```python
import jax
import jax.numpy as jnp

def _softmax(x, axis=-1):
    return jax.nn.softmax(x, axis=axis)

def _gelu(x):
    return jax.nn.gelu(x, approximate=True)

def _silu(x):
    return jax.nn.silu(x)

def _sigmoid(x):
    return jax.nn.sigmoid(x)

def _layernorm(x, axis=-1, eps=1e-05):
    m = jnp.mean(x, axis=axis, keepdims=True)
    v = jnp.var(x, axis=axis, keepdims=True)
    return (x - m) / jnp.sqrt(v + eps)

def _scatter_add(tgt, idx, src, axis=0):
    return tgt.at[idx].add(src)

def _segment_sum(src, seg, n):
    return jax.ops.segment_sum(src, seg, n)

class _Rng:

    def __init__(self, key):
        self._k = key

    def _next(self):
        self._k, sub = jax.random.split(self._k)
        return sub

    def normal(self, shape):
        return jax.random.normal(self._next(), shape, dtype=jnp.bfloat16)

    def randint(self, lo, hi, shape):
        return jax.random.randint(self._next(), shape, lo, hi, dtype=jnp.int32)

    def uniform(self, shape, lo=0.0, hi=1.0):
        return jax.random.uniform(self._next(), shape, jnp.bfloat16, lo, hi)

    def permutation(self, n):
        return jax.random.permutation(self._next(), n)
kernel_name = 'adaLN_cond__memory_aug_recurrent_mem_tr__dense_activation_gelu__prompt'

def setup_inputs():
    _rng = _Rng(jax.random.key(int.from_bytes(__import__("os").urandom(4), "little")))
    _w = lambda a: (lambda t: t.astype(jnp.bfloat16) if jnp.issubdtype(t.dtype, jnp.floating) else t)(jnp.asarray(a))

    def _A_setup():
        B, S, Dm = (1, 2048, 1024)
        H, Dh = (32, 128)
        M, seg = (8, 32)
        seg = min(seg, S)
        S = S // seg * seg
        return {'x': _w((lambda *s: _rng.normal(s) * 0.05)(B, S, Dm)), 'mem0': _w((lambda *s: _rng.normal(s) * 0.05)(B, M, Dm)), 'Wq': _w((lambda *s: _rng.normal(s) * 0.05)(Dm, H, Dh) * Dm ** (-0.5)), 'Wk': _w((lambda *s: _rng.normal(s) * 0.05)(Dm, H, Dh) * Dm ** (-0.5)), 'Wv': _w((lambda *s: _rng.normal(s) * 0.05)(Dm, H, Dh) * Dm ** (-0.5)), 'Wo': _w((lambda *s: _rng.normal(s) * 0.05)(H, Dh, Dm) * (H * Dh) ** (-0.5)), 'seg_len': seg}
    _A_in = _A_setup()

    def _B_setup():
        B, S, D, F = (1, 2048, 1024, 3584)
        return {'x': _w((lambda *s: _rng.normal(s) * 0.05)(B, S, D)), 'w1': _w((lambda *s: _rng.normal(s) * 0.05)(D, F) * D ** (-0.5)), 'b1': _w((lambda *s: _rng.normal(s) * 0.05)(F) * 0.01), 'w2': _w((lambda *s: _rng.normal(s) * 0.05)(F, D) * F ** (-0.5)), 'b2': _w((lambda *s: _rng.normal(s) * 0.05)(D) * 0.01)}
    _B_in = _B_setup()
    return {'A_x': _A_in['x'], 'A_mem0': _A_in['mem0'], 'A_Wq': _A_in['Wq'], 'A_Wk': _A_in['Wk'], 'A_Wv': _A_in['Wv'], 'A_Wo': _A_in['Wo'], 'A_seg_len': _A_in['seg_len'], 'B_x': _B_in['x'], 'B_w1': _B_in['w1'], 'B_b1': _B_in['b1'], 'B_w2': _B_in['w2'], 'B_b2': _B_in['b2'], 'c': _w((lambda *s: _rng.normal(s) * 0.05)(1, 1024)), 'w_mod': _w((lambda *s: _rng.normal(s) * 0.05)(1024, 6 * 1024) * 1024 ** (-0.5))}

def reference(A_x, A_mem0, A_Wq, A_Wk, A_Wv, A_Wo, A_seg_len, B_x, B_w1, B_b1, B_w2, B_b2, c, w_mod):

    def _A_ref(x, mem0, Wq, Wk, Wv, Wo, seg_len):
        B, S, Dm = x.shape
        H, Dh = (Wq.shape[1], Wq.shape[2])
        M = mem0.shape[1]
        scale = Dh ** (-0.5)
        n_seg = S // seg_len
        L = M + seg_len
        idx = jnp.arange(L)
        mask = (idx[:, None] < M) | (idx[:, None] >= idx[None, :])
        mem = mem0
        outs = []
        for s in range(n_seg):
            xs = x[:, s * seg_len:(s + 1) * seg_len, :].copy()
            h = jnp.concatenate([mem, xs], axis=1)
            q = jnp.einsum('btd,dhe->bhte', h, Wq)
            k = jnp.einsum('btd,dhe->bhte', h, Wk)
            v = jnp.einsum('btd,dhe->bhte', h, Wv)
            scores = jnp.einsum('bhqe,bhke->bhqk', q, k) * scale
            scores = jnp.where(mask[None, None], scores, -1000000000.0)
            p = _softmax(scores, axis=-1)
            o = jnp.einsum('bhqk,bhke->bhqe', p, v)
            o = jnp.einsum('bhte,hed->btd', o, Wo)
            mem = o[:, :M, :].copy()
            outs.append(o[:, M:, :])
        return jnp.concatenate(outs, axis=1)

    def _B_ref(x, w1, b1, w2, b2):
        h = jnp.einsum('bsd,df->bsf', x, w1) + b1
        h = _gelu(h)
        return jnp.einsum('bsf,fd->bsd', h, w2) + b2
    x = A_x
    mod = (_silu(c) @ w_mod).reshape(c.shape[0], 6, 1, -1)
    sa, ca, ga, sb, cb, gb = (mod[:, 0].copy(), mod[:, 1].copy(), mod[:, 2].copy(), mod[:, 3].copy(), mod[:, 4].copy(), mod[:, 5].copy())
    h = _layernorm(x, axis=-1) * (1 + ca) + sa
    x = x + ga * _A_ref(h, A_mem0, A_Wq, A_Wk, A_Wv, A_Wo, A_seg_len)
    h = _layernorm(x, axis=-1) * (1 + cb) + sb
    x = x + gb * _B_ref(h, B_w1, B_b1, B_w2, B_b2)
    return x
```

```python
import functools
import math

import jax
import jax.numpy as jnp
from jax import lax
import jax.experimental.pallas as pl
import jax.experimental.pallas.tpu as pltpu

F32 = jnp.float32
BF16 = jnp.bfloat16
U32 = jnp.uint32

S = 2048
D = 1024
H = 32
E = 128
M = 8
SEG = 32
NSEG = S // SEG
FF = 3584
NP = H // 2
TOK = 24
PRE = S - NSEG * TOK
RING = 576
OOFF = (-NSEG * TOK) % RING
LN_EPS = 1e-5
FB = 256
LNB = (S - PRE) // NP


def _ln(x):
    m = jnp.mean(x, axis=-1, keepdims=True)
    xc = x - m
    v = jnp.mean(xc * xc, axis=-1, keepdims=True)
    return xc * lax.rsqrt(v + LN_EPS)


def _bf(w32):
    return pltpu.bitcast(w32, BF16)


def _dot(a, b):
    return jnp.dot(a, b, preferred_element_type=F32)


def _kernel(x_hbm, mem0_ref, wq_hbm, wk_hbm, wv_hbm, wo_hbm, w1_hbm, b1_ref, w2_hbm, b2_ref,
            c_ref, wmod_hbm, out_hbm,
            xs, wqkv, wo, w1, w2, wmod, ring, oring, ha, hb, memb, modb, fillb, obuf,
            sem_qkv, sem_x, sem_mod, sem_w, sem_out):
    qkv_hbm = [r.bitcast(U32) for r in (wq_hbm, wk_hbm, wv_hbm)]
    wo32 = wo_hbm.bitcast(U32)
    wmod32 = wmod_hbm.bitcast(U32)

    def qkv_copy(j, m, p):
        c = 6 * j + 2 * m + p
        return pltpu.make_async_copy(qkv_hbm[m].at[:, p, j, :], wqkv.at[c], sem_qkv.at[c])

    def mod_copy(n):
        return pltpu.make_async_copy(wmod32.at[:, pl.ds(n * 128, 128)], wmod.at[n],
                                     sem_mod.at[0 if n < 16 else 1])

    def x_copy(part):
        rows = pl.ds(0, PRE) if part == 0 else pl.ds(PRE, S - PRE)
        return pltpu.make_async_copy(x_hbm.at[rows], xs.at[rows], sem_x.at[part])

    def wo_copy(n):
        return pltpu.make_async_copy(wo32.at[:, pl.ds(n * 128, 128)], wo.at[n], sem_w.at[0])

    w1_copy = pltpu.make_async_copy(w1_hbm, w1, sem_w.at[1])
    w2_copy = pltpu.make_async_copy(w2_hbm, w2, sem_w.at[2])

    def start_pair(j):
        for m in range(3):
            for p in range(2):
                qkv_copy(j, m, p).start()

    def wait_pair(j):
        for m in range(3):
            for p in range(2):
                qkv_copy(j, m, p).wait()

    def deinterleave(j):
        for m in range(3):
            c = 6 * j + 2 * m
            a = wqkv[c]
            b = wqkv[c + 1]
            wqkv[c] = (a & jnp.uint32(0xFFFF)) | (b << 16)
            wqkv[c + 1] = (a >> 16) | (b & jnp.uint32(0xFFFF0000))

    x_copy(0).start()
    for n in range(16):
        mod_copy(n).start()
    start_pair(0)
    start_pair(1)
    x_copy(1).start()
    start_pair(2)

    r = lax.broadcasted_iota(jnp.int32, (80, 128), 0)
    q = lax.broadcasted_iota(jnp.int32, (80, 128), 1)
    r_tok = r < 64
    q_tok = q < 64
    r_head = jnp.where(r_tok, r >> 5, (r - 64) >> 3)
    q_head = jnp.where(q_tok, q >> 5, (q - 64) >> 3)
    same = (r_head == q_head) & (q < 80)
    causal_ok = jnp.logical_not(r_tok & q_tok & ((q & 31) > (r & 31)))
    scale = E ** (-0.5)
    fillb[...] = jnp.where(same, jnp.where(causal_ok, 0.0, -1e9 / scale), -jnp.inf).astype(F32)

    cf = c_ref[...].astype(F32)
    sc = (cf * jax.nn.sigmoid(cf)).astype(BF16)
    sc16 = jnp.broadcast_to(sc, (16, D))

    def mod_part(lo, hi):
        for n in range(lo, hi):
            y = _dot(sc16, _bf(wmod[n]))[0:8]
            modb[n // 8, :, pl.ds((n % 8) * 128, 128)] = y.astype(BF16).astype(F32)

    memb[...] = mem0_ref[...].astype(F32)

    x_copy(0).wait()
    for n in range(16):
        mod_copy(n).wait()
    mod_part(0, 16)

    def ln1(rows):
        sa = modb[0, 0:1, :]
        ca1 = 1.0 + modb[1, 0:1, :]
        return _ln(xs[rows, :].astype(F32)) * ca1 + sa

    def pre_ln(i, carry):
        r0 = pl.multiple_of(i * 64, 64)
        hb[pl.ds(pl.multiple_of(i * 32, 32), 32), :] = pltpu.bitcast(
            ln1(pl.ds(r0, 64)).astype(BF16), U32)
        return carry

    with jax.named_scope("p0_ln"):
        lax.fori_loop(0, PRE // 64, pre_ln, 0)

    wait_pair(0)
    deinterleave(0)
    x_copy(1).wait()

    def bulk_qkv(j):
        lhs = _bf(hb[...])
        for t in range(6):
            c = 6 * j + t
            ring[c, pl.ds(RING - PRE, PRE), :] = _dot(lhs, _bf(wqkv[c]))
        r0 = pl.multiple_of(PRE + j * LNB, 32)
        ha[pl.ds(r0, LNB), :] = ln1(pl.ds(r0, LNB))

    def phase1(j, carry):
        @pl.when(j + 3 < NP)
        def _():
            start_pair(j + 3)

        @pl.when(j == 8)
        def _():
            for n in range(8):
                wo_copy(n).start()

        @pl.when(j == 13)
        def _():
            for n in range(16, 48):
                mod_copy(n).start()
            w1_copy.start()
            w2_copy.start()

        wait_pair(j + 1)
        deinterleave(j + 1)
        bulk_qkv(j)
        return carry

    with jax.named_scope("p1_bulk_qkv"):
        lax.fori_loop(0, NP - 1, phase1, 0)
    bulk_qkv(NP - 1)
    for n in range(8):
        wo_copy(n).wait()

    cexp = scale * math.log2(math.e)
    zpad = jnp.zeros((48, E), BF16)

    def step(s, carry):
        w0 = pl.multiple_of(lax.rem(TOK * s, RING), 8)
        r0 = pl.multiple_of(lax.rem(SEG * s + (RING - PRE), RING), 32)
        ow = pl.multiple_of(lax.rem(SEG * s + OOFF, RING), 32)
        o0 = pl.multiple_of(lax.rem(TOK * s + OOFF, RING), 8)
        h0 = pl.multiple_of(PRE + TOK * s, 8)
        a0 = pl.multiple_of(TOK * s, 8)
        X = jnp.concatenate([ha[pl.ds(h0, TOK), :], memb[...]], axis=0).astype(BF16)
        ym = [None] * 96
        probs = [None] * NP
        lhs_o = [None] * H

        def proj(j):
            for t in range(6):
                c = 6 * j + t
                y = _dot(X, _bf(wqkv[c]))
                ring[c, pl.ds(w0, TOK), :] = y[0:TOK]
                ym[c] = y[TOK:TOK + M]

        def gather(j, m):
            c = 6 * j + 2 * m
            return jnp.concatenate(
                [ring[c, pl.ds(r0, SEG), :], ring[c + 1, pl.ds(r0, SEG), :],
                 ym[c], ym[c + 1]], axis=0).astype(BF16)

        def scores(j):
            Q = gather(j, 0)
            K = jnp.concatenate([gather(j, 1), zpad], axis=0)
            sc_ = lax.dot_general(Q, K, (((1,), (1,)), ((), ())), preferred_element_type=F32)
            fill = fillb[...]
            sc_ = jnp.where(fill == 0.0, sc_, fill)
            mx = jnp.max(sc_, axis=-1, keepdims=True)
            p = jnp.exp2((sc_ - mx) * cexp)
            l = jnp.sum(p, axis=-1, keepdims=True)
            rl = pl.reciprocal(l, approx=True)
            rl = rl * (2.0 - l * rl)
            probs[j] = (p * rl).astype(BF16)

        def pv(j):
            V = jnp.concatenate([gather(j, 2), zpad], axis=0)
            o = _dot(probs[j], V)
            oring[2 * j, pl.ds(ow, SEG), :] = o[0:32]
            oring[2 * j + 1, pl.ds(ow, SEG), :] = o[32:64]
            for u in range(2):
                lhs_o[2 * j + u] = jnp.concatenate(
                    [oring[2 * j + u, pl.ds(o0, TOK), :], o[64 + 8 * u:72 + 8 * u]],
                    axis=0).astype(BF16)

        def oproj(n, h_lo, h_hi):
            lo = jnp.concatenate(lhs_o[h_lo:h_hi], axis=1)
            return _dot(lo, _bf(wo[n, pl.ds(h_lo * 64, (h_hi - h_lo) * 64), :]))

        NG = NP // 2
        for g in range(NG):
            proj(2 * g)
            if g >= 1:
                scores(2 * g - 2)
                scores(2 * g - 1)
            if g >= 2:
                pv(2 * g - 4)
                pv(2 * g - 3)
            proj(2 * g + 1)
        HS = 24
        acc = [None] * 8
        for n in range(8):
            acc[n] = oproj(n, 0, HS)
            if n == 1:
                scores(NP - 2)
                scores(NP - 1)
                pv(NP - 4)
                pv(NP - 3)
            if n == 5:
                pv(NP - 2)
                pv(NP - 1)
        for n in range(8):
            a = acc[n] + oproj(n, HS, H)
            ha[pl.ds(a0, TOK), pl.ds(n * 128, 128)] = a[0:TOK]
            memb[:, pl.ds(n * 128, 128)] = a[TOK:TOK + M]
        return carry

    with jax.named_scope("p2_steps"):
        lax.fori_loop(0, NSEG, step, 0)

    def bulk_o(i, carry):
        rr = pl.multiple_of(i * 256, 256)
        lo = jnp.concatenate([oring[h, pl.ds(rr, 256), :].astype(BF16) for h in range(H)], axis=1)
        for n in range(8):
            ha[pl.ds(NSEG * TOK + rr, 256), pl.ds(n * 128, 128)] = _dot(lo, _bf(wo[n]))
        return carry

    with jax.named_scope("p3_bulk_o"):
        lax.fori_loop(0, PRE // 256, bulk_o, 0)

    for n in range(16, 48):
        mod_copy(n).wait()
    mod_part(16, 48)
    w1_copy.wait()
    w2_copy.wait()

    def out_copy(i, slot):
        return pltpu.make_async_copy(obuf.at[slot], out_hbm.at[pl.ds(i * FB, FB)], sem_out.at[slot])

    def ffn(i, carry):
        slot = i % 2

        @pl.when(i >= 2)
        def _():
            out_copy(i - 2, slot).wait()

        rows = pl.ds(pl.multiple_of(i * FB, FB), FB)
        ga = modb[2, 0:1, :]
        sb = modb[3, 0:1, :]
        cb1 = 1.0 + modb[4, 0:1, :]
        gb = modb[5, 0:1, :]
        x2 = xs[rows, :].astype(F32) + ga * ha[rows, :]
        h2 = (_ln(x2) * cb1 + sb).astype(BF16)
        b1 = b1_ref[...].astype(F32).reshape(1, FF)
        g = jax.nn.gelu(_dot(h2, w1[...]) + b1, approximate=True).astype(BF16)
        y = _dot(g, w2[...]) + b2_ref[...].astype(F32).reshape(1, D)
        obuf[slot] = (x2 + gb * y).astype(BF16)
        out_copy(i, slot).start()
        return carry

    nb = S // FB
    with jax.named_scope("p4_ffn"):
        lax.fori_loop(0, nb, ffn, 0)
    out_copy(nb - 2, (nb - 2) % 2).wait()
    out_copy(nb - 1, (nb - 1) % 2).wait()


@functools.partial(jax.jit, static_argnames=("A_seg_len",))
def pallas_adaLN_cond__memory_aug_recurrent_mem_tr__dense_activation_gelu__prompt_kernel(
    A_x, A_mem0, A_Wq, A_Wk, A_Wv, A_Wo, A_seg_len, B_x, B_w1, B_b1, B_w2, B_b2, c, w_mod,
):
    assert A_seg_len == SEG and A_x.shape == (1, S, D) and A_Wq.shape == (D, H, E)
    any_spec = pl.BlockSpec(memory_space=pl.ANY)
    vmem_spec = pl.BlockSpec(memory_space=pltpu.VMEM)
    out = pl.pallas_call(
        _kernel,
        out_shape=jax.ShapeDtypeStruct((S, D), BF16),
        in_specs=[any_spec, vmem_spec, any_spec, any_spec, any_spec, any_spec, any_spec, vmem_spec,
                  any_spec, vmem_spec, vmem_spec, any_spec],
        out_specs=any_spec,
        scratch_shapes=[
            pltpu.VMEM((S, D), BF16),
            pltpu.VMEM((96, D // 2, E), U32),
            pltpu.VMEM((8, H * E // 2, 128), U32),
            pltpu.VMEM((D, FF), BF16),
            pltpu.VMEM((FF, D), BF16),
            pltpu.VMEM((48, D // 2, 128), U32),
            pltpu.VMEM((96, RING, E), F32),
            pltpu.VMEM((H, RING, E), F32),
            pltpu.VMEM((S, D), F32),
            pltpu.VMEM((PRE // 2, D), U32),
            pltpu.VMEM((M, D), F32),
            pltpu.VMEM((6, 8, D), F32),
            pltpu.VMEM((80, 128), F32),
            pltpu.VMEM((2, FB, D), BF16),
            pltpu.SemaphoreType.DMA((96,)),
            pltpu.SemaphoreType.DMA((2,)),
            pltpu.SemaphoreType.DMA((2,)),
            pltpu.SemaphoreType.DMA((3,)),
            pltpu.SemaphoreType.DMA((2,)),
        ],
        compiler_params=pltpu.CompilerParams(vmem_limit_bytes=126 * 1024 * 1024),
    )(
        A_x.reshape(S, D), A_mem0.reshape(M, D),
        A_Wq.reshape(D // 2, 2, H, E), A_Wk.reshape(D // 2, 2, H, E), A_Wv.reshape(D // 2, 2, H, E),
        A_Wo.reshape(H * E, D), B_w1, B_b1, B_w2, B_b2, c, w_mod,
    )
    return out.reshape(1, S, D)
```

```python
import functools
import math

import jax
import jax.numpy as jnp
from jax import lax
import jax.experimental.pallas as pl
import jax.experimental.pallas.tpu as pltpu

F32 = jnp.float32
BF16 = jnp.bfloat16
U32 = jnp.uint32

S = 2048
D = 1024
H = 32
E = 128
M = 8
SEG = 32
NSEG = S // SEG
FF = 3584
NP = H // 2
TOK = 24
PRE = S - NSEG * TOK
RING = 576
OOFF = (-NSEG * TOK) % RING
LN_EPS = 1e-5
FB = 256
LNB = (S - PRE) // NP


def _ln(x):
    m = jnp.mean(x, axis=-1, keepdims=True)
    xc = x - m
    v = jnp.mean(xc * xc, axis=-1, keepdims=True)
    return xc * lax.rsqrt(v + LN_EPS)


def _bf(w32):
    return pltpu.bitcast(w32, BF16)


def _dot(a, b):
    return jnp.dot(a, b, preferred_element_type=F32)


def _kernel(x_hbm, mem0_ref, wq_hbm, wk_hbm, wv_hbm, wo_hbm, w1_hbm, b1_ref, w2_hbm, b2_ref,
            c_ref, wmod_hbm, out_hbm,
            xs, wqkv, wo, w1, w2, wmod, qka, qkb, vring, oring, ha, hb, memb, modb, fillb, accb, obuf,
            sem_qkv, sem_x, sem_mod, sem_w, sem_out):
    qkv_hbm = [r.bitcast(U32) for r in (wq_hbm, wk_hbm, wv_hbm)]
    wo32 = wo_hbm.bitcast(U32)
    wmod32 = wmod_hbm.bitcast(U32)

    def qkv_copy(j, m, p):
        c = 6 * j + 2 * m + p
        return pltpu.make_async_copy(qkv_hbm[m].at[:, p, j, :], wqkv.at[c], sem_qkv.at[c])

    def mod_copy(n):
        return pltpu.make_async_copy(wmod32.at[:, pl.ds(n * 128, 128)], wmod.at[n],
                                     sem_mod.at[0 if n < 16 else 1])

    def x_copy(part):
        rows = pl.ds(0, PRE) if part == 0 else pl.ds(PRE, S - PRE)
        return pltpu.make_async_copy(x_hbm.at[rows], xs.at[rows], sem_x.at[part])

    def wo_copy(n):
        return pltpu.make_async_copy(wo32.at[:, pl.ds(n * 128, 128)], wo.at[n], sem_w.at[0])

    w1_copy = pltpu.make_async_copy(w1_hbm, w1, sem_w.at[1])
    w2_copy = pltpu.make_async_copy(w2_hbm, w2, sem_w.at[2])

    def start_pair(j):
        for m in range(3):
            for p in range(2):
                qkv_copy(j, m, p).start()

    def wait_pair(j):
        for m in range(3):
            for p in range(2):
                qkv_copy(j, m, p).wait()

    def deinterleave(j):
        for m in range(3):
            c = 6 * j + 2 * m
            a = wqkv[c]
            b = wqkv[c + 1]
            wqkv[c] = (a & jnp.uint32(0xFFFF)) | (b << 16)
            wqkv[c + 1] = (a >> 16) | (b & jnp.uint32(0xFFFF0000))

    x_copy(0).start()
    for n in range(16):
        mod_copy(n).start()
    start_pair(0)
    start_pair(1)
    x_copy(1).start()
    start_pair(2)
    start_pair(3)

    r = lax.broadcasted_iota(jnp.int32, (80, 128), 0)
    q = lax.broadcasted_iota(jnp.int32, (80, 128), 1)
    r_tok = r < 64
    q_tok = q < 64
    r_head = jnp.where(r_tok, r >> 5, (r - 64) >> 3)
    q_head = jnp.where(q_tok, q >> 5, (q - 64) >> 3)
    same = (r_head == q_head) & (q < 80)
    causal_ok = jnp.logical_not(r_tok & q_tok & ((q & 31) > (r & 31)))
    scale = E ** (-0.5)
    fillb[...] = jnp.where(same, jnp.where(causal_ok, 0.0, -1e9 / scale), -jnp.inf).astype(F32)

    cf = c_ref[...].astype(F32)
    sc = (cf * jax.nn.sigmoid(cf)).astype(BF16)
    sc16 = jnp.broadcast_to(sc, (16, D))

    def mod_part(lo, hi):
        for n in range(lo, hi):
            y = _dot(sc16, _bf(wmod[n]))[0:8]
            modb[n // 8, :, pl.ds((n % 8) * 128, 128)] = y.astype(BF16).astype(F32)

    memb[...] = mem0_ref[...].astype(F32)

    x_copy(0).wait()
    for n in range(16):
        mod_copy(n).wait()
    mod_part(0, 16)

    def ln1(rows):
        sa = modb[0, 0:1, :]
        ca1 = 1.0 + modb[1, 0:1, :]
        return _ln(xs[rows, :].astype(F32)) * ca1 + sa

    def pre_ln(i, carry):
        r0 = pl.multiple_of(i * 64, 64)
        hb[pl.ds(pl.multiple_of(i * 32, 32), 32), :] = pltpu.bitcast(
            ln1(pl.ds(r0, 64)).astype(BF16), U32)
        return carry

    with jax.named_scope("p0_ln"):
        lax.fori_loop(0, PRE // 64, pre_ln, 0)

    wait_pair(0)
    deinterleave(0)
    wait_pair(1)
    deinterleave(1)
    x_copy(1).wait()

    def bulk_qkv(i):
        lhs = _bf(hb[...])
        rows = pl.ds(RING - PRE, PRE)
        for u in range(2):
            j = 2 * i + u
            for t in range(6):
                y = _dot(lhs, _bf(wqkv[6 * j + t]))
                if t >= 4:
                    vring[2 * j + t - 4, rows, :] = y
                else:
                    (qka, qkb)[u][4 * i + t, rows, :] = y
        r0 = pl.multiple_of(PRE + i * 2 * LNB, 32)
        ha[pl.ds(r0, 2 * LNB), :] = ln1(pl.ds(r0, 2 * LNB))

    def phase1(i, carry):
        @pl.when(i + 2 < NP // 2)
        def _():
            start_pair(2 * i + 4)
            start_pair(2 * i + 5)

        @pl.when(i == 4)
        def _():
            for n in range(8):
                wo_copy(n).start()

        @pl.when(i == 6)
        def _():
            for n in range(16, 48):
                mod_copy(n).start()
            w1_copy.start()
            w2_copy.start()

        wait_pair(2 * i + 2)
        wait_pair(2 * i + 3)
        deinterleave(2 * i + 2)
        deinterleave(2 * i + 3)
        bulk_qkv(i)
        return carry

    with jax.named_scope("p1_bulk_qkv"):
        lax.fori_loop(0, NP // 2 - 1, phase1, 0)
    bulk_qkv(NP // 2 - 1)
    for n in range(8):
        wo_copy(n).wait()

    cexp = scale * math.log2(math.e)
    zpad = jnp.zeros((48, E), BF16)

    def step(s, carry):
        w0 = pl.multiple_of(lax.rem(TOK * s, RING), 8)
        r0 = pl.multiple_of(lax.rem(SEG * s + (RING - PRE), RING), 32)
        ow = pl.multiple_of(lax.rem(SEG * s + OOFF, RING), 32)
        o0 = pl.multiple_of(lax.rem(TOK * s + OOFF, RING), 8)
        h0 = pl.multiple_of(PRE + TOK * s, 8)
        a0 = pl.multiple_of(TOK * s, 8)
        X = jnp.concatenate([ha[pl.ds(h0, TOK), :], memb[...]], axis=0).astype(BF16)
        ym = [None] * 96
        probs = [None] * NP
        lhs_o = [None] * H

        def slot(j, t):
            if t >= 4:
                return vring, 2 * j + t - 4
            return (qka, qkb)[j % 2], 4 * (j // 2) + t

        def proj(j):
            for t in (4, 5, 0, 1, 2, 3):
                c = 6 * j + t
                y = _dot(X, _bf(wqkv[c]))
                ref, k = slot(j, t)
                ref[k, pl.ds(w0, TOK), :] = y[0:TOK]
                ym[c] = y[TOK:TOK + M]

        def gather(j, m):
            c = 6 * j + 2 * m
            ref, k = slot(j, 2 * m)
            return jnp.concatenate(
                [ref[k, pl.ds(r0, SEG), :], ref[k + 1, pl.ds(r0, SEG), :],
                 ym[c], ym[c + 1]], axis=0).astype(BF16)

        def scores(j):
            Q = gather(j, 0)
            K = jnp.concatenate([gather(j, 1), zpad], axis=0)
            sc_ = lax.dot_general(Q, K, (((1,), (1,)), ((), ())), preferred_element_type=F32)
            fill = fillb[...]
            sc_ = jnp.where(fill == 0.0, sc_, fill)
            mx = jnp.max(sc_, axis=-1, keepdims=True)
            p = jnp.exp2((sc_ - mx) * cexp)
            l = jnp.sum(p, axis=-1, keepdims=True)
            rl = pl.reciprocal(l, approx=True)
            rl = rl * (2.0 - l * rl)
            probs[j] = (p * rl).astype(BF16)

        def pv(j):
            V = jnp.concatenate([gather(j, 2), zpad], axis=0)
            o = _dot(probs[j], V)
            oring[2 * j, pl.ds(ow, SEG), :] = o[0:32]
            oring[2 * j + 1, pl.ds(ow, SEG), :] = o[32:64]
            for u in range(2):
                lhs_o[2 * j + u] = jnp.concatenate(
                    [oring[2 * j + u, pl.ds(o0, TOK), :], o[64 + 8 * u:72 + 8 * u]],
                    axis=0).astype(BF16)

        def oproj(n, h_lo, h_hi):
            lo = jnp.concatenate(lhs_o[h_lo:h_hi], axis=1)
            return _dot(lo, _bf(wo[n, pl.ds(h_lo * 64, (h_hi - h_lo) * 64), :]))

        NG = NP // 2
        grp = [(4 * (g // 2) + (g % 2), 4 * (g // 2) + (g % 2) + 2) for g in range(NG)]
        for g in range(NG):
            proj(grp[g][0])
            if g >= 1:
                scores(grp[g - 1][0])
                scores(grp[g - 1][1])
            if g >= 2:
                pv(grp[g - 2][0])
                pv(grp[g - 2][1])
            proj(grp[g][1])
        HS = 24
        for n in range(8):
            accb[n] = oproj(n, 0, HS)
            if n == 1:
                scores(grp[NG - 1][0])
                scores(grp[NG - 1][1])
                pv(grp[NG - 2][0])
                pv(grp[NG - 2][1])
            if n == 5:
                pv(grp[NG - 1][0])
                pv(grp[NG - 1][1])
        for n in range(8):
            a = accb[n] + oproj(n, HS, H)
            ha[pl.ds(a0, TOK), pl.ds(n * 128, 128)] = a[0:TOK]
            memb[:, pl.ds(n * 128, 128)] = a[TOK:TOK + M]
        return carry

    with jax.named_scope("p2_steps"):
        lax.fori_loop(0, NSEG, step, 0)

    def bulk_o(i, carry):
        rr = pl.multiple_of(i * 256, 256)
        lo = jnp.concatenate([oring[h, pl.ds(rr, 256), :].astype(BF16) for h in range(H)], axis=1)
        for n in range(8):
            ha[pl.ds(NSEG * TOK + rr, 256), pl.ds(n * 128, 128)] = _dot(lo, _bf(wo[n]))
        return carry

    with jax.named_scope("p3_bulk_o"):
        lax.fori_loop(0, PRE // 256, bulk_o, 0)

    for n in range(16, 48):
        mod_copy(n).wait()
    mod_part(16, 48)
    w1_copy.wait()
    w2_copy.wait()

    def out_copy(i, slot):
        return pltpu.make_async_copy(obuf.at[slot], out_hbm.at[pl.ds(i * FB, FB)], sem_out.at[slot])

    def ffn(i, carry):
        slot = i % 2

        @pl.when(i >= 2)
        def _():
            out_copy(i - 2, slot).wait()

        rows = pl.ds(pl.multiple_of(i * FB, FB), FB)
        ga = modb[2, 0:1, :]
        sb = modb[3, 0:1, :]
        cb1 = 1.0 + modb[4, 0:1, :]
        gb = modb[5, 0:1, :]
        x2 = xs[rows, :].astype(F32) + ga * ha[rows, :]
        h2 = (_ln(x2) * cb1 + sb).astype(BF16)
        b1 = b1_ref[...].astype(F32).reshape(1, FF)
        g = jax.nn.gelu(_dot(h2, w1[...]) + b1, approximate=True).astype(BF16)
        y = _dot(g, w2[...]) + b2_ref[...].astype(F32).reshape(1, D)
        obuf[slot] = (x2 + gb * y).astype(BF16)
        out_copy(i, slot).start()
        return carry

    nb = S // FB
    with jax.named_scope("p4_ffn"):
        lax.fori_loop(0, nb, ffn, 0)
    out_copy(nb - 2, (nb - 2) % 2).wait()
    out_copy(nb - 1, (nb - 1) % 2).wait()


@functools.partial(jax.jit, static_argnames=("A_seg_len",))
def pallas_adaLN_cond__memory_aug_recurrent_mem_tr__dense_activation_gelu__prompt_kernel(
    A_x, A_mem0, A_Wq, A_Wk, A_Wv, A_Wo, A_seg_len, B_x, B_w1, B_b1, B_w2, B_b2, c, w_mod,
):
    assert A_seg_len == SEG and A_x.shape == (1, S, D) and A_Wq.shape == (D, H, E)
    any_spec = pl.BlockSpec(memory_space=pl.ANY)
    vmem_spec = pl.BlockSpec(memory_space=pltpu.VMEM)
    out = pl.pallas_call(
        _kernel,
        out_shape=jax.ShapeDtypeStruct((S, D), BF16),
        in_specs=[any_spec, vmem_spec, any_spec, any_spec, any_spec, any_spec, any_spec, vmem_spec,
                  any_spec, vmem_spec, vmem_spec, any_spec],
        out_specs=any_spec,
        scratch_shapes=[
            pltpu.VMEM((S, D), BF16),
            pltpu.VMEM((96, D // 2, E), U32),
            pltpu.VMEM((8, H * E // 2, 128), U32),
            pltpu.VMEM((D, FF), BF16),
            pltpu.VMEM((FF, D), BF16),
            pltpu.VMEM((48, D // 2, 128), U32),
            pltpu.VMEM((32, RING, E), F32),
            pltpu.VMEM((32, RING, E), F32),
            pltpu.VMEM((32, RING, E), F32),
            pltpu.VMEM((H, RING, E), F32),
            pltpu.VMEM((S, D), F32),
            pltpu.VMEM((PRE // 2, D), U32),
            pltpu.VMEM((M, D), F32),
            pltpu.VMEM((6, 8, D), F32),
            pltpu.VMEM((80, 128), F32),
            pltpu.VMEM((8, 32, 128), F32),
            pltpu.VMEM((2, FB, D), BF16),
            pltpu.SemaphoreType.DMA((96,)),
            pltpu.SemaphoreType.DMA((2,)),
            pltpu.SemaphoreType.DMA((2,)),
            pltpu.SemaphoreType.DMA((3,)),
            pltpu.SemaphoreType.DMA((2,)),
        ],
        compiler_params=pltpu.CompilerParams(vmem_limit_bytes=126 * 1024 * 1024),
    )(
        A_x.reshape(S, D), A_mem0.reshape(M, D),
        A_Wq.reshape(D // 2, 2, H, E), A_Wk.reshape(D // 2, 2, H, E), A_Wv.reshape(D // 2, 2, H, E),
        A_Wo.reshape(H * E, D), B_w1, B_b1, B_w2, B_b2, c, w_mod,
    )
    return out.reshape(1, S, D)
```

```python
import functools
import math

import jax
import jax.numpy as jnp
from jax import lax
import jax.experimental.pallas as pl
import jax.experimental.pallas.tpu as pltpu

F32 = jnp.float32
BF16 = jnp.bfloat16
U32 = jnp.uint32

S = 2048
D = 1024
H = 32
E = 128
M = 8
SEG = 32
NSEG = S // SEG
FF = 3584
NP = H // 2
TOK = 24
PRE = S - NSEG * TOK
RING = 576
OOFF = (-NSEG * TOK) % RING
LN_EPS = 1e-5
FB = 256


def _ln(x):
    m = jnp.mean(x, axis=-1, keepdims=True)
    xc = x - m
    v = jnp.mean(xc * xc, axis=-1, keepdims=True)
    return xc * lax.rsqrt(v + LN_EPS)


def _bf(w32):
    return pltpu.bitcast(w32, BF16)


def _dot(a, b):
    return jnp.dot(a, b, preferred_element_type=F32)


SEM_SMALL = 0
SEM_MISC = 1
SEM_X0 = 2
SEM_MOD = 3
SEM_UNIT = 8
SEM_XC = SEM_UNIT + 48
SEM_WO = SEM_XC + 6
SEM_W1 = SEM_WO + 1
SEM_W2 = SEM_W1 + 1
SEM_OUT = SEM_W2 + 1
NSEM = SEM_OUT + 2
XC = (S - PRE) // 6


def _kernel(x_hbm, mem0_hbm, wq_hbm, wk_hbm, wv_hbm, wo_hbm, w1_hbm, b1_hbm, w2_hbm, b2_hbm,
            c_hbm, wmod_hbm, out_hbm,
            xs, wqkv, wo, w1, w2, wmod, qka, qkb, vring, oring, ha, hb, memb, modb, fillb, accb, obuf,
            mem0_ref, b1_ref, b2_ref, c_ref, sem):
    qkv_hbm = [r.bitcast(U32) for r in (wq_hbm, wk_hbm, wv_hbm)]
    wo32 = wo_hbm.bitcast(U32)
    wmod32 = wmod_hbm.bitcast(U32)

    def unit_start(u):
        j, m = u // 3, u % 3
        for p in range(2):
            pltpu.make_async_copy(qkv_hbm[m].at[:, p, j, :], wqkv.at[2 * u + p],
                                  sem.at[SEM_UNIT + u]).start()

    def unit_wait(u):
        both = wqkv.at[pl.ds(2 * u, 2)]
        pltpu.make_async_copy(both, both, sem.at[SEM_UNIT + u]).wait()

    def mod_copy(g):
        return pltpu.make_async_copy(wmod32.at[:, pl.ds(g * 512, 512)], wmod.at[g],
                                     sem.at[SEM_MOD + min(g, 4)])

    x0_copy = pltpu.make_async_copy(x_hbm.at[pl.ds(0, PRE)], xs.at[pl.ds(0, PRE)], sem.at[SEM_X0])

    def xc_copy(i):
        rows = pl.ds(pl.multiple_of(PRE + i * XC, 64), XC)
        return pltpu.make_async_copy(x_hbm.at[rows], xs.at[rows], sem.at[SEM_XC + i])

    def wo_copy(n):
        return pltpu.make_async_copy(wo32.at[:, pl.ds(n * 128, 128)], wo.at[n], sem.at[SEM_WO])

    w1_copy = pltpu.make_async_copy(w1_hbm, w1, sem.at[SEM_W1])
    w2_copy = pltpu.make_async_copy(w2_hbm, w2, sem.at[SEM_W2])
    c_copy = pltpu.make_async_copy(c_hbm, c_ref, sem.at[SEM_SMALL])
    misc_copies = [pltpu.make_async_copy(a, b, sem.at[SEM_MISC])
                   for a, b in ((mem0_hbm, mem0_ref), (b1_hbm, b1_ref), (b2_hbm, b2_ref))]

    def deinterleave(u):
        for k in range(D // 2 // 64):
            rows = pl.ds(k * 64, 64)
            a = wqkv[2 * u, rows, :]
            b = wqkv[2 * u + 1, rows, :]
            wqkv[2 * u, rows, :] = (a & jnp.uint32(0xFFFF)) | (b << 16)
            wqkv[2 * u + 1, rows, :] = (a >> 16) | (b & jnp.uint32(0xFFFF0000))

    c_copy.start()
    x0_copy.start()
    for g in range(4):
        mod_copy(g).start()

    def start_units(lo, hi):
        for u in range(lo, hi):
            if u % 6 == 0 and 12 <= u:
                xc_copy(u // 6 - 2).start()
            unit_start(u)

    start_units(0, 28)

    def start_rest():
        for cp in misc_copies:
            cp.start()
        for n in range(8):
            wo_copy(n).start()
        for g in range(4, 12):
            mod_copy(g).start()
        w1_copy.start()
        w2_copy.start()

    r = lax.broadcasted_iota(jnp.int32, (80, 128), 0)
    q = lax.broadcasted_iota(jnp.int32, (80, 128), 1)
    r_tok = r < 64
    q_tok = q < 64
    r_head = jnp.where(r_tok, r >> 5, (r - 64) >> 3)
    q_head = jnp.where(q_tok, q >> 5, (q - 64) >> 3)
    same = (r_head == q_head) & (q < 80)
    causal_ok = jnp.logical_not(r_tok & q_tok & ((q & 31) > (r & 31)))
    scale = E ** (-0.5)
    fillb[...] = jnp.where(same, jnp.where(causal_ok, 0.0, -1e9 / scale), -jnp.inf).astype(F32)

    def silu_c():
        cf = c_ref[...].astype(F32)
        return jnp.broadcast_to((cf * jax.nn.sigmoid(cf)).astype(BF16), (16, D))

    def mod_part(sc16, lo, hi):
        for g in range(lo, hi):
            y = _dot(sc16, _bf(wmod[g]))[0:8]
            modb[g // 2, :, pl.ds((g % 2) * 512, 512)] = y.astype(BF16).astype(F32)

    def pre_norm(i, carry):
        rows = pl.ds(pl.multiple_of(i * 64, 64), 64)
        ha[rows, :] = _ln(xs[rows, :].astype(F32))
        return carry

    c_copy.wait()
    x0_copy.wait()
    with jax.named_scope("p0_ln"):
        lax.fori_loop(0, PRE // 64, pre_norm, 0)

    sc16 = silu_c()
    for g in range(4):
        mod_copy(g).wait()
        mod_part(sc16, g, g + 1)

    def modulate1(n):
        return n * (1.0 + modb[1, 0:1, :]) + modb[0, 0:1, :]

    for i in range(PRE // 64):
        hb[pl.ds(i * 32, 32), :] = pltpu.bitcast(
            modulate1(ha[pl.ds(i * 64, 64), :]).astype(BF16), U32)

    unit_wait(0)
    deinterleave(0)

    def bulk_qkv(i, waits, last, with_ln):
        rows = pl.ds(RING - PRE, PRE)
        for k in range(6):
            u = 6 * i + k
            cls, m = k // 3, k % 3
            for p in range(2):
                y = _dot(_bf(hb[...]), _bf(wqkv[2 * u + p]))
                if m == 2:
                    vring[4 * i + 2 * cls + p, rows, :] = y
                else:
                    (qka, qkb)[cls][4 * i + 2 * m + p, rows, :] = y
                if p == 0:
                    for w in waits.get(k, ()):
                        unit_wait(6 * i + w)
                    if not (last and k == 5):
                        deinterleave(u + 1)
                if with_ln and k >= 2:
                    for z in range(2):
                        r0 = pl.multiple_of(PRE + (i - 1) * XC + (4 * k + 2 * p + z - 8) * 16, 16)
                        rr = pl.ds(r0, 16)
                        ha[rr, :] = modulate1(_ln(xs[rr, :].astype(F32)))

    def phase1(i, carry):
        @pl.when(i == 2)
        def _():
            start_units(28, 48)

        @pl.when(i == 4)
        def _():
            start_rest()

        xc_copy(i - 1).wait()
        for w in range(1, 7):
            unit_wait(6 * i + w)
        bulk_qkv(i, {}, False, True)
        return carry

    bulk_qkv(0, {0: (1,), 1: (2, 3), 3: (4, 5, 6)}, False, False)
    with jax.named_scope("p1_bulk_qkv"):
        lax.fori_loop(1, 7, phase1, 0)
    for w in range(43, 48):
        unit_wait(w)
    bulk_qkv(7, {}, True, False)
    for cp in misc_copies:
        cp.wait()
    memb[...] = mem0_ref[...].astype(F32)
    for n in range(8):
        wo_copy(n).wait()

    cexp = scale * math.log2(math.e)
    zpad = jnp.zeros((48, E), BF16)

    def step(s, carry):
        w0 = pl.multiple_of(lax.rem(TOK * s, RING), 8)
        r0 = pl.multiple_of(lax.rem(SEG * s + (RING - PRE), RING), 32)
        ow = pl.multiple_of(lax.rem(SEG * s + OOFF, RING), 32)
        o0 = pl.multiple_of(lax.rem(TOK * s + OOFF, RING), 8)
        h0 = pl.multiple_of(PRE + TOK * s, 8)
        a0 = pl.multiple_of(TOK * s, 8)
        X = jnp.concatenate([ha[pl.ds(h0, TOK), :], memb[...]], axis=0).astype(BF16)
        ym = [None] * 96
        probs = [None] * NP
        lhs_o = [None] * H

        def slot(j, t):
            if t >= 4:
                return vring, 2 * j + t - 4
            return (qka, qkb)[j % 2], 4 * (j // 2) + t

        def proj(j):
            for t in (4, 5, 0, 1, 2, 3):
                c = 6 * j + t
                y = _dot(X, _bf(wqkv[c]))
                ref, k = slot(j, t)
                ref[k, pl.ds(w0, TOK), :] = y[0:TOK]
                ym[c] = y[TOK:TOK + M]

        def gather(j, m):
            c = 6 * j + 2 * m
            ref, k = slot(j, 2 * m)
            return jnp.concatenate(
                [ref[k, pl.ds(r0, SEG), :], ref[k + 1, pl.ds(r0, SEG), :],
                 ym[c], ym[c + 1]], axis=0).astype(BF16)

        def scores(j):
            Q = gather(j, 0)
            K = jnp.concatenate([gather(j, 1), zpad], axis=0)
            sc_ = lax.dot_general(Q, K, (((1,), (1,)), ((), ())), preferred_element_type=F32)
            fill = fillb[...]
            sc_ = jnp.where(fill == 0.0, sc_, fill)
            mx = jnp.max(sc_, axis=-1, keepdims=True)
            p = jnp.exp2((sc_ - mx) * cexp)
            l = jnp.sum(p, axis=-1, keepdims=True)
            rl = pl.reciprocal(l, approx=True)
            rl = rl * (2.0 - l * rl)
            probs[j] = (p * rl).astype(BF16)

        def pv(j):
            V = jnp.concatenate([gather(j, 2), zpad], axis=0)
            o = _dot(probs[j], V)
            oring[2 * j, pl.ds(ow, SEG), :] = o[0:32]
            oring[2 * j + 1, pl.ds(ow, SEG), :] = o[32:64]
            for u in range(2):
                lhs_o[2 * j + u] = jnp.concatenate(
                    [oring[2 * j + u, pl.ds(o0, TOK), :], o[64 + 8 * u:72 + 8 * u]],
                    axis=0).astype(BF16)

        def oproj(n, h_lo, h_hi):
            lo = jnp.concatenate(lhs_o[h_lo:h_hi], axis=1)
            return _dot(lo, _bf(wo[n, pl.ds(h_lo * 64, (h_hi - h_lo) * 64), :]))

        NG = NP // 2
        grp = [(4 * (g // 2) + (g % 2), 4 * (g // 2) + (g % 2) + 2) for g in range(NG)]
        for g in range(NG):
            proj(grp[g][0])
            if g >= 1:
                scores(grp[g - 1][0])
                scores(grp[g - 1][1])
            if g >= 2:
                pv(grp[g - 2][0])
                pv(grp[g - 2][1])
            proj(grp[g][1])
        HS = 24
        for n in range(8):
            accb[n] = oproj(n, 0, HS)
            if n == 1:
                scores(grp[NG - 1][0])
                scores(grp[NG - 1][1])
                pv(grp[NG - 2][0])
                pv(grp[NG - 2][1])
            if n == 5:
                pv(grp[NG - 1][0])
                pv(grp[NG - 1][1])
        for n in range(8):
            a = accb[n] + oproj(n, HS, H)
            ha[pl.ds(a0, TOK), pl.ds(n * 128, 128)] = a[0:TOK]
            memb[:, pl.ds(n * 128, 128)] = a[TOK:TOK + M]
        return carry

    with jax.named_scope("p2_steps"):
        lax.fori_loop(0, NSEG, step, 0)

    def bulk_o(i, carry):
        rr = pl.multiple_of(i * 256, 256)
        lo = jnp.concatenate([oring[h, pl.ds(rr, 256), :].astype(BF16) for h in range(H)], axis=1)
        for n in range(8):
            ha[pl.ds(NSEG * TOK + rr, 256), pl.ds(n * 128, 128)] = _dot(lo, _bf(wo[n]))
        return carry

    with jax.named_scope("p3_bulk_o"):
        lax.fori_loop(0, PRE // 256, bulk_o, 0)

    for g in range(4, 12):
        mod_copy(g).wait()
    mod_part(silu_c(), 4, 12)
    w1_copy.wait()
    w2_copy.wait()

    def out_copy(i, slot):
        return pltpu.make_async_copy(obuf.at[slot], out_hbm.at[pl.ds(i * FB, FB)], sem.at[SEM_OUT + slot])

    def ffn(i, carry):
        slot = i % 2

        @pl.when(i >= 2)
        def _():
            out_copy(i - 2, slot).wait()

        rows = pl.ds(pl.multiple_of(i * FB, FB), FB)
        ga = modb[2, 0:1, :]
        sb = modb[3, 0:1, :]
        cb1 = 1.0 + modb[4, 0:1, :]
        gb = modb[5, 0:1, :]
        x2 = xs[rows, :].astype(F32) + ga * ha[rows, :]
        h2 = (_ln(x2) * cb1 + sb).astype(BF16)
        b1 = b1_ref[...].astype(F32).reshape(1, FF)
        g = jax.nn.gelu(_dot(h2, w1[...]) + b1, approximate=True).astype(BF16)
        y = _dot(g, w2[...]) + b2_ref[...].astype(F32).reshape(1, D)
        obuf[slot] = (x2 + gb * y).astype(BF16)
        out_copy(i, slot).start()
        return carry

    nb = S // FB
    with jax.named_scope("p4_ffn"):
        lax.fori_loop(0, nb, ffn, 0)
    out_copy(nb - 2, (nb - 2) % 2).wait()
    out_copy(nb - 1, (nb - 1) % 2).wait()


@functools.partial(jax.jit, static_argnames=("A_seg_len",))
def pallas_adaLN_cond__memory_aug_recurrent_mem_tr__dense_activation_gelu__prompt_kernel(
    A_x, A_mem0, A_Wq, A_Wk, A_Wv, A_Wo, A_seg_len, B_x, B_w1, B_b1, B_w2, B_b2, c, w_mod,
):
    assert A_seg_len == SEG and A_x.shape == (1, S, D) and A_Wq.shape == (D, H, E)
    any_spec = pl.BlockSpec(memory_space=pl.ANY)
    out = pl.pallas_call(
        _kernel,
        out_shape=jax.ShapeDtypeStruct((S, D), BF16),
        in_specs=[any_spec] * 12,
        out_specs=any_spec,
        scratch_shapes=[
            pltpu.VMEM((S, D), BF16),
            pltpu.VMEM((96, D // 2, E), U32),
            pltpu.VMEM((8, H * E // 2, 128), U32),
            pltpu.VMEM((D, FF), BF16),
            pltpu.VMEM((FF, D), BF16),
            pltpu.VMEM((12, D // 2, 512), U32),
            pltpu.VMEM((32, RING, E), F32),
            pltpu.VMEM((32, RING, E), F32),
            pltpu.VMEM((32, RING, E), F32),
            pltpu.VMEM((H, RING, E), F32),
            pltpu.VMEM((S, D), F32),
            pltpu.VMEM((PRE // 2, D), U32),
            pltpu.VMEM((M, D), F32),
            pltpu.VMEM((6, 8, D), F32),
            pltpu.VMEM((80, 128), F32),
            pltpu.VMEM((8, 32, 128), F32),
            pltpu.VMEM((2, FB, D), BF16),
            pltpu.VMEM((M, D), BF16),
            pltpu.VMEM((FF,), BF16),
            pltpu.VMEM((D,), BF16),
            pltpu.VMEM((1, D), BF16),
            pltpu.SemaphoreType.DMA((NSEM,)),
        ],
        compiler_params=pltpu.CompilerParams(vmem_limit_bytes=126 * 1024 * 1024),
    )(
        A_x.reshape(S, D), A_mem0.reshape(M, D),
        A_Wq.reshape(D // 2, 2, H, E), A_Wk.reshape(D // 2, 2, H, E), A_Wv.reshape(D // 2, 2, H, E),
        A_Wo.reshape(H * E, D), B_w1, B_b1, B_w2, B_b2, c, w_mod,
    )
    return out.reshape(1, S, D)
```

```python
import math

import jax
import jax.numpy as jnp
from jax import lax
import jax.experimental.pallas as pl
import jax.experimental.pallas.tpu as pltpu

F32 = jnp.float32
BF16 = jnp.bfloat16
U32 = jnp.uint32

S = 2048
D = 1024
H = 32
E = 128
M = 8
SEG = 32
NSEG = S // SEG
FF = 3584
NP = H // 2
TOK = 24
PRE = S - NSEG * TOK
RING = 576
OOFF = (-NSEG * TOK) % RING
LN_EPS = 1e-5
FB = 256
XC = (S - PRE) // 6
UNROLL = 4

UNIT_GROUPS = [(0, 1), (1, 2), (2, 4), (4, 7)] + [(6 * i + 1, min(6 * i + 7, 48)) for i in range(1, 8)]

SEM_C = 0
SEM_MISC = 1
SEM_X0 = 2
SEM_MOD = 3
SEM_UNIT = 8
SEM_XC = SEM_UNIT + len(UNIT_GROUPS)
SEM_WO = SEM_XC + 6
SEM_W1 = SEM_WO + 1
SEM_W2 = SEM_W1 + 1
SEM_OUT = SEM_W2 + 1
NSEM = SEM_OUT + 2


def _ln(x):
    m = jnp.mean(x, axis=-1, keepdims=True)
    xc = x - m
    v = jnp.mean(xc * xc, axis=-1, keepdims=True)
    return xc * lax.rsqrt(v + LN_EPS)


def _bf(w32):
    return pltpu.bitcast(w32, BF16)


def _dot(a, b):
    return jnp.dot(a, b, preferred_element_type=F32)


def _kernel(x_hbm, mem0_hbm, wq_hbm, wk_hbm, wv_hbm, wo_hbm, w1_hbm, b1_hbm, w2_hbm, b2_hbm,
            c_hbm, wmod_hbm, out_hbm,
            xs, wqkv, wo, w1, w2, wmod, qka, qkb, vring, oring, ha, hn, hb, memb, modb, biasb,
            fillb, accb, zerob, obuf, mem0_ref, b1_ref, b2_ref, c_ref, sem):
    qkv_hbm = [r.bitcast(U32) for r in (wq_hbm, wk_hbm, wv_hbm)]
    x32 = x_hbm.bitcast(U32)
    wo32 = wo_hbm.bitcast(U32)
    wmod32 = wmod_hbm.bitcast(U32)

    def unit_start(u):
        j, m = u // 3, u % 3
        grp = [k for k, (lo, hi) in enumerate(UNIT_GROUPS) if lo <= u < hi][0]
        for p in range(2):
            pltpu.make_async_copy(qkv_hbm[m].at[:, p, j, :], wqkv.at[2 * u + p],
                                  sem.at[SEM_UNIT + grp]).start()

    def units_wait(grp, lo, n):
        blk = wqkv.at[pl.ds(2 * lo, 2 * n)]
        pltpu.make_async_copy(blk, blk, sem.at[SEM_UNIT + grp]).wait()

    def static_units_wait(grp):
        lo, hi = UNIT_GROUPS[grp]
        units_wait(grp, lo, hi - lo)

    def mod_copy(g):
        return pltpu.make_async_copy(wmod32.at[:, pl.ds(g * 512, 512)], wmod.at[g],
                                     sem.at[SEM_MOD + min(g, 4)])

    x0_copy = pltpu.make_async_copy(x32.at[pl.ds(0, PRE // 2)], xs.at[pl.ds(0, PRE // 2)],
                                    sem.at[SEM_X0])

    def xc_copy(i):
        rows = pl.ds(pl.multiple_of(PRE // 2 + i * (XC // 2), 64), XC // 2)
        return pltpu.make_async_copy(x32.at[rows], xs.at[rows], sem.at[SEM_XC + i])

    def wo_copy(n):
        return pltpu.make_async_copy(wo32.at[:, pl.ds(n * 128, 128)], wo.at[n], sem.at[SEM_WO])

    w1_copy = pltpu.make_async_copy(w1_hbm.bitcast(U32), w1, sem.at[SEM_W1])
    w2_copy = pltpu.make_async_copy(w2_hbm.bitcast(U32), w2, sem.at[SEM_W2])
    c_copy = pltpu.make_async_copy(c_hbm, c_ref, sem.at[SEM_C])
    misc_copies = [pltpu.make_async_copy(a, b, sem.at[SEM_MISC])
                   for a, b in ((mem0_hbm, mem0_ref), (b1_hbm, b1_ref), (b2_hbm, b2_ref))]

    def deinterleave(u):
        for k in range(D // 2 // 64):
            rows = pl.ds(k * 64, 64)
            a = wqkv[2 * u, rows, :]
            b = wqkv[2 * u + 1, rows, :]
            wqkv[2 * u, rows, :] = (a & jnp.uint32(0xFFFF)) | (b << 16)
            wqkv[2 * u + 1, rows, :] = (a >> 16) | (b & jnp.uint32(0xFFFF0000))

    def load_x16(row2, dep):
        xw = xs[pl.ds(row2, 8), :]
        if dep is not None:
            first = xw[:, 0:128] | (dep & zerob[...])
            xw = jnp.concatenate([first, xw[:, 128:]], axis=1)
        return _bf(xw).astype(F32)

    def mrow(k):
        return modb[k, 0:1, :]

    c_copy.start()
    x0_copy.start()
    for g in range(4):
        mod_copy(g).start()

    def start_units(lo, hi):
        for u in range(lo, hi):
            if u % 6 == 0 and 12 <= u:
                xc_copy(u // 6 - 2).start()
            unit_start(u)

    start_units(0, 28)

    def start_rest():
        for cp in misc_copies:
            cp.start()
        for n in range(8):
            wo_copy(n).start()
        for g in range(4, 12):
            mod_copy(g).start()
        w1_copy.start()
        w2_copy.start()

    r = lax.broadcasted_iota(jnp.int32, (80, 128), 0)
    q = lax.broadcasted_iota(jnp.int32, (80, 128), 1)
    r_tok = r < 64
    q_tok = q < 64
    r_head = jnp.where(r_tok, r >> 5, (r - 64) >> 3)
    q_head = jnp.where(q_tok, q >> 5, (q - 64) >> 3)
    same = (r_head == q_head) & (q < 80)
    causal_ok = jnp.logical_not(r_tok & q_tok & ((q & 31) > (r & 31)))
    scale = E ** (-0.5)
    fillb[...] = jnp.where(same, jnp.where(causal_ok, 0.0, -1e9 / scale), -jnp.inf).astype(F32)
    zerob[...] = jnp.zeros((8, 128), U32)

    def silu_c():
        cf = c_ref[...].astype(F32)
        return jnp.broadcast_to((cf * jax.nn.sigmoid(cf)).astype(BF16), (16, D))

    def mod_part(sc16, lo, hi):
        for g in range(lo, hi):
            y = _dot(sc16, _bf(wmod[g]))[0:8].astype(BF16).astype(F32)
            if g // 2 in (1, 4):
                y = 1.0 + y
            modb[g // 2, :, pl.ds((g % 2) * 512, 512)] = y

    def pre_norm(i, carry):
        rows = pl.ds(pl.multiple_of(i * 64, 64), 64)
        ha[rows, :] = _ln(_bf(xs[pl.ds(pl.multiple_of(i * 32, 32), 32), :]).astype(F32))
        return carry

    c_copy.wait()
    x0_copy.wait()
    with jax.named_scope("p0_ln"):
        lax.fori_loop(0, PRE // 64, pre_norm, 0)

    sc16 = silu_c()
    for g in range(4):
        mod_copy(g).wait()
        mod_part(sc16, g, g + 1)

    for i in range(PRE // 64):
        hb[pl.ds(i * 32, 32), :] = pltpu.bitcast(
            (ha[pl.ds(i * 64, 64), :] * mrow(1) + mrow(0)).astype(BF16), U32)

    static_units_wait(0)
    deinterleave(0)

    def bulk_qkv(i, waits, last, with_ln):
        rows = pl.ds(RING - PRE, PRE)
        dep = None
        for k in range(6):
            u = 6 * i + k
            cls, m = k // 3, k % 3
            for p in range(2):
                y = _dot(_bf(hb[...]), _bf(wqkv[2 * u + p]))
                if m == 2:
                    vring[4 * i + 2 * cls + p, rows, :] = y
                else:
                    (qka, qkb)[cls][4 * i + 2 * m + p, rows, :] = y
                if p == 0:
                    if k in waits:
                        static_units_wait(waits[k])
                    if not (last and k == 5):
                        deinterleave(u + 1)
                if with_ln and k >= 2:
                    for z in range(2):
                        r0 = (i - 1) * XC + (4 * k + 2 * p + z - 8) * 16
                        x16 = load_x16(pl.multiple_of(PRE // 2 + r0 // 2, 8), dep)
                        h16 = _ln(x16) * mrow(1) + mrow(0)
                        hn[pl.ds(pl.multiple_of(r0, 16), 16), :] = h16
                        dep = pltpu.bitcast(h16[8:16, D - 128:], U32)

    def phase1(i, carry):
        @pl.when(i == 2)
        def _():
            start_units(28, 48)

        @pl.when(i == 4)
        def _():
            start_rest()

        xc_copy(i - 1).wait()
        units_wait(3 + i, 6 * i + 1, 6)
        bulk_qkv(i, {}, False, True)
        return carry

    bulk_qkv(0, {0: 1, 1: 2, 3: 3}, False, False)
    with jax.named_scope("p1_bulk_qkv"):
        lax.fori_loop(1, 7, phase1, 0)
    static_units_wait(10)
    bulk_qkv(7, {}, True, False)
    for cp in misc_copies:
        cp.wait()
    memb[...] = mem0_ref[...].astype(F32)
    biasb[:, pl.ds(0, FF)] = jnp.broadcast_to(b1_ref[...].astype(F32).reshape(1, FF), (8, FF))
    biasb[:, pl.ds(FF, D)] = jnp.broadcast_to(b2_ref[...].astype(F32).reshape(1, D), (8, D))
    for n in range(8):
        wo_copy(n).wait()

    cexp = scale * math.log2(math.e)
    NG = NP // 2
    grp = [(4 * (g // 2) + (g % 2), 4 * (g // 2) + (g % 2) + 2) for g in range(NG)]
    HS = 24

    def step(s, split):
        w0 = pl.multiple_of(lax.rem(TOK * s, RING), 8)
        r0 = pl.multiple_of(lax.rem(SEG * s + (RING - PRE), RING), 32)
        ow = pl.multiple_of(lax.rem(SEG * s + OOFF, RING), 32)
        o0 = pl.multiple_of(lax.rem(TOK * s + OOFF, RING), 8)
        a0 = pl.multiple_of(TOK * s, 8)
        X = jnp.concatenate([hn[pl.ds(a0, TOK), :], memb[...]], axis=0).astype(BF16)
        ym = [None] * 96
        probs = [None] * NP
        om = [None] * H
        order = (4, 5, 0, 1, 2, 3)

        if split:
            for t in order:
                accb[t] = _dot(X[:, :D // 2], _bf(wqkv[t, pl.ds(0, D // 4), :]))

        def slot(j, t):
            if t >= 4:
                return vring, 2 * j + t - 4
            return (qka, qkb)[j % 2], 4 * (j // 2) + t

        def proj(j):
            for t in order:
                c = 6 * j + t
                if split and j == 0:
                    y = accb[t] + _dot(X[:, D // 2:], _bf(wqkv[c, pl.ds(D // 4, D // 4), :]))
                else:
                    y = _dot(X, _bf(wqkv[c]))
                ref, k = slot(j, t)
                ref[k, pl.ds(w0, TOK), :] = y[0:TOK]
                ym[c] = y[TOK:TOK + M]

        def gather(j, m, pad):
            c = 6 * j + 2 * m
            ref, k = slot(j, 2 * m)
            parts = [ref[k, pl.ds(r0, SEG), :], ref[k + 1, pl.ds(r0, SEG), :], ym[c], ym[c + 1]]
            if pad:
                parts.append(jnp.zeros((48, E), F32))
            return jnp.concatenate(parts, axis=0).astype(BF16)

        def scores(j):
            sc_ = lax.dot_general(gather(j, 0, False), gather(j, 1, True),
                                  (((1,), (1,)), ((), ())), preferred_element_type=F32)
            fill = fillb[...]
            sc_ = jnp.where(fill == 0.0, sc_, fill)
            mx = jnp.max(sc_, axis=-1, keepdims=True)
            p = jnp.exp2((sc_ - mx) * cexp)
            l = jnp.sum(p, axis=-1, keepdims=True)
            rl = pl.reciprocal(l, approx=True)
            rl = rl * (2.0 - l * rl)
            probs[j] = (p * rl).astype(BF16)

        def park(j):
            vring[H, pl.ds(40 * (j % 8), 40), :] = pltpu.bitcast(probs[j], F32)
            probs[j] = None

        def pv(j):
            P = probs[j]
            if P is None:
                P = _bf(vring[H, pl.ds(40 * (j % 8), 40), :])
            o = _dot(P, gather(j, 2, True))
            oring[2 * j, pl.ds(ow, SEG), :] = o[0:32]
            oring[2 * j + 1, pl.ds(ow, SEG), :] = o[32:64]
            om[2 * j] = o[64:72]
            om[2 * j + 1] = o[72:80]

        def att(gs, gp):
            if gp is not None:
                pv(grp[gp][0])
                pv(grp[gp][1])
            if gs is not None:
                scores(grp[gs][0])
                scores(grp[gs][1])

        def o_lhs(h_lo, h_hi):
            return jnp.concatenate(
                [jnp.concatenate([oring[h, pl.ds(o0, TOK), :], om[h]], axis=0)
                 for h in range(h_lo, h_hi)], axis=1).astype(BF16)

        for g in range(NG):
            if g >= 2:
                park(grp[g - 2][0])
                park(grp[g - 2][1])
            proj(grp[g][0])
            att(g - 1 if g >= 1 else None, g - 2 if g >= 2 else None)
            proj(grp[g][1])
        lo = o_lhs(0, HS)
        for n in range(8):
            accb[n] = _dot(lo, _bf(wo[n, pl.ds(0, HS * 64), :]))
            if n == 1:
                att(NG - 1, NG - 2)
            if n == 5:
                att(None, NG - 1)
        lo = o_lhs(HS, H)
        for n in range(8):
            a = accb[n] + _dot(lo, _bf(wo[n, pl.ds(HS * 64, (H - HS) * 64), :]))
            ha[pl.ds(a0, TOK), pl.ds(n * 128, 128)] = a[0:TOK]
            memb[:, pl.ds(n * 128, 128)] = a[TOK:TOK + M]

    def steps(i, carry):
        for k in range(UNROLL):
            step(i * UNROLL + k, k > 0)
        return carry

    with jax.named_scope("p2_steps"):
        lax.fori_loop(0, NSEG // UNROLL, steps, 0)

    for g in range(4, 12):
        mod_copy(g).wait()
    mod_part(silu_c(), 4, 12)

    def ln2_piece(r0, dep):
        r2 = pl.multiple_of(r0 // 2, 8)
        x2 = load_x16(r2, dep) + mrow(2) * ha[pl.ds(pl.multiple_of(r0, 16), 16), :]
        h2 = pltpu.bitcast((_ln(x2) * mrow(4) + mrow(3)).astype(BF16), F32)
        hn[pl.ds(r2, 8), :] = h2
        return pltpu.bitcast(h2[:, D - 128:], U32)

    def bulk_o(i, carry):
        rr = pl.multiple_of(i * 256, 256)
        lo = jnp.concatenate([oring[h, pl.ds(rr, 256), :] for h in range(H)], axis=1).astype(BF16)
        dep = None
        for n in range(8):
            dep = ln2_piece(i * (FB // 2) + n * 16, dep)
            ha[pl.ds(NSEG * TOK + rr, 256), pl.ds(n * 128, 128)] = _dot(lo, _bf(wo[n]))
        return carry

    with jax.named_scope("p3_bulk_o"):
        lax.fori_loop(0, PRE // 256, bulk_o, 0)

    w1_copy.wait()
    w2_copy.wait()

    nb = S // FB

    def out_copy(i, slot):
        return pltpu.make_async_copy(obuf.at[slot], out_hbm.at[pl.ds(i * FB, FB)], sem.at[SEM_OUT + slot])

    def ffn(i, carry):
        slot = i % 2

        @pl.when(i >= 2)
        def _():
            out_copy(i - 2, slot).wait()

        rows = pl.ds(pl.multiple_of(i * FB, FB), FB)
        rows2 = pl.ds(pl.multiple_of(i * (FB // 2), FB // 2), FB // 2)
        h2 = _bf(hn[rows2, :])
        g = jax.nn.gelu(_dot(h2, _bf(w1[...])) + biasb[0:1, pl.ds(0, FF)], approximate=True).astype(BF16)
        nxt = jnp.minimum(i + 1, nb - 1) * FB
        dep = None
        for n in range(8):
            cols = pl.ds(n * 128, 128)
            y = _dot(g, _bf(w2[:, cols])) + biasb[0:1, pl.ds(FF + n * 128, 128)]
            x2 = _bf(xs[rows2, cols]).astype(F32) + modb[2, 0:1, cols] * ha[rows, cols]
            obuf[slot, :, cols] = (x2 + modb[5, 0:1, cols] * y).astype(BF16)
            for z in range(2):
                dep = ln2_piece(nxt + (2 * n + z) * 16, dep)
        out_copy(i, slot).start()
        return carry

    with jax.named_scope("p4_ffn"):
        lax.fori_loop(0, nb, ffn, 0)
    out_copy(nb - 2, (nb - 2) % 2).wait()
    out_copy(nb - 1, (nb - 1) % 2).wait()


@jax.jit
def pallas_adaLN_cond__memory_aug_recurrent_mem_tr__dense_activation_gelu__prompt_kernel(
    A_x, A_mem0, A_Wq, A_Wk, A_Wv, A_Wo, A_seg_len, B_x, B_w1, B_b1, B_w2, B_b2, c, w_mod,
):
    assert A_x.shape == (1, S, D) and A_Wq.shape == (D, H, E) and A_mem0.shape == (1, M, D)
    any_spec = pl.BlockSpec(memory_space=pl.ANY)
    out = pl.pallas_call(
        _kernel,
        out_shape=jax.ShapeDtypeStruct((S, D), BF16),
        in_specs=[any_spec] * 12,
        out_specs=any_spec,
        scratch_shapes=[
            pltpu.VMEM((S // 2, D), U32),
            pltpu.VMEM((96, D // 2, E), U32),
            pltpu.VMEM((8, H * E // 2, 128), U32),
            pltpu.VMEM((D // 2, FF), U32),
            pltpu.VMEM((FF // 2, D), U32),
            pltpu.VMEM((12, D // 2, 512), U32),
            pltpu.VMEM((H, RING, E), F32),
            pltpu.VMEM((H, RING, E), F32),
            pltpu.VMEM((H + 1, RING, E), F32),
            pltpu.VMEM((H, RING, E), F32),
            pltpu.VMEM((S, D), F32),
            pltpu.VMEM((S - PRE, D), F32),
            pltpu.VMEM((PRE // 2, D), U32),
            pltpu.VMEM((M, D), F32),
            pltpu.VMEM((6, 8, D), F32),
            pltpu.VMEM((8, FF + D), F32),
            pltpu.VMEM((80, 128), F32),
            pltpu.VMEM((8, 32, 128), F32),
            pltpu.VMEM((8, 128), U32),
            pltpu.VMEM((2, FB, D), BF16),
            pltpu.VMEM((M, D), BF16),
            pltpu.VMEM((FF,), BF16),
            pltpu.VMEM((D,), BF16),
            pltpu.VMEM((1, D), BF16),
            pltpu.SemaphoreType.DMA((NSEM,)),
        ],
        compiler_params=pltpu.CompilerParams(vmem_limit_bytes=127 * 1024 * 1024),
    )(
        A_x.reshape(S, D), A_mem0.reshape(M, D),
        A_Wq.reshape(D // 2, 2, H, E), A_Wk.reshape(D // 2, 2, H, E), A_Wv.reshape(D // 2, 2, H, E),
        A_Wo.reshape(H * E, D), B_w1, B_b1, B_w2, B_b2, c, w_mod,
    )
    return out.reshape(1, S, D)
```

```python
import math

import jax
import jax.numpy as jnp
from jax import lax
import jax.experimental.pallas as pl
import jax.experimental.pallas.tpu as pltpu

F32 = jnp.float32
BF16 = jnp.bfloat16
U32 = jnp.uint32

S = 2048
D = 1024
H = 32
E = 128
M = 8
SEG = 32
NSEG = S // SEG
FF = 3584
NP = H // 2
TOK = 24
PRE = S - NSEG * TOK
RING = 576
OOFF = (-NSEG * TOK) % RING
LN_EPS = 1e-5
FB = 256
XC = (S - PRE) // 6
UNROLL = 4

UNIT_GROUPS = [(0, 1), (1, 2), (2, 4), (4, 7)] + [(6 * i + 1, min(6 * i + 7, 48)) for i in range(1, 8)]

SEM_C = 0
SEM_MISC = 1
SEM_X0 = 2
SEM_MOD = 3
SEM_UNIT = 8
SEM_XC = SEM_UNIT + len(UNIT_GROUPS)
SEM_WO = SEM_XC + 6
SEM_W1 = SEM_WO + 1
SEM_W2 = SEM_W1 + 1
SEM_OUT = SEM_W2 + 1
NSEM = SEM_OUT + 1


def _ln(x):
    m = jnp.mean(x, axis=-1, keepdims=True)
    xc = x - m
    v = jnp.mean(xc * xc, axis=-1, keepdims=True)
    return xc * lax.rsqrt(v + LN_EPS)


def _bf(w32):
    return pltpu.bitcast(w32, BF16)


def _dot(a, b):
    return jnp.dot(a, b, preferred_element_type=F32)


def _kernel(x_hbm, mem0_hbm, wq_hbm, wk_hbm, wv_hbm, wo_hbm, w1_hbm, b1_hbm, w2_hbm, b2_hbm,
            c_hbm, wmod_hbm, out_hbm,
            xs, wqkv, wo, w1, w2, wmod, qka, qkb, vring, oring, ha, hn, hb, memb, modb, biasb,
            fillb, accb, zerob, colb, zero_s, mem0_ref, b1_ref, b2_ref, c_ref, sem):
    qkv_hbm = [r.bitcast(U32) for r in (wq_hbm, wk_hbm, wv_hbm)]
    x32 = x_hbm.bitcast(U32)
    wo32 = wo_hbm.bitcast(U32)
    wmod32 = wmod_hbm.bitcast(U32)

    def unit_start(u):
        j, m = u // 3, u % 3
        grp = [k for k, (lo, hi) in enumerate(UNIT_GROUPS) if lo <= u < hi][0]
        for p in range(2):
            pltpu.make_async_copy(qkv_hbm[m].at[:, p, j, :], wqkv.at[2 * u + p],
                                  sem.at[SEM_UNIT + grp]).start()

    def units_wait(grp, lo, n):
        blk = wqkv.at[pl.ds(2 * lo, 2 * n)]
        pltpu.make_async_copy(blk, blk, sem.at[SEM_UNIT + grp]).wait()

    def static_units_wait(grp):
        lo, hi = UNIT_GROUPS[grp]
        units_wait(grp, lo, hi - lo)

    def mod_copy(g):
        return pltpu.make_async_copy(wmod32.at[:, pl.ds(g * 512, 512)], wmod.at[g],
                                     sem.at[SEM_MOD + min(g, 4)])

    x0_copy = pltpu.make_async_copy(x32.at[pl.ds(0, PRE // 2)], xs.at[pl.ds(0, PRE // 2)],
                                    sem.at[SEM_X0])

    def xc_copy(i):
        rows = pl.ds(pl.multiple_of(PRE // 2 + i * (XC // 2), 64), XC // 2)
        return pltpu.make_async_copy(x32.at[rows], xs.at[rows], sem.at[SEM_XC + i])

    def wo_copy(n):
        return pltpu.make_async_copy(wo32.at[:, pl.ds(n * 128, 128)], wo.at[n], sem.at[SEM_WO])

    w1_copy = pltpu.make_async_copy(w1_hbm.bitcast(U32), w1, sem.at[SEM_W1])
    w2_copy = pltpu.make_async_copy(w2_hbm.bitcast(U32), w2, sem.at[SEM_W2])
    c_copy = pltpu.make_async_copy(c_hbm, c_ref, sem.at[SEM_C])
    misc_copies = [pltpu.make_async_copy(a, b, sem.at[SEM_MISC])
                   for a, b in ((mem0_hbm, mem0_ref), (b1_hbm, b1_ref), (b2_hbm, b2_ref))]

    def deinterleave(u):
        for k in range(D // 2 // 64):
            rows = pl.ds(k * 64, 64)
            a = wqkv[2 * u, rows, :]
            b = wqkv[2 * u + 1, rows, :]
            wqkv[2 * u, rows, :] = (a & jnp.uint32(0xFFFF)) | (b << 16)
            wqkv[2 * u + 1, rows, :] = (a >> 16) | (b & jnp.uint32(0xFFFF0000))

    def load_x16(row2, dep):
        xw = xs[pl.ds(row2, 8), :]
        if dep is not None:
            first = xw[:, 0:128] | (dep & zerob[...])
            xw = jnp.concatenate([first, xw[:, 128:]], axis=1)
        return _bf(xw).astype(F32)

    def rep(v8, n):
        return jnp.concatenate([v8] * (n // 8), axis=0)

    def mrow(k, n):
        return rep(modb[k], n)

    c_copy.start()
    x0_copy.start()
    for g in range(4):
        mod_copy(g).start()

    def start_units(lo, hi):
        for u in range(lo, hi):
            if u % 6 == 0 and 12 <= u:
                xc_copy(u // 6 - 2).start()
            unit_start(u)

    start_units(0, 28)

    def start_rest():
        for cp in misc_copies:
            cp.start()
        for n in range(8):
            wo_copy(n).start()
        for g in range(4, 12):
            mod_copy(g).start()
        w1_copy.start()
        w2_copy.start()

    r = lax.broadcasted_iota(jnp.int32, (80, 128), 0)
    q = lax.broadcasted_iota(jnp.int32, (80, 128), 1)
    r_tok = r < 64
    q_tok = q < 64
    r_head = jnp.where(r_tok, r >> 5, (r - 64) >> 3)
    q_head = jnp.where(q_tok, q >> 5, (q - 64) >> 3)
    same = (r_head == q_head) & (q < 80)
    causal_ok = jnp.logical_not(r_tok & q_tok & ((q & 31) > (r & 31)))
    scale = E ** (-0.5)
    fillb[...] = jnp.where(same, jnp.where(causal_ok, 0.0, -1e9 / scale), -jnp.inf).astype(F32)
    zerob[...] = jnp.zeros((8, 128), U32)
    zero_s[0] = 0

    def silu_c():
        cf = c_ref[...].astype(F32)
        return jnp.broadcast_to((cf * jax.nn.sigmoid(cf)).astype(BF16), (16, D))

    def mod_part(sc16, lo, hi):
        for g in range(lo, hi):
            y = _dot(sc16, _bf(wmod[g]))[0:8].astype(BF16).astype(F32)
            if g // 2 in (1, 4):
                y = 1.0 + y
            modb[g // 2, :, pl.ds((g % 2) * 512, 512)] = y

    def pre_norm(i, carry):
        rows = pl.ds(pl.multiple_of(i * 64, 64), 64)
        ha[rows, :] = _ln(_bf(xs[pl.ds(pl.multiple_of(i * 32, 32), 32), :]).astype(F32))
        return carry

    c_copy.wait()
    x0_copy.wait()
    with jax.named_scope("p0_ln"):
        lax.fori_loop(0, PRE // 64, pre_norm, 0)

    sc16 = silu_c()
    scf = jnp.broadcast_to(sc16[0:1].astype(F32), (128, D))
    for k in range(8):
        colb[pl.ds(k * 64, 64), :] = pltpu.bitcast(scf[:, k * 128:(k + 1) * 128].T.astype(BF16), U32)
    for g in range(4):
        mod_copy(g).wait()
        mod_part(sc16, g, g + 1)

    for i in range(PRE // 64):
        hb[pl.ds(i * 32, 32), :] = pltpu.bitcast(
            (ha[pl.ds(i * 64, 64), :] * mrow(1, 64) + mrow(0, 64)).astype(BF16), U32)

    static_units_wait(0)
    deinterleave(0)

    def bulk_qkv(i, waits, last, with_ln):
        rows = pl.ds(RING - PRE, PRE)
        dep = None
        for k in range(6):
            u = 6 * i + k
            cls, m = k // 3, k % 3
            for p in range(2):
                y = _dot(_bf(hb[...]), _bf(wqkv[2 * u + p]))
                if m == 2:
                    vring[4 * i + 2 * cls + p, rows, :] = y
                else:
                    (qka, qkb)[cls][4 * i + 2 * m + p, rows, :] = y
                if p == 0:
                    if k in waits:
                        static_units_wait(waits[k])
                    if not (last and k == 5):
                        deinterleave(u + 1)
                if with_ln and k >= 2:
                    for z in range(2):
                        r0 = (i - 1) * XC + (4 * k + 2 * p + z - 8) * 16
                        x16 = load_x16(pl.multiple_of(PRE // 2 + r0 // 2, 8), dep)
                        h16 = _ln(x16) * mrow(1, 16) + mrow(0, 16)
                        hn[pl.ds(pl.multiple_of(r0, 16), 16), :] = h16
                        dep = pltpu.bitcast(h16[8:16, D - 128:], U32)

    def phase1(i, carry):
        @pl.when(i == 2)
        def _():
            start_units(28, 48)

        @pl.when(i == 4)
        def _():
            start_rest()

        xc_copy(i - 1).wait()
        units_wait(3 + i, 6 * i + 1, 6)
        bulk_qkv(i, {}, False, True)
        return carry

    bulk_qkv(0, {0: 1, 1: 2, 3: 3}, False, False)
    with jax.named_scope("p1_bulk_qkv"):
        lax.fori_loop(1, 7, phase1, 0)
    static_units_wait(10)
    bulk_qkv(7, {}, True, False)
    for cp in misc_copies:
        cp.wait()
    memb[...] = mem0_ref[...].astype(F32)
    biasb[:, pl.ds(0, FF)] = jnp.broadcast_to(b1_ref[...].astype(F32).reshape(1, FF), (8, FF))
    biasb[:, pl.ds(FF, D)] = jnp.broadcast_to(b2_ref[...].astype(F32).reshape(1, D), (8, D))
    for n in range(8):
        wo_copy(n).wait()

    cexp = scale * math.log2(math.e)
    NG = NP // 2
    grp = [(4 * (g // 2) + (g % 2), 4 * (g // 2) + (g % 2) + 2) for g in range(NG)]
    HS = 24

    def step(s, split):
        w0 = pl.multiple_of(lax.rem(TOK * s, RING), 8)
        r0 = pl.multiple_of(lax.rem(SEG * s + (RING - PRE), RING), 32)
        ow = pl.multiple_of(lax.rem(SEG * s + OOFF, RING), 32)
        o0 = pl.multiple_of(lax.rem(TOK * s + OOFF, RING), 8)
        a0 = pl.multiple_of(TOK * s, 8)
        X = jnp.concatenate([hn[pl.ds(a0, TOK), :], memb[...]], axis=0).astype(BF16)
        ym = [None] * 96
        probs = [None] * NP
        om = [None] * H
        order = (4, 5, 0, 1, 2, 3)

        if split:
            for t in order:
                accb[t] = _dot(X[:, :D // 2], _bf(wqkv[t, pl.ds(0, D // 4), :]))

        def slot(j, t):
            if t >= 4:
                return vring, 2 * j + t - 4
            return (qka, qkb)[j % 2], 4 * (j // 2) + t

        def proj(j):
            for t in order:
                c = 6 * j + t
                if split and j == 0:
                    y = accb[t] + _dot(X[:, D // 2:], _bf(wqkv[c, pl.ds(D // 4, D // 4), :]))
                else:
                    y = _dot(X, _bf(wqkv[c]))
                ref, k = slot(j, t)
                ref[k, pl.ds(w0, TOK), :] = y[0:TOK]
                ym[c] = y[TOK:TOK + M]

        def gather(j, m, pad):
            c = 6 * j + 2 * m
            ref, k = slot(j, 2 * m)
            parts = [ref[k, pl.ds(r0, SEG), :], ref[k + 1, pl.ds(r0, SEG), :], ym[c], ym[c + 1]]
            if pad:
                parts.append(jnp.zeros((48, E), F32))
            return jnp.concatenate(parts, axis=0).astype(BF16)

        def scores(j):
            sc_ = lax.dot_general(gather(j, 0, False), gather(j, 1, True),
                                  (((1,), (1,)), ((), ())), preferred_element_type=F32)
            fill = fillb[...]
            sc_ = jnp.where(fill == 0.0, sc_, fill)
            mx = jnp.max(sc_, axis=-1, keepdims=True)
            p = jnp.exp2((sc_ - mx) * cexp)
            l = jnp.sum(p, axis=-1, keepdims=True)
            rl = pl.reciprocal(l, approx=True)
            rl = rl * (2.0 - l * rl)
            probs[j] = (p * rl).astype(BF16)

        def park(j):
            vring[H, pl.ds(40 * (j % 8), 40), :] = pltpu.bitcast(probs[j], F32)
            probs[j] = None

        def pv(j):
            P = probs[j]
            if P is None:
                P = _bf(vring[H, pl.ds(40 * (j % 8), 40), :])
            o = _dot(P, gather(j, 2, True))
            oring[2 * j, pl.ds(ow, SEG), :] = o[0:32]
            oring[2 * j + 1, pl.ds(ow, SEG), :] = o[32:64]
            om[2 * j] = o[64:72]
            om[2 * j + 1] = o[72:80]

        def att(gs, gp):
            if gp is not None:
                pv(grp[gp][0])
                pv(grp[gp][1])
            if gs is not None:
                scores(grp[gs][0])
                scores(grp[gs][1])

        def o_lhs(h_lo, h_hi):
            return jnp.concatenate(
                [jnp.concatenate([oring[h, pl.ds(o0, TOK), :], om[h]], axis=0)
                 for h in range(h_lo, h_hi)], axis=1).astype(BF16)

        for g in range(NG):
            if g >= 2:
                park(grp[g - 2][0])
                park(grp[g - 2][1])
            proj(grp[g][0])
            att(g - 1 if g >= 1 else None, g - 2 if g >= 2 else None)
            proj(grp[g][1])
        lo = o_lhs(0, HS)
        for n in range(8):
            accb[n] = _dot(lo, _bf(wo[n, pl.ds(0, HS * 64), :]))
            if n == 1:
                att(NG - 1, NG - 2)
            if n == 5:
                att(None, NG - 1)
        lo = o_lhs(HS, H)
        for n in range(8):
            a = accb[n] + _dot(lo, _bf(wo[n, pl.ds(HS * 64, (H - HS) * 64), :]))
            ha[pl.ds(a0, TOK), pl.ds(n * 128, 128)] = a[0:TOK]
            memb[:, pl.ds(n * 128, 128)] = a[TOK:TOK + M]

    def steps(i, carry):
        for k in range(UNROLL):
            step(i * UNROLL + k, k > 0)
        return carry

    with jax.named_scope("p2_steps"):
        lax.fori_loop(0, NSEG // UNROLL, steps, 0)

    for g in range(4, 12):
        mod_copy(g).wait()

    def lo16(w):
        return pltpu.bitcast(w << 16, F32)

    def hi16(w):
        return pltpu.bitcast(w & jnp.uint32(0xFFFF0000), F32)

    def mod_vpu(g, dep):
        for t in range(4):
            acc = None if dep is None else pltpu.bitcast(dep & zerob[...], F32)
            for k in range(D // 16):
                cw = colb[pl.ds(k * 8, 8), :]
                w = wmod[g, pl.ds(k * 8, 8), pl.ds(t * 128, 128)]
                pe = lo16(w) * lo16(cw)
                acc = pe if acc is None else acc + pe
                acc = acc + hi16(w) * hi16(cw)
            dep = pltpu.bitcast(acc, U32)
            y = jnp.sum(acc, axis=0, keepdims=True).astype(BF16).astype(F32)
            if g // 2 == 4:
                y = 1.0 + y
            modb[g // 2, :, pl.ds((g % 2) * 512 + t * 128, 128)] = jnp.broadcast_to(y, (8, 128))
        return dep

    def ln2_piece(r0, dep):
        r2 = pl.multiple_of(r0 // 2, 8)
        x2 = load_x16(r2, dep) + mrow(2, 16) * ha[pl.ds(pl.multiple_of(r0, 16), 16), :]
        h2 = pltpu.bitcast((_ln(x2) * mrow(4, 16) + mrow(3, 16)).astype(BF16), F32)
        hn[pl.ds(r2, 8), :] = h2
        return pltpu.bitcast(h2[:, D - 128:], U32)

    def bulk_o(one, carry):
        dep = None
        for i in range(2):
            lo = jnp.concatenate([oring[h, pl.ds(i * 256, 256), :] for h in range(H)], axis=1).astype(BF16)
            for n in range(8):
                if i == 0:
                    dep = mod_vpu(4 + n, dep)
                else:
                    for z in range(2):
                        dep = ln2_piece(one * FB + (2 * n + z) * 16, dep)
                ha[pl.ds(NSEG * TOK + i * 256, 256), pl.ds(n * 128, 128)] = _dot(lo, _bf(wo[n]))
        return carry

    with jax.named_scope("p3_bulk_o"):
        bulk_o(zero_s[0], 0)

    w1_copy.wait()
    w2_copy.wait()

    nb = S // FB

    out32 = out_hbm.bitcast(U32)
    HB = FB // 2

    def ffn(i, carry):
        rows2 = pl.ds(pl.multiple_of(i * HB, HB), HB)
        h2 = _bf(hn[rows2, :])
        g = jax.nn.gelu(_dot(h2, _bf(w1[...])) + rep(biasb[:, pl.ds(0, FF)], FB), approximate=True).astype(BF16)
        nxt = lax.rem(i + 1, nb) * FB
        dep = None
        for n in range(8):
            cols = pl.ds(n * 128, 128)
            for z in range(2):
                dep = ln2_piece(nxt + (2 * n + z) * 16, dep)
                y = _dot(g[z * HB:(z + 1) * HB], _bf(w2[:, cols])) + rep(biasb[:, pl.ds(FF + n * 128, 128)], HB)
                xr = pl.ds(pl.multiple_of(i * HB + z * (HB // 2), HB // 2), HB // 2)
                ar = pl.ds(pl.multiple_of(i * FB + z * HB, HB), HB)
                x2 = _bf(xs[xr, cols]).astype(F32) + rep(modb[2, :, cols], HB) * ha[ar, cols]
                xs[xr, cols] = pltpu.bitcast((x2 + rep(modb[5, :, cols], HB) * y).astype(BF16), U32)
        pltpu.make_async_copy(xs.at[rows2], out32.at[rows2], sem.at[SEM_OUT]).start()
        return carry

    with jax.named_scope("p4_ffn"):
        lax.fori_loop(0, nb, ffn, 0)
    pltpu.make_async_copy(xs, out32, sem.at[SEM_OUT]).wait()


@jax.jit
def pallas_adaLN_cond__memory_aug_recurrent_mem_tr__dense_activation_gelu__prompt_kernel(
    A_x, A_mem0, A_Wq, A_Wk, A_Wv, A_Wo, A_seg_len, B_x, B_w1, B_b1, B_w2, B_b2, c, w_mod,
):
    assert A_x.shape == (1, S, D) and A_Wq.shape == (D, H, E) and A_mem0.shape == (1, M, D)
    any_spec = pl.BlockSpec(memory_space=pl.ANY)
    out = pl.pallas_call(
        _kernel,
        out_shape=jax.ShapeDtypeStruct((S, D), BF16),
        in_specs=[any_spec] * 12,
        out_specs=any_spec,
        scratch_shapes=[
            pltpu.VMEM((S // 2, D), U32),
            pltpu.VMEM((96, D // 2, E), U32),
            pltpu.VMEM((8, H * E // 2, 128), U32),
            pltpu.VMEM((D // 2, FF), U32),
            pltpu.VMEM((FF // 2, D), U32),
            pltpu.VMEM((12, D // 2, 512), U32),
            pltpu.VMEM((H, RING, E), F32),
            pltpu.VMEM((H, RING, E), F32),
            pltpu.VMEM((H + 1, RING, E), F32),
            pltpu.VMEM((H, RING, E), F32),
            pltpu.VMEM((S, D), F32),
            pltpu.VMEM((S - PRE, D), F32),
            pltpu.VMEM((PRE // 2, D), U32),
            pltpu.VMEM((M, D), F32),
            pltpu.VMEM((6, 8, D), F32),
            pltpu.VMEM((8, FF + D), F32),
            pltpu.VMEM((80, 128), F32),
            pltpu.VMEM((8, 32, 128), F32),
            pltpu.VMEM((8, 128), U32),
            pltpu.VMEM((D // 2, 128), U32),
            pltpu.SMEM((1,), jnp.int32),
            pltpu.VMEM((M, D), BF16),
            pltpu.VMEM((FF,), BF16),
            pltpu.VMEM((D,), BF16),
            pltpu.VMEM((1, D), BF16),
            pltpu.SemaphoreType.DMA((NSEM,)),
        ],
        compiler_params=pltpu.CompilerParams(vmem_limit_bytes=127 * 1024 * 1024),
    )(
        A_x.reshape(S, D), A_mem0.reshape(M, D),
        A_Wq.reshape(D // 2, 2, H, E), A_Wk.reshape(D // 2, 2, H, E), A_Wv.reshape(D // 2, 2, H, E),
        A_Wo.reshape(H * E, D), B_w1, B_b1, B_w2, B_b2, c, w_mod,
    )
    return out.reshape(1, S, D)
```

```python
import math

import jax
import jax.numpy as jnp
from jax import lax
import jax.experimental.pallas as pl
import jax.experimental.pallas.tpu as pltpu

F32 = jnp.float32
BF16 = jnp.bfloat16
U32 = jnp.uint32

S = 2048
D = 1024
H = 32
E = 128
M = 8
SEG = 32
NSEG = S // SEG
FF = 3584
NP = H // 2
TOK = 24
PRE = S - NSEG * TOK
RING = 576
OOFF = (-NSEG * TOK) % RING
LN_EPS = 1e-5
FB = 256
XC = (S - PRE) // 6
UNROLL = 4

UNIT_GROUPS = [(0, 1), (1, 2), (2, 4), (4, 7)] + [(6 * i + 1, min(6 * i + 7, 48)) for i in range(1, 8)]

SEM_C = 0
SEM_MISC = 1
SEM_X0 = 2
SEM_MOD = 3
SEM_UNIT = 8
SEM_XC = SEM_UNIT + len(UNIT_GROUPS)
SEM_WO = SEM_XC + 6
SEM_W1 = SEM_WO + 1
SEM_W2 = SEM_W1 + 1
SEM_OUT = SEM_W2 + 1
NSEM = SEM_OUT + 1


def _ln(x):
    m = jnp.mean(x, axis=-1, keepdims=True)
    xc = x - m
    v = jnp.mean(xc * xc, axis=-1, keepdims=True)
    return xc * lax.rsqrt(v + LN_EPS)


def _bf(w32):
    return pltpu.bitcast(w32, BF16)


def _dot(a, b):
    return jnp.dot(a, b, preferred_element_type=F32)


def _kernel(x_hbm, mem0_hbm, wq_hbm, wk_hbm, wv_hbm, wo_hbm, w1_hbm, b1_hbm, w2_hbm, b2_hbm,
            c_hbm, wmod_hbm, out_hbm,
            xs, wqkv, wo, w1, w2, wmod, qka, qkb, vring, oring, ha, hn, hb, memb, modb, biasb,
            fillb, accb, zerob, colb, zero_s, mem0_ref, b1_ref, b2_ref, c_ref, sem):
    qkv_hbm = [r.bitcast(U32) for r in (wq_hbm, wk_hbm, wv_hbm)]
    x32 = x_hbm.bitcast(U32)
    wo32 = wo_hbm.bitcast(U32)
    wmod32 = wmod_hbm.bitcast(U32)

    def unit_start(u):
        j, m = u // 3, u % 3
        grp = [k for k, (lo, hi) in enumerate(UNIT_GROUPS) if lo <= u < hi][0]
        for p in range(2):
            pltpu.make_async_copy(qkv_hbm[m].at[:, p, j, :], wqkv.at[2 * u + p],
                                  sem.at[SEM_UNIT + grp]).start()

    def units_wait(grp, lo, n):
        blk = wqkv.at[pl.ds(2 * lo, 2 * n)]
        pltpu.make_async_copy(blk, blk, sem.at[SEM_UNIT + grp]).wait()

    def static_units_wait(grp):
        lo, hi = UNIT_GROUPS[grp]
        units_wait(grp, lo, hi - lo)

    def mod_copy(g):
        return pltpu.make_async_copy(wmod32.at[:, pl.ds(g * 512, 512)], wmod.at[g],
                                     sem.at[SEM_MOD + min(g, 4)])

    x0_copy = pltpu.make_async_copy(x32.at[pl.ds(0, PRE // 2)], xs.at[pl.ds(0, PRE // 2)],
                                    sem.at[SEM_X0])

    def xc_copy(i):
        rows = pl.ds(pl.multiple_of(PRE // 2 + i * (XC // 2), 64), XC // 2)
        return pltpu.make_async_copy(x32.at[rows], xs.at[rows], sem.at[SEM_XC + i])

    def wo_copy(n):
        return pltpu.make_async_copy(wo32.at[:, pl.ds(n * 128, 128)], wo.at[n], sem.at[SEM_WO])

    w1_copy = pltpu.make_async_copy(w1_hbm.bitcast(U32), w1, sem.at[SEM_W1])
    w2_copy = pltpu.make_async_copy(w2_hbm.bitcast(U32), w2, sem.at[SEM_W2])
    c_copy = pltpu.make_async_copy(c_hbm, c_ref, sem.at[SEM_C])
    misc_copies = [pltpu.make_async_copy(a, b, sem.at[SEM_MISC])
                   for a, b in ((mem0_hbm, mem0_ref), (b1_hbm, b1_ref), (b2_hbm, b2_ref))]

    def deinterleave(u):
        for k in range(D // 2 // 64):
            rows = pl.ds(k * 64, 64)
            a = wqkv[2 * u, rows, :]
            b = wqkv[2 * u + 1, rows, :]
            wqkv[2 * u, rows, :] = (a & jnp.uint32(0xFFFF)) | (b << 16)
            wqkv[2 * u + 1, rows, :] = (a >> 16) | (b & jnp.uint32(0xFFFF0000))

    def load_x16(row2, dep):
        xw = xs[pl.ds(row2, 8), :]
        if dep is not None:
            first = xw[:, 0:128] | (dep & zerob[...])
            xw = jnp.concatenate([first, xw[:, 128:]], axis=1)
        return _bf(xw).astype(F32)

    def rep(v8, n):
        return jnp.concatenate([v8] * (n // 8), axis=0)

    def mrow(k, n):
        return rep(modb[k], n)

    c_copy.start()
    x0_copy.start()
    for g in range(4):
        mod_copy(g).start()

    def start_units(lo, hi):
        for u in range(lo, hi):
            if u % 6 == 0 and 12 <= u:
                xc_copy(u // 6 - 2).start()
            unit_start(u)

    start_units(0, 28)

    def start_rest():
        for cp in misc_copies:
            cp.start()
        for n in range(8):
            wo_copy(n).start()
        for g in range(4, 12):
            mod_copy(g).start()
        w1_copy.start()
        w2_copy.start()

    r = lax.broadcasted_iota(jnp.int32, (80, 128), 0)
    q = lax.broadcasted_iota(jnp.int32, (80, 128), 1)
    r_tok = r < 64
    q_tok = q < 64
    r_head = jnp.where(r_tok, r >> 5, (r - 64) >> 3)
    q_head = jnp.where(q_tok, q >> 5, (q - 64) >> 3)
    same = (r_head == q_head) & (q < 80)
    causal_ok = jnp.logical_not(r_tok & q_tok & ((q & 31) > (r & 31)))
    scale = E ** (-0.5)
    fillb[...] = jnp.where(same, jnp.where(causal_ok, 0.0, -1e9 / scale), -jnp.inf).astype(F32)
    zerob[...] = jnp.zeros((8, 128), U32)
    zero_s[0] = 0

    def silu_c():
        cf = c_ref[...].astype(F32)
        return jnp.broadcast_to((cf * jax.nn.sigmoid(cf)).astype(BF16), (16, D))

    def mod_part(sc16, lo, hi):
        for g in range(lo, hi):
            y = _dot(sc16, _bf(wmod[g]))[0:8].astype(BF16).astype(F32)
            if g // 2 in (1, 4):
                y = 1.0 + y
            modb[g // 2, :, pl.ds((g % 2) * 512, 512)] = y

    def pre_norm(i, carry):
        rows = pl.ds(pl.multiple_of(i * 64, 64), 64)
        ha[rows, :] = _ln(_bf(xs[pl.ds(pl.multiple_of(i * 32, 32), 32), :]).astype(F32))
        return carry

    c_copy.wait()
    x0_copy.wait()
    with jax.named_scope("p0_ln"):
        lax.fori_loop(0, PRE // 64, pre_norm, 0)

    sc16 = silu_c()
    scf = jnp.broadcast_to(sc16[0:1].astype(F32), (128, D))
    for k in range(8):
        colb[pl.ds(k * 64, 64), :] = pltpu.bitcast(scf[:, k * 128:(k + 1) * 128].T.astype(BF16), U32)
    for g in range(4):
        mod_copy(g).wait()
        mod_part(sc16, g, g + 1)

    for i in range(PRE // 64):
        hb[pl.ds(i * 32, 32), :] = pltpu.bitcast(
            (ha[pl.ds(i * 64, 64), :] * mrow(1, 64) + mrow(0, 64)).astype(BF16), U32)

    static_units_wait(0)
    deinterleave(0)

    def bulk_qkv(i, waits, last, with_ln):
        rows = pl.ds(RING - PRE, PRE)
        dep = None
        for k in range(6):
            u = 6 * i + k
            cls, m = k // 3, k % 3
            for p in range(2):
                y = _dot(_bf(hb[...]), _bf(wqkv[2 * u + p]))
                if m == 2:
                    vring[4 * i + 2 * cls + p, rows, :] = y
                else:
                    (qka, qkb)[cls][4 * i + 2 * m + p, rows, :] = y
                if p == 0:
                    if k in waits:
                        static_units_wait(waits[k])
                    if not (last and k == 5):
                        deinterleave(u + 1)
                if with_ln and k >= 2:
                    for z in range(2):
                        r0 = (i - 1) * XC + (4 * k + 2 * p + z - 8) * 16
                        x16 = load_x16(pl.multiple_of(PRE // 2 + r0 // 2, 8), dep)
                        h16 = _ln(x16) * mrow(1, 16) + mrow(0, 16)
                        hn[pl.ds(pl.multiple_of(r0, 16), 16), :] = h16
                        dep = pltpu.bitcast(h16[8:16, D - 128:], U32)

    def phase1(i, carry):
        @pl.when(i == 2)
        def _():
            start_units(28, 48)

        @pl.when(i == 4)
        def _():
            start_rest()

        xc_copy(i - 1).wait()
        units_wait(3 + i, 6 * i + 1, 6)
        bulk_qkv(i, {}, False, True)
        return carry

    bulk_qkv(0, {0: 1, 1: 2, 3: 3}, False, False)
    with jax.named_scope("p1_bulk_qkv"):
        lax.fori_loop(1, 7, phase1, 0)
    static_units_wait(10)
    bulk_qkv(7, {}, True, False)
    for cp in misc_copies:
        cp.wait()
    memb[...] = mem0_ref[...].astype(F32)
    biasb[:, pl.ds(0, FF)] = jnp.broadcast_to(b1_ref[...].astype(F32).reshape(1, FF), (8, FF))
    biasb[:, pl.ds(FF, D)] = jnp.broadcast_to(b2_ref[...].astype(F32).reshape(1, D), (8, D))
    for n in range(8):
        wo_copy(n).wait()

    cexp = scale * math.log2(math.e)
    NG = NP // 2
    grp = [(4 * (g // 2) + (g % 2), 4 * (g // 2) + (g % 2) + 2) for g in range(NG)]
    early = [2 * j + u for g in range(NG - 3) for j in grp[g] for u in range(2)]
    late = [h for h in range(H) if h not in early]

    def step(s, split):
        w0 = pl.multiple_of(lax.rem(TOK * s, RING), 8)
        r0 = pl.multiple_of(lax.rem(SEG * s + (RING - PRE), RING), 32)
        ow = pl.multiple_of(lax.rem(SEG * s + OOFF, RING), 32)
        o0 = pl.multiple_of(lax.rem(TOK * s + OOFF, RING), 8)
        a0 = pl.multiple_of(TOK * s, 8)
        X = jnp.concatenate([hn[pl.ds(a0, TOK), :], memb[...]], axis=0).astype(BF16)
        ym = [None] * 96
        probs = [None] * NP
        om = [None] * H
        order = (4, 5, 0, 1, 2, 3)

        if split:
            for t in order:
                accb[t] = _dot(X[:, :D // 2], _bf(wqkv[t, pl.ds(0, D // 4), :]))

        def slot(j, t):
            if t >= 4:
                return vring, 2 * j + t - 4
            return (qka, qkb)[j % 2], 4 * (j // 2) + t

        def proj(j, t):
            c = 6 * j + t
            if split and j == 0:
                y = accb[t] + _dot(X[:, D // 2:], _bf(wqkv[c, pl.ds(D // 4, D // 4), :]))
            else:
                y = _dot(X, _bf(wqkv[c]))
            ref, k = slot(j, t)
            ref[k, pl.ds(w0, TOK), :] = y[0:TOK]
            ym[c] = y[TOK:TOK + M]

        def gather(j, m, pad):
            c = 6 * j + 2 * m
            ref, k = slot(j, 2 * m)
            parts = [ref[k, pl.ds(r0, SEG), :], ref[k + 1, pl.ds(r0, SEG), :], ym[c], ym[c + 1]]
            if pad:
                parts.append(jnp.zeros((48, E), F32))
            return jnp.concatenate(parts, axis=0).astype(BF16)

        def scores(j):
            sc_ = lax.dot_general(gather(j, 0, False), gather(j, 1, True),
                                  (((1,), (1,)), ((), ())), preferred_element_type=F32)
            fill = fillb[...]
            sc_ = jnp.where(fill == 0.0, sc_, fill)
            mx = jnp.max(sc_, axis=-1, keepdims=True)
            p = jnp.exp2((sc_ - mx) * cexp)
            l = jnp.sum(p, axis=-1, keepdims=True)
            rl = pl.reciprocal(l, approx=True)
            rl = rl * (2.0 - l * rl)
            probs[j] = (p * rl).astype(BF16)

        def park(j):
            vring[H, pl.ds(40 * (j % 8), 40), :] = pltpu.bitcast(probs[j], F32)
            probs[j] = None

        def pv(j):
            P = probs[j]
            if P is None:
                P = _bf(vring[H, pl.ds(40 * (j % 8), 40), :])
            o = _dot(P, gather(j, 2, True))
            oring[2 * j, pl.ds(ow, SEG), :] = o[0:32]
            oring[2 * j + 1, pl.ds(ow, SEG), :] = o[32:64]
            om[2 * j] = o[64:72]
            om[2 * j + 1] = o[72:80]

        def o_lhs(hs):
            return jnp.concatenate(
                [jnp.concatenate([oring[h, pl.ds(o0, TOK), :], om[h]], axis=0) for h in hs],
                axis=1).astype(BF16)

        def o_rhs(n, hs):
            return _bf(jnp.concatenate([wo[n, pl.ds(h * 64, 64), :] for h in hs], axis=0))

        for g in range(NG):
            cols = [(j, t) for j in grp[g] for t in order]
            if g == 2:
                cols = ([(j, t) for j in grp[g] for t in (4, 5)]
                        + [(j, t) for j in grp[g] for t in range(4)])
            for j in (grp[0] + grp[1] if g == 3 else grp[g - 2] if g >= 4 else ()):
                park(j)
            for ci, (j, t) in enumerate(cols):
                if g == 2 and ci == 4:
                    for jj in grp[0] + grp[1]:
                        scores(jj)
                if g >= 3 and ci == 6:
                    for jj in grp[g - 1]:
                        scores(jj)
                    for jj in grp[g - 3]:
                        pv(jj)
                proj(j, t)
        lo = o_lhs(early)
        for n in range(8):
            accb[n] = _dot(lo, o_rhs(n, early))
            if n == 1:
                for jj in grp[NG - 1]:
                    scores(jj)
                for jj in grp[NG - 3]:
                    pv(jj)
            if n == 4:
                for jj in grp[NG - 2] + grp[NG - 1]:
                    pv(jj)
        lo = o_lhs(late)
        for n in range(8):
            a = accb[n] + _dot(lo, o_rhs(n, late))
            ha[pl.ds(a0, TOK), pl.ds(n * 128, 128)] = a[0:TOK]
            memb[:, pl.ds(n * 128, 128)] = a[TOK:TOK + M]

    def steps(i, carry):
        for k in range(UNROLL):
            step(i * UNROLL + k, k > 0)
        return carry

    with jax.named_scope("p2_steps"):
        lax.fori_loop(0, NSEG // UNROLL, steps, 0)

    for g in range(4, 12):
        mod_copy(g).wait()

    def lo16(w):
        return pltpu.bitcast(w << 16, F32)

    def hi16(w):
        return pltpu.bitcast(w & jnp.uint32(0xFFFF0000), F32)

    def mod_vpu(g, dep):
        for t in range(4):
            acc = None if dep is None else pltpu.bitcast(dep & zerob[...], F32)
            for k in range(D // 16):
                cw = colb[pl.ds(k * 8, 8), :]
                w = wmod[g, pl.ds(k * 8, 8), pl.ds(t * 128, 128)]
                pe = lo16(w) * lo16(cw)
                acc = pe if acc is None else acc + pe
                acc = acc + hi16(w) * hi16(cw)
            dep = pltpu.bitcast(acc, U32)
            y = jnp.sum(acc, axis=0, keepdims=True).astype(BF16).astype(F32)
            if g // 2 == 4:
                y = 1.0 + y
            modb[g // 2, :, pl.ds((g % 2) * 512 + t * 128, 128)] = jnp.broadcast_to(y, (8, 128))
        return dep

    def ln2_piece(r0, dep):
        r2 = pl.multiple_of(r0 // 2, 8)
        x2 = load_x16(r2, dep) + mrow(2, 16) * ha[pl.ds(pl.multiple_of(r0, 16), 16), :]
        h2 = pltpu.bitcast((_ln(x2) * mrow(4, 16) + mrow(3, 16)).astype(BF16), F32)
        hn[pl.ds(r2, 8), :] = h2
        return pltpu.bitcast(h2[:, D - 128:], U32)

    def bulk_o(one, carry):
        dep = None
        for i in range(2):
            lo = jnp.concatenate([oring[h, pl.ds(i * 256, 256), :] for h in range(H)], axis=1).astype(BF16)
            for n in range(8):
                if i == 0:
                    dep = mod_vpu(4 + n, dep)
                else:
                    for z in range(2):
                        dep = ln2_piece(one * FB + (2 * n + z) * 16, dep)
                ha[pl.ds(NSEG * TOK + i * 256, 256), pl.ds(n * 128, 128)] = _dot(lo, _bf(wo[n]))
        return carry

    with jax.named_scope("p3_bulk_o"):
        bulk_o(zero_s[0], 0)

    w1_copy.wait()
    w2_copy.wait()

    nb = S // FB

    out32 = out_hbm.bitcast(U32)
    HB = FB // 2

    def ffn(i, carry):
        rows2 = pl.ds(pl.multiple_of(i * HB, HB), HB)
        h2 = _bf(hn[rows2, :])
        g = jax.nn.gelu(_dot(h2, _bf(w1[...])) + rep(biasb[:, pl.ds(0, FF)], FB), approximate=True).astype(BF16)
        nxt = lax.rem(i + 1, nb) * FB
        dep = None
        for n in range(8):
            cols = pl.ds(n * 128, 128)
            for z in range(2):
                dep = ln2_piece(nxt + (2 * n + z) * 16, dep)
                y = _dot(g[z * HB:(z + 1) * HB], _bf(w2[:, cols])) + rep(biasb[:, pl.ds(FF + n * 128, 128)], HB)
                xr = pl.ds(pl.multiple_of(i * HB + z * (HB // 2), HB // 2), HB // 2)
                ar = pl.ds(pl.multiple_of(i * FB + z * HB, HB), HB)
                x2 = _bf(xs[xr, cols]).astype(F32) + rep(modb[2, :, cols], HB) * ha[ar, cols]
                xs[xr, cols] = pltpu.bitcast((x2 + rep(modb[5, :, cols], HB) * y).astype(BF16), U32)
        pltpu.make_async_copy(xs.at[rows2], out32.at[rows2], sem.at[SEM_OUT]).start()
        return carry

    with jax.named_scope("p4_ffn"):
        lax.fori_loop(0, nb, ffn, 0)
    pltpu.make_async_copy(xs, out32, sem.at[SEM_OUT]).wait()


@jax.jit
def pallas_adaLN_cond__memory_aug_recurrent_mem_tr__dense_activation_gelu__prompt_kernel(
    A_x, A_mem0, A_Wq, A_Wk, A_Wv, A_Wo, A_seg_len, B_x, B_w1, B_b1, B_w2, B_b2, c, w_mod,
):
    assert A_x.shape == (1, S, D) and A_Wq.shape == (D, H, E) and A_mem0.shape == (1, M, D)
    any_spec = pl.BlockSpec(memory_space=pl.ANY)
    out = pl.pallas_call(
        _kernel,
        out_shape=jax.ShapeDtypeStruct((S, D), BF16),
        in_specs=[any_spec] * 12,
        out_specs=any_spec,
        scratch_shapes=[
            pltpu.VMEM((S // 2, D), U32),
            pltpu.VMEM((96, D // 2, E), U32),
            pltpu.VMEM((8, H * E // 2, 128), U32),
            pltpu.VMEM((D // 2, FF), U32),
            pltpu.VMEM((FF // 2, D), U32),
            pltpu.VMEM((12, D // 2, 512), U32),
            pltpu.VMEM((H, RING, E), F32),
            pltpu.VMEM((H, RING, E), F32),
            pltpu.VMEM((H + 1, RING, E), F32),
            pltpu.VMEM((H, RING, E), F32),
            pltpu.VMEM((S, D), F32),
            pltpu.VMEM((S - PRE, D), F32),
            pltpu.VMEM((PRE // 2, D), U32),
            pltpu.VMEM((M, D), F32),
            pltpu.VMEM((6, 8, D), F32),
            pltpu.VMEM((8, FF + D), F32),
            pltpu.VMEM((80, 128), F32),
            pltpu.VMEM((8, 32, 128), F32),
            pltpu.VMEM((8, 128), U32),
            pltpu.VMEM((D // 2, 128), U32),
            pltpu.SMEM((1,), jnp.int32),
            pltpu.VMEM((M, D), BF16),
            pltpu.VMEM((FF,), BF16),
            pltpu.VMEM((D,), BF16),
            pltpu.VMEM((1, D), BF16),
            pltpu.SemaphoreType.DMA((NSEM,)),
        ],
        compiler_params=pltpu.CompilerParams(vmem_limit_bytes=127 * 1024 * 1024),
    )(
        A_x.reshape(S, D), A_mem0.reshape(M, D),
        A_Wq.reshape(D // 2, 2, H, E), A_Wk.reshape(D // 2, 2, H, E), A_Wv.reshape(D // 2, 2, H, E),
        A_Wo.reshape(H * E, D), B_w1, B_b1, B_w2, B_b2, c, w_mod,
    )
    return out.reshape(1, S, D)
```

```python
import math

import jax
import jax.numpy as jnp
from jax import lax
import jax.experimental.pallas as pl
import jax.experimental.pallas.tpu as pltpu

F32 = jnp.float32
BF16 = jnp.bfloat16
U32 = jnp.uint32

S = 2048
D = 1024
H = 32
E = 128
M = 8
SEG = 32
NSEG = S // SEG
FF = 3584
NP = H // 2
TOK = 24
PRE = S - NSEG * TOK
RING = 576
OOFF = (-NSEG * TOK) % RING
LN_EPS = 1e-5
FB = 256
XC = (S - PRE) // 6
UNROLL = 4

NQ = 4
KQ = D // NQ

FIRST_STARTS = [('m', 0), ('w', 0, 0), ('w', 0, 1), ('m', 1), ('w', 1, 0), ('m', 2), ('w', 1, 1)]
P1A_BLOCKS = [
    ([], [('m', 0)]),
    ([], [('w', 0, 0)]),
    ([('w', 2, 0), ('m', 3), ('w', 2, 1)], [('m', 1), ('w', 0, 1)]),
    ([('w', 3, 0), ('w', 3, 1)], [('m', 2), ('w', 1, 0)]),
    ([('g', 2), ('g', 3)], [('w', 1, 1), ('w', 2, 0)]),
    ([], [('m', 3), ('w', 2, 1), ('w', 3, 0)]),
    ([('g', 4), ('g', 5)], [('w', 3, 1)]),
]

SEM_C = 0
SEM_X0 = 1
SEM_MOD = 2
SEM_WA = SEM_MOD + NQ + 1
SEM_WB = SEM_WA + 2 * NQ
SEM_XC = SEM_WB + 6
SEM_WO = SEM_XC + 6
SEM_W1 = SEM_WO + 1
SEM_W2 = SEM_W1 + 1
SEM_OUT = SEM_W2 + 1
NSEM = SEM_OUT + 1


def _ln(x):
    m = jnp.mean(x, axis=-1, keepdims=True)
    xc = x - m
    v = jnp.mean(xc * xc, axis=-1, keepdims=True)
    return xc * lax.rsqrt(v + LN_EPS)


def _bf(w32):
    return pltpu.bitcast(w32, BF16)


def _dot(a, b):
    return jnp.dot(a, b, preferred_element_type=F32)


def _kernel(x_hbm, mem0_hbm, wq_hbm, wk_hbm, wv_hbm, wo_hbm, w1_hbm, b1_hbm, w2_hbm, b2_hbm,
            c_hbm, wmod_hbm, out_hbm,
            xs, wqkv, wo, w1, w2, wmoda, wmod, qka, qkb, vring, oring, ha, hn, hb, memb, moda, modb, scb, biasb,
            fillb, accb, zerob, colb, zero_s, mem0_ref, b1_ref, b2_ref, c_ref, sem):
    qkv_hbm = [r.bitcast(U32) for r in (wq_hbm, wk_hbm, wv_hbm)]
    x32 = x_hbm.bitcast(U32)
    wo32 = wo_hbm.bitcast(U32)
    wmod32 = wmod_hbm.bitcast(U32)

    def group_start(i, rows, sem_idx):
        for u in range(6 * i, 6 * i + 6):
            j, m = u // 3, u % 3
            for p in range(2):
                pltpu.make_async_copy(qkv_hbm[m].at[rows, p, j, :], wqkv.at[2 * u + p, rows, :],
                                      sem.at[sem_idx]).start()

    def group_wait(i, rows, sem_idx):
        blk = wqkv.at[pl.ds(12 * i, 12), rows, :]
        pltpu.make_async_copy(blk, blk, sem.at[sem_idx]).wait()

    def item_start(item):
        if item[0] == 'm':
            qq = item[1]
            for k in range(2):
                pltpu.make_async_copy(wmod32.at[:, pl.ds(k * D + qq * KQ, KQ)], wmoda.at[qq, k],
                                      sem.at[SEM_MOD + qq]).start()
        elif item[0] == 'w':
            _, qq, i = item
            group_start(i, pl.ds(qq * (KQ // 2), KQ // 2), SEM_WA + 2 * qq + i)
        else:
            whole_start(item[1])

    def item_wait(item):
        if item[0] == 'm':
            qq = item[1]
            pltpu.make_async_copy(wmoda.at[qq], wmoda.at[qq], sem.at[SEM_MOD + qq]).wait()
        else:
            _, qq, i = item
            group_wait(i, pl.ds(qq * (KQ // 2), KQ // 2), SEM_WA + 2 * qq + i)

    def whole_start(i):
        xc_copy(i - 2).start()
        group_start(i, pl.ds(0, D // 2), SEM_WB + i - 2)

    def mod_copy(g):
        return pltpu.make_async_copy(wmod32.at[:, pl.ds(2 * D + g * 512, 512)], wmod.at[g],
                                     sem.at[SEM_MOD + NQ])

    x0_copy = pltpu.make_async_copy(x32.at[pl.ds(0, PRE // 2)], xs.at[pl.ds(0, PRE // 2)],
                                    sem.at[SEM_X0])

    def xc_copy(i):
        rows = pl.ds(pl.multiple_of(PRE // 2 + i * (XC // 2), 64), XC // 2)
        return pltpu.make_async_copy(x32.at[rows], xs.at[rows], sem.at[SEM_XC + i])

    def wo_copy(n):
        return pltpu.make_async_copy(wo32.at[:, pl.ds(n * 128, 128)], wo.at[n], sem.at[SEM_WO])

    w1_copy = pltpu.make_async_copy(w1_hbm.bitcast(U32), w1, sem.at[SEM_W1])
    w2_copy = pltpu.make_async_copy(w2_hbm.bitcast(U32), w2, sem.at[SEM_W2])
    small_copies = [pltpu.make_async_copy(a, b, sem.at[SEM_C])
                    for a, b in ((c_hbm, c_ref), (mem0_hbm, mem0_ref), (b1_hbm, b1_ref),
                                 (b2_hbm, b2_ref))]

    def deinterleave(u, row0, nrows):
        for k in range(nrows // 64):
            rows = pl.ds(row0 + k * 64, 64)
            a = wqkv[2 * u, rows, :]
            b = wqkv[2 * u + 1, rows, :]
            wqkv[2 * u, rows, :] = (a & jnp.uint32(0xFFFF)) | (b << 16)
            wqkv[2 * u + 1, rows, :] = (a >> 16) | (b & jnp.uint32(0xFFFF0000))

    def load_x16(row2, dep):
        xw = xs[pl.ds(row2, 8), :]
        if dep is not None:
            first = xw[:, 0:128] | (dep & zerob[...])
            xw = jnp.concatenate([first, xw[:, 128:]], axis=1)
        return _bf(xw).astype(F32)

    def rep(v8, n):
        return jnp.concatenate([v8] * (n // 8), axis=0)

    def mrow(k, n):
        if k < 2:
            return rep(jnp.concatenate([moda[qq, k] for qq in range(NQ)], axis=1), n)
        return rep(modb[k - 2], n)

    for cp in small_copies:
        cp.start()
    x0_copy.start()
    for item in FIRST_STARTS:
        item_start(item)

    def start_rest():
        for n in range(8):
            wo_copy(n).start()
        for g in range(8):
            mod_copy(g).start()
        w1_copy.start()
        w2_copy.start()

    r = lax.broadcasted_iota(jnp.int32, (80, 128), 0)
    q = lax.broadcasted_iota(jnp.int32, (80, 128), 1)
    r_tok = r < 64
    q_tok = q < 64
    r_head = jnp.where(r_tok, r >> 5, (r - 64) >> 3)
    q_head = jnp.where(q_tok, q >> 5, (q - 64) >> 3)
    same = (r_head == q_head) & (q < 80)
    causal_ok = jnp.logical_not(r_tok & q_tok & ((q & 31) > (r & 31)))
    scale = E ** (-0.5)
    fillb[...] = jnp.where(same, jnp.where(causal_ok, 0.0, -1e9 / scale), -jnp.inf).astype(F32)
    zerob[...] = jnp.zeros((8, 128), U32)
    zero_s[0] = 0

    pre_rows = pl.ds(RING - PRE, PRE)

    for cp in small_copies:
        cp.wait()
    cf = c_ref[...].astype(F32)
    sc = (cf * jax.nn.sigmoid(cf)).astype(BF16)
    scb[...] = pltpu.bitcast(jnp.broadcast_to(sc, (16, D)), U32)
    scf = jnp.broadcast_to(sc.astype(F32), (128, D))
    for k in range(8):
        colb[pl.ds(k * 64, 64), :] = pltpu.bitcast(scf[:, k * 128:(k + 1) * 128].T.astype(BF16), U32)
    memb[...] = mem0_ref[...].astype(F32)
    biasb[:, pl.ds(0, FF)] = jnp.broadcast_to(b1_ref[...].astype(F32).reshape(1, FF), (8, FF))
    biasb[:, pl.ds(FF, D)] = jnp.broadcast_to(b2_ref[...].astype(F32).reshape(1, D), (8, D))

    def pre_norm(i, carry):
        xn = _ln(_bf(xs[pl.ds(pl.multiple_of(i * 32, 32), 32), :]).astype(F32))
        for n in range(8):
            oring[n, pl.ds(pl.multiple_of(i * 64, 64), 64), :] = xn[:, n * 128:(n + 1) * 128]
        return carry

    x0_copy.wait()
    with jax.named_scope("p0_ln"):
        lax.fori_loop(0, PRE // 64, pre_norm, 0)

    def dst_slot(i, k, p):
        cls, m = k // 3, k % 3
        if m == 2:
            return vring, 4 * i + 2 * cls + p
        return (qka, qkb)[cls], 4 * i + 2 * m + p

    NT = KQ // 128

    def item_run(item):
        if item[0] == 'm':
            qq = item[1]
            sc16 = _bf(scb[...])
            ca1 = 1.0 + _dot(sc16, _bf(wmoda[qq, 1]))[0:8].astype(BF16).astype(F32)
            sa = _dot(sc16, _bf(wmoda[qq, 0]))[0:8].astype(BF16).astype(F32)
            moda[qq, 0] = sa
            moda[qq, 1] = ca1
            for n in range(NT):
                cols = slice(n * 128, (n + 1) * 128)
                for z in range(PRE // 64):
                    hq = (oring[NT * qq + n, pl.ds(z * 64, 64), :] * rep(ca1[:, cols], 64)
                          + rep(sa[:, cols], 64))
                    hb[NT * qq + n, pl.ds(z * 32, 32), :] = pltpu.bitcast(hq.astype(BF16), U32)
            return
        _, qq, i = item
        row0 = qq * (KQ // 2)
        for k in range(6):
            u = 6 * i + k
            deinterleave(u, row0, KQ // 2)
            for p in range(2):
                lhs = _bf(jnp.concatenate([hb[NT * qq + n] for n in range(NT)], axis=1))
                ref, idx = dst_slot(i, k, p)
                y = _dot(lhs, _bf(wqkv[2 * u + p, pl.ds(row0, KQ // 2), :]))
                if qq > 0:
                    y = y + ref[idx, pre_rows, :]
                ref[idx, pre_rows, :] = y

    def phase1b(i, carry):
        @pl.when(i == 3)
        def _():
            whole_start(6)
            whole_start(7)

        @pl.when(i == 4)
        def _():
            start_rest()

        xc_copy(i - 2).wait()
        group_wait(i, pl.ds(0, D // 2), SEM_WB + i - 2)
        deinterleave(6 * i, 0, D // 2)
        dep = None
        for k in range(6):
            u = 6 * i + k
            for p in range(2):
                lhs = _bf(jnp.concatenate([hb[n] for n in range(8)], axis=1))
                ref, idx = dst_slot(i, k, p)
                ref[idx, pre_rows, :] = _dot(lhs, _bf(wqkv[2 * u + p]))
                if p == 0 and k < 5:
                    deinterleave(u + 1, 0, D // 2)
                if k >= 2:
                    for z in range(2):
                        r0 = (i - 2) * XC + (4 * k + 2 * p + z - 8) * 16
                        x16 = load_x16(pl.multiple_of(PRE // 2 + r0 // 2, 8), dep)
                        h16 = _ln(x16) * mrow(1, 16) + mrow(0, 16)
                        hn[pl.ds(pl.multiple_of(r0, 16), 16), :] = h16
                        dep = pltpu.bitcast(h16[8:16, D - 128:], U32)
        return carry

    for bi, (starts, items) in enumerate(P1A_BLOCKS):
        for item in starts:
            item_start(item)
        with jax.named_scope("p1a_wait%d" % bi):
            for item in items:
                item_wait(item)
        for item in items:
            item_run(item)
    with jax.named_scope("p1b"):
        lax.fori_loop(2, 8, phase1b, 0)
    for n in range(8):
        wo_copy(n).wait()

    cexp = scale * math.log2(math.e)
    NG = NP // 2
    grp = [(4 * (g // 2) + (g % 2), 4 * (g // 2) + (g % 2) + 2) for g in range(NG)]
    early = [2 * j + u for g in range(NG - 3) for j in grp[g] for u in range(2)]
    late = [h for h in range(H) if h not in early]

    def step(s, split):
        w0 = pl.multiple_of(lax.rem(TOK * s, RING), 8)
        r0 = pl.multiple_of(lax.rem(SEG * s + (RING - PRE), RING), 32)
        ow = pl.multiple_of(lax.rem(SEG * s + OOFF, RING), 32)
        o0 = pl.multiple_of(lax.rem(TOK * s + OOFF, RING), 8)
        a0 = pl.multiple_of(TOK * s, 8)
        X = jnp.concatenate([hn[pl.ds(a0, TOK), :], memb[...]], axis=0).astype(BF16)
        ym = [None] * 96
        probs = [None] * NP
        om = [None] * H
        order = (4, 5, 0, 1, 2, 3)

        if split:
            for t in order:
                accb[t] = _dot(X[:, :D // 2], _bf(wqkv[t, pl.ds(0, D // 4), :]))

        def slot(j, t):
            if t >= 4:
                return vring, 2 * j + t - 4
            return (qka, qkb)[j % 2], 4 * (j // 2) + t

        def proj(j, t):
            c = 6 * j + t
            if split and j == 0:
                y = accb[t] + _dot(X[:, D // 2:], _bf(wqkv[c, pl.ds(D // 4, D // 4), :]))
            else:
                y = _dot(X, _bf(wqkv[c]))
            ref, k = slot(j, t)
            ref[k, pl.ds(w0, TOK), :] = y[0:TOK]
            ym[c] = y[TOK:TOK + M]

        def gather(j, m, pad):
            c = 6 * j + 2 * m
            ref, k = slot(j, 2 * m)
            parts = [ref[k, pl.ds(r0, SEG), :], ref[k + 1, pl.ds(r0, SEG), :], ym[c], ym[c + 1]]
            if pad:
                parts.append(jnp.zeros((48, E), F32))
            return jnp.concatenate(parts, axis=0).astype(BF16)

        def scores(j):
            sc_ = lax.dot_general(gather(j, 0, False), gather(j, 1, True),
                                  (((1,), (1,)), ((), ())), preferred_element_type=F32)
            fill = fillb[...]
            sc_ = jnp.where(fill == 0.0, sc_, fill)
            mx = jnp.max(sc_, axis=-1, keepdims=True)
            p = jnp.exp2((sc_ - mx) * cexp)
            l = jnp.sum(p, axis=-1, keepdims=True)
            rl = pl.reciprocal(l, approx=True)
            rl = rl * (2.0 - l * rl)
            probs[j] = (p * rl).astype(BF16)

        def park(j):
            vring[H, pl.ds(40 * (j % 8), 40), :] = pltpu.bitcast(probs[j], F32)
            probs[j] = None

        def pv(j):
            P = probs[j]
            if P is None:
                P = _bf(vring[H, pl.ds(40 * (j % 8), 40), :])
            o = _dot(P, gather(j, 2, True))
            oring[2 * j, pl.ds(ow, SEG), :] = o[0:32]
            oring[2 * j + 1, pl.ds(ow, SEG), :] = o[32:64]
            om[2 * j] = o[64:72]
            om[2 * j + 1] = o[72:80]

        def o_lhs(hs):
            return jnp.concatenate(
                [jnp.concatenate([oring[h, pl.ds(o0, TOK), :], om[h]], axis=0) for h in hs],
                axis=1).astype(BF16)

        def o_rhs(n, hs):
            return _bf(jnp.concatenate([wo[n, pl.ds(h * 64, 64), :] for h in hs], axis=0))

        for g in range(NG):
            cols = [(j, t) for j in grp[g] for t in order]
            if g == 2:
                cols = ([(j, t) for j in grp[g] for t in (4, 5)]
                        + [(j, t) for j in grp[g] for t in range(4)])
            for j in (grp[0] + grp[1] if g == 3 else grp[g - 2] if g >= 4 else ()):
                park(j)
            for ci, (j, t) in enumerate(cols):
                if g == 2 and ci == 4:
                    for jj in grp[0] + grp[1]:
                        scores(jj)
                if g >= 3 and ci == 6:
                    for jj in grp[g - 1]:
                        scores(jj)
                    for jj in grp[g - 3]:
                        pv(jj)
                proj(j, t)
        lo = o_lhs(early)
        for n in range(8):
            accb[n] = _dot(lo, o_rhs(n, early))
            if n == 1:
                for jj in grp[NG - 1]:
                    scores(jj)
                for jj in grp[NG - 3]:
                    pv(jj)
            if n == 4:
                for jj in grp[NG - 2] + grp[NG - 1]:
                    pv(jj)
        lo = o_lhs(late)
        for n in range(8):
            a = accb[n] + _dot(lo, o_rhs(n, late))
            ha[pl.ds(a0, TOK), pl.ds(n * 128, 128)] = a[0:TOK]
            memb[:, pl.ds(n * 128, 128)] = a[TOK:TOK + M]

    def steps(i, carry):
        for k in range(UNROLL):
            step(i * UNROLL + k, k > 0)
        return carry

    with jax.named_scope("p2_steps"):
        lax.fori_loop(0, NSEG // UNROLL, steps, 0)

    for g in range(8):
        mod_copy(g).wait()

    def lo16(w):
        return pltpu.bitcast(w << 16, F32)

    def hi16(w):
        return pltpu.bitcast(w & jnp.uint32(0xFFFF0000), F32)

    def mod_vpu(g, dep):
        for t in range(4):
            acc = None if dep is None else pltpu.bitcast(dep & zerob[...], F32)
            for k in range(D // 16):
                cw = colb[pl.ds(k * 8, 8), :]
                w = wmod[g, pl.ds(k * 8, 8), pl.ds(t * 128, 128)]
                pe = lo16(w) * lo16(cw)
                acc = pe if acc is None else acc + pe
                acc = acc + hi16(w) * hi16(cw)
            dep = pltpu.bitcast(acc, U32)
            y = jnp.sum(acc, axis=0, keepdims=True).astype(BF16).astype(F32)
            if g // 2 == 2:
                y = 1.0 + y
            modb[g // 2, :, pl.ds((g % 2) * 512 + t * 128, 128)] = jnp.broadcast_to(y, (8, 128))
        return dep

    def ln2_piece(r0, dep):
        r2 = pl.multiple_of(r0 // 2, 8)
        x2 = load_x16(r2, dep) + mrow(2, 16) * ha[pl.ds(pl.multiple_of(r0, 16), 16), :]
        h2 = pltpu.bitcast((_ln(x2) * mrow(4, 16) + mrow(3, 16)).astype(BF16), F32)
        hn[pl.ds(r2, 8), :] = h2
        return pltpu.bitcast(h2[:, D - 128:], U32)

    def bulk_o(one, carry):
        dep = None
        for i in range(2):
            lo = jnp.concatenate([oring[h, pl.ds(i * 256, 256), :] for h in range(H)], axis=1).astype(BF16)
            for n in range(8):
                if i == 0:
                    dep = mod_vpu(n, dep)
                else:
                    for z in range(2):
                        dep = ln2_piece(one * FB + (2 * n + z) * 16, dep)
                ha[pl.ds(NSEG * TOK + i * 256, 256), pl.ds(n * 128, 128)] = _dot(lo, _bf(wo[n]))
        return carry

    with jax.named_scope("p3_bulk_o"):
        bulk_o(zero_s[0], 0)

    w1_copy.wait()
    w2_copy.wait()

    nb = S // FB

    out32 = out_hbm.bitcast(U32)
    HB = FB // 2

    def ffn(i, carry):
        rows2 = pl.ds(pl.multiple_of(i * HB, HB), HB)
        h2 = _bf(hn[rows2, :])
        g = jax.nn.gelu(_dot(h2, _bf(w1[...])) + rep(biasb[:, pl.ds(0, FF)], FB), approximate=True).astype(BF16)
        nxt = lax.rem(i + 1, nb) * FB
        dep = None
        for n in range(8):
            cols = pl.ds(n * 128, 128)
            for z in range(2):
                dep = ln2_piece(nxt + (2 * n + z) * 16, dep)
                y = _dot(g[z * HB:(z + 1) * HB], _bf(w2[:, cols])) + rep(biasb[:, pl.ds(FF + n * 128, 128)], HB)
                xr = pl.ds(pl.multiple_of(i * HB + z * (HB // 2), HB // 2), HB // 2)
                ar = pl.ds(pl.multiple_of(i * FB + z * HB, HB), HB)
                x2 = _bf(xs[xr, cols]).astype(F32) + rep(modb[0, :, cols], HB) * ha[ar, cols]
                xs[xr, cols] = pltpu.bitcast((x2 + rep(modb[3, :, cols], HB) * y).astype(BF16), U32)
        pltpu.make_async_copy(xs.at[rows2], out32.at[rows2], sem.at[SEM_OUT]).start()
        return carry

    with jax.named_scope("p4_ffn"):
        lax.fori_loop(0, nb, ffn, 0)
    pltpu.make_async_copy(xs, out32, sem.at[SEM_OUT]).wait()


@jax.jit
def pallas_adaLN_cond__memory_aug_recurrent_mem_tr__dense_activation_gelu__prompt_kernel(
    A_x, A_mem0, A_Wq, A_Wk, A_Wv, A_Wo, A_seg_len, B_x, B_w1, B_b1, B_w2, B_b2, c, w_mod,
):
    assert A_x.shape == (1, S, D) and A_Wq.shape == (D, H, E) and A_mem0.shape == (1, M, D)
    any_spec = pl.BlockSpec(memory_space=pl.ANY)
    out = pl.pallas_call(
        _kernel,
        out_shape=jax.ShapeDtypeStruct((S, D), BF16),
        in_specs=[any_spec] * 12,
        out_specs=any_spec,
        scratch_shapes=[
            pltpu.VMEM((S // 2, D), U32),
            pltpu.VMEM((96, D // 2, E), U32),
            pltpu.VMEM((8, H * E // 2, 128), U32),
            pltpu.VMEM((D // 2, FF), U32),
            pltpu.VMEM((FF // 2, D), U32),
            pltpu.VMEM((NQ, 2, D // 2, KQ), U32),
            pltpu.VMEM((8, D // 2, 512), U32),
            pltpu.VMEM((H, RING, E), F32),
            pltpu.VMEM((H, RING, E), F32),
            pltpu.VMEM((H + 1, RING, E), F32),
            pltpu.VMEM((H, RING, E), F32),
            pltpu.VMEM((S, D), F32),
            pltpu.VMEM((S - PRE, D), F32),
            pltpu.VMEM((8, PRE // 2, 128), U32),
            pltpu.VMEM((M, D), F32),
            pltpu.VMEM((NQ, 2, 8, KQ), F32),
            pltpu.VMEM((4, 8, D), F32),
            pltpu.VMEM((8, D), U32),
            pltpu.VMEM((8, FF + D), F32),
            pltpu.VMEM((80, 128), F32),
            pltpu.VMEM((8, 32, 128), F32),
            pltpu.VMEM((8, 128), U32),
            pltpu.VMEM((D // 2, 128), U32),
            pltpu.SMEM((1,), jnp.int32),
            pltpu.VMEM((M, D), BF16),
            pltpu.VMEM((FF,), BF16),
            pltpu.VMEM((D,), BF16),
            pltpu.VMEM((1, D), BF16),
            pltpu.SemaphoreType.DMA((NSEM,)),
        ],
        compiler_params=pltpu.CompilerParams(vmem_limit_bytes=127 * 1024 * 1024),
    )(
        A_x.reshape(S, D), A_mem0.reshape(M, D),
        A_Wq.reshape(D // 2, 2, H, E), A_Wk.reshape(D // 2, 2, H, E), A_Wv.reshape(D // 2, 2, H, E),
        A_Wo.reshape(H * E, D), B_w1, B_b1, B_w2, B_b2, c, w_mod,
    )
    return out.reshape(1, S, D)
```

```python
import math

import jax
import jax.numpy as jnp
from jax import lax
import jax.experimental.pallas as pl
import jax.experimental.pallas.tpu as pltpu

F32 = jnp.float32
BF16 = jnp.bfloat16
U32 = jnp.uint32

S = 2048
D = 1024
H = 32
E = 128
M = 8
SEG = 32
NSEG = S // SEG
FF = 3584
NP = H // 2
TOK = 24
PRE = S - NSEG * TOK
RING = 576
OOFF = (-NSEG * TOK) % RING
LN_EPS = 1e-5
FB = 256
XC = (S - PRE) // 6
UNROLL = 4

NQ = 4
KQ = D // NQ

FIRST_STARTS = [('m', 0), ('w', 0, 0, 2), ('w', 0, 2, 6), ('w', 0, 6, 12), ('m', 1), ('w', 1, 0, 6),
                ('w', 1, 6, 12), ('m', 2)]
P1A_BLOCKS = [
    ([], [('m', 0)]),
    ([], [('w', 0, 0, 2)]),
    ([], [('w', 0, 2, 6)]),
    ([('w', 2, 0, 6), ('w', 2, 6, 12)], [('w', 0, 6, 12)]),
    ([('m', 3), ('w', 3, 0, 6), ('w', 3, 6, 12)], [('m', 1), ('w', 1, 0, 6)]),
    ([], [('m', 2), ('w', 1, 6, 12)]),
    ([('g', 2), ('g', 3)], [('w', 2, 0, 6), ('w', 2, 6, 12)]),
    ([('g', 4), ('g', 5)], [('m', 3), ('w', 3, 0, 6), ('w', 3, 6, 12)]),
]
W_ITEMS = [it for _, items in P1A_BLOCKS for it in items if it[0] == 'w']
NX0 = 4

SEM_C = 0
SEM_X0 = 1
SEM_MOD = SEM_X0 + NX0
SEM_WA = SEM_MOD + NQ + 1
SEM_WB = SEM_WA + len(W_ITEMS)
SEM_XC = SEM_WB + 6
SEM_WO = SEM_XC + 6
SEM_W1 = SEM_WO + 1
SEM_W2 = SEM_W1 + 1
SEM_OUT = SEM_W2 + 1
NSEM = SEM_OUT + 1


def _ln(x):
    m = jnp.mean(x, axis=-1, keepdims=True)
    xc = x - m
    v = jnp.mean(xc * xc, axis=-1, keepdims=True)
    return xc * lax.rsqrt(v + LN_EPS)


def _bf(w32):
    return pltpu.bitcast(w32, BF16)


def _dot(a, b):
    return jnp.dot(a, b, preferred_element_type=F32)


def _kernel(x_hbm, mem0_hbm, wq_hbm, wk_hbm, wv_hbm, wo_hbm, w1_hbm, b1_hbm, w2_hbm, b2_hbm,
            c_hbm, wmod_hbm, out_hbm,
            xs, wqkv, wo, w1, w2, wmoda, wmod, qka, qkb, vring, oring, ha, hn, hb, memb, moda, modb, scb, biasb,
            fillb, accb, zerob, colb, zero_s, mem0_ref, b1_ref, b2_ref, c_ref, sem):
    qkv_hbm = [r.bitcast(U32) for r in (wq_hbm, wk_hbm, wv_hbm)]
    x32 = x_hbm.bitcast(U32)
    wo32 = wo_hbm.bitcast(U32)
    wmod32 = wmod_hbm.bitcast(U32)

    def units_start(lo, hi, rows, sem_idx):
        for u in range(lo, hi):
            j, m = u // 3, u % 3
            for p in range(2):
                pltpu.make_async_copy(qkv_hbm[m].at[rows, p, j, :], wqkv.at[2 * u + p, rows, :],
                                      sem.at[sem_idx]).start()

    def units_wait(lo, n, rows, sem_idx):
        blk = wqkv.at[pl.ds(2 * lo, 2 * n), rows, :]
        pltpu.make_async_copy(blk, blk, sem.at[sem_idx]).wait()

    def item_start(item):
        if item[0] == 'm':
            qq = item[1]
            for k in range(2):
                pltpu.make_async_copy(wmod32.at[:, pl.ds(k * D + qq * KQ, KQ)], wmoda.at[qq, k],
                                      sem.at[SEM_MOD + qq]).start()
        elif item[0] == 'w':
            _, qq, lo, hi = item
            units_start(lo, hi, pl.ds(qq * (KQ // 2), KQ // 2), SEM_WA + W_ITEMS.index(item))
        else:
            whole_start(item[1])

    def item_wait(item):
        if item[0] == 'm':
            qq = item[1]
            pltpu.make_async_copy(wmoda.at[qq], wmoda.at[qq], sem.at[SEM_MOD + qq]).wait()
        else:
            _, qq, lo, hi = item
            units_wait(lo, hi - lo, pl.ds(qq * (KQ // 2), KQ // 2), SEM_WA + W_ITEMS.index(item))

    def whole_start(i):
        xc_copy(i - 2).start()
        units_start(6 * i, 6 * i + 6, pl.ds(0, D // 2), SEM_WB + i - 2)

    def mod_copy(g):
        return pltpu.make_async_copy(wmod32.at[:, pl.ds(2 * D + g * 512, 512)], wmod.at[g],
                                     sem.at[SEM_MOD + NQ])

    def x0_copy(i):
        n = PRE // 2 // NX0
        rows = pl.ds(pl.multiple_of(i * n, n), n)
        return pltpu.make_async_copy(x32.at[rows], xs.at[rows], sem.at[SEM_X0 + i])

    def xc_copy(i):
        rows = pl.ds(pl.multiple_of(PRE // 2 + i * (XC // 2), 64), XC // 2)
        return pltpu.make_async_copy(x32.at[rows], xs.at[rows], sem.at[SEM_XC + i])

    def wo_copy(n):
        return pltpu.make_async_copy(wo32.at[:, pl.ds(n * 128, 128)], wo.at[n], sem.at[SEM_WO])

    w1_copy = pltpu.make_async_copy(w1_hbm.bitcast(U32), w1, sem.at[SEM_W1])
    w2_copy = pltpu.make_async_copy(w2_hbm.bitcast(U32), w2, sem.at[SEM_W2])
    small_copies = [pltpu.make_async_copy(a, b, sem.at[SEM_C])
                    for a, b in ((c_hbm, c_ref), (mem0_hbm, mem0_ref), (b1_hbm, b1_ref),
                                 (b2_hbm, b2_ref))]

    def deinterleave(u, row0, nrows):
        for k in range(nrows // 64):
            rows = pl.ds(row0 + k * 64, 64)
            a = wqkv[2 * u, rows, :]
            b = wqkv[2 * u + 1, rows, :]
            wqkv[2 * u, rows, :] = (a & jnp.uint32(0xFFFF)) | (b << 16)
            wqkv[2 * u + 1, rows, :] = (a >> 16) | (b & jnp.uint32(0xFFFF0000))

    def load_x16(row2, dep):
        xw = xs[pl.ds(row2, 8), :]
        if dep is not None:
            first = xw[:, 0:128] | (dep & zerob[...])
            xw = jnp.concatenate([first, xw[:, 128:]], axis=1)
        return _bf(xw).astype(F32)

    def rep(v8, n):
        return jnp.concatenate([v8] * (n // 8), axis=0)

    def mrow(k, n):
        if k < 2:
            return rep(jnp.concatenate([moda[qq, k] for qq in range(NQ)], axis=1), n)
        return rep(modb[k - 2], n)

    for cp in small_copies:
        cp.start()
    for i in range(NX0):
        x0_copy(i).start()
    for item in FIRST_STARTS:
        item_start(item)

    def start_rest():
        for n in range(8):
            wo_copy(n).start()
        for g in range(8):
            mod_copy(g).start()
        w1_copy.start()
        w2_copy.start()

    r = lax.broadcasted_iota(jnp.int32, (80, 128), 0)
    q = lax.broadcasted_iota(jnp.int32, (80, 128), 1)
    r_tok = r < 64
    q_tok = q < 64
    r_head = jnp.where(r_tok, r >> 5, (r - 64) >> 3)
    q_head = jnp.where(q_tok, q >> 5, (q - 64) >> 3)
    same = (r_head == q_head) & (q < 80)
    causal_ok = jnp.logical_not(r_tok & q_tok & ((q & 31) > (r & 31)))
    scale = E ** (-0.5)
    fillb[...] = jnp.where(same, jnp.where(causal_ok, 0.0, -1e9 / scale), -jnp.inf).astype(F32)
    zerob[...] = jnp.zeros((8, 128), U32)
    zero_s[0] = 0

    pre_rows = pl.ds(RING - PRE, PRE)

    for cp in small_copies:
        cp.wait()
    cf = c_ref[...].astype(F32)
    sc = (cf * jax.nn.sigmoid(cf)).astype(BF16)
    scb[...] = pltpu.bitcast(jnp.broadcast_to(sc, (16, D)), U32)
    scf = jnp.broadcast_to(sc.astype(F32), (128, D))
    for k in range(8):
        colb[pl.ds(k * 64, 64), :] = pltpu.bitcast(scf[:, k * 128:(k + 1) * 128].T.astype(BF16), U32)
    memb[...] = mem0_ref[...].astype(F32)
    biasb[:, pl.ds(0, FF)] = jnp.broadcast_to(b1_ref[...].astype(F32).reshape(1, FF), (8, FF))
    biasb[:, pl.ds(FF, D)] = jnp.broadcast_to(b2_ref[...].astype(F32).reshape(1, D), (8, D))

    def pre_norm(i, carry):
        x0_copy(i).wait()
        nr = PRE // NX0
        for z in range(nr // 16):
            xn = _ln(load_x16(pl.multiple_of(i * (nr // 2) + z * 8, 8), None))
            for n in range(8):
                oring[n, pl.ds(pl.multiple_of(i * nr + z * 16, 16), 16), :] = xn[:, n * 128:(n + 1) * 128]
        return carry

    with jax.named_scope("p0_ln"):
        lax.fori_loop(0, NX0, pre_norm, 0)

    def dst_slot(i, k, p):
        cls, m = k // 3, k % 3
        if m == 2:
            return vring, 4 * i + 2 * cls + p
        return (qka, qkb)[cls], 4 * i + 2 * m + p

    NT = KQ // 128

    def item_run(item):
        if item[0] == 'm':
            qq = item[1]
            sc16 = _bf(scb[...])
            ca1 = 1.0 + _dot(sc16, _bf(wmoda[qq, 1]))[0:8].astype(BF16).astype(F32)
            sa = _dot(sc16, _bf(wmoda[qq, 0]))[0:8].astype(BF16).astype(F32)
            moda[qq, 0] = sa
            moda[qq, 1] = ca1
            for n in range(NT):
                cols = slice(n * 128, (n + 1) * 128)
                for z in range(PRE // 64):
                    hq = (oring[NT * qq + n, pl.ds(z * 64, 64), :] * rep(ca1[:, cols], 64)
                          + rep(sa[:, cols], 64))
                    hb[NT * qq + n, pl.ds(z * 32, 32), :] = pltpu.bitcast(hq.astype(BF16), U32)
            return
        _, qq, lo, hi = item
        row0 = qq * (KQ // 2)
        for u in range(lo, hi):
            i, k = u // 6, u % 6
            deinterleave(u, row0, KQ // 2)
            for p in range(2):
                lhs = _bf(jnp.concatenate([hb[NT * qq + n] for n in range(NT)], axis=1))
                ref, idx = dst_slot(i, k, p)
                y = _dot(lhs, _bf(wqkv[2 * u + p, pl.ds(row0, KQ // 2), :]))
                if qq > 0:
                    y = y + ref[idx, pre_rows, :]
                ref[idx, pre_rows, :] = y

    def phase1b(i, carry):
        @pl.when(i == 3)
        def _():
            whole_start(6)
            whole_start(7)

        @pl.when(i == 4)
        def _():
            start_rest()

        xc_copy(i - 2).wait()
        units_wait(6 * i, 6, pl.ds(0, D // 2), SEM_WB + i - 2)
        deinterleave(6 * i, 0, D // 2)
        dep = None
        for k in range(6):
            u = 6 * i + k
            for p in range(2):
                lhs = _bf(jnp.concatenate([hb[n] for n in range(8)], axis=1))
                ref, idx = dst_slot(i, k, p)
                ref[idx, pre_rows, :] = _dot(lhs, _bf(wqkv[2 * u + p]))
                if p == 0 and k < 5:
                    deinterleave(u + 1, 0, D // 2)
                if k >= 2:
                    for z in range(2):
                        r0 = (i - 2) * XC + (4 * k + 2 * p + z - 8) * 16
                        x16 = load_x16(pl.multiple_of(PRE // 2 + r0 // 2, 8), dep)
                        h16 = _ln(x16) * mrow(1, 16) + mrow(0, 16)
                        hn[pl.ds(pl.multiple_of(r0, 16), 16), :] = h16
                        dep = pltpu.bitcast(h16[8:16, D - 128:], U32)
        return carry

    for bi, (starts, items) in enumerate(P1A_BLOCKS):
        for item in starts:
            item_start(item)
        with jax.named_scope("p1a_wait%d" % bi):
            for item in items:
                item_wait(item)
        for item in items:
            item_run(item)
    with jax.named_scope("p1b"):
        lax.fori_loop(2, 8, phase1b, 0)
    for n in range(8):
        wo_copy(n).wait()

    cexp = scale * math.log2(math.e)
    NG = NP // 2
    grp = [(4 * (g // 2) + (g % 2), 4 * (g // 2) + (g % 2) + 2) for g in range(NG)]
    early = [2 * j + u for g in range(NG - 3) for j in grp[g] for u in range(2)]
    late = [h for h in range(H) if h not in early]

    def step(s, split):
        w0 = pl.multiple_of(lax.rem(TOK * s, RING), 8)
        r0 = pl.multiple_of(lax.rem(SEG * s + (RING - PRE), RING), 32)
        ow = pl.multiple_of(lax.rem(SEG * s + OOFF, RING), 32)
        o0 = pl.multiple_of(lax.rem(TOK * s + OOFF, RING), 8)
        a0 = pl.multiple_of(TOK * s, 8)
        X = jnp.concatenate([hn[pl.ds(a0, TOK), :], memb[...]], axis=0).astype(BF16)
        ym = [None] * 96
        probs = [None] * NP
        om = [None] * H
        order = (4, 5, 0, 1, 2, 3)

        if split:
            for t in order:
                accb[t] = _dot(X[:, :D // 2], _bf(wqkv[t, pl.ds(0, D // 4), :]))

        def slot(j, t):
            if t >= 4:
                return vring, 2 * j + t - 4
            return (qka, qkb)[j % 2], 4 * (j // 2) + t

        def proj(j, t):
            c = 6 * j + t
            if split and j == 0:
                y = accb[t] + _dot(X[:, D // 2:], _bf(wqkv[c, pl.ds(D // 4, D // 4), :]))
            else:
                y = _dot(X, _bf(wqkv[c]))
            ref, k = slot(j, t)
            ref[k, pl.ds(w0, TOK), :] = y[0:TOK]
            ym[c] = y[TOK:TOK + M]

        def gather(j, m, pad):
            c = 6 * j + 2 * m
            ref, k = slot(j, 2 * m)
            parts = [ref[k, pl.ds(r0, SEG), :], ref[k + 1, pl.ds(r0, SEG), :], ym[c], ym[c + 1]]
            if pad:
                parts.append(jnp.zeros((48, E), F32))
            return jnp.concatenate(parts, axis=0).astype(BF16)

        def scores(j):
            sc_ = lax.dot_general(gather(j, 0, False), gather(j, 1, True),
                                  (((1,), (1,)), ((), ())), preferred_element_type=F32)
            fill = fillb[...]
            sc_ = jnp.where(fill == 0.0, sc_, fill)
            mx = jnp.max(sc_, axis=-1, keepdims=True)
            p = jnp.exp2((sc_ - mx) * cexp)
            l = jnp.sum(p, axis=-1, keepdims=True)
            rl = pl.reciprocal(l, approx=True)
            rl = rl * (2.0 - l * rl)
            probs[j] = (p * rl).astype(BF16)

        def park(j):
            vring[H, pl.ds(40 * (j % 8), 40), :] = pltpu.bitcast(probs[j], F32)
            probs[j] = None

        def pv(j):
            P = probs[j]
            if P is None:
                P = _bf(vring[H, pl.ds(40 * (j % 8), 40), :])
            o = _dot(P, gather(j, 2, True))
            oring[2 * j, pl.ds(ow, SEG), :] = o[0:32]
            oring[2 * j + 1, pl.ds(ow, SEG), :] = o[32:64]
            om[2 * j] = o[64:72]
            om[2 * j + 1] = o[72:80]

        def o_lhs(hs):
            return jnp.concatenate(
                [jnp.concatenate([oring[h, pl.ds(o0, TOK), :], om[h]], axis=0) for h in hs],
                axis=1).astype(BF16)

        def o_rhs(n, hs):
            return _bf(jnp.concatenate([wo[n, pl.ds(h * 64, 64), :] for h in hs], axis=0))

        for g in range(NG):
            cols = [(j, t) for j in grp[g] for t in order]
            if g == 2:
                cols = ([(j, t) for j in grp[g] for t in (4, 5)]
                        + [(j, t) for j in grp[g] for t in range(4)])
            for j in (grp[0] + grp[1] if g == 3 else grp[g - 2] if g >= 4 else ()):
                park(j)
            for ci, (j, t) in enumerate(cols):
                if g == 2 and ci == 4:
                    for jj in grp[0] + grp[1]:
                        scores(jj)
                if g >= 3 and ci == 6:
                    for jj in grp[g - 1]:
                        scores(jj)
                    for jj in grp[g - 3]:
                        pv(jj)
                proj(j, t)
        lo = o_lhs(early)
        for n in range(8):
            accb[n] = _dot(lo, o_rhs(n, early))
            if n == 1:
                for jj in grp[NG - 1]:
                    scores(jj)
                for jj in grp[NG - 3]:
                    pv(jj)
            if n == 4:
                for jj in grp[NG - 2] + grp[NG - 1]:
                    pv(jj)
        lo = o_lhs(late)
        for n in range(8):
            a = accb[n] + _dot(lo, o_rhs(n, late))
            ha[pl.ds(a0, TOK), pl.ds(n * 128, 128)] = a[0:TOK]
            memb[:, pl.ds(n * 128, 128)] = a[TOK:TOK + M]

    def steps(i, carry):
        for k in range(UNROLL):
            step(i * UNROLL + k, k > 0)
        return carry

    with jax.named_scope("p2_steps"):
        lax.fori_loop(0, NSEG // UNROLL, steps, 0)

    for g in range(8):
        mod_copy(g).wait()

    def lo16(w):
        return pltpu.bitcast(w << 16, F32)

    def hi16(w):
        return pltpu.bitcast(w & jnp.uint32(0xFFFF0000), F32)

    def mod_vpu(g, dep):
        for t in range(4):
            acc = None if dep is None else pltpu.bitcast(dep & zerob[...], F32)
            for k in range(D // 16):
                cw = colb[pl.ds(k * 8, 8), :]
                w = wmod[g, pl.ds(k * 8, 8), pl.ds(t * 128, 128)]
                pe = lo16(w) * lo16(cw)
                acc = pe if acc is None else acc + pe
                acc = acc + hi16(w) * hi16(cw)
            dep = pltpu.bitcast(acc, U32)
            y = jnp.sum(acc, axis=0, keepdims=True).astype(BF16).astype(F32)
            if g // 2 == 2:
                y = 1.0 + y
            modb[g // 2, :, pl.ds((g % 2) * 512 + t * 128, 128)] = jnp.broadcast_to(y, (8, 128))
        return dep

    def ln2_piece(r0, dep):
        r2 = pl.multiple_of(r0 // 2, 8)
        x2 = load_x16(r2, dep) + mrow(2, 16) * ha[pl.ds(pl.multiple_of(r0, 16), 16), :]
        h2 = pltpu.bitcast((_ln(x2) * mrow(4, 16) + mrow(3, 16)).astype(BF16), F32)
        hn[pl.ds(r2, 8), :] = h2
        return pltpu.bitcast(h2[:, D - 128:], U32)

    def bulk_o(one, carry):
        dep = None
        for i in range(2):
            lo = jnp.concatenate([oring[h, pl.ds(i * 256, 256), :] for h in range(H)], axis=1).astype(BF16)
            for n in range(8):
                if i == 0:
                    dep = mod_vpu(n, dep)
                else:
                    for z in range(2):
                        dep = ln2_piece(one * FB + (2 * n + z) * 16, dep)
                ha[pl.ds(NSEG * TOK + i * 256, 256), pl.ds(n * 128, 128)] = _dot(lo, _bf(wo[n]))
        return carry

    with jax.named_scope("p3_bulk_o"):
        bulk_o(zero_s[0], 0)

    w1_copy.wait()
    w2_copy.wait()

    nb = S // FB

    out32 = out_hbm.bitcast(U32)
    HB = FB // 2

    def ffn(i, carry):
        rows2 = pl.ds(pl.multiple_of(i * HB, HB), HB)
        h2 = _bf(hn[rows2, :])
        g = jax.nn.gelu(_dot(h2, _bf(w1[...])) + rep(biasb[:, pl.ds(0, FF)], FB), approximate=True).astype(BF16)
        nxt = lax.rem(i + 1, nb) * FB
        dep = None
        for n in range(8):
            cols = pl.ds(n * 128, 128)
            for z in range(2):
                dep = ln2_piece(nxt + (2 * n + z) * 16, dep)
                y = _dot(g[z * HB:(z + 1) * HB], _bf(w2[:, cols])) + rep(biasb[:, pl.ds(FF + n * 128, 128)], HB)
                xr = pl.ds(pl.multiple_of(i * HB + z * (HB // 2), HB // 2), HB // 2)
                ar = pl.ds(pl.multiple_of(i * FB + z * HB, HB), HB)
                x2 = _bf(xs[xr, cols]).astype(F32) + rep(modb[0, :, cols], HB) * ha[ar, cols]
                xs[xr, cols] = pltpu.bitcast((x2 + rep(modb[3, :, cols], HB) * y).astype(BF16), U32)
        pltpu.make_async_copy(xs.at[rows2], out32.at[rows2], sem.at[SEM_OUT]).start()
        return carry

    with jax.named_scope("p4_ffn"):
        lax.fori_loop(0, nb, ffn, 0)
    pltpu.make_async_copy(xs, out32, sem.at[SEM_OUT]).wait()


@jax.jit
def pallas_adaLN_cond__memory_aug_recurrent_mem_tr__dense_activation_gelu__prompt_kernel(
    A_x, A_mem0, A_Wq, A_Wk, A_Wv, A_Wo, A_seg_len, B_x, B_w1, B_b1, B_w2, B_b2, c, w_mod,
):
    assert A_x.shape == (1, S, D) and A_Wq.shape == (D, H, E) and A_mem0.shape == (1, M, D)
    any_spec = pl.BlockSpec(memory_space=pl.ANY)
    out = pl.pallas_call(
        _kernel,
        out_shape=jax.ShapeDtypeStruct((S, D), BF16),
        in_specs=[any_spec] * 12,
        out_specs=any_spec,
        scratch_shapes=[
            pltpu.VMEM((S // 2, D), U32),
            pltpu.VMEM((96, D // 2, E), U32),
            pltpu.VMEM((8, H * E // 2, 128), U32),
            pltpu.VMEM((D // 2, FF), U32),
            pltpu.VMEM((FF // 2, D), U32),
            pltpu.VMEM((NQ, 2, D // 2, KQ), U32),
            pltpu.VMEM((8, D // 2, 512), U32),
            pltpu.VMEM((H, RING, E), F32),
            pltpu.VMEM((H, RING, E), F32),
            pltpu.VMEM((H + 1, RING, E), F32),
            pltpu.VMEM((H, RING, E), F32),
            pltpu.VMEM((S, D), F32),
            pltpu.VMEM((S - PRE, D), F32),
            pltpu.VMEM((8, PRE // 2, 128), U32),
            pltpu.VMEM((M, D), F32),
            pltpu.VMEM((NQ, 2, 8, KQ), F32),
            pltpu.VMEM((4, 8, D), F32),
            pltpu.VMEM((8, D), U32),
            pltpu.VMEM((8, FF + D), F32),
            pltpu.VMEM((80, 128), F32),
            pltpu.VMEM((8, 32, 128), F32),
            pltpu.VMEM((8, 128), U32),
            pltpu.VMEM((D // 2, 128), U32),
            pltpu.SMEM((1,), jnp.int32),
            pltpu.VMEM((M, D), BF16),
            pltpu.VMEM((FF,), BF16),
            pltpu.VMEM((D,), BF16),
            pltpu.VMEM((1, D), BF16),
            pltpu.SemaphoreType.DMA((NSEM,)),
        ],
        compiler_params=pltpu.CompilerParams(vmem_limit_bytes=127 * 1024 * 1024),
    )(
        A_x.reshape(S, D), A_mem0.reshape(M, D),
        A_Wq.reshape(D // 2, 2, H, E), A_Wk.reshape(D // 2, 2, H, E), A_Wv.reshape(D // 2, 2, H, E),
        A_Wo.reshape(H * E, D), B_w1, B_b1, B_w2, B_b2, c, w_mod,
    )
    return out.reshape(1, S, D)
```

```python
import math

import jax
import jax.numpy as jnp
from jax import lax
import jax.experimental.pallas as pl
import jax.experimental.pallas.tpu as pltpu

F32 = jnp.float32
BF16 = jnp.bfloat16
U32 = jnp.uint32

S = 2048
D = 1024
H = 32
E = 128
M = 8
SEG = 32
NSEG = S // SEG
FF = 3584
NP = H // 2
TOK = 24
PRE = S - NSEG * TOK
RING = 576
OOFF = (-NSEG * TOK) % RING
LN_EPS = 1e-5
FB = 256
XC = (S - PRE) // 6
UNROLL = 4

NQ = 4
KQ = D // NQ

FIRST_STARTS = [('m', 0), ('w', 0, 0, 2), ('w', 0, 2, 6), ('w', 0, 6, 12), ('m', 1), ('w', 1, 0, 6),
                ('w', 1, 6, 12), ('m', 2)]
P1A_BLOCKS = [
    ([], [('m', 0)]),
    ([], [('w', 0, 0, 2)]),
    ([], [('w', 0, 2, 6)]),
    ([('w', 2, 0, 6), ('w', 2, 6, 12)], [('w', 0, 6, 12)]),
    ([('m', 3), ('w', 3, 0, 6), ('w', 3, 6, 12)], [('m', 1), ('w', 1, 0, 6)]),
    ([], [('m', 2), ('w', 1, 6, 12)]),
    ([('g', 2), ('g', 3)], [('w', 2, 0, 6), ('w', 2, 6, 12)]),
    ([('g', 4), ('g', 5)], [('m', 3), ('w', 3, 0, 6), ('w', 3, 6, 12)]),
]
W_ITEMS = [it for _, items in P1A_BLOCKS for it in items if it[0] == 'w']
NX0 = 4

SEM_C = 0
SEM_X0 = 1
SEM_MOD = SEM_X0 + NX0
SEM_WA = SEM_MOD + NQ + 1
SEM_WB = SEM_WA + len(W_ITEMS)
SEM_XC = SEM_WB + 6
SEM_WO = SEM_XC + 6
SEM_W1 = SEM_WO + 1
SEM_W2 = SEM_W1 + 1
SEM_OUT = SEM_W2 + 1
NSEM = SEM_OUT + 1


def _ln(x):
    m = jnp.mean(x, axis=-1, keepdims=True)
    xc = x - m
    v = jnp.mean(xc * xc, axis=-1, keepdims=True)
    return xc * lax.rsqrt(v + LN_EPS)


def _bf(w32):
    return pltpu.bitcast(w32, BF16)


def _dot(a, b):
    return jnp.dot(a, b, preferred_element_type=F32)


def _kernel(x_hbm, mem0_hbm, wq_hbm, wk_hbm, wv_hbm, wo_hbm, w1_hbm, b1_hbm, w2_hbm, b2_hbm,
            c_hbm, wmod_hbm, out_hbm,
            xs, wqkv, wo, w1, w2, wmoda, wmod, qka, qkb, vring, oring, ha, hn, hb, memb, moda, modb, scb, biasb,
            fillb, accb, zerob, colb, zero_s, mem0_ref, b1_ref, b2_ref, c_ref, sem):
    qkv_hbm = [r.bitcast(U32) for r in (wq_hbm, wk_hbm, wv_hbm)]
    x32 = x_hbm.bitcast(U32)
    wo32 = wo_hbm.bitcast(U32)
    wmod32 = wmod_hbm.bitcast(U32)

    def units_start(lo, hi, rows, sem_idx):
        for u in range(lo, hi):
            j, m = u // 3, u % 3
            for p in range(2):
                pltpu.make_async_copy(qkv_hbm[m].at[rows, p, j, :], wqkv.at[2 * u + p, rows, :],
                                      sem.at[sem_idx]).start()

    def units_wait(lo, n, rows, sem_idx):
        blk = wqkv.at[pl.ds(2 * lo, 2 * n), rows, :]
        pltpu.make_async_copy(blk, blk, sem.at[sem_idx]).wait()

    def item_start(item):
        if item[0] == 'm':
            qq = item[1]
            for k in range(2):
                pltpu.make_async_copy(wmod32.at[:, pl.ds(k * D + qq * KQ, KQ)], wmoda.at[qq, k],
                                      sem.at[SEM_MOD + qq]).start()
        elif item[0] == 'w':
            _, qq, lo, hi = item
            units_start(lo, hi, pl.ds(qq * (KQ // 2), KQ // 2), SEM_WA + W_ITEMS.index(item))
        else:
            whole_start(item[1])

    def item_wait(item):
        if item[0] == 'm':
            qq = item[1]
            pltpu.make_async_copy(wmoda.at[qq], wmoda.at[qq], sem.at[SEM_MOD + qq]).wait()
        else:
            _, qq, lo, hi = item
            units_wait(lo, hi - lo, pl.ds(qq * (KQ // 2), KQ // 2), SEM_WA + W_ITEMS.index(item))

    def whole_start(i):
        xc_copy(i - 2).start()
        units_start(6 * i, 6 * i + 6, pl.ds(0, D // 2), SEM_WB + i - 2)

    def mod_copy(g):
        return pltpu.make_async_copy(wmod32.at[:, pl.ds(2 * D + g * 512, 512)], wmod.at[g],
                                     sem.at[SEM_MOD + NQ])

    def x0_copy(i):
        n = PRE // 2 // NX0
        rows = pl.ds(pl.multiple_of(i * n, n), n)
        return pltpu.make_async_copy(x32.at[rows], xs.at[rows], sem.at[SEM_X0 + i])

    def xc_copy(i):
        rows = pl.ds(pl.multiple_of(PRE // 2 + i * (XC // 2), 64), XC // 2)
        return pltpu.make_async_copy(x32.at[rows], xs.at[rows], sem.at[SEM_XC + i])

    def wo_copy(n):
        return pltpu.make_async_copy(wo32.at[:, pl.ds(n * 128, 128)], wo.at[n], sem.at[SEM_WO])

    w1_copy = pltpu.make_async_copy(w1_hbm.bitcast(U32), w1, sem.at[SEM_W1])
    w2_copy = pltpu.make_async_copy(w2_hbm.bitcast(U32), w2, sem.at[SEM_W2])
    small_copies = [pltpu.make_async_copy(a, b, sem.at[SEM_C])
                    for a, b in ((c_hbm, c_ref), (mem0_hbm, mem0_ref), (b1_hbm, b1_ref),
                                 (b2_hbm, b2_ref))]

    def deinterleave(u, row0, nrows):
        for k in range(nrows // 64):
            rows = pl.ds(row0 + k * 64, 64)
            a = wqkv[2 * u, rows, :]
            b = wqkv[2 * u + 1, rows, :]
            wqkv[2 * u, rows, :] = (a & jnp.uint32(0xFFFF)) | (b << 16)
            wqkv[2 * u + 1, rows, :] = (a >> 16) | (b & jnp.uint32(0xFFFF0000))

    def load_x16(row2, dep):
        xw = xs[pl.ds(row2, 8), :]
        if dep is not None:
            first = xw[:, 0:128] | (dep & zerob[...])
            xw = jnp.concatenate([first, xw[:, 128:]], axis=1)
        return _bf(xw).astype(F32)

    def rep(v8, n):
        return jnp.concatenate([v8] * (n // 8), axis=0)

    def mrow(k, n):
        if k < 2:
            return rep(jnp.concatenate([moda[qq, k] for qq in range(NQ)], axis=1), n)
        return rep(modb[k - 2], n)

    for cp in small_copies:
        cp.start()
    for i in range(NX0):
        x0_copy(i).start()
    for item in FIRST_STARTS:
        item_start(item)

    def start_rest():
        for n in range(8):
            wo_copy(n).start()
        for g in range(8):
            mod_copy(g).start()
        w1_copy.start()
        w2_copy.start()

    r = lax.broadcasted_iota(jnp.int32, (80, 128), 0)
    q = lax.broadcasted_iota(jnp.int32, (80, 128), 1)
    r_tok = r < 64
    q_tok = q < 64
    r_head = jnp.where(r_tok, r >> 5, (r - 64) >> 3)
    q_head = jnp.where(q_tok, q >> 5, (q - 64) >> 3)
    same = (r_head == q_head) & (q < 80)
    causal_ok = jnp.logical_not(r_tok & q_tok & ((q & 31) > (r & 31)))
    scale = E ** (-0.5)
    fillb[...] = jnp.where(same, jnp.where(causal_ok, 0.0, -1e9 / scale), -jnp.inf).astype(F32)
    zerob[...] = jnp.zeros((8, 128), U32)
    zero_s[0] = 0

    pre_rows = pl.ds(RING - PRE, PRE)

    for cp in small_copies:
        cp.wait()
    cf = c_ref[...].astype(F32)
    sc = (cf * jax.nn.sigmoid(cf)).astype(BF16)
    scb[...] = pltpu.bitcast(jnp.broadcast_to(sc, (16, D)), U32)
    scf = jnp.broadcast_to(sc.astype(F32), (128, D))
    for k in range(8):
        colb[pl.ds(k * 64, 64), :] = pltpu.bitcast(scf[:, k * 128:(k + 1) * 128].T.astype(BF16), U32)
    memb[...] = mem0_ref[...].astype(F32)
    biasb[:, pl.ds(0, FF)] = jnp.broadcast_to(b1_ref[...].astype(F32).reshape(1, FF), (8, FF))
    biasb[:, pl.ds(FF, D)] = jnp.broadcast_to(b2_ref[...].astype(F32).reshape(1, D), (8, D))

    def pre_norm(i, carry):
        x0_copy(i).wait()
        nr = PRE // NX0
        for z in range(nr // 16):
            xn = _ln(load_x16(pl.multiple_of(i * (nr // 2) + z * 8, 8), None))
            for n in range(8):
                oring[n, pl.ds(pl.multiple_of(i * nr + z * 16, 16), 16), :] = xn[:, n * 128:(n + 1) * 128]
        return carry

    with jax.named_scope("p0_ln"):
        lax.fori_loop(0, NX0, pre_norm, 0)

    def dst_slot(i, k, p):
        cls, m = k // 3, k % 3
        if m == 2:
            return vring, 4 * i + 2 * cls + p
        return (qka, qkb)[cls], 4 * i + 2 * m + p

    NT = KQ // 128

    def item_run(item):
        if item[0] == 'm':
            qq = item[1]
            sc16 = _bf(scb[...])
            ca1 = 1.0 + _dot(sc16, _bf(wmoda[qq, 1]))[0:8].astype(BF16).astype(F32)
            sa = _dot(sc16, _bf(wmoda[qq, 0]))[0:8].astype(BF16).astype(F32)
            moda[qq, 0] = sa
            moda[qq, 1] = ca1
            for n in range(NT):
                cols = slice(n * 128, (n + 1) * 128)
                for z in range(PRE // 64):
                    hq = (oring[NT * qq + n, pl.ds(z * 64, 64), :] * rep(ca1[:, cols], 64)
                          + rep(sa[:, cols], 64))
                    hb[NT * qq + n, pl.ds(z * 32, 32), :] = pltpu.bitcast(hq.astype(BF16), U32)
            return
        _, qq, lo, hi = item
        row0 = qq * (KQ // 2)
        for u in range(lo, hi):
            i, k = u // 6, u % 6
            deinterleave(u, row0, KQ // 2)
            for p in range(2):
                lhs = _bf(jnp.concatenate([hb[NT * qq + n] for n in range(NT)], axis=1))
                ref, idx = dst_slot(i, k, p)
                y = _dot(lhs, _bf(wqkv[2 * u + p, pl.ds(row0, KQ // 2), :]))
                if qq > 0:
                    y = y + ref[idx, pre_rows, :]
                ref[idx, pre_rows, :] = y

    def phase1b(i, carry):
        @pl.when(i == 3)
        def _():
            whole_start(6)
            whole_start(7)

        @pl.when(i == 4)
        def _():
            start_rest()

        xc_copy(i - 2).wait()
        units_wait(6 * i, 6, pl.ds(0, D // 2), SEM_WB + i - 2)
        deinterleave(6 * i, 0, D // 2)
        dep = None
        for k in range(6):
            u = 6 * i + k
            for p in range(2):
                lhs = _bf(jnp.concatenate([hb[n] for n in range(8)], axis=1))
                ref, idx = dst_slot(i, k, p)
                ref[idx, pre_rows, :] = _dot(lhs, _bf(wqkv[2 * u + p]))
                if p == 0 and k < 5:
                    deinterleave(u + 1, 0, D // 2)
                if k >= 2:
                    for z in range(2):
                        r0 = (i - 2) * XC + (4 * k + 2 * p + z - 8) * 16
                        x16 = load_x16(pl.multiple_of(PRE // 2 + r0 // 2, 8), dep)
                        h16 = _ln(x16) * mrow(1, 16) + mrow(0, 16)
                        hn[pl.ds(pl.multiple_of(r0, 16), 16), :] = h16
                        dep = pltpu.bitcast(h16[8:16, D - 128:], U32)
        return carry

    for bi, (starts, items) in enumerate(P1A_BLOCKS):
        for item in starts:
            item_start(item)
        with jax.named_scope("p1a_wait%d" % bi):
            for item in items:
                item_wait(item)
        for item in items:
            item_run(item)
    with jax.named_scope("p1b"):
        lax.fori_loop(2, 8, phase1b, 0)
    for n in range(8):
        wo_copy(n).wait()

    cexp = scale * math.log2(math.e)
    NG = NP // 2
    grp = [(4 * (g // 2) + (g % 2), 4 * (g // 2) + (g % 2) + 2) for g in range(NG)]
    early = [2 * j + u for g in range(NG - 3) for j in grp[g] for u in range(2)]
    late = [h for h in range(H) if h not in early]

    def step(it, k):
        s = it * UNROLL + k
        split = k > 0
        base = TOK * UNROLL * it
        w0 = pl.multiple_of(lax.rem(base, RING), 32) + TOK * k
        r0 = pl.multiple_of(lax.rem(SEG * s + (RING - PRE), RING), 32)
        ow = pl.multiple_of(lax.rem(SEG * s + OOFF, RING), 32)
        o0 = pl.multiple_of(lax.rem(base + OOFF, RING), 32) + TOK * k
        a0 = pl.multiple_of(base, 32) + TOK * k
        X = jnp.concatenate([hn[pl.ds(a0, TOK), :], memb[...]], axis=0).astype(BF16)
        ym = [None] * 96
        probs = [None] * NP
        om = [None] * H
        order = (4, 5, 0, 1, 2, 3)

        if split:
            for t in order:
                accb[t] = _dot(X[:, :D // 2], _bf(wqkv[t, pl.ds(0, D // 4), :]))

        def slot(j, t):
            if t >= 4:
                return vring, 2 * j + t - 4
            return (qka, qkb)[j % 2], 4 * (j // 2) + t

        def proj(j, t):
            c = 6 * j + t
            if split and j == 0:
                y = accb[t] + _dot(X[:, D // 2:], _bf(wqkv[c, pl.ds(D // 4, D // 4), :]))
            else:
                y = _dot(X, _bf(wqkv[c]))
            ref, k = slot(j, t)
            ref[k, pl.ds(w0, TOK), :] = y[0:TOK]
            ym[c] = y[TOK:TOK + M]

        def gather(j, m, pad):
            c = 6 * j + 2 * m
            ref, k = slot(j, 2 * m)
            parts = [ref[k, pl.ds(r0, SEG), :], ref[k + 1, pl.ds(r0, SEG), :], ym[c], ym[c + 1]]
            if pad:
                parts.append(jnp.zeros((48, E), F32))
            return jnp.concatenate(parts, axis=0).astype(BF16)

        def scores(j):
            sc_ = lax.dot_general(gather(j, 0, False), gather(j, 1, True),
                                  (((1,), (1,)), ((), ())), preferred_element_type=F32)
            fill = fillb[...]
            sc_ = jnp.where(fill == 0.0, sc_, fill)
            mx = jnp.max(sc_, axis=-1, keepdims=True)
            p = jnp.exp2((sc_ - mx) * cexp)
            l = jnp.sum(p, axis=-1, keepdims=True)
            rl = pl.reciprocal(l, approx=True)
            rl = rl * (2.0 - l * rl)
            probs[j] = (p * rl).astype(BF16)

        def park(j):
            vring[H, pl.ds(40 * (j % 8), 40), :] = pltpu.bitcast(probs[j], F32)
            probs[j] = None

        def pv(j):
            P = probs[j]
            if P is None:
                P = _bf(vring[H, pl.ds(40 * (j % 8), 40), :])
            o = _dot(P, gather(j, 2, True))
            oring[2 * j, pl.ds(ow, SEG), :] = o[0:32]
            oring[2 * j + 1, pl.ds(ow, SEG), :] = o[32:64]
            om[2 * j] = o[64:72]
            om[2 * j + 1] = o[72:80]

        def o_lhs(hs):
            return jnp.concatenate(
                [jnp.concatenate([oring[h, pl.ds(o0, TOK), :], om[h]], axis=0) for h in hs],
                axis=1).astype(BF16)

        def o_rhs(n, hs):
            return _bf(jnp.concatenate([wo[n, pl.ds(h * 64, 64), :] for h in hs], axis=0))

        for g in range(NG):
            cols = [(j, t) for j in grp[g] for t in order]
            if g == 2:
                cols = ([(j, t) for j in grp[g] for t in (4, 5)]
                        + [(j, t) for j in grp[g] for t in range(4)])
            for j in (grp[0] + grp[1] if g == 3 else grp[g - 2] if g >= 4 else ()):
                park(j)
            for ci, (j, t) in enumerate(cols):
                if g == 2 and ci == 4:
                    for jj in grp[0] + grp[1]:
                        scores(jj)
                if g >= 3 and ci == 6:
                    for jj in grp[g - 1]:
                        scores(jj)
                    for jj in grp[g - 3]:
                        pv(jj)
                proj(j, t)
        lo = o_lhs(early)
        for n in range(8):
            accb[n] = _dot(lo, o_rhs(n, early))
            if n == 1:
                for jj in grp[NG - 1]:
                    scores(jj)
                for jj in grp[NG - 3]:
                    pv(jj)
            if n == 4:
                for jj in grp[NG - 2] + grp[NG - 1]:
                    pv(jj)
        lo = o_lhs(late)
        for n in range(8):
            a = accb[n] + _dot(lo, o_rhs(n, late))
            ha[pl.ds(a0, TOK), pl.ds(n * 128, 128)] = a[0:TOK]
            memb[:, pl.ds(n * 128, 128)] = a[TOK:TOK + M]

    def steps(i, carry):
        for k in range(UNROLL):
            step(i, k)
        return carry

    with jax.named_scope("p2_steps"):
        lax.fori_loop(0, NSEG // UNROLL, steps, 0)

    for g in range(8):
        mod_copy(g).wait()

    def lo16(w):
        return pltpu.bitcast(w << 16, F32)

    def hi16(w):
        return pltpu.bitcast(w & jnp.uint32(0xFFFF0000), F32)

    def mod_vpu(g, dep):
        for t in range(4):
            acc = None if dep is None else pltpu.bitcast(dep & zerob[...], F32)
            for k in range(D // 16):
                cw = colb[pl.ds(k * 8, 8), :]
                w = wmod[g, pl.ds(k * 8, 8), pl.ds(t * 128, 128)]
                pe = lo16(w) * lo16(cw)
                acc = pe if acc is None else acc + pe
                acc = acc + hi16(w) * hi16(cw)
            dep = pltpu.bitcast(acc, U32)
            y = jnp.sum(acc, axis=0, keepdims=True).astype(BF16).astype(F32)
            if g // 2 == 2:
                y = 1.0 + y
            modb[g // 2, :, pl.ds((g % 2) * 512 + t * 128, 128)] = jnp.broadcast_to(y, (8, 128))
        return dep

    def ln2_piece(r0, dep):
        r2 = pl.multiple_of(r0 // 2, 8)
        x2 = load_x16(r2, dep) + mrow(2, 16) * ha[pl.ds(pl.multiple_of(r0, 16), 16), :]
        h2 = pltpu.bitcast((_ln(x2) * mrow(4, 16) + mrow(3, 16)).astype(BF16), F32)
        hn[pl.ds(r2, 8), :] = h2
        return pltpu.bitcast(h2[:, D - 128:], U32)

    def bulk_o(one, carry):
        dep = None
        for i in range(2):
            lo = jnp.concatenate([oring[h, pl.ds(i * 256, 256), :] for h in range(H)], axis=1).astype(BF16)
            for n in range(8):
                if i == 0:
                    dep = mod_vpu(n, dep)
                else:
                    for z in range(2):
                        dep = ln2_piece(one * FB + (2 * n + z) * 16, dep)
                ha[pl.ds(NSEG * TOK + i * 256, 256), pl.ds(n * 128, 128)] = _dot(lo, _bf(wo[n]))
        return carry

    with jax.named_scope("p3_bulk_o"):
        bulk_o(zero_s[0], 0)

    w1_copy.wait()
    w2_copy.wait()

    nb = S // FB

    out32 = out_hbm.bitcast(U32)
    HB = FB // 2

    def ffn(i, carry):
        rows2 = pl.ds(pl.multiple_of(i * HB, HB), HB)
        h2 = _bf(hn[rows2, :])
        g = jax.nn.gelu(_dot(h2, _bf(w1[...])) + rep(biasb[:, pl.ds(0, FF)], FB), approximate=True).astype(BF16)
        nxt = lax.rem(i + 1, nb) * FB
        dep = None
        for n in range(8):
            cols = pl.ds(n * 128, 128)
            for z in range(2):
                dep = ln2_piece(nxt + (2 * n + z) * 16, dep)
                y = _dot(g[z * HB:(z + 1) * HB], _bf(w2[:, cols])) + rep(biasb[:, pl.ds(FF + n * 128, 128)], HB)
                xr = pl.ds(pl.multiple_of(i * HB + z * (HB // 2), HB // 2), HB // 2)
                ar = pl.ds(pl.multiple_of(i * FB + z * HB, HB), HB)
                x2 = _bf(xs[xr, cols]).astype(F32) + rep(modb[0, :, cols], HB) * ha[ar, cols]
                xs[xr, cols] = pltpu.bitcast((x2 + rep(modb[3, :, cols], HB) * y).astype(BF16), U32)
        pltpu.make_async_copy(xs.at[rows2], out32.at[rows2], sem.at[SEM_OUT]).start()
        return carry

    with jax.named_scope("p4_ffn"):
        lax.fori_loop(0, nb, ffn, 0)
    pltpu.make_async_copy(xs, out32, sem.at[SEM_OUT]).wait()


@jax.jit
def pallas_adaLN_cond__memory_aug_recurrent_mem_tr__dense_activation_gelu__prompt_kernel(
    A_x, A_mem0, A_Wq, A_Wk, A_Wv, A_Wo, A_seg_len, B_x, B_w1, B_b1, B_w2, B_b2, c, w_mod,
):
    assert A_x.shape == (1, S, D) and A_Wq.shape == (D, H, E) and A_mem0.shape == (1, M, D)
    any_spec = pl.BlockSpec(memory_space=pl.ANY)
    out = pl.pallas_call(
        _kernel,
        out_shape=jax.ShapeDtypeStruct((S, D), BF16),
        in_specs=[any_spec] * 12,
        out_specs=any_spec,
        scratch_shapes=[
            pltpu.VMEM((S // 2, D), U32),
            pltpu.VMEM((96, D // 2, E), U32),
            pltpu.VMEM((8, H * E // 2, 128), U32),
            pltpu.VMEM((D // 2, FF), U32),
            pltpu.VMEM((FF // 2, D), U32),
            pltpu.VMEM((NQ, 2, D // 2, KQ), U32),
            pltpu.VMEM((8, D // 2, 512), U32),
            pltpu.VMEM((H, RING, E), F32),
            pltpu.VMEM((H, RING, E), F32),
            pltpu.VMEM((H + 1, RING, E), F32),
            pltpu.VMEM((H, RING, E), F32),
            pltpu.VMEM((S, D), F32),
            pltpu.VMEM((S - PRE, D), F32),
            pltpu.VMEM((8, PRE // 2, 128), U32),
            pltpu.VMEM((M, D), F32),
            pltpu.VMEM((NQ, 2, 8, KQ), F32),
            pltpu.VMEM((4, 8, D), F32),
            pltpu.VMEM((8, D), U32),
            pltpu.VMEM((8, FF + D), F32),
            pltpu.VMEM((80, 128), F32),
            pltpu.VMEM((8, 32, 128), F32),
            pltpu.VMEM((8, 128), U32),
            pltpu.VMEM((D // 2, 128), U32),
            pltpu.SMEM((1,), jnp.int32),
            pltpu.VMEM((M, D), BF16),
            pltpu.VMEM((FF,), BF16),
            pltpu.VMEM((D,), BF16),
            pltpu.VMEM((1, D), BF16),
            pltpu.SemaphoreType.DMA((NSEM,)),
        ],
        compiler_params=pltpu.CompilerParams(vmem_limit_bytes=127 * 1024 * 1024),
    )(
        A_x.reshape(S, D), A_mem0.reshape(M, D),
        A_Wq.reshape(D // 2, 2, H, E), A_Wk.reshape(D // 2, 2, H, E), A_Wv.reshape(D // 2, 2, H, E),
        A_Wo.reshape(H * E, D), B_w1, B_b1, B_w2, B_b2, c, w_mod,
    )
    return out.reshape(1, S, D)
```

```python
import math

import jax
import jax.numpy as jnp
from jax import lax
import jax.experimental.pallas as pl
import jax.experimental.pallas.tpu as pltpu

F32 = jnp.float32
BF16 = jnp.bfloat16
U32 = jnp.uint32

S = 2048
D = 1024
H = 32
E = 128
M = 8
SEG = 32
NSEG = S // SEG
FF = 3584
NP = H // 2
TOK = 24
PRE = S - NSEG * TOK
RING = 576
OOFF = (-NSEG * TOK) % RING
LN_EPS = 1e-5
FB = 256
XC = (S - PRE) // 6
UNROLL = 4

NQ = 4
KQ = D // NQ

FIRST_STARTS = [('m', 0), ('w', 0, 0, 2), ('w', 0, 2, 6), ('w', 0, 6, 12), ('m', 1), ('w', 1, 0, 6),
                ('w', 1, 6, 12), ('m', 2)]
P1A_BLOCKS = [
    ([], [('m', 0)]),
    ([], [('w', 0, 0, 2)]),
    ([], [('w', 0, 2, 6)]),
    ([('w', 2, 0, 6), ('w', 2, 6, 12)], [('w', 0, 6, 12)]),
    ([('m', 3), ('w', 3, 0, 6), ('w', 3, 6, 12)], [('m', 1), ('w', 1, 0, 6)]),
    ([], [('m', 2), ('w', 1, 6, 12)]),
    ([('g', 2), ('g', 3)], [('w', 2, 0, 6), ('w', 2, 6, 12)]),
    ([('g', 4), ('g', 5)], [('m', 3), ('w', 3, 0, 6), ('w', 3, 6, 12)]),
]
W_ITEMS = [it for _, items in P1A_BLOCKS for it in items if it[0] == 'w']
NX0 = 4

SEM_C = 0
SEM_X0 = 1
SEM_MOD = SEM_X0 + NX0
SEM_WA = SEM_MOD + NQ + 1
SEM_WB = SEM_WA + len(W_ITEMS)
SEM_XC = SEM_WB + 6
SEM_WO = SEM_XC + 6
SEM_W1 = SEM_WO + 1
SEM_W2 = SEM_W1 + 1
SEM_OUT = SEM_W2 + 1
NSEM = SEM_OUT + 1


def _ln(x):
    m = jnp.mean(x, axis=-1, keepdims=True)
    xc = x - m
    v = jnp.mean(xc * xc, axis=-1, keepdims=True)
    return xc * lax.rsqrt(v + LN_EPS)


def _bf(w32):
    return pltpu.bitcast(w32, BF16)


def _dot(a, b):
    return jnp.dot(a, b, preferred_element_type=F32)


def _kernel(x_hbm, mem0_hbm, wq_hbm, wk_hbm, wv_hbm, wo_hbm, w1_hbm, b1_hbm, w2_hbm, b2_hbm,
            c_hbm, wmod_hbm, out_hbm,
            xs, wqkv, wo, w1, w2, wmoda, wmod, qka, qkb, vring, oring, ha, hn, hb, memb, moda, modb, scb, biasb,
            fillb, accb, zerob, colb, zero_s, mem0_ref, b1_ref, b2_ref, c_ref, sem):
    qkv_hbm = [r.bitcast(U32) for r in (wq_hbm, wk_hbm, wv_hbm)]
    x32 = x_hbm.bitcast(U32)
    wo32 = wo_hbm.bitcast(U32)
    wmod32 = wmod_hbm.bitcast(U32)

    def units_start(lo, hi, rows, sem_idx):
        for u in range(lo, hi):
            j, m = u // 3, u % 3
            for p in range(2):
                pltpu.make_async_copy(qkv_hbm[m].at[rows, p, j, :], wqkv.at[2 * u + p, rows, :],
                                      sem.at[sem_idx]).start()

    def units_wait(lo, n, rows, sem_idx):
        blk = wqkv.at[pl.ds(2 * lo, 2 * n), rows, :]
        pltpu.make_async_copy(blk, blk, sem.at[sem_idx]).wait()

    def item_start(item):
        if item[0] == 'm':
            qq = item[1]
            for k in range(2):
                pltpu.make_async_copy(wmod32.at[:, pl.ds(k * D + qq * KQ, KQ)], wmoda.at[qq, k],
                                      sem.at[SEM_MOD + qq]).start()
        elif item[0] == 'w':
            _, qq, lo, hi = item
            units_start(lo, hi, pl.ds(qq * (KQ // 2), KQ // 2), SEM_WA + W_ITEMS.index(item))
        else:
            whole_start(item[1])

    def item_wait(item):
        if item[0] == 'm':
            qq = item[1]
            pltpu.make_async_copy(wmoda.at[qq], wmoda.at[qq], sem.at[SEM_MOD + qq]).wait()
        else:
            _, qq, lo, hi = item
            units_wait(lo, hi - lo, pl.ds(qq * (KQ // 2), KQ // 2), SEM_WA + W_ITEMS.index(item))

    def whole_start(i):
        xc_copy(i - 2).start()
        units_start(6 * i, 6 * i + 6, pl.ds(0, D // 2), SEM_WB + i - 2)

    def mod_copy(g):
        return pltpu.make_async_copy(wmod32.at[:, pl.ds(2 * D + g * 512, 512)], wmod.at[g],
                                     sem.at[SEM_MOD + NQ])

    def x0_copy(i):
        n = PRE // 2 // NX0
        rows = pl.ds(pl.multiple_of(i * n, n), n)
        return pltpu.make_async_copy(x32.at[rows], xs.at[rows], sem.at[SEM_X0 + i])

    def xc_copy(i):
        rows = pl.ds(pl.multiple_of(PRE // 2 + i * (XC // 2), 64), XC // 2)
        return pltpu.make_async_copy(x32.at[rows], xs.at[rows], sem.at[SEM_XC + i])

    def wo_copy(n):
        return pltpu.make_async_copy(wo32.at[:, pl.ds(n * 128, 128)], wo.at[n], sem.at[SEM_WO])

    w1_copy = pltpu.make_async_copy(w1_hbm.bitcast(U32), w1, sem.at[SEM_W1])
    w2_copy = pltpu.make_async_copy(w2_hbm.bitcast(U32), w2, sem.at[SEM_W2])
    small_copies = [pltpu.make_async_copy(a, b, sem.at[SEM_C])
                    for a, b in ((c_hbm, c_ref), (mem0_hbm, mem0_ref), (b1_hbm, b1_ref),
                                 (b2_hbm, b2_ref))]

    def deinterleave(u, row0, nrows):
        for k in range(nrows // 64):
            rows = pl.ds(row0 + k * 64, 64)
            a = wqkv[2 * u, rows, :]
            b = wqkv[2 * u + 1, rows, :]
            wqkv[2 * u, rows, :] = (a & jnp.uint32(0xFFFF)) | (b << 16)
            wqkv[2 * u + 1, rows, :] = (a >> 16) | (b & jnp.uint32(0xFFFF0000))

    def load_x16(row2, dep):
        xw = xs[pl.ds(row2, 8), :]
        if dep is not None:
            first = xw[:, 0:128] | (dep & zerob[...])
            xw = jnp.concatenate([first, xw[:, 128:]], axis=1)
        return _bf(xw).astype(F32)

    def rep(v8, n):
        return jnp.concatenate([v8] * (n // 8), axis=0)

    def mrow(k, n):
        if k < 2:
            return rep(jnp.concatenate([moda[qq, k] for qq in range(NQ)], axis=1), n)
        return rep(modb[k - 2], n)

    for cp in small_copies:
        cp.start()
    for i in range(NX0):
        x0_copy(i).start()
    for item in FIRST_STARTS:
        item_start(item)

    def start_rest():
        for n in range(8):
            wo_copy(n).start()
        for g in range(8):
            mod_copy(g).start()
        w1_copy.start()
        w2_copy.start()

    r = lax.broadcasted_iota(jnp.int32, (80, 128), 0)
    q = lax.broadcasted_iota(jnp.int32, (80, 128), 1)
    r_tok = r < 64
    q_tok = q < 64
    r_head = jnp.where(r_tok, r >> 5, (r - 64) >> 3)
    q_head = jnp.where(q_tok, q >> 5, (q - 64) >> 3)
    same = (r_head == q_head) & (q < 80)
    causal_ok = jnp.logical_not(r_tok & q_tok & ((q & 31) > (r & 31)))
    scale = E ** (-0.5)
    fillb[...] = jnp.where(same, jnp.where(causal_ok, 0.0, -1e9 / scale), -jnp.inf).astype(F32)
    zerob[...] = jnp.zeros((8, 128), U32)
    zero_s[0] = 0

    pre_rows = pl.ds(RING - PRE, PRE)

    for cp in small_copies:
        cp.wait()
    cf = c_ref[...].astype(F32)
    sc = (cf * jax.nn.sigmoid(cf)).astype(BF16)
    scb[...] = pltpu.bitcast(jnp.broadcast_to(sc, (16, D)), U32)
    scf = jnp.broadcast_to(sc.astype(F32), (128, D))
    for k in range(8):
        colb[pl.ds(k * 64, 64), :] = pltpu.bitcast(scf[:, k * 128:(k + 1) * 128].T.astype(BF16), U32)
    memb[...] = mem0_ref[...].astype(F32)
    biasb[:, pl.ds(0, FF)] = jnp.broadcast_to(b1_ref[...].astype(F32).reshape(1, FF), (8, FF))
    biasb[:, pl.ds(FF, D)] = jnp.broadcast_to(b2_ref[...].astype(F32).reshape(1, D), (8, D))

    def pre_norm(i, carry):
        x0_copy(i).wait()
        nr = PRE // NX0
        for z in range(nr // 16):
            xn = _ln(load_x16(pl.multiple_of(i * (nr // 2) + z * 8, 8), None))
            for n in range(8):
                oring[n, pl.ds(pl.multiple_of(i * nr + z * 16, 16), 16), :] = xn[:, n * 128:(n + 1) * 128]
        return carry

    with jax.named_scope("p0_ln"):
        lax.fori_loop(0, NX0, pre_norm, 0)

    def dst_slot(i, k, p):
        cls, m = k // 3, k % 3
        if m == 2:
            return vring, 4 * i + 2 * cls + p
        return (qka, qkb)[cls], 4 * i + 2 * m + p

    NT = KQ // 128

    def item_run(item):
        if item[0] == 'm':
            qq = item[1]
            sc16 = _bf(scb[...])
            ca1 = 1.0 + _dot(sc16, _bf(wmoda[qq, 1]))[0:8].astype(BF16).astype(F32)
            sa = _dot(sc16, _bf(wmoda[qq, 0]))[0:8].astype(BF16).astype(F32)
            moda[qq, 0] = sa
            moda[qq, 1] = ca1
            for n in range(NT):
                cols = slice(n * 128, (n + 1) * 128)
                for z in range(PRE // 64):
                    hq = (oring[NT * qq + n, pl.ds(z * 64, 64), :] * rep(ca1[:, cols], 64)
                          + rep(sa[:, cols], 64))
                    hb[NT * qq + n, pl.ds(z * 32, 32), :] = pltpu.bitcast(hq.astype(BF16), U32)
            return
        _, qq, lo, hi = item
        row0 = qq * (KQ // 2)
        for u in range(lo, hi):
            i, k = u // 6, u % 6
            deinterleave(u, row0, KQ // 2)
            for p in range(2):
                lhs = _bf(jnp.concatenate([hb[NT * qq + n] for n in range(NT)], axis=1))
                ref, idx = dst_slot(i, k, p)
                y = _dot(lhs, _bf(wqkv[2 * u + p, pl.ds(row0, KQ // 2), :]))
                if qq > 0:
                    y = y + ref[idx, pre_rows, :]
                ref[idx, pre_rows, :] = y

    def phase1b(i, carry):
        @pl.when(i == 3)
        def _():
            whole_start(6)
            whole_start(7)

        @pl.when(i == 4)
        def _():
            start_rest()

        xc_copy(i - 2).wait()
        units_wait(6 * i, 6, pl.ds(0, D // 2), SEM_WB + i - 2)
        deinterleave(6 * i, 0, D // 2)
        dep = None
        for k in range(6):
            u = 6 * i + k
            for p in range(2):
                lhs = _bf(jnp.concatenate([hb[n] for n in range(8)], axis=1))
                ref, idx = dst_slot(i, k, p)
                ref[idx, pre_rows, :] = _dot(lhs, _bf(wqkv[2 * u + p]))
                if p == 0 and k < 5:
                    deinterleave(u + 1, 0, D // 2)
                if k >= 2:
                    for z in range(2):
                        r0 = (i - 2) * XC + (4 * k + 2 * p + z - 8) * 16
                        x16 = load_x16(pl.multiple_of(PRE // 2 + r0 // 2, 8), dep)
                        h16 = _ln(x16) * mrow(1, 16) + mrow(0, 16)
                        hn[pl.ds(pl.multiple_of(r0, 16), 16), :] = h16
                        dep = pltpu.bitcast(h16[8:16, D - 128:], U32)
        return carry

    for bi, (starts, items) in enumerate(P1A_BLOCKS):
        for item in starts:
            item_start(item)
        with jax.named_scope("p1a_wait%d" % bi):
            for item in items:
                item_wait(item)
        for item in items:
            item_run(item)
    with jax.named_scope("p1b"):
        lax.fori_loop(2, 8, phase1b, 0)
    for n in range(8):
        wo_copy(n).wait()

    cexp = scale * math.log2(math.e)
    NG = NP // 2
    grp = [(4 * (g // 2) + (g % 2), 4 * (g // 2) + (g % 2) + 2) for g in range(NG)]
    early = [2 * j + u for g in range(NG - 3) for j in grp[g] for u in range(2)]
    late = [h for h in range(H) if h not in early]

    def step(it, k):
        s = it * UNROLL + k
        split = k > 0
        base = TOK * UNROLL * it
        w0 = pl.multiple_of(lax.rem(base, RING), 32) + TOK * k
        r0 = pl.multiple_of(lax.rem(SEG * s + (RING - PRE), RING), 32)
        ow = pl.multiple_of(lax.rem(SEG * s + OOFF, RING), 32)
        o0 = pl.multiple_of(lax.rem(base + OOFF, RING), 32) + TOK * k
        a0 = pl.multiple_of(base, 32) + TOK * k
        X = jnp.concatenate([hn[pl.ds(a0, TOK), :], memb[...]], axis=0).astype(BF16)
        ym = [None] * 96
        probs = [None] * NP
        om = [None] * H
        order = (4, 5, 0, 1, 2, 3)

        if split:
            for t in order:
                accb[t] = _dot(X[:, :D // 2], _bf(wqkv[t, pl.ds(0, D // 4), :]))

        def slot(j, t):
            if t >= 4:
                return vring, 2 * j + t - 4
            return (qka, qkb)[j % 2], 4 * (j // 2) + t

        def proj(j, t):
            c = 6 * j + t
            if split and j == 0:
                y = accb[t] + _dot(X[:, D // 2:], _bf(wqkv[c, pl.ds(D // 4, D // 4), :]))
            else:
                y = _dot(X, _bf(wqkv[c]))
            ref, k = slot(j, t)
            ref[k, pl.ds(w0, TOK), :] = y[0:TOK]
            ym[c] = y[TOK:TOK + M]

        def gather(j, m, pad):
            c = 6 * j + 2 * m
            ref, k = slot(j, 2 * m)
            parts = [ref[k, pl.ds(r0, SEG), :], ref[k + 1, pl.ds(r0, SEG), :], ym[c], ym[c + 1]]
            if pad:
                parts.append(jnp.zeros((48, E), F32))
            return jnp.concatenate(parts, axis=0).astype(BF16)

        def scores(j):
            sc_ = lax.dot_general(gather(j, 0, False), gather(j, 1, True),
                                  (((1,), (1,)), ((), ())), preferred_element_type=F32)
            fill = fillb[...]
            sc_ = jnp.where(fill == 0.0, sc_, fill)
            mx = jnp.max(sc_, axis=-1, keepdims=True)
            p = jnp.exp2((sc_ - mx) * cexp)
            l = jnp.sum(p, axis=-1, keepdims=True)
            rl = pl.reciprocal(l, approx=True)
            rl = rl * (2.0 - l * rl)
            probs[j] = (p * rl).astype(BF16)

        def park(j):
            vring[H, pl.ds(40 * (j % 8), 40), :] = pltpu.bitcast(probs[j], F32)
            probs[j] = None

        def pv(j):
            P = probs[j]
            if P is None:
                P = _bf(vring[H, pl.ds(40 * (j % 8), 40), :])
            o = _dot(P, gather(j, 2, True))
            oring[2 * j, pl.ds(ow, SEG), :] = o[0:32]
            oring[2 * j + 1, pl.ds(ow, SEG), :] = o[32:64]
            om[2 * j] = o[64:72]
            om[2 * j + 1] = o[72:80]

        def o_lhs(hs):
            return jnp.concatenate(
                [jnp.concatenate([oring[h, pl.ds(o0, TOK), :], om[h]], axis=0) for h in hs],
                axis=1).astype(BF16)

        def o_rhs(n, hs):
            return _bf(jnp.concatenate([wo[n, pl.ds(h * 64, 64), :] for h in hs], axis=0))

        for g in range(NG):
            cols = [(j, t) for j in grp[g] for t in order]
            if g == 2:
                cols = ([(j, t) for j in grp[g] for t in (4, 5)]
                        + [(j, t) for j in grp[g] for t in range(4)])
            for j in (grp[0] + grp[1] if g == 3 else grp[g - 2] if g >= 4 else ()):
                park(j)
            for ci, (j, t) in enumerate(cols):
                if g == 2 and ci == 4:
                    for jj in grp[0] + grp[1]:
                        scores(jj)
                if g >= 3 and ci == 6:
                    for jj in grp[g - 1]:
                        scores(jj)
                    for jj in grp[g - 3]:
                        pv(jj)
                proj(j, t)
        lo = o_lhs(early)
        for n in range(8):
            accb[n] = _dot(lo, o_rhs(n, early))
            if n == 1:
                for jj in grp[NG - 1]:
                    scores(jj)
                for jj in grp[NG - 3]:
                    pv(jj)
            if n == 4:
                for jj in grp[NG - 2] + grp[NG - 1]:
                    pv(jj)
        lo = o_lhs(late)
        for n in range(8):
            a = accb[n] + _dot(lo, o_rhs(n, late))
            ha[pl.ds(a0, TOK), pl.ds(n * 128, 128)] = a[0:TOK]
            memb[:, pl.ds(n * 128, 128)] = a[TOK:TOK + M]

    def steps(i, carry):
        for k in range(UNROLL):
            step(i, k)
        return carry

    with jax.named_scope("p2_steps"):
        lax.fori_loop(0, NSEG // UNROLL, steps, 0)

    for g in range(8):
        mod_copy(g).wait()

    def lo16(w):
        return pltpu.bitcast(w << 16, F32)

    def hi16(w):
        return pltpu.bitcast(w & jnp.uint32(0xFFFF0000), F32)

    def mod_vpu(g, dep):
        for t in range(4):
            acc = None if dep is None else pltpu.bitcast(dep & zerob[...], F32)
            for k in range(D // 16):
                cw = colb[pl.ds(k * 8, 8), :]
                w = wmod[g, pl.ds(k * 8, 8), pl.ds(t * 128, 128)]
                pe = lo16(w) * lo16(cw)
                acc = pe if acc is None else acc + pe
                acc = acc + hi16(w) * hi16(cw)
            dep = pltpu.bitcast(acc, U32)
            y = jnp.sum(acc, axis=0, keepdims=True).astype(BF16).astype(F32)
            if g // 2 == 2:
                y = 1.0 + y
            modb[g // 2, :, pl.ds((g % 2) * 512 + t * 128, 128)] = jnp.broadcast_to(y, (8, 128))
        return dep

    def ln2_piece(r0, dep):
        r2 = pl.multiple_of(r0 // 2, 8)
        x2 = load_x16(r2, dep) + mrow(2, 16) * ha[pl.ds(pl.multiple_of(r0, 16), 16), :]
        h2 = pltpu.bitcast((_ln(x2) * mrow(4, 16) + mrow(3, 16)).astype(BF16), F32)
        hn[pl.ds(r2, 8), :] = h2
        return pltpu.bitcast(h2[:, D - 128:], U32)

    def bulk_o(one, carry):
        dep = None
        for i in range(2):
            lo = jnp.concatenate([oring[h, pl.ds(i * 256, 256), :] for h in range(H)], axis=1).astype(BF16)
            for n in range(8):
                if i == 0:
                    dep = mod_vpu(n, dep)
                else:
                    for z in range(2):
                        dep = ln2_piece(one * FB + (2 * n + z) * 16, dep)
                ha[pl.ds(NSEG * TOK + i * 256, 256), pl.ds(n * 128, 128)] = _dot(lo, _bf(wo[n]))
        return carry

    with jax.named_scope("p3_bulk_o"):
        bulk_o(zero_s[0], 0)

    w1_copy.wait()
    w2_copy.wait()

    nb = S // FB

    out32 = out_hbm.bitcast(F32)
    HB = FB // 2
    qka[16, pl.ds(0, 8), :] = jnp.zeros((8, E), F32)

    def ffn(i, carry):
        rows2 = pl.ds(pl.multiple_of(i * HB, HB), HB)
        h2 = _bf(hn[rows2, :])
        g = jax.nn.gelu(_dot(h2, _bf(w1[...])) + rep(biasb[:, pl.ds(0, FF)], FB), approximate=True).astype(BF16)
        nxt = lax.rem(i + 1, nb) * FB
        half = i // 4
        srow = pl.multiple_of(lax.rem(i, 4) * HB, HB)
        dep = None
        for n in range(8):
            cols = pl.ds(n * 128, 128)
            for z in range(2):
                pin = pltpu.bitcast(qka[16, pl.ds(0, 8), :], U32)
                dep = ln2_piece(nxt + (2 * n + z) * 16, pin if dep is None else dep | pin)
                y = _dot(g[z * HB:(z + 1) * HB], _bf(w2[:, cols])) + rep(biasb[:, pl.ds(FF + n * 128, 128)], HB)
                xr = pl.ds(pl.multiple_of(i * HB + z * (HB // 2), HB // 2), HB // 2)
                ar = pl.ds(pl.multiple_of(i * FB + z * HB, HB), HB)
                x2 = _bf(xs[xr, cols]).astype(F32) + rep(modb[0, :, cols], HB) * ha[ar, cols]
                qka[2 * n + half, pl.ds(srow + z * (HB // 2), HB // 2), :] = pltpu.bitcast(
                    (x2 + rep(modb[3, :, cols], HB) * y).astype(BF16), F32)
            pltpu.make_async_copy(qka.at[2 * n + half, pl.ds(srow, HB), :], out32.at[rows2, cols],
                                  sem.at[SEM_OUT]).start()
        return carry

    with jax.named_scope("p4_ffn"):
        lax.fori_loop(0, nb, ffn, 0)
    pltpu.make_async_copy(out32, out32, sem.at[SEM_OUT]).wait()


@jax.jit
def pallas_adaLN_cond__memory_aug_recurrent_mem_tr__dense_activation_gelu__prompt_kernel(
    A_x, A_mem0, A_Wq, A_Wk, A_Wv, A_Wo, A_seg_len, B_x, B_w1, B_b1, B_w2, B_b2, c, w_mod,
):
    assert A_x.shape == (1, S, D) and A_Wq.shape == (D, H, E) and A_mem0.shape == (1, M, D)
    any_spec = pl.BlockSpec(memory_space=pl.ANY)
    out = pl.pallas_call(
        _kernel,
        out_shape=jax.ShapeDtypeStruct((S, D), BF16),
        in_specs=[any_spec] * 12,
        out_specs=any_spec,
        scratch_shapes=[
            pltpu.VMEM((S // 2, D), U32),
            pltpu.VMEM((96, D // 2, E), U32),
            pltpu.VMEM((8, H * E // 2, 128), U32),
            pltpu.VMEM((D // 2, FF), U32),
            pltpu.VMEM((FF // 2, D), U32),
            pltpu.VMEM((NQ, 2, D // 2, KQ), U32),
            pltpu.VMEM((8, D // 2, 512), U32),
            pltpu.VMEM((H, RING, E), F32),
            pltpu.VMEM((H, RING, E), F32),
            pltpu.VMEM((H + 1, RING, E), F32),
            pltpu.VMEM((H, RING, E), F32),
            pltpu.VMEM((S, D), F32),
            pltpu.VMEM((S - PRE, D), F32),
            pltpu.VMEM((8, PRE // 2, 128), U32),
            pltpu.VMEM((M, D), F32),
            pltpu.VMEM((NQ, 2, 8, KQ), F32),
            pltpu.VMEM((4, 8, D), F32),
            pltpu.VMEM((8, D), U32),
            pltpu.VMEM((8, FF + D), F32),
            pltpu.VMEM((80, 128), F32),
            pltpu.VMEM((8, 32, 128), F32),
            pltpu.VMEM((8, 128), U32),
            pltpu.VMEM((D // 2, 128), U32),
            pltpu.SMEM((1,), jnp.int32),
            pltpu.VMEM((M, D), BF16),
            pltpu.VMEM((FF,), BF16),
            pltpu.VMEM((D,), BF16),
            pltpu.VMEM((1, D), BF16),
            pltpu.SemaphoreType.DMA((NSEM,)),
        ],
        compiler_params=pltpu.CompilerParams(vmem_limit_bytes=127 * 1024 * 1024, disable_bounds_checks=True,
                                             disable_semaphore_checks=True),
    )(
        A_x.reshape(S, D), A_mem0.reshape(M, D),
        A_Wq.reshape(D // 2, 2, H, E), A_Wk.reshape(D // 2, 2, H, E), A_Wv.reshape(D // 2, 2, H, E),
        A_Wo.reshape(H * E, D), B_w1, B_b1, B_w2, B_b2, c, w_mod,
    )
    return out.reshape(1, S, D)
```

```python
import functools
import math

import jax
import jax.numpy as jnp
from jax import lax
import jax.experimental.pallas as pl
import jax.experimental.pallas.tpu as pltpu

F32 = jnp.float32
BF16 = jnp.bfloat16
U32 = jnp.uint32

S = 2048
D = 1024
H = 32
E = 128
M = 8
SEG = 32
NSEG = S // SEG
FF = 3584
NP = H // 2
TOK = 24
PRE = S - NSEG * TOK
RING = 576
OOFF = (-NSEG * TOK) % RING
LN_EPS = 1e-5
FB = 256
XC = (S - PRE) // 6
UNROLL = 4

NQ = 4
KQ = D // NQ

FIRST_STARTS = [('m', 0), ('w', 0, 0, 2), ('w', 0, 2, 6), ('w', 0, 6, 12), ('m', 1), ('w', 1, 0, 6),
                ('w', 1, 6, 12), ('m', 2)]
P1A_BLOCKS = [
    ([], [('m', 0)]),
    ([], [('w', 0, 0, 2)]),
    ([], [('w', 0, 2, 6)]),
    ([('w', 2, 0, 6), ('w', 2, 6, 12)], [('w', 0, 6, 12)]),
    ([('m', 3), ('w', 3, 0, 6), ('w', 3, 6, 12)], [('m', 1), ('w', 1, 0, 6)]),
    ([], [('m', 2), ('w', 1, 6, 12)]),
    ([('g', 2), ('g', 3)], [('w', 2, 0, 6), ('w', 2, 6, 12)]),
    ([('g', 4), ('g', 5)], [('m', 3), ('w', 3, 0, 6), ('w', 3, 6, 12)]),
]
W_ITEMS = [it for _, items in P1A_BLOCKS for it in items if it[0] == 'w']
NX0 = 4

SEM_C = 0
SEM_X0 = 1
SEM_MOD = SEM_X0 + NX0
SEM_WA = SEM_MOD + NQ + 1
SEM_WB = SEM_WA + len(W_ITEMS)
SEM_XC = SEM_WB + 6
SEM_WO = SEM_XC + 6
SEM_W1 = SEM_WO + 1
SEM_W2 = SEM_W1 + 1
SEM_OUT = SEM_W2 + 1
NSEM = SEM_OUT + 1


def _ln(x):
    m = jnp.mean(x, axis=-1, keepdims=True)
    xc = x - m
    v = jnp.mean(xc * xc, axis=-1, keepdims=True)
    return xc * lax.rsqrt(v + LN_EPS)


def _bf(w32):
    return pltpu.bitcast(w32, BF16)


def _dot(a, b):
    return jnp.dot(a, b, preferred_element_type=F32)


def _lhs_combos(a11, a12, a21, a22):
    return [a11 + a22, a21 + a22, a11, a22, a11 + a12, a21 - a11, a12 - a22]


def _rhs_combos(b11, b12, b21, b22):
    return [b11 + b22, b12 - b22, b21 - b11, b11 + b12, b21 + b22]


_RHS_IDX = {0: 0, 2: 1, 3: 2, 5: 3, 6: 4}
_RHS_TERMS = {0: ((0, 0), (1, 1), 1), 1: ((0, 0), None, 0), 2: ((0, 1), (1, 1), -1), 3: ((1, 0), (0, 0), -1),
              4: ((1, 1), None, 0), 5: ((0, 0), (0, 1), 1), 6: ((1, 0), (1, 1), 1)}


def _rhs_operand(c, blk, wrap=lambda raw: raw):
    p, q, sign = _RHS_TERMS[c]
    a = _bf(wrap(blk(*p)))
    if q is None:
        return a
    a = a.astype(F32)
    b = _bf(blk(*q)).astype(F32)
    return (a + b if sign > 0 else a - b).astype(BF16)


def _strassen(prod, finish, side=lambda: None):
    side()
    m1 = prod(1)
    m3 = prod(3)
    finish(m1 + m3, 1, 0)
    side()
    m2 = prod(2)
    m4 = prod(4)
    finish(m2 + m4, 0, 1)
    side()
    m0 = prod(0)
    m5 = prod(5)
    finish((m2 - m1) + m0 + m5, 1, 1)
    side()
    m6 = prod(6)
    finish((m3 - m4) + m0 + m6, 0, 0)


def _kernel(x_hbm, mem0_hbm, wq_hbm, wk_hbm, wv_hbm, wo_hbm, w1_hbm, b1_hbm, w2_hbm, b2_hbm,
            c_hbm, wmod_hbm, out_hbm,
            xs, wqkv, wo, w1, w2, wmod, qka, qkb, vring, oring, ha, hn, hb, memb, moda, modb, scb, biasb,
            fillb, accb, zerob, colb, tb, zero_s, mem0_ref, b1_ref, b2_ref, c_ref, sem):
    qkv_hbm = [r.bitcast(U32) for r in (wq_hbm, wk_hbm, wv_hbm)]
    x32 = x_hbm.bitcast(U32)
    wo32 = wo_hbm.bitcast(U32)
    wmod32 = wmod_hbm.bitcast(U32)

    def units_start(lo, hi, rows, sem_idx):
        for u in range(lo, hi):
            j, m = u // 3, u % 3
            for p in range(2):
                pltpu.make_async_copy(qkv_hbm[m].at[rows, p, j, :], wqkv.at[2 * u + p, rows, :],
                                      sem.at[sem_idx]).start()

    def units_wait(lo, n, rows, sem_idx):
        blk = wqkv.at[pl.ds(2 * lo, 2 * n), rows, :]
        pltpu.make_async_copy(blk, blk, sem.at[sem_idx]).wait()

    def item_start(item):
        if item[0] == 'm':
            qq = item[1]
            for k in range(2):
                pltpu.make_async_copy(wmod32.at[:, pl.ds(k * D + qq * KQ, KQ)], wmod.at[qq, :, pl.ds(k * KQ, KQ)],
                                      sem.at[SEM_MOD + qq]).start()
        elif item[0] == 'w':
            _, qq, lo, hi = item
            units_start(lo, hi, pl.ds(qq * (KQ // 2), KQ // 2), SEM_WA + W_ITEMS.index(item))
        else:
            whole_start(item[1])

    def item_wait(item):
        if item[0] == 'm':
            qq = item[1]
            pltpu.make_async_copy(wmod.at[qq], wmod.at[qq], sem.at[SEM_MOD + qq]).wait()
        else:
            _, qq, lo, hi = item
            units_wait(lo, hi - lo, pl.ds(qq * (KQ // 2), KQ // 2), SEM_WA + W_ITEMS.index(item))

    def whole_start(i):
        xc_copy(i - 2).start()
        units_start(6 * i, 6 * i + 6, pl.ds(0, D // 2), SEM_WB + i - 2)

    def mod_copy(g):
        return pltpu.make_async_copy(wmod32.at[:, pl.ds(2 * D + g * 512, 512)], wmod.at[g],
                                     sem.at[SEM_MOD + NQ])

    def x0_copy(i):
        n = PRE // 2 // NX0
        rows = pl.ds(pl.multiple_of(i * n, n), n)
        return pltpu.make_async_copy(x32.at[rows], xs.at[rows], sem.at[SEM_X0 + i])

    def xc_copy(i):
        rows = pl.ds(pl.multiple_of(PRE // 2 + i * (XC // 2), 64), XC // 2)
        return pltpu.make_async_copy(x32.at[rows], xs.at[rows], sem.at[SEM_XC + i])

    def wo_copy(n):
        return pltpu.make_async_copy(wo32.at[:, pl.ds(n * 128, 128)], wo.at[n], sem.at[SEM_WO])

    w1_copy = pltpu.make_async_copy(w1_hbm.bitcast(U32), w1, sem.at[SEM_W1])
    w2_copy = pltpu.make_async_copy(w2_hbm.bitcast(U32), w2, sem.at[SEM_W2])
    small_copies = [pltpu.make_async_copy(a, b, sem.at[SEM_C])
                    for a, b in ((c_hbm, c_ref), (mem0_hbm, mem0_ref), (b1_hbm, b1_ref),
                                 (b2_hbm, b2_ref))]

    def deinterleave(u, row0, nrows):
        for k in range(nrows // 64):
            rows = pl.ds(row0 + k * 64, 64)
            a = wqkv[2 * u, rows, :]
            b = wqkv[2 * u + 1, rows, :]
            wqkv[2 * u, rows, :] = (a & jnp.uint32(0xFFFF)) | (b << 16)
            wqkv[2 * u + 1, rows, :] = (a >> 16) | (b & jnp.uint32(0xFFFF0000))

    def load_x16(row2, dep):
        xw = xs[pl.ds(row2, 8), :]
        if dep is not None:
            first = xw[:, 0:128] | (dep & zerob[...])
            xw = jnp.concatenate([first, xw[:, 128:]], axis=1)
        return _bf(xw).astype(F32)

    def rep(v8, n):
        return jnp.concatenate([v8] * (n // 8), axis=0)

    def mrow(k, n):
        if k < 2:
            return rep(jnp.concatenate([moda[qq, k] for qq in range(NQ)], axis=1), n)
        return rep(modb[k - 2], n)

    for cp in small_copies:
        cp.start()
    for i in range(NX0):
        x0_copy(i).start()
    for item in FIRST_STARTS:
        item_start(item)

    def start_rest():
        for n in range(8):
            wo_copy(n).start()
        for g in range(8):
            mod_copy(g).start()
        w1_copy.start()
        w2_copy.start()

    r = lax.broadcasted_iota(jnp.int32, (80, 128), 0)
    q = lax.broadcasted_iota(jnp.int32, (80, 128), 1)
    r_tok = r < 64
    q_tok = q < 64
    r_head = jnp.where(r_tok, r >> 5, (r - 64) >> 3)
    q_head = jnp.where(q_tok, q >> 5, (q - 64) >> 3)
    same = (r_head == q_head) & (q < 80)
    causal_ok = jnp.logical_not(r_tok & q_tok & ((q & 31) > (r & 31)))
    scale = E ** (-0.5)
    fillb[...] = jnp.where(same, jnp.where(causal_ok, 0.0, -1e9 / scale), -jnp.inf).astype(F32)
    zerob[...] = jnp.zeros((8, 128), U32)
    zero_s[0] = 0

    pre_rows = pl.ds(RING - PRE, PRE)

    for cp in small_copies:
        cp.wait()
    cf = c_ref[...].astype(F32)
    sc = (cf * jax.nn.sigmoid(cf)).astype(BF16)
    scb[...] = pltpu.bitcast(jnp.broadcast_to(sc, (16, D)), U32)
    scf = jnp.broadcast_to(sc.astype(F32), (128, D))
    for k in range(8):
        colb[pl.ds(k * 64, 64), :] = pltpu.bitcast(scf[:, k * 128:(k + 1) * 128].T.astype(BF16), U32)
    memb[...] = mem0_ref[...].astype(F32)
    biasb[:, pl.ds(0, FF)] = jnp.broadcast_to(b1_ref[...].astype(F32).reshape(1, FF), (8, FF))
    biasb[:, pl.ds(FF, D)] = jnp.broadcast_to(b2_ref[...].astype(F32).reshape(1, D), (8, D))

    def pre_norm(i, carry):
        x0_copy(i).wait()
        nr = PRE // NX0
        for z in range(nr // 16):
            xn = _ln(load_x16(pl.multiple_of(i * (nr // 2) + z * 8, 8), None))
            for n in range(8):
                oring[n, pl.ds(pl.multiple_of(i * nr + z * 16, 16), 16), :] = xn[:, n * 128:(n + 1) * 128]
        return carry

    with jax.named_scope("p0_ln"):
        lax.fori_loop(0, NX0, pre_norm, 0)

    def dst_slot(i, k, p):
        cls, m = k // 3, k % 3
        if m == 2:
            return vring, 4 * i + 2 * cls + p
        return (qka, qkb)[cls], 4 * i + 2 * m + p

    NT = KQ // 128

    def item_run(item):
        if item[0] == 'm':
            qq = item[1]
            sc16 = _bf(scb[...])
            ca1 = 1.0 + _dot(sc16, _bf(wmod[qq, :, pl.ds(KQ, KQ)]))[0:8].astype(BF16).astype(F32)
            sa = _dot(sc16, _bf(wmod[qq, :, pl.ds(0, KQ)]))[0:8].astype(BF16).astype(F32)
            moda[qq, 0] = sa
            moda[qq, 1] = ca1
            for n in range(NT):
                cols = slice(n * 128, (n + 1) * 128)
                for z in range(PRE // 64):
                    hq = (oring[NT * qq + n, pl.ds(z * 64, 64), :] * rep(ca1[:, cols], 64)
                          + rep(sa[:, cols], 64))
                    hb[NT * qq + n, pl.ds(z * 32, 32), :] = pltpu.bitcast(hq.astype(BF16), U32)
            return
        _, qq, lo, hi = item
        row0 = qq * (KQ // 2)
        for u in range(lo, hi):
            i, k = u // 6, u % 6
            deinterleave(u, row0, KQ // 2)
            for p in range(2):
                lhs = _bf(jnp.concatenate([hb[NT * qq + n] for n in range(NT)], axis=1))
                ref, idx = dst_slot(i, k, p)
                y = _dot(lhs, _bf(wqkv[2 * u + p, pl.ds(row0, KQ // 2), :]))
                if qq > 0:
                    y = y + ref[idx, pre_rows, :]
                ref[idx, pre_rows, :] = y

    def phase1b(i, carry):
        @pl.when(i == 3)
        def _():
            whole_start(6)
            whole_start(7)

        @pl.when(i == 4)
        def _():
            start_rest()

        xc_copy(i - 2).wait()
        units_wait(6 * i, 6, pl.ds(0, D // 2), SEM_WB + i - 2)
        deinterleave(6 * i, 0, D // 2)
        dep = None
        for k in range(6):
            u = 6 * i + k
            for p in range(2):
                lhs = _bf(jnp.concatenate([hb[n] for n in range(8)], axis=1))
                ref, idx = dst_slot(i, k, p)
                ref[idx, pre_rows, :] = _dot(lhs, _bf(wqkv[2 * u + p]))
                if p == 0 and k < 5:
                    deinterleave(u + 1, 0, D // 2)
                if k >= 2:
                    for z in range(2):
                        r0 = (i - 2) * XC + (4 * k + 2 * p + z - 8) * 16
                        x16 = load_x16(pl.multiple_of(PRE // 2 + r0 // 2, 8), dep)
                        h16 = _ln(x16) * mrow(1, 16) + mrow(0, 16)
                        hn[pl.ds(pl.multiple_of(r0, 16), 16), :] = h16
                        dep = pltpu.bitcast(h16[8:16, D - 128:], U32)
        return carry

    for bi, (starts, items) in enumerate(P1A_BLOCKS):
        for item in starts:
            item_start(item)
        with jax.named_scope("p1a_wait%d" % bi):
            for item in items:
                item_wait(item)
        for item in items:
            item_run(item)
    with jax.named_scope("p1b"):
        lax.fori_loop(2, 8, phase1b, 0)
    for n in range(8):
        wo_copy(n).wait()

    cexp = scale * math.log2(math.e)
    NG = NP // 2
    grp = [(4 * (g // 2) + (g % 2), 4 * (g // 2) + (g % 2) + 2) for g in range(NG)]
    early = [2 * j + u for g in range(NG - 3) for j in grp[g] for u in range(2)]
    late = [h for h in range(H) if h not in early]

    def step(it, k):
        s = it * UNROLL + k
        split = k > 0
        base = TOK * UNROLL * it
        w0 = pl.multiple_of(lax.rem(base, RING), 32) + TOK * k
        r0 = pl.multiple_of(lax.rem(SEG * s + (RING - PRE), RING), 32)
        ow = pl.multiple_of(lax.rem(SEG * s + OOFF, RING), 32)
        o0 = pl.multiple_of(lax.rem(base + OOFF, RING), 32) + TOK * k
        a0 = pl.multiple_of(base, 32) + TOK * k
        X = jnp.concatenate([hn[pl.ds(a0, TOK), :], memb[...]], axis=0).astype(BF16)
        ym = [None] * 96
        probs = [None] * NP
        om = [None] * H
        order = (4, 5, 0, 1, 2, 3)

        if split:
            for t in order:
                accb[t] = _dot(X[:, :D // 2], _bf(wqkv[t, pl.ds(0, D // 4), :]))

        def slot(j, t):
            if t >= 4:
                return vring, 2 * j + t - 4
            return (qka, qkb)[j % 2], 4 * (j // 2) + t

        def proj(j, t):
            c = 6 * j + t
            if split and j == 0:
                y = accb[t] + _dot(X[:, D // 2:], _bf(wqkv[c, pl.ds(D // 4, D // 4), :]))
            else:
                y = _dot(X, _bf(wqkv[c]))
            ref, k = slot(j, t)
            ref[k, pl.ds(w0, TOK), :] = y[0:TOK]
            ym[c] = y[TOK:TOK + M]

        def gather(j, m, pad):
            c = 6 * j + 2 * m
            ref, k = slot(j, 2 * m)
            parts = [ref[k, pl.ds(r0, SEG), :], ref[k + 1, pl.ds(r0, SEG), :], ym[c], ym[c + 1]]
            if pad:
                parts.append(jnp.zeros((48, E), F32))
            return jnp.concatenate(parts, axis=0).astype(BF16)

        def scores(j):
            sc_ = lax.dot_general(gather(j, 0, False), gather(j, 1, True),
                                  (((1,), (1,)), ((), ())), preferred_element_type=F32)
            fill = fillb[...]
            sc_ = jnp.where(fill == 0.0, sc_, fill)
            mx = jnp.max(sc_, axis=-1, keepdims=True)
            p = jnp.exp2((sc_ - mx) * cexp)
            l = jnp.sum(p, axis=-1, keepdims=True)
            rl = pl.reciprocal(l, approx=True)
            rl = rl * (2.0 - l * rl)
            probs[j] = (p * rl).astype(BF16)

        def park(j):
            vring[H, pl.ds(40 * (j % 8), 40), :] = pltpu.bitcast(probs[j], F32)
            probs[j] = None

        def pv(j):
            P = probs[j]
            if P is None:
                P = _bf(vring[H, pl.ds(40 * (j % 8), 40), :])
            o = _dot(P, gather(j, 2, True))
            oring[2 * j, pl.ds(ow, SEG), :] = o[0:32]
            oring[2 * j + 1, pl.ds(ow, SEG), :] = o[32:64]
            om[2 * j] = o[64:72]
            om[2 * j + 1] = o[72:80]

        def o_lhs(hs):
            return jnp.concatenate(
                [jnp.concatenate([oring[h, pl.ds(o0, TOK), :], om[h]], axis=0) for h in hs],
                axis=1).astype(BF16)

        def o_rhs(n, hs):
            return _bf(jnp.concatenate([wo[n, pl.ds(h * 64, 64), :] for h in hs], axis=0))

        for g in range(NG):
            cols = [(j, t) for j in grp[g] for t in order]
            if g == 2:
                cols = ([(j, t) for j in grp[g] for t in (4, 5)]
                        + [(j, t) for j in grp[g] for t in range(4)])
            for j in (grp[0] + grp[1] if g == 3 else grp[g - 2] if g >= 4 else ()):
                park(j)
            for ci, (j, t) in enumerate(cols):
                if g == 2 and ci == 4:
                    for jj in grp[0] + grp[1]:
                        scores(jj)
                if g >= 3 and ci == 6:
                    for jj in grp[g - 1]:
                        scores(jj)
                    for jj in grp[g - 3]:
                        pv(jj)
                proj(j, t)
        lo = o_lhs(early)
        for n in range(8):
            accb[n] = _dot(lo, o_rhs(n, early))
            if n == 1:
                for jj in grp[NG - 1]:
                    scores(jj)
                for jj in grp[NG - 3]:
                    pv(jj)
            if n == 4:
                for jj in grp[NG - 2] + grp[NG - 1]:
                    pv(jj)
        lo = o_lhs(late)
        for n in range(8):
            a = accb[n] + _dot(lo, o_rhs(n, late))
            ha[pl.ds(a0, TOK), pl.ds(n * 128, 128)] = a[0:TOK]
            memb[:, pl.ds(n * 128, 128)] = a[TOK:TOK + M]

    def steps(i, carry):
        for k in range(UNROLL):
            step(i, k)
        return carry

    with jax.named_scope("p2_steps"):
        lax.fori_loop(0, NSEG // UNROLL, steps, 0)

    for g in range(8):
        mod_copy(g).wait()
    w1_copy.wait()
    w2_copy.wait()

    def lo16(w):
        return pltpu.bitcast(w << 16, F32)

    def hi16(w):
        return pltpu.bitcast(w & jnp.uint32(0xFFFF0000), F32)

    macc = {}

    def mod_job(g, k):
        cw = colb[pl.ds(k * 8, 8), :]
        bits = None
        for t in range(4):
            w = wmod[g, pl.ds(k * 8, 8), pl.ds(t * 128, 128)]
            v = lo16(w) * lo16(cw) + hi16(w) * hi16(cw)
            macc[t] = v if k == 0 else macc[t] + v
            b = pltpu.bitcast(v, U32)
            bits = b if bits is None else bits | b
            if k == D // 16 - 1:
                y = jnp.sum(macc[t], axis=0, keepdims=True).astype(BF16).astype(F32)
                if g // 2 == 2:
                    y = 1.0 + y
                modb[g // 2, :, pl.ds((g % 2) * 512 + t * 128, 128)] = jnp.broadcast_to(y, (8, 128))
        return bits

    nb = S // FB
    HB = FB // 2

    def h2_16(blk, off, dep):
        x2 = (load_x16(pl.multiple_of(blk * HB, HB) + off // 2, dep)
              + mrow(2, 16) * ha[pl.ds(pl.multiple_of(blk * FB, FB) + off, 16), :])
        return _ln(x2) * mrow(4, 16) + mrow(3, 16)

    def ln2_piece(blk, base, piece, dep):
        k = piece // 2
        if piece % 2 == 0:
            h = h2_16(blk, 16 * k, dep)
            tb[pl.ds(16 * k, 16), :] = h
            return pltpu.bitcast(h[8:16, D - 128:], U32)
        h = h2_16(blk, HB + 16 * k, dep)
        for t in range(4):
            c1, c2 = t * 128, D // 2 + t * 128
            combos = _lhs_combos(tb[pl.ds(16 * k, 16), pl.ds(c1, 128)], tb[pl.ds(16 * k, 16), pl.ds(c2, 128)],
                                 h[:, c1:c1 + 128], h[:, c2:c2 + 128])
            for c, v in enumerate(combos):
                last = pltpu.bitcast(v.astype(BF16), F32)
                hn[pl.ds(base + 64 * (c // 2) + 8 * k, 8), pl.ds(512 * (c % 2) + t * 128, 128)] = last
        return pltpu.bitcast(last, U32)

    def rhs1_loc(cc, n, r):
        return 3 * n + cc // 2, 256 * (cc % 2) + r

    def rhs2_loc(cc, n, r):
        return 42 + 2 * (5 * n + cc) + r // 512, r % 512

    def rhs_job(w, kh, nh, n, loc, r):
        raw = [w[pl.ds(r + a * kh, 8), pl.ds(n * 128 + b * nh, 128)] for a in range(2) for b in range(2)]
        bits = None
        for cc, v in enumerate(_rhs_combos(*[_bf(v).astype(F32) for v in raw])):
            sl, row = loc(cc, n, r)
            wqkv[sl, pl.ds(row, 8), :] = pltpu.bitcast(v.astype(BF16), U32)
            b = pltpu.bitcast(v[8 * (cc % 2):8 * (cc % 2) + 8], U32)
            bits = b if bits is None else bits | b
        return bits

    def rhs1(c, n):
        if c == 1:
            return _bf(w1[pl.ds(0, D // 4), pl.ds(n * 128, 128)])
        if c == 4:
            return _bf(w1[pl.ds(D // 4, D // 4), pl.ds(FF // 2 + n * 128, 128)])
        sl, row = rhs1_loc(_RHS_IDX[c], n, 0)
        return _bf(wqkv[sl, pl.ds(row, D // 4), :])

    def rhs2(c, n):
        if c == 1:
            return _bf(w2[pl.ds(0, FF // 4), pl.ds(n * 128, 128)])
        if c == 4:
            return _bf(w2[pl.ds(FF // 4, FF // 4), pl.ds(D // 2 + n * 128, 128)])
        sl, _ = rhs2_loc(_RHS_IDX[c], n, 0)
        return _bf(jnp.concatenate([wqkv[sl], wqkv[sl + 1, pl.ds(0, FF // 4 - 512), :]], axis=0))

    def bulk_o(zero):
        jobs = ([functools.partial(mod_job, g, k) for g in range(8) for k in range(D // 16)]
                + [functools.partial(rhs_job, w1, D // 4, FF // 2, n, rhs1_loc, r)
                   for n in range(FF // 256) for r in range(0, D // 4, 8)]
                + [functools.partial(rhs_job, w2, FF // 4, D // 2, n, rhs2_loc, r)
                   for n in range(D // 256) for r in range(0, FF // 4, 8)])[::-1]
        state = dict(credit=-16.0, dep=None, piece=0)

        def tie(raw, density):
            parts = []
            for r in range(0, raw.shape[0], 8):
                v = raw[r:r + 8]
                state['credit'] += density
                if jobs and state['credit'] >= 1.0:
                    state['credit'] -= 1.0
                    v = v | (jobs.pop()() & zerob[...])
                parts.append(v)
            return jnp.concatenate(parts, axis=0)

        def a_blk(rh, kh):
            return jnp.concatenate([oring[h, pl.ds(rh * 256, 256), :]
                                    for h in range(16 * kh, 16 * kh + 16)], axis=1)

        lhs = [v.astype(BF16) for v in _lhs_combos(a_blk(0, 0), a_blk(0, 1), a_blk(1, 0), a_blk(1, 1))]
        for n in range(4):
            def prod(c):
                rhs = _rhs_operand(c, lambda a, b: wo[n + 4 * b, pl.ds(a * 1024, 1024), :],
                                   lambda raw: tie(raw, 0.56 if c in (1, 4) else 0.34))
                return _dot(lhs[c], rhs)

            def side():
                if n >= 2:
                    for _ in range(2):
                        state['dep'] = ln2_piece(zero, 0, state['piece'], state['dep'])
                        state['piece'] += 1

            def finish(y, rh, ch):
                ha[pl.ds(NSEG * TOK + rh * 256, 256), pl.ds((n + 4 * ch) * 128, 128)] = y

            _strassen(prod, finish, side)
        assert not jobs

    qka[16, pl.ds(0, 8), :] = jnp.zeros((8, E), F32)
    with jax.named_scope("p3_bulk_o"):
        bulk_o(zero_s[0])

    out32 = out_hbm.bitcast(F32)

    def ffn(i, carry):
        base = pl.multiple_of(lax.rem(i, 2) * 256, 256)
        nbase = pl.multiple_of(lax.rem(i + 1, 2) * 256, 256)
        nxt = lax.rem(i + 1, nb)
        half = i // 4
        srow = pl.multiple_of(lax.rem(i, 4) * HB, HB)

        def gelu(v):
            return jax.nn.gelu(v, approximate=True)

        g = [[] for _ in range(7)]
        for n in range(FF // 256):
            m = [None] * 7
            for c in (1, 3, 2, 4, 0, 5, 6):
                lhs = _bf(hn[pl.ds(base + 64 * (c // 2), 64), pl.ds(512 * (c % 2), 512)])
                m[c] = _dot(lhs, rhs1(c, n))
            b1a = rep(biasb[:, pl.ds(n * 128, 128)], HB)
            b1b = rep(biasb[:, pl.ds(FF // 2 + n * 128, 128)], HB)
            combos = _lhs_combos(gelu((m[3] - m[4]) + m[0] + m[6] + b1a), gelu(m[2] + m[4] + b1b),
                                 gelu(m[1] + m[3] + b1a), gelu((m[2] - m[1]) + m[0] + m[5] + b1b))
            for c, v in enumerate(combos):
                g[c].append(v.astype(BF16))
        g = [jnp.concatenate(v, axis=1) for v in g]

        state = dict(dep=None, piece=0)

        def ln_next():
            pin = pltpu.bitcast(qka[16, pl.ds(0, 8), :], U32)
            dep = pin if state['dep'] is None else state['dep'] | pin
            state['dep'] = ln2_piece(nxt, nbase, state['piece'], dep)
            state['piece'] += 1

        def finish(y, rh, nn):
            cols = pl.ds(nn * 128, 128)
            y = y + rep(biasb[:, pl.ds(FF + nn * 128, 128)], HB)
            xr = pl.ds(pl.multiple_of(i * HB, HB) + rh * (HB // 2), HB // 2)
            ar = pl.ds(pl.multiple_of(i * FB, FB) + rh * HB, HB)
            x2 = _bf(xs[xr, cols]).astype(F32) + rep(modb[0, :, cols], HB) * ha[ar, cols]
            qka[2 * nn + half, pl.ds(srow + rh * (HB // 2), HB // 2), :] = pltpu.bitcast(
                (x2 + rep(modb[3, :, cols], HB) * y).astype(BF16), F32)

        def copy_out(nn):
            pltpu.make_async_copy(qka.at[2 * nn + half, pl.ds(srow, HB), :],
                                  out32.at[pl.ds(pl.multiple_of(i * HB, HB), HB), pl.ds(nn * 128, 128)],
                                  sem.at[SEM_OUT]).start()

        for n in range(D // 256):
            def finish_n(y, rh, ch):
                finish(y, rh, n + 4 * ch)
                if rh == ch:
                    copy_out(n + 4 * ch)

            _strassen(lambda c: _dot(g[c], rhs2(c, n)), finish_n, ln_next)
        return carry

    with jax.named_scope("p4_ffn"):
        lax.fori_loop(0, nb, ffn, 0)
    pltpu.make_async_copy(out32, out32, sem.at[SEM_OUT]).wait()


@jax.jit
def pallas_adaLN_cond__memory_aug_recurrent_mem_tr__dense_activation_gelu__prompt_kernel(
    A_x, A_mem0, A_Wq, A_Wk, A_Wv, A_Wo, A_seg_len, B_x, B_w1, B_b1, B_w2, B_b2, c, w_mod,
):
    assert A_x.shape == (1, S, D) and A_Wq.shape == (D, H, E) and A_mem0.shape == (1, M, D)
    any_spec = pl.BlockSpec(memory_space=pl.ANY)
    out = pl.pallas_call(
        _kernel,
        out_shape=jax.ShapeDtypeStruct((S, D), BF16),
        in_specs=[any_spec] * 12,
        out_specs=any_spec,
        scratch_shapes=[
            pltpu.VMEM((S // 2, D), U32),
            pltpu.VMEM((96, D // 2, E), U32),
            pltpu.VMEM((8, H * E // 2, 128), U32),
            pltpu.VMEM((D // 2, FF), U32),
            pltpu.VMEM((FF // 2, D), U32),
            pltpu.VMEM((8, D // 2, 512), U32),
            pltpu.VMEM((H, RING, E), F32),
            pltpu.VMEM((H, RING, E), F32),
            pltpu.VMEM((H + 1, RING, E), F32),
            pltpu.VMEM((H, RING, E), F32),
            pltpu.VMEM((S, D), F32),
            pltpu.VMEM((S - PRE, D), F32),
            pltpu.VMEM((8, PRE // 2, 128), U32),
            pltpu.VMEM((M, D), F32),
            pltpu.VMEM((NQ, 2, 8, KQ), F32),
            pltpu.VMEM((4, 8, D), F32),
            pltpu.VMEM((8, D), U32),
            pltpu.VMEM((8, FF + D), F32),
            pltpu.VMEM((80, 128), F32),
            pltpu.VMEM((8, 32, 128), F32),
            pltpu.VMEM((8, 128), U32),
            pltpu.VMEM((D // 2, 128), U32),
            pltpu.VMEM((FB // 2, D), F32),
            pltpu.SMEM((1,), jnp.int32),
            pltpu.VMEM((M, D), BF16),
            pltpu.VMEM((FF,), BF16),
            pltpu.VMEM((D,), BF16),
            pltpu.VMEM((1, D), BF16),
            pltpu.SemaphoreType.DMA((NSEM,)),
        ],
        compiler_params=pltpu.CompilerParams(vmem_limit_bytes=127 * 1024 * 1024, disable_bounds_checks=True,
                                             disable_semaphore_checks=True),
    )(
        A_x.reshape(S, D), A_mem0.reshape(M, D),
        A_Wq.reshape(D // 2, 2, H, E), A_Wk.reshape(D // 2, 2, H, E), A_Wv.reshape(D // 2, 2, H, E),
        A_Wo.reshape(H * E, D), B_w1, B_b1, B_w2, B_b2, c, w_mod,
    )
    return out.reshape(1, S, D)
```

```python
import functools
import math

import jax
import jax.numpy as jnp
from jax import lax
import jax.experimental.pallas as pl
import jax.experimental.pallas.tpu as pltpu

F32 = jnp.float32
BF16 = jnp.bfloat16
U32 = jnp.uint32

S = 2048
D = 1024
H = 32
E = 128
M = 8
SEG = 32
NSEG = S // SEG
FF = 3584
NP = H // 2
TOK = 24
PRE = S - NSEG * TOK
RING = 576
OOFF = (-NSEG * TOK) % RING
LN_EPS = 1e-5
FB = 256
XC = (S - PRE) // 6
UNROLL = 4

NQ = 4
KQ = D // NQ

FIRST_STARTS = [('m', 0), ('w', 0, 0, 2), ('w', 0, 2, 6), ('w', 0, 6, 12), ('m', 1), ('w', 1, 0, 6),
                ('w', 1, 6, 12), ('m', 2)]
P1A_BLOCKS = [
    ([], [('m', 0)]),
    ([], [('w', 0, 0, 2)]),
    ([], [('w', 0, 2, 6)]),
    ([('w', 2, 0, 6), ('w', 2, 6, 12)], [('w', 0, 6, 12)]),
    ([('m', 3), ('w', 3, 0, 6), ('w', 3, 6, 12)], [('m', 1), ('w', 1, 0, 6)]),
    ([], [('m', 2), ('w', 1, 6, 12)]),
    ([('g', 2), ('g', 3)], [('w', 2, 0, 6), ('w', 2, 6, 12)]),
    ([('g', 4), ('g', 5)], [('m', 3), ('w', 3, 0, 6), ('w', 3, 6, 12)]),
]
W_ITEMS = [it for _, items in P1A_BLOCKS for it in items if it[0] == 'w']
NX0 = 4

SEM_C = 0
SEM_X0 = 1
SEM_MOD = SEM_X0 + NX0
SEM_WA = SEM_MOD + NQ + 1
SEM_WB = SEM_WA + len(W_ITEMS)
SEM_XC = SEM_WB + 6
SEM_WO = SEM_XC + 6
SEM_W1 = SEM_WO + 1
SEM_W2 = SEM_W1 + 1
SEM_OUT = SEM_W2 + 1
NSEM = SEM_OUT + 1


def _ln(x):
    m = jnp.mean(x, axis=-1, keepdims=True)
    xc = x - m
    v = jnp.mean(xc * xc, axis=-1, keepdims=True)
    return xc * lax.rsqrt(v + LN_EPS)


def _bf(w32):
    return pltpu.bitcast(w32, BF16)


def _dot(a, b):
    return jnp.dot(a, b, preferred_element_type=F32)


def _lhs_combos(a11, a12, a21, a22):
    return [a11 + a22, a21 + a22, a11, a22, a11 + a12, a21 - a11, a12 - a22]


def _rhs_combos(b11, b12, b21, b22):
    return [b11 + b22, b12 - b22, b21 - b11, b11 + b12, b21 + b22]


_RHS_IDX = {0: 0, 2: 1, 3: 2, 5: 3, 6: 4}
_RHS_TERMS = {0: ((0, 0), (1, 1), 1), 1: ((0, 0), None, 0), 2: ((0, 1), (1, 1), -1), 3: ((1, 0), (0, 0), -1),
              4: ((1, 1), None, 0), 5: ((0, 0), (0, 1), 1), 6: ((1, 0), (1, 1), 1)}


def _rhs_operand(c, blk, wrap=lambda raw: raw):
    p, q, sign = _RHS_TERMS[c]
    a = _bf(wrap(blk(*p)))
    if q is None:
        return a
    a = a.astype(F32)
    b = _bf(blk(*q)).astype(F32)
    return (a + b if sign > 0 else a - b).astype(BF16)


def _strassen(prod, finish, side=lambda: None):
    side()
    m1 = prod(1)
    m3 = prod(3)
    finish(m1 + m3, 1, 0)
    side()
    m2 = prod(2)
    m4 = prod(4)
    finish(m2 + m4, 0, 1)
    side()
    m0 = prod(0)
    m5 = prod(5)
    finish((m2 - m1) + m0 + m5, 1, 1)
    side()
    m6 = prod(6)
    finish((m3 - m4) + m0 + m6, 0, 0)


def _kernel(x_hbm, mem0_hbm, wq_hbm, wk_hbm, wv_hbm, wo_hbm, w1_hbm, b1_hbm, w2_hbm, b2_hbm,
            c_hbm, wmod_hbm, out_hbm,
            xs, wqkv, wo, w1, w2, wmod, qka, qkb, vring, oring, ha, hn, hb, memb, moda, modb, scb, biasb,
            fillb, accb, zerob, colb, tb, zero_s, mem0_ref, b1_ref, b2_ref, c_ref, sem):
    qkv_hbm = [r.bitcast(U32) for r in (wq_hbm, wk_hbm, wv_hbm)]
    x32 = x_hbm.bitcast(U32)
    wo32 = wo_hbm.bitcast(U32)
    wmod32 = wmod_hbm.bitcast(U32)

    def units_start(lo, hi, rows, sem_idx):
        for u in range(lo, hi):
            j, m = u // 3, u % 3
            for p in range(2):
                pltpu.make_async_copy(qkv_hbm[m].at[rows, p, j, :], wqkv.at[2 * u + p, rows, :],
                                      sem.at[sem_idx]).start()

    def units_wait(lo, n, rows, sem_idx):
        blk = wqkv.at[pl.ds(2 * lo, 2 * n), rows, :]
        pltpu.make_async_copy(blk, blk, sem.at[sem_idx]).wait()

    def item_start(item):
        if item[0] == 'm':
            qq = item[1]
            for k in range(2):
                pltpu.make_async_copy(wmod32.at[:, pl.ds(k * D + qq * KQ, KQ)], wmod.at[qq, :, pl.ds(k * KQ, KQ)],
                                      sem.at[SEM_MOD + qq]).start()
        elif item[0] == 'w':
            _, qq, lo, hi = item
            units_start(lo, hi, pl.ds(qq * (KQ // 2), KQ // 2), SEM_WA + W_ITEMS.index(item))
        else:
            whole_start(item[1])

    def item_wait(item):
        if item[0] == 'm':
            qq = item[1]
            pltpu.make_async_copy(wmod.at[qq], wmod.at[qq], sem.at[SEM_MOD + qq]).wait()
        else:
            _, qq, lo, hi = item
            units_wait(lo, hi - lo, pl.ds(qq * (KQ // 2), KQ // 2), SEM_WA + W_ITEMS.index(item))

    def whole_start(i):
        xc_copy(i - 2).start()
        units_start(6 * i, 6 * i + 6, pl.ds(0, D // 2), SEM_WB + i - 2)

    def mod_copy(g):
        return pltpu.make_async_copy(wmod32.at[:, pl.ds(2 * D + g * 512, 512)], wmod.at[g],
                                     sem.at[SEM_MOD + NQ])

    def x0_copy(i):
        n = PRE // 2 // NX0
        rows = pl.ds(pl.multiple_of(i * n, n), n)
        return pltpu.make_async_copy(x32.at[rows], xs.at[rows], sem.at[SEM_X0 + i])

    def xc_copy(i):
        rows = pl.ds(pl.multiple_of(PRE // 2 + i * (XC // 2), 64), XC // 2)
        return pltpu.make_async_copy(x32.at[rows], xs.at[rows], sem.at[SEM_XC + i])

    def wo_copy(n):
        return pltpu.make_async_copy(wo32.at[:, pl.ds(n * 128, 128)], wo.at[n], sem.at[SEM_WO])

    w1_copy = pltpu.make_async_copy(w1_hbm.bitcast(U32), w1, sem.at[SEM_W1])
    w2_copy = pltpu.make_async_copy(w2_hbm.bitcast(U32), w2, sem.at[SEM_W2])
    small_copies = [pltpu.make_async_copy(a, b, sem.at[SEM_C])
                    for a, b in ((c_hbm, c_ref), (mem0_hbm, mem0_ref), (b1_hbm, b1_ref),
                                 (b2_hbm, b2_ref))]

    def deinterleave(u, row0, nrows):
        for k in range(nrows // 64):
            rows = pl.ds(row0 + k * 64, 64)
            a = wqkv[2 * u, rows, :]
            b = wqkv[2 * u + 1, rows, :]
            wqkv[2 * u, rows, :] = (a & jnp.uint32(0xFFFF)) | (b << 16)
            wqkv[2 * u + 1, rows, :] = (a >> 16) | (b & jnp.uint32(0xFFFF0000))

    def load_x16(row2, dep):
        xw = xs[pl.ds(row2, 8), :]
        if dep is not None:
            first = xw[:, 0:128] | (dep & zerob[...])
            xw = jnp.concatenate([first, xw[:, 128:]], axis=1)
        return _bf(xw).astype(F32)

    def rep(v8, n):
        return jnp.concatenate([v8] * (n // 8), axis=0)

    def mrow(k, n):
        if k < 2:
            return rep(jnp.concatenate([moda[qq, k] for qq in range(NQ)], axis=1), n)
        return rep(modb[k - 2], n)

    for cp in small_copies:
        cp.start()
    for i in range(NX0):
        x0_copy(i).start()
    for item in FIRST_STARTS:
        item_start(item)

    def start_rest():
        for n in range(8):
            wo_copy(n).start()
        for g in range(8):
            mod_copy(g).start()
        w1_copy.start()
        w2_copy.start()

    r = lax.broadcasted_iota(jnp.int32, (80, 128), 0)
    q = lax.broadcasted_iota(jnp.int32, (80, 128), 1)
    r_tok = r < 64
    q_tok = q < 64
    r_head = jnp.where(r_tok, r >> 5, (r - 64) >> 3)
    q_head = jnp.where(q_tok, q >> 5, (q - 64) >> 3)
    same = (r_head == q_head) & (q < 80)
    causal_ok = jnp.logical_not(r_tok & q_tok & ((q & 31) > (r & 31)))
    scale = E ** (-0.5)
    fillb[...] = jnp.where(same, jnp.where(causal_ok, 0.0, -1e9 / scale), -jnp.inf).astype(F32)
    zerob[...] = jnp.zeros((8, 128), U32)
    zero_s[0] = 0

    for cp in small_copies:
        cp.wait()
    cf = c_ref[...].astype(F32)
    sc = (cf * jax.nn.sigmoid(cf)).astype(BF16)
    scb[...] = pltpu.bitcast(jnp.broadcast_to(sc, (16, D)), U32)
    scf = jnp.broadcast_to(sc.astype(F32), (128, D))
    for k in range(8):
        colb[pl.ds(k * 64, 64), :] = pltpu.bitcast(scf[:, k * 128:(k + 1) * 128].T.astype(BF16), U32)
    memb[...] = mem0_ref[...].astype(F32)
    biasb[:, pl.ds(0, FF)] = jnp.broadcast_to(b1_ref[...].astype(F32).reshape(1, FF), (8, FF))
    biasb[:, pl.ds(FF, D)] = jnp.broadcast_to(b2_ref[...].astype(F32).reshape(1, D), (8, D))

    def pre_norm(i, carry):
        x0_copy(i).wait()
        nr = PRE // NX0
        for z in range(nr // 16):
            xn = _ln(load_x16(pl.multiple_of(i * (nr // 2) + z * 8, 8), None))
            for n in range(8):
                oring[n, pl.ds(pl.multiple_of(i * nr + z * 16, 16), 16), :] = xn[:, n * 128:(n + 1) * 128]
        return carry

    with jax.named_scope("p0_ln"):
        lax.fori_loop(0, NX0, pre_norm, 0)

    def dst_slot(i, k, p):
        cls, m = k // 3, k % 3
        if m == 2:
            return vring, 4 * i + 2 * cls + p
        return (qka, qkb)[cls], 4 * i + 2 * m + p

    PH = PRE // 2
    assert KQ == 256

    def item_run(item):
        if item[0] == 'm':
            qq = item[1]
            sc16 = _bf(scb[...])
            ca1 = 1.0 + _dot(sc16, _bf(wmod[qq, :, pl.ds(KQ, KQ)]))[0:8].astype(BF16).astype(F32)
            sa = _dot(sc16, _bf(wmod[qq, :, pl.ds(0, KQ)]))[0:8].astype(BF16).astype(F32)
            moda[qq, 0] = sa
            moda[qq, 1] = ca1
            for z in range(PH // 32):
                def h_blk(rh, kh):
                    cols = slice(kh * 128, (kh + 1) * 128)
                    return (oring[2 * qq + kh, pl.ds(rh * PH + z * 32, 32), :] * rep(ca1[:, cols], 32)
                            + rep(sa[:, cols], 32))

                for c, v in enumerate(_lhs_combos(h_blk(0, 0), h_blk(0, 1), h_blk(1, 0), h_blk(1, 1))):
                    hb[c, qq, pl.ds(z * 16, 16), :] = pltpu.bitcast(v.astype(BF16), U32)
            return
        _, qq, lo, hi = item
        for u in range(lo, hi):
            deinterleave(u, qq * (KQ // 2), KQ // 2)
            unit_proj(u // 6, u % 6, [qq], qq > 0)

    def unit_proj(i, k, slices, accumulate, side=lambda: None):
        u = 6 * i + k

        def prod(c):
            lhs = _bf(jnp.concatenate([hb[c, qq] for qq in slices], axis=1))
            rhs = _rhs_operand(c, lambda a, b: jnp.concatenate(
                [wqkv[2 * u + b, pl.ds((2 * qq + a) * 64, 64), :] for qq in slices], axis=0))
            return _dot(lhs, rhs)

        def finish(y, rh, ch):
            ref, idx = dst_slot(i, k, ch)
            rows = pl.ds(RING - PRE + rh * PH, PH)
            if accumulate:
                y = y + ref[idx, rows, :]
            ref[idx, rows, :] = y

        _strassen(prod, finish, side)

    def phase1b(i, carry):
        @pl.when(i == 3)
        def _():
            whole_start(6)
            whole_start(7)

        @pl.when(i == 4)
        def _():
            start_rest()

        xc_copy(i - 2).wait()
        units_wait(6 * i, 6, pl.ds(0, D // 2), SEM_WB + i - 2)
        deinterleave(6 * i, 0, D // 2)
        state = dict(dep=None, piece=0, slot=0)

        def side():
            state['slot'] += 1
            if state['slot'] % 4 != 0 and state['piece'] < XC // 16:
                off = state['piece'] * 16
                x16 = load_x16(pl.multiple_of((i - 2) * (XC // 2), XC // 2) + (PRE + off) // 2, state['dep'])
                h16 = _ln(x16) * mrow(1, 16) + mrow(0, 16)
                hn[pl.ds(pl.multiple_of((i - 2) * XC, XC) + off, 16), :] = h16
                state['dep'] = pltpu.bitcast(h16[8:16, D - 128:], U32)
                state['piece'] += 1

        for k in range(6):
            if k < 5:
                deinterleave(6 * i + k + 1, 0, D // 2)
            unit_proj(i, k, range(NQ), False, side)
        return carry

    for bi, (starts, items) in enumerate(P1A_BLOCKS):
        for item in starts:
            item_start(item)
        with jax.named_scope("p1a_wait%d" % bi):
            for item in items:
                item_wait(item)
        for item in items:
            item_run(item)
    with jax.named_scope("p1b"):
        lax.fori_loop(2, 8, phase1b, 0)
    for n in range(8):
        wo_copy(n).wait()

    cexp = scale * math.log2(math.e)
    NG = NP // 2
    grp = [(4 * (g // 2) + (g % 2), 4 * (g // 2) + (g % 2) + 2) for g in range(NG)]
    early = [2 * j + u for g in range(NG - 3) for j in grp[g] for u in range(2)]
    late = [h for h in range(H) if h not in early]

    def step(it, k):
        s = it * UNROLL + k
        split = k > 0
        base = TOK * UNROLL * it
        w0 = pl.multiple_of(lax.rem(base, RING), 32) + TOK * k
        r0 = pl.multiple_of(lax.rem(SEG * s + (RING - PRE), RING), 32)
        ow = pl.multiple_of(lax.rem(SEG * s + OOFF, RING), 32)
        o0 = pl.multiple_of(lax.rem(base + OOFF, RING), 32) + TOK * k
        a0 = pl.multiple_of(base, 32) + TOK * k
        X = jnp.concatenate([hn[pl.ds(a0, TOK), :], memb[...]], axis=0).astype(BF16)
        ym = [None] * 96
        probs = [None] * NP
        om = [None] * H
        order = (4, 5, 0, 1, 2, 3)

        if split:
            for t in order:
                accb[t] = _dot(X[:, :D // 2], _bf(wqkv[t, pl.ds(0, D // 4), :]))

        def slot(j, t):
            if t >= 4:
                return vring, 2 * j + t - 4
            return (qka, qkb)[j % 2], 4 * (j // 2) + t

        def proj(j, t):
            c = 6 * j + t
            if split and j == 0:
                y = accb[t] + _dot(X[:, D // 2:], _bf(wqkv[c, pl.ds(D // 4, D // 4), :]))
            else:
                y = _dot(X, _bf(wqkv[c]))
            ref, k = slot(j, t)
            ref[k, pl.ds(w0, TOK), :] = y[0:TOK]
            ym[c] = y[TOK:TOK + M]

        def gather(j, m, pad):
            c = 6 * j + 2 * m
            ref, k = slot(j, 2 * m)
            parts = [ref[k, pl.ds(r0, SEG), :], ref[k + 1, pl.ds(r0, SEG), :], ym[c], ym[c + 1]]
            if pad:
                parts.append(jnp.zeros((48, E), F32))
            return jnp.concatenate(parts, axis=0).astype(BF16)

        def scores(j):
            sc_ = lax.dot_general(gather(j, 0, False), gather(j, 1, True),
                                  (((1,), (1,)), ((), ())), preferred_element_type=F32)
            fill = fillb[...]
            sc_ = jnp.where(fill == 0.0, sc_, fill)
            mx = jnp.max(sc_, axis=-1, keepdims=True)
            p = jnp.exp2((sc_ - mx) * cexp)
            l = jnp.sum(p, axis=-1, keepdims=True)
            rl = pl.reciprocal(l, approx=True)
            rl = rl * (2.0 - l * rl)
            probs[j] = (p * rl).astype(BF16)

        def park(j):
            vring[H, pl.ds(40 * (j % 8), 40), :] = pltpu.bitcast(probs[j], F32)
            probs[j] = None

        def pv(j):
            P = probs[j]
            if P is None:
                P = _bf(vring[H, pl.ds(40 * (j % 8), 40), :])
            o = _dot(P, gather(j, 2, True))
            oring[2 * j, pl.ds(ow, SEG), :] = o[0:32]
            oring[2 * j + 1, pl.ds(ow, SEG), :] = o[32:64]
            om[2 * j] = o[64:72]
            om[2 * j + 1] = o[72:80]

        def o_lhs(hs):
            return jnp.concatenate(
                [jnp.concatenate([oring[h, pl.ds(o0, TOK), :], om[h]], axis=0) for h in hs],
                axis=1).astype(BF16)

        def o_rhs(n, hs):
            return _bf(jnp.concatenate([wo[n, pl.ds(h * 64, 64), :] for h in hs], axis=0))

        for g in range(NG):
            cols = [(j, t) for j in grp[g] for t in order]
            if g == 2:
                cols = ([(j, t) for j in grp[g] for t in (4, 5)]
                        + [(j, t) for j in grp[g] for t in range(4)])
            for j in (grp[0] + grp[1] if g == 3 else grp[g - 2] if g >= 4 else ()):
                park(j)
            for ci, (j, t) in enumerate(cols):
                if g == 2 and ci == 4:
                    for jj in grp[0] + grp[1]:
                        scores(jj)
                if g >= 3 and ci == 6:
                    for jj in grp[g - 1]:
                        scores(jj)
                    for jj in grp[g - 3]:
                        pv(jj)
                proj(j, t)
        lo = o_lhs(early)
        for n in range(8):
            accb[n] = _dot(lo, o_rhs(n, early))
            if n == 1:
                for jj in grp[NG - 1]:
                    scores(jj)
                for jj in grp[NG - 3]:
                    pv(jj)
            if n == 4:
                for jj in grp[NG - 2] + grp[NG - 1]:
                    pv(jj)
        lo = o_lhs(late)
        for n in range(8):
            a = accb[n] + _dot(lo, o_rhs(n, late))
            ha[pl.ds(a0, TOK), pl.ds(n * 128, 128)] = a[0:TOK]
            memb[:, pl.ds(n * 128, 128)] = a[TOK:TOK + M]

    def steps(i, carry):
        for k in range(UNROLL):
            step(i, k)
        return carry

    with jax.named_scope("p2_steps"):
        lax.fori_loop(0, NSEG // UNROLL, steps, 0)

    for g in range(8):
        mod_copy(g).wait()
    w1_copy.wait()
    w2_copy.wait()

    def lo16(w):
        return pltpu.bitcast(w << 16, F32)

    def hi16(w):
        return pltpu.bitcast(w & jnp.uint32(0xFFFF0000), F32)

    macc = {}

    def mod_job(g, k):
        cw = colb[pl.ds(k * 8, 8), :]
        bits = None
        for t in range(4):
            w = wmod[g, pl.ds(k * 8, 8), pl.ds(t * 128, 128)]
            v = lo16(w) * lo16(cw) + hi16(w) * hi16(cw)
            macc[t] = v if k == 0 else macc[t] + v
            b = pltpu.bitcast(v, U32)
            bits = b if bits is None else bits | b
            if k == D // 16 - 1:
                y = jnp.sum(macc[t], axis=0, keepdims=True).astype(BF16).astype(F32)
                if g // 2 == 2:
                    y = 1.0 + y
                modb[g // 2, :, pl.ds((g % 2) * 512 + t * 128, 128)] = jnp.broadcast_to(y, (8, 128))
        return bits

    nb = S // FB
    HB = FB // 2

    def h2_16(blk, off, dep):
        x2 = (load_x16(pl.multiple_of(blk * HB, HB) + off // 2, dep)
              + mrow(2, 16) * ha[pl.ds(pl.multiple_of(blk * FB, FB) + off, 16), :])
        return _ln(x2) * mrow(4, 16) + mrow(3, 16)

    def ln2_piece(blk, base, piece, dep):
        k = piece // 2
        if piece % 2 == 0:
            h = h2_16(blk, 16 * k, dep)
            tb[pl.ds(16 * k, 16), :] = h
            return pltpu.bitcast(h[8:16, D - 128:], U32)
        h = h2_16(blk, HB + 16 * k, dep)
        for t in range(4):
            c1, c2 = t * 128, D // 2 + t * 128
            combos = _lhs_combos(tb[pl.ds(16 * k, 16), pl.ds(c1, 128)], tb[pl.ds(16 * k, 16), pl.ds(c2, 128)],
                                 h[:, c1:c1 + 128], h[:, c2:c2 + 128])
            for c, v in enumerate(combos):
                last = pltpu.bitcast(v.astype(BF16), F32)
                hn[pl.ds(base + 64 * (c // 2) + 8 * k, 8), pl.ds(512 * (c % 2) + t * 128, 128)] = last
        return pltpu.bitcast(last, U32)

    def rhs1_loc(cc, n, r):
        return 3 * n + cc // 2, 256 * (cc % 2) + r

    def rhs2_loc(cc, n, r):
        return 42 + 2 * (5 * n + cc) + r // 512, r % 512

    def rhs_job(w, kh, nh, n, loc, r):
        raw = [w[pl.ds(r + a * kh, 8), pl.ds(n * 128 + b * nh, 128)] for a in range(2) for b in range(2)]
        bits = None
        for cc, v in enumerate(_rhs_combos(*[_bf(v).astype(F32) for v in raw])):
            sl, row = loc(cc, n, r)
            wqkv[sl, pl.ds(row, 8), :] = pltpu.bitcast(v.astype(BF16), U32)
            b = pltpu.bitcast(v[8 * (cc % 2):8 * (cc % 2) + 8], U32)
            bits = b if bits is None else bits | b
        return bits

    def rhs1(c, n):
        if c == 1:
            return _bf(w1[pl.ds(0, D // 4), pl.ds(n * 128, 128)])
        if c == 4:
            return _bf(w1[pl.ds(D // 4, D // 4), pl.ds(FF // 2 + n * 128, 128)])
        sl, row = rhs1_loc(_RHS_IDX[c], n, 0)
        return _bf(wqkv[sl, pl.ds(row, D // 4), :])

    def rhs2(c, n):
        if c == 1:
            return _bf(w2[pl.ds(0, FF // 4), pl.ds(n * 128, 128)])
        if c == 4:
            return _bf(w2[pl.ds(FF // 4, FF // 4), pl.ds(D // 2 + n * 128, 128)])
        sl, _ = rhs2_loc(_RHS_IDX[c], n, 0)
        return _bf(jnp.concatenate([wqkv[sl], wqkv[sl + 1, pl.ds(0, FF // 4 - 512), :]], axis=0))

    def bulk_o(zero):
        jobs = ([functools.partial(mod_job, g, k) for g in range(8) for k in range(D // 16)]
                + [functools.partial(rhs_job, w1, D // 4, FF // 2, n, rhs1_loc, r)
                   for n in range(FF // 256) for r in range(0, D // 4, 8)]
                + [functools.partial(rhs_job, w2, FF // 4, D // 2, n, rhs2_loc, r)
                   for n in range(D // 256) for r in range(0, FF // 4, 8)])[::-1]
        state = dict(credit=-16.0, dep=None, piece=0)

        def tie(raw, density):
            parts = []
            for r in range(0, raw.shape[0], 8):
                v = raw[r:r + 8]
                state['credit'] += density
                if jobs and state['credit'] >= 1.0:
                    state['credit'] -= 1.0
                    v = v | (jobs.pop()() & zerob[...])
                parts.append(v)
            return jnp.concatenate(parts, axis=0)

        def a_blk(rh, kh):
            return jnp.concatenate([oring[h, pl.ds(rh * 256, 256), :]
                                    for h in range(16 * kh, 16 * kh + 16)], axis=1)

        lhs = [v.astype(BF16) for v in _lhs_combos(a_blk(0, 0), a_blk(0, 1), a_blk(1, 0), a_blk(1, 1))]
        for n in range(4):
            def prod(c):
                rhs = _rhs_operand(c, lambda a, b: wo[n + 4 * b, pl.ds(a * 1024, 1024), :],
                                   lambda raw: tie(raw, 0.56 if c in (1, 4) else 0.34))
                return _dot(lhs[c], rhs)

            def side():
                if n >= 2:
                    for _ in range(2):
                        state['dep'] = ln2_piece(zero, 0, state['piece'], state['dep'])
                        state['piece'] += 1

            def finish(y, rh, ch):
                ha[pl.ds(NSEG * TOK + rh * 256, 256), pl.ds((n + 4 * ch) * 128, 128)] = y

            _strassen(prod, finish, side)
        assert not jobs

    qka[16, pl.ds(0, 8), :] = jnp.zeros((8, E), F32)
    with jax.named_scope("p3_bulk_o"):
        bulk_o(zero_s[0])

    out32 = out_hbm.bitcast(F32)

    def ffn(i, carry):
        base = pl.multiple_of(lax.rem(i, 2) * 256, 256)
        nbase = pl.multiple_of(lax.rem(i + 1, 2) * 256, 256)
        nxt = lax.rem(i + 1, nb)
        half = i // 4
        srow = pl.multiple_of(lax.rem(i, 4) * HB, HB)

        def gelu(v):
            return jax.nn.gelu(v, approximate=True)

        g = [[] for _ in range(7)]
        for n in range(FF // 256):
            m = [None] * 7
            for c in (1, 3, 2, 4, 0, 5, 6):
                lhs = _bf(hn[pl.ds(base + 64 * (c // 2), 64), pl.ds(512 * (c % 2), 512)])
                m[c] = _dot(lhs, rhs1(c, n))
            b1a = rep(biasb[:, pl.ds(n * 128, 128)], HB)
            b1b = rep(biasb[:, pl.ds(FF // 2 + n * 128, 128)], HB)
            combos = _lhs_combos(gelu((m[3] - m[4]) + m[0] + m[6] + b1a), gelu(m[2] + m[4] + b1b),
                                 gelu(m[1] + m[3] + b1a), gelu((m[2] - m[1]) + m[0] + m[5] + b1b))
            for c, v in enumerate(combos):
                g[c].append(v.astype(BF16))
        g = [jnp.concatenate(v, axis=1) for v in g]

        state = dict(dep=None, piece=0)

        def ln_next():
            pin = pltpu.bitcast(qka[16, pl.ds(0, 8), :], U32)
            dep = pin if state['dep'] is None else state['dep'] | pin
            state['dep'] = ln2_piece(nxt, nbase, state['piece'], dep)
            state['piece'] += 1

        def finish(y, rh, nn):
            cols = pl.ds(nn * 128, 128)
            y = y + rep(biasb[:, pl.ds(FF + nn * 128, 128)], HB)
            xr = pl.ds(pl.multiple_of(i * HB, HB) + rh * (HB // 2), HB // 2)
            ar = pl.ds(pl.multiple_of(i * FB, FB) + rh * HB, HB)
            x2 = _bf(xs[xr, cols]).astype(F32) + rep(modb[0, :, cols], HB) * ha[ar, cols]
            qka[2 * nn + half, pl.ds(srow + rh * (HB // 2), HB // 2), :] = pltpu.bitcast(
                (x2 + rep(modb[3, :, cols], HB) * y).astype(BF16), F32)

        def copy_out(nn):
            pltpu.make_async_copy(qka.at[2 * nn + half, pl.ds(srow, HB), :],
                                  out32.at[pl.ds(pl.multiple_of(i * HB, HB), HB), pl.ds(nn * 128, 128)],
                                  sem.at[SEM_OUT]).start()

        for n in range(D // 256):
            def finish_n(y, rh, ch):
                finish(y, rh, n + 4 * ch)
                if rh == ch:
                    copy_out(n + 4 * ch)

            _strassen(lambda c: _dot(g[c], rhs2(c, n)), finish_n, ln_next)
        return carry

    with jax.named_scope("p4_ffn"):
        lax.fori_loop(0, nb, ffn, 0)
    pltpu.make_async_copy(out32, out32, sem.at[SEM_OUT]).wait()


@jax.jit
def pallas_adaLN_cond__memory_aug_recurrent_mem_tr__dense_activation_gelu__prompt_kernel(
    A_x, A_mem0, A_Wq, A_Wk, A_Wv, A_Wo, A_seg_len, B_x, B_w1, B_b1, B_w2, B_b2, c, w_mod,
):
    assert A_x.shape == (1, S, D) and A_Wq.shape == (D, H, E) and A_mem0.shape == (1, M, D)
    any_spec = pl.BlockSpec(memory_space=pl.ANY)
    out = pl.pallas_call(
        _kernel,
        out_shape=jax.ShapeDtypeStruct((S, D), BF16),
        in_specs=[any_spec] * 12,
        out_specs=any_spec,
        scratch_shapes=[
            pltpu.VMEM((S // 2, D), U32),
            pltpu.VMEM((96, D // 2, E), U32),
            pltpu.VMEM((8, H * E // 2, 128), U32),
            pltpu.VMEM((D // 2, FF), U32),
            pltpu.VMEM((FF // 2, D), U32),
            pltpu.VMEM((8, D // 2, 512), U32),
            pltpu.VMEM((H, RING, E), F32),
            pltpu.VMEM((H, RING, E), F32),
            pltpu.VMEM((H + 1, RING, E), F32),
            pltpu.VMEM((H, RING, E), F32),
            pltpu.VMEM((S, D), F32),
            pltpu.VMEM((S - PRE, D), F32),
            pltpu.VMEM((7, NQ, PRE // 4, 128), U32),
            pltpu.VMEM((M, D), F32),
            pltpu.VMEM((NQ, 2, 8, KQ), F32),
            pltpu.VMEM((4, 8, D), F32),
            pltpu.VMEM((8, D), U32),
            pltpu.VMEM((8, FF + D), F32),
            pltpu.VMEM((80, 128), F32),
            pltpu.VMEM((8, 32, 128), F32),
            pltpu.VMEM((8, 128), U32),
            pltpu.VMEM((D // 2, 128), U32),
            pltpu.VMEM((FB // 2, D), F32),
            pltpu.SMEM((1,), jnp.int32),
            pltpu.VMEM((M, D), BF16),
            pltpu.VMEM((FF,), BF16),
            pltpu.VMEM((D,), BF16),
            pltpu.VMEM((1, D), BF16),
            pltpu.SemaphoreType.DMA((NSEM,)),
        ],
        compiler_params=pltpu.CompilerParams(vmem_limit_bytes=127 * 1024 * 1024, disable_bounds_checks=True,
                                             disable_semaphore_checks=True),
    )(
        A_x.reshape(S, D), A_mem0.reshape(M, D),
        A_Wq.reshape(D // 2, 2, H, E), A_Wk.reshape(D // 2, 2, H, E), A_Wv.reshape(D // 2, 2, H, E),
        A_Wo.reshape(H * E, D), B_w1, B_b1, B_w2, B_b2, c, w_mod,
    )
    return out.reshape(1, S, D)
```

```python
import functools
import math

import jax
import jax.numpy as jnp
from jax import lax
import jax.experimental.pallas as pl
import jax.experimental.pallas.tpu as pltpu

F32 = jnp.float32
BF16 = jnp.bfloat16
U32 = jnp.uint32

S = 2048
D = 1024
H = 32
E = 128
M = 8
SEG = 32
NSEG = S // SEG
FF = 3584
NP = H // 2
TOK = 24
PRE = S - NSEG * TOK
RING = 576
OOFF = (-NSEG * TOK) % RING
LN_EPS = 1e-5
FB = 256
XC = (S - PRE) // 6
P3_DENSITY = 0.223
LN_PLAN = (1, 1, 1, 1, 1, 1, 1, 2, 2, 2, 2, 1, 0, 0)
UNROLL = 4

NQ = 4
KQ = D // NQ

FIRST_STARTS = [('m', 0), ('w', 0, 0, 2), ('w', 0, 2, 6), ('w', 0, 6, 12), ('m', 1), ('w', 1, 0, 6),
                ('w', 1, 6, 12), ('m', 2)]
P1A_BLOCKS = [
    ([], [('m', 0)]),
    ([], [('w', 0, 0, 2)]),
    ([], [('w', 0, 2, 6)]),
    ([('w', 2, 0, 6), ('w', 2, 6, 12)], [('w', 0, 6, 12)]),
    ([('m', 3), ('w', 3, 0, 6), ('w', 3, 6, 12)], [('m', 1), ('w', 1, 0, 6)]),
    ([], [('m', 2), ('w', 1, 6, 12)]),
    ([('g', 2), ('g', 3)], [('w', 2, 0, 6), ('w', 2, 6, 12)]),
    ([('g', 4), ('g', 5)], [('m', 3), ('w', 3, 0, 6), ('w', 3, 6, 12)]),
]
W_ITEMS = [it for _, items in P1A_BLOCKS for it in items if it[0] == 'w']
NX0 = 4

SEM_C = 0
SEM_X0 = 1
SEM_MOD = SEM_X0 + NX0
SEM_WA = SEM_MOD + NQ + 1
SEM_WB = SEM_WA + len(W_ITEMS)
SEM_XC = SEM_WB + 6
SEM_WO = SEM_XC + 6
SEM_W1 = SEM_WO + 1
SEM_W2 = SEM_W1 + 1
SEM_OUT = SEM_W2 + 1
NSEM = SEM_OUT + 1


def _ln(x):
    m = jnp.mean(x, axis=-1, keepdims=True)
    xc = x - m
    v = jnp.mean(xc * xc, axis=-1, keepdims=True)
    return xc * lax.rsqrt(v + LN_EPS)


def _bf(w32):
    return pltpu.bitcast(w32, BF16)


def _dot(a, b):
    return jnp.dot(a, b, preferred_element_type=F32)


def _lhs_combos(a11, a12, a21, a22):
    return [a11 + a22, a21 + a22, a11, a22, a11 + a12, a21 - a11, a12 - a22]


def _rhs_combos(b11, b12, b21, b22):
    return [b11 + b22, b11, b12 - b22, b21 - b11, b22, b11 + b12, b21 + b22]


_LHS_TERMS = {0: ((0, 0), (1, 1), 1), 1: ((1, 0), (1, 1), 1), 2: ((0, 0), None, 0), 3: ((1, 1), None, 0),
              4: ((0, 0), (0, 1), 1), 5: ((1, 0), (0, 0), -1), 6: ((0, 1), (1, 1), -1)}
_RHS_TERMS = {0: ((0, 0), (1, 1), 1), 1: ((0, 0), None, 0), 2: ((0, 1), (1, 1), -1), 3: ((1, 0), (0, 0), -1),
              4: ((1, 1), None, 0), 5: ((0, 0), (0, 1), 1), 6: ((1, 0), (1, 1), 1)}


def _combo(terms, c, blk):
    p, q, sign = terms[c]
    if q is None:
        return blk(*p)
    return blk(*p) + blk(*q) if sign > 0 else blk(*p) - blk(*q)


def _rhs_operand(c, blk, wrap=lambda raw: raw):
    p, q, sign = _RHS_TERMS[c]
    a = _bf(wrap(blk(*p)))
    if q is None:
        return a
    a = a.astype(F32)
    b = _bf(blk(*q)).astype(F32)
    return (a + b if sign > 0 else a - b).astype(BF16)


def _strassen(prod, finish, side=lambda: None):
    side()
    m1 = prod(1)
    m3 = prod(3)
    finish(m1 + m3, 1, 0)
    side()
    m2 = prod(2)
    m4 = prod(4)
    finish(m2 + m4, 0, 1)
    side()
    m0 = prod(0)
    m5 = prod(5)
    finish((m2 - m1) + m0 + m5, 1, 1)
    side()
    m6 = prod(6)
    finish((m3 - m4) + m0 + m6, 0, 0)


def _strassen_value(prod):
    r = {}
    _strassen(prod, lambda y, rh, ch: r.__setitem__((rh, ch), y))
    return jnp.concatenate([jnp.concatenate([r[0, 0], r[0, 1]], axis=1),
                            jnp.concatenate([r[1, 0], r[1, 1]], axis=1)], axis=0)


_PAIRS = [(c, d) for c in range(7) for d in range(7) if not (c in (1, 4) and d in (1, 4))]


def _kernel(x_hbm, mem0_hbm, wq_hbm, wk_hbm, wv_hbm, wo_hbm, w1_hbm, b1_hbm, w2_hbm, b2_hbm,
            c_hbm, wmod_hbm, out_hbm,
            xs, wqkv, wo, w1, w2, qka, qkb, vring, oring, ha, hn, memb, moda, modb, scb, biasb,
            fillb, accb, zerob, pk0, pk1, pk2, pk3, mem0_ref, b1_ref, b2_ref, c_ref, sem):
    qkv_hbm = [r.bitcast(U32) for r in (wq_hbm, wk_hbm, wv_hbm)]
    x32 = x_hbm.bitcast(U32)
    wo32 = wo_hbm.bitcast(U32)
    wmod32 = wmod_hbm.bitcast(F32)

    def wma(qq, k):
        return pl.ds(512 * (qq // 2), 512), pl.ds(512 * (qq % 2) + k * KQ, KQ)

    def hb_idx(c, q0, nq, row0=0, nrows=PRE // 4):
        return pl.ds(1024 + 128 * (c // 2) + row0, nrows), pl.ds(512 * (c % 2) + 128 * q0, 128 * nq)

    def units_start(lo, hi, rows, sem_idx):
        for u in range(lo, hi):
            j, m = u // 3, u % 3
            for p in range(2):
                pltpu.make_async_copy(qkv_hbm[m].at[rows, p, j, :], wqkv.at[2 * u + p, rows, :],
                                      sem.at[sem_idx]).start()

    def units_wait(lo, n, rows, sem_idx):
        blk = wqkv.at[pl.ds(2 * lo, 2 * n), rows, :]
        pltpu.make_async_copy(blk, blk, sem.at[sem_idx]).wait()

    def item_start(item):
        if item[0] == 'm':
            qq = item[1]
            for k in range(2):
                pltpu.make_async_copy(wmod32.at[:, pl.ds(k * D + qq * KQ, KQ)], ha.at[wma(qq, k)],
                                      sem.at[SEM_MOD + qq]).start()
        elif item[0] == 'w':
            _, qq, lo, hi = item
            units_start(lo, hi, pl.ds(qq * (KQ // 2), KQ // 2), SEM_WA + W_ITEMS.index(item))
        else:
            whole_start(item[1])

    def item_wait(item):
        if item[0] == 'm':
            qq = item[1]
            blk = ha.at[pl.ds(512 * (qq // 2), 512), pl.ds(512 * (qq % 2), 512)]
            pltpu.make_async_copy(blk, blk, sem.at[SEM_MOD + qq]).wait()
        else:
            _, qq, lo, hi = item
            units_wait(lo, hi - lo, pl.ds(qq * (KQ // 2), KQ // 2), SEM_WA + W_ITEMS.index(item))

    def whole_start(i):
        xc_copy(i - 2).start()
        units_start(6 * i, 6 * i + 6, pl.ds(0, D // 2), SEM_WB + i - 2)

    def mod_copy(n):
        return pltpu.make_async_copy(wmod32.at[:, pl.ds(2 * D + n * 128, 128)],
                                     qka.at[n, pl.ds(0, D // 2), :], sem.at[SEM_MOD + NQ])

    def x0_copy(i):
        n = PRE // 2 // NX0
        rows = pl.ds(pl.multiple_of(i * n, n), n)
        return pltpu.make_async_copy(x32.at[rows], xs.at[rows], sem.at[SEM_X0 + i])

    def xc_copy(i):
        rows = pl.ds(pl.multiple_of(PRE // 2 + i * (XC // 2), 64), XC // 2)
        return pltpu.make_async_copy(x32.at[rows], xs.at[rows], sem.at[SEM_XC + i])

    def wo_copy(n):
        return pltpu.make_async_copy(wo32.at[:, pl.ds(n * 128, 128)], wo.at[n], sem.at[SEM_WO])

    w1_copy = pltpu.make_async_copy(w1_hbm.bitcast(U32), w1, sem.at[SEM_W1])
    w2_copy = pltpu.make_async_copy(w2_hbm.bitcast(U32), w2, sem.at[SEM_W2])
    small_copies = [pltpu.make_async_copy(a, b, sem.at[SEM_C])
                    for a, b in ((c_hbm, c_ref), (mem0_hbm, mem0_ref), (b1_hbm, b1_ref),
                                 (b2_hbm, b2_ref))]

    def deinterleave(u, row0, nrows):
        for k in range(nrows // 64):
            rows = pl.ds(row0 + k * 64, 64)
            a = wqkv[2 * u, rows, :]
            b = wqkv[2 * u + 1, rows, :]
            wqkv[2 * u, rows, :] = (a & jnp.uint32(0xFFFF)) | (b << 16)
            wqkv[2 * u + 1, rows, :] = (a >> 16) | (b & jnp.uint32(0xFFFF0000))

    def load_x16(row2, dep):
        xw = xs[pl.ds(row2, 8), :]
        if dep is not None:
            first = xw[:, 0:128] | (dep & zerob[...])
            xw = jnp.concatenate([first, xw[:, 128:]], axis=1)
        return _bf(xw).astype(F32)

    pks = [pk0, pk1, pk2, pk3]

    def pack(v, dtype=U32):
        rows = pl.ds(0, v.shape[0] // 2)
        pk = pks[0]
        pk[rows, pl.ds(0, 128)] = pltpu.bitcast(v.astype(BF16), U32)
        return pltpu.bitcast(pk[rows, pl.ds(0, 128)], dtype)

    def rep(v8, n):
        return jnp.concatenate([v8] * (n // 8), axis=0)

    def mrow(k, n):
        if k < 2:
            return rep(jnp.concatenate([moda[qq, k] for qq in range(NQ)], axis=1), n)
        return rep(modb[k - 2], n)

    for cp in small_copies:
        cp.start()
    for i in range(NX0):
        x0_copy(i).start()
    for item in FIRST_STARTS:
        item_start(item)

    def start_rest():
        for n in range(8):
            wo_copy(n).start()
        w1_copy.start()
        w2_copy.start()

    r = lax.broadcasted_iota(jnp.int32, (80, 128), 0)
    q = lax.broadcasted_iota(jnp.int32, (80, 128), 1)
    r_tok = r < 64
    q_tok = q < 64
    r_head = jnp.where(r_tok, r >> 5, (r - 64) >> 3)
    q_head = jnp.where(q_tok, q >> 5, (q - 64) >> 3)
    same = (r_head == q_head) & (q < 80)
    causal_ok = jnp.logical_not(r_tok & q_tok & ((q & 31) > (r & 31)))
    scale = E ** (-0.5)
    fillb[...] = jnp.where(same, jnp.where(causal_ok, 0.0, -1e9 / scale), -jnp.inf).astype(F32)
    zerob[...] = jnp.zeros((8, 128), U32)

    for cp in small_copies:
        cp.wait()
    cf = c_ref[...].astype(F32)
    sc = (cf * jax.nn.sigmoid(cf)).astype(BF16)
    scb[...] = pltpu.bitcast(jnp.broadcast_to(sc, (16, D)), U32)
    memb[...] = mem0_ref[...].astype(F32)
    biasb[:, pl.ds(0, FF)] = jnp.broadcast_to(b1_ref[...].astype(F32).reshape(1, FF), (8, FF))
    biasb[:, pl.ds(FF, D)] = jnp.broadcast_to(b2_ref[...].astype(F32).reshape(1, D), (8, D))

    def pre_norm(i, carry):
        x0_copy(i).wait()
        nr = PRE // NX0
        for z in range(nr // 16):
            xn = _ln(load_x16(pl.multiple_of(i * (nr // 2) + z * 8, 8), None))
            for n in range(8):
                oring[n, pl.ds(pl.multiple_of(i * nr + z * 16, 16), 16), :] = xn[:, n * 128:(n + 1) * 128]
        return carry

    with jax.named_scope("p0_ln"):
        lax.fori_loop(0, NX0, pre_norm, 0)

    def dst_slot(i, k, p):
        cls, m = k // 3, k % 3
        if m == 2:
            return vring, 4 * i + 2 * cls + p
        return (qka, qkb)[cls], 4 * i + 2 * m + p

    PH = PRE // 2
    assert KQ == 256

    def item_run(item):
        if item[0] == 'm':
            qq = item[1]
            sc16 = _bf(scb[...])
            ca1 = 1.0 + _dot(sc16, _bf(ha[wma(qq, 1)]))[0:8].astype(BF16).astype(F32)
            sa = _dot(sc16, _bf(ha[wma(qq, 0)]))[0:8].astype(BF16).astype(F32)
            moda[qq, 0] = sa
            moda[qq, 1] = ca1
            for z in range(PH // 32):
                def h_blk(rh, kh):
                    cols = slice(kh * 128, (kh + 1) * 128)
                    return (oring[2 * qq + kh, pl.ds(rh * PH + z * 32, 32), :] * rep(ca1[:, cols], 32)
                            + rep(sa[:, cols], 32))

                for c, v in enumerate(_lhs_combos(h_blk(0, 0), h_blk(0, 1), h_blk(1, 0), h_blk(1, 1))):
                    ha[hb_idx(c, qq, 1, z * 16, 16)] = pltpu.bitcast(v.astype(BF16), F32)
            return
        _, qq, lo, hi = item
        for u in range(lo, hi):
            deinterleave(u, qq * (KQ // 2), KQ // 2)
            unit_proj(u // 6, u % 6, [qq], qq > 0)

    def unit_proj(i, k, slices, accumulate, side=lambda: None):
        u = 6 * i + k

        def prod(c):
            lhs = _bf(ha[hb_idx(c, slices[0], len(slices))])
            rhs = _rhs_operand(c, lambda a, b: jnp.concatenate(
                [wqkv[2 * u + b, pl.ds((2 * qq + a) * 64, 64), :] for qq in slices], axis=0))
            return _dot(lhs, rhs)

        def finish(y, rh, ch):
            ref, idx = dst_slot(i, k, ch)
            rows = pl.ds(RING - PRE + rh * PH, PH)
            if accumulate:
                y = y + ref[idx, rows, :]
            ref[idx, rows, :] = y

        _strassen(prod, finish, side)

    def phase1b(i, carry):
        @pl.when(i == 3)
        def _():
            whole_start(6)
            whole_start(7)

        @pl.when(i == 4)
        def _():
            start_rest()

        xc_copy(i - 2).wait()
        units_wait(6 * i, 6, pl.ds(0, D // 2), SEM_WB + i - 2)
        deinterleave(6 * i, 0, D // 2)
        state = dict(dep=None, piece=0, slot=0)

        def side():
            state['slot'] += 1
            if state['slot'] % 4 != 0 and state['piece'] < XC // 16:
                off = state['piece'] * 16
                x16 = load_x16(pl.multiple_of((i - 2) * (XC // 2), XC // 2) + (PRE + off) // 2, state['dep'])
                h16 = _ln(x16) * mrow(1, 16) + mrow(0, 16)
                hn[pl.ds(pl.multiple_of((i - 2) * XC, XC) + off, 16), :] = h16
                state['dep'] = pltpu.bitcast(h16[8:16, D - 128:], U32)
                state['piece'] += 1

        for k in range(6):
            if k < 5:
                deinterleave(6 * i + k + 1, 0, D // 2)
            unit_proj(i, k, list(range(NQ)), False, side)
        return carry

    for bi, (starts, items) in enumerate(P1A_BLOCKS):
        for item in starts:
            item_start(item)
        with jax.named_scope("p1a_wait%d" % bi):
            for item in items:
                item_wait(item)
        for item in items:
            item_run(item)
    with jax.named_scope("p1b"):
        lax.fori_loop(2, 8, phase1b, 0)
    for n in range(8):
        wo_copy(n).wait()

    cexp = scale * math.log2(math.e)
    NG = NP // 2
    grp = [(4 * (g // 2) + (g % 2), 4 * (g // 2) + (g % 2) + 2) for g in range(NG)]
    early = [2 * j + u for g in range(NG - 3) for j in grp[g] for u in range(2)]
    late = [h for h in range(H) if h not in early]

    def step(it, k):
        s = it * UNROLL + k
        split = k > 0
        base = TOK * UNROLL * it
        w0 = pl.multiple_of(lax.rem(base, RING), 32) + TOK * k
        r0 = pl.multiple_of(lax.rem(SEG * s + (RING - PRE), RING), 32)
        ow = pl.multiple_of(lax.rem(SEG * s + OOFF, RING), 32)
        o0 = pl.multiple_of(lax.rem(base + OOFF, RING), 32) + TOK * k
        a0 = pl.multiple_of(base, 32) + TOK * k
        X = jnp.concatenate([hn[pl.ds(a0, TOK), :], memb[...]], axis=0).astype(BF16)
        ym = [None] * 96
        probs = [None] * NP
        om = [None] * H
        order = (4, 5, 0, 1, 2, 3)

        if split:
            for t in order:
                accb[t] = _dot(X[:, :D // 2], _bf(wqkv[t, pl.ds(0, D // 4), :]))

        def slot(j, t):
            if t >= 4:
                return vring, 2 * j + t - 4
            return (qka, qkb)[j % 2], 4 * (j // 2) + t

        def proj(j, t):
            c = 6 * j + t
            if split and j == 0:
                y = accb[t] + _dot(X[:, D // 2:], _bf(wqkv[c, pl.ds(D // 4, D // 4), :]))
            else:
                y = _dot(X, _bf(wqkv[c]))
            ref, k = slot(j, t)
            ref[k, pl.ds(w0, TOK), :] = y[0:TOK]
            ym[c] = y[TOK:TOK + M]

        def gather(j, m, pad):
            c = 6 * j + 2 * m
            ref, k = slot(j, 2 * m)
            parts = [ref[k, pl.ds(r0, SEG), :], ref[k + 1, pl.ds(r0, SEG), :], ym[c], ym[c + 1]]
            if pad:
                parts.append(jnp.zeros((48, E), F32))
            return jnp.concatenate(parts, axis=0).astype(BF16)

        def scores(j):
            sc_ = lax.dot_general(gather(j, 0, False), gather(j, 1, True),
                                  (((1,), (1,)), ((), ())), preferred_element_type=F32)
            fill = fillb[...]
            sc_ = jnp.where(fill == 0.0, sc_, fill)
            mx = jnp.max(sc_, axis=-1, keepdims=True)
            p = jnp.exp2((sc_ - mx) * cexp)
            l = jnp.sum(p, axis=-1, keepdims=True)
            rl = pl.reciprocal(l, approx=True)
            rl = rl * (2.0 - l * rl)
            probs[j] = p * rl

        def park(j):
            vring[H, pl.ds(40 * (j % 8), 40), :] = pack(probs[j], F32)
            probs[j] = None

        def pv(j):
            if probs[j] is None:
                P = _bf(vring[H, pl.ds(40 * (j % 8), 40), :])
            else:
                P = probs[j].astype(BF16)
            o = _dot(P, gather(j, 2, True))
            oring[2 * j, pl.ds(ow, SEG), :] = o[0:32]
            oring[2 * j + 1, pl.ds(ow, SEG), :] = o[32:64]
            om[2 * j] = o[64:72]
            om[2 * j + 1] = o[72:80]

        def o_lhs(hs):
            return jnp.concatenate(
                [jnp.concatenate([oring[h, pl.ds(o0, TOK), :], om[h]], axis=0) for h in hs],
                axis=1).astype(BF16)

        def o_rhs(n, hs):
            return _bf(jnp.concatenate([wo[n, pl.ds(h * 64, 64), :] for h in hs], axis=0))

        for g in range(NG):
            cols = [(j, t) for j in grp[g] for t in order]
            if g == 2:
                cols = ([(j, t) for j in grp[g] for t in (4, 5)]
                        + [(j, t) for j in grp[g] for t in range(4)])
            for j in (grp[0] + grp[1] if g == 3 else grp[g - 2] if g >= 4 else ()):
                park(j)
            for ci, (j, t) in enumerate(cols):
                if g == 2 and ci == 4:
                    for jj in grp[0] + grp[1]:
                        scores(jj)
                if g >= 3 and ci == 6:
                    for jj in grp[g - 1]:
                        scores(jj)
                    for jj in grp[g - 3]:
                        pv(jj)
                proj(j, t)
        lo = o_lhs(early)
        for n in range(8):
            accb[n] = _dot(lo, o_rhs(n, early))
            if n == 1:
                for jj in grp[NG - 1]:
                    scores(jj)
                for jj in grp[NG - 3]:
                    pv(jj)
            if n == 4:
                for jj in grp[NG - 2] + grp[NG - 1]:
                    pv(jj)
        lo = o_lhs(late)
        for n in range(8):
            a = accb[n] + _dot(lo, o_rhs(n, late))
            ha[pl.ds(a0, TOK), pl.ds(n * 128, 128)] = a[0:TOK]
            memb[:, pl.ds(n * 128, 128)] = a[TOK:TOK + M]

    def steps(i, carry):
        for k in range(UNROLL):
            step(i, k)
        return carry

    with jax.named_scope("p2_steps"):
        lax.fori_loop(0, NSEG // UNROLL, steps, 0)

    for n in range(H):
        mod_copy(n).start()
    w1_copy.wait()
    w2_copy.wait()

    nb = S // FB
    HB = FB // 2
    QB = FB // 4

    def ln2_piece(blk, off, dep):
        x2 = (load_x16(pl.multiple_of(blk * HB + off // 2, 8), dep)
              + mrow(2, 16) * ha[pl.ds(pl.multiple_of(blk * FB + off, 16), 16), :])
        h = _ln(x2) * mrow(4, 16) + mrow(3, 16)
        for n in range(8):
            oring[n, pl.ds(pl.multiple_of(off, 16), 16), :] = h[:, n * 128:(n + 1) * 128]
        return pltpu.bitcast(h[8:16, D - 128:], U32)

    def lhs1_loc(base, c, d):
        e = 7 * c + d
        return base + 32 * (e // 4), 256 * (e % 4)

    def lhs1_job(base, k, t, c):
        def sub(ri, ki):
            return _combo(_LHS_TERMS, c, lambda ro, ko: oring[
                (2 * ko + ki) * 2 + t, pl.ds(pl.multiple_of((2 * ro + ri) * QB + 16 * k, 16), 16), :])

        bits = None
        for d, v in enumerate(_lhs_combos(sub(0, 0), sub(0, 1), sub(1, 0), sub(1, 1))):
            r0, c0 = lhs1_loc(base, c, d)
            hn[pl.ds(pl.multiple_of(r0 + 8 * k, 8), 8), pl.ds(c0 + t * 128, 128)] = pltpu.bitcast(
                v.astype(BF16), F32)
            if d not in (2, 3):
                b = pltpu.bitcast(v[8 * (d % 2):8 * (d % 2) + 8], U32)
                bits = b if bits is None else bits | b
        return bits

    K1, N1, K2, N2 = D // 8, FF // 4, FF // 8, D // 4

    def rhs1_loc(c, d, n):
        e = _PAIRS.index((c, d)) * 7 + n
        return wqkv, e // 4, K1 * (e % 4)

    rhs2_slots = ([(wo, e // 4, K2 * (e % 4)) for e in range(32)] + [(wqkv, e, 0) for e in range(79, 96)]
                  + [(qkb, e, 0) for e in range(H)] + [(vring, e, 0) for e in range(9)])

    def rhs2_loc(c, d, n):
        return rhs2_slots[_PAIRS.index((c, d)) * 2 + n]

    def rhs_job(w, kq, nq, loc, n, r, cs):
        cache = {}

        def blk(ko, no, ki, ni):
            key = (2 * ko + ki, 2 * no + ni)
            if key not in cache:
                cache[key] = _bf(w[pl.ds(r + key[0] * kq, 8), pl.ds(n * 128 + key[1] * nq, 128)]).astype(F32)
            return cache[key]

        bits = None
        for c in cs:
            def sub(ki, ni):
                return _combo(_RHS_TERMS, c, lambda ko, no: blk(ko, no, ki, ni))

            for d, v in enumerate(_rhs_combos(sub(0, 0), sub(0, 1), sub(1, 0), sub(1, 1))):
                if (c, d) in _PAIRS:
                    ref, idx, row = loc(c, d, n)
                    b = pack(v)
                    ref[idx, pl.ds(row + r, 8), :] = pltpu.bitcast(b, ref.dtype)
                    bits = b if bits is None else bits | b
        return bits

    def rhs_load(w, kq, nq, loc, c, d, n):
        if (c, d) not in _PAIRS:
            q = 2 * (c // 4) + d // 4
            return w[pl.ds(q * kq, kq), pl.ds(q * nq + n * 128, 128)]
        ref, idx, row = loc(c, d, n)
        return pltpu.bitcast(ref[idx, pl.ds(row, kq), :], U32)

    def make_tie(jobs, credit):
        state = [credit]

        def tie(raw, density):
            if not jobs:
                return raw
            parts = []
            for r in range(0, raw.shape[0], 8):
                v = raw[r:r + 8]
                state[0] += density
                if jobs and state[0] >= 1.0:
                    state[0] -= 1.0
                    v = v | (jobs.pop(0)() & zerob[...])
                parts.append(v)
            return jnp.concatenate(parts, axis=0)

        return tie

    def bulk_o():
        jobs = [functools.partial(rhs_job, w1, K1, N1, rhs1_loc, n, r, [c])
                for c in range(7) for n in range(7) for r in range(0, K1, 8)]
        tie = make_tie(jobs, -4.0)

        def a_blk(rh, kh):
            return jnp.concatenate([oring[h, pl.ds(rh * 256, 256), :]
                                    for h in range(16 * kh, 16 * kh + 16)], axis=1)

        lhs = [v.astype(BF16) for v in _lhs_combos(a_blk(0, 0), a_blk(0, 1), a_blk(1, 0), a_blk(1, 1))]
        for n in range(4):
            def prod(c):
                rhs = _rhs_operand(c, lambda a, b: wo[n + 4 * b, pl.ds(a * 1024, 1024), :],
                                   lambda raw: tie(raw, P3_DENSITY))
                return _dot(lhs[c], rhs)

            def finish(y, rh, ch):
                ha[pl.ds(NSEG * TOK + rh * 256, 256), pl.ds((n + 4 * ch) * 128, 128)] = y

            _strassen(prod, finish)
        assert not jobs

    pks.pop(0)
    with jax.named_scope("p3_bulk_o"):
        bulk_o()
    pks.pop(0)
    for n in range(H):
        mod_copy(n).wait()

    def w2_rows(r0, count):
        for j in range(count):
            for n in range(2):
                rhs_job(w2, K2, N2, rhs2_loc, n, r0 + 8 * j, range(7))

    def prep_a(g, carry):
        for n in range(8):
            y = _dot(_bf(scb[...]), _bf(qka[8 * g + n, pl.ds(0, D // 2), :]))[0:8].astype(BF16).astype(F32)
            modb[g, :, pl.ds(n * 128, 128)] = y + jnp.where(g == 2, 1.0, 0.0)
        w2_rows(pl.multiple_of(g * 56, 8), 7)
        return carry

    def prep_b(k, carry):
        for r in range(4):
            ln2_piece(0, r * QB + 16 * k, None)
        w2_rows(pl.multiple_of(224 + k * 56, 8), 7)
        for t in range(2):
            for c in range(7):
                lhs1_job(0, k, t, c)
        return carry

    with jax.named_scope("p3_prep"):
        lax.fori_loop(0, 4, prep_a, 0)
        lax.fori_loop(0, 4, prep_b, 0)

    pks.pop(0)
    out32 = out_hbm.bitcast(F32)
    qka[16, pl.ds(0, 8), :] = jnp.zeros((8, E), F32)

    def ffn(i, carry):
        base = pl.multiple_of((i & 1) * 512, 512)
        nbase = pl.multiple_of(((i + 1) & 1) * 512, 512)
        nxt = (i + 1) & (nb - 1)
        half = i >> 2
        srow = pl.multiple_of((i & 3) * HB, HB)

        g = {(c, d): [] for c in range(7) for d in range(7)}
        for n in range(7):
            act = {}

            def prod1(c, d):
                r0, c0 = lhs1_loc(base, c, d)
                return _dot(_bf(hn[pl.ds(r0, QB // 2), pl.ds(c0, 256)]),
                            _bf(rhs_load(w1, K1, N1, rhs1_loc, c, d, n)))

            def activate(y, rh, ch):
                b1 = jnp.concatenate([biasb[:, pl.ds((2 * ch + ci) * N1 + n * 128, 128)] for ci in range(2)],
                                     axis=1)
                act[rh, ch] = jax.nn.gelu(y + rep(b1, HB), approximate=True)

            _strassen(lambda c: _strassen_value(functools.partial(prod1, c)), activate)
            for c in range(7):
                o = _combo(_LHS_TERMS, c, lambda a, b: act[a, b])
                for d, v in enumerate(_lhs_combos(o[:QB, :128], o[:QB, 128:], o[QB:, :128], o[QB:, 128:])):
                    g[c, d].append(v.astype(BF16))

        state = dict(dep=None, piece=0, window=0)
        jobs, pending = [], []
        tie = make_tie(jobs, 0.0)

        def next_block_ln():
            jobs.extend(pending)
            del pending[:]
            for _ in range(LN_PLAN[state['window']]):
                k, r = state['piece'] // 4, state['piece'] % 4
                pin = pltpu.bitcast(qka[16, pl.ds(0, 8), :], U32)
                dep = pin if state['dep'] is None else state['dep'] | pin
                state['dep'] = ln2_piece(nxt, r * QB + 16 * k, dep)
                if r == 3:
                    pending.extend(functools.partial(lhs1_job, nbase, k, t, c)
                                   for t in range(2) for c in range(7))
                state['piece'] += 1
            state['window'] += 1

        for n in range(2):
            def prod2(c, d):
                return _dot(jnp.concatenate(g[c, d], axis=1),
                            _bf(tie(rhs_load(w2, K2, N2, rhs2_loc, c, d, n), 1.0 / 24)))

            def outer(c):
                next_block_ln()
                y = _strassen_value(functools.partial(prod2, c))
                qka[17, pl.ds(srow, 8), :] = y[0:8, 0:128]
                return y

            def finish(y, rh, ch):
                for ci in range(2):
                    nn = (2 * ch + ci) * 2 + n
                    cols = pl.ds(nn * 128, 128)
                    yy = y[:, ci * 128:(ci + 1) * 128] + rep(biasb[:, pl.ds(FF + nn * 128, 128)], HB)
                    xr = pl.ds(pl.multiple_of(i * HB, HB) + rh * (HB // 2), HB // 2)
                    ar = pl.ds(pl.multiple_of(i * FB, FB) + rh * HB, HB)
                    x2 = _bf(xs[xr, cols]).astype(F32) + rep(modb[0, :, cols], HB) * ha[ar, cols]
                    qka[2 * nn + half, pl.ds(srow + rh * (HB // 2), HB // 2), :] = pack(
                        x2 + rep(modb[3, :, cols], HB) * yy, F32)
                    if rh == ch:
                        pltpu.make_async_copy(
                            qka.at[2 * nn + half, pl.ds(srow, HB), :],
                            out32.at[pl.ds(pl.multiple_of(i * HB, HB), HB), cols],
                            sem.at[SEM_OUT]).start()

            _strassen(outer, finish)
        assert not jobs and not pending and state['piece'] == 16
        return carry

    with jax.named_scope("p4_ffn"):
        lax.fori_loop(0, nb, ffn, 0)
    pltpu.make_async_copy(out32, out32, sem.at[SEM_OUT]).wait()


@jax.jit
def pallas_adaLN_cond__memory_aug_recurrent_mem_tr__dense_activation_gelu__prompt_kernel(
    A_x, A_mem0, A_Wq, A_Wk, A_Wv, A_Wo, A_seg_len, B_x, B_w1, B_b1, B_w2, B_b2, c, w_mod,
):
    assert A_x.shape == (1, S, D) and A_Wq.shape == (D, H, E) and A_mem0.shape == (1, M, D)
    any_spec = pl.BlockSpec(memory_space=pl.ANY)
    out = pl.pallas_call(
        _kernel,
        out_shape=jax.ShapeDtypeStruct((S, D), BF16),
        in_specs=[any_spec] * 12,
        out_specs=any_spec,
        scratch_shapes=[
            pltpu.VMEM((S // 2, D), U32),
            pltpu.VMEM((96, D // 2, E), U32),
            pltpu.VMEM((8, H * E // 2, 128), U32),
            pltpu.VMEM((D // 2, FF), U32),
            pltpu.VMEM((FF // 2, D), U32),
            pltpu.VMEM((H, RING, E), F32),
            pltpu.VMEM((H, RING, E), F32),
            pltpu.VMEM((H + 1, RING, E), F32),
            pltpu.VMEM((H, RING, E), F32),
            pltpu.VMEM((S, D), F32),
            pltpu.VMEM((S - PRE, D), F32),
            pltpu.VMEM((M, D), F32),
            pltpu.VMEM((NQ, 2, 8, KQ), F32),
            pltpu.VMEM((4, 8, D), F32),
            pltpu.VMEM((8, D), U32),
            pltpu.VMEM((8, FF + D), F32),
            pltpu.VMEM((80, 128), F32),
            pltpu.VMEM((8, 32, 128), F32),
            pltpu.VMEM((8, 128), U32),
            pltpu.VMEM((128, 256), U32),
            pltpu.VMEM((128, 256), U32),
            pltpu.VMEM((128, 256), U32),
            pltpu.VMEM((128, 256), U32),
            pltpu.VMEM((M, D), BF16),
            pltpu.VMEM((FF,), BF16),
            pltpu.VMEM((D,), BF16),
            pltpu.VMEM((1, D), BF16),
            pltpu.SemaphoreType.DMA((NSEM,)),
        ],
        compiler_params=pltpu.CompilerParams(vmem_limit_bytes=127 * 1024 * 1024, disable_bounds_checks=True,
                                             disable_semaphore_checks=True),
    )(
        A_x.reshape(S, D), A_mem0.reshape(M, D),
        A_Wq.reshape(D // 2, 2, H, E), A_Wk.reshape(D // 2, 2, H, E), A_Wv.reshape(D // 2, 2, H, E),
        A_Wo.reshape(H * E, D), B_w1, B_b1, B_w2, B_b2, c, w_mod,
    )
    return out.reshape(1, S, D)
```

```python
import functools
import math

import jax
import jax.numpy as jnp
from jax import lax
import jax.experimental.pallas as pl
import jax.experimental.pallas.tpu as pltpu

F32 = jnp.float32
BF16 = jnp.bfloat16
U32 = jnp.uint32

S = 2048
D = 1024
H = 32
E = 128
M = 8
SEG = 32
NSEG = S // SEG
FF = 3584
NP = H // 2
TOK = 24
PRE = S - NSEG * TOK
RING = 576
OOFF = (-NSEG * TOK) % RING
LN_EPS = 1e-5
FB = 256
XC = (S - PRE) // 6
P3_SPLIT = ((4, 10), (4, 16), (4, 14))
MOD_DENSITY = 0.07
LN0_PLAN = (3, 3, 3, 3, 2, 2, 0)
LN_PLAN = (1, 1, 1, 1, 1, 1, 1, 2, 2, 2, 2, 1, 0, 0)
UNROLL = 4

NQ = 4
KQ = D // NQ

FIRST_STARTS = [('m', 0), ('w', 0, 0, 2), ('w', 0, 2, 6), ('w', 0, 6, 12), ('m', 1), ('w', 1, 0, 6),
                ('w', 1, 6, 12), ('m', 2)]
P1A_BLOCKS = [
    ([], [('m', 0)]),
    ([], [('w', 0, 0, 2)]),
    ([], [('w', 0, 2, 6)]),
    ([('w', 2, 0, 6), ('w', 2, 6, 12)], [('w', 0, 6, 12)]),
    ([('m', 3), ('w', 3, 0, 6), ('w', 3, 6, 12)], [('m', 1), ('w', 1, 0, 6)]),
    ([], [('m', 2), ('w', 1, 6, 12)]),
    ([('g', 2), ('g', 3)], [('w', 2, 0, 6), ('w', 2, 6, 12)]),
    ([('g', 4), ('g', 5)], [('m', 3), ('w', 3, 0, 6), ('w', 3, 6, 12)]),
]
W_ITEMS = [it for _, items in P1A_BLOCKS for it in items if it[0] == 'w']
NX0 = 4

SEM_C = 0
SEM_X0 = 1
SEM_MOD = SEM_X0 + NX0
SEM_WA = SEM_MOD + NQ + 1
SEM_WB = SEM_WA + len(W_ITEMS)
SEM_XC = SEM_WB + 6
SEM_WO = SEM_XC + 6
SEM_W1 = SEM_WO + 1
SEM_W2 = SEM_W1 + 1
SEM_OUT = SEM_W2 + 1
NSEM = SEM_OUT + 1


def _ln(x):
    m = jnp.mean(x, axis=-1, keepdims=True)
    xc = x - m
    v = jnp.mean(xc * xc, axis=-1, keepdims=True)
    return xc * lax.rsqrt(v + LN_EPS)


def _bf(w32):
    return pltpu.bitcast(w32, BF16)


def _dot(a, b):
    return jnp.dot(a, b, preferred_element_type=F32)


def _lhs_combos(a11, a12, a21, a22):
    return [a11 + a22, a21 + a22, a11, a22, a11 + a12, a21 - a11, a12 - a22]


def _rhs_combos(b11, b12, b21, b22):
    return [b11 + b22, b11, b12 - b22, b21 - b11, b22, b11 + b12, b21 + b22]


_LHS_TERMS = {0: ((0, 0), (1, 1), 1), 1: ((1, 0), (1, 1), 1), 2: ((0, 0), None, 0), 3: ((1, 1), None, 0),
              4: ((0, 0), (0, 1), 1), 5: ((1, 0), (0, 0), -1), 6: ((0, 1), (1, 1), -1)}
_RHS_TERMS = {0: ((0, 0), (1, 1), 1), 1: ((0, 0), None, 0), 2: ((0, 1), (1, 1), -1), 3: ((1, 0), (0, 0), -1),
              4: ((1, 1), None, 0), 5: ((0, 0), (0, 1), 1), 6: ((1, 0), (1, 1), 1)}


def _combo(terms, c, blk):
    p, q, sign = terms[c]
    if q is None:
        return blk(*p)
    return blk(*p) + blk(*q) if sign > 0 else blk(*p) - blk(*q)


def _rhs_operand(c, blk):
    p, q, sign = _RHS_TERMS[c]
    a = _bf(blk(*p))
    if q is None:
        return a
    a = a.astype(F32)
    b = _bf(blk(*q)).astype(F32)
    return (a + b if sign > 0 else a - b).astype(BF16)


def _strassen(prod, finish, side=lambda: None):
    side()
    m1 = prod(1)
    m3 = prod(3)
    finish(m1 + m3, 1, 0)
    side()
    m2 = prod(2)
    m4 = prod(4)
    finish(m2 + m4, 0, 1)
    side()
    m0 = prod(0)
    m5 = prod(5)
    finish((m2 - m1) + m0 + m5, 1, 1)
    side()
    m6 = prod(6)
    finish((m3 - m4) + m0 + m6, 0, 0)


def _strassen_value(prod):
    r = {}
    _strassen(prod, lambda y, rh, ch: r.__setitem__((rh, ch), y))
    return jnp.concatenate([jnp.concatenate([r[0, 0], r[0, 1]], axis=1),
                            jnp.concatenate([r[1, 0], r[1, 1]], axis=1)], axis=0)


_PAIRS = [(c, d) for c in range(7) for d in range(7) if not (c in (1, 4) and d in (1, 4))]


def _kernel(x_hbm, mem0_hbm, wq_hbm, wk_hbm, wv_hbm, wo_hbm, w1_hbm, b1_hbm, w2_hbm, b2_hbm,
            c_hbm, wmod_hbm, out_hbm,
            xs, wqkv, wo, w1, w2, qka, qkb, vring, oring, ha, hn, memb, moda, modb, scb, biasb,
            fillb, accb, zerob, zero_s, wx, pk0, pk1, pk2, pk3, pk4, mem0_ref, b1_ref, b2_ref, c_ref, sem):
    qkv_hbm = [r.bitcast(U32) for r in (wq_hbm, wk_hbm, wv_hbm)]
    x32 = x_hbm.bitcast(U32)
    wo32 = wo_hbm.bitcast(U32)
    wmod32 = wmod_hbm.bitcast(F32)

    def wma(qq, k):
        return pl.ds(512 * (qq // 2), 512), pl.ds(512 * (qq % 2) + k * KQ, KQ)

    def hb_idx(c, q0, nq, row0=0, nrows=PRE // 4):
        return pl.ds(1024 + 128 * (c // 2) + row0, nrows), pl.ds(512 * (c % 2) + 128 * q0, 128 * nq)

    def units_start(lo, hi, rows, sem_idx):
        for u in range(lo, hi):
            j, m = u // 3, u % 3
            for p in range(2):
                pltpu.make_async_copy(qkv_hbm[m].at[rows, p, j, :], wqkv.at[2 * u + p, rows, :],
                                      sem.at[sem_idx]).start()

    def units_wait(lo, n, rows, sem_idx):
        blk = wqkv.at[pl.ds(2 * lo, 2 * n), rows, :]
        pltpu.make_async_copy(blk, blk, sem.at[sem_idx]).wait()

    def item_start(item):
        if item[0] == 'm':
            qq = item[1]
            for k in range(2):
                pltpu.make_async_copy(wmod32.at[:, pl.ds(k * D + qq * KQ, KQ)], ha.at[wma(qq, k)],
                                      sem.at[SEM_MOD + qq]).start()
        elif item[0] == 'w':
            _, qq, lo, hi = item
            units_start(lo, hi, pl.ds(qq * (KQ // 2), KQ // 2), SEM_WA + W_ITEMS.index(item))
        else:
            whole_start(item[1])

    def item_wait(item):
        if item[0] == 'm':
            qq = item[1]
            blk = ha.at[pl.ds(512 * (qq // 2), 512), pl.ds(512 * (qq % 2), 512)]
            pltpu.make_async_copy(blk, blk, sem.at[SEM_MOD + qq]).wait()
        else:
            _, qq, lo, hi = item
            units_wait(lo, hi - lo, pl.ds(qq * (KQ // 2), KQ // 2), SEM_WA + W_ITEMS.index(item))

    def whole_start(i):
        xc_copy(i - 2).start()
        units_start(6 * i, 6 * i + 6, pl.ds(0, D // 2), SEM_WB + i - 2)

    def mod_copy(n):
        return pltpu.make_async_copy(wmod32.at[:, pl.ds(2 * D + n * 128, 128)],
                                     qka.at[n, pl.ds(0, D // 2), :], sem.at[SEM_MOD + NQ])

    def x0_copy(i):
        n = PRE // 2 // NX0
        rows = pl.ds(pl.multiple_of(i * n, n), n)
        return pltpu.make_async_copy(x32.at[rows], xs.at[rows], sem.at[SEM_X0 + i])

    def xc_copy(i):
        rows = pl.ds(pl.multiple_of(PRE // 2 + i * (XC // 2), 64), XC // 2)
        return pltpu.make_async_copy(x32.at[rows], xs.at[rows], sem.at[SEM_XC + i])

    def wo_copy(n):
        return pltpu.make_async_copy(wo32.at[:, pl.ds(n * 128, 128)], wo.at[n], sem.at[SEM_WO])

    w1_copy = pltpu.make_async_copy(w1_hbm.bitcast(U32), w1, sem.at[SEM_W1])
    w2_copy = pltpu.make_async_copy(w2_hbm.bitcast(U32), w2, sem.at[SEM_W2])
    small_copies = [pltpu.make_async_copy(a, b, sem.at[SEM_C])
                    for a, b in ((c_hbm, c_ref), (mem0_hbm, mem0_ref), (b1_hbm, b1_ref),
                                 (b2_hbm, b2_ref))]

    def deinterleave(u, row0, nrows):
        for k in range(nrows // 64):
            rows = pl.ds(row0 + k * 64, 64)
            a = wqkv[2 * u, rows, :]
            b = wqkv[2 * u + 1, rows, :]
            wqkv[2 * u, rows, :] = (a & jnp.uint32(0xFFFF)) | (b << 16)
            wqkv[2 * u + 1, rows, :] = (a >> 16) | (b & jnp.uint32(0xFFFF0000))

    def load_x16(row2, dep):
        xw = xs[pl.ds(row2, 8), :]
        if dep is not None:
            first = xw[:, 0:128] | (dep & zerob[...])
            xw = jnp.concatenate([first, xw[:, 128:]], axis=1)
        return _bf(xw).astype(F32)

    pks = [pk0, pk1, pk2, pk3, pk4]

    def pack(v, dtype=U32):
        rows = pl.ds(0, v.shape[0] // 2)
        pk = pks[0]
        pk[rows, pl.ds(0, 128)] = pltpu.bitcast(v.astype(BF16), U32)
        return pltpu.bitcast(pk[rows, pl.ds(0, 128)], dtype)

    def rep(v8, n):
        return jnp.concatenate([v8] * (n // 8), axis=0)

    def mrow(k, n):
        if k < 2:
            return rep(jnp.concatenate([moda[qq, k] for qq in range(NQ)], axis=1), n)
        return rep(modb[k - 2], n)

    for cp in small_copies:
        cp.start()
    for i in range(NX0):
        x0_copy(i).start()
    for item in FIRST_STARTS:
        item_start(item)

    def start_rest():
        for n in range(8):
            wo_copy(n).start()
        w1_copy.start()
        w2_copy.start()

    r = lax.broadcasted_iota(jnp.int32, (80, 128), 0)
    q = lax.broadcasted_iota(jnp.int32, (80, 128), 1)
    r_tok = r < 64
    q_tok = q < 64
    r_head = jnp.where(r_tok, r >> 5, (r - 64) >> 3)
    q_head = jnp.where(q_tok, q >> 5, (q - 64) >> 3)
    same = (r_head == q_head) & (q < 80)
    causal_ok = jnp.logical_not(r_tok & q_tok & ((q & 31) > (r & 31)))
    scale = E ** (-0.5)
    fillb[...] = jnp.where(same, jnp.where(causal_ok, 0.0, -1e9 / scale), -jnp.inf).astype(F32)
    zerob[...] = jnp.zeros((8, 128), U32)
    zero_s[0] = 0

    for cp in small_copies:
        cp.wait()
    cf = c_ref[...].astype(F32)
    sc = (cf * jax.nn.sigmoid(cf)).astype(BF16)
    scb[...] = pltpu.bitcast(jnp.broadcast_to(sc, (16, D)), U32)
    memb[...] = mem0_ref[...].astype(F32)
    biasb[:, pl.ds(0, FF)] = jnp.broadcast_to(b1_ref[...].astype(F32).reshape(1, FF), (8, FF))
    biasb[:, pl.ds(FF, D)] = jnp.broadcast_to(b2_ref[...].astype(F32).reshape(1, D), (8, D))

    def pre_norm(i, carry):
        x0_copy(i).wait()
        nr = PRE // NX0
        for z in range(nr // 16):
            xn = _ln(load_x16(pl.multiple_of(i * (nr // 2) + z * 8, 8), None))
            for n in range(8):
                oring[n, pl.ds(pl.multiple_of(i * nr + z * 16, 16), 16), :] = xn[:, n * 128:(n + 1) * 128]
        return carry

    with jax.named_scope("p0_ln"):
        lax.fori_loop(0, NX0, pre_norm, 0)

    def dst_slot(i, k, p):
        cls, m = k // 3, k % 3
        if m == 2:
            return vring, 4 * i + 2 * cls + p
        return (qka, qkb)[cls], 4 * i + 2 * m + p

    PH = PRE // 2
    assert KQ == 256

    def item_run(item):
        if item[0] == 'm':
            qq = item[1]
            sc16 = _bf(scb[...])
            ca1 = 1.0 + _dot(sc16, _bf(ha[wma(qq, 1)]))[0:8].astype(BF16).astype(F32)
            sa = _dot(sc16, _bf(ha[wma(qq, 0)]))[0:8].astype(BF16).astype(F32)
            moda[qq, 0] = sa
            moda[qq, 1] = ca1
            for z in range(PH // 32):
                def h_blk(rh, kh):
                    cols = slice(kh * 128, (kh + 1) * 128)
                    return (oring[2 * qq + kh, pl.ds(rh * PH + z * 32, 32), :] * rep(ca1[:, cols], 32)
                            + rep(sa[:, cols], 32))

                for c, v in enumerate(_lhs_combos(h_blk(0, 0), h_blk(0, 1), h_blk(1, 0), h_blk(1, 1))):
                    ha[hb_idx(c, qq, 1, z * 16, 16)] = pltpu.bitcast(v.astype(BF16), F32)
            return
        _, qq, lo, hi = item
        for u in range(lo, hi):
            deinterleave(u, qq * (KQ // 2), KQ // 2)
            unit_proj(u // 6, u % 6, [qq], qq > 0)

    def unit_proj(i, k, slices, accumulate, side=lambda: None):
        u = 6 * i + k

        def prod(c):
            lhs = _bf(ha[hb_idx(c, slices[0], len(slices))])
            rhs = _rhs_operand(c, lambda a, b: jnp.concatenate(
                [wqkv[2 * u + b, pl.ds((2 * qq + a) * 64, 64), :] for qq in slices], axis=0))
            return _dot(lhs, rhs)

        def finish(y, rh, ch):
            ref, idx = dst_slot(i, k, ch)
            rows = pl.ds(RING - PRE + rh * PH, PH)
            if accumulate:
                y = y + ref[idx, rows, :]
            ref[idx, rows, :] = y

        _strassen(prod, finish, side)

    def phase1b(i, carry):
        @pl.when(i == 3)
        def _():
            whole_start(6)
            whole_start(7)

        @pl.when(i == 4)
        def _():
            start_rest()

        xc_copy(i - 2).wait()
        units_wait(6 * i, 6, pl.ds(0, D // 2), SEM_WB + i - 2)
        deinterleave(6 * i, 0, D // 2)
        state = dict(dep=None, piece=0, slot=0)

        def side():
            state['slot'] += 1
            if state['slot'] % 4 != 0 and state['piece'] < XC // 16:
                off = state['piece'] * 16
                x16 = load_x16(pl.multiple_of((i - 2) * (XC // 2), XC // 2) + (PRE + off) // 2, state['dep'])
                h16 = _ln(x16) * mrow(1, 16) + mrow(0, 16)
                hn[pl.ds(pl.multiple_of((i - 2) * XC, XC) + off, 16), :] = h16
                state['dep'] = pltpu.bitcast(h16[8:16, D - 128:], U32)
                state['piece'] += 1

        for k in range(6):
            if k < 5:
                deinterleave(6 * i + k + 1, 0, D // 2)
            unit_proj(i, k, list(range(NQ)), False, side)
        return carry

    for bi, (starts, items) in enumerate(P1A_BLOCKS):
        for item in starts:
            item_start(item)
        with jax.named_scope("p1a_wait%d" % bi):
            for item in items:
                item_wait(item)
        for item in items:
            item_run(item)
    with jax.named_scope("p1b"):
        lax.fori_loop(2, 8, phase1b, 0)
    for n in range(8):
        wo_copy(n).wait()

    cexp = scale * math.log2(math.e)
    NG = NP // 2
    grp = [(4 * (g // 2) + (g % 2), 4 * (g // 2) + (g % 2) + 2) for g in range(NG)]
    early = [2 * j + u for g in range(NG - 3) for j in grp[g] for u in range(2)]
    late = [h for h in range(H) if h not in early]

    def step(it, k):
        s = it * UNROLL + k
        split = k > 0
        base = TOK * UNROLL * it
        w0 = pl.multiple_of(lax.rem(base, RING), 32) + TOK * k
        r0 = pl.multiple_of(lax.rem(SEG * s + (RING - PRE), RING), 32)
        ow = pl.multiple_of(lax.rem(SEG * s + OOFF, RING), 32)
        o0 = pl.multiple_of(lax.rem(base + OOFF, RING), 32) + TOK * k
        a0 = pl.multiple_of(base, 32) + TOK * k
        X = jnp.concatenate([hn[pl.ds(a0, TOK), :], memb[...]], axis=0).astype(BF16)
        ym = [None] * 96
        probs = [None] * NP
        om = [None] * H
        order = (4, 5, 0, 1, 2, 3)

        if split:
            for t in order:
                accb[t] = _dot(X[:, :D // 2], _bf(wqkv[t, pl.ds(0, D // 4), :]))

        def slot(j, t):
            if t >= 4:
                return vring, 2 * j + t - 4
            return (qka, qkb)[j % 2], 4 * (j // 2) + t

        def proj(j, t):
            c = 6 * j + t
            if split and j == 0:
                y = accb[t] + _dot(X[:, D // 2:], _bf(wqkv[c, pl.ds(D // 4, D // 4), :]))
            else:
                y = _dot(X, _bf(wqkv[c]))
            ref, k = slot(j, t)
            ref[k, pl.ds(w0, TOK), :] = y[0:TOK]
            ym[c] = y[TOK:TOK + M]

        def gather(j, m, pad):
            c = 6 * j + 2 * m
            ref, k = slot(j, 2 * m)
            parts = [ref[k, pl.ds(r0, SEG), :], ref[k + 1, pl.ds(r0, SEG), :], ym[c], ym[c + 1]]
            if pad:
                parts.append(jnp.zeros((48, E), F32))
            return jnp.concatenate(parts, axis=0).astype(BF16)

        def scores(j):
            sc_ = lax.dot_general(gather(j, 0, False), gather(j, 1, True),
                                  (((1,), (1,)), ((), ())), preferred_element_type=F32)
            fill = fillb[...]
            sc_ = jnp.where(fill == 0.0, sc_, fill)
            mx = jnp.max(sc_, axis=-1, keepdims=True)
            p = jnp.exp2((sc_ - mx) * cexp)
            l = jnp.sum(p, axis=-1, keepdims=True)
            rl = pl.reciprocal(l, approx=True)
            rl = rl * (2.0 - l * rl)
            probs[j] = p * rl

        def park(j):
            vring[H, pl.ds(40 * (j % 8), 40), :] = pack(probs[j], F32)
            probs[j] = None

        def pv(j):
            if probs[j] is None:
                P = _bf(vring[H, pl.ds(40 * (j % 8), 40), :])
            else:
                P = probs[j].astype(BF16)
            o = _dot(P, gather(j, 2, True))
            oring[2 * j, pl.ds(ow, SEG), :] = o[0:32]
            oring[2 * j + 1, pl.ds(ow, SEG), :] = o[32:64]
            om[2 * j] = o[64:72]
            om[2 * j + 1] = o[72:80]

        def o_lhs(hs):
            return jnp.concatenate(
                [jnp.concatenate([oring[h, pl.ds(o0, TOK), :], om[h]], axis=0) for h in hs],
                axis=1).astype(BF16)

        def o_rhs(n, hs):
            return _bf(jnp.concatenate([wo[n, pl.ds(h * 64, 64), :] for h in hs], axis=0))

        for g in range(NG):
            cols = [(j, t) for j in grp[g] for t in order]
            if g == 2:
                cols = ([(j, t) for j in grp[g] for t in (4, 5)]
                        + [(j, t) for j in grp[g] for t in range(4)])
            for j in (grp[0] + grp[1] if g == 3 else grp[g - 2] if g >= 4 else ()):
                park(j)
            for ci, (j, t) in enumerate(cols):
                if g == 2 and ci == 4:
                    for jj in grp[0] + grp[1]:
                        scores(jj)
                if g >= 3 and ci == 6:
                    for jj in grp[g - 1]:
                        scores(jj)
                    for jj in grp[g - 3]:
                        pv(jj)
                proj(j, t)
        lo = o_lhs(early)
        for n in range(8):
            accb[n] = _dot(lo, o_rhs(n, early))
            if n == 1:
                for jj in grp[NG - 1]:
                    scores(jj)
                for jj in grp[NG - 3]:
                    pv(jj)
            if n == 4:
                for jj in grp[NG - 2] + grp[NG - 1]:
                    pv(jj)
        lo = o_lhs(late)
        for n in range(8):
            a = accb[n] + _dot(lo, o_rhs(n, late))
            ha[pl.ds(a0, TOK), pl.ds(n * 128, 128)] = a[0:TOK]
            memb[:, pl.ds(n * 128, 128)] = a[TOK:TOK + M]

    def steps(i, carry):
        for k in range(UNROLL):
            step(i, k)
        return carry

    with jax.named_scope("p2_steps"):
        lax.fori_loop(0, NSEG // UNROLL, steps, 0)

    for n in range(H):
        mod_copy(n).start()
    w1_copy.wait()
    w2_copy.wait()

    nb = S // FB
    HB = FB // 2
    QB = FB // 4

    def ln2_piece(blk, off, dep):
        x2 = (load_x16(pl.multiple_of(blk * HB, HB) + off // 2, dep)
              + mrow(2, 16) * ha[pl.ds(pl.multiple_of(blk * FB, FB) + off, 16), :])
        h = _ln(x2) * mrow(4, 16) + mrow(3, 16)
        for n in range(8):
            oring[n, pl.ds(off, 16), :] = h[:, n * 128:(n + 1) * 128]
        return pltpu.bitcast(h[8:16, D - 128:], U32)

    def lhs1_loc(base, c, d):
        e = 7 * c + d
        return base + 32 * (e // 4), 256 * (e % 4)

    def lhs1_job(base, k, t, c):
        def sub(ri, ki):
            return _combo(_LHS_TERMS, c, lambda ro, ko: oring[
                (2 * ko + ki) * 2 + t, pl.ds((2 * ro + ri) * QB + 16 * k, 16), :])

        bits = None
        for d, v in enumerate(_lhs_combos(sub(0, 0), sub(0, 1), sub(1, 0), sub(1, 1))):
            r0, c0 = lhs1_loc(base, c, d)
            hn[pl.ds(r0 + 8 * k, 8), pl.ds(c0 + t * 128, 128)] = pltpu.bitcast(
                v.astype(BF16), F32)
            if d not in (2, 3):
                b = pltpu.bitcast(v[8 * (d % 2):8 * (d % 2) + 8], U32)
                bits = b if bits is None else bits | b
        return bits

    K1, N1, K2, N2 = D // 8, FF // 4, FF // 8, D // 4

    def rhs1_loc(c, d, n):
        e = _PAIRS.index((c, d)) * 7 + n
        return wqkv, e // 4, K1 * (e % 4)

    rhs2_slots = ([(wqkv, e, 0) for e in range(79, 96)] + [(qkb, e, 0) for e in range(H)]
                  + [(vring, e, 0) for e in range(H + 1)] + [(wx, e, 0) for e in range(8)])

    def rhs2_loc(c, d, n):
        return rhs2_slots[_PAIRS.index((c, d)) * 2 + n]

    def rhs_job(w, kq, nq, loc, n, r, cs):
        cache = {}

        def blk(ko, no, ki, ni):
            key = (2 * ko + ki, 2 * no + ni)
            if key not in cache:
                cache[key] = _bf(w[pl.ds(r + key[0] * kq, 8), pl.ds(n * 128 + key[1] * nq, 128)]).astype(F32)
            return cache[key]

        bits = None
        for c in cs:
            def sub(ki, ni):
                return _combo(_RHS_TERMS, c, lambda ko, no: blk(ko, no, ki, ni))

            for d, v in enumerate(_rhs_combos(sub(0, 0), sub(0, 1), sub(1, 0), sub(1, 1))):
                if (c, d) in _PAIRS:
                    ref, idx, row = loc(c, d, n)
                    b = pack(v)
                    ref[idx, pl.ds(row + r, 8), :] = pltpu.bitcast(b, ref.dtype)
                    bits = b if bits is None else bits | b
        return bits

    def rhs_load(w, kq, nq, loc, c, d, n):
        if (c, d) not in _PAIRS:
            q = 2 * (c // 4) + d // 4
            return w[pl.ds(q * kq, kq), pl.ds(q * nq + n * 128, 128)]
        ref, idx, row = loc(c, d, n)
        return pltpu.bitcast(ref[idx, pl.ds(row, kq), :], U32)

    def make_tie(jobs, credit):
        state = [credit]

        def tie(raw, density):
            if not jobs:
                return raw
            parts = []
            for r in range(0, raw.shape[0], 8):
                v = raw[r:r + 8]
                state[0] += density
                if jobs and state[0] >= 1.0:
                    state[0] -= 1.0
                    v = v | (jobs.pop(0)() & zerob[...])
                parts.append(v)
            return jnp.concatenate(parts, axis=0)

        return tie

    def w_jobs(r1, n1, r2, n2):
        return ([functools.partial(rhs_job, w1, K1, N1, rhs1_loc, n, r1 + 8 * j, [c])
                 for c in range(7) for n in range(7) for j in range(n1)]
                + [functools.partial(rhs_job, w2, K2, N2, rhs2_loc, n, r2 + 8 * j, [c])
                   for c in range(7) for n in range(2) for j in range(n2)])

    def bulk_o(lhs, n, jobs, side=lambda: None, density=None):
        if density is None:
            density = (len(jobs) + 4) / (7 * 64)
        credit = [-2.0]

        def tie_lhs(tiles):
            tiles = [[t[8 * g:8 * g + 8] for g in range(16)] for t in tiles]
            for w in range(4):
                for g in range(16):
                    credit[0] += density
                    if jobs and credit[0] >= 1.0:
                        credit[0] -= 1.0
                        t = tiles[4 * w + g % 4]
                        t[g] = t[g] | (jobs.pop(0)() & zerob[...])
            return _bf(jnp.concatenate([jnp.concatenate(t, axis=0) for t in tiles], axis=1))

        def prod(c):
            side()
            return _dot(tie_lhs(lhs[c]),
                        _rhs_operand(c, lambda a, b: wo[n + 4 * b, pl.ds(a * 1024, 1024), :]))

        def finish(y, rh, ch):
            cols = pl.ds(pl.multiple_of((n + 4 * ch) * 128, 128), 128)
            ha[pl.ds(NSEG * TOK + rh * 256, 256), cols] = y

        _strassen(prod, finish)
        assert not jobs

    def a_blk(rh, kh):
        return jnp.concatenate([oring[h, pl.ds(rh * 256, 256), :]
                                for h in range(16 * kh, 16 * kh + 16)], axis=1)

    (a1, a2), (m1, m2), (z1, z2) = P3_SPLIT
    assert a1 + 2 * m1 + z1 == K1 // 8 and a2 + 2 * m2 + z2 == K2 // 8
    pks.pop(0)
    with jax.named_scope("p3_first"):
        lhs_o = [[pack(v[:, 128 * t:128 * t + 128]) for t in range(16)]
                 for v in _lhs_combos(a_blk(0, 0), a_blk(0, 1), a_blk(1, 0), a_blk(1, 1))]
        bulk_o(lhs_o, 0, w_jobs(0, a1, 0, a2))
    pks.pop(0)

    def bulk_mid(n, carry):
        bulk_o(lhs_o, n, w_jobs(pl.multiple_of(8 * (a1 + (n - 1) * m1), 8), m1,
                                pl.multiple_of(8 * (a2 + (n - 1) * m2), 8), m2))
        return carry

    with jax.named_scope("p3_mid"):
        lax.fori_loop(1, 3, bulk_mid, 0)
    pks.pop(0)
    for n in range(H):
        mod_copy(n).wait()

    def bulk_last(zero):
        jobs = w_jobs(8 * (a1 + 2 * m1), z1, 8 * (a2 + 2 * m2), z2)
        tie = make_tie(jobs, 0.0)
        for g in range(4):
            for n in range(8):
                w = tie(pltpu.bitcast(qka[8 * g + n, pl.ds(0, D // 2), :], U32), MOD_DENSITY)
                y = _dot(_bf(scb[...]), _bf(w))[0:8].astype(BF16).astype(F32)
                modb[g, :, pl.ds(n * 128, 128)] = 1.0 + y if g == 2 else y
        density = (len(jobs) + 56 + 4) / (7 * 64)
        state = dict(dep=None, piece=0, window=0)
        pending = []

        def side():
            jobs.extend(pending)
            del pending[:]
            for _ in range(LN0_PLAN[state['window']]):
                k, r = state['piece'] // 4, state['piece'] % 4
                state['dep'] = ln2_piece(zero, r * QB + 16 * k, state['dep'])
                if r == 3:
                    pending.extend(functools.partial(lhs1_job, 0, k, t, c)
                                   for t in range(2) for c in range(7))
                state['piece'] += 1
            state['window'] += 1

        bulk_o(lhs_o, 3, jobs, side, density)
        assert not pending and state['piece'] == 16

    with jax.named_scope("p3_last"):
        bulk_last(zero_s[0])

    pks.pop(0)
    out32 = out_hbm.bitcast(F32)
    qka[16, pl.ds(0, 8), :] = jnp.zeros((8, E), F32)

    def ffn(i, carry):
        base = pl.multiple_of((i & 1) * 512, 512)
        nbase = pl.multiple_of(((i + 1) & 1) * 512, 512)
        nxt = (i + 1) & (nb - 1)
        half = i >> 2
        srow = pl.multiple_of((i & 3) * HB, HB)

        g = {(c, d): [] for c in range(7) for d in range(7)}
        for n in range(7):
            act = {}

            def prod1(c, d):
                r0, c0 = lhs1_loc(base, c, d)
                return _dot(_bf(hn[pl.ds(r0, QB // 2), pl.ds(c0, 256)]),
                            _bf(rhs_load(w1, K1, N1, rhs1_loc, c, d, n)))

            def activate(y, rh, ch):
                b1 = jnp.concatenate([biasb[:, pl.ds((2 * ch + ci) * N1 + n * 128, 128)] for ci in range(2)],
                                     axis=1)
                act[rh, ch] = jax.nn.gelu(y + rep(b1, HB), approximate=True)

            _strassen(lambda c: _strassen_value(functools.partial(prod1, c)), activate)
            for c in range(7):
                o = _combo(_LHS_TERMS, c, lambda a, b: act[a, b])
                for d, v in enumerate(_lhs_combos(o[:QB, :128], o[:QB, 128:], o[QB:, :128], o[QB:, 128:])):
                    g[c, d].append(v.astype(BF16))

        state = dict(dep=None, piece=0, window=0)
        jobs, pending = [], []
        tie = make_tie(jobs, 0.0)

        def next_block_ln():
            jobs.extend(pending)
            del pending[:]
            for _ in range(LN_PLAN[state['window']]):
                k, r = state['piece'] // 4, state['piece'] % 4
                pin = pltpu.bitcast(qka[16, pl.ds(0, 8), :], U32)
                dep = pin if state['dep'] is None else state['dep'] | pin
                state['dep'] = ln2_piece(nxt, r * QB + 16 * k, dep)
                if r == 3:
                    pending.extend(functools.partial(lhs1_job, nbase, k, t, c)
                                   for t in range(2) for c in range(7))
                state['piece'] += 1
            state['window'] += 1

        for n in range(2):
            def prod2(c, d):
                return _dot(jnp.concatenate(g[c, d], axis=1),
                            _bf(tie(rhs_load(w2, K2, N2, rhs2_loc, c, d, n), 1.0 / 24)))

            def outer(c):
                next_block_ln()
                y = _strassen_value(functools.partial(prod2, c))
                qka[17, pl.ds(srow, 8), :] = y[0:8, 0:128]
                return y

            def finish(y, rh, ch):
                for ci in range(2):
                    nn = (2 * ch + ci) * 2 + n
                    cols = pl.ds(nn * 128, 128)
                    yy = y[:, ci * 128:(ci + 1) * 128] + rep(biasb[:, pl.ds(FF + nn * 128, 128)], HB)
                    xr = pl.ds(pl.multiple_of(i * HB, HB) + rh * (HB // 2), HB // 2)
                    ar = pl.ds(pl.multiple_of(i * FB, FB) + rh * HB, HB)
                    x2 = _bf(xs[xr, cols]).astype(F32) + rep(modb[0, :, cols], HB) * ha[ar, cols]
                    qka[2 * nn + half, pl.ds(srow + rh * (HB // 2), HB // 2), :] = pack(
                        x2 + rep(modb[3, :, cols], HB) * yy, F32)
                    if rh == ch:
                        pltpu.make_async_copy(
                            qka.at[2 * nn + half, pl.ds(srow, HB), :],
                            out32.at[pl.ds(pl.multiple_of(i * HB, HB), HB), cols],
                            sem.at[SEM_OUT]).start()

            _strassen(outer, finish)
        assert not jobs and not pending and state['piece'] == 16
        return carry

    with jax.named_scope("p4_ffn"):
        lax.fori_loop(0, nb, ffn, 0)
    pltpu.make_async_copy(out32, out32, sem.at[SEM_OUT]).wait()


@jax.jit
def pallas_adaLN_cond__memory_aug_recurrent_mem_tr__dense_activation_gelu__prompt_kernel(
    A_x, A_mem0, A_Wq, A_Wk, A_Wv, A_Wo, A_seg_len, B_x, B_w1, B_b1, B_w2, B_b2, c, w_mod,
):
    assert A_x.shape == (1, S, D) and A_Wq.shape == (D, H, E) and A_mem0.shape == (1, M, D)
    any_spec = pl.BlockSpec(memory_space=pl.ANY)
    out = pl.pallas_call(
        _kernel,
        out_shape=jax.ShapeDtypeStruct((S, D), BF16),
        in_specs=[any_spec] * 12,
        out_specs=any_spec,
        scratch_shapes=[
            pltpu.VMEM((S // 2, D), U32),
            pltpu.VMEM((96, D // 2, E), U32),
            pltpu.VMEM((8, H * E // 2, 128), U32),
            pltpu.VMEM((D // 2, FF), U32),
            pltpu.VMEM((FF // 2, D), U32),
            pltpu.VMEM((H, RING, E), F32),
            pltpu.VMEM((H, RING, E), F32),
            pltpu.VMEM((H + 1, RING, E), F32),
            pltpu.VMEM((H, RING, E), F32),
            pltpu.VMEM((S, D), F32),
            pltpu.VMEM((S - PRE, D), F32),
            pltpu.VMEM((M, D), F32),
            pltpu.VMEM((NQ, 2, 8, KQ), F32),
            pltpu.VMEM((4, 8, D), F32),
            pltpu.VMEM((8, D), U32),
            pltpu.VMEM((8, FF + D), F32),
            pltpu.VMEM((80, 128), F32),
            pltpu.VMEM((8, 32, 128), F32),
            pltpu.VMEM((8, 128), U32),
            pltpu.SMEM((1,), jnp.int32),
            pltpu.VMEM((8, FF // 8, 128), U32),
            pltpu.VMEM((128, 256), U32),
            pltpu.VMEM((128, 256), U32),
            pltpu.VMEM((128, 256), U32),
            pltpu.VMEM((128, 256), U32),
            pltpu.VMEM((128, 256), U32),
            pltpu.VMEM((M, D), BF16),
            pltpu.VMEM((FF,), BF16),
            pltpu.VMEM((D,), BF16),
            pltpu.VMEM((1, D), BF16),
            pltpu.SemaphoreType.DMA((NSEM,)),
        ],
        compiler_params=pltpu.CompilerParams(vmem_limit_bytes=127 * 1024 * 1024, disable_bounds_checks=True,
                                             disable_semaphore_checks=True),
    )(
        A_x.reshape(S, D), A_mem0.reshape(M, D),
        A_Wq.reshape(D // 2, 2, H, E), A_Wk.reshape(D // 2, 2, H, E), A_Wv.reshape(D // 2, 2, H, E),
        A_Wo.reshape(H * E, D), B_w1, B_b1, B_w2, B_b2, c, w_mod,
    )
    return out.reshape(1, S, D)
```

```python
import functools
import math

import jax
import jax.numpy as jnp
from jax import lax
import jax.experimental.pallas as pl
import jax.experimental.pallas.tpu as pltpu

F32 = jnp.float32
BF16 = jnp.bfloat16
U32 = jnp.uint32

S = 2048
D = 1024
H = 32
E = 128
M = 8
SEG = 32
NSEG = S // SEG
FF = 3584
NP = H // 2
TOK = 24
PRE = S - NSEG * TOK
RING = 576
OOFF = (-NSEG * TOK) % RING
LN_EPS = 1e-5
FB = 256
XC = (S - PRE) // 6
P3_SPLIT = ((4, 8), (4, 16), (4, 16))
MOD_DENSITY = 0.07
LN0_PLAN = (6, 2, 2, 2, 2, 2, 0)
LN_PLAN = (1, 1, 1, 1, 1, 1, 1, 2, 2, 2, 2, 1, 0, 0)
UNROLL = 4

NQ = 4
KQ = D // NQ

FIRST_STARTS = [('m', 0), ('w', 0, 0, 2), ('w', 0, 2, 6), ('w', 0, 6, 12), ('m', 1), ('w', 1, 0, 6),
                ('w', 1, 6, 12), ('m', 2)]
P1A_BLOCKS = [
    ([], [('m', 0)]),
    ([], [('w', 0, 0, 2)]),
    ([], [('w', 0, 2, 6)]),
    ([('w', 2, 0, 6), ('w', 2, 6, 12)], [('w', 0, 6, 12)]),
    ([('m', 3), ('w', 3, 0, 6), ('w', 3, 6, 12)], [('m', 1), ('w', 1, 0, 6)]),
    ([], [('m', 2), ('w', 1, 6, 12)]),
    ([('g', 2), ('g', 3)], [('w', 2, 0, 6), ('w', 2, 6, 12)]),
    ([('g', 4), ('g', 5)], [('m', 3), ('w', 3, 0, 6), ('w', 3, 6, 12)]),
]
W_ITEMS = [it for _, items in P1A_BLOCKS for it in items if it[0] == 'w']
NX0 = 4

SEM_C = 0
SEM_X0 = 1
SEM_MOD = SEM_X0 + NX0
SEM_WA = SEM_MOD + NQ + 1
SEM_WB = SEM_WA + len(W_ITEMS)
SEM_XC = SEM_WB + 6
SEM_WO = SEM_XC + 6
SEM_W1 = SEM_WO + 1
SEM_W2 = SEM_W1 + 1
SEM_OUT = SEM_W2 + 1
NSEM = SEM_OUT + 1


def _ln(x):
    m = jnp.mean(x, axis=-1, keepdims=True)
    xc = x - m
    v = jnp.mean(xc * xc, axis=-1, keepdims=True)
    return xc * lax.rsqrt(v + LN_EPS)


def _bf(w32):
    return pltpu.bitcast(w32, BF16)


def _dot(a, b):
    return jnp.dot(a, b, preferred_element_type=F32)


def _lhs_combos(a11, a12, a21, a22):
    return [a11 + a22, a21 + a22, a11, a22, a11 + a12, a21 - a11, a12 - a22]


def _rhs_combos(b11, b12, b21, b22):
    return [b11 + b22, b11, b12 - b22, b21 - b11, b22, b11 + b12, b21 + b22]


_LHS_TERMS = {0: ((0, 0), (1, 1), 1), 1: ((1, 0), (1, 1), 1), 2: ((0, 0), None, 0), 3: ((1, 1), None, 0),
              4: ((0, 0), (0, 1), 1), 5: ((1, 0), (0, 0), -1), 6: ((0, 1), (1, 1), -1)}
_RHS_TERMS = {0: ((0, 0), (1, 1), 1), 1: ((0, 0), None, 0), 2: ((0, 1), (1, 1), -1), 3: ((1, 0), (0, 0), -1),
              4: ((1, 1), None, 0), 5: ((0, 0), (0, 1), 1), 6: ((1, 0), (1, 1), 1)}


def _combo(terms, c, blk):
    p, q, sign = terms[c]
    if q is None:
        return blk(*p)
    return blk(*p) + blk(*q) if sign > 0 else blk(*p) - blk(*q)


def _rhs_operand(c, blk):
    p, q, sign = _RHS_TERMS[c]
    a = _bf(blk(*p))
    if q is None:
        return a
    a = a.astype(F32)
    b = _bf(blk(*q)).astype(F32)
    return (a + b if sign > 0 else a - b).astype(BF16)


def _strassen(prod, finish, side=lambda: None):
    side()
    m1 = prod(1)
    m3 = prod(3)
    finish(m1 + m3, 1, 0)
    side()
    m2 = prod(2)
    m4 = prod(4)
    finish(m2 + m4, 0, 1)
    side()
    m0 = prod(0)
    m5 = prod(5)
    finish((m2 - m1) + m0 + m5, 1, 1)
    side()
    m6 = prod(6)
    finish((m3 - m4) + m0 + m6, 0, 0)


def _strassen_value(prod):
    r = {}
    _strassen(prod, lambda y, rh, ch: r.__setitem__((rh, ch), y))
    return jnp.concatenate([jnp.concatenate([r[0, 0], r[0, 1]], axis=1),
                            jnp.concatenate([r[1, 0], r[1, 1]], axis=1)], axis=0)


_PAIRS = [(c, d) for c in range(7) for d in range(7) if not (c in (1, 4) and d in (1, 4))]


def _kernel(x_hbm, mem0_hbm, wq_hbm, wk_hbm, wv_hbm, wo_hbm, w1_hbm, b1_hbm, w2_hbm, b2_hbm,
            c_hbm, wmod_hbm, out_hbm,
            xs, wqkv, wo, w1, w2, qka, qkb, vring, oring, ha, hn, memb, moda, modb, scb, biasb,
            fillb, accb, zerob, zero_s, wx, pk0, pk1, pk2, pk3, pk4, mem0_ref, b1_ref, b2_ref, c_ref, sem):
    qkv_hbm = [r.bitcast(U32) for r in (wq_hbm, wk_hbm, wv_hbm)]
    x32 = x_hbm.bitcast(U32)
    wo32 = wo_hbm.bitcast(U32)
    wmod32 = wmod_hbm.bitcast(F32)

    def wma(qq, k):
        return pl.ds(512 * (qq // 2), 512), pl.ds(512 * (qq % 2) + k * KQ, KQ)

    def hb_idx(c, q0, nq, row0=0, nrows=PRE // 4):
        return pl.ds(1024 + 128 * (c // 2) + row0, nrows), pl.ds(512 * (c % 2) + 128 * q0, 128 * nq)

    def units_start(lo, hi, rows, sem_idx):
        for u in range(lo, hi):
            j, m = u // 3, u % 3
            for p in range(2):
                pltpu.make_async_copy(qkv_hbm[m].at[rows, p, j, :], wqkv.at[2 * u + p, rows, :],
                                      sem.at[sem_idx]).start()

    def units_wait(lo, n, rows, sem_idx):
        blk = wqkv.at[pl.ds(2 * lo, 2 * n), rows, :]
        pltpu.make_async_copy(blk, blk, sem.at[sem_idx]).wait()

    def item_start(item):
        if item[0] == 'm':
            qq = item[1]
            for k in range(2):
                pltpu.make_async_copy(wmod32.at[:, pl.ds(k * D + qq * KQ, KQ)], ha.at[wma(qq, k)],
                                      sem.at[SEM_MOD + qq]).start()
        elif item[0] == 'w':
            _, qq, lo, hi = item
            units_start(lo, hi, pl.ds(qq * (KQ // 2), KQ // 2), SEM_WA + W_ITEMS.index(item))
        else:
            whole_start(item[1])

    def item_wait(item):
        if item[0] == 'm':
            qq = item[1]
            blk = ha.at[pl.ds(512 * (qq // 2), 512), pl.ds(512 * (qq % 2), 512)]
            pltpu.make_async_copy(blk, blk, sem.at[SEM_MOD + qq]).wait()
        else:
            _, qq, lo, hi = item
            units_wait(lo, hi - lo, pl.ds(qq * (KQ // 2), KQ // 2), SEM_WA + W_ITEMS.index(item))

    def whole_start(i):
        xc_copy(i - 2).start()
        units_start(6 * i, 6 * i + 6, pl.ds(0, D // 2), SEM_WB + i - 2)

    def mod_copy(n):
        return pltpu.make_async_copy(wmod32.at[:, pl.ds(2 * D + n * 128, 128)],
                                     qka.at[n, pl.ds(0, D // 2), :], sem.at[SEM_MOD + NQ])

    def x0_copy(i):
        n = PRE // 2 // NX0
        rows = pl.ds(pl.multiple_of(i * n, n), n)
        return pltpu.make_async_copy(x32.at[rows], xs.at[rows], sem.at[SEM_X0 + i])

    def xc_copy(i):
        rows = pl.ds(pl.multiple_of(PRE // 2 + i * (XC // 2), 64), XC // 2)
        return pltpu.make_async_copy(x32.at[rows], xs.at[rows], sem.at[SEM_XC + i])

    def wo_copy(n):
        return pltpu.make_async_copy(wo32.at[:, pl.ds(n * 128, 128)], wo.at[n], sem.at[SEM_WO])

    w1_copy = pltpu.make_async_copy(w1_hbm.bitcast(U32), w1, sem.at[SEM_W1])
    w2_copy = pltpu.make_async_copy(w2_hbm.bitcast(U32), w2, sem.at[SEM_W2])
    small_copies = [pltpu.make_async_copy(a, b, sem.at[SEM_C])
                    for a, b in ((c_hbm, c_ref), (mem0_hbm, mem0_ref), (b1_hbm, b1_ref),
                                 (b2_hbm, b2_ref))]

    def deinterleave(u, row0, nrows):
        for k in range(nrows // 64):
            rows = pl.ds(row0 + k * 64, 64)
            a = wqkv[2 * u, rows, :]
            b = wqkv[2 * u + 1, rows, :]
            wqkv[2 * u, rows, :] = (a & jnp.uint32(0xFFFF)) | (b << 16)
            wqkv[2 * u + 1, rows, :] = (a >> 16) | (b & jnp.uint32(0xFFFF0000))

    def load_x16(row2, dep):
        xw = xs[pl.ds(row2, 8), :]
        if dep is not None:
            first = xw[:, 0:128] | (dep & zerob[...])
            xw = jnp.concatenate([first, xw[:, 128:]], axis=1)
        return _bf(xw).astype(F32)

    pks = [pk0, pk1, pk2, pk3, pk4]

    def pack(v, dtype=U32):
        rows = pl.ds(0, v.shape[0] // 2)
        pk = pks[0]
        pk[rows, pl.ds(0, 128)] = pltpu.bitcast(v.astype(BF16), U32)
        return pltpu.bitcast(pk[rows, pl.ds(0, 128)], dtype)

    def rep(v8, n):
        return jnp.concatenate([v8] * (n // 8), axis=0)

    def mrow(k, n):
        if k < 2:
            return rep(jnp.concatenate([moda[qq, k] for qq in range(NQ)], axis=1), n)
        return rep(modb[k - 2], n)

    for cp in small_copies:
        cp.start()
    for i in range(NX0):
        x0_copy(i).start()
    for item in FIRST_STARTS:
        item_start(item)

    def start_rest():
        for n in range(8):
            wo_copy(n).start()
        w1_copy.start()
        w2_copy.start()

    r = lax.broadcasted_iota(jnp.int32, (80, 128), 0)
    q = lax.broadcasted_iota(jnp.int32, (80, 128), 1)
    r_tok = r < 64
    q_tok = q < 64
    r_head = jnp.where(r_tok, r >> 5, (r - 64) >> 3)
    q_head = jnp.where(q_tok, q >> 5, (q - 64) >> 3)
    same = (r_head == q_head) & (q < 80)
    causal_ok = jnp.logical_not(r_tok & q_tok & ((q & 31) > (r & 31)))
    scale = E ** (-0.5)
    fillb[...] = jnp.where(same, jnp.where(causal_ok, 0.0, -1e9 / scale), -jnp.inf).astype(F32)
    zerob[...] = jnp.zeros((8, 128), U32)
    zero_s[0] = 0

    for cp in small_copies:
        cp.wait()
    cf = c_ref[...].astype(F32)
    sc = (cf * jax.nn.sigmoid(cf)).astype(BF16)
    scb[...] = pltpu.bitcast(jnp.broadcast_to(sc, (16, D)), U32)
    memb[...] = mem0_ref[...].astype(F32)
    biasb[:, pl.ds(0, FF)] = jnp.broadcast_to(b1_ref[...].astype(F32).reshape(1, FF), (8, FF))
    biasb[:, pl.ds(FF, D)] = jnp.broadcast_to(b2_ref[...].astype(F32).reshape(1, D), (8, D))

    def pre_norm(i, carry):
        x0_copy(i).wait()
        nr = PRE // NX0
        for z in range(nr // 16):
            xn = _ln(load_x16(pl.multiple_of(i * (nr // 2) + z * 8, 8), None))
            for n in range(8):
                oring[n, pl.ds(pl.multiple_of(i * nr + z * 16, 16), 16), :] = xn[:, n * 128:(n + 1) * 128]
        return carry

    with jax.named_scope("p0_ln"):
        lax.fori_loop(0, NX0, pre_norm, 0)

    def dst_slot(i, k, p):
        cls, m = k // 3, k % 3
        if m == 2:
            return vring, 4 * i + 2 * cls + p
        return (qka, qkb)[cls], 4 * i + 2 * m + p

    PH = PRE // 2
    assert KQ == 256

    def item_run(item):
        if item[0] == 'm':
            qq = item[1]
            sc16 = _bf(scb[...])
            ca1 = 1.0 + _dot(sc16, _bf(ha[wma(qq, 1)]))[0:8].astype(BF16).astype(F32)
            sa = _dot(sc16, _bf(ha[wma(qq, 0)]))[0:8].astype(BF16).astype(F32)
            moda[qq, 0] = sa
            moda[qq, 1] = ca1
            for z in range(PH // 32):
                def h_blk(rh, kh):
                    cols = slice(kh * 128, (kh + 1) * 128)
                    return (oring[2 * qq + kh, pl.ds(rh * PH + z * 32, 32), :] * rep(ca1[:, cols], 32)
                            + rep(sa[:, cols], 32))

                for c, v in enumerate(_lhs_combos(h_blk(0, 0), h_blk(0, 1), h_blk(1, 0), h_blk(1, 1))):
                    ha[hb_idx(c, qq, 1, z * 16, 16)] = pltpu.bitcast(v.astype(BF16), F32)
            return
        _, qq, lo, hi = item
        for u in range(lo, hi):
            deinterleave(u, qq * (KQ // 2), KQ // 2)
            unit_proj(u // 6, u % 6, [qq], qq > 0)

    def unit_proj(i, k, slices, accumulate, side=lambda: None):
        u = 6 * i + k

        def prod(c):
            lhs = _bf(ha[hb_idx(c, slices[0], len(slices))])
            rhs = _rhs_operand(c, lambda a, b: jnp.concatenate(
                [wqkv[2 * u + b, pl.ds((2 * qq + a) * 64, 64), :] for qq in slices], axis=0))
            return _dot(lhs, rhs)

        def finish(y, rh, ch):
            ref, idx = dst_slot(i, k, ch)
            rows = pl.ds(RING - PRE + rh * PH, PH)
            if accumulate:
                y = y + ref[idx, rows, :]
            ref[idx, rows, :] = y

        _strassen(prod, finish, side)

    def phase1b(i, carry):
        @pl.when(i == 3)
        def _():
            whole_start(6)
            whole_start(7)

        @pl.when(i == 4)
        def _():
            start_rest()

        xc_copy(i - 2).wait()
        units_wait(6 * i, 6, pl.ds(0, D // 2), SEM_WB + i - 2)
        deinterleave(6 * i, 0, D // 2)
        state = dict(dep=None, piece=0, slot=0)

        def side():
            state['slot'] += 1
            if state['slot'] % 4 != 0 and state['piece'] < XC // 16:
                off = state['piece'] * 16
                x16 = load_x16(pl.multiple_of((i - 2) * (XC // 2), XC // 2) + (PRE + off) // 2, state['dep'])
                h16 = _ln(x16) * mrow(1, 16) + mrow(0, 16)
                hn[pl.ds(pl.multiple_of((i - 2) * XC, XC) + off, 16), :] = h16
                state['dep'] = pltpu.bitcast(h16[8:16, D - 128:], U32)
                state['piece'] += 1

        for k in range(6):
            if k < 5:
                deinterleave(6 * i + k + 1, 0, D // 2)
            unit_proj(i, k, list(range(NQ)), False, side)
        return carry

    for bi, (starts, items) in enumerate(P1A_BLOCKS):
        for item in starts:
            item_start(item)
        with jax.named_scope("p1a_wait%d" % bi):
            for item in items:
                item_wait(item)
        for item in items:
            item_run(item)
    with jax.named_scope("p1b"):
        lax.fori_loop(2, 8, phase1b, 0)
    for n in range(8):
        wo_copy(n).wait()

    cexp = scale * math.log2(math.e)
    NG = NP // 2
    grp = [(4 * (g // 2) + (g % 2), 4 * (g // 2) + (g % 2) + 2) for g in range(NG)]
    early = [2 * j + u for g in range(NG - 3) for j in grp[g] for u in range(2)]
    late = [h for h in range(H) if h not in early]

    def step(it, k):
        s = it * UNROLL + k
        split = k > 0
        base = TOK * UNROLL * it
        w0 = pl.multiple_of(lax.rem(base, RING), 32) + TOK * k
        r0 = pl.multiple_of(lax.rem(SEG * s + (RING - PRE), RING), 32)
        ow = pl.multiple_of(lax.rem(SEG * s + OOFF, RING), 32)
        o0 = pl.multiple_of(lax.rem(base + OOFF, RING), 32) + TOK * k
        a0 = pl.multiple_of(base, 32) + TOK * k
        X = jnp.concatenate([hn[pl.ds(a0, TOK), :], memb[...]], axis=0).astype(BF16)
        ym = [None] * 96
        probs = [None] * NP
        om = [None] * H
        order = (4, 5, 0, 1, 2, 3)

        if split:
            for t in order:
                accb[t] = _dot(X[:, :D // 2], _bf(wqkv[t, pl.ds(0, D // 4), :]))

        def slot(j, t):
            if t >= 4:
                return vring, 2 * j + t - 4
            return (qka, qkb)[j % 2], 4 * (j // 2) + t

        def proj(j, t):
            c = 6 * j + t
            if split and j == 0:
                y = accb[t] + _dot(X[:, D // 2:], _bf(wqkv[c, pl.ds(D // 4, D // 4), :]))
            else:
                y = _dot(X, _bf(wqkv[c]))
            ref, k = slot(j, t)
            ref[k, pl.ds(w0, TOK), :] = y[0:TOK]
            ym[c] = y[TOK:TOK + M]

        def gather(j, m, pad):
            c = 6 * j + 2 * m
            ref, k = slot(j, 2 * m)
            parts = [ref[k, pl.ds(r0, SEG), :], ref[k + 1, pl.ds(r0, SEG), :], ym[c], ym[c + 1]]
            if pad:
                parts.append(jnp.zeros((48, E), F32))
            return jnp.concatenate(parts, axis=0).astype(BF16)

        def scores(j):
            sc_ = lax.dot_general(gather(j, 0, False), gather(j, 1, True),
                                  (((1,), (1,)), ((), ())), preferred_element_type=F32)
            fill = fillb[...]
            sc_ = jnp.where(fill == 0.0, sc_, fill)
            mx = jnp.max(sc_, axis=-1, keepdims=True)
            p = jnp.exp2((sc_ - mx) * cexp)
            l = jnp.sum(p, axis=-1, keepdims=True)
            rl = pl.reciprocal(l, approx=True)
            rl = rl * (2.0 - l * rl)
            probs[j] = p * rl

        def park(j):
            vring[H, pl.ds(40 * (j % 8), 40), :] = pack(probs[j], F32)
            probs[j] = None

        def pv(j):
            if probs[j] is None:
                P = _bf(vring[H, pl.ds(40 * (j % 8), 40), :])
            else:
                P = probs[j].astype(BF16)
            o = _dot(P, gather(j, 2, True))
            oring[2 * j, pl.ds(ow, SEG), :] = o[0:32]
            oring[2 * j + 1, pl.ds(ow, SEG), :] = o[32:64]
            om[2 * j] = o[64:72]
            om[2 * j + 1] = o[72:80]

        def o_lhs(hs):
            return jnp.concatenate(
                [jnp.concatenate([oring[h, pl.ds(o0, TOK), :], om[h]], axis=0) for h in hs],
                axis=1).astype(BF16)

        def o_rhs(n, hs):
            return _bf(jnp.concatenate([wo[n, pl.ds(h * 64, 64), :] for h in hs], axis=0))

        for g in range(NG):
            cols = [(j, t) for j in grp[g] for t in order]
            if g == 2:
                cols = ([(j, t) for j in grp[g] for t in (4, 5)]
                        + [(j, t) for j in grp[g] for t in range(4)])
            for j in (grp[0] + grp[1] if g == 3 else grp[g - 2] if g >= 4 else ()):
                park(j)
            for ci, (j, t) in enumerate(cols):
                if g == 2 and ci == 4:
                    for jj in grp[0] + grp[1]:
                        scores(jj)
                if g >= 3 and ci == 6:
                    for jj in grp[g - 1]:
                        scores(jj)
                    for jj in grp[g - 3]:
                        pv(jj)
                proj(j, t)
        lo = o_lhs(early)
        for n in range(8):
            accb[n] = _dot(lo, o_rhs(n, early))
            if n == 1:
                for jj in grp[NG - 1]:
                    scores(jj)
                for jj in grp[NG - 3]:
                    pv(jj)
            if n == 4:
                for jj in grp[NG - 2] + grp[NG - 1]:
                    pv(jj)
        lo = o_lhs(late)
        for n in range(8):
            a = accb[n] + _dot(lo, o_rhs(n, late))
            ha[pl.ds(a0, TOK), pl.ds(n * 128, 128)] = a[0:TOK]
            memb[:, pl.ds(n * 128, 128)] = a[TOK:TOK + M]

    def steps(i, carry):
        for k in range(UNROLL):
            step(i, k)
        return carry

    with jax.named_scope("p2_steps"):
        lax.fori_loop(0, NSEG // UNROLL, steps, 0)

    for n in range(H):
        mod_copy(n).start()
    w1_copy.wait()
    w2_copy.wait()

    nb = S // FB
    HB = FB // 2
    QB = FB // 4

    def ln2_piece(hs, blk, off, dep):
        x2 = (load_x16(pl.multiple_of(blk * HB, HB) + off // 2, dep)
              + mrow(2, 16) * ha[pl.ds(pl.multiple_of(blk * FB, FB) + off, 16), :])
        h = _ln(x2) * mrow(4, 16) + mrow(3, 16)
        hs[off] = h
        return pltpu.bitcast(h[8:16, D - 128:], U32)

    def lhs1_loc(base, c, d):
        e = 7 * c + d
        return base + 32 * (e // 4), 256 * (e % 4)

    def lhs1_job(hs, base, k, t, c):
        def sub(ri, ki):
            def blk(ro, ko):
                c0 = (2 * ko + ki) * 256 + t * 128
                return hs[(2 * ro + ri) * QB + 16 * k][:, c0:c0 + 128]

            return _combo(_LHS_TERMS, c, blk)

        bits = None
        for d, v in enumerate(_lhs_combos(sub(0, 0), sub(0, 1), sub(1, 0), sub(1, 1))):
            r0, c0 = lhs1_loc(base, c, d)
            hn[pl.ds(r0 + 8 * k, 8), pl.ds(c0 + t * 128, 128)] = pltpu.bitcast(
                v.astype(BF16), F32)
            if d not in (2, 3):
                b = pltpu.bitcast(v[8 * (d % 2):8 * (d % 2) + 8], U32)
                bits = b if bits is None else bits | b
        return bits

    K1, N1, K2, N2 = D // 8, FF // 4, FF // 8, D // 4

    def rhs1_loc(c, d, n):
        e = _PAIRS.index((c, d)) * 7 + n
        return wqkv, e // 4, K1 * (e % 4)

    rhs2_slots = ([(wqkv, e, 0) for e in range(79, 96)] + [(qkb, e, 0) for e in range(H)]
                  + [(vring, e, 0) for e in range(H + 1)] + [(wx, e, 0) for e in range(8)])

    def rhs2_loc(c, d, n):
        return rhs2_slots[_PAIRS.index((c, d)) * 2 + n]

    def rhs_job(w, kq, nq, loc, n, r, cs):
        cache = {}

        def blk(ko, no, ki, ni):
            key = (2 * ko + ki, 2 * no + ni)
            if key not in cache:
                cache[key] = _bf(w[pl.ds(r + key[0] * kq, 8), pl.ds(n * 128 + key[1] * nq, 128)]).astype(F32)
            return cache[key]

        bits = None
        for c in cs:
            def sub(ki, ni):
                return _combo(_RHS_TERMS, c, lambda ko, no: blk(ko, no, ki, ni))

            for d, v in enumerate(_rhs_combos(sub(0, 0), sub(0, 1), sub(1, 0), sub(1, 1))):
                if (c, d) in _PAIRS:
                    ref, idx, row = loc(c, d, n)
                    b = pack(v)
                    ref[idx, pl.ds(row + r, 8), :] = pltpu.bitcast(b, ref.dtype)
                    bits = b if bits is None else bits | b
        return bits

    def rhs_load(w, kq, nq, loc, c, d, n):
        if (c, d) not in _PAIRS:
            q = 2 * (c // 4) + d // 4
            return w[pl.ds(q * kq, kq), pl.ds(q * nq + n * 128, 128)]
        ref, idx, row = loc(c, d, n)
        return pltpu.bitcast(ref[idx, pl.ds(row, kq), :], U32)

    def make_tie(jobs, credit):
        state = [credit]

        def tie(raw, density):
            if not jobs:
                return raw
            parts = []
            for r in range(0, raw.shape[0], 8):
                v = raw[r:r + 8]
                state[0] += density
                if jobs and state[0] >= 1.0:
                    state[0] -= 1.0
                    v = v | (jobs.pop(0)() & zerob[...])
                parts.append(v)
            return jnp.concatenate(parts, axis=0)

        return tie

    def w_jobs(r1, n1, r2, n2):
        return ([functools.partial(rhs_job, w1, K1, N1, rhs1_loc, n, r1 + 8 * j, [c])
                 for c in range(7) for n in range(7) for j in range(n1)]
                + [functools.partial(rhs_job, w2, K2, N2, rhs2_loc, n, r2 + 8 * j, [c])
                   for c in range(7) for n in range(2) for j in range(n2)])

    def bulk_o(lhs, n, jobs, side=lambda: None, density=None):
        if density is None:
            density = (len(jobs) + 4) / (7 * 64)
        credit = [-2.0]

        def tie_lhs(tiles):
            tiles = [[t[8 * g:8 * g + 8] for g in range(16)] for t in tiles]
            for w in range(4):
                for g in range(16):
                    credit[0] += density
                    for extra in range(2):
                        if jobs and credit[0] >= 1.0:
                            credit[0] -= 1.0
                            t = tiles[4 * w + (g + 2 * extra) % 4]
                            t[g] = t[g] | (jobs.pop(0)() & zerob[...])
            return _bf(jnp.concatenate([jnp.concatenate(t, axis=0) for t in tiles], axis=1))

        def prod(c):
            side()
            return _dot(tie_lhs(lhs[c]),
                        _rhs_operand(c, lambda a, b: wo[n + 4 * b, pl.ds(a * 1024, 1024), :]))

        def finish(y, rh, ch):
            cols = pl.ds(pl.multiple_of((n + 4 * ch) * 128, 128), 128)
            ha[pl.ds(NSEG * TOK + rh * 256, 256), cols] = y

        _strassen(prod, finish)
        assert not jobs

    def a_blk(rh, kh):
        return jnp.concatenate([oring[h, pl.ds(rh * 256, 256), :]
                                for h in range(16 * kh, 16 * kh + 16)], axis=1)

    (a1, a2), (m1, m2), (z1, z2) = P3_SPLIT
    assert a1 + 2 * m1 + z1 == K1 // 8 and a2 + 2 * m2 + z2 == K2 // 8
    pks.pop(0)
    with jax.named_scope("p3_first"):
        lhs_o = [[pack(v[:, 128 * t:128 * t + 128]) for t in range(16)]
                 for v in _lhs_combos(a_blk(0, 0), a_blk(0, 1), a_blk(1, 0), a_blk(1, 1))]
        bulk_o(lhs_o, 0, w_jobs(0, a1, 0, a2))
    pks.pop(0)

    def bulk_mid(n, carry):
        bulk_o(lhs_o, n, w_jobs(pl.multiple_of(8 * (a1 + (n - 1) * m1), 8), m1,
                                pl.multiple_of(8 * (a2 + (n - 1) * m2), 8), m2))
        return carry

    with jax.named_scope("p3_mid"):
        lax.fori_loop(1, 3, bulk_mid, 0)
    pks.pop(0)
    for n in range(H):
        mod_copy(n).wait()

    def bulk_last(zero):
        jobs = w_jobs(8 * (a1 + 2 * m1), z1, 8 * (a2 + 2 * m2), z2)
        tie = make_tie(jobs, 0.0)
        for g in range(4):
            for n in range(8):
                w = tie(pltpu.bitcast(qka[8 * g + n, pl.ds(0, D // 2), :], U32), MOD_DENSITY)
                y = _dot(_bf(scb[...]), _bf(w))[0:8].astype(BF16).astype(F32)
                modb[g, :, pl.ds(n * 128, 128)] = 1.0 + y if g == 2 else y
        density = (len(jobs) + 56 + 4) / (7 * 64)
        state = dict(dep=None, piece=0, window=0)
        pending = []
        hs = {}

        def side():
            jobs.extend(pending)
            del pending[:]
            for _ in range(LN0_PLAN[state['window']]):
                k, r = state['piece'] // 4, state['piece'] % 4
                state['dep'] = ln2_piece(hs, zero, r * QB + 16 * k, state['dep'])
                if r == 3:
                    pending.extend(functools.partial(lhs1_job, hs, 0, k, t, c)
                                   for t in range(2) for c in range(7))
                state['piece'] += 1
            state['window'] += 1

        bulk_o(lhs_o, 3, jobs, side, density)
        assert not pending and state['piece'] == 16

    with jax.named_scope("p3_last"):
        bulk_last(zero_s[0])

    pks.pop(0)
    out32 = out_hbm.bitcast(F32)
    qka[16, pl.ds(0, 8), :] = jnp.zeros((8, E), F32)

    def ffn(i, carry):
        base = pl.multiple_of((i & 1) * 512, 512)
        nbase = pl.multiple_of(((i + 1) & 1) * 512, 512)
        nxt = (i + 1) & (nb - 1)
        half = i >> 2
        srow = pl.multiple_of((i & 3) * HB, HB)

        g = {(c, d): [] for c in range(7) for d in range(7)}
        for n in range(7):
            act = {}

            def prod1(c, d):
                r0, c0 = lhs1_loc(base, c, d)
                return _dot(_bf(hn[pl.ds(r0, QB // 2), pl.ds(c0, 256)]),
                            _bf(rhs_load(w1, K1, N1, rhs1_loc, c, d, n)))

            def activate(y, rh, ch):
                b1 = jnp.concatenate([biasb[:, pl.ds((2 * ch + ci) * N1 + n * 128, 128)] for ci in range(2)],
                                     axis=1)
                act[rh, ch] = jax.nn.gelu(y + rep(b1, HB), approximate=True)

            _strassen(lambda c: _strassen_value(functools.partial(prod1, c)), activate)
            for c in range(7):
                o = _combo(_LHS_TERMS, c, lambda a, b: act[a, b])
                for d, v in enumerate(_lhs_combos(o[:QB, :128], o[:QB, 128:], o[QB:, :128], o[QB:, 128:])):
                    g[c, d].append(v.astype(BF16))

        state = dict(dep=None, piece=0, window=0)
        jobs, pending, hs = [], [], {}
        tie = make_tie(jobs, 0.0)

        def next_block_ln():
            jobs.extend(pending)
            del pending[:]
            for _ in range(LN_PLAN[state['window']]):
                k, r = state['piece'] // 4, state['piece'] % 4
                pin = pltpu.bitcast(qka[16, pl.ds(0, 8), :], U32)
                dep = pin if state['dep'] is None else state['dep'] | pin
                state['dep'] = ln2_piece(hs, nxt, r * QB + 16 * k, dep)
                if r == 3:
                    pending.extend(functools.partial(lhs1_job, hs, nbase, k, t, c)
                                   for t in range(2) for c in range(7))
                state['piece'] += 1
            state['window'] += 1

        for n in range(2):
            def prod2(c, d):
                return _dot(jnp.concatenate(g[c, d], axis=1),
                            _bf(tie(rhs_load(w2, K2, N2, rhs2_loc, c, d, n), 1.0 / 24)))

            def outer(c):
                next_block_ln()
                y = _strassen_value(functools.partial(prod2, c))
                qka[17, pl.ds(srow, 8), :] = y[0:8, 0:128]
                return y

            def finish(y, rh, ch):
                for ci in range(2):
                    nn = (2 * ch + ci) * 2 + n
                    cols = pl.ds(nn * 128, 128)
                    yy = y[:, ci * 128:(ci + 1) * 128] + rep(biasb[:, pl.ds(FF + nn * 128, 128)], HB)
                    xr = pl.ds(pl.multiple_of(i * HB, HB) + rh * (HB // 2), HB // 2)
                    ar = pl.ds(pl.multiple_of(i * FB, FB) + rh * HB, HB)
                    x2 = _bf(xs[xr, cols]).astype(F32) + rep(modb[0, :, cols], HB) * ha[ar, cols]
                    qka[2 * nn + half, pl.ds(srow + rh * (HB // 2), HB // 2), :] = pack(
                        x2 + rep(modb[3, :, cols], HB) * yy, F32)
                    if rh == ch:
                        pltpu.make_async_copy(
                            qka.at[2 * nn + half, pl.ds(srow, HB), :],
                            out32.at[pl.ds(pl.multiple_of(i * HB, HB), HB), cols],
                            sem.at[SEM_OUT]).start()

            _strassen(outer, finish)
        assert not jobs and not pending and state['piece'] == 16
        return carry

    with jax.named_scope("p4_ffn"):
        lax.fori_loop(0, nb, ffn, 0)
    pltpu.make_async_copy(out32, out32, sem.at[SEM_OUT]).wait()


@jax.jit
def pallas_adaLN_cond__memory_aug_recurrent_mem_tr__dense_activation_gelu__prompt_kernel(
    A_x, A_mem0, A_Wq, A_Wk, A_Wv, A_Wo, A_seg_len, B_x, B_w1, B_b1, B_w2, B_b2, c, w_mod,
):
    assert A_x.shape == (1, S, D) and A_Wq.shape == (D, H, E) and A_mem0.shape == (1, M, D)
    any_spec = pl.BlockSpec(memory_space=pl.ANY)
    out = pl.pallas_call(
        _kernel,
        out_shape=jax.ShapeDtypeStruct((S, D), BF16),
        in_specs=[any_spec] * 12,
        out_specs=any_spec,
        scratch_shapes=[
            pltpu.VMEM((S // 2, D), U32),
            pltpu.VMEM((96, D // 2, E), U32),
            pltpu.VMEM((8, H * E // 2, 128), U32),
            pltpu.VMEM((D // 2, FF), U32),
            pltpu.VMEM((FF // 2, D), U32),
            pltpu.VMEM((H, RING, E), F32),
            pltpu.VMEM((H, RING, E), F32),
            pltpu.VMEM((H + 1, RING, E), F32),
            pltpu.VMEM((H, RING, E), F32),
            pltpu.VMEM((S, D), F32),
            pltpu.VMEM((S - PRE, D), F32),
            pltpu.VMEM((M, D), F32),
            pltpu.VMEM((NQ, 2, 8, KQ), F32),
            pltpu.VMEM((4, 8, D), F32),
            pltpu.VMEM((8, D), U32),
            pltpu.VMEM((8, FF + D), F32),
            pltpu.VMEM((80, 128), F32),
            pltpu.VMEM((8, 32, 128), F32),
            pltpu.VMEM((8, 128), U32),
            pltpu.SMEM((1,), jnp.int32),
            pltpu.VMEM((8, FF // 8, 128), U32),
            pltpu.VMEM((128, 256), U32),
            pltpu.VMEM((128, 256), U32),
            pltpu.VMEM((128, 256), U32),
            pltpu.VMEM((128, 256), U32),
            pltpu.VMEM((128, 256), U32),
            pltpu.VMEM((M, D), BF16),
            pltpu.VMEM((FF,), BF16),
            pltpu.VMEM((D,), BF16),
            pltpu.VMEM((1, D), BF16),
            pltpu.SemaphoreType.DMA((NSEM,)),
        ],
        compiler_params=pltpu.CompilerParams(vmem_limit_bytes=127 * 1024 * 1024, disable_bounds_checks=True,
                                             disable_semaphore_checks=True),
    )(
        A_x.reshape(S, D), A_mem0.reshape(M, D),
        A_Wq.reshape(D // 2, 2, H, E), A_Wk.reshape(D // 2, 2, H, E), A_Wv.reshape(D // 2, 2, H, E),
        A_Wo.reshape(H * E, D), B_w1, B_b1, B_w2, B_b2, c, w_mod,
    )
    return out.reshape(1, S, D)
```

```python
import functools
import math

import jax
import jax.numpy as jnp
from jax import lax
import jax.experimental.pallas as pl
import jax.experimental.pallas.tpu as pltpu

F32 = jnp.float32
BF16 = jnp.bfloat16
U32 = jnp.uint32

S = 2048
D = 1024
H = 32
E = 128
M = 8
SEG = 32
NSEG = S // SEG
FF = 3584
NP = H // 2
TOK = 24
PRE = S - NSEG * TOK
RING = 576
OOFF = (-NSEG * TOK) % RING
LN_EPS = 1e-5
FB = 256
XC = (S - PRE) // 6
P3_SPLIT = ((4, 8), (4, 16), (4, 16))
MOD_DENSITY = 0.07
LN0_PLAN = (6, 2, 2, 2, 2, 2, 0)
LN_PLAN = (1, 1, 1, 1, 1, 1, 1, 2, 2, 2, 2, 1, 0, 0)
FFN_DENSITY = 1.0 / 24
ATT_COL, ATT_N1, ATT_N2 = 6, 2, 5
UNROLL = 4

NQ = 4
KQ = D // NQ

FIRST_STARTS = [('m', 0), ('w', 0, 0, 2), ('w', 0, 2, 6), ('w', 0, 6, 12), ('m', 1), ('w', 1, 0, 6),
                ('w', 1, 6, 12), ('m', 2)]
P1A_BLOCKS = [
    ([], [('m', 0)]),
    ([], [('w', 0, 0, 2)]),
    ([], [('w', 0, 2, 6)]),
    ([('w', 2, 0, 6), ('w', 2, 6, 12)], [('w', 0, 6, 12)]),
    ([('m', 3), ('w', 3, 0, 6), ('w', 3, 6, 12)], [('m', 1), ('w', 1, 0, 6)]),
    ([], [('m', 2), ('w', 1, 6, 12)]),
    ([('g', 2), ('g', 3)], [('w', 2, 0, 6), ('w', 2, 6, 12)]),
    ([('g', 4), ('g', 5)], [('m', 3), ('w', 3, 0, 6), ('w', 3, 6, 12)]),
]
W_ITEMS = [it for _, items in P1A_BLOCKS for it in items if it[0] == 'w']
NX0 = 4

SEM_C = 0
SEM_X0 = 1
SEM_MOD = SEM_X0 + NX0
SEM_WA = SEM_MOD + NQ + 1
SEM_WB = SEM_WA + len(W_ITEMS)
SEM_XC = SEM_WB + 6
SEM_WO = SEM_XC + 6
SEM_W1 = SEM_WO + 1
SEM_W2 = SEM_W1 + 1
SEM_OUT = SEM_W2 + 1
NSEM = SEM_OUT + 1


def _ln(x):
    m = jnp.mean(x, axis=-1, keepdims=True)
    xc = x - m
    v = jnp.mean(xc * xc, axis=-1, keepdims=True)
    return xc * lax.rsqrt(v + LN_EPS)


def _bf(w32):
    return pltpu.bitcast(w32, BF16)


def _dot(a, b):
    return jnp.dot(a, b, preferred_element_type=F32)


def _lhs_combos(a11, a12, a21, a22):
    return [a11 + a22, a21 + a22, a11, a22, a11 + a12, a21 - a11, a12 - a22]


def _rhs_combos(b11, b12, b21, b22):
    return [b11 + b22, b11, b12 - b22, b21 - b11, b22, b11 + b12, b21 + b22]


_LHS_TERMS = {0: ((0, 0), (1, 1), 1), 1: ((1, 0), (1, 1), 1), 2: ((0, 0), None, 0), 3: ((1, 1), None, 0),
              4: ((0, 0), (0, 1), 1), 5: ((1, 0), (0, 0), -1), 6: ((0, 1), (1, 1), -1)}
_RHS_TERMS = {0: ((0, 0), (1, 1), 1), 1: ((0, 0), None, 0), 2: ((0, 1), (1, 1), -1), 3: ((1, 0), (0, 0), -1),
              4: ((1, 1), None, 0), 5: ((0, 0), (0, 1), 1), 6: ((1, 0), (1, 1), 1)}


def _combo(terms, c, blk):
    p, q, sign = terms[c]
    if q is None:
        return blk(*p)
    return blk(*p) + blk(*q) if sign > 0 else blk(*p) - blk(*q)


def _rhs_operand(c, blk):
    p, q, sign = _RHS_TERMS[c]
    a = _bf(blk(*p))
    if q is None:
        return a
    a = a.astype(F32)
    b = _bf(blk(*q)).astype(F32)
    return (a + b if sign > 0 else a - b).astype(BF16)


def _strassen(prod, finish, side=lambda: None):
    side()
    m1 = prod(1)
    m3 = prod(3)
    finish(m1 + m3, 1, 0)
    side()
    m2 = prod(2)
    m4 = prod(4)
    finish(m2 + m4, 0, 1)
    side()
    m0 = prod(0)
    m5 = prod(5)
    finish((m2 - m1) + m0 + m5, 1, 1)
    side()
    m6 = prod(6)
    finish((m3 - m4) + m0 + m6, 0, 0)


def _strassen_value(prod):
    r = {}
    _strassen(prod, lambda y, rh, ch: r.__setitem__((rh, ch), y))
    return jnp.concatenate([jnp.concatenate([r[0, 0], r[0, 1]], axis=1),
                            jnp.concatenate([r[1, 0], r[1, 1]], axis=1)], axis=0)


_ORDER = (1, 3, 2, 4, 0, 5, 6)

_PAIRS = [(c, d) for c in range(7) for d in range(7) if not (c in (1, 4) and d in (1, 4))]


def _kernel(x_hbm, mem0_hbm, wq_hbm, wk_hbm, wv_hbm, wo_hbm, w1_hbm, b1_hbm, w2_hbm, b2_hbm,
            c_hbm, wmod_hbm, out_hbm,
            xs, wqkv, wo, w1, w2, qka, qkb, vring, oring, ha, hn, memb, moda, modb, scb, biasb,
            fillb, accb, zerob, zero_s, wx, hb2, pk0, pk1, pk2, pk3, pk4, pk5, mem0_ref, b1_ref, b2_ref, c_ref, sem):
    qkv_hbm = [r.bitcast(U32) for r in (wq_hbm, wk_hbm, wv_hbm)]
    x32 = x_hbm.bitcast(U32)
    wo32 = wo_hbm.bitcast(U32)
    wmod32 = wmod_hbm.bitcast(F32)

    def wma(qq, k):
        return pl.ds(512 * (qq // 2), 512), pl.ds(512 * (qq % 2) + k * KQ, KQ)

    def hb_idx(c, q0, nq, row0=0, nrows=PRE // 4):
        return pl.ds(1024 + 128 * (c // 2) + row0, nrows), pl.ds(512 * (c % 2) + 128 * q0, 128 * nq)

    def units_start(lo, hi, rows, sem_idx):
        for u in range(lo, hi):
            j, m = u // 3, u % 3
            for p in range(2):
                pltpu.make_async_copy(qkv_hbm[m].at[rows, p, j, :], wqkv.at[2 * u + p, rows, :],
                                      sem.at[sem_idx]).start()

    def units_wait(lo, n, rows, sem_idx):
        blk = wqkv.at[pl.ds(2 * lo, 2 * n), rows, :]
        pltpu.make_async_copy(blk, blk, sem.at[sem_idx]).wait()

    def item_start(item):
        if item[0] == 'm':
            qq = item[1]
            for k in range(2):
                pltpu.make_async_copy(wmod32.at[:, pl.ds(k * D + qq * KQ, KQ)], ha.at[wma(qq, k)],
                                      sem.at[SEM_MOD + qq]).start()
        elif item[0] == 'w':
            _, qq, lo, hi = item
            units_start(lo, hi, pl.ds(qq * (KQ // 2), KQ // 2), SEM_WA + W_ITEMS.index(item))
        else:
            whole_start(item[1])

    def item_wait(item):
        if item[0] == 'm':
            qq = item[1]
            blk = ha.at[pl.ds(512 * (qq // 2), 512), pl.ds(512 * (qq % 2), 512)]
            pltpu.make_async_copy(blk, blk, sem.at[SEM_MOD + qq]).wait()
        else:
            _, qq, lo, hi = item
            units_wait(lo, hi - lo, pl.ds(qq * (KQ // 2), KQ // 2), SEM_WA + W_ITEMS.index(item))

    def whole_start(i):
        xc_copy(i - 2).start()
        units_start(6 * i, 6 * i + 6, pl.ds(0, D // 2), SEM_WB + i - 2)

    def mod_copy(n):
        return pltpu.make_async_copy(wmod32.at[:, pl.ds(2 * D + n * 128, 128)],
                                     qka.at[n, pl.ds(0, D // 2), :], sem.at[SEM_MOD + NQ])

    def x0_copy(i):
        n = PRE // 2 // NX0
        rows = pl.ds(pl.multiple_of(i * n, n), n)
        return pltpu.make_async_copy(x32.at[rows], xs.at[rows], sem.at[SEM_X0 + i])

    def xc_copy(i):
        rows = pl.ds(pl.multiple_of(PRE // 2 + i * (XC // 2), 64), XC // 2)
        return pltpu.make_async_copy(x32.at[rows], xs.at[rows], sem.at[SEM_XC + i])

    def wo_copy(n):
        return pltpu.make_async_copy(wo32.at[:, pl.ds(n * 128, 128)], wo.at[n], sem.at[SEM_WO])

    w1_copy = pltpu.make_async_copy(w1_hbm.bitcast(U32), w1, sem.at[SEM_W1])
    w2_copy = pltpu.make_async_copy(w2_hbm.bitcast(U32), w2, sem.at[SEM_W2])
    small_copies = [pltpu.make_async_copy(a, b, sem.at[SEM_C])
                    for a, b in ((c_hbm, c_ref), (mem0_hbm, mem0_ref), (b1_hbm, b1_ref),
                                 (b2_hbm, b2_ref))]

    def deinterleave(u, row0, nrows):
        for k in range(nrows // 64):
            rows = pl.ds(row0 + k * 64, 64)
            a = wqkv[2 * u, rows, :]
            b = wqkv[2 * u + 1, rows, :]
            wqkv[2 * u, rows, :] = (a & jnp.uint32(0xFFFF)) | (b << 16)
            wqkv[2 * u + 1, rows, :] = (a >> 16) | (b & jnp.uint32(0xFFFF0000))

    def load_x16(row2, dep):
        xw = xs[pl.ds(row2, 8), :]
        if dep is not None:
            first = xw[:, 0:128] | (dep & zerob[...])
            xw = jnp.concatenate([first, xw[:, 128:]], axis=1)
        return _bf(xw).astype(F32)

    pks = [pk0, pk1, pk2, pk3, pk4, pk5]

    def pack(v, dtype=U32):
        rows = pl.ds(0, v.shape[0] // 2)
        pk = pks[0]
        pk[rows, pl.ds(0, 128)] = pltpu.bitcast(v.astype(BF16), U32)
        return pltpu.bitcast(pk[rows, pl.ds(0, 128)], dtype)

    def rep(v8, n):
        return jnp.concatenate([v8] * (n // 8), axis=0)

    def mrow(k, n):
        if k < 2:
            return rep(jnp.concatenate([moda[qq, k] for qq in range(NQ)], axis=1), n)
        return rep(modb[k - 2], n)

    for cp in small_copies:
        cp.start()
    for i in range(NX0):
        x0_copy(i).start()
    for item in FIRST_STARTS:
        item_start(item)

    def start_rest():
        for n in range(8):
            wo_copy(n).start()
        w1_copy.start()
        w2_copy.start()

    r = lax.broadcasted_iota(jnp.int32, (80, 128), 0)
    q = lax.broadcasted_iota(jnp.int32, (80, 128), 1)
    r_tok = r < 64
    q_tok = q < 64
    r_head = jnp.where(r_tok, r >> 5, (r - 64) >> 3)
    q_head = jnp.where(q_tok, q >> 5, (q - 64) >> 3)
    same = (r_head == q_head) & (q < 80)
    causal_ok = jnp.logical_not(r_tok & q_tok & ((q & 31) > (r & 31)))
    scale = E ** (-0.5)
    fillb[...] = jnp.where(same, jnp.where(causal_ok, 0.0, -1e9 / scale), -jnp.inf).astype(F32)
    zerob[...] = jnp.zeros((8, 128), U32)
    zero_s[0] = 0

    for cp in small_copies:
        cp.wait()
    cf = c_ref[...].astype(F32)
    sc = (cf * jax.nn.sigmoid(cf)).astype(BF16)
    scb[...] = pltpu.bitcast(jnp.broadcast_to(sc, (16, D)), U32)
    memb[...] = mem0_ref[...].astype(F32)
    biasb[:, pl.ds(0, FF)] = jnp.broadcast_to(b1_ref[...].astype(F32).reshape(1, FF), (8, FF))
    biasb[:, pl.ds(FF, D)] = jnp.broadcast_to(b2_ref[...].astype(F32).reshape(1, D), (8, D))

    def pre_norm(i, carry):
        x0_copy(i).wait()
        nr = PRE // NX0
        for z in range(nr // 16):
            xn = _ln(load_x16(pl.multiple_of(i * (nr // 2) + z * 8, 8), None))
            for n in range(8):
                oring[n, pl.ds(pl.multiple_of(i * nr + z * 16, 16), 16), :] = xn[:, n * 128:(n + 1) * 128]
        return carry

    with jax.named_scope("p0_ln"):
        lax.fori_loop(0, NX0, pre_norm, 0)

    def dst_slot(i, k, p):
        cls, m = k // 3, k % 3
        if m == 2:
            return vring, 4 * i + 2 * cls + p
        return (qka, qkb)[cls], 4 * i + 2 * m + p

    PH = PRE // 2
    assert KQ == 256

    def item_run(item):
        if item[0] == 'm':
            qq = item[1]
            sc16 = _bf(scb[...])
            ca1 = 1.0 + _dot(sc16, _bf(ha[wma(qq, 1)]))[0:8].astype(BF16).astype(F32)
            sa = _dot(sc16, _bf(ha[wma(qq, 0)]))[0:8].astype(BF16).astype(F32)
            moda[qq, 0] = sa
            moda[qq, 1] = ca1
            for z in range(PH // 32):
                def h_blk(rh, kh):
                    cols = slice(kh * 128, (kh + 1) * 128)
                    return (oring[2 * qq + kh, pl.ds(rh * PH + z * 32, 32), :] * rep(ca1[:, cols], 32)
                            + rep(sa[:, cols], 32))

                for c, v in enumerate(_lhs_combos(h_blk(0, 0), h_blk(0, 1), h_blk(1, 0), h_blk(1, 1))):
                    ha[hb_idx(c, qq, 1, z * 16, 16)] = pltpu.bitcast(v.astype(BF16), F32)
            return
        _, qq, lo, hi = item
        if lo == 0 and qq >= 2:
            a_jobs.extend(functools.partial(lhs0_job, k, qq - 2, c) for k in range(PQ // 16) for c in range(7))
        for u in range(lo, hi):
            deinterleave(u, qq * (KQ // 2), KQ // 2)
            i, k = u // 6, u % 6

            def prod(c):
                lhs = pltpu.bitcast(ha[hb_idx(c, qq, 1)], U32)
                if u >= 2:
                    lhs = tie_rows(lhs, a_jobs, (8,))
                rhs = _rhs_operand(c, lambda a, b: wqkv[2 * u + b, pl.ds((2 * qq + a) * 64, 64), :])
                return _dot(_bf(lhs), rhs)

            def finish(y, rh, ch):
                ref, idx = dst_slot(i, k, ch)
                rows = pl.ds(RING - PRE + rh * PH, PH)
                if qq > 0:
                    y = y + ref[idx, rows, :]
                ref[idx, rows, :] = y

            _strassen(prod, finish)

    def tie_rows(w, jobs, groups):
        if not jobs:
            return w
        parts = [w[8 * g:8 * g + 8, 0:128] for g in range(w.shape[0] // 8)]
        for g in groups:
            if jobs:
                parts[g] = parts[g] | (jobs.pop(0)() & zerob[...])
        first = jnp.concatenate(parts, axis=0)
        return first if w.shape[1] == 128 else jnp.concatenate([first, w[:, 128:]], axis=1)

    PQ = PRE // 4
    a_jobs = []

    def lhs0_idx(c, d, k, nk, t, nt):
        e = 7 * c + d
        return pl.ds(64 * (e // 4) + 8 * k, 8 * nk), pl.ds(256 * (e % 4) + 128 * t, 128 * nt)

    def lhs0_job(k, t, c):
        def sub(ri, ki):
            def blk(ro, ko):
                n = 2 * ko + ki + 4 * t
                cols = pl.ds((n % 2) * 128, 128)
                return (oring[n, pl.ds((2 * ro + ri) * PQ + 16 * k, 16), :] * rep(moda[n // 2, 1, :, cols], 16)
                        + rep(moda[n // 2, 0, :, cols], 16))

            return _combo(_LHS_TERMS, c, blk)

        bits = None
        for d, v in enumerate(_lhs_combos(sub(0, 0), sub(0, 1), sub(1, 0), sub(1, 1))):
            hb2[lhs0_idx(c, d, k, 1, t, 1)] = pltpu.bitcast(v.astype(BF16), U32)
            if d not in (2, 3):
                b = pltpu.bitcast(v[8 * (d % 2):8 * (d % 2) + 8], U32)
                bits = b if bits is None else bits | b
        return bits

    def phase1b(i, carry):
        @pl.when(i == 3)
        def _():
            whole_start(6)
            whole_start(7)

        @pl.when(i == 4)
        def _():
            start_rest()

        xc_copy(i - 2).wait()
        units_wait(6 * i, 6, pl.ds(0, D // 2), SEM_WB + i - 2)
        state = dict(dep=None, piece=0)

        def ln1_piece():
            if state['piece'] < XC // 16:
                off = state['piece'] * 16
                x16 = load_x16(pl.multiple_of((i - 2) * (XC // 2), XC // 2) + (PRE + off) // 2, state['dep'])
                h16 = _ln(x16) * mrow(1, 16) + mrow(0, 16)
                hn[pl.ds(pl.multiple_of((i - 2) * XC, XC) + off, 16), :] = h16
                state['dep'] = pltpu.bitcast(h16[8:16, D - 128:], U32)
                state['piece'] += 1

        def raw(m, kq, nq, g):
            u = 6 * i + m + 3 * (nq // 2)
            return wqkv[2 * u + nq % 2, pl.ds((kq + 4 * (g // 8)) * 64 + 8 * (g % 8), 8), :]

        ops = {}

        def rhs0_job(m, c, g):
            def sub(ki, ni):
                return _combo(_RHS_TERMS, c,
                              lambda ko, no: _bf(raw(m, 2 * ko + ki, 2 * no + ni, g)).astype(F32))

            bits = None
            for d, v in enumerate(_rhs_combos(sub(0, 0), sub(0, 1), sub(1, 0), sub(1, 1))):
                if (c, d) in _PAIRS:
                    ops[m, c, d, g] = pack(v)
                    bits = ops[m, c, d, g] if bits is None else bits | ops[m, c, d, g]
            return bits

        seq = [(m, c) for m in range(3) for c in _ORDER]
        jobs = []
        deinterleave(6 * i, 0, D // 2)
        deinterleave(6 * i + 3, 0, D // 2)
        for g in range(16):
            rhs0_job(*seq[0], g)
        for m in range(3):
            if m < 2:
                deinterleave(6 * i + m + 1, 0, D // 2)
                deinterleave(6 * i + m + 4, 0, D // 2)

            def prod(c, d):
                if (c, d) in _PAIRS:
                    rhs = [ops[m, c, d, g] for g in range(16)]
                else:
                    q = 2 * (c // 4) + d // 4
                    rhs = [raw(m, q, q, g) for g in range(16)]
                lhs = tie_rows(hb2[lhs0_idx(c, d, 0, 8, 0, 2)], jobs, (1, 4, 7))
                return _dot(_bf(lhs), _bf(jnp.concatenate(rhs, axis=0)))

            def outer(c):
                ln1_piece()
                assert not jobs
                nx = seq.index((m, c)) + 1
                if nx < len(seq):
                    jobs.extend(functools.partial(rhs0_job, *seq[nx], g) for g in range(16))
                return _strassen_value(functools.partial(prod, c))

            def finish(y, rh, ch):
                for ci in range(2):
                    ref, idx = dst_slot(i, m + 3 * ch, ci)
                    ref[idx, pl.ds(RING - PRE + rh * PH, PH), :] = y[:, ci * 128:(ci + 1) * 128]

            _strassen(outer, finish)
        return carry

    for bi, (starts, items) in enumerate(P1A_BLOCKS):
        for item in starts:
            item_start(item)
        with jax.named_scope("p1a_wait%d" % bi):
            for item in items:
                item_wait(item)
        for item in items:
            item_run(item)
    assert not a_jobs
    with jax.named_scope("p1b"):
        lax.fori_loop(2, 8, phase1b, 0)
    pks.pop(0)
    for n in range(8):
        wo_copy(n).wait()

    cexp = scale * math.log2(math.e)
    NG = NP // 2
    grp = [(4 * (g // 2) + (g % 2), 4 * (g // 2) + (g % 2) + 2) for g in range(NG)]
    early = [2 * j + u for g in range(NG - 3) for j in grp[g] for u in range(2)]
    late = [h for h in range(H) if h not in early]

    def step(it, k):
        s = it * UNROLL + k
        split = k > 0
        base = TOK * UNROLL * it
        w0 = pl.multiple_of(lax.rem(base, RING), 32) + TOK * k
        r0 = pl.multiple_of(lax.rem(SEG * s + (RING - PRE), RING), 32)
        ow = pl.multiple_of(lax.rem(SEG * s + OOFF, RING), 32)
        o0 = pl.multiple_of(lax.rem(base + OOFF, RING), 32) + TOK * k
        a0 = pl.multiple_of(base, 32) + TOK * k
        X = jnp.concatenate([hn[pl.ds(a0, TOK), :], memb[...]], axis=0).astype(BF16)
        ym = [None] * 96
        probs = [None] * NP
        om = [None] * H
        order = (4, 5, 0, 1, 2, 3)

        if split:
            for t in order:
                accb[t] = _dot(X[:, :D // 2], _bf(wqkv[t, pl.ds(0, D // 4), :]))

        def slot(j, t):
            if t >= 4:
                return vring, 2 * j + t - 4
            return (qka, qkb)[j % 2], 4 * (j // 2) + t

        def proj(j, t):
            c = 6 * j + t
            if split and j == 0:
                y = accb[t] + _dot(X[:, D // 2:], _bf(wqkv[c, pl.ds(D // 4, D // 4), :]))
            else:
                y = _dot(X, _bf(wqkv[c]))
            ref, k = slot(j, t)
            ref[k, pl.ds(w0, TOK), :] = y[0:TOK]
            ym[c] = y[TOK:TOK + M]

        def gather(j, m, pad):
            c = 6 * j + 2 * m
            ref, k = slot(j, 2 * m)
            parts = [ref[k, pl.ds(r0, SEG), :], ref[k + 1, pl.ds(r0, SEG), :], ym[c], ym[c + 1]]
            if pad:
                parts.append(jnp.zeros((48, E), F32))
            return jnp.concatenate(parts, axis=0).astype(BF16)

        def scores(j):
            sc_ = lax.dot_general(gather(j, 0, False), gather(j, 1, True),
                                  (((1,), (1,)), ((), ())), preferred_element_type=F32)
            fill = fillb[...]
            sc_ = jnp.where(fill == 0.0, sc_, fill)
            mx = jnp.max(sc_, axis=-1, keepdims=True)
            p = jnp.exp2((sc_ - mx) * cexp)
            l = jnp.sum(p, axis=-1, keepdims=True)
            rl = pl.reciprocal(l, approx=True)
            rl = rl * (2.0 - l * rl)
            probs[j] = p * rl

        def park(j):
            vring[H, pl.ds(40 * (j % 8), 40), :] = pack(probs[j], F32)
            probs[j] = None

        def pv(j):
            if probs[j] is None:
                P = _bf(vring[H, pl.ds(40 * (j % 8), 40), :])
            else:
                P = probs[j].astype(BF16)
            o = _dot(P, gather(j, 2, True))
            oring[2 * j, pl.ds(ow, SEG), :] = o[0:32]
            oring[2 * j + 1, pl.ds(ow, SEG), :] = o[32:64]
            om[2 * j] = o[64:72]
            om[2 * j + 1] = o[72:80]

        def o_lhs(hs):
            return jnp.concatenate(
                [jnp.concatenate([oring[h, pl.ds(o0, TOK), :], om[h]], axis=0) for h in hs],
                axis=1).astype(BF16)

        def o_rhs(n, hs):
            return _bf(jnp.concatenate([wo[n, pl.ds(h * 64, 64), :] for h in hs], axis=0))

        for g in range(NG):
            cols = [(j, t) for j in grp[g] for t in order]
            if g == 2:
                cols = ([(j, t) for j in grp[g] for t in (4, 5)]
                        + [(j, t) for j in grp[g] for t in range(4)])
            for j in (grp[0] + grp[1] if g == 3 else grp[g - 2] if g >= 4 else ()):
                park(j)
            for ci, (j, t) in enumerate(cols):
                if g == 2 and ci == 4:
                    for jj in grp[0] + grp[1]:
                        scores(jj)
                if g >= 3 and ci == ATT_COL:
                    for jj in grp[g - 1]:
                        scores(jj)
                    for jj in grp[g - 3]:
                        pv(jj)
                proj(j, t)
        lo = o_lhs(early)
        for n in range(8):
            accb[n] = _dot(lo, o_rhs(n, early))
            if n == ATT_N1:
                for jj in grp[NG - 1]:
                    scores(jj)
                for jj in grp[NG - 3]:
                    pv(jj)
            if n == ATT_N2:
                for jj in grp[NG - 2] + grp[NG - 1]:
                    pv(jj)
        lo = o_lhs(late)
        for n in range(8):
            a = accb[n] + _dot(lo, o_rhs(n, late))
            ha[pl.ds(a0, TOK), pl.ds(n * 128, 128)] = a[0:TOK]
            memb[:, pl.ds(n * 128, 128)] = a[TOK:TOK + M]

    def steps(i, carry):
        for k in range(UNROLL):
            step(i, k)
        return carry

    with jax.named_scope("p2_steps"):
        lax.fori_loop(0, NSEG // UNROLL, steps, 0)

    for n in range(H):
        mod_copy(n).start()
    w1_copy.wait()
    w2_copy.wait()

    nb = S // FB
    HB = FB // 2
    QB = FB // 4

    def ln2_piece(hs, blk, off, dep):
        x2 = (load_x16(pl.multiple_of(blk * HB, HB) + off // 2, dep)
              + mrow(2, 16) * ha[pl.ds(pl.multiple_of(blk * FB, FB) + off, 16), :])
        h = _ln(x2) * mrow(4, 16) + mrow(3, 16)
        hs[off] = h
        return pltpu.bitcast(h[8:16, D - 128:], U32)

    def lhs1_loc(base, c, d):
        e = 7 * c + d
        return base + 32 * (e // 4), 256 * (e % 4)

    def lhs1_job(hs, base, k, t, c):
        def sub(ri, ki):
            def blk(ro, ko):
                c0 = (2 * ko + ki) * 256 + t * 128
                return hs[(2 * ro + ri) * QB + 16 * k][:, c0:c0 + 128]

            return _combo(_LHS_TERMS, c, blk)

        bits = None
        for d, v in enumerate(_lhs_combos(sub(0, 0), sub(0, 1), sub(1, 0), sub(1, 1))):
            r0, c0 = lhs1_loc(base, c, d)
            hn[pl.ds(r0 + 8 * k, 8), pl.ds(c0 + t * 128, 128)] = pltpu.bitcast(
                v.astype(BF16), F32)
            if d not in (2, 3):
                b = pltpu.bitcast(v[8 * (d % 2):8 * (d % 2) + 8], U32)
                bits = b if bits is None else bits | b
        return bits

    K1, N1, K2, N2 = D // 8, FF // 4, FF // 8, D // 4

    def rhs1_loc(c, d, n):
        e = _PAIRS.index((c, d)) * 7 + n
        return wqkv, e // 4, K1 * (e % 4)

    rhs2_slots = ([(wqkv, e, 0) for e in range(79, 96)] + [(qkb, e, 0) for e in range(H)]
                  + [(vring, e, 0) for e in range(H + 1)] + [(wx, e, 0) for e in range(8)])

    def rhs2_loc(c, d, n):
        return rhs2_slots[_PAIRS.index((c, d)) * 2 + n]

    def rhs_job(w, kq, nq, loc, n, r, cs):
        cache = {}

        def blk(ko, no, ki, ni):
            key = (2 * ko + ki, 2 * no + ni)
            if key not in cache:
                cache[key] = _bf(w[pl.ds(r + key[0] * kq, 8), pl.ds(n * 128 + key[1] * nq, 128)]).astype(F32)
            return cache[key]

        bits = None
        for c in cs:
            def sub(ki, ni):
                return _combo(_RHS_TERMS, c, lambda ko, no: blk(ko, no, ki, ni))

            for d, v in enumerate(_rhs_combos(sub(0, 0), sub(0, 1), sub(1, 0), sub(1, 1))):
                if (c, d) in _PAIRS:
                    ref, idx, row = loc(c, d, n)
                    b = pack(v)
                    ref[idx, pl.ds(row + r, 8), :] = pltpu.bitcast(b, ref.dtype)
                    bits = b if bits is None else bits | b
        return bits

    def rhs_load(w, kq, nq, loc, c, d, n):
        if (c, d) not in _PAIRS:
            q = 2 * (c // 4) + d // 4
            return w[pl.ds(q * kq, kq), pl.ds(q * nq + n * 128, 128)]
        ref, idx, row = loc(c, d, n)
        return pltpu.bitcast(ref[idx, pl.ds(row, kq), :], U32)

    def make_tie(jobs, credit):
        state = [credit]

        def tie(raw, density):
            if not jobs:
                return raw
            parts = []
            for r in range(0, raw.shape[0], 8):
                v = raw[r:r + 8]
                state[0] += density
                if jobs and state[0] >= 1.0:
                    state[0] -= 1.0
                    v = v | (jobs.pop(0)() & zerob[...])
                parts.append(v)
            return jnp.concatenate(parts, axis=0)

        return tie

    def w_jobs(r1, n1, r2, n2):
        return ([functools.partial(rhs_job, w1, K1, N1, rhs1_loc, n, r1 + 8 * j, [c])
                 for c in range(7) for n in range(7) for j in range(n1)]
                + [functools.partial(rhs_job, w2, K2, N2, rhs2_loc, n, r2 + 8 * j, [c])
                   for c in range(7) for n in range(2) for j in range(n2)])

    def bulk_o(lhs, n, jobs, side=lambda: None, density=None):
        if density is None:
            density = (len(jobs) + 4) / (7 * 64)
        credit = [-2.0]

        def tie_lhs(tiles):
            tiles = [[t[8 * g:8 * g + 8] for g in range(16)] for t in tiles]
            for w in range(4):
                for g in range(16):
                    credit[0] += density
                    for extra in range(2):
                        if jobs and credit[0] >= 1.0:
                            credit[0] -= 1.0
                            t = tiles[4 * w + (g + 2 * extra) % 4]
                            t[g] = t[g] | (jobs.pop(0)() & zerob[...])
            return _bf(jnp.concatenate([jnp.concatenate(t, axis=0) for t in tiles], axis=1))

        def prod(c):
            side()
            return _dot(tie_lhs(lhs[c]),
                        _rhs_operand(c, lambda a, b: wo[n + 4 * b, pl.ds(a * 1024, 1024), :]))

        def finish(y, rh, ch):
            cols = pl.ds(pl.multiple_of((n + 4 * ch) * 128, 128), 128)
            ha[pl.ds(NSEG * TOK + rh * 256, 256), cols] = y

        _strassen(prod, finish)
        assert not jobs

    def a_blk(rh, kh):
        return jnp.concatenate([oring[h, pl.ds(rh * 256, 256), :]
                                for h in range(16 * kh, 16 * kh + 16)], axis=1)

    (a1, a2), (m1, m2), (z1, z2) = P3_SPLIT
    assert a1 + 2 * m1 + z1 == K1 // 8 and a2 + 2 * m2 + z2 == K2 // 8
    pks.pop(0)
    with jax.named_scope("p3_first"):
        lhs_o = [[pack(v[:, 128 * t:128 * t + 128]) for t in range(16)]
                 for v in _lhs_combos(a_blk(0, 0), a_blk(0, 1), a_blk(1, 0), a_blk(1, 1))]
        bulk_o(lhs_o, 0, w_jobs(0, a1, 0, a2))
    pks.pop(0)

    def bulk_mid(n, carry):
        bulk_o(lhs_o, n, w_jobs(pl.multiple_of(8 * (a1 + (n - 1) * m1), 8), m1,
                                pl.multiple_of(8 * (a2 + (n - 1) * m2), 8), m2))
        return carry

    with jax.named_scope("p3_mid"):
        lax.fori_loop(1, 3, bulk_mid, 0)
    pks.pop(0)
    for n in range(H):
        mod_copy(n).wait()

    def bulk_last(zero):
        jobs = w_jobs(8 * (a1 + 2 * m1), z1, 8 * (a2 + 2 * m2), z2)
        tie = make_tie(jobs, 0.0)
        for g in range(4):
            for n in range(8):
                w = tie(pltpu.bitcast(qka[8 * g + n, pl.ds(0, D // 2), :], U32), MOD_DENSITY)
                y = _dot(_bf(scb[...]), _bf(w))[0:8].astype(BF16).astype(F32)
                modb[g, :, pl.ds(n * 128, 128)] = 1.0 + y if g == 2 else y
        density = (len(jobs) + 56 + 4) / (7 * 64)
        state = dict(dep=None, piece=0, window=0)
        pending = []
        hs = {}

        def side():
            jobs.extend(pending)
            del pending[:]
            for _ in range(LN0_PLAN[state['window']]):
                k, r = state['piece'] // 4, state['piece'] % 4
                state['dep'] = ln2_piece(hs, zero, r * QB + 16 * k, state['dep'])
                if r == 3:
                    pending.extend(functools.partial(lhs1_job, hs, 0, k, t, c)
                                   for t in range(2) for c in range(7))
                state['piece'] += 1
            state['window'] += 1

        bulk_o(lhs_o, 3, jobs, side, density)
        assert not pending and state['piece'] == 16

    with jax.named_scope("p3_last"):
        bulk_last(zero_s[0])

    pks.pop(0)
    out32 = out_hbm.bitcast(F32)
    qka[16, pl.ds(0, 8), :] = jnp.zeros((8, E), F32)

    def ffn(i, carry):
        base = pl.multiple_of((i & 1) * 512, 512)
        nbase = pl.multiple_of(((i + 1) & 1) * 512, 512)
        nxt = (i + 1) & (nb - 1)
        half = i >> 2
        srow = pl.multiple_of((i & 3) * HB, HB)

        g = {(c, d): [] for c in range(7) for d in range(7)}
        for n in range(7):
            act = {}

            def prod1(c, d):
                r0, c0 = lhs1_loc(base, c, d)
                return _dot(_bf(hn[pl.ds(r0, QB // 2), pl.ds(c0, 256)]),
                            _bf(rhs_load(w1, K1, N1, rhs1_loc, c, d, n)))

            def activate(y, rh, ch):
                b1 = jnp.concatenate([biasb[:, pl.ds((2 * ch + ci) * N1 + n * 128, 128)] for ci in range(2)],
                                     axis=1)
                act[rh, ch] = jax.nn.gelu(y + rep(b1, HB), approximate=True)

            _strassen(lambda c: _strassen_value(functools.partial(prod1, c)), activate)
            for c in range(7):
                o = _combo(_LHS_TERMS, c, lambda a, b: act[a, b])
                for d, v in enumerate(_lhs_combos(o[:QB, :128], o[:QB, 128:], o[QB:, :128], o[QB:, 128:])):
                    g[c, d].append(v.astype(BF16))

        state = dict(dep=None, piece=0, window=0)
        jobs, pending, hs = [], [], {}
        tie = make_tie(jobs, 0.0)

        def next_block_ln():
            jobs.extend(pending)
            del pending[:]
            for _ in range(LN_PLAN[state['window']]):
                k, r = state['piece'] // 4, state['piece'] % 4
                pin = pltpu.bitcast(qka[16, pl.ds(0, 8), :], U32)
                dep = pin if state['dep'] is None else state['dep'] | pin
                state['dep'] = ln2_piece(hs, nxt, r * QB + 16 * k, dep)
                if r == 3:
                    pending.extend(functools.partial(lhs1_job, hs, nbase, k, t, c)
                                   for t in range(2) for c in range(7))
                state['piece'] += 1
            state['window'] += 1

        for n in range(2):
            def prod2(c, d):
                return _dot(jnp.concatenate(g[c, d], axis=1),
                            _bf(tie(rhs_load(w2, K2, N2, rhs2_loc, c, d, n), FFN_DENSITY)))

            def outer(c):
                next_block_ln()
                y = _strassen_value(functools.partial(prod2, c))
                qka[17, pl.ds(srow, 8), :] = y[0:8, 0:128]
                return y

            def finish(y, rh, ch):
                for ci in range(2):
                    nn = (2 * ch + ci) * 2 + n
                    cols = pl.ds(nn * 128, 128)
                    yy = y[:, ci * 128:(ci + 1) * 128] + rep(biasb[:, pl.ds(FF + nn * 128, 128)], HB)
                    xr = pl.ds(pl.multiple_of(i * HB, HB) + rh * (HB // 2), HB // 2)
                    ar = pl.ds(pl.multiple_of(i * FB, FB) + rh * HB, HB)
                    x2 = _bf(xs[xr, cols]).astype(F32) + rep(modb[0, :, cols], HB) * ha[ar, cols]
                    qka[2 * nn + half, pl.ds(srow + rh * (HB // 2), HB // 2), :] = pack(
                        x2 + rep(modb[3, :, cols], HB) * yy, F32)
                    if rh == ch:
                        pltpu.make_async_copy(
                            qka.at[2 * nn + half, pl.ds(srow, HB), :],
                            out32.at[pl.ds(pl.multiple_of(i * HB, HB), HB), cols],
                            sem.at[SEM_OUT]).start()

            _strassen(outer, finish)
        assert not jobs and not pending and state['piece'] == 16
        return carry

    with jax.named_scope("p4_ffn"):
        lax.fori_loop(0, nb, ffn, 0)
    pltpu.make_async_copy(out32, out32, sem.at[SEM_OUT]).wait()


@jax.jit
def pallas_adaLN_cond__memory_aug_recurrent_mem_tr__dense_activation_gelu__prompt_kernel(
    A_x, A_mem0, A_Wq, A_Wk, A_Wv, A_Wo, A_seg_len, B_x, B_w1, B_b1, B_w2, B_b2, c, w_mod,
):
    assert A_x.shape == (1, S, D) and A_Wq.shape == (D, H, E) and A_mem0.shape == (1, M, D)
    any_spec = pl.BlockSpec(memory_space=pl.ANY)
    out = pl.pallas_call(
        _kernel,
        out_shape=jax.ShapeDtypeStruct((S, D), BF16),
        in_specs=[any_spec] * 12,
        out_specs=any_spec,
        scratch_shapes=[
            pltpu.VMEM((S // 2, D), U32),
            pltpu.VMEM((96, D // 2, E), U32),
            pltpu.VMEM((8, H * E // 2, 128), U32),
            pltpu.VMEM((D // 2, FF), U32),
            pltpu.VMEM((FF // 2, D), U32),
            pltpu.VMEM((H, RING, E), F32),
            pltpu.VMEM((H, RING, E), F32),
            pltpu.VMEM((H + 1, RING, E), F32),
            pltpu.VMEM((H, RING, E), F32),
            pltpu.VMEM((S, D), F32),
            pltpu.VMEM((S - PRE, D), F32),
            pltpu.VMEM((M, D), F32),
            pltpu.VMEM((NQ, 2, 8, KQ), F32),
            pltpu.VMEM((4, 8, D), F32),
            pltpu.VMEM((8, D), U32),
            pltpu.VMEM((8, FF + D), F32),
            pltpu.VMEM((80, 128), F32),
            pltpu.VMEM((8, 32, 128), F32),
            pltpu.VMEM((8, 128), U32),
            pltpu.SMEM((1,), jnp.int32),
            pltpu.VMEM((8, FF // 8, 128), U32),
            pltpu.VMEM((13 * 64, D), U32),
            pltpu.VMEM((128, 256), U32),
            pltpu.VMEM((128, 256), U32),
            pltpu.VMEM((128, 256), U32),
            pltpu.VMEM((128, 256), U32),
            pltpu.VMEM((128, 256), U32),
            pltpu.VMEM((128, 256), U32),
            pltpu.VMEM((M, D), BF16),
            pltpu.VMEM((FF,), BF16),
            pltpu.VMEM((D,), BF16),
            pltpu.VMEM((1, D), BF16),
            pltpu.SemaphoreType.DMA((NSEM,)),
        ],
        compiler_params=pltpu.CompilerParams(vmem_limit_bytes=127 * 1024 * 1024, disable_bounds_checks=True,
                                             disable_semaphore_checks=True),
    )(
        A_x.reshape(S, D), A_mem0.reshape(M, D),
        A_Wq.reshape(D // 2, 2, H, E), A_Wk.reshape(D // 2, 2, H, E), A_Wv.reshape(D // 2, 2, H, E),
        A_Wo.reshape(H * E, D), B_w1, B_b1, B_w2, B_b2, c, w_mod,
    )
    return out.reshape(1, S, D)
```

```python
import functools
import math

import jax
import jax.numpy as jnp
from jax import lax
import jax.experimental.pallas as pl
import jax.experimental.pallas.tpu as pltpu

F32 = jnp.float32
BF16 = jnp.bfloat16
U32 = jnp.uint32

S = 2048
D = 1024
H = 32
E = 128
M = 8
SEG = 32
NSEG = S // SEG
FF = 3584
NP = H // 2
TOK = 24
PRE = S - NSEG * TOK
RING = 576
OOFF = (-NSEG * TOK) % RING
LN_EPS = 1e-5
FB = 256
XC = (S - PRE) // 6
P3_SPLIT = ((4, 8), (4, 16), (4, 16))
MOD_DENSITY = 0.07
LN0_PLAN = (6, 2, 2, 2, 2, 2, 0)
LN_PLAN = (1, 1, 1, 1, 1, 1, 1, 2, 2, 2, 2, 1, 0, 0)
FFN_DENSITY = 1.0 / 24
ATT_COL, ATT_N1, ATT_N2 = 6, 2, 5
UNROLL = 4

NQ = 4
KQ = D // NQ

FIRST_STARTS = [('m', 0), ('w', 0, 0, 2), ('w', 0, 2, 6), ('w', 0, 6, 12), ('m', 1), ('w', 1, 0, 6),
                ('w', 1, 6, 12), ('m', 2)]
P1A_BLOCKS = [
    ([], [('m', 0)]),
    ([], [('w', 0, 0, 2)]),
    ([], [('w', 0, 2, 6)]),
    ([('w', 2, 0, 6), ('w', 2, 6, 12)], [('w', 0, 6, 12)]),
    ([('m', 3), ('w', 3, 0, 6), ('w', 3, 6, 12)], [('m', 1), ('w', 1, 0, 6)]),
    ([], [('m', 2), ('w', 1, 6, 12)]),
    ([('g', 2), ('g', 3)], [('w', 2, 0, 6), ('w', 2, 6, 12)]),
    ([('g', 4), ('g', 5)], [('m', 3), ('w', 3, 0, 6), ('w', 3, 6, 12)]),
]
W_ITEMS = [it for _, items in P1A_BLOCKS for it in items if it[0] == 'w']
NX0 = 4

SEM_C = 0
SEM_X0 = 1
SEM_MOD = SEM_X0 + NX0
SEM_WA = SEM_MOD + NQ + 1
SEM_WB = SEM_WA + len(W_ITEMS)
SEM_XC = SEM_WB + 6
SEM_WO = SEM_XC + 6
SEM_W1 = SEM_WO + 1
SEM_W2 = SEM_W1 + 1
SEM_OUT = SEM_W2 + 1
NSEM = SEM_OUT + 1


def _ln(x):
    m = jnp.mean(x, axis=-1, keepdims=True)
    xc = x - m
    v = jnp.mean(xc * xc, axis=-1, keepdims=True)
    return xc * lax.rsqrt(v + LN_EPS)


def _bf(w32):
    return pltpu.bitcast(w32, BF16)


def _dot(a, b):
    return jnp.dot(a, b, preferred_element_type=F32)


def _lhs_combos(a11, a12, a21, a22):
    return [a11 - a22, a21 - a22, a11, a22, a12 - a11, a21 - a11, a12 - a22]


def _rhs_combos(b11, b12, b21, b22):
    return [b11 - b22, b11, b12 + b22, b21 + b11, b22, b11 + b12, b21 + b22]


_LHS_TERMS = {0: ((0, 0), (1, 1), -1), 1: ((1, 0), (1, 1), -1), 2: ((0, 0), None, 0), 3: ((1, 1), None, 0),
              4: ((0, 1), (0, 0), -1), 5: ((1, 0), (0, 0), -1), 6: ((0, 1), (1, 1), -1)}
_RHS_TERMS = {0: ((0, 0), (1, 1), -1), 1: ((0, 0), None, 0), 2: ((0, 1), (1, 1), 1), 3: ((1, 0), (0, 0), 1),
              4: ((1, 1), None, 0), 5: ((0, 0), (0, 1), 1), 6: ((1, 0), (1, 1), 1)}
_SWAP = {c: int(c in (2, 4, 5, 6)) for c in range(7)}


def _combo(terms, c, blk):
    p, q, sign = terms[c]
    if q is None:
        return blk(*p)
    return blk(*p) + blk(*q) if sign > 0 else blk(*p) - blk(*q)


def _rhs_operand(c, blk):
    p, q, sign = _RHS_TERMS[c]
    a = _bf(blk(*p))
    if q is None:
        return a
    a = a.astype(F32)
    b = _bf(blk(*q)).astype(F32)
    return (a + b if sign > 0 else a - b).astype(BF16)


def _strassen(prod, finish, side=lambda: None):
    side()
    m1 = prod(1)
    m3 = prod(3)
    finish(m1 + m3, 1, 0)
    side()
    m2 = prod(2)
    m4 = prod(4)
    finish(m2 + m4, 0, 1)
    side()
    m0 = prod(0)
    m5 = prod(5)
    finish((m2 - m1) + m0 + m5, 1, 1)
    side()
    m6 = prod(6)
    finish((m3 - m4) + m0 + m6, 0, 0)


def _strassen_value(prod2, c):
    r = {}
    _strassen(functools.partial(prod2, c), lambda y, rh, ch: r.__setitem__((rh, ch ^ _SWAP[c]), y))
    return jnp.concatenate([jnp.concatenate([r[0, 0], r[0, 1]], axis=1),
                            jnp.concatenate([r[1, 0], r[1, 1]], axis=1)], axis=0)


_ORDER = (1, 3, 2, 4, 0, 5, 6)

_PAIRS = [(c, d) for c in range(7) for d in range(7) if not (c in (1, 4) and d in (1, 4))]


def _plain_block(c, d):
    return 2 * (c // 4) + d // 4, 2 * (c // 4) + ((d // 4) ^ _SWAP[c])


def _kernel(x_hbm, mem0_hbm, wq_hbm, wk_hbm, wv_hbm, wo_hbm, w1_hbm, b1_hbm, w2_hbm, b2_hbm,
            c_hbm, wmod_hbm, out_hbm,
            xs, wqkv, wo, w1, w2, qka, qkb, vring, oring, ha, hn, memb, moda, modb, scb, biasb,
            fillb, accb, zerob, zero_s, wx, hb2, pk0, pk1, pk2, pk3, pk4, pk5, mem0_ref, b1_ref, b2_ref, c_ref, sem):
    qkv_hbm = [r.bitcast(U32) for r in (wq_hbm, wk_hbm, wv_hbm)]
    x32 = x_hbm.bitcast(U32)
    wo32 = wo_hbm.bitcast(U32)
    wmod32 = wmod_hbm.bitcast(F32)

    def wma(qq, k):
        return pl.ds(512 * (qq // 2), 512), pl.ds(512 * (qq % 2) + k * KQ, KQ)

    def hb_idx(c, q0, nq, row0=0, nrows=PRE // 4):
        return pl.ds(1024 + 128 * (c // 2) + row0, nrows), pl.ds(512 * (c % 2) + 128 * q0, 128 * nq)

    def units_start(lo, hi, rows, sem_idx):
        for u in range(lo, hi):
            j, m = u // 3, u % 3
            for p in range(2):
                pltpu.make_async_copy(qkv_hbm[m].at[rows, p, j, :], wqkv.at[2 * u + p, rows, :],
                                      sem.at[sem_idx]).start()

    def units_wait(lo, n, rows, sem_idx):
        blk = wqkv.at[pl.ds(2 * lo, 2 * n), rows, :]
        pltpu.make_async_copy(blk, blk, sem.at[sem_idx]).wait()

    def item_start(item):
        if item[0] == 'm':
            qq = item[1]
            for k in range(2):
                pltpu.make_async_copy(wmod32.at[:, pl.ds(k * D + qq * KQ, KQ)], ha.at[wma(qq, k)],
                                      sem.at[SEM_MOD + qq]).start()
        elif item[0] == 'w':
            _, qq, lo, hi = item
            units_start(lo, hi, pl.ds(qq * (KQ // 2), KQ // 2), SEM_WA + W_ITEMS.index(item))
        else:
            whole_start(item[1])

    def item_wait(item):
        if item[0] == 'm':
            qq = item[1]
            blk = ha.at[pl.ds(512 * (qq // 2), 512), pl.ds(512 * (qq % 2), 512)]
            pltpu.make_async_copy(blk, blk, sem.at[SEM_MOD + qq]).wait()
        else:
            _, qq, lo, hi = item
            units_wait(lo, hi - lo, pl.ds(qq * (KQ // 2), KQ // 2), SEM_WA + W_ITEMS.index(item))

    def whole_start(i):
        xc_copy(i - 2).start()
        units_start(6 * i, 6 * i + 6, pl.ds(0, D // 2), SEM_WB + i - 2)

    def mod_copy(n):
        return pltpu.make_async_copy(wmod32.at[:, pl.ds(2 * D + n * 128, 128)],
                                     qka.at[n, pl.ds(0, D // 2), :], sem.at[SEM_MOD + NQ])

    def x0_copy(i):
        n = PRE // 2 // NX0
        rows = pl.ds(pl.multiple_of(i * n, n), n)
        return pltpu.make_async_copy(x32.at[rows], xs.at[rows], sem.at[SEM_X0 + i])

    def xc_copy(i):
        rows = pl.ds(pl.multiple_of(PRE // 2 + i * (XC // 2), 64), XC // 2)
        return pltpu.make_async_copy(x32.at[rows], xs.at[rows], sem.at[SEM_XC + i])

    def wo_copy(n):
        return pltpu.make_async_copy(wo32.at[:, pl.ds(n * 128, 128)], wo.at[n], sem.at[SEM_WO])

    w1_copy = pltpu.make_async_copy(w1_hbm.bitcast(U32), w1, sem.at[SEM_W1])
    w2_copy = pltpu.make_async_copy(w2_hbm.bitcast(U32), w2, sem.at[SEM_W2])
    small_copies = [pltpu.make_async_copy(a, b, sem.at[SEM_C])
                    for a, b in ((c_hbm, c_ref), (mem0_hbm, mem0_ref), (b1_hbm, b1_ref),
                                 (b2_hbm, b2_ref))]

    def deinterleave(u, row0, nrows):
        for k in range(nrows // 64):
            rows = pl.ds(row0 + k * 64, 64)
            a = wqkv[2 * u, rows, :]
            b = wqkv[2 * u + 1, rows, :]
            wqkv[2 * u, rows, :] = (a & jnp.uint32(0xFFFF)) | (b << 16)
            wqkv[2 * u + 1, rows, :] = (a >> 16) | (b & jnp.uint32(0xFFFF0000))

    def load_x16(row2, dep):
        xw = xs[pl.ds(row2, 8), :]
        if dep is not None:
            first = xw[:, 0:128] | (dep & zerob[...])
            xw = jnp.concatenate([first, xw[:, 128:]], axis=1)
        return _bf(xw).astype(F32)

    pks = [pk0, pk1, pk2, pk3, pk4, pk5]

    def pack(v, dtype=U32):
        rows = pl.ds(0, v.shape[0] // 2)
        pk = pks[0]
        pk[rows, pl.ds(0, 128)] = pltpu.bitcast(v.astype(BF16), U32)
        return pltpu.bitcast(pk[rows, pl.ds(0, 128)], dtype)

    def rep(v8, n):
        return jnp.concatenate([v8] * (n // 8), axis=0)

    def mrow(k, n):
        if k < 2:
            return rep(jnp.concatenate([moda[qq, k] for qq in range(NQ)], axis=1), n)
        return rep(modb[k - 2], n)

    for cp in small_copies:
        cp.start()
    for i in range(NX0):
        x0_copy(i).start()
    for item in FIRST_STARTS:
        item_start(item)

    def start_rest():
        for n in range(8):
            wo_copy(n).start()
        w1_copy.start()
        w2_copy.start()

    r = lax.broadcasted_iota(jnp.int32, (80, 128), 0)
    q = lax.broadcasted_iota(jnp.int32, (80, 128), 1)
    r_tok = r < 64
    q_tok = q < 64
    r_head = jnp.where(r_tok, r >> 5, (r - 64) >> 3)
    q_head = jnp.where(q_tok, q >> 5, (q - 64) >> 3)
    same = (r_head == q_head) & (q < 80)
    causal_ok = jnp.logical_not(r_tok & q_tok & ((q & 31) > (r & 31)))
    scale = E ** (-0.5)
    fillb[...] = jnp.where(same, jnp.where(causal_ok, 0.0, -1e9 / scale), -jnp.inf).astype(F32)
    zerob[...] = jnp.zeros((8, 128), U32)
    zero_s[0] = 0

    for cp in small_copies:
        cp.wait()
    cf = c_ref[...].astype(F32)
    sc = (cf * jax.nn.sigmoid(cf)).astype(BF16)
    scb[...] = pltpu.bitcast(jnp.broadcast_to(sc, (16, D)), U32)
    memb[...] = mem0_ref[...].astype(F32)
    biasb[:, pl.ds(0, FF)] = jnp.broadcast_to(b1_ref[...].astype(F32).reshape(1, FF), (8, FF))
    biasb[:, pl.ds(FF, D)] = jnp.broadcast_to(b2_ref[...].astype(F32).reshape(1, D), (8, D))

    def pre_norm(i, carry):
        x0_copy(i).wait()
        nr = PRE // NX0
        for z in range(nr // 16):
            xn = _ln(load_x16(pl.multiple_of(i * (nr // 2) + z * 8, 8), None))
            for n in range(8):
                oring[n, pl.ds(pl.multiple_of(i * nr + z * 16, 16), 16), :] = xn[:, n * 128:(n + 1) * 128]
        return carry

    with jax.named_scope("p0_ln"):
        lax.fori_loop(0, NX0, pre_norm, 0)

    def dst_slot(i, k, p):
        cls, m = k // 3, k % 3
        if m == 2:
            return vring, 4 * i + 2 * cls + p
        return (qka, qkb)[cls], 4 * i + 2 * m + p

    PH = PRE // 2
    assert KQ == 256

    def item_run(item):
        if item[0] == 'm':
            qq = item[1]
            sc16 = _bf(scb[...])
            ca1 = 1.0 + _dot(sc16, _bf(ha[wma(qq, 1)]))[0:8].astype(BF16).astype(F32)
            sa = _dot(sc16, _bf(ha[wma(qq, 0)]))[0:8].astype(BF16).astype(F32)
            moda[qq, 0] = sa
            moda[qq, 1] = ca1
            for z in range(PH // 32):
                def h_blk(rh, kh):
                    cols = slice(kh * 128, (kh + 1) * 128)
                    return (oring[2 * qq + kh, pl.ds(rh * PH + z * 32, 32), :] * rep(ca1[:, cols], 32)
                            + rep(sa[:, cols], 32))

                for c, v in enumerate(_lhs_combos(h_blk(0, 0), h_blk(0, 1), h_blk(1, 0), h_blk(1, 1))):
                    ha[hb_idx(c, qq, 1, z * 16, 16)] = pltpu.bitcast(v.astype(BF16), F32)
            return
        _, qq, lo, hi = item
        if lo == 0 and qq >= 2:
            a_jobs.extend(functools.partial(lhs0_job, k, qq - 2, c) for k in range(PQ // 16) for c in range(7))
        for u in range(lo, hi):
            deinterleave(u, qq * (KQ // 2), KQ // 2)
            i, k = u // 6, u % 6

            def prod(c):
                lhs = pltpu.bitcast(ha[hb_idx(c, qq, 1)], U32)
                if u >= 2:
                    lhs = tie_rows(lhs, a_jobs, (8,))
                rhs = _rhs_operand(c, lambda a, b: wqkv[2 * u + b, pl.ds((2 * qq + a) * 64, 64), :])
                return _dot(_bf(lhs), rhs)

            def finish(y, rh, ch):
                ref, idx = dst_slot(i, k, ch)
                rows = pl.ds(RING - PRE + rh * PH, PH)
                if qq > 0:
                    y = y + ref[idx, rows, :]
                ref[idx, rows, :] = y

            _strassen(prod, finish)

    def tie_rows(w, jobs, groups):
        if not jobs:
            return w
        parts = [w[8 * g:8 * g + 8, 0:128] for g in range(w.shape[0] // 8)]
        for g in groups:
            if jobs:
                parts[g] = parts[g] | (jobs.pop(0)() & zerob[...])
        first = jnp.concatenate(parts, axis=0)
        return first if w.shape[1] == 128 else jnp.concatenate([first, w[:, 128:]], axis=1)

    PQ = PRE // 4
    a_jobs = []

    def lhs0_idx(c, d, k, nk, t, nt):
        e = 7 * c + d
        return pl.ds(64 * (e // 4) + 8 * k, 8 * nk), pl.ds(256 * (e % 4) + 128 * t, 128 * nt)

    def lhs0_job(k, t, c):
        def sub(ri, ki):
            def blk(ro, ko):
                n = 2 * ko + ki + 4 * t
                cols = pl.ds((n % 2) * 128, 128)
                return (oring[n, pl.ds((2 * ro + ri) * PQ + 16 * k, 16), :] * rep(moda[n // 2, 1, :, cols], 16)
                        + rep(moda[n // 2, 0, :, cols], 16))

            return _combo(_LHS_TERMS, c, blk)

        bits = None
        for d, v in enumerate(_lhs_combos(sub(0, 0), sub(0, 1), sub(1, 0), sub(1, 1))):
            hb2[lhs0_idx(c, d, k, 1, t, 1)] = pltpu.bitcast(v.astype(BF16), U32)
            if d not in (2, 3):
                b = pltpu.bitcast(v[8 * (d % 2):8 * (d % 2) + 8], U32)
                bits = b if bits is None else bits | b
        return bits

    def phase1b(i, carry):
        @pl.when(i == 3)
        def _():
            whole_start(6)
            whole_start(7)

        @pl.when(i == 4)
        def _():
            start_rest()

        xc_copy(i - 2).wait()
        units_wait(6 * i, 6, pl.ds(0, D // 2), SEM_WB + i - 2)
        state = dict(dep=None, piece=0)

        def ln1_piece():
            if state['piece'] < XC // 16:
                off = state['piece'] * 16
                x16 = load_x16(pl.multiple_of((i - 2) * (XC // 2), XC // 2) + (PRE + off) // 2, state['dep'])
                h16 = _ln(x16) * mrow(1, 16) + mrow(0, 16)
                hn[pl.ds(pl.multiple_of((i - 2) * XC, XC) + off, 16), :] = h16
                state['dep'] = pltpu.bitcast(h16[8:16, D - 128:], U32)
                state['piece'] += 1

        def raw(m, kq, nq, g):
            u = 6 * i + m + 3 * (nq // 2)
            return wqkv[2 * u + nq % 2, pl.ds((kq + 4 * (g // 8)) * 64 + 8 * (g % 8), 8), :]

        ops = {}

        def rhs0_job(m, c, g):
            def sub(ki, ni):
                return _combo(_RHS_TERMS, c,
                              lambda ko, no: _bf(raw(m, 2 * ko + ki, 2 * no + (ni ^ _SWAP[c]), g)).astype(F32))

            bits = None
            for d, v in enumerate(_rhs_combos(sub(0, 0), sub(0, 1), sub(1, 0), sub(1, 1))):
                if (c, d) in _PAIRS:
                    ops[m, c, d, g] = pack(v)
                    bits = ops[m, c, d, g] if bits is None else bits | ops[m, c, d, g]
            return bits

        seq = [(m, c) for m in range(3) for c in _ORDER]
        jobs = []
        deinterleave(6 * i, 0, D // 2)
        deinterleave(6 * i + 3, 0, D // 2)
        for g in range(16):
            rhs0_job(*seq[0], g)
        for m in range(3):
            if m < 2:
                deinterleave(6 * i + m + 1, 0, D // 2)
                deinterleave(6 * i + m + 4, 0, D // 2)

            def prod(c, d):
                if (c, d) in _PAIRS:
                    rhs = [ops[m, c, d, g] for g in range(16)]
                else:
                    rhs = [raw(m, *_plain_block(c, d), g) for g in range(16)]
                lhs = tie_rows(hb2[lhs0_idx(c, d, 0, 8, 0, 2)], jobs, (1, 4, 7))
                return _dot(_bf(lhs), _bf(jnp.concatenate(rhs, axis=0)))

            def outer(c):
                ln1_piece()
                assert not jobs
                nx = seq.index((m, c)) + 1
                if nx < len(seq):
                    jobs.extend(functools.partial(rhs0_job, *seq[nx], g) for g in range(16))
                return _strassen_value(prod, c)

            def finish(y, rh, ch):
                for ci in range(2):
                    ref, idx = dst_slot(i, m + 3 * ch, ci)
                    ref[idx, pl.ds(RING - PRE + rh * PH, PH), :] = y[:, ci * 128:(ci + 1) * 128]

            _strassen(outer, finish)
        return carry

    for bi, (starts, items) in enumerate(P1A_BLOCKS):
        for item in starts:
            item_start(item)
        with jax.named_scope("p1a_wait%d" % bi):
            for item in items:
                item_wait(item)
        for item in items:
            item_run(item)
    assert not a_jobs
    with jax.named_scope("p1b"):
        lax.fori_loop(2, 8, phase1b, 0)
    pks.pop(0)
    for n in range(8):
        wo_copy(n).wait()

    cexp = scale * math.log2(math.e)
    NG = NP // 2
    grp = [(4 * (g // 2) + (g % 2), 4 * (g // 2) + (g % 2) + 2) for g in range(NG)]
    early = [2 * j + u for g in range(NG - 3) for j in grp[g] for u in range(2)]
    late = [h for h in range(H) if h not in early]

    def step(it, k):
        s = it * UNROLL + k
        split = k > 0
        base = TOK * UNROLL * it
        w0 = pl.multiple_of(lax.rem(base, RING), 32) + TOK * k
        r0 = pl.multiple_of(lax.rem(SEG * s + (RING - PRE), RING), 32)
        ow = pl.multiple_of(lax.rem(SEG * s + OOFF, RING), 32)
        o0 = pl.multiple_of(lax.rem(base + OOFF, RING), 32) + TOK * k
        a0 = pl.multiple_of(base, 32) + TOK * k
        X = jnp.concatenate([hn[pl.ds(a0, TOK), :], memb[...]], axis=0).astype(BF16)
        ym = [None] * 96
        probs = [None] * NP
        om = [None] * H
        order = (4, 5, 0, 1, 2, 3)

        if split:
            for t in order:
                accb[t] = _dot(X[:, :D // 2], _bf(wqkv[t, pl.ds(0, D // 4), :]))

        def slot(j, t):
            if t >= 4:
                return vring, 2 * j + t - 4
            return (qka, qkb)[j % 2], 4 * (j // 2) + t

        def proj(j, t):
            c = 6 * j + t
            if split and j == 0:
                y = accb[t] + _dot(X[:, D // 2:], _bf(wqkv[c, pl.ds(D // 4, D // 4), :]))
            else:
                y = _dot(X, _bf(wqkv[c]))
            ref, k = slot(j, t)
            ref[k, pl.ds(w0, TOK), :] = y[0:TOK]
            ym[c] = y[TOK:TOK + M]

        def gather(j, m, pad):
            c = 6 * j + 2 * m
            ref, k = slot(j, 2 * m)
            parts = [ref[k, pl.ds(r0, SEG), :], ref[k + 1, pl.ds(r0, SEG), :], ym[c], ym[c + 1]]
            if pad:
                parts.append(jnp.zeros((48, E), F32))
            return jnp.concatenate(parts, axis=0).astype(BF16)

        def scores(j):
            sc_ = lax.dot_general(gather(j, 0, False), gather(j, 1, True),
                                  (((1,), (1,)), ((), ())), preferred_element_type=F32)
            fill = fillb[...]
            sc_ = jnp.where(fill == 0.0, sc_, fill)
            mx = jnp.max(sc_, axis=-1, keepdims=True)
            p = jnp.exp2((sc_ - mx) * cexp)
            l = jnp.sum(p, axis=-1, keepdims=True)
            rl = pl.reciprocal(l, approx=True)
            rl = rl * (2.0 - l * rl)
            probs[j] = p * rl

        def park(j):
            vring[H, pl.ds(40 * (j % 8), 40), :] = pack(probs[j], F32)
            probs[j] = None

        def pv(j):
            if probs[j] is None:
                P = _bf(vring[H, pl.ds(40 * (j % 8), 40), :])
            else:
                P = probs[j].astype(BF16)
            o = _dot(P, gather(j, 2, True))
            oring[2 * j, pl.ds(ow, SEG), :] = o[0:32]
            oring[2 * j + 1, pl.ds(ow, SEG), :] = o[32:64]
            om[2 * j] = o[64:72]
            om[2 * j + 1] = o[72:80]

        def o_lhs(hs):
            return jnp.concatenate(
                [jnp.concatenate([oring[h, pl.ds(o0, TOK), :], om[h]], axis=0) for h in hs],
                axis=1).astype(BF16)

        def o_rhs(n, hs):
            return _bf(jnp.concatenate([wo[n, pl.ds(h * 64, 64), :] for h in hs], axis=0))

        for g in range(NG):
            cols = [(j, t) for j in grp[g] for t in order]
            if g == 2:
                cols = ([(j, t) for j in grp[g] for t in (4, 5)]
                        + [(j, t) for j in grp[g] for t in range(4)])
            for j in (grp[0] + grp[1] if g == 3 else grp[g - 2] if g >= 4 else ()):
                park(j)
            for ci, (j, t) in enumerate(cols):
                if g == 2 and ci == 4:
                    for jj in grp[0] + grp[1]:
                        scores(jj)
                if g >= 3 and ci == ATT_COL:
                    for jj in grp[g - 1]:
                        scores(jj)
                    for jj in grp[g - 3]:
                        pv(jj)
                proj(j, t)
        lo = o_lhs(early)
        for n in range(8):
            accb[n] = _dot(lo, o_rhs(n, early))
            if n == ATT_N1:
                for jj in grp[NG - 1]:
                    scores(jj)
                for jj in grp[NG - 3]:
                    pv(jj)
            if n == ATT_N2:
                for jj in grp[NG - 2] + grp[NG - 1]:
                    pv(jj)
        lo = o_lhs(late)
        for n in range(8):
            a = accb[n] + _dot(lo, o_rhs(n, late))
            ha[pl.ds(a0, TOK), pl.ds(n * 128, 128)] = a[0:TOK]
            memb[:, pl.ds(n * 128, 128)] = a[TOK:TOK + M]

    def steps(i, carry):
        for k in range(UNROLL):
            step(i, k)
        return carry

    with jax.named_scope("p2_steps"):
        lax.fori_loop(0, NSEG // UNROLL, steps, 0)

    for n in range(H):
        mod_copy(n).start()
    w1_copy.wait()
    w2_copy.wait()

    nb = S // FB
    HB = FB // 2
    QB = FB // 4

    def ln2_piece(hs, blk, off, dep):
        x2 = (load_x16(pl.multiple_of(blk * HB, HB) + off // 2, dep)
              + mrow(2, 16) * ha[pl.ds(pl.multiple_of(blk * FB, FB) + off, 16), :])
        h = _ln(x2) * mrow(4, 16) + mrow(3, 16)
        hs[off] = h
        return pltpu.bitcast(h[8:16, D - 128:], U32)

    def lhs1_loc(base, c, d):
        e = 7 * c + d
        return base + 32 * (e // 4), 256 * (e % 4)

    def lhs1_job(hs, base, k, t, c):
        def sub(ri, ki):
            def blk(ro, ko):
                c0 = (2 * ko + ki) * 256 + t * 128
                return hs[(2 * ro + ri) * QB + 16 * k][:, c0:c0 + 128]

            return _combo(_LHS_TERMS, c, blk)

        bits = None
        for d, v in enumerate(_lhs_combos(sub(0, 0), sub(0, 1), sub(1, 0), sub(1, 1))):
            r0, c0 = lhs1_loc(base, c, d)
            hn[pl.ds(r0 + 8 * k, 8), pl.ds(c0 + t * 128, 128)] = pltpu.bitcast(
                v.astype(BF16), F32)
            if d not in (2, 3):
                b = pltpu.bitcast(v[8 * (d % 2):8 * (d % 2) + 8], U32)
                bits = b if bits is None else bits | b
        return bits

    K1, N1, K2, N2 = D // 8, FF // 4, FF // 8, D // 4

    def rhs1_loc(c, d, n):
        e = _PAIRS.index((c, d)) * 7 + n
        return wqkv, e // 4, K1 * (e % 4)

    rhs2_slots = ([(wqkv, e, 0) for e in range(79, 96)] + [(qkb, e, 0) for e in range(H)]
                  + [(vring, e, 0) for e in range(H + 1)] + [(wx, e, 0) for e in range(8)])

    def rhs2_loc(c, d, n):
        return rhs2_slots[_PAIRS.index((c, d)) * 2 + n]

    def rhs_job(w, kq, nq, loc, n, r, cs):
        cache = {}

        def blk(ko, no, ki, ni):
            key = (2 * ko + ki, 2 * no + ni)
            if key not in cache:
                cache[key] = _bf(w[pl.ds(r + key[0] * kq, 8), pl.ds(n * 128 + key[1] * nq, 128)]).astype(F32)
            return cache[key]

        bits = None
        for c in cs:
            def sub(ki, ni):
                return _combo(_RHS_TERMS, c, lambda ko, no: blk(ko, no, ki, ni ^ _SWAP[c]))

            for d, v in enumerate(_rhs_combos(sub(0, 0), sub(0, 1), sub(1, 0), sub(1, 1))):
                if (c, d) in _PAIRS:
                    ref, idx, row = loc(c, d, n)
                    b = pack(v)
                    ref[idx, pl.ds(row + r, 8), :] = pltpu.bitcast(b, ref.dtype)
                    bits = b if bits is None else bits | b
        return bits

    def rhs_load(w, kq, nq, loc, c, d, n):
        if (c, d) not in _PAIRS:
            qk, qn = _plain_block(c, d)
            return w[pl.ds(qk * kq, kq), pl.ds(qn * nq + n * 128, 128)]
        ref, idx, row = loc(c, d, n)
        return pltpu.bitcast(ref[idx, pl.ds(row, kq), :], U32)

    def make_tie(jobs, credit):
        state = [credit]

        def tie(raw, density):
            if not jobs:
                return raw
            parts = []
            for r in range(0, raw.shape[0], 8):
                v = raw[r:r + 8]
                state[0] += density
                if jobs and state[0] >= 1.0:
                    state[0] -= 1.0
                    v = v | (jobs.pop(0)() & zerob[...])
                parts.append(v)
            return jnp.concatenate(parts, axis=0)

        return tie

    def w_jobs(r1, n1, r2, n2):
        return ([functools.partial(rhs_job, w1, K1, N1, rhs1_loc, n, r1 + 8 * j, [c])
                 for c in range(7) for n in range(7) for j in range(n1)]
                + [functools.partial(rhs_job, w2, K2, N2, rhs2_loc, n, r2 + 8 * j, [c])
                   for c in range(7) for n in range(2) for j in range(n2)])

    def bulk_o(lhs, n, jobs, side=lambda: None, density=None):
        if density is None:
            density = (len(jobs) + 4) / (7 * 64)
        credit = [-2.0]

        def tie_lhs(tiles):
            tiles = [[t[8 * g:8 * g + 8] for g in range(16)] for t in tiles]
            for w in range(4):
                for g in range(16):
                    credit[0] += density
                    for extra in range(2):
                        if jobs and credit[0] >= 1.0:
                            credit[0] -= 1.0
                            t = tiles[4 * w + (g + 2 * extra) % 4]
                            t[g] = t[g] | (jobs.pop(0)() & zerob[...])
            return _bf(jnp.concatenate([jnp.concatenate(t, axis=0) for t in tiles], axis=1))

        def prod(c):
            side()
            return _dot(tie_lhs(lhs[c]),
                        _rhs_operand(c, lambda a, b: wo[n + 4 * b, pl.ds(a * 1024, 1024), :]))

        def finish(y, rh, ch):
            cols = pl.ds(pl.multiple_of((n + 4 * ch) * 128, 128), 128)
            ha[pl.ds(NSEG * TOK + rh * 256, 256), cols] = y

        _strassen(prod, finish)
        assert not jobs

    def a_blk(rh, kh):
        return jnp.concatenate([oring[h, pl.ds(rh * 256, 256), :]
                                for h in range(16 * kh, 16 * kh + 16)], axis=1)

    (a1, a2), (m1, m2), (z1, z2) = P3_SPLIT
    assert a1 + 2 * m1 + z1 == K1 // 8 and a2 + 2 * m2 + z2 == K2 // 8
    pks.pop(0)
    with jax.named_scope("p3_first"):
        lhs_o = [[pack(v[:, 128 * t:128 * t + 128]) for t in range(16)]
                 for v in _lhs_combos(a_blk(0, 0), a_blk(0, 1), a_blk(1, 0), a_blk(1, 1))]
        bulk_o(lhs_o, 0, w_jobs(0, a1, 0, a2))
    pks.pop(0)

    def bulk_mid(n, carry):
        bulk_o(lhs_o, n, w_jobs(pl.multiple_of(8 * (a1 + (n - 1) * m1), 8), m1,
                                pl.multiple_of(8 * (a2 + (n - 1) * m2), 8), m2))
        return carry

    with jax.named_scope("p3_mid"):
        lax.fori_loop(1, 3, bulk_mid, 0)
    pks.pop(0)
    for n in range(H):
        mod_copy(n).wait()

    def bulk_last(zero):
        jobs = w_jobs(8 * (a1 + 2 * m1), z1, 8 * (a2 + 2 * m2), z2)
        tie = make_tie(jobs, 0.0)
        for g in range(4):
            for n in range(8):
                w = tie(pltpu.bitcast(qka[8 * g + n, pl.ds(0, D // 2), :], U32), MOD_DENSITY)
                y = _dot(_bf(scb[...]), _bf(w))[0:8].astype(BF16).astype(F32)
                modb[g, :, pl.ds(n * 128, 128)] = 1.0 + y if g == 2 else y
        density = (len(jobs) + 56 + 4) / (7 * 64)
        state = dict(dep=None, piece=0, window=0)
        pending = []
        hs = {}

        def side():
            jobs.extend(pending)
            del pending[:]
            for _ in range(LN0_PLAN[state['window']]):
                k, r = state['piece'] // 4, state['piece'] % 4
                state['dep'] = ln2_piece(hs, zero, r * QB + 16 * k, state['dep'])
                if r == 3:
                    pending.extend(functools.partial(lhs1_job, hs, 0, k, t, c)
                                   for t in range(2) for c in range(7))
                state['piece'] += 1
            state['window'] += 1

        bulk_o(lhs_o, 3, jobs, side, density)
        assert not pending and state['piece'] == 16

    with jax.named_scope("p3_last"):
        bulk_last(zero_s[0])

    pks.pop(0)
    out32 = out_hbm.bitcast(F32)
    qka[16, pl.ds(0, 8), :] = jnp.zeros((8, E), F32)

    def ffn(i, carry):
        base = pl.multiple_of((i & 1) * 512, 512)
        nbase = pl.multiple_of(((i + 1) & 1) * 512, 512)
        nxt = (i + 1) & (nb - 1)
        half = i >> 2
        srow = pl.multiple_of((i & 3) * HB, HB)

        g = {(c, d): [] for c in range(7) for d in range(7)}
        for n in range(7):
            act = {}

            def prod1(c, d):
                r0, c0 = lhs1_loc(base, c, d)
                return _dot(_bf(hn[pl.ds(r0, QB // 2), pl.ds(c0, 256)]),
                            _bf(rhs_load(w1, K1, N1, rhs1_loc, c, d, n)))

            def activate(y, rh, ch):
                b1 = jnp.concatenate([biasb[:, pl.ds((2 * ch + ci) * N1 + n * 128, 128)] for ci in range(2)],
                                     axis=1)
                act[rh, ch] = jax.nn.gelu(y + rep(b1, HB), approximate=True)

            _strassen(lambda c: _strassen_value(prod1, c), activate)
            for c in range(7):
                o = _combo(_LHS_TERMS, c, lambda a, b: act[a, b])
                for d, v in enumerate(_lhs_combos(o[:QB, :128], o[:QB, 128:], o[QB:, :128], o[QB:, 128:])):
                    g[c, d].append(v.astype(BF16))

        state = dict(dep=None, piece=0, window=0)
        jobs, pending, hs = [], [], {}
        tie = make_tie(jobs, 0.0)

        def next_block_ln():
            jobs.extend(pending)
            del pending[:]
            for _ in range(LN_PLAN[state['window']]):
                k, r = state['piece'] // 4, state['piece'] % 4
                pin = pltpu.bitcast(qka[16, pl.ds(0, 8), :], U32)
                dep = pin if state['dep'] is None else state['dep'] | pin
                state['dep'] = ln2_piece(hs, nxt, r * QB + 16 * k, dep)
                if r == 3:
                    pending.extend(functools.partial(lhs1_job, hs, nbase, k, t, c)
                                   for t in range(2) for c in range(7))
                state['piece'] += 1
            state['window'] += 1

        for n in range(2):
            def prod2(c, d):
                return _dot(jnp.concatenate(g[c, d], axis=1),
                            _bf(tie(rhs_load(w2, K2, N2, rhs2_loc, c, d, n), FFN_DENSITY)))

            def outer(c):
                next_block_ln()
                y = _strassen_value(prod2, c)
                qka[17, pl.ds(srow, 8), :] = y[0:8, 0:128]
                return y

            def finish(y, rh, ch):
                for ci in range(2):
                    nn = (2 * ch + ci) * 2 + n
                    cols = pl.ds(nn * 128, 128)
                    yy = y[:, ci * 128:(ci + 1) * 128] + rep(biasb[:, pl.ds(FF + nn * 128, 128)], HB)
                    xr = pl.ds(pl.multiple_of(i * HB, HB) + rh * (HB // 2), HB // 2)
                    ar = pl.ds(pl.multiple_of(i * FB, FB) + rh * HB, HB)
                    x2 = _bf(xs[xr, cols]).astype(F32) + rep(modb[0, :, cols], HB) * ha[ar, cols]
                    qka[2 * nn + half, pl.ds(srow + rh * (HB // 2), HB // 2), :] = pack(
                        x2 + rep(modb[3, :, cols], HB) * yy, F32)
                    if rh == ch:
                        pltpu.make_async_copy(
                            qka.at[2 * nn + half, pl.ds(srow, HB), :],
                            out32.at[pl.ds(pl.multiple_of(i * HB, HB), HB), cols],
                            sem.at[SEM_OUT]).start()

            _strassen(outer, finish)
        assert not jobs and not pending and state['piece'] == 16
        return carry

    with jax.named_scope("p4_ffn"):
        lax.fori_loop(0, nb, ffn, 0)
    pltpu.make_async_copy(out32, out32, sem.at[SEM_OUT]).wait()


@jax.jit
def pallas_adaLN_cond__memory_aug_recurrent_mem_tr__dense_activation_gelu__prompt_kernel(
    A_x, A_mem0, A_Wq, A_Wk, A_Wv, A_Wo, A_seg_len, B_x, B_w1, B_b1, B_w2, B_b2, c, w_mod,
):
    assert A_x.shape == (1, S, D) and A_Wq.shape == (D, H, E) and A_mem0.shape == (1, M, D)
    any_spec = pl.BlockSpec(memory_space=pl.ANY)
    out = pl.pallas_call(
        _kernel,
        out_shape=jax.ShapeDtypeStruct((S, D), BF16),
        in_specs=[any_spec] * 12,
        out_specs=any_spec,
        scratch_shapes=[
            pltpu.VMEM((S // 2, D), U32),
            pltpu.VMEM((96, D // 2, E), U32),
            pltpu.VMEM((8, H * E // 2, 128), U32),
            pltpu.VMEM((D // 2, FF), U32),
            pltpu.VMEM((FF // 2, D), U32),
            pltpu.VMEM((H, RING, E), F32),
            pltpu.VMEM((H, RING, E), F32),
            pltpu.VMEM((H + 1, RING, E), F32),
            pltpu.VMEM((H, RING, E), F32),
            pltpu.VMEM((S, D), F32),
            pltpu.VMEM((S - PRE, D), F32),
            pltpu.VMEM((M, D), F32),
            pltpu.VMEM((NQ, 2, 8, KQ), F32),
            pltpu.VMEM((4, 8, D), F32),
            pltpu.VMEM((8, D), U32),
            pltpu.VMEM((8, FF + D), F32),
            pltpu.VMEM((80, 128), F32),
            pltpu.VMEM((8, 32, 128), F32),
            pltpu.VMEM((8, 128), U32),
            pltpu.SMEM((1,), jnp.int32),
            pltpu.VMEM((8, FF // 8, 128), U32),
            pltpu.VMEM((13 * 64, D), U32),
            pltpu.VMEM((128, 256), U32),
            pltpu.VMEM((128, 256), U32),
            pltpu.VMEM((128, 256), U32),
            pltpu.VMEM((128, 256), U32),
            pltpu.VMEM((128, 256), U32),
            pltpu.VMEM((128, 256), U32),
            pltpu.VMEM((M, D), BF16),
            pltpu.VMEM((FF,), BF16),
            pltpu.VMEM((D,), BF16),
            pltpu.VMEM((1, D), BF16),
            pltpu.SemaphoreType.DMA((NSEM,)),
        ],
        compiler_params=pltpu.CompilerParams(vmem_limit_bytes=127 * 1024 * 1024, disable_bounds_checks=True,
                                             disable_semaphore_checks=True),
    )(
        A_x.reshape(S, D), A_mem0.reshape(M, D),
        A_Wq.reshape(D // 2, 2, H, E), A_Wk.reshape(D // 2, 2, H, E), A_Wv.reshape(D // 2, 2, H, E),
        A_Wo.reshape(H * E, D), B_w1, B_b1, B_w2, B_b2, c, w_mod,
    )
    return out.reshape(1, S, D)
```

```python
import functools
import math

import jax
import jax.numpy as jnp
from jax import lax
import jax.experimental.pallas as pl
import jax.experimental.pallas.tpu as pltpu

F32 = jnp.float32
BF16 = jnp.bfloat16
U32 = jnp.uint32

S = 2048
D = 1024
H = 32
E = 128
M = 8
SEG = 32
NSEG = S // SEG
FF = 3584
NP = H // 2
TOK = 24
PRE = S - NSEG * TOK
RING = 576
OOFF = (-NSEG * TOK) % RING
LN_EPS = 1e-5
FB = 256
P3_SPLIT = ((4, 10), (4, 18), (4, 10))
LN0_PLAN = (3, 3, 3, 3, 2, 2, 0)
LN_PLAN = (1, 1, 1, 1, 1, 1, 1, 2, 2, 2, 2, 1, 0, 0)
FFN_DENSITY = 1.0 / 24
ATT_COL, ATT_N1, ATT_N2 = 6, 2, 5
UNROLL = 4

NQ = 4
KQ = D // NQ

FIRST_STARTS = [('m', 0), ('w', 0, 0, 2), ('w', 0, 2, 6), ('w', 0, 6, 12), ('m', 1), ('w', 1, 0, 6),
                ('w', 1, 6, 12), ('m', 2)]
P1A_BLOCKS = [
    ([], [('m', 0)]),
    ([], [('w', 0, 0, 2)]),
    ([], [('w', 0, 2, 6)]),
    ([('w', 2, 0, 6), ('w', 2, 6, 12)], [('w', 0, 6, 12)]),
    ([('m', 3), ('w', 3, 0, 6), ('w', 3, 6, 12)], [('m', 1), ('w', 1, 0, 6)]),
    ([], [('m', 2), ('w', 1, 6, 12)]),
    ([('g', 2), ('g', 3)], [('w', 2, 0, 6), ('w', 2, 6, 12)]),
    ([('g', 4), ('g', 5)], [('m', 3), ('w', 3, 0, 6), ('w', 3, 6, 12)]),
]
W_ITEMS = [it for _, items in P1A_BLOCKS for it in items if it[0] == 'w']
IT_ROWS = TOK * UNROLL
X_CHUNKS = (PRE, PRE + IT_ROWS, PRE + 3 * IT_ROWS, S)
LN_SLOTS = ((0, 10), (1, 6))
MOD_SLOTS = tuple((g, 2) for g in range(8))
NX0 = 4

SEM_C = 0
SEM_X0 = 1
SEM_MOD = SEM_X0 + NX0
SEM_WA = SEM_MOD + NQ + 2
SEM_WB = SEM_WA + len(W_ITEMS)
SEM_XC = SEM_WB + 6
SEM_WO = SEM_XC + 3
SEM_W1 = SEM_WO + 1
SEM_W2 = SEM_W1 + 1
SEM_OUT = SEM_W2 + 1
NSEM = SEM_OUT + 1


def _ln(x):
    m = jnp.mean(x, axis=-1, keepdims=True)
    xc = x - m
    v = jnp.mean(xc * xc, axis=-1, keepdims=True)
    return xc * lax.rsqrt(v + LN_EPS)


def _bf(w32):
    return pltpu.bitcast(w32, BF16)


def _dot(a, b):
    return jnp.dot(a, b, preferred_element_type=F32)


def _lhs_combos(a11, a12, a21, a22):
    return [a11 - a22, a21 - a22, a11, a22, a12 - a11, a21 - a11, a12 - a22]


def _rhs_combos(b11, b12, b21, b22):
    return [b11 - b22, b11, b12 + b22, b21 + b11, b22, b11 + b12, b21 + b22]


_LHS_TERMS = {0: ((0, 0), (1, 1), -1), 1: ((1, 0), (1, 1), -1), 2: ((0, 0), None, 0), 3: ((1, 1), None, 0),
              4: ((0, 1), (0, 0), -1), 5: ((1, 0), (0, 0), -1), 6: ((0, 1), (1, 1), -1)}
_RHS_TERMS = {0: ((0, 0), (1, 1), -1), 1: ((0, 0), None, 0), 2: ((0, 1), (1, 1), 1), 3: ((1, 0), (0, 0), 1),
              4: ((1, 1), None, 0), 5: ((0, 0), (0, 1), 1), 6: ((1, 0), (1, 1), 1)}
_SWAP = {c: int(c in (2, 4, 5, 6)) for c in range(7)}


def _combo(terms, c, blk):
    p, q, sign = terms[c]
    if q is None:
        return blk(*p)
    return blk(*p) + blk(*q) if sign > 0 else blk(*p) - blk(*q)


def _rhs_operand(c, blk):
    p, q, sign = _RHS_TERMS[c]
    a = _bf(blk(*p))
    if q is None:
        return a
    a = a.astype(F32)
    b = _bf(blk(*q)).astype(F32)
    return (a + b if sign > 0 else a - b).astype(BF16)


def _strassen(prod, finish, side=lambda: None):
    side()
    m1 = prod(1)
    m3 = prod(3)
    finish(m1 + m3, 1, 0)
    side()
    m2 = prod(2)
    m4 = prod(4)
    finish(m2 + m4, 0, 1)
    side()
    m0 = prod(0)
    m5 = prod(5)
    finish((m2 - m1) + m0 + m5, 1, 1)
    side()
    m6 = prod(6)
    finish((m3 - m4) + m0 + m6, 0, 0)


def _strassen_value(prod2, c):
    r = {}
    _strassen(functools.partial(prod2, c), lambda y, rh, ch: r.__setitem__((rh, ch ^ _SWAP[c]), y))
    return jnp.concatenate([jnp.concatenate([r[0, 0], r[0, 1]], axis=1),
                            jnp.concatenate([r[1, 0], r[1, 1]], axis=1)], axis=0)


_ORDER = (1, 3, 2, 4, 0, 5, 6)

_PAIRS = [(c, d) for c in range(7) for d in range(7) if not (c in (1, 4) and d in (1, 4))]


def _plain_block(c, d):
    return 2 * (c // 4) + d // 4, 2 * (c // 4) + ((d // 4) ^ _SWAP[c])


def _kernel(x_hbm, mem0_hbm, wq_hbm, wk_hbm, wv_hbm, wo_hbm, w1_hbm, b1_hbm, w2_hbm, b2_hbm,
            c_hbm, wmod_hbm, out_hbm,
            xs, wqkv, wo, w1, w2, qka, qkb, vring, oring, ha, hn, memb, moda, modb, scb, colb, slab, biasb,
            fillb, accb, zerob, zero_s, wx, hb2, pk0, pk1, pk2, pk3, pk4, pk5, mem0_ref, b1_ref, b2_ref, c_ref, sem):
    qkv_hbm = [r.bitcast(U32) for r in (wq_hbm, wk_hbm, wv_hbm)]
    x32 = x_hbm.bitcast(U32)
    wo32 = wo_hbm.bitcast(U32)
    wmod32 = wmod_hbm.bitcast(F32)

    def wma(qq, k):
        return pl.ds(512 * (qq // 2), 512), pl.ds(512 * (qq % 2) + k * KQ, KQ)

    def hb_idx(c, q0, nq, row0=0, nrows=PRE // 4):
        return pl.ds(1024 + 128 * (c // 2) + row0, nrows), pl.ds(512 * (c % 2) + 128 * q0, 128 * nq)

    def units_start(lo, hi, rows, sem_idx):
        for u in range(lo, hi):
            j, m = u // 3, u % 3
            for p in range(2):
                pltpu.make_async_copy(qkv_hbm[m].at[rows, p, j, :], wqkv.at[2 * u + p, rows, :],
                                      sem.at[sem_idx]).start()

    def units_wait(lo, n, rows, sem_idx):
        blk = wqkv.at[pl.ds(2 * lo, 2 * n), rows, :]
        pltpu.make_async_copy(blk, blk, sem.at[sem_idx]).wait()

    def item_start(item):
        if item[0] == 'm':
            qq = item[1]
            for k in range(2):
                pltpu.make_async_copy(wmod32.at[:, pl.ds(k * D + qq * KQ, KQ)], ha.at[wma(qq, k)],
                                      sem.at[SEM_MOD + qq]).start()
        elif item[0] == 'w':
            _, qq, lo, hi = item
            units_start(lo, hi, pl.ds(qq * (KQ // 2), KQ // 2), SEM_WA + W_ITEMS.index(item))
        else:
            whole_start(item[1])

    def item_wait(item):
        if item[0] == 'm':
            qq = item[1]
            blk = ha.at[pl.ds(512 * (qq // 2), 512), pl.ds(512 * (qq % 2), 512)]
            pltpu.make_async_copy(blk, blk, sem.at[SEM_MOD + qq]).wait()
        else:
            _, qq, lo, hi = item
            units_wait(lo, hi - lo, pl.ds(qq * (KQ // 2), KQ // 2), SEM_WA + W_ITEMS.index(item))

    def whole_start(i):
        if i == 2:
            xc_copy(0).start()
        units_start(6 * i, 6 * i + 6, pl.ds(0, D // 2), SEM_WB + i - 2)

    def slab_copies(it):
        return [pltpu.make_async_copy(
            wmod32.at[:, pl.ds(pl.multiple_of(2 * D + it * 256 + t * 128, 128), 128)],
            slab.at[it & 1, t], sem.at[SEM_MOD + NQ + (it & 1)]) for t in range(2)]

    def x0_copy(i):
        n = PRE // 2 // NX0
        rows = pl.ds(pl.multiple_of(i * n, n), n)
        return pltpu.make_async_copy(x32.at[rows], xs.at[rows], sem.at[SEM_X0 + i])

    def xc_copy(i):
        rows = pl.ds(X_CHUNKS[i] // 2, (X_CHUNKS[i + 1] - X_CHUNKS[i]) // 2)
        return pltpu.make_async_copy(x32.at[rows], xs.at[rows], sem.at[SEM_XC + i])

    def wo_copy(n):
        return pltpu.make_async_copy(wo32.at[:, pl.ds(n * 128, 128)], wo.at[n], sem.at[SEM_WO])

    w1_copy = pltpu.make_async_copy(w1_hbm.bitcast(U32), w1, sem.at[SEM_W1])
    w2_copy = pltpu.make_async_copy(w2_hbm.bitcast(U32), w2, sem.at[SEM_W2])
    small_copies = [pltpu.make_async_copy(a, b, sem.at[SEM_C])
                    for a, b in ((c_hbm, c_ref), (mem0_hbm, mem0_ref), (b1_hbm, b1_ref),
                                 (b2_hbm, b2_ref))]

    def deinterleave(u, row0, nrows):
        for k in range(nrows // 64):
            rows = pl.ds(row0 + k * 64, 64)
            a = wqkv[2 * u, rows, :]
            b = wqkv[2 * u + 1, rows, :]
            wqkv[2 * u, rows, :] = (a & jnp.uint32(0xFFFF)) | (b << 16)
            wqkv[2 * u + 1, rows, :] = (a >> 16) | (b & jnp.uint32(0xFFFF0000))

    def load_x16(row2, dep):
        xw = xs[pl.ds(row2, 8), :]
        if dep is not None:
            first = xw[:, 0:128] | (dep & zerob[...])
            xw = jnp.concatenate([first, xw[:, 128:]], axis=1)
        return _bf(xw).astype(F32)

    pks = [pk0, pk1, pk2, pk3, pk4, pk5]

    def pack(v, dtype=U32):
        rows = pl.ds(0, v.shape[0] // 2)
        pk = pks[0]
        pk[rows, pl.ds(0, 128)] = pltpu.bitcast(v.astype(BF16), U32)
        return pltpu.bitcast(pk[rows, pl.ds(0, 128)], dtype)

    def rep(v8, n):
        return jnp.concatenate([v8] * (n // 8), axis=0)

    def mrow(k, n):
        if k < 2:
            return rep(jnp.concatenate([moda[qq, k] for qq in range(NQ)], axis=1), n)
        return rep(jnp.concatenate([modb[4 * (k - 2) + q] for q in range(4)], axis=1), n)

    for cp in small_copies:
        cp.start()
    for i in range(NX0):
        x0_copy(i).start()
    for item in FIRST_STARTS:
        item_start(item)

    def start_rest():
        xc_copy(1).start()
        for n in range(8):
            wo_copy(n).start()
        for cp in slab_copies(0):
            cp.start()
        xc_copy(2).start()
        w1_copy.start()
        w2_copy.start()

    r = lax.broadcasted_iota(jnp.int32, (80, 128), 0)
    q = lax.broadcasted_iota(jnp.int32, (80, 128), 1)
    r_tok = r < 64
    q_tok = q < 64
    r_head = jnp.where(r_tok, r >> 5, (r - 64) >> 3)
    q_head = jnp.where(q_tok, q >> 5, (q - 64) >> 3)
    same = (r_head == q_head) & (q < 80)
    causal_ok = jnp.logical_not(r_tok & q_tok & ((q & 31) > (r & 31)))
    scale = E ** (-0.5)
    fillb[...] = jnp.where(same, jnp.where(causal_ok, 0.0, -1e9 / scale), -jnp.inf).astype(F32)
    zerob[...] = jnp.zeros((8, 128), U32)
    zero_s[0] = 0

    for cp in small_copies:
        cp.wait()
    cf = c_ref[...].astype(F32)
    sc = (cf * jax.nn.sigmoid(cf)).astype(BF16)
    scb[...] = pltpu.bitcast(jnp.broadcast_to(sc, (16, D)), U32)
    scf = jnp.broadcast_to(sc.astype(F32), (128, D))
    for k in range(8):
        colb[pl.ds(k * 64, 64), :] = pltpu.bitcast(scf[:, k * 128:(k + 1) * 128].T.astype(BF16), U32)
    memb[...] = mem0_ref[...].astype(F32)
    biasb[:, pl.ds(0, FF)] = jnp.broadcast_to(b1_ref[...].astype(F32).reshape(1, FF), (8, FF))
    biasb[:, pl.ds(FF, D)] = jnp.broadcast_to(b2_ref[...].astype(F32).reshape(1, D), (8, D))

    def pre_norm(i, carry):
        x0_copy(i).wait()
        nr = PRE // NX0
        for z in range(nr // 16):
            xn = _ln(load_x16(pl.multiple_of(i * (nr // 2) + z * 8, 8), None))
            for n in range(8):
                oring[n, pl.ds(pl.multiple_of(i * nr + z * 16, 16), 16), :] = xn[:, n * 128:(n + 1) * 128]
        return carry

    with jax.named_scope("p0_ln"):
        lax.fori_loop(0, NX0, pre_norm, 0)

    def dst_slot(i, k, p):
        cls, m = k // 3, k % 3
        if m == 2:
            return vring, 4 * i + 2 * cls + p
        return (qka, qkb)[cls], 4 * i + 2 * m + p

    PH = PRE // 2
    assert KQ == 256

    def item_run(item):
        if item[0] == 'm':
            qq = item[1]
            sc16 = _bf(scb[...])
            ca1 = 1.0 + _dot(sc16, _bf(ha[wma(qq, 1)]))[0:8].astype(BF16).astype(F32)
            sa = _dot(sc16, _bf(ha[wma(qq, 0)]))[0:8].astype(BF16).astype(F32)
            moda[qq, 0] = sa
            moda[qq, 1] = ca1
            for z in range(PH // 32):
                def h_blk(rh, kh):
                    cols = slice(kh * 128, (kh + 1) * 128)
                    return (oring[2 * qq + kh, pl.ds(rh * PH + z * 32, 32), :] * rep(ca1[:, cols], 32)
                            + rep(sa[:, cols], 32))

                for c, v in enumerate(_lhs_combos(h_blk(0, 0), h_blk(0, 1), h_blk(1, 0), h_blk(1, 1))):
                    ha[hb_idx(c, qq, 1, z * 16, 16)] = pltpu.bitcast(v.astype(BF16), F32)
            return
        _, qq, lo, hi = item
        if lo == 0 and qq >= 2:
            a_jobs.extend(functools.partial(lhs0_job, k, qq - 2, c) for k in range(PQ // 16) for c in range(7))
        for u in range(lo, hi):
            deinterleave(u, qq * (KQ // 2), KQ // 2)
            i, k = u // 6, u % 6

            def prod(c):
                lhs = pltpu.bitcast(ha[hb_idx(c, qq, 1)], U32)
                if u >= 2:
                    lhs = tie_rows(lhs, a_jobs, (8,))
                rhs = _rhs_operand(c, lambda a, b: wqkv[2 * u + b, pl.ds((2 * qq + a) * 64, 64), :])
                return _dot(_bf(lhs), rhs)

            def finish(y, rh, ch):
                ref, idx = dst_slot(i, k, ch)
                rows = pl.ds(RING - PRE + rh * PH, PH)
                if qq > 0:
                    y = y + ref[idx, rows, :]
                ref[idx, rows, :] = y

            _strassen(prod, finish)

    def tie_rows(w, jobs, groups):
        if not jobs:
            return w
        parts = [w[8 * g:8 * g + 8, 0:128] for g in range(w.shape[0] // 8)]
        for g in groups:
            if jobs:
                parts[g] = parts[g] | (jobs.pop(0)() & zerob[...])
        first = jnp.concatenate(parts, axis=0)
        return first if w.shape[1] == 128 else jnp.concatenate([first, w[:, 128:]], axis=1)

    PQ = PRE // 4
    a_jobs = []

    def lhs0_idx(c, d, k, nk, t, nt):
        e = 7 * c + d
        return pl.ds(64 * (e // 4) + 8 * k, 8 * nk), pl.ds(256 * (e % 4) + 128 * t, 128 * nt)

    def lhs0_job(k, t, c):
        def sub(ri, ki):
            def blk(ro, ko):
                n = 2 * ko + ki + 4 * t
                cols = pl.ds((n % 2) * 128, 128)
                return (oring[n, pl.ds((2 * ro + ri) * PQ + 16 * k, 16), :] * rep(moda[n // 2, 1, :, cols], 16)
                        + rep(moda[n // 2, 0, :, cols], 16))

            return _combo(_LHS_TERMS, c, blk)

        bits = None
        for d, v in enumerate(_lhs_combos(sub(0, 0), sub(0, 1), sub(1, 0), sub(1, 1))):
            hb2[lhs0_idx(c, d, k, 1, t, 1)] = pltpu.bitcast(v.astype(BF16), U32)
            if d not in (2, 3):
                b = pltpu.bitcast(v[8 * (d % 2):8 * (d % 2) + 8], U32)
                bits = b if bits is None else bits | b
        return bits

    def ln1_piece(row2):
        h16 = _ln(load_x16(PRE // 2 + row2, None)) * mrow(1, 16) + mrow(0, 16)
        hn[pl.ds(pl.multiple_of(2 * row2, 16), 16), :] = h16
        return pltpu.bitcast(h16[8:16, D - 128:], U32)

    def phase1b(i, carry):
        @pl.when(i == 3)
        def _():
            whole_start(6)
            whole_start(7)

        @pl.when(i == 4)
        def _():
            start_rest()

        units_wait(6 * i, 6, pl.ds(0, D // 2), SEM_WB + i - 2)
        ln1_piece(pl.multiple_of((i - 2) * 8, 8))

        def raw(m, kq, nq, g):
            u = 6 * i + m + 3 * (nq // 2)
            return wqkv[2 * u + nq % 2, pl.ds((kq + 4 * (g // 8)) * 64 + 8 * (g % 8), 8), :]

        ops = {}

        def rhs0_job(m, c, g):
            def sub(ki, ni):
                return _combo(_RHS_TERMS, c,
                              lambda ko, no: _bf(raw(m, 2 * ko + ki, 2 * no + (ni ^ _SWAP[c]), g)).astype(F32))

            bits = None
            for d, v in enumerate(_rhs_combos(sub(0, 0), sub(0, 1), sub(1, 0), sub(1, 1))):
                if (c, d) in _PAIRS:
                    ops[m, c, d, g] = pack(v)
                    bits = ops[m, c, d, g] if bits is None else bits | ops[m, c, d, g]
            return bits

        seq = [(m, c) for m in range(3) for c in _ORDER]
        jobs = []
        count = [0]
        deinterleave(6 * i, 0, D // 2)
        deinterleave(6 * i + 3, 0, D // 2)
        for g in range(16):
            rhs0_job(*seq[0], g)
        for m in range(3):
            if m < 2:
                deinterleave(6 * i + m + 1, 0, D // 2)
                deinterleave(6 * i + m + 4, 0, D // 2)

            def prod(c, d):
                if (c, d) in _PAIRS:
                    rhs = [ops[m, c, d, g] for g in range(16)]
                else:
                    rhs = [raw(m, *_plain_block(c, d), g) for g in range(16)]
                lhs = tie_rows(hb2[lhs0_idx(c, d, 0, 8, 0, 2)], jobs, ((0, 3, 6), (1, 4, 7))[count[0] % 2])
                count[0] += 1
                return _dot(_bf(lhs), _bf(jnp.concatenate(rhs, axis=0)))

            def outer(c):
                assert not jobs
                count[0] = 0
                nx = seq.index((m, c)) + 1
                if nx < len(seq):
                    jobs.extend(functools.partial(rhs0_job, *seq[nx], g) for g in range(16))
                return _strassen_value(prod, c)

            def finish(y, rh, ch):
                for ci in range(2):
                    ref, idx = dst_slot(i, m + 3 * ch, ci)
                    ref[idx, pl.ds(RING - PRE + rh * PH, PH), :] = y[:, ci * 128:(ci + 1) * 128]

            _strassen(outer, finish)
        return carry

    for bi, (starts, items) in enumerate(P1A_BLOCKS):
        for item in starts:
            item_start(item)
        with jax.named_scope("p1a_wait%d" % bi):
            for item in items:
                item_wait(item)
        for item in items:
            item_run(item)
    assert not a_jobs
    xc_copy(0).wait()
    with jax.named_scope("p1b"):
        lax.fori_loop(2, 8, phase1b, 0)
    pks.pop(0)
    xc_copy(1).wait()
    for n in range(8):
        wo_copy(n).wait()

    cexp = scale * math.log2(math.e)
    NG = NP // 2
    grp = [(4 * (g // 2) + (g % 2), 4 * (g // 2) + (g % 2) + 2) for g in range(NG)]
    early = [2 * j + u for g in range(NG - 3) for j in grp[g] for u in range(2)]
    late = [h for h in range(H) if h not in early]

    def step(it, k, side_jobs):
        s = it * UNROLL + k
        split = k > 0
        base = TOK * UNROLL * it
        w0 = pl.multiple_of(lax.rem(base, RING), 32) + TOK * k
        r0 = pl.multiple_of(lax.rem(SEG * s + (RING - PRE), RING), 32)
        ow = pl.multiple_of(lax.rem(SEG * s + OOFF, RING), 32)
        o0 = pl.multiple_of(lax.rem(base + OOFF, RING), 32) + TOK * k
        a0 = pl.multiple_of(base, 32) + TOK * k
        X = jnp.concatenate([hn[pl.ds(a0, TOK), :], memb[...]], axis=0).astype(BF16)
        ym = [None] * 96
        probs = [None] * NP
        om = [None] * H
        order = (4, 5, 0, 1, 2, 3)

        if split:
            for t in order:
                accb[t] = _dot(X[:, :D // 2], _bf(wqkv[t, pl.ds(0, D // 4), :]))

        def slot(j, t):
            if t >= 4:
                return vring, 2 * j + t - 4
            return (qka, qkb)[j % 2], 4 * (j // 2) + t

        def proj(j, t, job):
            c = 6 * j + t
            bits = None if job is None else job()
            if split and j == 0:
                y = accb[t] + _dot(X[:, D // 2:], _bf(wqkv[c, pl.ds(D // 4, D // 4), :]))
            else:
                y = _dot(X, _bf(wqkv[c]))
            ref, k = slot(j, t)
            if bits is not None:
                y0 = pltpu.bitcast(pltpu.bitcast(y[0:8], U32) | (bits & zerob[...]), F32)
                y = jnp.concatenate([y0, y[8:]], axis=0)
            ref[k, pl.ds(w0, TOK), :] = y[0:TOK]
            ym[c] = y[TOK:TOK + M]

        def gather(j, m, pad):
            c = 6 * j + 2 * m
            ref, k = slot(j, 2 * m)
            parts = [ref[k, pl.ds(r0, SEG), :], ref[k + 1, pl.ds(r0, SEG), :], ym[c], ym[c + 1]]
            if pad:
                parts.append(jnp.zeros((48, E), F32))
            return jnp.concatenate(parts, axis=0).astype(BF16)

        def scores(j):
            sc_ = lax.dot_general(gather(j, 0, False), gather(j, 1, True),
                                  (((1,), (1,)), ((), ())), preferred_element_type=F32)
            fill = fillb[...]
            sc_ = jnp.where(fill == 0.0, sc_, fill)
            mx = jnp.max(sc_, axis=-1, keepdims=True)
            p = jnp.exp2((sc_ - mx) * cexp)
            l = jnp.sum(p, axis=-1, keepdims=True)
            rl = pl.reciprocal(l, approx=True)
            rl = rl * (2.0 - l * rl)
            probs[j] = p * rl

        def park(j):
            vring[H, pl.ds(40 * (j % 8), 40), :] = pack(probs[j], F32)
            probs[j] = None

        def pv(j):
            if probs[j] is None:
                P = _bf(vring[H, pl.ds(40 * (j % 8), 40), :])
            else:
                P = probs[j].astype(BF16)
            o = _dot(P, gather(j, 2, True))
            oring[2 * j, pl.ds(ow, SEG), :] = o[0:32]
            oring[2 * j + 1, pl.ds(ow, SEG), :] = o[32:64]
            om[2 * j] = o[64:72]
            om[2 * j + 1] = o[72:80]

        def o_lhs(hs):
            return jnp.concatenate(
                [jnp.concatenate([oring[h, pl.ds(o0, TOK), :], om[h]], axis=0) for h in hs],
                axis=1).astype(BF16)

        def o_rhs(n, hs):
            return _bf(jnp.concatenate([wo[n, pl.ds(h * 64, 64), :] for h in hs], axis=0))

        for g in range(NG):
            cols = [(j, t) for j in grp[g] for t in order]
            if g == 2:
                cols = ([(j, t) for j in grp[g] for t in (4, 5)]
                        + [(j, t) for j in grp[g] for t in range(4)])
            for j in (grp[0] + grp[1] if g == 3 else grp[g - 2] if g >= 4 else ()):
                park(j)
            for ci, (j, t) in enumerate(cols):
                if g == 2 and ci == 4:
                    for jj in grp[0] + grp[1]:
                        scores(jj)
                if g >= 3 and ci == ATT_COL:
                    for jj in grp[g - 1]:
                        scores(jj)
                    for jj in grp[g - 3]:
                        pv(jj)
                proj(j, t, side_jobs.get((g, ci)))
        lo = o_lhs(early)
        for n in range(8):
            accb[n] = _dot(lo, o_rhs(n, early))
            if n == ATT_N1:
                for jj in grp[NG - 1]:
                    scores(jj)
                for jj in grp[NG - 3]:
                    pv(jj)
            if n == ATT_N2:
                for jj in grp[NG - 2] + grp[NG - 1]:
                    pv(jj)
        lo = o_lhs(late)
        for n in range(8):
            a = accb[n] + _dot(lo, o_rhs(n, late))
            ha[pl.ds(a0, TOK), pl.ds(n * 128, 128)] = a[0:TOK]
            memb[:, pl.ds(n * 128, 128)] = a[TOK:TOK + M]

    NIT = NSEG // UNROLL

    def lo16(w):
        return pltpu.bitcast(w << 16, F32)

    def hi16(w):
        return pltpu.bitcast(w & jnp.uint32(0xFFFF0000), F32)

    def steps(it, carry):
        @pl.when(it + 1 < NIT)
        def _():
            for cp in slab_copies(it + 1):
                cp.start()

        @pl.when(it == 1)
        def _():
            xc_copy(2).wait()

        for cp in slab_copies(it):
            cp.wait()
        acc = [None, None]

        def mod_job(q):
            for kk in range(2 * q, 2 * q + 2):
                cw = colb[pl.ds(kk * 8, 8), :]
                for t in range(2):
                    w = pltpu.bitcast(slab[it & 1, t, pl.ds(kk * 8, 8), :], U32)
                    v = lo16(w) * lo16(cw) + hi16(w) * hi16(cw)
                    acc[t] = v if acc[t] is None else acc[t] + v
            if q < D // 32 - 1:
                return pltpu.bitcast(acc[0], U32) | pltpu.bitcast(acc[1], U32)
            y = jnp.sum(jnp.concatenate(acc, axis=1), axis=0, keepdims=True).astype(BF16).astype(F32)
            y = jnp.broadcast_to(y + jnp.where((it >> 2) == 2, 1.0, 0.0), (8, 256))
            modb[it] = y
            return pltpu.bitcast(y[:, 0:128], U32)

        nxt2 = pl.multiple_of(jnp.minimum(it + 1, NIT - 1) * (IT_ROWS // 2), 16)
        pieces = list(range(IT_ROWS // 16))
        for k in range(UNROLL):
            side_jobs = {pos: functools.partial(mod_job, 8 * k + q) for q, pos in enumerate(MOD_SLOTS)}
            for pos in LN_SLOTS[k % 2:]:
                side_jobs[pos] = functools.partial(ln1_piece, nxt2 + 8 * pieces.pop(0))
            step(it, k, side_jobs)
        assert not pieces
        return carry

    with jax.named_scope("p2_steps"):
        lax.fori_loop(0, NIT, steps, 0)

    w1_copy.wait()
    w2_copy.wait()

    nb = S // FB
    HB = FB // 2
    QB = FB // 4

    def ln2_piece(hs, blk, off, dep):
        x2 = (load_x16(pl.multiple_of(blk * HB, HB) + off // 2, dep)
              + mrow(2, 16) * ha[pl.ds(pl.multiple_of(blk * FB, FB) + off, 16), :])
        h = _ln(x2) * mrow(4, 16) + mrow(3, 16)
        hs[off] = h
        return pltpu.bitcast(h[8:16, D - 128:], U32)

    def lhs1_loc(base, c, d):
        e = 7 * c + d
        return base + 32 * (e // 4), 256 * (e % 4)

    def lhs1_job(hs, base, k, t, c):
        def sub(ri, ki):
            def blk(ro, ko):
                c0 = (2 * ko + ki) * 256 + t * 128
                return hs[(2 * ro + ri) * QB + 16 * k][:, c0:c0 + 128]

            return _combo(_LHS_TERMS, c, blk)

        bits = None
        for d, v in enumerate(_lhs_combos(sub(0, 0), sub(0, 1), sub(1, 0), sub(1, 1))):
            r0, c0 = lhs1_loc(base, c, d)
            hn[pl.ds(r0 + 8 * k, 8), pl.ds(c0 + t * 128, 128)] = pltpu.bitcast(
                v.astype(BF16), F32)
            if d not in (2, 3):
                b = pltpu.bitcast(v[8 * (d % 2):8 * (d % 2) + 8], U32)
                bits = b if bits is None else bits | b
        return bits

    K1, N1, K2, N2 = D // 8, FF // 4, FF // 8, D // 4

    def rhs1_loc(c, d, n):
        e = _PAIRS.index((c, d)) * 7 + n
        return wqkv, e // 4, K1 * (e % 4)

    rhs2_slots = ([(wqkv, e, 0) for e in range(79, 96)] + [(qkb, e, 0) for e in range(H)]
                  + [(vring, e, 0) for e in range(H + 1)] + [(wx, e, 0) for e in range(8)])

    def rhs2_loc(c, d, n):
        return rhs2_slots[_PAIRS.index((c, d)) * 2 + n]

    def rhs_job(w, kq, nq, loc, n, r, cs):
        cache = {}

        def blk(ko, no, ki, ni):
            key = (2 * ko + ki, 2 * no + ni)
            if key not in cache:
                cache[key] = _bf(w[pl.ds(r + key[0] * kq, 8), pl.ds(n * 128 + key[1] * nq, 128)]).astype(F32)
            return cache[key]

        bits = None
        for c in cs:
            def sub(ki, ni):
                return _combo(_RHS_TERMS, c, lambda ko, no: blk(ko, no, ki, ni ^ _SWAP[c]))

            for d, v in enumerate(_rhs_combos(sub(0, 0), sub(0, 1), sub(1, 0), sub(1, 1))):
                if (c, d) in _PAIRS:
                    ref, idx, row = loc(c, d, n)
                    b = pack(v)
                    ref[idx, pl.ds(row + r, 8), :] = pltpu.bitcast(b, ref.dtype)
                    bits = b if bits is None else bits | b
        return bits

    def rhs_load(w, kq, nq, loc, c, d, n):
        if (c, d) not in _PAIRS:
            qk, qn = _plain_block(c, d)
            return w[pl.ds(qk * kq, kq), pl.ds(qn * nq + n * 128, 128)]
        ref, idx, row = loc(c, d, n)
        return pltpu.bitcast(ref[idx, pl.ds(row, kq), :], U32)

    def make_tie(jobs, credit):
        state = [credit]

        def tie(raw, density):
            if not jobs:
                return raw
            parts = []
            for r in range(0, raw.shape[0], 8):
                v = raw[r:r + 8]
                state[0] += density
                if jobs and state[0] >= 1.0:
                    state[0] -= 1.0
                    v = v | (jobs.pop(0)() & zerob[...])
                parts.append(v)
            return jnp.concatenate(parts, axis=0)

        return tie

    def w_jobs(r1, n1, r2, n2):
        return ([functools.partial(rhs_job, w1, K1, N1, rhs1_loc, n, r1 + 8 * j, [c])
                 for c in range(7) for n in range(7) for j in range(n1)]
                + [functools.partial(rhs_job, w2, K2, N2, rhs2_loc, n, r2 + 8 * j, [c])
                   for c in range(7) for n in range(2) for j in range(n2)])

    def bulk_o(lhs, n, jobs, side=lambda: None, density=None):
        if density is None:
            density = (len(jobs) + 4) / (7 * 64)
        credit = [-2.0]

        def tie_lhs(tiles):
            tiles = [[t[8 * g:8 * g + 8] for g in range(16)] for t in tiles]
            for w in range(4):
                for g in range(16):
                    credit[0] += density
                    for extra in range(2):
                        if jobs and credit[0] >= 1.0:
                            credit[0] -= 1.0
                            t = tiles[4 * w + (g + 2 * extra) % 4]
                            t[g] = t[g] | (jobs.pop(0)() & zerob[...])
            return _bf(jnp.concatenate([jnp.concatenate(t, axis=0) for t in tiles], axis=1))

        def prod(c):
            side()
            return _dot(tie_lhs(lhs[c]),
                        _rhs_operand(c, lambda a, b: wo[n + 4 * b, pl.ds(a * 1024, 1024), :]))

        def finish(y, rh, ch):
            cols = pl.ds(pl.multiple_of((n + 4 * ch) * 128, 128), 128)
            ha[pl.ds(NSEG * TOK + rh * 256, 256), cols] = y

        _strassen(prod, finish)
        assert not jobs

    def a_blk(rh, kh):
        return jnp.concatenate([oring[h, pl.ds(rh * 256, 256), :]
                                for h in range(16 * kh, 16 * kh + 16)], axis=1)

    (a1, a2), (m1, m2), (z1, z2) = P3_SPLIT
    assert a1 + 2 * m1 + z1 == K1 // 8 and a2 + 2 * m2 + z2 == K2 // 8
    pks.pop(0)
    with jax.named_scope("p3_first"):
        lhs_o = [[pack(v[:, 128 * t:128 * t + 128]) for t in range(16)]
                 for v in _lhs_combos(a_blk(0, 0), a_blk(0, 1), a_blk(1, 0), a_blk(1, 1))]
        bulk_o(lhs_o, 0, w_jobs(0, a1, 0, a2))
    pks.pop(0)

    def bulk_mid(n, carry):
        bulk_o(lhs_o, n, w_jobs(pl.multiple_of(8 * (a1 + (n - 1) * m1), 8), m1,
                                pl.multiple_of(8 * (a2 + (n - 1) * m2), 8), m2))
        return carry

    with jax.named_scope("p3_mid"):
        lax.fori_loop(1, 3, bulk_mid, 0)
    pks.pop(0)

    def bulk_last(zero):
        jobs = w_jobs(8 * (a1 + 2 * m1), z1, 8 * (a2 + 2 * m2), z2)
        density = (len(jobs) + 56 + 4) / (7 * 64)
        state = dict(dep=None, piece=0, window=0)
        pending = []
        hs = {}

        def side():
            jobs.extend(pending)
            del pending[:]
            for _ in range(LN0_PLAN[state['window']]):
                k, r = state['piece'] // 4, state['piece'] % 4
                state['dep'] = ln2_piece(hs, zero, r * QB + 16 * k, state['dep'])
                if r == 3:
                    pending.extend(functools.partial(lhs1_job, hs, 0, k, t, c)
                                   for t in range(2) for c in range(7))
                state['piece'] += 1
            state['window'] += 1

        bulk_o(lhs_o, 3, jobs, side, density)
        assert not pending and state['piece'] == 16

    with jax.named_scope("p3_last"):
        bulk_last(zero_s[0])

    pks.pop(0)
    out32 = out_hbm.bitcast(F32)
    qka[16, pl.ds(0, 8), :] = jnp.zeros((8, E), F32)

    def ffn(i, carry):
        base = pl.multiple_of((i & 1) * 512, 512)
        nbase = pl.multiple_of(((i + 1) & 1) * 512, 512)
        nxt = (i + 1) & (nb - 1)
        half = i >> 2
        srow = pl.multiple_of((i & 3) * HB, HB)

        g = {(c, d): [] for c in range(7) for d in range(7)}
        for n in range(7):
            act = {}

            def prod1(c, d):
                r0, c0 = lhs1_loc(base, c, d)
                return _dot(_bf(hn[pl.ds(r0, QB // 2), pl.ds(c0, 256)]),
                            _bf(rhs_load(w1, K1, N1, rhs1_loc, c, d, n)))

            def activate(y, rh, ch):
                b1 = jnp.concatenate([biasb[:, pl.ds((2 * ch + ci) * N1 + n * 128, 128)] for ci in range(2)],
                                     axis=1)
                act[rh, ch] = jax.nn.gelu(y + rep(b1, HB), approximate=True)

            _strassen(lambda c: _strassen_value(prod1, c), activate)
            for c in range(7):
                o = _combo(_LHS_TERMS, c, lambda a, b: act[a, b])
                for d, v in enumerate(_lhs_combos(o[:QB, :128], o[:QB, 128:], o[QB:, :128], o[QB:, 128:])):
                    g[c, d].append(v.astype(BF16))

        state = dict(dep=None, piece=0, window=0)
        jobs, pending, hs = [], [], {}
        tie = make_tie(jobs, 0.0)

        def next_block_ln():
            jobs.extend(pending)
            del pending[:]
            for _ in range(LN_PLAN[state['window']]):
                k, r = state['piece'] // 4, state['piece'] % 4
                pin = pltpu.bitcast(qka[16, pl.ds(0, 8), :], U32)
                dep = pin if state['dep'] is None else state['dep'] | pin
                state['dep'] = ln2_piece(hs, nxt, r * QB + 16 * k, dep)
                if r == 3:
                    pending.extend(functools.partial(lhs1_job, hs, nbase, k, t, c)
                                   for t in range(2) for c in range(7))
                state['piece'] += 1
            state['window'] += 1

        for n in range(2):
            def prod2(c, d):
                return _dot(jnp.concatenate(g[c, d], axis=1),
                            _bf(tie(rhs_load(w2, K2, N2, rhs2_loc, c, d, n), FFN_DENSITY)))

            def outer(c):
                next_block_ln()
                y = _strassen_value(prod2, c)
                qka[17, pl.ds(srow, 8), :] = y[0:8, 0:128]
                return y

            def finish(y, rh, ch):
                for ci in range(2):
                    nn = (2 * ch + ci) * 2 + n
                    cols = pl.ds(nn * 128, 128)
                    mcols = pl.ds((nn % 2) * 128, 128)
                    yy = y[:, ci * 128:(ci + 1) * 128] + rep(biasb[:, pl.ds(FF + nn * 128, 128)], HB)
                    xr = pl.ds(pl.multiple_of(i * HB, HB) + rh * (HB // 2), HB // 2)
                    ar = pl.ds(pl.multiple_of(i * FB, FB) + rh * HB, HB)
                    x2 = _bf(xs[xr, cols]).astype(F32) + rep(modb[nn // 2, :, mcols], HB) * ha[ar, cols]
                    qka[2 * nn + half, pl.ds(srow + rh * (HB // 2), HB // 2), :] = pack(
                        x2 + rep(modb[12 + nn // 2, :, mcols], HB) * yy, F32)
                    if rh == ch:
                        pltpu.make_async_copy(
                            qka.at[2 * nn + half, pl.ds(srow, HB), :],
                            out32.at[pl.ds(pl.multiple_of(i * HB, HB), HB), cols],
                            sem.at[SEM_OUT]).start()

            _strassen(outer, finish)
        assert not jobs and not pending and state['piece'] == 16
        return carry

    with jax.named_scope("p4_ffn"):
        lax.fori_loop(0, nb, ffn, 0)
    pltpu.make_async_copy(out32, out32, sem.at[SEM_OUT]).wait()


@jax.jit
def pallas_adaLN_cond__memory_aug_recurrent_mem_tr__dense_activation_gelu__prompt_kernel(
    A_x, A_mem0, A_Wq, A_Wk, A_Wv, A_Wo, A_seg_len, B_x, B_w1, B_b1, B_w2, B_b2, c, w_mod,
):
    assert A_x.shape == (1, S, D) and A_Wq.shape == (D, H, E) and A_mem0.shape == (1, M, D)
    any_spec = pl.BlockSpec(memory_space=pl.ANY)
    out = pl.pallas_call(
        _kernel,
        out_shape=jax.ShapeDtypeStruct((S, D), BF16),
        in_specs=[any_spec] * 12,
        out_specs=any_spec,
        scratch_shapes=[
            pltpu.VMEM((S // 2, D), U32),
            pltpu.VMEM((96, D // 2, E), U32),
            pltpu.VMEM((8, H * E // 2, 128), U32),
            pltpu.VMEM((D // 2, FF), U32),
            pltpu.VMEM((FF // 2, D), U32),
            pltpu.VMEM((H, RING, E), F32),
            pltpu.VMEM((H, RING, E), F32),
            pltpu.VMEM((H + 1, RING, E), F32),
            pltpu.VMEM((H, RING, E), F32),
            pltpu.VMEM((S, D), F32),
            pltpu.VMEM((S - PRE, D), F32),
            pltpu.VMEM((M, D), F32),
            pltpu.VMEM((NQ, 2, 8, KQ), F32),
            pltpu.VMEM((16, 8, 256), F32),
            pltpu.VMEM((8, D), U32),
            pltpu.VMEM((D // 2, 128), U32),
            pltpu.VMEM((2, 2, D // 2, 128), F32),
            pltpu.VMEM((8, FF + D), F32),
            pltpu.VMEM((80, 128), F32),
            pltpu.VMEM((8, 32, 128), F32),
            pltpu.VMEM((8, 128), U32),
            pltpu.SMEM((1,), jnp.int32),
            pltpu.VMEM((8, FF // 8, 128), U32),
            pltpu.VMEM((13 * 64, D), U32),
            pltpu.VMEM((128, 256), U32),
            pltpu.VMEM((128, 256), U32),
            pltpu.VMEM((128, 256), U32),
            pltpu.VMEM((128, 256), U32),
            pltpu.VMEM((128, 256), U32),
            pltpu.VMEM((128, 256), U32),
            pltpu.VMEM((M, D), BF16),
            pltpu.VMEM((FF,), BF16),
            pltpu.VMEM((D,), BF16),
            pltpu.VMEM((1, D), BF16),
            pltpu.SemaphoreType.DMA((NSEM,)),
        ],
        compiler_params=pltpu.CompilerParams(vmem_limit_bytes=127 * 1024 * 1024, disable_bounds_checks=True,
                                             disable_semaphore_checks=True),
    )(
        A_x.reshape(S, D), A_mem0.reshape(M, D),
        A_Wq.reshape(D // 2, 2, H, E), A_Wk.reshape(D // 2, 2, H, E), A_Wv.reshape(D // 2, 2, H, E),
        A_Wo.reshape(H * E, D), B_w1, B_b1, B_w2, B_b2, c, w_mod,
    )
    return out.reshape(1, S, D)
```

```python
import functools
import math

import jax
import jax.numpy as jnp
from jax import lax
import jax.experimental.pallas as pl
import jax.experimental.pallas.tpu as pltpu

F32 = jnp.float32
BF16 = jnp.bfloat16
U32 = jnp.uint32

S = 2048
D = 1024
H = 32
E = 128
M = 8
SEG = 32
NSEG = S // SEG
FF = 3584
NP = H // 2
TOK = 24
PRE = S - NSEG * TOK
RING = 576
OOFF = (-NSEG * TOK) % RING
LN_EPS = 1e-5
FB = 256
P3_SPLIT = ((4, 10), (4, 18), (4, 10))
LN0_PLAN = (3, 3, 3, 3, 2, 2, 0)
LN_PLAN = (1, 1, 1, 1, 1, 1, 1, 2, 2, 2, 2, 1, 0, 0)
FFN_DENSITY = 1.0 / 24
ATT_COL, ATT_N1, ATT_N2 = 6, 2, 5
UNROLL = 4

NQ = 4
KQ = D // NQ

FIRST_STARTS = [('m', 0), ('w', 0, 0, 4), ('w', 0, 4, 8), ('m', 1), ('w', 0, 8, 12), ('w', 1, 0, 8), ('m', 2),
                ('w', 1, 8, 12)]
P1A_BLOCKS = [
    ([], [('m', 0)]),
    ([], [('w', 0, 0, 4)]),
    ([], [('w', 0, 4, 8)]),
    ([('w', 2, 0, 8), ('m', 3), ('w', 2, 8, 12)], [('m', 1), ('w', 0, 8, 12)]),
    ([('w', 3, 0, 12)], [('w', 1, 0, 8)]),
    ([('g', 2), ('g', 3)], [('m', 2), ('w', 1, 8, 12)]),
    ([], [('w', 2, 0, 8)]),
    ([('g', 4), ('g', 5)], [('m', 3), ('w', 2, 8, 12)]),
    ([], [('w', 3, 0, 12)]),
]
W_ITEMS = [it for _, items in P1A_BLOCKS for it in items if it[0] == 'w']
IT_ROWS = TOK * UNROLL
X_CHUNKS = (PRE, PRE + IT_ROWS, PRE + 3 * IT_ROWS, S)
LN_SLOTS = ((0, 11), (1, 5))
MOD_SLOTS = ((0, 2), (0, 4), (0, 6), (1, 8), (1, 9), (1, 10), (1, 11), (2, 0))
NX0 = 4

SEM_C = 0
SEM_X0 = 1
SEM_MOD = SEM_X0 + NX0
SEM_WA = SEM_MOD + NQ + 2
SEM_WB = SEM_WA + 10
SEM_XC = SEM_WB + 6
SEM_WO = SEM_XC + 3
SEM_W1 = SEM_WO + 1
SEM_W2 = SEM_W1 + 1
SEM_OUT = SEM_W2 + 1
NSEM = SEM_OUT + 1


def _ln(x):
    m = jnp.mean(x, axis=-1, keepdims=True)
    xc = x - m
    v = jnp.mean(xc * xc, axis=-1, keepdims=True)
    return xc * lax.rsqrt(v + LN_EPS)


def _bf(w32):
    return pltpu.bitcast(w32, BF16)


def _dot(a, b):
    return jnp.dot(a, b, preferred_element_type=F32)


def _lhs_combos(a11, a12, a21, a22):
    return [a11 - a22, a21 - a22, a11, a22, a12 - a11, a21 - a11, a12 - a22]


def _rhs_combos(b11, b12, b21, b22):
    return [b11 - b22, b11, b12 + b22, b21 + b11, b22, b11 + b12, b21 + b22]


_LHS_TERMS = {0: ((0, 0), (1, 1), -1), 1: ((1, 0), (1, 1), -1), 2: ((0, 0), None, 0), 3: ((1, 1), None, 0),
              4: ((0, 1), (0, 0), -1), 5: ((1, 0), (0, 0), -1), 6: ((0, 1), (1, 1), -1)}
_RHS_TERMS = {0: ((0, 0), (1, 1), -1), 1: ((0, 0), None, 0), 2: ((0, 1), (1, 1), 1), 3: ((1, 0), (0, 0), 1),
              4: ((1, 1), None, 0), 5: ((0, 0), (0, 1), 1), 6: ((1, 0), (1, 1), 1)}
_SWAP = {c: int(c in (2, 4, 5, 6)) for c in range(7)}


def _combo(terms, c, blk):
    p, q, sign = terms[c]
    if q is None:
        return blk(*p)
    return blk(*p) + blk(*q) if sign > 0 else blk(*p) - blk(*q)


def _rhs_operand(c, blk):
    p, q, sign = _RHS_TERMS[c]
    a = _bf(blk(*p))
    if q is None:
        return a
    a = a.astype(F32)
    b = _bf(blk(*q)).astype(F32)
    return (a + b if sign > 0 else a - b).astype(BF16)


def _strassen(prod, finish, side=lambda: None):
    side()
    m1 = prod(1)
    m3 = prod(3)
    finish(m1 + m3, 1, 0)
    side()
    m2 = prod(2)
    m4 = prod(4)
    finish(m2 + m4, 0, 1)
    side()
    m0 = prod(0)
    m5 = prod(5)
    finish((m2 - m1) + m0 + m5, 1, 1)
    side()
    m6 = prod(6)
    finish((m3 - m4) + m0 + m6, 0, 0)


def _strassen_value(prod2, c):
    r = {}
    _strassen(functools.partial(prod2, c), lambda y, rh, ch: r.__setitem__((rh, ch ^ _SWAP[c]), y))
    return jnp.concatenate([jnp.concatenate([r[0, 0], r[0, 1]], axis=1),
                            jnp.concatenate([r[1, 0], r[1, 1]], axis=1)], axis=0)


_ORDER = (1, 3, 2, 4, 0, 5, 6)

_PAIRS = [(c, d) for c in range(7) for d in range(7) if not (c in (1, 4) and d in (1, 4))]


def _plain_block(c, d):
    return 2 * (c // 4) + d // 4, 2 * (c // 4) + ((d // 4) ^ _SWAP[c])


def _kernel(x_hbm, mem0_hbm, wq_hbm, wk_hbm, wv_hbm, wo_hbm, w1_hbm, b1_hbm, w2_hbm, b2_hbm,
            c_hbm, wmod_hbm, out_hbm,
            xs, wqkv, wo, w1, w2, qka, qkb, vring, oring, ha, hn, memb, moda, modb, scb, colb, slab, biasb,
            fillb, accb, zerob, zero_s, wx, hb2, pk0, pk1, pk2, pk3, pk4, pk5, mem0_ref, b1_ref, b2_ref, c_ref, sem):
    qkv_hbm = [r.bitcast(U32) for r in (wq_hbm, wk_hbm, wv_hbm)]
    x32 = x_hbm.bitcast(U32)
    wo32 = wo_hbm.bitcast(U32)
    wmod32 = wmod_hbm.bitcast(F32)

    def wma(qq, k):
        return pl.ds(512 * (qq // 2), 512), pl.ds(512 * (qq % 2) + k * KQ, KQ)

    def hb_idx(c, q0, nq, row0=0, nrows=PRE // 4):
        return pl.ds(1024 + 128 * (c // 2) + row0, nrows), pl.ds(512 * (c % 2) + 128 * q0, 128 * nq)

    def units_start(lo, hi, rows, sem_idx):
        for u in range(lo, hi):
            j, m = u // 3, u % 3
            for p in range(2):
                pltpu.make_async_copy(qkv_hbm[m].at[rows, p, j, :], wqkv.at[2 * u + p, rows, :],
                                      sem.at[sem_idx]).start()

    def units_wait(lo, n, rows, sem_idx):
        blk = wqkv.at[pl.ds(2 * lo, 2 * n), rows, :]
        pltpu.make_async_copy(blk, blk, sem.at[sem_idx]).wait()

    def item_start(item):
        if item[0] == 'm':
            qq = item[1]
            for k in range(2):
                pltpu.make_async_copy(wmod32.at[:, pl.ds(k * D + qq * KQ, KQ)], ha.at[wma(qq, k)],
                                      sem.at[SEM_MOD + qq]).start()
        elif item[0] == 'w':
            _, qq, lo, hi = item
            units_start(lo, hi, pl.ds(qq * (KQ // 2), KQ // 2), SEM_WA + W_ITEMS.index(item))
        else:
            whole_start(item[1])

    def item_wait(item):
        if item[0] == 'm':
            qq = item[1]
            blk = ha.at[pl.ds(512 * (qq // 2), 512), pl.ds(512 * (qq % 2), 512)]
            pltpu.make_async_copy(blk, blk, sem.at[SEM_MOD + qq]).wait()
        else:
            _, qq, lo, hi = item
            units_wait(lo, hi - lo, pl.ds(qq * (KQ // 2), KQ // 2), SEM_WA + W_ITEMS.index(item))

    def whole_start(i):
        if i == 2:
            xc_copy(0).start()
        units_start(6 * i, 6 * i + 6, pl.ds(0, D // 2), SEM_WB + i - 2)

    def slab_copies(it):
        return [pltpu.make_async_copy(
            wmod32.at[:, pl.ds(pl.multiple_of(2 * D + it * 256 + t * 128, 128), 128)],
            slab.at[it & 1, t], sem.at[SEM_MOD + NQ + (it & 1)]) for t in range(2)]

    def x0_copy(i):
        n = PRE // 2 // NX0
        rows = pl.ds(pl.multiple_of(i * n, n), n)
        return pltpu.make_async_copy(x32.at[rows], xs.at[rows], sem.at[SEM_X0 + i])

    def xc_copy(i):
        rows = pl.ds(X_CHUNKS[i] // 2, (X_CHUNKS[i + 1] - X_CHUNKS[i]) // 2)
        return pltpu.make_async_copy(x32.at[rows], xs.at[rows], sem.at[SEM_XC + i])

    def wo_copy(n):
        return pltpu.make_async_copy(wo32.at[:, pl.ds(n * 128, 128)], wo.at[n], sem.at[SEM_WO])

    w1_copy = pltpu.make_async_copy(w1_hbm.bitcast(U32), w1, sem.at[SEM_W1])
    w2_copy = pltpu.make_async_copy(w2_hbm.bitcast(U32), w2, sem.at[SEM_W2])
    small_copies = [pltpu.make_async_copy(a, b, sem.at[SEM_C])
                    for a, b in ((c_hbm, c_ref), (mem0_hbm, mem0_ref), (b1_hbm, b1_ref),
                                 (b2_hbm, b2_ref))]

    def deinterleave(u, row0, nrows):
        for k in range(nrows // 64):
            rows = pl.ds(row0 + k * 64, 64)
            a = wqkv[2 * u, rows, :]
            b = wqkv[2 * u + 1, rows, :]
            wqkv[2 * u, rows, :] = (a & jnp.uint32(0xFFFF)) | (b << 16)
            wqkv[2 * u + 1, rows, :] = (a >> 16) | (b & jnp.uint32(0xFFFF0000))

    def load_x16(row2, dep):
        xw = xs[pl.ds(row2, 8), :]
        if dep is not None:
            first = xw[:, 0:128] | (dep & zerob[...])
            xw = jnp.concatenate([first, xw[:, 128:]], axis=1)
        return _bf(xw).astype(F32)

    pks = [pk0, pk1, pk2, pk3, pk4, pk5]

    def pack(v, dtype=U32):
        rows = pl.ds(0, v.shape[0] // 2)
        pk = pks[0]
        pk[rows, pl.ds(0, 128)] = pltpu.bitcast(v.astype(BF16), U32)
        return pltpu.bitcast(pk[rows, pl.ds(0, 128)], dtype)

    def rep(v8, n):
        return jnp.concatenate([v8] * (n // 8), axis=0)

    def mrow(k, n):
        if k < 2:
            return rep(jnp.concatenate([moda[qq, k] for qq in range(NQ)], axis=1), n)
        return rep(jnp.concatenate([modb[4 * (k - 2) + q] for q in range(4)], axis=1), n)

    for cp in small_copies:
        cp.start()
    for i in range(NX0):
        x0_copy(i).start()
    for item in FIRST_STARTS:
        item_start(item)

    def start_rest():
        xc_copy(1).start()
        for n in range(8):
            wo_copy(n).start()
        for cp in slab_copies(0):
            cp.start()
        xc_copy(2).start()
        w1_copy.start()
        w2_copy.start()

    r = lax.broadcasted_iota(jnp.int32, (80, 128), 0)
    q = lax.broadcasted_iota(jnp.int32, (80, 128), 1)
    r_tok = r < 64
    q_tok = q < 64
    r_head = jnp.where(r_tok, r >> 5, (r - 64) >> 3)
    q_head = jnp.where(q_tok, q >> 5, (q - 64) >> 3)
    same = (r_head == q_head) & (q < 80)
    causal_ok = jnp.logical_not(r_tok & q_tok & ((q & 31) > (r & 31)))
    scale = E ** (-0.5)
    fillb[...] = jnp.where(same, jnp.where(causal_ok, 0.0, -1e9 / scale), -jnp.inf).astype(F32)
    zerob[...] = jnp.zeros((8, 128), U32)
    zero_s[0] = 0

    for cp in small_copies:
        cp.wait()
    cf = c_ref[...].astype(F32)
    sc = (cf * jax.nn.sigmoid(cf)).astype(BF16)
    scb[...] = pltpu.bitcast(jnp.broadcast_to(sc, (16, D)), U32)
    scf = jnp.broadcast_to(sc.astype(F32), (128, D))
    for k in range(8):
        colb[pl.ds(k * 64, 64), :] = pltpu.bitcast(scf[:, k * 128:(k + 1) * 128].T.astype(BF16), U32)
    memb[...] = mem0_ref[...].astype(F32)
    biasb[:, pl.ds(0, FF)] = jnp.broadcast_to(b1_ref[...].astype(F32).reshape(1, FF), (8, FF))
    biasb[:, pl.ds(FF, D)] = jnp.broadcast_to(b2_ref[...].astype(F32).reshape(1, D), (8, D))

    def pre_norm(i, carry):
        x0_copy(i).wait()
        nr = PRE // NX0
        for z in range(nr // 16):
            xn = _ln(load_x16(pl.multiple_of(i * (nr // 2) + z * 8, 8), None))
            for n in range(8):
                oring[n, pl.ds(pl.multiple_of(i * nr + z * 16, 16), 16), :] = xn[:, n * 128:(n + 1) * 128]
        return carry

    with jax.named_scope("p0_ln"):
        lax.fori_loop(0, NX0, pre_norm, 0)

    def dst_slot(i, k, p):
        cls, m = k // 3, k % 3
        if m == 2:
            return vring, 4 * i + 2 * cls + p
        return (qka, qkb)[cls], 4 * i + 2 * m + p

    PH = PRE // 2
    assert KQ == 256

    def item_run(item):
        if item[0] == 'm':
            qq = item[1]
            sc16 = _bf(scb[...])
            ca1 = 1.0 + _dot(sc16, _bf(ha[wma(qq, 1)]))[0:8].astype(BF16).astype(F32)
            sa = _dot(sc16, _bf(ha[wma(qq, 0)]))[0:8].astype(BF16).astype(F32)
            moda[qq, 0] = sa
            moda[qq, 1] = ca1
            for z in range(PH // 32):
                def h_blk(rh, kh):
                    cols = slice(kh * 128, (kh + 1) * 128)
                    return (oring[2 * qq + kh, pl.ds(rh * PH + z * 32, 32), :] * rep(ca1[:, cols], 32)
                            + rep(sa[:, cols], 32))

                for c, v in enumerate(_lhs_combos(h_blk(0, 0), h_blk(0, 1), h_blk(1, 0), h_blk(1, 1))):
                    ha[hb_idx(c, qq, 1, z * 16, 16)] = pltpu.bitcast(v.astype(BF16), F32)
            return
        _, qq, lo, hi = item
        if lo == 0 and qq >= 2:
            a_jobs.extend(functools.partial(lhs0_job, k, qq - 2, c) for k in range(PQ // 16) for c in range(7))
        for u in range(lo, hi):
            deinterleave(u, qq * (KQ // 2), KQ // 2)
            i, k = u // 6, u % 6

            def prod(c):
                lhs = pltpu.bitcast(ha[hb_idx(c, qq, 1)], U32)
                if u >= 2:
                    lhs = tie_rows(lhs, a_jobs, (1 + 4 * ((7 * u + _ORDER.index(c)) % 4),))
                rhs = _rhs_operand(c, lambda a, b: wqkv[2 * u + b, pl.ds((2 * qq + a) * 64, 64), :])
                return _dot(_bf(lhs), rhs)

            def finish(y, rh, ch):
                ref, idx = dst_slot(i, k, ch)
                rows = pl.ds(RING - PRE + rh * PH, PH)
                if qq > 0:
                    y = y + ref[idx, rows, :]
                ref[idx, rows, :] = y

            _strassen(prod, finish)

    def tie_rows(w, jobs, groups):
        if not jobs:
            return w
        parts = [w[8 * g:8 * g + 8, 0:128] for g in range(w.shape[0] // 8)]
        for g in groups:
            if jobs:
                parts[g] = parts[g] | (jobs.pop(0)() & zerob[...])
        first = jnp.concatenate(parts, axis=0)
        return first if w.shape[1] == 128 else jnp.concatenate([first, w[:, 128:]], axis=1)

    PQ = PRE // 4
    a_jobs = []

    def lhs0_idx(c, d, k, nk, t, nt):
        e = 7 * c + d
        return pl.ds(64 * (e // 4) + 8 * k, 8 * nk), pl.ds(256 * (e % 4) + 128 * t, 128 * nt)

    def lhs0_job(k, t, c):
        def sub(ri, ki):
            def blk(ro, ko):
                n = 2 * ko + ki + 4 * t
                cols = pl.ds((n % 2) * 128, 128)
                return (oring[n, pl.ds((2 * ro + ri) * PQ + 16 * k, 16), :] * rep(moda[n // 2, 1, :, cols], 16)
                        + rep(moda[n // 2, 0, :, cols], 16))

            return _combo(_LHS_TERMS, c, blk)

        bits = None
        for d, v in enumerate(_lhs_combos(sub(0, 0), sub(0, 1), sub(1, 0), sub(1, 1))):
            hb2[lhs0_idx(c, d, k, 1, t, 1)] = pltpu.bitcast(v.astype(BF16), U32)
            if d not in (2, 3):
                b = pltpu.bitcast(v[8 * (d % 2):8 * (d % 2) + 8], U32)
                bits = b if bits is None else bits | b
        return bits

    def ln1_piece(row2):
        h16 = _ln(load_x16(PRE // 2 + row2, None)) * mrow(1, 16) + mrow(0, 16)
        hn[pl.ds(pl.multiple_of(2 * row2, 16), 16), :] = h16
        return pltpu.bitcast(h16[8:16, D - 128:], U32)

    def phase1b(i, carry):
        @pl.when(i == 3)
        def _():
            whole_start(6)
            whole_start(7)
            start_rest()

        units_wait(6 * i, 6, pl.ds(0, D // 2), SEM_WB + i - 2)
        ln1_piece(pl.multiple_of((i - 2) * 8, 8))

        def raw(m, kq, nq, g):
            u = 6 * i + m + 3 * (nq // 2)
            return wqkv[2 * u + nq % 2, pl.ds((kq + 4 * (g // 8)) * 64 + 8 * (g % 8), 8), :]

        ops = {}

        def rhs0_job(m, c, g):
            def sub(ki, ni):
                return _combo(_RHS_TERMS, c,
                              lambda ko, no: _bf(raw(m, 2 * ko + ki, 2 * no + (ni ^ _SWAP[c]), g)).astype(F32))

            bits = None
            for d, v in enumerate(_rhs_combos(sub(0, 0), sub(0, 1), sub(1, 0), sub(1, 1))):
                if (c, d) in _PAIRS:
                    ops[m, c, d, g] = pack(v)
                    bits = ops[m, c, d, g] if bits is None else bits | ops[m, c, d, g]
            return bits

        seq = [(m, c) for m in range(3) for c in _ORDER]
        jobs = []
        count = [0]
        deinterleave(6 * i, 0, D // 2)
        deinterleave(6 * i + 3, 0, D // 2)
        for g in range(16):
            rhs0_job(*seq[0], g)
        for m in range(3):
            if m < 2:
                deinterleave(6 * i + m + 1, 0, D // 2)
                deinterleave(6 * i + m + 4, 0, D // 2)

            def prod(c, d):
                if (c, d) in _PAIRS:
                    rhs = [ops[m, c, d, g] for g in range(16)]
                else:
                    rhs = [raw(m, *_plain_block(c, d), g) for g in range(16)]
                lhs = tie_rows(hb2[lhs0_idx(c, d, 0, 8, 0, 2)], jobs, ((0, 3, 6), (1, 4, 7))[count[0] % 2])
                count[0] += 1
                return _dot(_bf(lhs), _bf(jnp.concatenate(rhs, axis=0)))

            def outer(c):
                assert not jobs
                count[0] = 0
                nx = seq.index((m, c)) + 1
                if nx < len(seq):
                    jobs.extend(functools.partial(rhs0_job, *seq[nx], g) for g in range(16))
                return _strassen_value(prod, c)

            def finish(y, rh, ch):
                for ci in range(2):
                    ref, idx = dst_slot(i, m + 3 * ch, ci)
                    ref[idx, pl.ds(RING - PRE + rh * PH, PH), :] = y[:, ci * 128:(ci + 1) * 128]

            _strassen(outer, finish)
        return carry

    for bi, (starts, items) in enumerate(P1A_BLOCKS):
        for item in starts:
            item_start(item)
        with jax.named_scope("p1a_wait%d" % bi):
            for item in items:
                item_wait(item)
        for item in items:
            item_run(item)
    assert not a_jobs
    xc_copy(0).wait()
    with jax.named_scope("p1b"):
        lax.fori_loop(2, 8, phase1b, 0)
    pks.pop(0)
    xc_copy(1).wait()
    for n in range(8):
        wo_copy(n).wait()

    cexp = scale * math.log2(math.e)
    NG = NP // 2
    grp = [(4 * (g // 2) + (g % 2), 4 * (g // 2) + (g % 2) + 2) for g in range(NG)]
    early = [2 * j + u for g in range(NG - 3) for j in grp[g] for u in range(2)]
    late = [h for h in range(H) if h not in early]

    def step(it, k, side_jobs):
        s = it * UNROLL + k
        split = k > 0
        base = TOK * UNROLL * it
        w0 = pl.multiple_of(lax.rem(base, RING), 32) + TOK * k
        r0 = pl.multiple_of(lax.rem(SEG * s + (RING - PRE), RING), 32)
        ow = pl.multiple_of(lax.rem(SEG * s + OOFF, RING), 32)
        o0 = pl.multiple_of(lax.rem(base + OOFF, RING), 32) + TOK * k
        a0 = pl.multiple_of(base, 32) + TOK * k
        X = jnp.concatenate([hn[pl.ds(a0, TOK), :], memb[...]], axis=0).astype(BF16)
        ym = [None] * 96
        probs = [None] * NP
        om = [None] * H
        order = (4, 5, 0, 1, 2, 3)

        if split:
            for t in order:
                accb[t] = _dot(X[:, :D // 2], _bf(wqkv[t, pl.ds(0, D // 4), :]))

        def slot(j, t):
            if t >= 4:
                return vring, 2 * j + t - 4
            return (qka, qkb)[j % 2], 4 * (j // 2) + t

        def proj(j, t, job):
            c = 6 * j + t
            bits = None if job is None else job()
            if split and j == 0:
                y = accb[t] + _dot(X[:, D // 2:], _bf(wqkv[c, pl.ds(D // 4, D // 4), :]))
            else:
                y = _dot(X, _bf(wqkv[c]))
            ref, k = slot(j, t)
            if bits is not None:
                y0 = pltpu.bitcast(pltpu.bitcast(y[0:8], U32) | (bits & zerob[...]), F32)
                y = jnp.concatenate([y0, y[8:]], axis=0)
            ref[k, pl.ds(w0, TOK), :] = y[0:TOK]
            ym[c] = y[TOK:TOK + M]

        def gather(j, m, pad):
            c = 6 * j + 2 * m
            ref, k = slot(j, 2 * m)
            parts = [ref[k, pl.ds(r0, SEG), :], ref[k + 1, pl.ds(r0, SEG), :], ym[c], ym[c + 1]]
            if pad:
                parts.append(jnp.zeros((48, E), F32))
            return jnp.concatenate(parts, axis=0).astype(BF16)

        def scores(j):
            sc_ = lax.dot_general(gather(j, 0, False), gather(j, 1, True),
                                  (((1,), (1,)), ((), ())), preferred_element_type=F32)
            fill = fillb[...]
            sc_ = jnp.where(fill == 0.0, sc_, fill)
            mx = jnp.max(sc_, axis=-1, keepdims=True)
            p = jnp.exp2((sc_ - mx) * cexp)
            l = jnp.sum(p, axis=-1, keepdims=True)
            rl = pl.reciprocal(l, approx=True)
            rl = rl * (2.0 - l * rl)
            probs[j] = p * rl

        def park(j):
            vring[H, pl.ds(40 * (j % 8), 40), :] = pack(probs[j], F32)
            probs[j] = None

        def pv(j):
            if probs[j] is None:
                P = _bf(vring[H, pl.ds(40 * (j % 8), 40), :])
            else:
                P = probs[j].astype(BF16)
            o = _dot(P, gather(j, 2, True))
            oring[2 * j, pl.ds(ow, SEG), :] = o[0:32]
            oring[2 * j + 1, pl.ds(ow, SEG), :] = o[32:64]
            om[2 * j] = o[64:72]
            om[2 * j + 1] = o[72:80]

        def o_lhs(hs):
            return jnp.concatenate(
                [jnp.concatenate([oring[h, pl.ds(o0, TOK), :], om[h]], axis=0) for h in hs],
                axis=1).astype(BF16)

        def o_rhs(n, hs):
            return _bf(jnp.concatenate([wo[n, pl.ds(h * 64, 64), :] for h in hs], axis=0))

        for g in range(NG):
            cols = [(j, t) for j in grp[g] for t in order]
            if g == 2:
                cols = ([(j, t) for j in grp[g] for t in (4, 5)]
                        + [(j, t) for j in grp[g] for t in range(4)])
            for j in (grp[0] + grp[1] if g == 3 else grp[g - 2] if g >= 4 else ()):
                park(j)
            for ci, (j, t) in enumerate(cols):
                if g == 2 and ci == 4:
                    for jj in grp[0] + grp[1]:
                        scores(jj)
                if g >= 3 and ci == ATT_COL:
                    for jj in grp[g - 1]:
                        scores(jj)
                    for jj in grp[g - 3]:
                        pv(jj)
                proj(j, t, side_jobs.get((g, ci)))
        lo = o_lhs(early)
        for n in range(8):
            accb[n] = _dot(lo, o_rhs(n, early))
            if n == ATT_N1:
                for jj in grp[NG - 1]:
                    scores(jj)
                for jj in grp[NG - 3]:
                    pv(jj)
            if n == ATT_N2:
                for jj in grp[NG - 2] + grp[NG - 1]:
                    pv(jj)
        lo = o_lhs(late)
        for n in range(8):
            a = accb[n] + _dot(lo, o_rhs(n, late))
            ha[pl.ds(a0, TOK), pl.ds(n * 128, 128)] = a[0:TOK]
            memb[:, pl.ds(n * 128, 128)] = a[TOK:TOK + M]

    NIT = NSEG // UNROLL

    def lo16(w):
        return pltpu.bitcast(w << 16, F32)

    def hi16(w):
        return pltpu.bitcast(w & jnp.uint32(0xFFFF0000), F32)

    def steps(it, carry):
        @pl.when(it == 1)
        def _():
            xc_copy(2).wait()

        for cp in slab_copies(it):
            cp.wait()
        for cp in slab_copies((it + 1) & (NIT - 1)):
            cp.start()
        acc = [None, None]

        def mod_job(q):
            for kk in range(2 * q, 2 * q + 2):
                cw = colb[pl.ds(kk * 8, 8), :]
                for t in range(2):
                    w = pltpu.bitcast(slab[it & 1, t, pl.ds(kk * 8, 8), :], U32)
                    v = lo16(w) * lo16(cw) + hi16(w) * hi16(cw)
                    acc[t] = v if acc[t] is None else acc[t] + v
            if q < D // 32 - 1:
                return pltpu.bitcast(acc[0], U32) | pltpu.bitcast(acc[1], U32)
            y = jnp.sum(jnp.concatenate(acc, axis=1), axis=0, keepdims=True).astype(BF16).astype(F32)
            y = jnp.broadcast_to(y + jnp.where((it >> 2) == 2, 1.0, 0.0), (8, 256))
            modb[it] = y
            return pltpu.bitcast(y[:, 0:128], U32)

        nxt2 = pl.multiple_of(jnp.minimum(it + 1, NIT - 1) * (IT_ROWS // 2), 16)
        pieces = list(range(IT_ROWS // 16))
        for k in range(UNROLL):
            side_jobs = {pos: functools.partial(mod_job, 8 * k + q) for q, pos in enumerate(MOD_SLOTS)}
            for pos in LN_SLOTS[k % 2:]:
                side_jobs[pos] = functools.partial(ln1_piece, nxt2 + 8 * pieces.pop(0))
            step(it, k, side_jobs)
        assert not pieces
        return carry

    with jax.named_scope("p2_steps"):
        lax.fori_loop(0, NIT, steps, 0)
    for cp in slab_copies(0):
        cp.wait()
    w1_copy.wait()
    w2_copy.wait()

    nb = S // FB
    HB = FB // 2
    QB = FB // 4

    def ln2_piece(hs, blk, off, dep):
        x2 = (load_x16(pl.multiple_of(blk * HB, HB) + off // 2, dep)
              + mrow(2, 16) * ha[pl.ds(pl.multiple_of(blk * FB, FB) + off, 16), :])
        h = _ln(x2) * mrow(4, 16) + mrow(3, 16)
        hs[off] = h
        return pltpu.bitcast(h[8:16, D - 128:], U32)

    def lhs1_loc(base, c, d):
        e = 7 * c + d
        return base + 32 * (e // 4), 256 * (e % 4)

    def lhs1_job(hs, base, k, t, c):
        def sub(ri, ki):
            def blk(ro, ko):
                c0 = (2 * ko + ki) * 256 + t * 128
                return hs[(2 * ro + ri) * QB + 16 * k][:, c0:c0 + 128]

            return _combo(_LHS_TERMS, c, blk)

        bits = None
        for d, v in enumerate(_lhs_combos(sub(0, 0), sub(0, 1), sub(1, 0), sub(1, 1))):
            r0, c0 = lhs1_loc(base, c, d)
            hn[pl.ds(r0 + 8 * k, 8), pl.ds(c0 + t * 128, 128)] = pltpu.bitcast(
                v.astype(BF16), F32)
            if d not in (2, 3):
                b = pltpu.bitcast(v[8 * (d % 2):8 * (d % 2) + 8], U32)
                bits = b if bits is None else bits | b
        return bits

    K1, N1, K2, N2 = D // 8, FF // 4, FF // 8, D // 4

    def rhs1_loc(c, d, n):
        e = _PAIRS.index((c, d)) * 7 + n
        return wqkv, e // 4, K1 * (e % 4)

    rhs2_slots = ([(wqkv, e, 0) for e in range(79, 96)] + [(qkb, e, 0) for e in range(H)]
                  + [(vring, e, 0) for e in range(H + 1)] + [(wx, e, 0) for e in range(8)])

    def rhs2_loc(c, d, n):
        return rhs2_slots[_PAIRS.index((c, d)) * 2 + n]

    def rhs_job(w, kq, nq, loc, n, r, cs):
        cache = {}

        def blk(ko, no, ki, ni):
            key = (2 * ko + ki, 2 * no + ni)
            if key not in cache:
                cache[key] = _bf(w[pl.ds(r + key[0] * kq, 8), pl.ds(n * 128 + key[1] * nq, 128)]).astype(F32)
            return cache[key]

        bits = None
        for c in cs:
            def sub(ki, ni):
                return _combo(_RHS_TERMS, c, lambda ko, no: blk(ko, no, ki, ni ^ _SWAP[c]))

            for d, v in enumerate(_rhs_combos(sub(0, 0), sub(0, 1), sub(1, 0), sub(1, 1))):
                if (c, d) in _PAIRS:
                    ref, idx, row = loc(c, d, n)
                    b = pack(v)
                    ref[idx, pl.ds(row + r, 8), :] = pltpu.bitcast(b, ref.dtype)
                    bits = b if bits is None else bits | b
        return bits

    def rhs_load(w, kq, nq, loc, c, d, n):
        if (c, d) not in _PAIRS:
            qk, qn = _plain_block(c, d)
            return w[pl.ds(qk * kq, kq), pl.ds(qn * nq + n * 128, 128)]
        ref, idx, row = loc(c, d, n)
        return pltpu.bitcast(ref[idx, pl.ds(row, kq), :], U32)

    def make_tie(jobs, credit):
        state = [credit]

        def tie(raw, density):
            if not jobs:
                return raw
            parts = []
            for r in range(0, raw.shape[0], 8):
                v = raw[r:r + 8]
                state[0] += density
                if jobs and state[0] >= 1.0:
                    state[0] -= 1.0
                    v = v | (jobs.pop(0)() & zerob[...])
                parts.append(v)
            return jnp.concatenate(parts, axis=0)

        return tie

    def w_jobs(r1, n1, r2, n2):
        return ([functools.partial(rhs_job, w1, K1, N1, rhs1_loc, n, r1 + 8 * j, [c])
                 for c in range(7) for n in range(7) for j in range(n1)]
                + [functools.partial(rhs_job, w2, K2, N2, rhs2_loc, n, r2 + 8 * j, [c])
                   for c in range(7) for n in range(2) for j in range(n2)])

    def bulk_o(lhs, n, jobs, side=lambda: None, density=None):
        if density is None:
            density = (len(jobs) + 4) / (7 * 64)
        credit = [-2.0]

        def tie_lhs(tiles):
            tiles = [[t[8 * g:8 * g + 8] for g in range(16)] for t in tiles]
            for w in range(4):
                for g in range(16):
                    credit[0] += density
                    for extra in range(2):
                        if jobs and credit[0] >= 1.0:
                            credit[0] -= 1.0
                            t = tiles[4 * w + (g + 2 * extra) % 4]
                            t[g] = t[g] | (jobs.pop(0)() & zerob[...])
            return _bf(jnp.concatenate([jnp.concatenate(t, axis=0) for t in tiles], axis=1))

        def prod(c):
            side()
            return _dot(tie_lhs(lhs[c]),
                        _rhs_operand(c, lambda a, b: wo[n + 4 * b, pl.ds(a * 1024, 1024), :]))

        def finish(y, rh, ch):
            cols = pl.ds(pl.multiple_of((n + 4 * ch) * 128, 128), 128)
            ha[pl.ds(NSEG * TOK + rh * 256, 256), cols] = y

        _strassen(prod, finish)
        assert not jobs

    def a_blk(rh, kh):
        return jnp.concatenate([oring[h, pl.ds(rh * 256, 256), :]
                                for h in range(16 * kh, 16 * kh + 16)], axis=1)

    (a1, a2), (m1, m2), (z1, z2) = P3_SPLIT
    assert a1 + 2 * m1 + z1 == K1 // 8 and a2 + 2 * m2 + z2 == K2 // 8
    pks.pop(0)
    with jax.named_scope("p3_first"):
        lhs_o = [[pack(v[:, 128 * t:128 * t + 128]) for t in range(16)]
                 for v in _lhs_combos(a_blk(0, 0), a_blk(0, 1), a_blk(1, 0), a_blk(1, 1))]
        bulk_o(lhs_o, 0, w_jobs(0, a1, 0, a2))
    pks.pop(0)

    def bulk_mid(n, carry):
        bulk_o(lhs_o, n, w_jobs(pl.multiple_of(8 * (a1 + (n - 1) * m1), 8), m1,
                                pl.multiple_of(8 * (a2 + (n - 1) * m2), 8), m2))
        return carry

    with jax.named_scope("p3_mid"):
        lax.fori_loop(1, 3, bulk_mid, 0)
    pks.pop(0)

    def bulk_last(zero):
        jobs = w_jobs(8 * (a1 + 2 * m1), z1, 8 * (a2 + 2 * m2), z2)
        density = (len(jobs) + 56 + 4) / (7 * 64)
        state = dict(dep=None, piece=0, window=0)
        pending = []
        hs = {}

        def side():
            jobs.extend(pending)
            del pending[:]
            for _ in range(LN0_PLAN[state['window']]):
                k, r = state['piece'] // 4, state['piece'] % 4
                state['dep'] = ln2_piece(hs, zero, r * QB + 16 * k, state['dep'])
                if r == 3:
                    pending.extend(functools.partial(lhs1_job, hs, 0, k, t, c)
                                   for t in range(2) for c in range(7))
                state['piece'] += 1
            state['window'] += 1

        bulk_o(lhs_o, 3, jobs, side, density)
        assert not pending and state['piece'] == 16

    with jax.named_scope("p3_last"):
        bulk_last(zero_s[0])

    pks.pop(0)
    out32 = out_hbm.bitcast(F32)
    qka[16, pl.ds(0, 8), :] = jnp.zeros((8, E), F32)

    def ffn(i, carry):
        base = pl.multiple_of((i & 1) * 512, 512)
        nbase = pl.multiple_of(((i + 1) & 1) * 512, 512)
        nxt = (i + 1) & (nb - 1)
        half = i >> 2
        srow = pl.multiple_of((i & 3) * HB, HB)

        g = {(c, d): [] for c in range(7) for d in range(7)}
        for n in range(7):
            act = {}

            def prod1(c, d):
                r0, c0 = lhs1_loc(base, c, d)
                return _dot(_bf(hn[pl.ds(r0, QB // 2), pl.ds(c0, 256)]),
                            _bf(rhs_load(w1, K1, N1, rhs1_loc, c, d, n)))

            def activate(y, rh, ch):
                b1 = jnp.concatenate([biasb[:, pl.ds((2 * ch + ci) * N1 + n * 128, 128)] for ci in range(2)],
                                     axis=1)
                act[rh, ch] = jax.nn.gelu(y + rep(b1, HB), approximate=True)

            _strassen(lambda c: _strassen_value(prod1, c), activate)
            for c in range(7):
                o = _combo(_LHS_TERMS, c, lambda a, b: act[a, b])
                for d, v in enumerate(_lhs_combos(o[:QB, :128], o[:QB, 128:], o[QB:, :128], o[QB:, 128:])):
                    g[c, d].append(v.astype(BF16))

        state = dict(dep=None, piece=0, window=0)
        jobs, pending, hs = [], [], {}
        tie = make_tie(jobs, 0.0)

        def next_block_ln():
            jobs.extend(pending)
            del pending[:]
            for _ in range(LN_PLAN[state['window']]):
                k, r = state['piece'] // 4, state['piece'] % 4
                pin = pltpu.bitcast(qka[16, pl.ds(0, 8), :], U32)
                dep = pin if state['dep'] is None else state['dep'] | pin
                state['dep'] = ln2_piece(hs, nxt, r * QB + 16 * k, dep)
                if r == 3:
                    pending.extend(functools.partial(lhs1_job, hs, nbase, k, t, c)
                                   for t in range(2) for c in range(7))
                state['piece'] += 1
            state['window'] += 1

        for n in range(2):
            def prod2(c, d):
                return _dot(jnp.concatenate(g[c, d], axis=1),
                            _bf(tie(rhs_load(w2, K2, N2, rhs2_loc, c, d, n), FFN_DENSITY)))

            def outer(c):
                next_block_ln()
                y = _strassen_value(prod2, c)
                qka[17, pl.ds(srow, 8), :] = y[0:8, 0:128]
                return y

            def finish(y, rh, ch):
                for ci in range(2):
                    nn = (2 * ch + ci) * 2 + n
                    cols = pl.ds(nn * 128, 128)
                    mcols = pl.ds((nn % 2) * 128, 128)
                    yy = y[:, ci * 128:(ci + 1) * 128] + rep(biasb[:, pl.ds(FF + nn * 128, 128)], HB)
                    xr = pl.ds(pl.multiple_of(i * HB, HB) + rh * (HB // 2), HB // 2)
                    ar = pl.ds(pl.multiple_of(i * FB, FB) + rh * HB, HB)
                    x2 = _bf(xs[xr, cols]).astype(F32) + rep(modb[nn // 2, :, mcols], HB) * ha[ar, cols]
                    qka[2 * nn + half, pl.ds(srow + rh * (HB // 2), HB // 2), :] = pack(
                        x2 + rep(modb[12 + nn // 2, :, mcols], HB) * yy, F32)
                    if rh == ch:
                        pltpu.make_async_copy(
                            qka.at[2 * nn + half, pl.ds(srow, HB), :],
                            out32.at[pl.ds(pl.multiple_of(i * HB, HB), HB), cols],
                            sem.at[SEM_OUT]).start()

            _strassen(outer, finish)
        assert not jobs and not pending and state['piece'] == 16
        return carry

    with jax.named_scope("p4_ffn"):
        lax.fori_loop(0, nb, ffn, 0)
    pltpu.make_async_copy(out32, out32, sem.at[SEM_OUT]).wait()


@jax.jit
def pallas_adaLN_cond__memory_aug_recurrent_mem_tr__dense_activation_gelu__prompt_kernel(
    A_x, A_mem0, A_Wq, A_Wk, A_Wv, A_Wo, A_seg_len, B_x, B_w1, B_b1, B_w2, B_b2, c, w_mod,
):
    assert A_x.shape == (1, S, D) and A_Wq.shape == (D, H, E) and A_mem0.shape == (1, M, D)
    any_spec = pl.BlockSpec(memory_space=pl.ANY)
    out = pl.pallas_call(
        _kernel,
        out_shape=jax.ShapeDtypeStruct((S, D), BF16),
        in_specs=[any_spec] * 12,
        out_specs=any_spec,
        scratch_shapes=[
            pltpu.VMEM((S // 2, D), U32),
            pltpu.VMEM((96, D // 2, E), U32),
            pltpu.VMEM((8, H * E // 2, 128), U32),
            pltpu.VMEM((D // 2, FF), U32),
            pltpu.VMEM((FF // 2, D), U32),
            pltpu.VMEM((H, RING, E), F32),
            pltpu.VMEM((H, RING, E), F32),
            pltpu.VMEM((H + 1, RING, E), F32),
            pltpu.VMEM((H, RING, E), F32),
            pltpu.VMEM((S, D), F32),
            pltpu.VMEM((S - PRE, D), F32),
            pltpu.VMEM((M, D), F32),
            pltpu.VMEM((NQ, 2, 8, KQ), F32),
            pltpu.VMEM((16, 8, 256), F32),
            pltpu.VMEM((8, D), U32),
            pltpu.VMEM((D // 2, 128), U32),
            pltpu.VMEM((2, 2, D // 2, 128), F32),
            pltpu.VMEM((8, FF + D), F32),
            pltpu.VMEM((80, 128), F32),
            pltpu.VMEM((8, 32, 128), F32),
            pltpu.VMEM((8, 128), U32),
            pltpu.SMEM((1,), jnp.int32),
            pltpu.VMEM((8, FF // 8, 128), U32),
            pltpu.VMEM((13 * 64, D), U32),
            pltpu.VMEM((128, 256), U32),
            pltpu.VMEM((128, 256), U32),
            pltpu.VMEM((128, 256), U32),
            pltpu.VMEM((128, 256), U32),
            pltpu.VMEM((128, 256), U32),
            pltpu.VMEM((128, 256), U32),
            pltpu.VMEM((M, D), BF16),
            pltpu.VMEM((FF,), BF16),
            pltpu.VMEM((D,), BF16),
            pltpu.VMEM((1, D), BF16),
            pltpu.SemaphoreType.DMA((NSEM,)),
        ],
        compiler_params=pltpu.CompilerParams(vmem_limit_bytes=127 * 1024 * 1024, disable_bounds_checks=True,
                                             disable_semaphore_checks=True),
    )(
        A_x.reshape(S, D), A_mem0.reshape(M, D),
        A_Wq.reshape(D // 2, 2, H, E), A_Wk.reshape(D // 2, 2, H, E), A_Wv.reshape(D // 2, 2, H, E),
        A_Wo.reshape(H * E, D), B_w1, B_b1, B_w2, B_b2, c, w_mod,
    )
    return out.reshape(1, S, D)
```

```python
import functools
import math

import jax
import jax.numpy as jnp
from jax import lax
import jax.experimental.pallas as pl
import jax.experimental.pallas.tpu as pltpu

F32 = jnp.float32
BF16 = jnp.bfloat16
U32 = jnp.uint32

S = 2048
D = 1024
H = 32
E = 128
M = 8
SEG = 32
NSEG = S // SEG
FF = 3584
NP = H // 2
TOK = 24
PRE = S - NSEG * TOK
RING = 576
OOFF = (-NSEG * TOK) % RING
LN_EPS = 1e-5
FB = 256
P3_WEIGHTS = (0.78, 1.0, 1.0, 1.0)
LN0_PLAN = (0, 0, 0, 0, 2, 2, 1, 1, 2, 2, 1, 1, 2, 2, 0, 0)
LN_PLAN = (1, 1, 1, 1, 1, 1, 1, 2, 2, 2, 2, 1, 0, 0)
FFN_DENSITY = 1.0 / 24
ATT_COL, ATT_N1, ATT_N2 = 6, 2, 5
TIE_R, TIE_R0, TIE_L = (5, 6), (0, 1, 2, 3, 4, 5, 6), (0, 5, 6)
UNROLL = 4

NQ = 4
KQ = D // NQ

FIRST_STARTS = [('m', 0), ('w', 0, 0, 4), ('w', 0, 4, 8), ('m', 1), ('w', 0, 8, 12), ('w', 1, 0, 8), ('m', 2),
                ('w', 1, 8, 12)]
P1A_BLOCKS = [
    ([], [('m', 0)]),
    ([], [('w', 0, 0, 4)]),
    ([], [('w', 0, 4, 8)]),
    ([('w', 2, 0, 8), ('m', 3), ('w', 2, 8, 12)], [('m', 1), ('w', 0, 8, 12)]),
    ([('w', 3, 0, 12)], [('w', 1, 0, 8)]),
    ([('g', 2), ('g', 3)], [('m', 2), ('w', 1, 8, 12)]),
    ([], [('w', 2, 0, 8)]),
    ([('g', 4), ('g', 5)], [('m', 3), ('w', 2, 8, 12)]),
    ([], [('w', 3, 0, 12)]),
]
W_ITEMS = [it for _, items in P1A_BLOCKS for it in items if it[0] == 'w']
IT_ROWS = TOK * UNROLL
X_CHUNKS = (PRE, PRE + IT_ROWS, PRE + 3 * IT_ROWS, S)
LN_SLOTS = ((0, 11), (1, 5))
MOD_SLOTS = ((0, 2), (0, 4), (0, 6), (1, 8), (1, 9), (1, 10), (1, 11), (2, 0))
NX0 = 4

SEM_C = 0
SEM_X0 = 1
SEM_MOD = SEM_X0 + NX0
SEM_WA = SEM_MOD + NQ + 2
SEM_WB = SEM_WA + 10
SEM_XC = SEM_WB + 6
SEM_WO = SEM_XC + 3
SEM_W1 = SEM_WO + 1
SEM_W2 = SEM_W1 + 1
SEM_OUT = SEM_W2 + 1
NSEM = SEM_OUT + 1


def _ln(x):
    m = jnp.mean(x, axis=-1, keepdims=True)
    xc = x - m
    v = jnp.mean(xc * xc, axis=-1, keepdims=True)
    return xc * lax.rsqrt(v + LN_EPS)


def _bf(w32):
    return pltpu.bitcast(w32, BF16)


def _dot(a, b):
    return jnp.dot(a, b, preferred_element_type=F32)


def _lhs_combos(a11, a12, a21, a22):
    return [a11 - a22, a21 - a22, a11, a22, a12 - a11, a21 - a11, a12 - a22]


def _rhs_combos(b11, b12, b21, b22):
    return [b11 - b22, b11, b12 + b22, b21 + b11, b22, b11 + b12, b21 + b22]


_LHS_TERMS = {0: ((0, 0), (1, 1), -1), 1: ((1, 0), (1, 1), -1), 2: ((0, 0), None, 0), 3: ((1, 1), None, 0),
              4: ((0, 1), (0, 0), -1), 5: ((1, 0), (0, 0), -1), 6: ((0, 1), (1, 1), -1)}
_RHS_TERMS = {0: ((0, 0), (1, 1), -1), 1: ((0, 0), None, 0), 2: ((0, 1), (1, 1), 1), 3: ((1, 0), (0, 0), 1),
              4: ((1, 1), None, 0), 5: ((0, 0), (0, 1), 1), 6: ((1, 0), (1, 1), 1)}
_SWAP = {c: int(c in (2, 4, 5, 6)) for c in range(7)}


def _combo(terms, c, blk):
    p, q, sign = terms[c]
    if q is None:
        return blk(*p)
    return blk(*p) + blk(*q) if sign > 0 else blk(*p) - blk(*q)


def _rhs_operand(c, blk):
    p, q, sign = _RHS_TERMS[c]
    a = _bf(blk(*p))
    if q is None:
        return a
    a = a.astype(F32)
    b = _bf(blk(*q)).astype(F32)
    return (a + b if sign > 0 else a - b).astype(BF16)


def _strassen(prod, finish, side=lambda: None):
    side()
    m1 = prod(1)
    m3 = prod(3)
    finish(m1 + m3, 1, 0)
    side()
    m2 = prod(2)
    m4 = prod(4)
    finish(m2 + m4, 0, 1)
    side()
    m0 = prod(0)
    m5 = prod(5)
    finish((m2 - m1) + m0 + m5, 1, 1)
    side()
    m6 = prod(6)
    finish((m3 - m4) + m0 + m6, 0, 0)


def _strassen_value(prod2, c):
    r = {}
    _strassen(functools.partial(prod2, c), lambda y, rh, ch: r.__setitem__((rh, ch ^ _SWAP[c]), y))
    return jnp.concatenate([jnp.concatenate([r[0, 0], r[0, 1]], axis=1),
                            jnp.concatenate([r[1, 0], r[1, 1]], axis=1)], axis=0)


_ORDER = (1, 3, 2, 4, 0, 5, 6)

_PAIRS = [(c, d) for c in range(7) for d in range(7) if not (c in (1, 4) and d in (1, 4))]


def _plain_block(c, d):
    return 2 * (c // 4) + d // 4, 2 * (c // 4) + ((d // 4) ^ _SWAP[c])


def _kernel(x_hbm, mem0_hbm, wq_hbm, wk_hbm, wv_hbm, wo_hbm, w1_hbm, b1_hbm, w2_hbm, b2_hbm,
            c_hbm, wmod_hbm, out_hbm,
            xs, wqkv, wo, w1, w2, qka, qkb, vring, oring, ha, hn, memb, moda, modb, scb, colb, slab, biasb,
            fillb, accb, zerob, zero_s, wx, hb2, pk0, pk1, pk2, pk3, mem0_ref, b1_ref, b2_ref, c_ref, sem):
    qkv_hbm = [r.bitcast(U32) for r in (wq_hbm, wk_hbm, wv_hbm)]
    x32 = x_hbm.bitcast(U32)
    wo32 = wo_hbm.bitcast(U32)
    wmod32 = wmod_hbm.bitcast(F32)

    def wma(qq, k):
        return pl.ds(512 * (qq // 2), 512), pl.ds(512 * (qq % 2) + k * KQ, KQ)

    def hb_idx(c, q0, nq, row0=0, nrows=PRE // 4):
        return pl.ds(1024 + 128 * (c // 2) + row0, nrows), pl.ds(512 * (c % 2) + 128 * q0, 128 * nq)

    def units_start(lo, hi, rows, sem_idx):
        for u in range(lo, hi):
            j, m = u // 3, u % 3
            for p in range(2):
                pltpu.make_async_copy(qkv_hbm[m].at[rows, p, j, :], wqkv.at[2 * u + p, rows, :],
                                      sem.at[sem_idx]).start()

    def units_wait(lo, n, rows, sem_idx):
        blk = wqkv.at[pl.ds(2 * lo, 2 * n), rows, :]
        pltpu.make_async_copy(blk, blk, sem.at[sem_idx]).wait()

    def item_start(item):
        if item[0] == 'm':
            qq = item[1]
            for k in range(2):
                pltpu.make_async_copy(wmod32.at[:, pl.ds(k * D + qq * KQ, KQ)], ha.at[wma(qq, k)],
                                      sem.at[SEM_MOD + qq]).start()
        elif item[0] == 'w':
            _, qq, lo, hi = item
            units_start(lo, hi, pl.ds(qq * (KQ // 2), KQ // 2), SEM_WA + W_ITEMS.index(item))
        else:
            whole_start(item[1])

    def item_wait(item):
        if item[0] == 'm':
            qq = item[1]
            blk = ha.at[pl.ds(512 * (qq // 2), 512), pl.ds(512 * (qq % 2), 512)]
            pltpu.make_async_copy(blk, blk, sem.at[SEM_MOD + qq]).wait()
        else:
            _, qq, lo, hi = item
            units_wait(lo, hi - lo, pl.ds(qq * (KQ // 2), KQ // 2), SEM_WA + W_ITEMS.index(item))

    def whole_start(i):
        if i == 2:
            xc_copy(0).start()
        units_start(6 * i, 6 * i + 6, pl.ds(0, D // 2), SEM_WB + i - 2)

    def slab_copies(it):
        return [pltpu.make_async_copy(
            wmod32.at[:, pl.ds(pl.multiple_of(2 * D + it * 256 + t * 128, 128), 128)],
            slab.at[it & 1, t], sem.at[SEM_MOD + NQ + (it & 1)]) for t in range(2)]

    def x0_copy(i):
        n = PRE // 2 // NX0
        rows = pl.ds(pl.multiple_of(i * n, n), n)
        return pltpu.make_async_copy(x32.at[rows], xs.at[rows], sem.at[SEM_X0 + i])

    def xc_copy(i):
        rows = pl.ds(X_CHUNKS[i] // 2, (X_CHUNKS[i + 1] - X_CHUNKS[i]) // 2)
        return pltpu.make_async_copy(x32.at[rows], xs.at[rows], sem.at[SEM_XC + i])

    def wo_copy(n):
        return pltpu.make_async_copy(wo32.at[:, pl.ds(n * 128, 128)], wo.at[n], sem.at[SEM_WO])

    w1_copy = pltpu.make_async_copy(w1_hbm.bitcast(U32), w1, sem.at[SEM_W1])
    w2_copy = pltpu.make_async_copy(w2_hbm.bitcast(U32), w2, sem.at[SEM_W2])
    small_copies = [pltpu.make_async_copy(a, b, sem.at[SEM_C])
                    for a, b in ((c_hbm, c_ref), (mem0_hbm, mem0_ref), (b1_hbm, b1_ref),
                                 (b2_hbm, b2_ref))]

    def deinterleave(u, row0, nrows):
        for k in range(nrows // 64):
            rows = pl.ds(row0 + k * 64, 64)
            a = wqkv[2 * u, rows, :]
            b = wqkv[2 * u + 1, rows, :]
            wqkv[2 * u, rows, :] = (a & jnp.uint32(0xFFFF)) | (b << 16)
            wqkv[2 * u + 1, rows, :] = (a >> 16) | (b & jnp.uint32(0xFFFF0000))

    def load_x16(row2, dep):
        xw = xs[pl.ds(row2, 8), :]
        if dep is not None:
            first = xw[:, 0:128] | (dep & zerob[...])
            xw = jnp.concatenate([first, xw[:, 128:]], axis=1)
        return _bf(xw).astype(F32)

    pks = [pk0, pk1, pk2, pk3]

    def pack(v, dtype=U32):
        rows = pl.ds(0, v.shape[0] // 2)
        pk = pks[0]
        pk[rows, pl.ds(0, 128)] = pltpu.bitcast(v.astype(BF16), U32)
        return pltpu.bitcast(pk[rows, pl.ds(0, 128)], dtype)

    def rep(v8, n):
        return jnp.concatenate([v8] * (n // 8), axis=0)

    def mrow(k, n):
        if k < 2:
            return rep(jnp.concatenate([moda[qq, k] for qq in range(NQ)], axis=1), n)
        return rep(jnp.concatenate([modb[4 * (k - 2) + q] for q in range(4)], axis=1), n)

    for cp in small_copies:
        cp.start()
    for i in range(NX0):
        x0_copy(i).start()
    for item in FIRST_STARTS:
        item_start(item)

    def start_rest():
        xc_copy(1).start()
        for n in range(8):
            wo_copy(n).start()
        for cp in slab_copies(0):
            cp.start()
        xc_copy(2).start()
        w1_copy.start()
        w2_copy.start()

    r = lax.broadcasted_iota(jnp.int32, (80, 128), 0)
    q = lax.broadcasted_iota(jnp.int32, (80, 128), 1)
    r_tok = r < 64
    q_tok = q < 64
    r_head = jnp.where(r_tok, r >> 5, (r - 64) >> 3)
    q_head = jnp.where(q_tok, q >> 5, (q - 64) >> 3)
    same = (r_head == q_head) & (q < 80)
    causal_ok = jnp.logical_not(r_tok & q_tok & ((q & 31) > (r & 31)))
    scale = E ** (-0.5)
    fillb[...] = jnp.where(same, jnp.where(causal_ok, 0.0, -1e9 / scale), -jnp.inf).astype(F32)
    zerob[...] = jnp.zeros((8, 128), U32)
    zero_s[0] = 0

    for cp in small_copies:
        cp.wait()
    cf = c_ref[...].astype(F32)
    sc = (cf * jax.nn.sigmoid(cf)).astype(BF16)
    scb[...] = pltpu.bitcast(jnp.broadcast_to(sc, (16, D)), U32)
    scf = jnp.broadcast_to(sc.astype(F32), (128, D))
    for k in range(8):
        colb[pl.ds(k * 64, 64), :] = pltpu.bitcast(scf[:, k * 128:(k + 1) * 128].T.astype(BF16), U32)
    memb[...] = mem0_ref[...].astype(F32)
    biasb[:, pl.ds(0, FF)] = jnp.broadcast_to(b1_ref[...].astype(F32).reshape(1, FF), (8, FF))
    biasb[:, pl.ds(FF, D)] = jnp.broadcast_to(b2_ref[...].astype(F32).reshape(1, D), (8, D))

    def pre_norm(i, carry):
        x0_copy(i).wait()
        nr = PRE // NX0
        for z in range(nr // 16):
            xn = _ln(load_x16(pl.multiple_of(i * (nr // 2) + z * 8, 8), None))
            for n in range(8):
                oring[n, pl.ds(pl.multiple_of(i * nr + z * 16, 16), 16), :] = xn[:, n * 128:(n + 1) * 128]
        return carry

    with jax.named_scope("p0_ln"):
        lax.fori_loop(0, NX0, pre_norm, 0)

    def dst_slot(i, k, p):
        cls, m = k // 3, k % 3
        if m == 2:
            return vring, 4 * i + 2 * cls + p
        return (qka, qkb)[cls], 4 * i + 2 * m + p

    PH = PRE // 2
    assert KQ == 256

    def item_run(item):
        if item[0] == 'm':
            qq = item[1]
            sc16 = _bf(scb[...])
            ca1 = 1.0 + _dot(sc16, _bf(ha[wma(qq, 1)]))[0:8].astype(BF16).astype(F32)
            sa = _dot(sc16, _bf(ha[wma(qq, 0)]))[0:8].astype(BF16).astype(F32)
            moda[qq, 0] = sa
            moda[qq, 1] = ca1
            for z in range(PH // 32):
                def h_blk(rh, kh):
                    cols = slice(kh * 128, (kh + 1) * 128)
                    return (oring[2 * qq + kh, pl.ds(rh * PH + z * 32, 32), :] * rep(ca1[:, cols], 32)
                            + rep(sa[:, cols], 32))

                for c, v in enumerate(_lhs_combos(h_blk(0, 0), h_blk(0, 1), h_blk(1, 0), h_blk(1, 1))):
                    ha[hb_idx(c, qq, 1, z * 16, 16)] = pltpu.bitcast(v.astype(BF16), F32)
            return
        _, qq, lo, hi = item
        if lo == 0 and qq >= 2:
            a_jobs.extend(functools.partial(lhs0_job, k, qq - 2, c) for k in range(PQ // 16) for c in range(7))
        for u in range(lo, hi):
            deinterleave(u, qq * (KQ // 2), KQ // 2)
            i, k = u // 6, u % 6

            def prod(c):
                lhs = pltpu.bitcast(ha[hb_idx(c, qq, 1)], U32)
                if u >= 2:
                    lhs = tie_rows(lhs, a_jobs, (1 + 4 * ((7 * u + _ORDER.index(c)) % 4),))
                rhs = _rhs_operand(c, lambda a, b: wqkv[2 * u + b, pl.ds((2 * qq + a) * 64, 64), :])
                return _dot(_bf(lhs), rhs)

            def finish(y, rh, ch):
                ref, idx = dst_slot(i, k, ch)
                rows = pl.ds(RING - PRE + rh * PH, PH)
                if qq > 0:
                    y = y + ref[idx, rows, :]
                ref[idx, rows, :] = y

            _strassen(prod, finish)

    def tie_rows(w, jobs, groups):
        if not jobs:
            return w
        parts = [w[8 * g:8 * g + 8, 0:128] for g in range(w.shape[0] // 8)]
        for g in groups:
            if jobs:
                parts[g] = parts[g] | (jobs.pop(0)() & zerob[...])
        first = jnp.concatenate(parts, axis=0)
        return first if w.shape[1] == 128 else jnp.concatenate([first, w[:, 128:]], axis=1)

    PQ = PRE // 4
    a_jobs = []

    def lhs0_idx(c, d, k, nk, t, nt):
        e = 7 * c + d
        return pl.ds(64 * (e // 4) + 8 * k, 8 * nk), pl.ds(256 * (e % 4) + 128 * t, 128 * nt)

    def lhs0_job(k, t, c):
        def sub(ri, ki):
            def blk(ro, ko):
                n = 2 * ko + ki + 4 * t
                cols = pl.ds((n % 2) * 128, 128)
                return (oring[n, pl.ds((2 * ro + ri) * PQ + 16 * k, 16), :] * rep(moda[n // 2, 1, :, cols], 16)
                        + rep(moda[n // 2, 0, :, cols], 16))

            return _combo(_LHS_TERMS, c, blk)

        bits = None
        for d, v in enumerate(_lhs_combos(sub(0, 0), sub(0, 1), sub(1, 0), sub(1, 1))):
            hb2[lhs0_idx(c, d, k, 1, t, 1)] = pltpu.bitcast(v.astype(BF16), U32)
            if d in TIE_L:
                b = pltpu.bitcast(v[8 * (d % 2):8 * (d % 2) + 8], U32)
                bits = b if bits is None else bits | b
        return bits

    def ln1_piece(row2):
        h16 = _ln(load_x16(PRE // 2 + row2, None)) * mrow(1, 16) + mrow(0, 16)
        hn[pl.ds(pl.multiple_of(2 * row2, 16), 16), :] = h16
        return pltpu.bitcast(h16[8:16, D - 128:], U32)

    def phase1b(i, carry):
        @pl.when(i == 3)
        def _():
            whole_start(6)
            whole_start(7)
            start_rest()

        units_wait(6 * i, 6, pl.ds(0, D // 2), SEM_WB + i - 2)
        ln1_piece(pl.multiple_of((i - 2) * 8, 8))

        def raw(m, kq, nq, g):
            u = 6 * i + m + 3 * (nq // 2)
            return wqkv[2 * u + nq % 2, pl.ds((kq + 4 * (g // 8)) * 64 + 8 * (g % 8), 8), :]

        ops = {}

        def rhs0_job(m, c, g):
            def sub(ki, ni):
                return _combo(_RHS_TERMS, c,
                              lambda ko, no: _bf(raw(m, 2 * ko + ki, 2 * no + (ni ^ _SWAP[c]), g)).astype(F32))

            bits = None
            for d, v in enumerate(_rhs_combos(sub(0, 0), sub(0, 1), sub(1, 0), sub(1, 1))):
                if (c, d) in _PAIRS:
                    ops[m, c, d, g] = pack(v)
                    if d in TIE_R0:
                        bits = ops[m, c, d, g] if bits is None else bits | ops[m, c, d, g]
            return bits

        seq = [(m, c) for m in range(3) for c in _ORDER]
        jobs = []
        count = [0]
        deinterleave(6 * i, 0, D // 2)
        deinterleave(6 * i + 3, 0, D // 2)
        for g in range(16):
            rhs0_job(*seq[0], g)
        for m in range(3):
            if m < 2:
                deinterleave(6 * i + m + 1, 0, D // 2)
                deinterleave(6 * i + m + 4, 0, D // 2)

            def prod(c, d):
                if (c, d) in _PAIRS:
                    rhs = [ops[m, c, d, g] for g in range(16)]
                else:
                    rhs = [raw(m, *_plain_block(c, d), g) for g in range(16)]
                lhs = tie_rows(hb2[lhs0_idx(c, d, 0, 8, 0, 2)], jobs, ((0, 3, 6), (1, 4, 7))[count[0] % 2])
                count[0] += 1
                return _dot(_bf(lhs), _bf(jnp.concatenate(rhs, axis=0)))

            def outer(c):
                assert not jobs
                count[0] = 0
                nx = seq.index((m, c)) + 1
                if nx < len(seq):
                    jobs.extend(functools.partial(rhs0_job, *seq[nx], g) for g in range(16))
                return _strassen_value(prod, c)

            def finish(y, rh, ch):
                for ci in range(2):
                    ref, idx = dst_slot(i, m + 3 * ch, ci)
                    ref[idx, pl.ds(RING - PRE + rh * PH, PH), :] = y[:, ci * 128:(ci + 1) * 128]

            _strassen(outer, finish)
        return carry

    for bi, (starts, items) in enumerate(P1A_BLOCKS):
        for item in starts:
            item_start(item)
        with jax.named_scope("p1a_wait%d" % bi):
            for item in items:
                item_wait(item)
        for item in items:
            item_run(item)
    assert not a_jobs
    xc_copy(0).wait()
    with jax.named_scope("p1b"):
        lax.fori_loop(2, 8, phase1b, 0)
    pks.pop(0)
    xc_copy(1).wait()
    for n in range(8):
        wo_copy(n).wait()

    cexp = scale * math.log2(math.e)
    NG = NP // 2
    grp = [(4 * (g // 2) + (g % 2), 4 * (g // 2) + (g % 2) + 2) for g in range(NG)]
    early = [2 * j + u for g in range(NG - 3) for j in grp[g] for u in range(2)]
    late = [h for h in range(H) if h not in early]

    def step(it, k, side_jobs):
        s = it * UNROLL + k
        split = k > 0
        base = TOK * UNROLL * it
        w0 = pl.multiple_of(lax.rem(base, RING), 32) + TOK * k
        r0 = pl.multiple_of(lax.rem(SEG * s + (RING - PRE), RING), 32)
        ow = pl.multiple_of(lax.rem(SEG * s + OOFF, RING), 32)
        o0 = pl.multiple_of(lax.rem(base + OOFF, RING), 32) + TOK * k
        a0 = pl.multiple_of(base, 32) + TOK * k
        X = jnp.concatenate([hn[pl.ds(a0, TOK), :], memb[...]], axis=0).astype(BF16)
        ym = [None] * 96
        probs = [None] * NP
        om = [None] * H
        order = (4, 5, 0, 1, 2, 3)

        if split:
            for t in order:
                accb[t] = _dot(X[:, :D // 2], _bf(wqkv[t, pl.ds(0, D // 4), :]))

        def slot(j, t):
            if t >= 4:
                return vring, 2 * j + t - 4
            return (qka, qkb)[j % 2], 4 * (j // 2) + t

        def proj(j, t, job):
            c = 6 * j + t
            bits = None if job is None else job()
            if split and j == 0:
                y = accb[t] + _dot(X[:, D // 2:], _bf(wqkv[c, pl.ds(D // 4, D // 4), :]))
            else:
                y = _dot(X, _bf(wqkv[c]))
            ref, k = slot(j, t)
            if bits is not None:
                y0 = pltpu.bitcast(pltpu.bitcast(y[0:8], U32) | (bits & zerob[...]), F32)
                y = jnp.concatenate([y0, y[8:]], axis=0)
            ref[k, pl.ds(w0, TOK), :] = y[0:TOK]
            ym[c] = y[TOK:TOK + M]

        def gather(j, m, pad):
            c = 6 * j + 2 * m
            ref, k = slot(j, 2 * m)
            parts = [ref[k, pl.ds(r0, SEG), :], ref[k + 1, pl.ds(r0, SEG), :], ym[c], ym[c + 1]]
            if pad:
                parts.append(jnp.zeros((48, E), F32))
            return jnp.concatenate(parts, axis=0).astype(BF16)

        def scores(j):
            sc_ = lax.dot_general(gather(j, 0, False), gather(j, 1, True),
                                  (((1,), (1,)), ((), ())), preferred_element_type=F32)
            fill = fillb[...]
            sc_ = jnp.where(fill == 0.0, sc_, fill)
            mx = jnp.max(sc_, axis=-1, keepdims=True)
            p = jnp.exp2((sc_ - mx) * cexp)
            l = jnp.sum(p, axis=-1, keepdims=True)
            rl = pl.reciprocal(l, approx=True)
            rl = rl * (2.0 - l * rl)
            probs[j] = p * rl

        def park(j):
            vring[H, pl.ds(40 * (j % 8), 40), :] = pack(probs[j], F32)
            probs[j] = None

        def pv(j):
            if probs[j] is None:
                P = _bf(vring[H, pl.ds(40 * (j % 8), 40), :])
            else:
                P = probs[j].astype(BF16)
            o = _dot(P, gather(j, 2, True))
            oring[2 * j, pl.ds(ow, SEG), :] = o[0:32]
            oring[2 * j + 1, pl.ds(ow, SEG), :] = o[32:64]
            om[2 * j] = o[64:72]
            om[2 * j + 1] = o[72:80]

        def o_lhs(hs):
            return jnp.concatenate(
                [jnp.concatenate([oring[h, pl.ds(o0, TOK), :], om[h]], axis=0) for h in hs],
                axis=1).astype(BF16)

        def o_rhs(n, hs):
            return _bf(jnp.concatenate([wo[n, pl.ds(h * 64, 64), :] for h in hs], axis=0))

        for g in range(NG):
            cols = [(j, t) for j in grp[g] for t in order]
            if g == 2:
                cols = ([(j, t) for j in grp[g] for t in (4, 5)]
                        + [(j, t) for j in grp[g] for t in range(4)])
            for j in (grp[0] + grp[1] if g == 3 else grp[g - 2] if g >= 4 else ()):
                park(j)
            for ci, (j, t) in enumerate(cols):
                if g == 2 and ci == 4:
                    for jj in grp[0] + grp[1]:
                        scores(jj)
                if g >= 3 and ci == ATT_COL:
                    for jj in grp[g - 1]:
                        scores(jj)
                    for jj in grp[g - 3]:
                        pv(jj)
                proj(j, t, side_jobs.get((g, ci)))
        lo = o_lhs(early)
        for n in range(8):
            accb[n] = _dot(lo, o_rhs(n, early))
            if n == ATT_N1:
                for jj in grp[NG - 1]:
                    scores(jj)
                for jj in grp[NG - 3]:
                    pv(jj)
            if n == ATT_N2:
                for jj in grp[NG - 2] + grp[NG - 1]:
                    pv(jj)
        lo = o_lhs(late)
        for n in range(8):
            a = accb[n] + _dot(lo, o_rhs(n, late))
            ha[pl.ds(a0, TOK), pl.ds(n * 128, 128)] = a[0:TOK]
            memb[:, pl.ds(n * 128, 128)] = a[TOK:TOK + M]

    NIT = NSEG // UNROLL

    def lo16(w):
        return pltpu.bitcast(w << 16, F32)

    def hi16(w):
        return pltpu.bitcast(w & jnp.uint32(0xFFFF0000), F32)

    def steps(it, carry):
        @pl.when(it == 1)
        def _():
            xc_copy(2).wait()

        for cp in slab_copies(it):
            cp.wait()
        for cp in slab_copies((it + 1) & (NIT - 1)):
            cp.start()
        acc = [None, None]

        def mod_job(q):
            for kk in range(2 * q, 2 * q + 2):
                cw = colb[pl.ds(kk * 8, 8), :]
                for t in range(2):
                    w = pltpu.bitcast(slab[it & 1, t, pl.ds(kk * 8, 8), :], U32)
                    v = lo16(w) * lo16(cw) + hi16(w) * hi16(cw)
                    acc[t] = v if acc[t] is None else acc[t] + v
            if q < D // 32 - 1:
                return pltpu.bitcast(acc[0], U32) | pltpu.bitcast(acc[1], U32)
            y = jnp.sum(jnp.concatenate(acc, axis=1), axis=0, keepdims=True).astype(BF16).astype(F32)
            y = jnp.broadcast_to(y + jnp.where((it >> 2) == 2, 1.0, 0.0), (8, 256))
            modb[it] = y
            return pltpu.bitcast(y[:, 0:128], U32)

        nxt2 = pl.multiple_of(jnp.minimum(it + 1, NIT - 1) * (IT_ROWS // 2), 16)
        pieces = list(range(IT_ROWS // 16))
        for k in range(UNROLL):
            side_jobs = {pos: functools.partial(mod_job, 8 * k + q) for q, pos in enumerate(MOD_SLOTS)}
            for pos in LN_SLOTS[k % 2:]:
                side_jobs[pos] = functools.partial(ln1_piece, nxt2 + 8 * pieces.pop(0))
            step(it, k, side_jobs)
        assert not pieces
        return carry

    with jax.named_scope("p2_steps"):
        lax.fori_loop(0, NIT, steps, 0)
    for cp in slab_copies(0):
        cp.wait()
    w1_copy.wait()
    w2_copy.wait()

    nb = S // FB
    HB = FB // 2
    QB = FB // 4

    def ln2_piece(hs, blk, off, dep):
        x2 = (load_x16(pl.multiple_of(blk * HB, HB) + off // 2, dep)
              + mrow(2, 16) * ha[pl.ds(pl.multiple_of(blk * FB, FB) + off, 16), :])
        h = _ln(x2) * mrow(4, 16) + mrow(3, 16)
        hs[off] = h
        return pltpu.bitcast(h[8:16, D - 128:], U32)

    def lhs1_loc(base, c, d):
        e = 7 * c + d
        return base + 32 * (e // 4), 256 * (e % 4)

    def lhs1_job(hs, base, k, t, c):
        def sub(ri, ki):
            def blk(ro, ko):
                c0 = (2 * ko + ki) * 256 + t * 128
                return hs[(2 * ro + ri) * QB + 16 * k][:, c0:c0 + 128]

            return _combo(_LHS_TERMS, c, blk)

        bits = None
        for d, v in enumerate(_lhs_combos(sub(0, 0), sub(0, 1), sub(1, 0), sub(1, 1))):
            r0, c0 = lhs1_loc(base, c, d)
            hn[pl.ds(r0 + 8 * k, 8), pl.ds(c0 + t * 128, 128)] = pltpu.bitcast(
                v.astype(BF16), F32)
            if d in TIE_L:
                b = pltpu.bitcast(v[8 * (d % 2):8 * (d % 2) + 8], U32)
                bits = b if bits is None else bits | b
        return bits

    K1, N1, K2, N2 = D // 8, FF // 4, FF // 8, D // 4

    def rhs1_loc(c, d, n):
        e = _PAIRS.index((c, d)) * 7 + n
        return wqkv, e // 4, K1 * (e % 4)

    rhs2_slots = ([(wqkv, e, 0) for e in range(79, 96)] + [(qkb, e, 0) for e in range(H)]
                  + [(vring, e, 0) for e in range(H + 1)] + [(wx, e, 0) for e in range(8)])

    def rhs2_loc(c, d, n):
        return rhs2_slots[_PAIRS.index((c, d)) * 2 + n]

    def rhs_job(w, kq, nq, loc, n, r, cs):
        cache = {}

        def blk(ko, no, ki, ni):
            key = (2 * ko + ki, 2 * no + ni)
            if key not in cache:
                cache[key] = _bf(w[pl.ds(r + key[0] * kq, 8), pl.ds(n * 128 + key[1] * nq, 128)]).astype(F32)
            return cache[key]

        bits = None
        for c in cs:
            def sub(ki, ni):
                return _combo(_RHS_TERMS, c, lambda ko, no: blk(ko, no, ki, ni ^ _SWAP[c]))

            for d, v in enumerate(_rhs_combos(sub(0, 0), sub(0, 1), sub(1, 0), sub(1, 1))):
                if (c, d) in _PAIRS:
                    ref, idx, row = loc(c, d, n)
                    b = pack(v)
                    ref[idx, pl.ds(row + r, 8), :] = pltpu.bitcast(b, ref.dtype)
                    if d in TIE_R:
                        bits = b if bits is None else bits | b
        return bits

    def rhs_load(w, kq, nq, loc, c, d, n):
        if (c, d) not in _PAIRS:
            qk, qn = _plain_block(c, d)
            return w[pl.ds(qk * kq, kq), pl.ds(qn * nq + n * 128, 128)]
        ref, idx, row = loc(c, d, n)
        return pltpu.bitcast(ref[idx, pl.ds(row, kq), :], U32)

    def make_tie(jobs, credit):
        state = [credit]

        def tie(raw, density):
            if not jobs:
                return raw
            parts = []
            for r in range(0, raw.shape[0], 8):
                v = raw[r:r + 8]
                state[0] += density
                if jobs and state[0] >= 1.0:
                    state[0] -= 1.0
                    v = v | (jobs.pop(0)() & zerob[...])
                parts.append(v)
            return jnp.concatenate(parts, axis=0)

        return tie

    def bulk_o(zero):
        jobs = ([functools.partial(rhs_job, w1, K1, N1, rhs1_loc, n, r, [c])
                 for c in range(7) for n in range(7) for r in range(0, K1, 8)]
                + [functools.partial(rhs_job, w2, K2, N2, rhs2_loc, n, r, [c])
                   for c in range(7) for n in range(2) for r in range(0, K2, 8)])
        scale_d = (len(jobs) + 56 + 6) / (7 * 64 * sum(P3_WEIGHTS))
        state = dict(dep=None, piece=0, window=0, credit=-2.0)
        pending = []
        hs = {}

        def tie_lhs(tiles, density):
            tiles = [[t[8 * g:8 * g + 8] for g in range(16)] for t in tiles]
            for w in range(4):
                for g in range(16):
                    state['credit'] += density
                    for extra in range(2):
                        if jobs and state['credit'] >= 1.0:
                            state['credit'] -= 1.0
                            t = tiles[4 * w + (g + 2 * extra) % 4]
                            t[g] = t[g] | (jobs.pop(0)() & zerob[...])
            return _bf(jnp.concatenate([jnp.concatenate(t, axis=0) for t in tiles], axis=1))

        def ln2_block0():
            jobs.extend(pending)
            del pending[:]
            for _ in range(LN0_PLAN[state['window']]):
                k, r = state['piece'] // 4, state['piece'] % 4
                state['dep'] = ln2_piece(hs, zero, r * QB + 16 * k, state['dep'])
                if r == 3:
                    pending.extend(functools.partial(lhs1_job, hs, 0, k, t, c)
                                   for t in range(2) for c in range(7))
                state['piece'] += 1
            state['window'] += 1

        def a_blk(rh, kh):
            return jnp.concatenate([oring[h, pl.ds(rh * 256, 256), :]
                                    for h in range(16 * kh, 16 * kh + 16)], axis=1)

        lhs = [[pack(v[:, 128 * t:128 * t + 128]) for t in range(16)]
               for v in _lhs_combos(a_blk(0, 0), a_blk(0, 1), a_blk(1, 0), a_blk(1, 1))]
        for n in range(4):
            def prod(c):
                return _dot(tie_lhs(lhs[c], scale_d * P3_WEIGHTS[n]),
                            _rhs_operand(c, lambda a, b: wo[n + 4 * b, pl.ds(a * 1024, 1024), :]))

            def finish(y, rh, ch):
                ha[pl.ds(NSEG * TOK + rh * 256, 256), pl.ds((n + 4 * ch) * 128, 128)] = y

            _strassen(prod, finish, ln2_block0)
        assert not jobs and not pending and state['piece'] == 16

    pks.pop(0)
    with jax.named_scope("p3_bulk_o"):
        bulk_o(zero_s[0])

    pks.pop(0)
    out32 = out_hbm.bitcast(F32)
    qka[16, pl.ds(0, 8), :] = jnp.zeros((8, E), F32)

    def ffn(i, carry):
        base = pl.multiple_of((i & 1) * 512, 512)
        nbase = pl.multiple_of(((i + 1) & 1) * 512, 512)
        nxt = (i + 1) & (nb - 1)
        half = i >> 2
        srow = pl.multiple_of((i & 3) * HB, HB)

        g = {(c, d): [] for c in range(7) for d in range(7)}
        for n in range(7):
            act = {}

            def prod1(c, d):
                r0, c0 = lhs1_loc(base, c, d)
                return _dot(_bf(hn[pl.ds(r0, QB // 2), pl.ds(c0, 256)]),
                            _bf(rhs_load(w1, K1, N1, rhs1_loc, c, d, n)))

            def activate(y, rh, ch):
                b1 = jnp.concatenate([biasb[:, pl.ds((2 * ch + ci) * N1 + n * 128, 128)] for ci in range(2)],
                                     axis=1)
                act[rh, ch] = jax.nn.gelu(y + rep(b1, HB), approximate=True)

            _strassen(lambda c: _strassen_value(prod1, c), activate)
            for c in range(7):
                o = _combo(_LHS_TERMS, c, lambda a, b: act[a, b])
                for d, v in enumerate(_lhs_combos(o[:QB, :128], o[:QB, 128:], o[QB:, :128], o[QB:, 128:])):
                    g[c, d].append(v.astype(BF16))

        state = dict(dep=None, piece=0, window=0)
        jobs, pending, hs = [], [], {}
        tie = make_tie(jobs, 0.0)

        def next_block_ln():
            jobs.extend(pending)
            del pending[:]
            for _ in range(LN_PLAN[state['window']]):
                k, r = state['piece'] // 4, state['piece'] % 4
                pin = pltpu.bitcast(qka[16, pl.ds(0, 8), :], U32)
                dep = pin if state['dep'] is None else state['dep'] | pin
                state['dep'] = ln2_piece(hs, nxt, r * QB + 16 * k, dep)
                if r == 3:
                    pending.extend(functools.partial(lhs1_job, hs, nbase, k, t, c)
                                   for t in range(2) for c in range(7))
                state['piece'] += 1
            state['window'] += 1

        for n in range(2):
            def prod2(c, d):
                return _dot(jnp.concatenate(g[c, d], axis=1),
                            _bf(tie(rhs_load(w2, K2, N2, rhs2_loc, c, d, n), FFN_DENSITY)))

            def outer(c):
                next_block_ln()
                y = _strassen_value(prod2, c)
                qka[17, pl.ds(srow, 8), :] = y[0:8, 0:128]
                return y

            def finish(y, rh, ch):
                for ci in range(2):
                    nn = (2 * ch + ci) * 2 + n
                    cols = pl.ds(nn * 128, 128)
                    mcols = pl.ds((nn % 2) * 128, 128)
                    yy = y[:, ci * 128:(ci + 1) * 128] + rep(biasb[:, pl.ds(FF + nn * 128, 128)], HB)
                    xr = pl.ds(pl.multiple_of(i * HB, HB) + rh * (HB // 2), HB // 2)
                    ar = pl.ds(pl.multiple_of(i * FB, FB) + rh * HB, HB)
                    x2 = _bf(xs[xr, cols]).astype(F32) + rep(modb[nn // 2, :, mcols], HB) * ha[ar, cols]
                    qka[2 * nn + half, pl.ds(srow + rh * (HB // 2), HB // 2), :] = pack(
                        x2 + rep(modb[12 + nn // 2, :, mcols], HB) * yy, F32)
                    if rh == ch:
                        pltpu.make_async_copy(
                            qka.at[2 * nn + half, pl.ds(srow, HB), :],
                            out32.at[pl.ds(pl.multiple_of(i * HB, HB), HB), cols],
                            sem.at[SEM_OUT]).start()

            _strassen(outer, finish)
        assert not jobs and not pending and state['piece'] == 16
        return carry

    with jax.named_scope("p4_ffn"):
        lax.fori_loop(0, nb, ffn, 0)
    pltpu.make_async_copy(out32, out32, sem.at[SEM_OUT]).wait()


@jax.jit
def pallas_adaLN_cond__memory_aug_recurrent_mem_tr__dense_activation_gelu__prompt_kernel(
    A_x, A_mem0, A_Wq, A_Wk, A_Wv, A_Wo, A_seg_len, B_x, B_w1, B_b1, B_w2, B_b2, c, w_mod,
):
    assert A_x.shape == (1, S, D) and A_Wq.shape == (D, H, E) and A_mem0.shape == (1, M, D)
    any_spec = pl.BlockSpec(memory_space=pl.ANY)
    out = pl.pallas_call(
        _kernel,
        out_shape=jax.ShapeDtypeStruct((S, D), BF16),
        in_specs=[any_spec] * 12,
        out_specs=any_spec,
        scratch_shapes=[
            pltpu.VMEM((S // 2, D), U32),
            pltpu.VMEM((96, D // 2, E), U32),
            pltpu.VMEM((8, H * E // 2, 128), U32),
            pltpu.VMEM((D // 2, FF), U32),
            pltpu.VMEM((FF // 2, D), U32),
            pltpu.VMEM((H, RING, E), F32),
            pltpu.VMEM((H, RING, E), F32),
            pltpu.VMEM((H + 1, RING, E), F32),
            pltpu.VMEM((H, RING, E), F32),
            pltpu.VMEM((S, D), F32),
            pltpu.VMEM((S - PRE, D), F32),
            pltpu.VMEM((M, D), F32),
            pltpu.VMEM((NQ, 2, 8, KQ), F32),
            pltpu.VMEM((16, 8, 256), F32),
            pltpu.VMEM((8, D), U32),
            pltpu.VMEM((D // 2, 128), U32),
            pltpu.VMEM((2, 2, D // 2, 128), F32),
            pltpu.VMEM((8, FF + D), F32),
            pltpu.VMEM((80, 128), F32),
            pltpu.VMEM((8, 32, 128), F32),
            pltpu.VMEM((8, 128), U32),
            pltpu.SMEM((1,), jnp.int32),
            pltpu.VMEM((8, FF // 8, 128), U32),
            pltpu.VMEM((13 * 64, D), U32),
            pltpu.VMEM((128, 256), U32),
            pltpu.VMEM((128, 256), U32),
            pltpu.VMEM((128, 256), U32),
            pltpu.VMEM((128, 256), U32),
            pltpu.VMEM((M, D), BF16),
            pltpu.VMEM((FF,), BF16),
            pltpu.VMEM((D,), BF16),
            pltpu.VMEM((1, D), BF16),
            pltpu.SemaphoreType.DMA((NSEM,)),
        ],
        compiler_params=pltpu.CompilerParams(vmem_limit_bytes=127 * 1024 * 1024, disable_bounds_checks=True,
                                             disable_semaphore_checks=True),
    )(
        A_x.reshape(S, D), A_mem0.reshape(M, D),
        A_Wq.reshape(D // 2, 2, H, E), A_Wk.reshape(D // 2, 2, H, E), A_Wv.reshape(D // 2, 2, H, E),
        A_Wo.reshape(H * E, D), B_w1, B_b1, B_w2, B_b2, c, w_mod,
    )
    return out.reshape(1, S, D)
```

```python
import functools
import math

import jax
import jax.numpy as jnp
from jax import lax
import jax.experimental.pallas as pl
import jax.experimental.pallas.tpu as pltpu

F32 = jnp.float32
BF16 = jnp.bfloat16
U32 = jnp.uint32

S = 2048
D = 1024
H = 32
E = 128
M = 8
SEG = 32
NSEG = S // SEG
FF = 3584
NP = H // 2
TOK = 24
PRE = S - NSEG * TOK
RING = 576
OOFF = (-NSEG * TOK) % RING
LN_EPS = 1e-5
FB = 256
P3_WEIGHTS = (0.78, 1.0, 1.0, 1.0)
LN0_PLAN = (0, 0, 0, 0, 2, 2, 1, 1, 2, 2, 1, 1, 2, 2, 0, 0)
LN_PLAN = (1, 1, 1, 1, 1, 1, 1, 2, 2, 2, 2, 1, 0, 0)
FFN_DENSITY = 1.0 / 24
ATT_COL, ATT_N1, ATT_N2 = 6, 2, 5
TIE_R, TIE_R0, TIE_L = (5, 6), (0, 1, 2, 3, 4, 5, 6), (0, 5, 6)
JOB_GROUPS = ([1, 3], [4, 2], [0], [5], [6])
UNROLL = 4

NQ = 4
KQ = D // NQ

FIRST_STARTS = [('m', 0), ('w', 0, 0, 4), ('w', 0, 4, 8), ('m', 1), ('w', 0, 8, 12), ('w', 1, 0, 8), ('m', 2),
                ('w', 1, 8, 12)]
P1A_BLOCKS = [
    ([], [('m', 0)]),
    ([], [('w', 0, 0, 4)]),
    ([], [('w', 0, 4, 8)]),
    ([('w', 2, 0, 8), ('m', 3), ('w', 2, 8, 12)], [('m', 1), ('w', 0, 8, 12)]),
    ([('w', 3, 0, 12)], [('w', 1, 0, 8)]),
    ([('g', 2), ('g', 3)], [('m', 2), ('w', 1, 8, 12)]),
    ([], [('w', 2, 0, 8)]),
    ([('g', 4), ('g', 5)], [('m', 3), ('w', 2, 8, 12)]),
    ([], [('w', 3, 0, 12)]),
]
W_ITEMS = [it for _, items in P1A_BLOCKS for it in items if it[0] == 'w']
IT_ROWS = TOK * UNROLL
X_CHUNKS = (PRE, PRE + IT_ROWS, PRE + 3 * IT_ROWS, S)
LN_SLOTS = ((0, 11), (1, 5))
MOD_SLOTS = ((0, 2), (0, 4), (0, 6), (1, 8), (1, 9), (1, 10), (1, 11), (2, 0))
NX0 = 4

SEM_C = 0
SEM_X0 = 1
SEM_MOD = SEM_X0 + NX0
SEM_WA = SEM_MOD + NQ + 2
SEM_WB = SEM_WA + 10
SEM_XC = SEM_WB + 6
SEM_WO = SEM_XC + 3
SEM_W1 = SEM_WO + 1
SEM_W2 = SEM_W1 + 1
SEM_OUT = SEM_W2 + 1
NSEM = SEM_OUT + 1


def _ln(x):
    m = jnp.mean(x, axis=-1, keepdims=True)
    xc = x - m
    v = jnp.mean(xc * xc, axis=-1, keepdims=True)
    return xc * lax.rsqrt(v + LN_EPS)


def _bf(w32):
    return pltpu.bitcast(w32, BF16)


def _dot(a, b):
    return jnp.dot(a, b, preferred_element_type=F32)


def _lhs_combos(a11, a12, a21, a22):
    return [a11 - a22, a21 - a22, a11, a22, a12 - a11, a21 - a11, a12 - a22]


def _rhs_combos(b11, b12, b21, b22):
    return [b11 - b22, b11, b12 + b22, b21 + b11, b22, b11 + b12, b21 + b22]


_LHS_TERMS = {0: ((0, 0), (1, 1), -1), 1: ((1, 0), (1, 1), -1), 2: ((0, 0), None, 0), 3: ((1, 1), None, 0),
              4: ((0, 1), (0, 0), -1), 5: ((1, 0), (0, 0), -1), 6: ((0, 1), (1, 1), -1)}
_RHS_TERMS = {0: ((0, 0), (1, 1), -1), 1: ((0, 0), None, 0), 2: ((0, 1), (1, 1), 1), 3: ((1, 0), (0, 0), 1),
              4: ((1, 1), None, 0), 5: ((0, 0), (0, 1), 1), 6: ((1, 0), (1, 1), 1)}
_SWAP = {c: int(c in (2, 4, 5, 6)) for c in range(7)}


def _combo(terms, c, blk):
    p, q, sign = terms[c]
    if q is None:
        return blk(*p)
    return blk(*p) + blk(*q) if sign > 0 else blk(*p) - blk(*q)


def _rhs_operand(c, blk):
    p, q, sign = _RHS_TERMS[c]
    a = _bf(blk(*p))
    if q is None:
        return a
    a = a.astype(F32)
    b = _bf(blk(*q)).astype(F32)
    return (a + b if sign > 0 else a - b).astype(BF16)


def _strassen(prod, finish, side=lambda: None):
    side()
    m1 = prod(1)
    m3 = prod(3)
    finish(m1 + m3, 1, 0)
    side()
    m2 = prod(2)
    m4 = prod(4)
    finish(m2 + m4, 0, 1)
    side()
    m0 = prod(0)
    m5 = prod(5)
    finish((m2 - m1) + m0 + m5, 1, 1)
    side()
    m6 = prod(6)
    finish((m3 - m4) + m0 + m6, 0, 0)


def _strassen_value(prod2, c):
    r = {}
    _strassen(functools.partial(prod2, c), lambda y, rh, ch: r.__setitem__((rh, ch ^ _SWAP[c]), y))
    return jnp.concatenate([jnp.concatenate([r[0, 0], r[0, 1]], axis=1),
                            jnp.concatenate([r[1, 0], r[1, 1]], axis=1)], axis=0)


_ORDER = (1, 3, 2, 4, 0, 5, 6)

_PAIRS = [(c, d) for c in range(7) for d in range(7) if not (c in (1, 4) and d in (1, 4))]


def _plain_block(c, d):
    return 2 * (c // 4) + d // 4, 2 * (c // 4) + ((d // 4) ^ _SWAP[c])


def _kernel(x_hbm, mem0_hbm, wq_hbm, wk_hbm, wv_hbm, wo_hbm, w1_hbm, b1_hbm, w2_hbm, b2_hbm,
            c_hbm, wmod_hbm, out_hbm,
            xs, wqkv, wo, w1, w2, qka, qkb, vring, oring, ha, hn, memb, moda, modb, scb, colb, slab, biasb,
            fillb, accb, zerob, zero_s, wx, hb2, pk0, pk1, pk2, pk3, mem0_ref, b1_ref, b2_ref, c_ref, sem):
    qkv_hbm = [r.bitcast(U32) for r in (wq_hbm, wk_hbm, wv_hbm)]
    x32 = x_hbm.bitcast(U32)
    wo32 = wo_hbm.bitcast(U32)
    wmod32 = wmod_hbm.bitcast(F32)

    def wma(qq, k):
        return pl.ds(512 * (qq // 2), 512), pl.ds(512 * (qq % 2) + k * KQ, KQ)

    def hb_idx(c, q0, nq, row0=0, nrows=PRE // 4):
        return pl.ds(1024 + 128 * (c // 2) + row0, nrows), pl.ds(512 * (c % 2) + 128 * q0, 128 * nq)

    def units_start(lo, hi, rows, sem_idx):
        for u in range(lo, hi):
            j, m = u // 3, u % 3
            for p in range(2):
                pltpu.make_async_copy(qkv_hbm[m].at[rows, p, j, :], wqkv.at[2 * u + p, rows, :],
                                      sem.at[sem_idx]).start()

    def units_wait(lo, n, rows, sem_idx):
        blk = wqkv.at[pl.ds(2 * lo, 2 * n), rows, :]
        pltpu.make_async_copy(blk, blk, sem.at[sem_idx]).wait()

    def item_start(item):
        if item[0] == 'm':
            qq = item[1]
            for k in range(2):
                pltpu.make_async_copy(wmod32.at[:, pl.ds(k * D + qq * KQ, KQ)], ha.at[wma(qq, k)],
                                      sem.at[SEM_MOD + qq]).start()
        elif item[0] == 'w':
            _, qq, lo, hi = item
            units_start(lo, hi, pl.ds(qq * (KQ // 2), KQ // 2), SEM_WA + W_ITEMS.index(item))
        else:
            whole_start(item[1])

    def item_wait(item):
        if item[0] == 'm':
            qq = item[1]
            blk = ha.at[pl.ds(512 * (qq // 2), 512), pl.ds(512 * (qq % 2), 512)]
            pltpu.make_async_copy(blk, blk, sem.at[SEM_MOD + qq]).wait()
        else:
            _, qq, lo, hi = item
            units_wait(lo, hi - lo, pl.ds(qq * (KQ // 2), KQ // 2), SEM_WA + W_ITEMS.index(item))

    def whole_start(i):
        if i == 2:
            xc_copy(0).start()
        units_start(6 * i, 6 * i + 6, pl.ds(0, D // 2), SEM_WB + i - 2)

    def slab_copies(it):
        return [pltpu.make_async_copy(
            wmod32.at[:, pl.ds(pl.multiple_of(2 * D + it * 256 + t * 128, 128), 128)],
            slab.at[it & 1, t], sem.at[SEM_MOD + NQ + (it & 1)]) for t in range(2)]

    def x0_copy(i):
        n = PRE // 2 // NX0
        rows = pl.ds(pl.multiple_of(i * n, n), n)
        return pltpu.make_async_copy(x32.at[rows], xs.at[rows], sem.at[SEM_X0 + i])

    def xc_copy(i):
        rows = pl.ds(X_CHUNKS[i] // 2, (X_CHUNKS[i + 1] - X_CHUNKS[i]) // 2)
        return pltpu.make_async_copy(x32.at[rows], xs.at[rows], sem.at[SEM_XC + i])

    def wo_copy(n):
        return pltpu.make_async_copy(wo32.at[:, pl.ds(n * 128, 128)], wo.at[n], sem.at[SEM_WO])

    w1_copy = pltpu.make_async_copy(w1_hbm.bitcast(U32), w1, sem.at[SEM_W1])
    w2_copy = pltpu.make_async_copy(w2_hbm.bitcast(U32), w2, sem.at[SEM_W2])
    small_copies = [pltpu.make_async_copy(a, b, sem.at[SEM_C])
                    for a, b in ((c_hbm, c_ref), (mem0_hbm, mem0_ref), (b1_hbm, b1_ref),
                                 (b2_hbm, b2_ref))]

    def deinterleave(u, row0, nrows):
        for k in range(nrows // 64):
            rows = pl.ds(row0 + k * 64, 64)
            a = wqkv[2 * u, rows, :]
            b = wqkv[2 * u + 1, rows, :]
            wqkv[2 * u, rows, :] = (a & jnp.uint32(0xFFFF)) | (b << 16)
            wqkv[2 * u + 1, rows, :] = (a >> 16) | (b & jnp.uint32(0xFFFF0000))

    def load_x16(row2, dep):
        xw = xs[pl.ds(row2, 8), :]
        if dep is not None:
            first = xw[:, 0:128] | (dep & zerob[...])
            xw = jnp.concatenate([first, xw[:, 128:]], axis=1)
        return _bf(xw).astype(F32)

    pks = [pk0, pk1, pk2, pk3]

    def pack(v, dtype=U32):
        rows = pl.ds(0, v.shape[0] // 2)
        pk = pks[0]
        pk[rows, pl.ds(0, 128)] = pltpu.bitcast(v.astype(BF16), U32)
        return pltpu.bitcast(pk[rows, pl.ds(0, 128)], dtype)

    def rep(v8, n):
        return jnp.concatenate([v8] * (n // 8), axis=0)

    def mrow(k, n):
        if k < 2:
            return rep(jnp.concatenate([moda[qq, k] for qq in range(NQ)], axis=1), n)
        return rep(jnp.concatenate([modb[4 * (k - 2) + q] for q in range(4)], axis=1), n)

    for cp in small_copies:
        cp.start()
    for i in range(NX0):
        x0_copy(i).start()
    for item in FIRST_STARTS:
        item_start(item)

    def start_rest():
        xc_copy(1).start()
        for n in range(8):
            wo_copy(n).start()
        for cp in slab_copies(0):
            cp.start()
        xc_copy(2).start()
        w1_copy.start()
        w2_copy.start()

    r = lax.broadcasted_iota(jnp.int32, (80, 128), 0)
    q = lax.broadcasted_iota(jnp.int32, (80, 128), 1)
    r_tok = r < 64
    q_tok = q < 64
    r_head = jnp.where(r_tok, r >> 5, (r - 64) >> 3)
    q_head = jnp.where(q_tok, q >> 5, (q - 64) >> 3)
    same = (r_head == q_head) & (q < 80)
    causal_ok = jnp.logical_not(r_tok & q_tok & ((q & 31) > (r & 31)))
    scale = E ** (-0.5)
    fillb[...] = jnp.where(same, jnp.where(causal_ok, 0.0, -1e9 / scale), -jnp.inf).astype(F32)
    zerob[...] = jnp.zeros((8, 128), U32)
    zero_s[0] = 0

    for cp in small_copies:
        cp.wait()
    cf = c_ref[...].astype(F32)
    sc = (cf * jax.nn.sigmoid(cf)).astype(BF16)
    scb[...] = pltpu.bitcast(jnp.broadcast_to(sc, (16, D)), U32)
    scf = jnp.broadcast_to(sc.astype(F32), (128, D))
    for k in range(8):
        colb[pl.ds(k * 64, 64), :] = pltpu.bitcast(scf[:, k * 128:(k + 1) * 128].T.astype(BF16), U32)
    memb[...] = mem0_ref[...].astype(F32)
    biasb[:, pl.ds(0, FF)] = jnp.broadcast_to(b1_ref[...].astype(F32).reshape(1, FF), (8, FF))
    biasb[:, pl.ds(FF, D)] = jnp.broadcast_to(b2_ref[...].astype(F32).reshape(1, D), (8, D))

    def pre_norm(i, carry):
        x0_copy(i).wait()
        nr = PRE // NX0
        for z in range(nr // 16):
            xn = _ln(load_x16(pl.multiple_of(i * (nr // 2) + z * 8, 8), None))
            for n in range(8):
                oring[n, pl.ds(pl.multiple_of(i * nr + z * 16, 16), 16), :] = xn[:, n * 128:(n + 1) * 128]
        return carry

    with jax.named_scope("p0_ln"):
        lax.fori_loop(0, NX0, pre_norm, 0)

    def dst_slot(i, k, p):
        cls, m = k // 3, k % 3
        if m == 2:
            return vring, 4 * i + 2 * cls + p
        return (qka, qkb)[cls], 4 * i + 2 * m + p

    PH = PRE // 2
    assert KQ == 256

    def item_run(item):
        if item[0] == 'm':
            qq = item[1]
            sc16 = _bf(scb[...])
            ca1 = 1.0 + _dot(sc16, _bf(ha[wma(qq, 1)]))[0:8].astype(BF16).astype(F32)
            sa = _dot(sc16, _bf(ha[wma(qq, 0)]))[0:8].astype(BF16).astype(F32)
            moda[qq, 0] = sa
            moda[qq, 1] = ca1
            for z in range(PH // 32):
                def h_blk(rh, kh):
                    cols = slice(kh * 128, (kh + 1) * 128)
                    return (oring[2 * qq + kh, pl.ds(rh * PH + z * 32, 32), :] * rep(ca1[:, cols], 32)
                            + rep(sa[:, cols], 32))

                for c, v in enumerate(_lhs_combos(h_blk(0, 0), h_blk(0, 1), h_blk(1, 0), h_blk(1, 1))):
                    ha[hb_idx(c, qq, 1, z * 16, 16)] = pltpu.bitcast(v.astype(BF16), F32)
            return
        _, qq, lo, hi = item
        if lo == 0 and qq >= 2:
            a_jobs.extend(functools.partial(lhs0_job, k, qq - 2, c) for k in range(PQ // 16) for c in range(7))
        for u in range(lo, hi):
            deinterleave(u, qq * (KQ // 2), KQ // 2)
            i, k = u // 6, u % 6

            def prod(c):
                lhs = pltpu.bitcast(ha[hb_idx(c, qq, 1)], U32)
                if u >= 2:
                    lhs = tie_rows(lhs, a_jobs, (1 + 4 * ((7 * u + _ORDER.index(c)) % 4),))
                rhs = _rhs_operand(c, lambda a, b: wqkv[2 * u + b, pl.ds((2 * qq + a) * 64, 64), :])
                return _dot(_bf(lhs), rhs)

            def finish(y, rh, ch):
                ref, idx = dst_slot(i, k, ch)
                rows = pl.ds(RING - PRE + rh * PH, PH)
                if qq > 0:
                    y = y + ref[idx, rows, :]
                ref[idx, rows, :] = y

            _strassen(prod, finish)

    def tie_rows(w, jobs, groups):
        if not jobs:
            return w
        parts = [w[8 * g:8 * g + 8, 0:128] for g in range(w.shape[0] // 8)]
        for g in groups:
            if jobs:
                parts[g] = parts[g] | (jobs.pop(0)() & zerob[...])
        first = jnp.concatenate(parts, axis=0)
        return first if w.shape[1] == 128 else jnp.concatenate([first, w[:, 128:]], axis=1)

    PQ = PRE // 4
    a_jobs = []

    def lhs0_idx(c, d, k, nk, t, nt):
        e = 7 * c + d
        return pl.ds(64 * (e // 4) + 8 * k, 8 * nk), pl.ds(256 * (e % 4) + 128 * t, 128 * nt)

    def lhs0_job(k, t, c):
        def sub(ri, ki):
            def blk(ro, ko):
                n = 2 * ko + ki + 4 * t
                cols = pl.ds((n % 2) * 128, 128)
                return (oring[n, pl.ds((2 * ro + ri) * PQ + 16 * k, 16), :] * rep(moda[n // 2, 1, :, cols], 16)
                        + rep(moda[n // 2, 0, :, cols], 16))

            return _combo(_LHS_TERMS, c, blk)

        bits = None
        for d, v in enumerate(_lhs_combos(sub(0, 0), sub(0, 1), sub(1, 0), sub(1, 1))):
            hb2[lhs0_idx(c, d, k, 1, t, 1)] = pltpu.bitcast(v.astype(BF16), U32)
            if d in TIE_L:
                b = pltpu.bitcast(v[8 * (d % 2):8 * (d % 2) + 8], U32)
                bits = b if bits is None else bits | b
        return bits

    def ln1_piece(row2):
        h16 = _ln(load_x16(PRE // 2 + row2, None)) * mrow(1, 16) + mrow(0, 16)
        hn[pl.ds(pl.multiple_of(2 * row2, 16), 16), :] = h16
        return pltpu.bitcast(h16[8:16, D - 128:], U32)

    def phase1b(i, carry):
        @pl.when(i == 3)
        def _():
            whole_start(6)
            whole_start(7)
            start_rest()

        units_wait(6 * i, 6, pl.ds(0, D // 2), SEM_WB + i - 2)
        ln1_piece(pl.multiple_of((i - 2) * 8, 8))

        def raw(m, kq, nq, g):
            u = 6 * i + m + 3 * (nq // 2)
            return wqkv[2 * u + nq % 2, pl.ds((kq + 4 * (g // 8)) * 64 + 8 * (g % 8), 8), :]

        ops = {}

        def rhs0_job(m, c, g):
            def sub(ki, ni):
                return _combo(_RHS_TERMS, c,
                              lambda ko, no: _bf(raw(m, 2 * ko + ki, 2 * no + (ni ^ _SWAP[c]), g)).astype(F32))

            bits = None
            for d, v in enumerate(_rhs_combos(sub(0, 0), sub(0, 1), sub(1, 0), sub(1, 1))):
                if (c, d) in _PAIRS:
                    ops[m, c, d, g] = pack(v)
                    if d in TIE_R0:
                        bits = ops[m, c, d, g] if bits is None else bits | ops[m, c, d, g]
            return bits

        seq = [(m, c) for m in range(3) for c in _ORDER]
        jobs = []
        count = [0]
        deinterleave(6 * i, 0, D // 2)
        deinterleave(6 * i + 3, 0, D // 2)
        for g in range(16):
            rhs0_job(*seq[0], g)
        for m in range(3):
            if m < 2:
                deinterleave(6 * i + m + 1, 0, D // 2)
                deinterleave(6 * i + m + 4, 0, D // 2)

            def prod(c, d):
                if (c, d) in _PAIRS:
                    rhs = [ops[m, c, d, g] for g in range(16)]
                else:
                    rhs = [raw(m, *_plain_block(c, d), g) for g in range(16)]
                lhs = tie_rows(hb2[lhs0_idx(c, d, 0, 8, 0, 2)], jobs, ((0, 3, 6), (1, 4, 7))[count[0] % 2])
                count[0] += 1
                return _dot(_bf(lhs), _bf(jnp.concatenate(rhs, axis=0)))

            def outer(c):
                assert not jobs
                count[0] = 0
                nx = seq.index((m, c)) + 1
                if nx < len(seq):
                    jobs.extend(functools.partial(rhs0_job, *seq[nx], g) for g in range(16))
                return _strassen_value(prod, c)

            def finish(y, rh, ch):
                for ci in range(2):
                    ref, idx = dst_slot(i, m + 3 * ch, ci)
                    ref[idx, pl.ds(RING - PRE + rh * PH, PH), :] = y[:, ci * 128:(ci + 1) * 128]

            _strassen(outer, finish)
        return carry

    for bi, (starts, items) in enumerate(P1A_BLOCKS):
        for item in starts:
            item_start(item)
        with jax.named_scope("p1a_wait%d" % bi):
            for item in items:
                item_wait(item)
        for item in items:
            item_run(item)
    assert not a_jobs
    xc_copy(0).wait()
    with jax.named_scope("p1b"):
        lax.fori_loop(2, 8, phase1b, 0)
    pks.pop(0)
    xc_copy(1).wait()
    for n in range(8):
        wo_copy(n).wait()

    cexp = scale * math.log2(math.e)
    NG = NP // 2
    grp = [(4 * (g // 2) + (g % 2), 4 * (g // 2) + (g % 2) + 2) for g in range(NG)]
    early = [2 * j + u for g in range(NG - 3) for j in grp[g] for u in range(2)]
    late = [h for h in range(H) if h not in early]

    def step(it, k, side_jobs):
        s = it * UNROLL + k
        split = k > 0
        base = TOK * UNROLL * it
        w0 = pl.multiple_of(lax.rem(base, RING), 32) + TOK * k
        r0 = pl.multiple_of(lax.rem(SEG * s + (RING - PRE), RING), 32)
        ow = pl.multiple_of(lax.rem(SEG * s + OOFF, RING), 32)
        o0 = pl.multiple_of(lax.rem(base + OOFF, RING), 32) + TOK * k
        a0 = pl.multiple_of(base, 32) + TOK * k
        X = jnp.concatenate([hn[pl.ds(a0, TOK), :], memb[...]], axis=0).astype(BF16)
        ym = [None] * 96
        probs = [None] * NP
        om = [None] * H
        order = (4, 5, 0, 1, 2, 3)

        if split:
            for t in order:
                accb[t] = _dot(X[:, :D // 2], _bf(wqkv[t, pl.ds(0, D // 4), :]))

        def slot(j, t):
            if t >= 4:
                return vring, 2 * j + t - 4
            return (qka, qkb)[j % 2], 4 * (j // 2) + t

        def proj(j, t, job):
            c = 6 * j + t
            bits = None if job is None else job()
            if split and j == 0:
                y = accb[t] + _dot(X[:, D // 2:], _bf(wqkv[c, pl.ds(D // 4, D // 4), :]))
            else:
                y = _dot(X, _bf(wqkv[c]))
            ref, k = slot(j, t)
            if bits is not None:
                y0 = pltpu.bitcast(pltpu.bitcast(y[0:8], U32) | (bits & zerob[...]), F32)
                y = jnp.concatenate([y0, y[8:]], axis=0)
            ref[k, pl.ds(w0, TOK), :] = y[0:TOK]
            ym[c] = y[TOK:TOK + M]

        def gather(j, m, pad):
            c = 6 * j + 2 * m
            ref, k = slot(j, 2 * m)
            parts = [ref[k, pl.ds(r0, SEG), :], ref[k + 1, pl.ds(r0, SEG), :], ym[c], ym[c + 1]]
            if pad:
                parts.append(jnp.zeros((48, E), F32))
            return jnp.concatenate(parts, axis=0).astype(BF16)

        def scores(j):
            sc_ = lax.dot_general(gather(j, 0, False), gather(j, 1, True),
                                  (((1,), (1,)), ((), ())), preferred_element_type=F32)
            fill = fillb[...]
            sc_ = jnp.where(fill == 0.0, sc_, fill)
            mx = jnp.max(sc_, axis=-1, keepdims=True)
            p = jnp.exp2((sc_ - mx) * cexp)
            l = jnp.sum(p, axis=-1, keepdims=True)
            rl = pl.reciprocal(l, approx=True)
            rl = rl * (2.0 - l * rl)
            probs[j] = p * rl

        def park(j):
            vring[H, pl.ds(40 * (j % 8), 40), :] = pack(probs[j], F32)
            probs[j] = None

        def pv(j):
            if probs[j] is None:
                P = _bf(vring[H, pl.ds(40 * (j % 8), 40), :])
            else:
                P = probs[j].astype(BF16)
            o = _dot(P, gather(j, 2, True))
            oring[2 * j, pl.ds(ow, SEG), :] = o[0:32]
            oring[2 * j + 1, pl.ds(ow, SEG), :] = o[32:64]
            om[2 * j] = o[64:72]
            om[2 * j + 1] = o[72:80]

        def o_lhs(hs):
            return jnp.concatenate(
                [jnp.concatenate([oring[h, pl.ds(o0, TOK), :], om[h]], axis=0) for h in hs],
                axis=1).astype(BF16)

        def o_rhs(n, hs):
            return _bf(jnp.concatenate([wo[n, pl.ds(h * 64, 64), :] for h in hs], axis=0))

        for g in range(NG):
            cols = [(j, t) for j in grp[g] for t in order]
            if g == 2:
                cols = ([(j, t) for j in grp[g] for t in (4, 5)]
                        + [(j, t) for j in grp[g] for t in range(4)])
            for j in (grp[0] + grp[1] if g == 3 else grp[g - 2] if g >= 4 else ()):
                park(j)
            for ci, (j, t) in enumerate(cols):
                if g == 2 and ci == 4:
                    for jj in grp[0] + grp[1]:
                        scores(jj)
                if g >= 3 and ci == ATT_COL:
                    for jj in grp[g - 1]:
                        scores(jj)
                    for jj in grp[g - 3]:
                        pv(jj)
                proj(j, t, side_jobs.get((g, ci)))
        lo = o_lhs(early)
        for n in range(8):
            accb[n] = _dot(lo, o_rhs(n, early))
            if n == ATT_N1:
                for jj in grp[NG - 1]:
                    scores(jj)
                for jj in grp[NG - 3]:
                    pv(jj)
            if n == ATT_N2:
                for jj in grp[NG - 2] + grp[NG - 1]:
                    pv(jj)
        lo = o_lhs(late)
        for n in range(8):
            a = accb[n] + _dot(lo, o_rhs(n, late))
            ha[pl.ds(a0, TOK), pl.ds(n * 128, 128)] = a[0:TOK]
            memb[:, pl.ds(n * 128, 128)] = a[TOK:TOK + M]

    NIT = NSEG // UNROLL

    def lo16(w):
        return pltpu.bitcast(w << 16, F32)

    def hi16(w):
        return pltpu.bitcast(w & jnp.uint32(0xFFFF0000), F32)

    def steps(it, carry):
        @pl.when(it == 1)
        def _():
            xc_copy(2).wait()

        for cp in slab_copies(it):
            cp.wait()
        for cp in slab_copies((it + 1) & (NIT - 1)):
            cp.start()
        acc = [None, None]

        def mod_job(q):
            for kk in range(2 * q, 2 * q + 2):
                cw = colb[pl.ds(kk * 8, 8), :]
                for t in range(2):
                    w = pltpu.bitcast(slab[it & 1, t, pl.ds(kk * 8, 8), :], U32)
                    v = lo16(w) * lo16(cw) + hi16(w) * hi16(cw)
                    acc[t] = v if acc[t] is None else acc[t] + v
            if q < D // 32 - 1:
                return pltpu.bitcast(acc[0], U32) | pltpu.bitcast(acc[1], U32)
            y = jnp.sum(jnp.concatenate(acc, axis=1), axis=0, keepdims=True).astype(BF16).astype(F32)
            y = jnp.broadcast_to(y + jnp.where((it >> 2) == 2, 1.0, 0.0), (8, 256))
            modb[it] = y
            return pltpu.bitcast(y[:, 0:128], U32)

        nxt2 = pl.multiple_of(jnp.minimum(it + 1, NIT - 1) * (IT_ROWS // 2), 16)
        pieces = list(range(IT_ROWS // 16))
        for k in range(UNROLL):
            side_jobs = {pos: functools.partial(mod_job, 8 * k + q) for q, pos in enumerate(MOD_SLOTS)}
            for pos in LN_SLOTS[k % 2:]:
                side_jobs[pos] = functools.partial(ln1_piece, nxt2 + 8 * pieces.pop(0))
            step(it, k, side_jobs)
        assert not pieces
        return carry

    with jax.named_scope("p2_steps"):
        lax.fori_loop(0, NIT, steps, 0)
    for cp in slab_copies(0):
        cp.wait()
    w1_copy.wait()
    w2_copy.wait()

    nb = S // FB
    HB = FB // 2
    QB = FB // 4

    def ln2_piece(hs, blk, off, dep):
        x2 = (load_x16(pl.multiple_of(blk * HB, HB) + off // 2, dep)
              + mrow(2, 16) * ha[pl.ds(pl.multiple_of(blk * FB, FB) + off, 16), :])
        h = _ln(x2) * mrow(4, 16) + mrow(3, 16)
        hs[off] = h
        return pltpu.bitcast(h[8:16, D - 128:], U32)

    def lhs1_loc(base, c, d):
        e = 7 * c + d
        return base + 32 * (e // 4), 256 * (e % 4)

    def lhs1_job(hs, base, k, t, c):
        def sub(ri, ki):
            def blk(ro, ko):
                c0 = (2 * ko + ki) * 256 + t * 128
                return hs[(2 * ro + ri) * QB + 16 * k][:, c0:c0 + 128]

            return _combo(_LHS_TERMS, c, blk)

        bits = None
        for d, v in enumerate(_lhs_combos(sub(0, 0), sub(0, 1), sub(1, 0), sub(1, 1))):
            r0, c0 = lhs1_loc(base, c, d)
            hn[pl.ds(r0 + 8 * k, 8), pl.ds(c0 + t * 128, 128)] = pltpu.bitcast(
                v.astype(BF16), F32)
            if d in TIE_L:
                b = pltpu.bitcast(v[8 * (d % 2):8 * (d % 2) + 8], U32)
                bits = b if bits is None else bits | b
        return bits

    K1, N1, K2, N2 = D // 8, FF // 4, FF // 8, D // 4

    def rhs1_loc(c, d, n):
        e = _PAIRS.index((c, d)) * 7 + n
        return wqkv, e // 4, K1 * (e % 4)

    rhs2_slots = ([(wqkv, e, 0) for e in range(79, 96)] + [(qkb, e, 0) for e in range(H)]
                  + [(vring, e, 0) for e in range(H + 1)] + [(wx, e, 0) for e in range(8)])

    def rhs2_loc(c, d, n):
        return rhs2_slots[_PAIRS.index((c, d)) * 2 + n]

    def rhs_job(w, kq, nq, loc, n, r, cs):
        cache = {}

        def blk(ko, no, ki, ni):
            key = (2 * ko + ki, 2 * no + ni)
            if key not in cache:
                cache[key] = _bf(w[pl.ds(r + key[0] * kq, 8), pl.ds(n * 128 + key[1] * nq, 128)]).astype(F32)
            return cache[key]

        bits = None
        for c in cs:
            def sub(ki, ni):
                return _combo(_RHS_TERMS, c, lambda ko, no: blk(ko, no, ki, ni ^ _SWAP[c]))

            for d, v in enumerate(_rhs_combos(sub(0, 0), sub(0, 1), sub(1, 0), sub(1, 1))):
                if (c, d) in _PAIRS:
                    ref, idx, row = loc(c, d, n)
                    b = pack(v)
                    ref[idx, pl.ds(row + r, 8), :] = pltpu.bitcast(b, ref.dtype)
                    if d in TIE_R:
                        bits = b if bits is None else bits | b
        return bits

    def rhs_load(w, kq, nq, loc, c, d, n):
        if (c, d) not in _PAIRS:
            qk, qn = _plain_block(c, d)
            return w[pl.ds(qk * kq, kq), pl.ds(qn * nq + n * 128, 128)]
        ref, idx, row = loc(c, d, n)
        return pltpu.bitcast(ref[idx, pl.ds(row, kq), :], U32)

    def make_tie(jobs, credit):
        state = [credit]

        def tie(raw, density):
            if not jobs:
                return raw
            parts = []
            for r in range(0, raw.shape[0], 8):
                v = raw[r:r + 8]
                state[0] += density
                if jobs and state[0] >= 1.0:
                    state[0] -= 1.0
                    v = v | (jobs.pop(0)() & zerob[...])
                parts.append(v)
            return jnp.concatenate(parts, axis=0)

        return tie

    def bulk_o(zero):
        spots = ([(w1, K1, N1, rhs1_loc, n, r) for n in range(7) for r in range(0, K1, 8)]
                 + [(w2, K2, N2, rhs2_loc, n, r) for n in range(2) for r in range(0, K2, 8)])
        ng = len(JOB_GROUPS)
        jobs = [functools.partial(rhs_job, *spots[(e + (len(spots) // ng) * gi) % len(spots)], cs)
                for e in range(len(spots)) for gi, cs in enumerate(JOB_GROUPS)]
        scale_d = (len(jobs) + 56 + 6) / (7 * 64 * sum(P3_WEIGHTS))
        state = dict(dep=None, piece=0, window=0, credit=-2.0)
        pending = []
        hs = {}

        def tie_lhs(tiles, density):
            tiles = [[t[8 * g:8 * g + 8] for g in range(16)] for t in tiles]
            for w in range(4):
                for g in range(16):
                    state['credit'] += density
                    for extra in range(2):
                        if jobs and state['credit'] >= 1.0:
                            state['credit'] -= 1.0
                            t = tiles[4 * w + (g + 2 * extra) % 4]
                            t[g] = t[g] | (jobs.pop(0)() & zerob[...])
            return _bf(jnp.concatenate([jnp.concatenate(t, axis=0) for t in tiles], axis=1))

        def ln2_block0():
            jobs.extend(pending)
            del pending[:]
            for _ in range(LN0_PLAN[state['window']]):
                k, r = state['piece'] // 4, state['piece'] % 4
                state['dep'] = ln2_piece(hs, zero, r * QB + 16 * k, state['dep'])
                if r == 3:
                    pending.extend(functools.partial(lhs1_job, hs, 0, k, t, c)
                                   for t in range(2) for c in range(7))
                state['piece'] += 1
            state['window'] += 1

        def a_blk(rh, kh):
            return jnp.concatenate([oring[h, pl.ds(rh * 256, 256), :]
                                    for h in range(16 * kh, 16 * kh + 16)], axis=1)

        lhs = [[pack(v[:, 128 * t:128 * t + 128]) for t in range(16)]
               for v in _lhs_combos(a_blk(0, 0), a_blk(0, 1), a_blk(1, 0), a_blk(1, 1))]
        for n in range(4):
            def prod(c):
                return _dot(tie_lhs(lhs[c], scale_d * P3_WEIGHTS[n]),
                            _rhs_operand(c, lambda a, b: wo[n + 4 * b, pl.ds(a * 1024, 1024), :]))

            def finish(y, rh, ch):
                ha[pl.ds(NSEG * TOK + rh * 256, 256), pl.ds((n + 4 * ch) * 128, 128)] = y

            _strassen(prod, finish, ln2_block0)
        assert not jobs and not pending and state['piece'] == 16

    pks.pop(0)
    with jax.named_scope("p3_bulk_o"):
        bulk_o(zero_s[0])

    pks.pop(0)
    out32 = out_hbm.bitcast(F32)
    qka[16, pl.ds(0, 8), :] = jnp.zeros((8, E), F32)

    def ffn(i, carry):
        base = pl.multiple_of((i & 1) * 512, 512)
        nbase = pl.multiple_of(((i + 1) & 1) * 512, 512)
        nxt = (i + 1) & (nb - 1)
        half = i >> 2
        srow = pl.multiple_of((i & 3) * HB, HB)

        g = {(c, d): [] for c in range(7) for d in range(7)}
        for n in range(7):
            act = {}

            def prod1(c, d):
                r0, c0 = lhs1_loc(base, c, d)
                return _dot(_bf(hn[pl.ds(r0, QB // 2), pl.ds(c0, 256)]),
                            _bf(rhs_load(w1, K1, N1, rhs1_loc, c, d, n)))

            def activate(y, rh, ch):
                b1 = jnp.concatenate([biasb[:, pl.ds((2 * ch + ci) * N1 + n * 128, 128)] for ci in range(2)],
                                     axis=1)
                act[rh, ch] = jax.nn.gelu(y + rep(b1, HB), approximate=True)

            _strassen(lambda c: _strassen_value(prod1, c), activate)
            for c in range(7):
                o = _combo(_LHS_TERMS, c, lambda a, b: act[a, b])
                for d, v in enumerate(_lhs_combos(o[:QB, :128], o[:QB, 128:], o[QB:, :128], o[QB:, 128:])):
                    g[c, d].append(v.astype(BF16))

        state = dict(dep=None, piece=0, window=0)
        jobs, pending, hs = [], [], {}
        tie = make_tie(jobs, 0.0)

        def next_block_ln():
            jobs.extend(pending)
            del pending[:]
            for _ in range(LN_PLAN[state['window']]):
                k, r = state['piece'] // 4, state['piece'] % 4
                pin = pltpu.bitcast(qka[16, pl.ds(0, 8), :], U32)
                dep = pin if state['dep'] is None else state['dep'] | pin
                state['dep'] = ln2_piece(hs, nxt, r * QB + 16 * k, dep)
                if r == 3:
                    pending.extend(functools.partial(lhs1_job, hs, nbase, k, t, c)
                                   for t in range(2) for c in range(7))
                state['piece'] += 1
            state['window'] += 1

        for n in range(2):
            def prod2(c, d):
                return _dot(jnp.concatenate(g[c, d], axis=1),
                            _bf(tie(rhs_load(w2, K2, N2, rhs2_loc, c, d, n), FFN_DENSITY)))

            def outer(c):
                next_block_ln()
                y = _strassen_value(prod2, c)
                qka[17, pl.ds(srow, 8), :] = y[0:8, 0:128]
                return y

            def finish(y, rh, ch):
                for ci in range(2):
                    nn = (2 * ch + ci) * 2 + n
                    cols = pl.ds(nn * 128, 128)
                    mcols = pl.ds((nn % 2) * 128, 128)
                    yy = y[:, ci * 128:(ci + 1) * 128] + rep(biasb[:, pl.ds(FF + nn * 128, 128)], HB)
                    xr = pl.ds(pl.multiple_of(i * HB, HB) + rh * (HB // 2), HB // 2)
                    ar = pl.ds(pl.multiple_of(i * FB, FB) + rh * HB, HB)
                    x2 = _bf(xs[xr, cols]).astype(F32) + rep(modb[nn // 2, :, mcols], HB) * ha[ar, cols]
                    qka[2 * nn + half, pl.ds(srow + rh * (HB // 2), HB // 2), :] = pack(
                        x2 + rep(modb[12 + nn // 2, :, mcols], HB) * yy, F32)
                    if rh == ch:
                        pltpu.make_async_copy(
                            qka.at[2 * nn + half, pl.ds(srow, HB), :],
                            out32.at[pl.ds(pl.multiple_of(i * HB, HB), HB), cols],
                            sem.at[SEM_OUT]).start()

            _strassen(outer, finish)
        assert not jobs and not pending and state['piece'] == 16
        return carry

    with jax.named_scope("p4_ffn"):
        lax.fori_loop(0, nb, ffn, 0)
    pltpu.make_async_copy(out32, out32, sem.at[SEM_OUT]).wait()


@jax.jit
def pallas_adaLN_cond__memory_aug_recurrent_mem_tr__dense_activation_gelu__prompt_kernel(
    A_x, A_mem0, A_Wq, A_Wk, A_Wv, A_Wo, A_seg_len, B_x, B_w1, B_b1, B_w2, B_b2, c, w_mod,
):
    assert A_x.shape == (1, S, D) and A_Wq.shape == (D, H, E) and A_mem0.shape == (1, M, D)
    any_spec = pl.BlockSpec(memory_space=pl.ANY)
    out = pl.pallas_call(
        _kernel,
        out_shape=jax.ShapeDtypeStruct((S, D), BF16),
        in_specs=[any_spec] * 12,
        out_specs=any_spec,
        scratch_shapes=[
            pltpu.VMEM((S // 2, D), U32),
            pltpu.VMEM((96, D // 2, E), U32),
            pltpu.VMEM((8, H * E // 2, 128), U32),
            pltpu.VMEM((D // 2, FF), U32),
            pltpu.VMEM((FF // 2, D), U32),
            pltpu.VMEM((H, RING, E), F32),
            pltpu.VMEM((H, RING, E), F32),
            pltpu.VMEM((H + 1, RING, E), F32),
            pltpu.VMEM((H, RING, E), F32),
            pltpu.VMEM((S, D), F32),
            pltpu.VMEM((S - PRE, D), F32),
            pltpu.VMEM((M, D), F32),
            pltpu.VMEM((NQ, 2, 8, KQ), F32),
            pltpu.VMEM((16, 8, 256), F32),
            pltpu.VMEM((8, D), U32),
            pltpu.VMEM((D // 2, 128), U32),
            pltpu.VMEM((2, 2, D // 2, 128), F32),
            pltpu.VMEM((8, FF + D), F32),
            pltpu.VMEM((80, 128), F32),
            pltpu.VMEM((8, 32, 128), F32),
            pltpu.VMEM((8, 128), U32),
            pltpu.SMEM((1,), jnp.int32),
            pltpu.VMEM((8, FF // 8, 128), U32),
            pltpu.VMEM((13 * 64, D), U32),
            pltpu.VMEM((128, 256), U32),
            pltpu.VMEM((128, 256), U32),
            pltpu.VMEM((128, 256), U32),
            pltpu.VMEM((128, 256), U32),
            pltpu.VMEM((M, D), BF16),
            pltpu.VMEM((FF,), BF16),
            pltpu.VMEM((D,), BF16),
            pltpu.VMEM((1, D), BF16),
            pltpu.SemaphoreType.DMA((NSEM,)),
        ],
        compiler_params=pltpu.CompilerParams(vmem_limit_bytes=127 * 1024 * 1024, disable_bounds_checks=True,
                                             disable_semaphore_checks=True),
    )(
        A_x.reshape(S, D), A_mem0.reshape(M, D),
        A_Wq.reshape(D // 2, 2, H, E), A_Wk.reshape(D // 2, 2, H, E), A_Wv.reshape(D // 2, 2, H, E),
        A_Wo.reshape(H * E, D), B_w1, B_b1, B_w2, B_b2, c, w_mod,
    )
    return out.reshape(1, S, D)
```

```python
import functools
import math

import jax
import jax.numpy as jnp
from jax import lax
import jax.experimental.pallas as pl
import jax.experimental.pallas.tpu as pltpu

F32 = jnp.float32
BF16 = jnp.bfloat16
U32 = jnp.uint32

S = 2048
D = 1024
H = 32
E = 128
M = 8
SEG = 32
NSEG = S // SEG
FF = 3584
NP = H // 2
TOK = 24
PRE = S - NSEG * TOK
RING = 576
OOFF = (-NSEG * TOK) % RING
LN_EPS = 1e-5
FB = 256
P3_WEIGHTS = (0.78, 1.0, 1.0, 1.0)
LN0_PLAN = (0,) * 8 + (1,) * 16 + (0,) * 4
LN_PLAN = (1, 1, 1, 1, 1, 1, 1, 2, 2, 2, 2, 1, 0, 0)
FFN_DENSITY = 1.0 / 24
ATT_COL, ATT_N1, ATT_N2 = 6, 2, 5
TIE_R, TIE_R0, TIE_L = (5, 6), (0, 1, 2, 3, 4, 5, 6), (0, 5, 6)
JOB_GROUPS = ([1, 3], [4, 2], [0], [5], [6])
UNROLL = 4

NQ = 4
KQ = D // NQ

FIRST_STARTS = [('m', 0), ('w', 0, 0, 4), ('w', 0, 4, 8), ('m', 1), ('w', 0, 8, 12), ('w', 1, 0, 8), ('m', 2),
                ('w', 1, 8, 12)]
P1A_BLOCKS = [
    ([], [('m', 0)]),
    ([], [('w', 0, 0, 4)]),
    ([], [('w', 0, 4, 8)]),
    ([('w', 2, 0, 8), ('m', 3), ('w', 2, 8, 12)], [('m', 1), ('w', 0, 8, 12)]),
    ([('w', 3, 0, 12)], [('w', 1, 0, 8)]),
    ([('g', 2), ('g', 3)], [('m', 2), ('w', 1, 8, 12)]),
    ([], [('w', 2, 0, 8)]),
    ([('g', 4), ('g', 5)], [('m', 3), ('w', 2, 8, 12)]),
    ([], [('w', 3, 0, 12)]),
]
W_ITEMS = [it for _, items in P1A_BLOCKS for it in items if it[0] == 'w']
IT_ROWS = TOK * UNROLL
X_CHUNKS = (PRE, PRE + IT_ROWS, PRE + 3 * IT_ROWS, S)
LN_SLOTS = ((0, 11), (1, 5))
MOD_SLOTS = ((0, 2), (0, 4), (0, 6), (1, 8), (1, 9), (1, 10), (1, 11), (2, 0))
NX0 = 4

SEM_C = 0
SEM_X0 = 1
SEM_MOD = SEM_X0 + NX0
SEM_WA = SEM_MOD + NQ + 2
SEM_WB = SEM_WA + 10
SEM_XC = SEM_WB + 6
SEM_WO = SEM_XC + 3
SEM_W1 = SEM_WO + 1
SEM_W2 = SEM_W1 + 1
SEM_OUT = SEM_W2 + 1
NSEM = SEM_OUT + 1


def _ln(x):
    m = jnp.mean(x, axis=-1, keepdims=True)
    xc = x - m
    v = jnp.mean(xc * xc, axis=-1, keepdims=True)
    return xc * lax.rsqrt(v + LN_EPS)


def _bf(w32):
    return pltpu.bitcast(w32, BF16)


def _dot(a, b):
    return jnp.dot(a, b, preferred_element_type=F32)


def _lhs_combos(a11, a12, a21, a22):
    return [a11 - a22, a21 - a22, a11, a22, a12 - a11, a21 - a11, a12 - a22]


def _rhs_combos(b11, b12, b21, b22):
    return [b11 - b22, b11, b12 + b22, b21 + b11, b22, b11 + b12, b21 + b22]


_LHS_TERMS = {0: ((0, 0), (1, 1), -1), 1: ((1, 0), (1, 1), -1), 2: ((0, 0), None, 0), 3: ((1, 1), None, 0),
              4: ((0, 1), (0, 0), -1), 5: ((1, 0), (0, 0), -1), 6: ((0, 1), (1, 1), -1)}
_RHS_TERMS = {0: ((0, 0), (1, 1), -1), 1: ((0, 0), None, 0), 2: ((0, 1), (1, 1), 1), 3: ((1, 0), (0, 0), 1),
              4: ((1, 1), None, 0), 5: ((0, 0), (0, 1), 1), 6: ((1, 0), (1, 1), 1)}
_SWAP = {c: int(c in (2, 4, 5, 6)) for c in range(7)}


def _combo(terms, c, blk):
    p, q, sign = terms[c]
    if q is None:
        return blk(*p)
    return blk(*p) + blk(*q) if sign > 0 else blk(*p) - blk(*q)


def _rhs_operand(c, blk):
    p, q, sign = _RHS_TERMS[c]
    a = _bf(blk(*p))
    if q is None:
        return a
    a = a.astype(F32)
    b = _bf(blk(*q)).astype(F32)
    return (a + b if sign > 0 else a - b).astype(BF16)


def _strassen(prod, finish):
    m1 = prod(1)
    m3 = prod(3)
    finish(m1 + m3, 1, 0)
    m2 = prod(2)
    m4 = prod(4)
    finish(m2 + m4, 0, 1)
    m0 = prod(0)
    m5 = prod(5)
    finish((m2 - m1) + m0 + m5, 1, 1)
    m6 = prod(6)
    finish((m3 - m4) + m0 + m6, 0, 0)


def _strassen_value(prod2, c):
    r = {}
    _strassen(functools.partial(prod2, c), lambda y, rh, ch: r.__setitem__((rh, ch ^ _SWAP[c]), y))
    return jnp.concatenate([jnp.concatenate([r[0, 0], r[0, 1]], axis=1),
                            jnp.concatenate([r[1, 0], r[1, 1]], axis=1)], axis=0)


_ORDER = (1, 3, 2, 4, 0, 5, 6)

_PAIRS = [(c, d) for c in range(7) for d in range(7) if not (c in (1, 4) and d in (1, 4))]


def _plain_block(c, d):
    return 2 * (c // 4) + d // 4, 2 * (c // 4) + ((d // 4) ^ _SWAP[c])


def _kernel(x_hbm, mem0_hbm, wq_hbm, wk_hbm, wv_hbm, wo_hbm, w1_hbm, b1_hbm, w2_hbm, b2_hbm,
            c_hbm, wmod_hbm, out_hbm,
            xs, wqkv, wo, w1, w2, qka, qkb, vring, oring, ha, hn, memb, moda, modb, scb, colb, slab, biasb,
            fillb, accb, zerob, wx, hb2, pk0, pk1, pk2, pk3, mem0_ref, b1_ref, b2_ref, c_ref, sem):
    qkv_hbm = [r.bitcast(U32) for r in (wq_hbm, wk_hbm, wv_hbm)]
    x32 = x_hbm.bitcast(U32)
    wo32 = wo_hbm.bitcast(U32)
    wmod32 = wmod_hbm.bitcast(F32)

    def wma(qq, k):
        return pl.ds(512 * (qq // 2), 512), pl.ds(512 * (qq % 2) + k * KQ, KQ)

    def hb_idx(c, q0, nq, row0=0, nrows=PRE // 4):
        return pl.ds(1024 + 128 * (c // 2) + row0, nrows), pl.ds(512 * (c % 2) + 128 * q0, 128 * nq)

    def units_start(lo, hi, rows, sem_idx):
        for u in range(lo, hi):
            j, m = u // 3, u % 3
            for p in range(2):
                pltpu.make_async_copy(qkv_hbm[m].at[rows, p, j, :], wqkv.at[2 * u + p, rows, :],
                                      sem.at[sem_idx]).start()

    def units_wait(lo, n, rows, sem_idx):
        blk = wqkv.at[pl.ds(2 * lo, 2 * n), rows, :]
        pltpu.make_async_copy(blk, blk, sem.at[sem_idx]).wait()

    def item_start(item):
        if item[0] == 'm':
            qq = item[1]
            for k in range(2):
                pltpu.make_async_copy(wmod32.at[:, pl.ds(k * D + qq * KQ, KQ)], ha.at[wma(qq, k)],
                                      sem.at[SEM_MOD + qq]).start()
        elif item[0] == 'w':
            _, qq, lo, hi = item
            units_start(lo, hi, pl.ds(qq * (KQ // 2), KQ // 2), SEM_WA + W_ITEMS.index(item))
        else:
            whole_start(item[1])

    def item_wait(item):
        if item[0] == 'm':
            qq = item[1]
            blk = ha.at[pl.ds(512 * (qq // 2), 512), pl.ds(512 * (qq % 2), 512)]
            pltpu.make_async_copy(blk, blk, sem.at[SEM_MOD + qq]).wait()
        else:
            _, qq, lo, hi = item
            units_wait(lo, hi - lo, pl.ds(qq * (KQ // 2), KQ // 2), SEM_WA + W_ITEMS.index(item))

    def whole_start(i):
        if i == 2:
            xc_copy(0).start()
        units_start(6 * i, 6 * i + 6, pl.ds(0, D // 2), SEM_WB + i - 2)

    def slab_copies(it):
        return [pltpu.make_async_copy(
            wmod32.at[:, pl.ds(pl.multiple_of(2 * D + it * 256 + t * 128, 128), 128)],
            slab.at[it & 1, t], sem.at[SEM_MOD + NQ + (it & 1)]) for t in range(2)]

    def x0_copy(i):
        n = PRE // 2 // NX0
        rows = pl.ds(pl.multiple_of(i * n, n), n)
        return pltpu.make_async_copy(x32.at[rows], xs.at[rows], sem.at[SEM_X0 + i])

    def xc_copy(i):
        rows = pl.ds(X_CHUNKS[i] // 2, (X_CHUNKS[i + 1] - X_CHUNKS[i]) // 2)
        return pltpu.make_async_copy(x32.at[rows], xs.at[rows], sem.at[SEM_XC + i])

    def wo_copy(n):
        return pltpu.make_async_copy(wo32.at[:, pl.ds(n * 128, 128)], wo.at[n], sem.at[SEM_WO])

    w1_copy = pltpu.make_async_copy(w1_hbm.bitcast(U32), w1, sem.at[SEM_W1])
    w2_copy = pltpu.make_async_copy(w2_hbm.bitcast(U32), w2, sem.at[SEM_W2])
    small_copies = [pltpu.make_async_copy(a, b, sem.at[SEM_C])
                    for a, b in ((c_hbm, c_ref), (mem0_hbm, mem0_ref), (b1_hbm, b1_ref),
                                 (b2_hbm, b2_ref))]

    def deinterleave(u, row0, nrows):
        for k in range(nrows // 64):
            rows = pl.ds(row0 + k * 64, 64)
            a = wqkv[2 * u, rows, :]
            b = wqkv[2 * u + 1, rows, :]
            wqkv[2 * u, rows, :] = (a & jnp.uint32(0xFFFF)) | (b << 16)
            wqkv[2 * u + 1, rows, :] = (a >> 16) | (b & jnp.uint32(0xFFFF0000))

    def load_x16(row2):
        return _bf(xs[pl.ds(row2, 8), :]).astype(F32)

    pks = [pk0, pk1, pk2, pk3]

    def pack(v, dtype=U32):
        rows = pl.ds(0, v.shape[0] // 2)
        pk = pks[0]
        pk[rows, pl.ds(0, 128)] = pltpu.bitcast(v.astype(BF16), U32)
        return pltpu.bitcast(pk[rows, pl.ds(0, 128)], dtype)

    def after(y, bits, t=0):
        if not bits:
            return y
        top = [y[0:8, u * 128:(u + 1) * 128] for u in range(y.shape[1] // 128)]
        top[t] = pltpu.bitcast(pltpu.bitcast(top[t], U32)
                               | (functools.reduce(jnp.bitwise_or, bits) & zerob[...]), F32)
        return jnp.concatenate([jnp.concatenate(top, axis=1), y[8:]], axis=0)

    def rep(v8, n):
        return jnp.concatenate([v8] * (n // 8), axis=0)

    def mrow(k, n):
        if k < 2:
            return rep(jnp.concatenate([moda[qq, k] for qq in range(NQ)], axis=1), n)
        return rep(jnp.concatenate([modb[4 * (k - 2) + q] for q in range(4)], axis=1), n)

    for cp in small_copies:
        cp.start()
    for i in range(NX0):
        x0_copy(i).start()
    for item in FIRST_STARTS:
        item_start(item)

    def start_rest():
        xc_copy(1).start()
        for n in range(8):
            wo_copy(n).start()
        for cp in slab_copies(0):
            cp.start()
        xc_copy(2).start()
        w1_copy.start()
        w2_copy.start()

    r = lax.broadcasted_iota(jnp.int32, (80, 128), 0)
    q = lax.broadcasted_iota(jnp.int32, (80, 128), 1)
    r_tok = r < 64
    q_tok = q < 64
    r_head = jnp.where(r_tok, r >> 5, (r - 64) >> 3)
    q_head = jnp.where(q_tok, q >> 5, (q - 64) >> 3)
    same = (r_head == q_head) & (q < 80)
    causal_ok = jnp.logical_not(r_tok & q_tok & ((q & 31) > (r & 31)))
    scale = E ** (-0.5)
    fillb[...] = jnp.where(same, jnp.where(causal_ok, 0.0, -1e9 / scale), -jnp.inf).astype(F32)
    zerob[...] = jnp.zeros((8, 128), U32)

    for cp in small_copies:
        cp.wait()
    cf = c_ref[...].astype(F32)
    sc = (cf * jax.nn.sigmoid(cf)).astype(BF16)
    scb[...] = pltpu.bitcast(jnp.broadcast_to(sc, (16, D)), U32)
    scf = jnp.broadcast_to(sc.astype(F32), (128, D))
    for k in range(8):
        colb[pl.ds(k * 64, 64), :] = pltpu.bitcast(scf[:, k * 128:(k + 1) * 128].T.astype(BF16), U32)
    memb[...] = mem0_ref[...].astype(F32)
    biasb[:, pl.ds(0, FF)] = jnp.broadcast_to(b1_ref[...].astype(F32).reshape(1, FF), (8, FF))
    biasb[:, pl.ds(FF, D)] = jnp.broadcast_to(b2_ref[...].astype(F32).reshape(1, D), (8, D))

    def pre_norm(i, carry):
        x0_copy(i).wait()
        nr = PRE // NX0
        for z in range(nr // 16):
            xn = _ln(load_x16(pl.multiple_of(i * (nr // 2) + z * 8, 8)))
            for n in range(8):
                oring[n, pl.ds(pl.multiple_of(i * nr + z * 16, 16), 16), :] = xn[:, n * 128:(n + 1) * 128]
        return carry

    with jax.named_scope("p0_ln"):
        lax.fori_loop(0, NX0, pre_norm, 0)

    def dst_slot(i, k, p):
        cls, m = k // 3, k % 3
        if m == 2:
            return vring, 4 * i + 2 * cls + p
        return (qka, qkb)[cls], 4 * i + 2 * m + p

    PH = PRE // 2
    assert KQ == 256

    def item_run(item):
        if item[0] == 'm':
            qq = item[1]
            sc16 = _bf(scb[...])
            ca1 = 1.0 + _dot(sc16, _bf(ha[wma(qq, 1)]))[0:8].astype(BF16).astype(F32)
            sa = _dot(sc16, _bf(ha[wma(qq, 0)]))[0:8].astype(BF16).astype(F32)
            moda[qq, 0] = sa
            moda[qq, 1] = ca1
            for z in range(PH // 32):
                def h_blk(rh, kh):
                    cols = slice(kh * 128, (kh + 1) * 128)
                    return (oring[2 * qq + kh, pl.ds(rh * PH + z * 32, 32), :] * rep(ca1[:, cols], 32)
                            + rep(sa[:, cols], 32))

                for c, v in enumerate(_lhs_combos(h_blk(0, 0), h_blk(0, 1), h_blk(1, 0), h_blk(1, 1))):
                    ha[hb_idx(c, qq, 1, z * 16, 16)] = pltpu.bitcast(v.astype(BF16), F32)
            return
        _, qq, lo, hi = item
        if lo == 0 and qq >= 2:
            a_jobs.extend(functools.partial(lhs0_job, k, qq - 2, c) for k in range(PQ // 16) for c in range(7))
        for u in range(lo, hi):
            deinterleave(u, qq * (KQ // 2), KQ // 2)
            i, k = u // 6, u % 6

            def prod(c):
                lhs = pltpu.bitcast(ha[hb_idx(c, qq, 1)], U32)
                if u >= 2:
                    lhs = tie_rows(lhs, a_jobs, (1 + 4 * ((7 * u + _ORDER.index(c)) % 4),))
                rhs = _rhs_operand(c, lambda a, b: wqkv[2 * u + b, pl.ds((2 * qq + a) * 64, 64), :])
                return _dot(_bf(lhs), rhs)

            def finish(y, rh, ch):
                ref, idx = dst_slot(i, k, ch)
                rows = pl.ds(RING - PRE + rh * PH, PH)
                if qq > 0:
                    y = y + ref[idx, rows, :]
                ref[idx, rows, :] = y

            _strassen(prod, finish)

    def tie_rows(w, jobs, groups):
        if not jobs:
            return w
        parts = [w[8 * g:8 * g + 8, 0:128] for g in range(w.shape[0] // 8)]
        for g in groups:
            if jobs:
                parts[g] = parts[g] | (jobs.pop(0)() & zerob[...])
        first = jnp.concatenate(parts, axis=0)
        return first if w.shape[1] == 128 else jnp.concatenate([first, w[:, 128:]], axis=1)

    PQ = PRE // 4
    a_jobs = []

    def lhs0_idx(c, d, k, nk, t, nt):
        e = 7 * c + d
        return pl.ds(64 * (e // 4) + 8 * k, 8 * nk), pl.ds(256 * (e % 4) + 128 * t, 128 * nt)

    def lhs0_job(k, t, c):
        def sub(ri, ki):
            def blk(ro, ko):
                n = 2 * ko + ki + 4 * t
                cols = pl.ds((n % 2) * 128, 128)
                return (oring[n, pl.ds((2 * ro + ri) * PQ + 16 * k, 16), :] * rep(moda[n // 2, 1, :, cols], 16)
                        + rep(moda[n // 2, 0, :, cols], 16))

            return _combo(_LHS_TERMS, c, blk)

        bits = None
        for d, v in enumerate(_lhs_combos(sub(0, 0), sub(0, 1), sub(1, 0), sub(1, 1))):
            hb2[lhs0_idx(c, d, k, 1, t, 1)] = pltpu.bitcast(v.astype(BF16), U32)
            if d in TIE_L:
                b = pltpu.bitcast(v[8 * (d % 2):8 * (d % 2) + 8], U32)
                bits = b if bits is None else bits | b
        return bits

    def ln1_piece(row2):
        h16 = _ln(load_x16(PRE // 2 + row2)) * mrow(1, 16) + mrow(0, 16)
        hn[pl.ds(pl.multiple_of(2 * row2, 16), 16), :] = h16
        return pltpu.bitcast(h16[8:16, D - 128:], U32)

    def phase1b(i, carry):
        @pl.when(i == 3)
        def _():
            whole_start(6)
            whole_start(7)
            start_rest()

        units_wait(6 * i, 6, pl.ds(0, D // 2), SEM_WB + i - 2)
        ln1_piece(pl.multiple_of((i - 2) * 8, 8))

        def raw(m, kq, nq, g):
            u = 6 * i + m + 3 * (nq // 2)
            return wqkv[2 * u + nq % 2, pl.ds((kq + 4 * (g // 8)) * 64 + 8 * (g % 8), 8), :]

        ops = {}

        def rhs0_job(m, c, g):
            def sub(ki, ni):
                return _combo(_RHS_TERMS, c,
                              lambda ko, no: _bf(raw(m, 2 * ko + ki, 2 * no + (ni ^ _SWAP[c]), g)).astype(F32))

            bits = None
            for d, v in enumerate(_rhs_combos(sub(0, 0), sub(0, 1), sub(1, 0), sub(1, 1))):
                if (c, d) in _PAIRS:
                    ops[m, c, d, g] = pack(v)
                    if d in TIE_R0:
                        bits = ops[m, c, d, g] if bits is None else bits | ops[m, c, d, g]
            return bits

        seq = [(m, c) for m in range(3) for c in _ORDER]
        jobs = []
        count = [0]
        deinterleave(6 * i, 0, D // 2)
        deinterleave(6 * i + 3, 0, D // 2)
        for g in range(16):
            rhs0_job(*seq[0], g)
        for m in range(3):
            if m < 2:
                deinterleave(6 * i + m + 1, 0, D // 2)
                deinterleave(6 * i + m + 4, 0, D // 2)

            def prod(c, d):
                if (c, d) in _PAIRS:
                    rhs = [ops[m, c, d, g] for g in range(16)]
                else:
                    rhs = [raw(m, *_plain_block(c, d), g) for g in range(16)]
                lhs = tie_rows(hb2[lhs0_idx(c, d, 0, 8, 0, 2)], jobs, ((0, 3, 6), (1, 4, 7))[count[0] % 2])
                count[0] += 1
                return _dot(_bf(lhs), _bf(jnp.concatenate(rhs, axis=0)))

            def outer(c):
                assert not jobs
                count[0] = 0
                nx = seq.index((m, c)) + 1
                if nx < len(seq):
                    jobs.extend(functools.partial(rhs0_job, *seq[nx], g) for g in range(16))
                return _strassen_value(prod, c)

            def finish(y, rh, ch):
                for ci in range(2):
                    ref, idx = dst_slot(i, m + 3 * ch, ci)
                    ref[idx, pl.ds(RING - PRE + rh * PH, PH), :] = y[:, ci * 128:(ci + 1) * 128]

            _strassen(outer, finish)
        return carry

    for bi, (starts, items) in enumerate(P1A_BLOCKS):
        for item in starts:
            item_start(item)
        with jax.named_scope("p1a_wait%d" % bi):
            for item in items:
                item_wait(item)
        for item in items:
            item_run(item)
    assert not a_jobs
    xc_copy(0).wait()
    with jax.named_scope("p1b"):
        lax.fori_loop(2, 8, phase1b, 0)
    pks.pop(0)
    xc_copy(1).wait()
    for n in range(8):
        wo_copy(n).wait()

    cexp = scale * math.log2(math.e)
    NG = NP // 2
    grp = [(4 * (g // 2) + (g % 2), 4 * (g // 2) + (g % 2) + 2) for g in range(NG)]
    early = [2 * j + u for g in range(NG - 3) for j in grp[g] for u in range(2)]
    late = [h for h in range(H) if h not in early]

    def step(it, k, side_jobs):
        s = it * UNROLL + k
        split = k > 0
        base = TOK * UNROLL * it
        w0 = pl.multiple_of(lax.rem(base, RING), 32) + TOK * k
        r0 = pl.multiple_of(lax.rem(SEG * s + (RING - PRE), RING), 32)
        ow = pl.multiple_of(lax.rem(SEG * s + OOFF, RING), 32)
        o0 = pl.multiple_of(lax.rem(base + OOFF, RING), 32) + TOK * k
        a0 = pl.multiple_of(base, 32) + TOK * k
        X = jnp.concatenate([hn[pl.ds(a0, TOK), :], memb[...]], axis=0).astype(BF16)
        ym = [None] * 96
        probs = [None] * NP
        om = [None] * H
        order = (4, 5, 0, 1, 2, 3)

        if split:
            for t in order:
                accb[t] = _dot(X[:, :D // 2], _bf(wqkv[t, pl.ds(0, D // 4), :]))

        def slot(j, t):
            if t >= 4:
                return vring, 2 * j + t - 4
            return (qka, qkb)[j % 2], 4 * (j // 2) + t

        def proj(j, t, job):
            c = 6 * j + t
            bits = [] if job is None else [job()]
            if split and j == 0:
                y = accb[t] + _dot(X[:, D // 2:], _bf(wqkv[c, pl.ds(D // 4, D // 4), :]))
            else:
                y = _dot(X, _bf(wqkv[c]))
            ref, k = slot(j, t)
            ref[k, pl.ds(w0, TOK), :] = after(y, bits)[0:TOK]
            ym[c] = y[TOK:TOK + M]

        def gather(j, m, pad):
            c = 6 * j + 2 * m
            ref, k = slot(j, 2 * m)
            parts = [ref[k, pl.ds(r0, SEG), :], ref[k + 1, pl.ds(r0, SEG), :], ym[c], ym[c + 1]]
            if pad:
                parts.append(jnp.zeros((48, E), F32))
            return jnp.concatenate(parts, axis=0).astype(BF16)

        def scores(j):
            sc_ = lax.dot_general(gather(j, 0, False), gather(j, 1, True),
                                  (((1,), (1,)), ((), ())), preferred_element_type=F32)
            fill = fillb[...]
            sc_ = jnp.where(fill == 0.0, sc_, fill)
            mx = jnp.max(sc_, axis=-1, keepdims=True)
            p = jnp.exp2((sc_ - mx) * cexp)
            l = jnp.sum(p, axis=-1, keepdims=True)
            rl = pl.reciprocal(l, approx=True)
            rl = rl * (2.0 - l * rl)
            probs[j] = p * rl

        def park(j):
            vring[H, pl.ds(40 * (j % 8), 40), :] = pack(probs[j], F32)
            probs[j] = None

        def pv(j):
            if probs[j] is None:
                P = _bf(vring[H, pl.ds(40 * (j % 8), 40), :])
            else:
                P = probs[j].astype(BF16)
            o = _dot(P, gather(j, 2, True))
            oring[2 * j, pl.ds(ow, SEG), :] = o[0:32]
            oring[2 * j + 1, pl.ds(ow, SEG), :] = o[32:64]
            om[2 * j] = o[64:72]
            om[2 * j + 1] = o[72:80]

        def o_lhs(hs):
            return jnp.concatenate(
                [jnp.concatenate([oring[h, pl.ds(o0, TOK), :], om[h]], axis=0) for h in hs],
                axis=1).astype(BF16)

        def o_rhs(n, hs):
            return _bf(jnp.concatenate([wo[n, pl.ds(h * 64, 64), :] for h in hs], axis=0))

        for g in range(NG):
            cols = [(j, t) for j in grp[g] for t in order]
            if g == 2:
                cols = ([(j, t) for j in grp[g] for t in (4, 5)]
                        + [(j, t) for j in grp[g] for t in range(4)])
            for j in (grp[0] + grp[1] if g == 3 else grp[g - 2] if g >= 4 else ()):
                park(j)
            for ci, (j, t) in enumerate(cols):
                if g == 2 and ci == 4:
                    for jj in grp[0] + grp[1]:
                        scores(jj)
                if g >= 3 and ci == ATT_COL:
                    for jj in grp[g - 1]:
                        scores(jj)
                    for jj in grp[g - 3]:
                        pv(jj)
                proj(j, t, side_jobs.get((g, ci)))
        lo = o_lhs(early)
        for n in range(8):
            accb[n] = _dot(lo, o_rhs(n, early))
            if n == ATT_N1:
                for jj in grp[NG - 1]:
                    scores(jj)
                for jj in grp[NG - 3]:
                    pv(jj)
            if n == ATT_N2:
                for jj in grp[NG - 2] + grp[NG - 1]:
                    pv(jj)
        lo = o_lhs(late)
        for n in range(8):
            a = accb[n] + _dot(lo, o_rhs(n, late))
            ha[pl.ds(a0, TOK), pl.ds(n * 128, 128)] = a[0:TOK]
            memb[:, pl.ds(n * 128, 128)] = a[TOK:TOK + M]

    NIT = NSEG // UNROLL

    def lo16(w):
        return pltpu.bitcast(w << 16, F32)

    def hi16(w):
        return pltpu.bitcast(w & jnp.uint32(0xFFFF0000), F32)

    def steps(it, carry):
        @pl.when(it == 1)
        def _():
            xc_copy(2).wait()

        for cp in slab_copies(it):
            cp.wait()
        for cp in slab_copies((it + 1) & (NIT - 1)):
            cp.start()
        acc = [None, None]

        def mod_job(q):
            for kk in range(2 * q, 2 * q + 2):
                cw = colb[pl.ds(kk * 8, 8), :]
                for t in range(2):
                    w = pltpu.bitcast(slab[it & 1, t, pl.ds(kk * 8, 8), :], U32)
                    v = lo16(w) * lo16(cw) + hi16(w) * hi16(cw)
                    acc[t] = v if acc[t] is None else acc[t] + v
            if q < D // 32 - 1:
                return pltpu.bitcast(acc[0], U32) | pltpu.bitcast(acc[1], U32)
            y = jnp.sum(jnp.concatenate(acc, axis=1), axis=0, keepdims=True).astype(BF16).astype(F32)
            y = jnp.broadcast_to(y + jnp.where((it >> 2) == 2, 1.0, 0.0), (8, 256))
            modb[it] = y
            return pltpu.bitcast(y[:, 0:128], U32)

        nxt2 = pl.multiple_of(jnp.minimum(it + 1, NIT - 1) * (IT_ROWS // 2), 16)
        pieces = list(range(IT_ROWS // 16))
        for k in range(UNROLL):
            side_jobs = {pos: functools.partial(mod_job, 8 * k + q) for q, pos in enumerate(MOD_SLOTS)}
            for pos in LN_SLOTS[k % 2:]:
                side_jobs[pos] = functools.partial(ln1_piece, nxt2 + 8 * pieces.pop(0))
            step(it, k, side_jobs)
        assert not pieces
        return carry

    with jax.named_scope("p2_steps"):
        lax.fori_loop(0, NIT, steps, 0)
    for cp in slab_copies(0):
        cp.wait()
    w1_copy.wait()
    w2_copy.wait()

    nb = S // FB
    HB = FB // 2
    QB = FB // 4

    def ln2_piece(hs, blk, off):
        x2 = (load_x16(pl.multiple_of(blk * HB, HB) + off // 2)
              + mrow(2, 16) * ha[pl.ds(pl.multiple_of(blk * FB, FB) + off, 16), :])
        h = _ln(x2) * mrow(4, 16) + mrow(3, 16)
        hs[off] = h
        return pltpu.bitcast(h[8:16, D - 128:], U32)

    def lhs1_loc(base, c, d):
        e = 7 * c + d
        return base + 32 * (e // 4), 256 * (e % 4)

    def lhs1_job(hs, base, k, t, c):
        def sub(ri, ki):
            def blk(ro, ko):
                c0 = (2 * ko + ki) * 256 + t * 128
                return hs[(2 * ro + ri) * QB + 16 * k][:, c0:c0 + 128]

            return _combo(_LHS_TERMS, c, blk)

        bits = None
        for d, v in enumerate(_lhs_combos(sub(0, 0), sub(0, 1), sub(1, 0), sub(1, 1))):
            r0, c0 = lhs1_loc(base, c, d)
            hn[pl.ds(r0 + 8 * k, 8), pl.ds(c0 + t * 128, 128)] = pltpu.bitcast(
                v.astype(BF16), F32)
            if d in TIE_L:
                b = pltpu.bitcast(v[8 * (d % 2):8 * (d % 2) + 8], U32)
                bits = b if bits is None else bits | b
        return bits

    def make_ln2(blk, base, plan, jobs):
        state = dict(piece=0, call=0)
        pending, hs = [], {}

        def issue():
            jobs.extend(pending)
            del pending[:]
            bits = []
            for _ in range(plan[state['call']]):
                k, r = state['piece'] // 4, state['piece'] % 4
                bits.append(ln2_piece(hs, blk, r * QB + 16 * k))
                if r == 3:
                    pending.extend(functools.partial(lhs1_job, hs, base, k, t, c)
                                   for t in range(2) for c in range(7))
                state['piece'] += 1
            state['call'] += 1
            return bits

        assert sum(plan) == FB // 16 and plan[-1] == 0
        return issue

    K1, N1, K2, N2 = D // 8, FF // 4, FF // 8, D // 4

    def rhs1_loc(c, d, n):
        e = _PAIRS.index((c, d)) * 7 + n
        return wqkv, e // 4, K1 * (e % 4)

    rhs2_slots = ([(wqkv, e, 0) for e in range(79, 96)] + [(qkb, e, 0) for e in range(H)]
                  + [(vring, e, 0) for e in range(H + 1)] + [(wx, e, 0) for e in range(8)])

    def rhs2_loc(c, d, n):
        return rhs2_slots[_PAIRS.index((c, d)) * 2 + n]

    def rhs_job(w, kq, nq, loc, n, r, cs):
        cache = {}

        def blk(ko, no, ki, ni):
            key = (2 * ko + ki, 2 * no + ni)
            if key not in cache:
                cache[key] = _bf(w[pl.ds(r + key[0] * kq, 8), pl.ds(n * 128 + key[1] * nq, 128)]).astype(F32)
            return cache[key]

        bits = None
        for c in cs:
            def sub(ki, ni):
                return _combo(_RHS_TERMS, c, lambda ko, no: blk(ko, no, ki, ni ^ _SWAP[c]))

            for d, v in enumerate(_rhs_combos(sub(0, 0), sub(0, 1), sub(1, 0), sub(1, 1))):
                if (c, d) in _PAIRS:
                    ref, idx, row = loc(c, d, n)
                    b = pack(v)
                    ref[idx, pl.ds(row + r, 8), :] = pltpu.bitcast(b, ref.dtype)
                    if d in TIE_R:
                        bits = b if bits is None else bits | b
        return bits

    def rhs_load(w, kq, nq, loc, c, d, n):
        if (c, d) not in _PAIRS:
            qk, qn = _plain_block(c, d)
            return w[pl.ds(qk * kq, kq), pl.ds(qn * nq + n * 128, 128)]
        ref, idx, row = loc(c, d, n)
        return pltpu.bitcast(ref[idx, pl.ds(row, kq), :], U32)

    def make_tie(jobs, credit):
        state = [credit]

        def tie(raw, density):
            if not jobs:
                return raw
            parts = []
            for r in range(0, raw.shape[0], 8):
                v = raw[r:r + 8]
                state[0] += density
                if jobs and state[0] >= 1.0:
                    state[0] -= 1.0
                    v = v | (jobs.pop(0)() & zerob[...])
                parts.append(v)
            return jnp.concatenate(parts, axis=0)

        return tie

    def bulk_o():
        spots = ([(w1, K1, N1, rhs1_loc, n, r) for n in range(7) for r in range(0, K1, 8)]
                 + [(w2, K2, N2, rhs2_loc, n, r) for n in range(2) for r in range(0, K2, 8)])
        ng = len(JOB_GROUPS)
        jobs = [functools.partial(rhs_job, *spots[(e + (len(spots) // ng) * gi) % len(spots)], cs)
                for e in range(len(spots)) for gi, cs in enumerate(JOB_GROUPS)]
        scale_d = (len(jobs) + 56 + 6) / (7 * 64 * sum(P3_WEIGHTS))
        state = dict(credit=-2.0)
        ln2_block0 = make_ln2(0, 0, LN0_PLAN, jobs)

        def tie_lhs(tiles, density):
            tiles = [[t[8 * g:8 * g + 8] for g in range(16)] for t in tiles]
            for w in range(4):
                for g in range(16):
                    state['credit'] += density
                    for extra in range(2):
                        if jobs and state['credit'] >= 1.0:
                            state['credit'] -= 1.0
                            t = tiles[4 * w + (g + 2 * extra) % 4]
                            t[g] = t[g] | (jobs.pop(0)() & zerob[...])
            return _bf(jnp.concatenate([jnp.concatenate(t, axis=0) for t in tiles], axis=1))

        def a_blk(rh, kh):
            return jnp.concatenate([oring[h, pl.ds(rh * 256, 256), :]
                                    for h in range(16 * kh, 16 * kh + 16)], axis=1)

        lhs = [[pack(v[:, 128 * t:128 * t + 128]) for t in range(16)]
               for v in _lhs_combos(a_blk(0, 0), a_blk(0, 1), a_blk(1, 0), a_blk(1, 1))]
        for n in range(4):
            def prod(c):
                bits = ln2_block0()
                return after(_dot(tie_lhs(lhs[c], scale_d * P3_WEIGHTS[n]),
                                  _rhs_operand(c, lambda a, b: wo[n + 4 * b, pl.ds(a * 1024, 1024), :])), bits)

            def finish(y, rh, ch):
                ha[pl.ds(NSEG * TOK + rh * 256, 256), pl.ds((n + 4 * ch) * 128, 128)] = y

            _strassen(prod, finish)
        assert not jobs

    pks.pop(0)
    with jax.named_scope("p3_bulk_o"):
        bulk_o()

    pks.pop(0)
    out32 = out_hbm.bitcast(F32)

    def ffn(i, carry):
        base = pl.multiple_of((i & 1) * 512, 512)
        nbase = pl.multiple_of(((i + 1) & 1) * 512, 512)
        nxt = (i + 1) & (nb - 1)
        half = i >> 2
        srow = pl.multiple_of((i & 3) * HB, HB)

        g = {(c, d): [] for c in range(7) for d in range(7)}
        for n in range(7):
            act = {}

            def prod1(c, d):
                r0, c0 = lhs1_loc(base, c, d)
                return _dot(_bf(hn[pl.ds(r0, QB // 2), pl.ds(c0, 256)]),
                            _bf(rhs_load(w1, K1, N1, rhs1_loc, c, d, n)))

            def activate(y, rh, ch):
                b1 = jnp.concatenate([biasb[:, pl.ds((2 * ch + ci) * N1 + n * 128, 128)] for ci in range(2)],
                                     axis=1)
                act[rh, ch] = jax.nn.gelu(y + rep(b1, HB), approximate=True)

            _strassen(lambda c: _strassen_value(prod1, c), activate)
            for c in range(7):
                o = _combo(_LHS_TERMS, c, lambda a, b: act[a, b])
                for d, v in enumerate(_lhs_combos(o[:QB, :128], o[:QB, 128:], o[QB:, :128], o[QB:, 128:])):
                    g[c, d].append(v.astype(BF16))

        jobs = []
        tie = make_tie(jobs, 0.0)
        next_block_ln = make_ln2(nxt, nbase, LN_PLAN, jobs)

        for n in range(2):
            def prod2(c, d):
                return _dot(jnp.concatenate(g[c, d], axis=1),
                            _bf(tie(rhs_load(w2, K2, N2, rhs2_loc, c, d, n), FFN_DENSITY)))

            def outer(c):
                bits = next_block_ln()
                return after(_strassen_value(prod2, c), bits, _SWAP[c])

            def finish(y, rh, ch):
                for ci in range(2):
                    nn = (2 * ch + ci) * 2 + n
                    cols = pl.ds(nn * 128, 128)
                    mcols = pl.ds((nn % 2) * 128, 128)
                    yy = y[:, ci * 128:(ci + 1) * 128] + rep(biasb[:, pl.ds(FF + nn * 128, 128)], HB)
                    xr = pl.ds(pl.multiple_of(i * HB, HB) + rh * (HB // 2), HB // 2)
                    ar = pl.ds(pl.multiple_of(i * FB, FB) + rh * HB, HB)
                    x2 = _bf(xs[xr, cols]).astype(F32) + rep(modb[nn // 2, :, mcols], HB) * ha[ar, cols]
                    qka[2 * nn + half, pl.ds(srow + rh * (HB // 2), HB // 2), :] = pack(
                        x2 + rep(modb[12 + nn // 2, :, mcols], HB) * yy, F32)
                    if rh == ch:
                        pltpu.make_async_copy(
                            qka.at[2 * nn + half, pl.ds(srow, HB), :],
                            out32.at[pl.ds(pl.multiple_of(i * HB, HB), HB), cols],
                            sem.at[SEM_OUT]).start()

            _strassen(outer, finish)
        assert not jobs
        return carry

    with jax.named_scope("p4_ffn"):
        lax.fori_loop(0, nb, ffn, 0)
    pltpu.make_async_copy(out32, out32, sem.at[SEM_OUT]).wait()


@jax.jit
def pallas_adaLN_cond__memory_aug_recurrent_mem_tr__dense_activation_gelu__prompt_kernel(
    A_x, A_mem0, A_Wq, A_Wk, A_Wv, A_Wo, A_seg_len, B_x, B_w1, B_b1, B_w2, B_b2, c, w_mod,
):
    assert A_x.shape == (1, S, D) and A_Wq.shape == (D, H, E) and A_mem0.shape == (1, M, D)
    any_spec = pl.BlockSpec(memory_space=pl.ANY)
    out = pl.pallas_call(
        _kernel,
        out_shape=jax.ShapeDtypeStruct((S, D), BF16),
        in_specs=[any_spec] * 12,
        out_specs=any_spec,
        scratch_shapes=[
            pltpu.VMEM((S // 2, D), U32),
            pltpu.VMEM((96, D // 2, E), U32),
            pltpu.VMEM((8, H * E // 2, 128), U32),
            pltpu.VMEM((D // 2, FF), U32),
            pltpu.VMEM((FF // 2, D), U32),
            pltpu.VMEM((H, RING, E), F32),
            pltpu.VMEM((H, RING, E), F32),
            pltpu.VMEM((H + 1, RING, E), F32),
            pltpu.VMEM((H, RING, E), F32),
            pltpu.VMEM((S, D), F32),
            pltpu.VMEM((S - PRE, D), F32),
            pltpu.VMEM((M, D), F32),
            pltpu.VMEM((NQ, 2, 8, KQ), F32),
            pltpu.VMEM((16, 8, 256), F32),
            pltpu.VMEM((8, D), U32),
            pltpu.VMEM((D // 2, 128), U32),
            pltpu.VMEM((2, 2, D // 2, 128), F32),
            pltpu.VMEM((8, FF + D), F32),
            pltpu.VMEM((80, 128), F32),
            pltpu.VMEM((8, 32, 128), F32),
            pltpu.VMEM((8, 128), U32),
            pltpu.VMEM((8, FF // 8, 128), U32),
            pltpu.VMEM((13 * 64, D), U32),
            pltpu.VMEM((128, 256), U32),
            pltpu.VMEM((128, 256), U32),
            pltpu.VMEM((128, 256), U32),
            pltpu.VMEM((128, 256), U32),
            pltpu.VMEM((M, D), BF16),
            pltpu.VMEM((FF,), BF16),
            pltpu.VMEM((D,), BF16),
            pltpu.VMEM((1, D), BF16),
            pltpu.SemaphoreType.DMA((NSEM,)),
        ],
        compiler_params=pltpu.CompilerParams(vmem_limit_bytes=127 * 1024 * 1024, disable_bounds_checks=True,
                                             disable_semaphore_checks=True),
    )(
        A_x.reshape(S, D), A_mem0.reshape(M, D),
        A_Wq.reshape(D // 2, 2, H, E), A_Wk.reshape(D // 2, 2, H, E), A_Wv.reshape(D // 2, 2, H, E),
        A_Wo.reshape(H * E, D), B_w1, B_b1, B_w2, B_b2, c, w_mod,
    )
    return out.reshape(1, S, D)
```

```python
import functools
import math

import jax
import jax.numpy as jnp
from jax import lax
import jax.experimental.pallas as pl
import jax.experimental.pallas.tpu as pltpu

F32 = jnp.float32
BF16 = jnp.bfloat16
U32 = jnp.uint32

S = 2048
D = 1024
H = 32
E = 128
M = 8
SEG = 32
NSEG = S // SEG
FF = 3584
NP = H // 2
TOK = 24
PRE = S - NSEG * TOK
RING = 576
OOFF = (-NSEG * TOK) % RING
LN_EPS = 1e-5
FB = 256
UNROLL = 4

ATT_COL, ATT_N1, ATT_N2 = 6, 2, 5
P3_WEIGHTS = (0.78, 1.0, 1.0, 1.0)
JOB_GROUPS = ([1, 3], [4, 2], [0], [5], [6])
LN0_PLAN = (0,) * 8 + (1,) * 16 + (0,) * 4
LN_PLAN = (1, 1, 1, 1, 1, 1, 1, 2, 2, 2, 2, 1, 0, 0)
FFN_DENSITY = 1.0 / 24
TIE_R, TIE_R0, TIE_L = (5, 6), (0, 1, 2, 3, 4, 5, 6), (0, 5, 6)

NQ = 4
KQ = D // NQ

FIRST_STARTS = [('m', 0), ('w', 0, 0, 4), ('w', 0, 4, 8), ('m', 1), ('w', 0, 8, 12), ('w', 1, 0, 8), ('m', 2),
                ('w', 1, 8, 12)]
P1A_BLOCKS = [
    ([], [('m', 0)]),
    ([], [('w', 0, 0, 4)]),
    ([], [('w', 0, 4, 8)]),
    ([('w', 2, 0, 8), ('m', 3), ('w', 2, 8, 12)], [('m', 1), ('w', 0, 8, 12)]),
    ([('w', 3, 0, 12)], [('w', 1, 0, 8)]),
    ([('g', 2), ('g', 3)], [('m', 2), ('w', 1, 8, 12)]),
    ([], [('w', 2, 0, 8)]),
    ([('g', 4), ('g', 5)], [('m', 3), ('w', 2, 8, 12)]),
    ([], [('w', 3, 0, 12)]),
]
W_ITEMS = [it for _, items in P1A_BLOCKS for it in items if it[0] == 'w']
IT_ROWS = TOK * UNROLL
X_CHUNKS = (PRE, PRE + IT_ROWS, PRE + 3 * IT_ROWS, S)
LN_SLOTS = ((0, 11), (1, 5))
MOD_SLOTS = ((0, 2), (0, 4), (0, 6), (1, 8), (1, 9), (1, 10), (1, 11), (2, 0))
NX0 = 4

SEM_C = 0
SEM_X0 = 1
SEM_MOD = SEM_X0 + NX0
SEM_WA = SEM_MOD + NQ + 2
SEM_WB = SEM_WA + len(W_ITEMS)
SEM_XC = SEM_WB + 6
SEM_WO = SEM_XC + 3
SEM_W1 = SEM_WO + 1
SEM_W2 = SEM_W1 + 1
SEM_OUT = SEM_W2 + 1
NSEM = SEM_OUT + 1


def _ln(x):
    m = jnp.mean(x, axis=-1, keepdims=True)
    xc = x - m
    v = jnp.mean(xc * xc, axis=-1, keepdims=True)
    return xc * lax.rsqrt(v + LN_EPS)


def _bf(w32):
    return pltpu.bitcast(w32, BF16)


def _dot(a, b):
    return jnp.dot(a, b, preferred_element_type=F32)


def _lhs_combos(a11, a12, a21, a22):
    return [a11 - a22, a21 - a22, a11, a22, a12 - a11, a21 - a11, a12 - a22]


def _rhs_combos(b11, b12, b21, b22):
    return [b11 - b22, b11, b12 + b22, b21 + b11, b22, b11 + b12, b21 + b22]


_LHS_TERMS = {0: ((0, 0), (1, 1), -1), 1: ((1, 0), (1, 1), -1), 2: ((0, 0), None, 0), 3: ((1, 1), None, 0),
              4: ((0, 1), (0, 0), -1), 5: ((1, 0), (0, 0), -1), 6: ((0, 1), (1, 1), -1)}
_RHS_TERMS = {0: ((0, 0), (1, 1), -1), 1: ((0, 0), None, 0), 2: ((0, 1), (1, 1), 1), 3: ((1, 0), (0, 0), 1),
              4: ((1, 1), None, 0), 5: ((0, 0), (0, 1), 1), 6: ((1, 0), (1, 1), 1)}
_SWAP = {c: int(c in (2, 4, 5, 6)) for c in range(7)}


def _combo(terms, c, blk):
    p, q, sign = terms[c]
    if q is None:
        return blk(*p)
    return blk(*p) + blk(*q) if sign > 0 else blk(*p) - blk(*q)


def _rhs_operand(c, blk):
    p, q, sign = _RHS_TERMS[c]
    a = _bf(blk(*p))
    if q is None:
        return a
    a = a.astype(F32)
    b = _bf(blk(*q)).astype(F32)
    return (a + b if sign > 0 else a - b).astype(BF16)


def _strassen(prod, finish):
    m1 = prod(1)
    m3 = prod(3)
    finish(m1 + m3, 1, 0)
    m2 = prod(2)
    m4 = prod(4)
    finish(m2 + m4, 0, 1)
    m0 = prod(0)
    m5 = prod(5)
    finish((m2 - m1) + m0 + m5, 1, 1)
    m6 = prod(6)
    finish((m3 - m4) + m0 + m6, 0, 0)


def _strassen_value(prod2, c):
    r = {}
    _strassen(functools.partial(prod2, c), lambda y, rh, ch: r.__setitem__((rh, ch ^ _SWAP[c]), y))
    return jnp.concatenate([jnp.concatenate([r[0, 0], r[0, 1]], axis=1),
                            jnp.concatenate([r[1, 0], r[1, 1]], axis=1)], axis=0)


_ORDER = (1, 3, 2, 4, 0, 5, 6)

_PAIRS = [(c, d) for c in range(7) for d in range(7) if not (c in (1, 4) and d in (1, 4))]


def _plain_block(c, d):
    return 2 * (c // 4) + d // 4, 2 * (c // 4) + ((d // 4) ^ _SWAP[c])


def _kernel(x_hbm, mem0_hbm, wq_hbm, wk_hbm, wv_hbm, wo_hbm, w1_hbm, b1_hbm, w2_hbm, b2_hbm,
            c_hbm, wmod_hbm, out_hbm,
            xs, wqkv, wo, w1, w2, qka, qkb, vring, oring, ha, hn, memb, moda, modb, scb, colb, slab, biasb,
            fillb, accb, zerob, wx, hb2, pk0, pk1, pk2, pk3, mem0_ref, b1_ref, b2_ref, c_ref, sem):
    qkv_hbm = [r.bitcast(U32) for r in (wq_hbm, wk_hbm, wv_hbm)]
    x32 = x_hbm.bitcast(U32)
    wo32 = wo_hbm.bitcast(U32)
    wmod32 = wmod_hbm.bitcast(F32)

    def wma(qq, k):
        return pl.ds(512 * (qq // 2), 512), pl.ds(512 * (qq % 2) + k * KQ, KQ)

    def hb_idx(c, q0, nq, row0=0, nrows=PRE // 4):
        return pl.ds(1024 + 128 * (c // 2) + row0, nrows), pl.ds(512 * (c % 2) + 128 * q0, 128 * nq)

    def units_start(lo, hi, rows, sem_idx):
        for u in range(lo, hi):
            j, m = u // 3, u % 3
            for p in range(2):
                pltpu.make_async_copy(qkv_hbm[m].at[rows, p, j, :], wqkv.at[2 * u + p, rows, :],
                                      sem.at[sem_idx]).start()

    def units_wait(lo, n, rows, sem_idx):
        blk = wqkv.at[pl.ds(2 * lo, 2 * n), rows, :]
        pltpu.make_async_copy(blk, blk, sem.at[sem_idx]).wait()

    def item_start(item):
        if item[0] == 'm':
            qq = item[1]
            for k in range(2):
                pltpu.make_async_copy(wmod32.at[:, pl.ds(k * D + qq * KQ, KQ)], ha.at[wma(qq, k)],
                                      sem.at[SEM_MOD + qq]).start()
        elif item[0] == 'w':
            _, qq, lo, hi = item
            units_start(lo, hi, pl.ds(qq * (KQ // 2), KQ // 2), SEM_WA + W_ITEMS.index(item))
        else:
            whole_start(item[1])

    def item_wait(item):
        if item[0] == 'm':
            qq = item[1]
            blk = ha.at[pl.ds(512 * (qq // 2), 512), pl.ds(512 * (qq % 2), 512)]
            pltpu.make_async_copy(blk, blk, sem.at[SEM_MOD + qq]).wait()
        else:
            _, qq, lo, hi = item
            units_wait(lo, hi - lo, pl.ds(qq * (KQ // 2), KQ // 2), SEM_WA + W_ITEMS.index(item))

    def whole_start(i):
        if i == 2:
            xc_copy(0).start()
        units_start(6 * i, 6 * i + 6, pl.ds(0, D // 2), SEM_WB + i - 2)

    def slab_copies(it):
        return [pltpu.make_async_copy(
            wmod32.at[:, pl.ds(pl.multiple_of(2 * D + it * 256 + t * 128, 128), 128)],
            slab.at[it & 1, t], sem.at[SEM_MOD + NQ + (it & 1)]) for t in range(2)]

    def x0_copy(i):
        n = PRE // 2 // NX0
        rows = pl.ds(pl.multiple_of(i * n, n), n)
        return pltpu.make_async_copy(x32.at[rows], xs.at[rows], sem.at[SEM_X0 + i])

    def xc_copy(i):
        rows = pl.ds(X_CHUNKS[i] // 2, (X_CHUNKS[i + 1] - X_CHUNKS[i]) // 2)
        return pltpu.make_async_copy(x32.at[rows], xs.at[rows], sem.at[SEM_XC + i])

    def wo_copy(n):
        return pltpu.make_async_copy(wo32.at[:, pl.ds(n * 128, 128)], wo.at[n], sem.at[SEM_WO])

    w1_copy = pltpu.make_async_copy(w1_hbm.bitcast(U32), w1, sem.at[SEM_W1])
    w2_copy = pltpu.make_async_copy(w2_hbm.bitcast(U32), w2, sem.at[SEM_W2])
    small_copies = [pltpu.make_async_copy(a, b, sem.at[SEM_C])
                    for a, b in ((c_hbm, c_ref), (mem0_hbm, mem0_ref), (b1_hbm, b1_ref),
                                 (b2_hbm, b2_ref))]

    def deinterleave(u, row0, nrows):
        for k in range(nrows // 64):
            rows = pl.ds(row0 + k * 64, 64)
            a = wqkv[2 * u, rows, :]
            b = wqkv[2 * u + 1, rows, :]
            wqkv[2 * u, rows, :] = (a & jnp.uint32(0xFFFF)) | (b << 16)
            wqkv[2 * u + 1, rows, :] = (a >> 16) | (b & jnp.uint32(0xFFFF0000))

    def load_x16(row2):
        return _bf(xs[pl.ds(row2, 8), :]).astype(F32)

    pks = [pk0, pk1, pk2, pk3]

    def pack(v, dtype=U32):
        rows = pl.ds(0, v.shape[0] // 2)
        pk = pks[0]
        pk[rows, pl.ds(0, 128)] = pltpu.bitcast(v.astype(BF16), U32)
        return pltpu.bitcast(pk[rows, pl.ds(0, 128)], dtype)

    def after(y, bits, t=0):
        if not bits:
            return y
        top = [y[0:8, u * 128:(u + 1) * 128] for u in range(y.shape[1] // 128)]
        top[t] = pltpu.bitcast(pltpu.bitcast(top[t], U32)
                               | (functools.reduce(jnp.bitwise_or, bits) & zerob[...]), F32)
        return jnp.concatenate([jnp.concatenate(top, axis=1), y[8:]], axis=0)

    def rep(v8, n):
        return jnp.concatenate([v8] * (n // 8), axis=0)

    def mrow(k, n):
        if k < 2:
            return rep(jnp.concatenate([moda[qq, k] for qq in range(NQ)], axis=1), n)
        return rep(jnp.concatenate([modb[4 * (k - 2) + q] for q in range(4)], axis=1), n)

    for cp in small_copies:
        cp.start()
    for i in range(NX0):
        x0_copy(i).start()
    for item in FIRST_STARTS:
        item_start(item)

    def start_rest():
        xc_copy(1).start()
        for n in range(8):
            wo_copy(n).start()
        for cp in slab_copies(0):
            cp.start()
        xc_copy(2).start()
        w1_copy.start()
        w2_copy.start()

    r = lax.broadcasted_iota(jnp.int32, (80, 128), 0)
    q = lax.broadcasted_iota(jnp.int32, (80, 128), 1)
    r_tok = r < 64
    q_tok = q < 64
    r_head = jnp.where(r_tok, r >> 5, (r - 64) >> 3)
    q_head = jnp.where(q_tok, q >> 5, (q - 64) >> 3)
    same = (r_head == q_head) & (q < 80)
    causal_ok = jnp.logical_not(r_tok & q_tok & ((q & 31) > (r & 31)))
    scale = E ** (-0.5)
    fillb[...] = jnp.where(same, jnp.where(causal_ok, 0.0, -1e9 / scale), -jnp.inf).astype(F32)
    zerob[...] = jnp.zeros((8, 128), U32)

    for cp in small_copies:
        cp.wait()
    cf = c_ref[...].astype(F32)
    sc = (cf * jax.nn.sigmoid(cf)).astype(BF16)
    scb[...] = pltpu.bitcast(jnp.broadcast_to(sc, (16, D)), U32)
    scf = jnp.broadcast_to(sc.astype(F32), (128, D))
    for k in range(8):
        colb[pl.ds(k * 64, 64), :] = pltpu.bitcast(scf[:, k * 128:(k + 1) * 128].T.astype(BF16), U32)
    memb[...] = mem0_ref[...].astype(F32)
    biasb[:, pl.ds(0, FF)] = jnp.broadcast_to(b1_ref[...].astype(F32).reshape(1, FF), (8, FF))
    biasb[:, pl.ds(FF, D)] = jnp.broadcast_to(b2_ref[...].astype(F32).reshape(1, D), (8, D))

    def pre_norm(i, carry):
        x0_copy(i).wait()
        nr = PRE // NX0
        for z in range(nr // 16):
            xn = _ln(load_x16(pl.multiple_of(i * (nr // 2) + z * 8, 8)))
            for n in range(8):
                oring[n, pl.ds(pl.multiple_of(i * nr + z * 16, 16), 16), :] = xn[:, n * 128:(n + 1) * 128]
        return carry

    with jax.named_scope("p0_ln"):
        lax.fori_loop(0, NX0, pre_norm, 0)

    def dst_slot(i, k, p):
        cls, m = k // 3, k % 3
        if m == 2:
            return vring, 4 * i + 2 * cls + p
        return (qka, qkb)[cls], 4 * i + 2 * m + p

    PH = PRE // 2
    assert KQ == 256

    def item_run(item):
        if item[0] == 'm':
            qq = item[1]
            sc16 = _bf(scb[...])
            ca1 = 1.0 + _dot(sc16, _bf(ha[wma(qq, 1)]))[0:8].astype(BF16).astype(F32)
            sa = _dot(sc16, _bf(ha[wma(qq, 0)]))[0:8].astype(BF16).astype(F32)
            moda[qq, 0] = sa
            moda[qq, 1] = ca1
            for z in range(PH // 32):
                def h_blk(rh, kh):
                    cols = slice(kh * 128, (kh + 1) * 128)
                    return (oring[2 * qq + kh, pl.ds(rh * PH + z * 32, 32), :] * rep(ca1[:, cols], 32)
                            + rep(sa[:, cols], 32))

                for c, v in enumerate(_lhs_combos(h_blk(0, 0), h_blk(0, 1), h_blk(1, 0), h_blk(1, 1))):
                    ha[hb_idx(c, qq, 1, z * 16, 16)] = pltpu.bitcast(v.astype(BF16), F32)
            return
        _, qq, lo, hi = item
        if lo == 0 and qq >= 2:
            a_jobs.extend(functools.partial(lhs0_job, k, qq - 2, c) for k in range(PQ // 16) for c in range(7))
        for u in range(lo, hi):
            deinterleave(u, qq * (KQ // 2), KQ // 2)
            i, k = u // 6, u % 6

            def prod(c):
                lhs = pltpu.bitcast(ha[hb_idx(c, qq, 1)], U32)
                if u >= 2:
                    lhs = tie_rows(lhs, a_jobs, (1 + 4 * ((7 * u + _ORDER.index(c)) % 4),))
                rhs = _rhs_operand(c, lambda a, b: wqkv[2 * u + b, pl.ds((2 * qq + a) * 64, 64), :])
                return _dot(_bf(lhs), rhs)

            def finish(y, rh, ch):
                ref, idx = dst_slot(i, k, ch)
                rows = pl.ds(RING - PRE + rh * PH, PH)
                if qq > 0:
                    y = y + ref[idx, rows, :]
                ref[idx, rows, :] = y

            _strassen(prod, finish)

    def tie_rows(w, jobs, groups):
        if not jobs:
            return w
        parts = [w[8 * g:8 * g + 8, 0:128] for g in range(w.shape[0] // 8)]
        for g in groups:
            if jobs:
                parts[g] = parts[g] | (jobs.pop(0)() & zerob[...])
        first = jnp.concatenate(parts, axis=0)
        return first if w.shape[1] == 128 else jnp.concatenate([first, w[:, 128:]], axis=1)

    PQ = PRE // 4
    a_jobs = []

    def lhs0_idx(c, d, k, nk, t, nt):
        e = 7 * c + d
        return pl.ds(64 * (e // 4) + 8 * k, 8 * nk), pl.ds(256 * (e % 4) + 128 * t, 128 * nt)

    def lhs0_job(k, t, c):
        def sub(ri, ki):
            def blk(ro, ko):
                n = 2 * ko + ki + 4 * t
                cols = pl.ds((n % 2) * 128, 128)
                return (oring[n, pl.ds((2 * ro + ri) * PQ + 16 * k, 16), :] * rep(moda[n // 2, 1, :, cols], 16)
                        + rep(moda[n // 2, 0, :, cols], 16))

            return _combo(_LHS_TERMS, c, blk)

        bits = None
        for d, v in enumerate(_lhs_combos(sub(0, 0), sub(0, 1), sub(1, 0), sub(1, 1))):
            hb2[lhs0_idx(c, d, k, 1, t, 1)] = pltpu.bitcast(v.astype(BF16), U32)
            if d in TIE_L:
                b = pltpu.bitcast(v[8 * (d % 2):8 * (d % 2) + 8], U32)
                bits = b if bits is None else bits | b
        return bits

    def ln1_piece(row2):
        h16 = _ln(load_x16(PRE // 2 + row2)) * mrow(1, 16) + mrow(0, 16)
        hn[pl.ds(pl.multiple_of(2 * row2, 16), 16), :] = h16
        return pltpu.bitcast(h16[8:16, D - 128:], U32)

    def phase1b(i, carry):
        @pl.when(i == 3)
        def _():
            whole_start(6)
            whole_start(7)
            start_rest()

        units_wait(6 * i, 6, pl.ds(0, D // 2), SEM_WB + i - 2)
        ln1_piece(pl.multiple_of((i - 2) * 8, 8))

        def raw(m, kq, nq, g):
            u = 6 * i + m + 3 * (nq // 2)
            return wqkv[2 * u + nq % 2, pl.ds((kq + 4 * (g // 8)) * 64 + 8 * (g % 8), 8), :]

        ops = {}

        def rhs0_job(m, c, g):
            def sub(ki, ni):
                return _combo(_RHS_TERMS, c,
                              lambda ko, no: _bf(raw(m, 2 * ko + ki, 2 * no + (ni ^ _SWAP[c]), g)).astype(F32))

            bits = None
            for d, v in enumerate(_rhs_combos(sub(0, 0), sub(0, 1), sub(1, 0), sub(1, 1))):
                if (c, d) in _PAIRS:
                    ops[m, c, d, g] = pack(v)
                    if d in TIE_R0:
                        bits = ops[m, c, d, g] if bits is None else bits | ops[m, c, d, g]
            return bits

        seq = [(m, c) for m in range(3) for c in _ORDER]
        jobs = []
        count = [0]
        deinterleave(6 * i, 0, D // 2)
        deinterleave(6 * i + 3, 0, D // 2)
        for g in range(16):
            rhs0_job(*seq[0], g)
        for m in range(3):
            if m < 2:
                deinterleave(6 * i + m + 1, 0, D // 2)
                deinterleave(6 * i + m + 4, 0, D // 2)

            def prod(c, d):
                if (c, d) in _PAIRS:
                    rhs = [ops[m, c, d, g] for g in range(16)]
                else:
                    rhs = [raw(m, *_plain_block(c, d), g) for g in range(16)]
                lhs = tie_rows(hb2[lhs0_idx(c, d, 0, 8, 0, 2)], jobs, ((0, 3, 6), (1, 4, 7))[count[0] % 2])
                count[0] += 1
                return _dot(_bf(lhs), _bf(jnp.concatenate(rhs, axis=0)))

            def outer(c):
                assert not jobs
                count[0] = 0
                nx = seq.index((m, c)) + 1
                if nx < len(seq):
                    jobs.extend(functools.partial(rhs0_job, *seq[nx], g) for g in range(16))
                return _strassen_value(prod, c)

            def finish(y, rh, ch):
                for ci in range(2):
                    ref, idx = dst_slot(i, m + 3 * ch, ci)
                    ref[idx, pl.ds(RING - PRE + rh * PH, PH), :] = y[:, ci * 128:(ci + 1) * 128]

            _strassen(outer, finish)
        return carry

    for bi, (starts, items) in enumerate(P1A_BLOCKS):
        for item in starts:
            item_start(item)
        with jax.named_scope("p1a_wait%d" % bi):
            for item in items:
                item_wait(item)
        for item in items:
            item_run(item)
    assert not a_jobs
    xc_copy(0).wait()
    with jax.named_scope("p1b"):
        lax.fori_loop(2, 8, phase1b, 0)
    pks.pop(0)
    xc_copy(1).wait()
    for n in range(8):
        wo_copy(n).wait()

    cexp = scale * math.log2(math.e)
    NG = NP // 2
    grp = [(4 * (g // 2) + (g % 2), 4 * (g // 2) + (g % 2) + 2) for g in range(NG)]
    early = [2 * j + u for g in range(NG - 3) for j in grp[g] for u in range(2)]
    late = [h for h in range(H) if h not in early]

    def step(it, k, side_jobs):
        s = it * UNROLL + k
        split = k > 0
        base = TOK * UNROLL * it
        w0 = pl.multiple_of(lax.rem(base, RING), 32) + TOK * k
        r0 = pl.multiple_of(lax.rem(SEG * s + (RING - PRE), RING), 32)
        ow = pl.multiple_of(lax.rem(SEG * s + OOFF, RING), 32)
        o0 = pl.multiple_of(lax.rem(base + OOFF, RING), 32) + TOK * k
        a0 = pl.multiple_of(base, 32) + TOK * k
        X = jnp.concatenate([hn[pl.ds(a0, TOK), :], memb[...]], axis=0).astype(BF16)
        ym = [None] * 96
        probs = [None] * NP
        om = [None] * H
        order = (4, 5, 0, 1, 2, 3)

        if split:
            for t in order:
                accb[t] = _dot(X[:, :D // 2], _bf(wqkv[t, pl.ds(0, D // 4), :]))

        def slot(j, t):
            if t >= 4:
                return vring, 2 * j + t - 4
            return (qka, qkb)[j % 2], 4 * (j // 2) + t

        def proj(j, t, job):
            c = 6 * j + t
            bits = [] if job is None else [job()]
            if split and j == 0:
                y = accb[t] + _dot(X[:, D // 2:], _bf(wqkv[c, pl.ds(D // 4, D // 4), :]))
            else:
                y = _dot(X, _bf(wqkv[c]))
            ref, k = slot(j, t)
            ref[k, pl.ds(w0, TOK), :] = after(y, bits)[0:TOK]
            ym[c] = y[TOK:TOK + M]

        def gather(j, m, pad):
            c = 6 * j + 2 * m
            ref, k = slot(j, 2 * m)
            parts = [ref[k, pl.ds(r0, SEG), :], ref[k + 1, pl.ds(r0, SEG), :], ym[c], ym[c + 1]]
            if pad:
                parts.append(jnp.zeros((48, E), F32))
            return jnp.concatenate(parts, axis=0).astype(BF16)

        def scores(j):
            sc_ = lax.dot_general(gather(j, 0, False), gather(j, 1, True),
                                  (((1,), (1,)), ((), ())), preferred_element_type=F32)
            fill = fillb[...]
            sc_ = jnp.where(fill == 0.0, sc_, fill)
            mx = jnp.max(sc_, axis=-1, keepdims=True)
            p = jnp.exp2((sc_ - mx) * cexp)
            l = jnp.sum(p, axis=-1, keepdims=True)
            rl = pl.reciprocal(l, approx=True)
            rl = rl * (2.0 - l * rl)
            probs[j] = p * rl

        def park(j):
            vring[H, pl.ds(40 * (j % 8), 40), :] = pack(probs[j], F32)
            probs[j] = None

        def pv(j):
            if probs[j] is None:
                P = _bf(vring[H, pl.ds(40 * (j % 8), 40), :])
            else:
                P = probs[j].astype(BF16)
            o = _dot(P, gather(j, 2, True))
            oring[2 * j, pl.ds(ow, SEG), :] = o[0:32]
            oring[2 * j + 1, pl.ds(ow, SEG), :] = o[32:64]
            om[2 * j] = o[64:72]
            om[2 * j + 1] = o[72:80]

        def o_lhs(hs):
            return jnp.concatenate(
                [jnp.concatenate([oring[h, pl.ds(o0, TOK), :], om[h]], axis=0) for h in hs],
                axis=1).astype(BF16)

        def o_rhs(n, hs):
            return _bf(jnp.concatenate([wo[n, pl.ds(h * 64, 64), :] for h in hs], axis=0))

        for g in range(NG):
            cols = [(j, t) for j in grp[g] for t in order]
            if g == 2:
                cols = ([(j, t) for j in grp[g] for t in (4, 5)]
                        + [(j, t) for j in grp[g] for t in range(4)])
            for j in (grp[0] + grp[1] if g == 3 else grp[g - 2] if g >= 4 else ()):
                park(j)
            for ci, (j, t) in enumerate(cols):
                if g == 2 and ci == 4:
                    for jj in grp[0] + grp[1]:
                        scores(jj)
                if g >= 3 and ci == ATT_COL:
                    for jj in grp[g - 1]:
                        scores(jj)
                    for jj in grp[g - 3]:
                        pv(jj)
                proj(j, t, side_jobs.get((g, ci)))
        lo = o_lhs(early)
        for n in range(8):
            accb[n] = _dot(lo, o_rhs(n, early))
            if n == ATT_N1:
                for jj in grp[NG - 1]:
                    scores(jj)
                for jj in grp[NG - 3]:
                    pv(jj)
            if n == ATT_N2:
                for jj in grp[NG - 2] + grp[NG - 1]:
                    pv(jj)
        lo = o_lhs(late)
        for n in range(8):
            a = accb[n] + _dot(lo, o_rhs(n, late))
            ha[pl.ds(a0, TOK), pl.ds(n * 128, 128)] = a[0:TOK]
            memb[:, pl.ds(n * 128, 128)] = a[TOK:TOK + M]

    NIT = NSEG // UNROLL

    def lo16(w):
        return pltpu.bitcast(w << 16, F32)

    def hi16(w):
        return pltpu.bitcast(w & jnp.uint32(0xFFFF0000), F32)

    def steps(it, carry):
        @pl.when(it == 1)
        def _():
            xc_copy(2).wait()

        for cp in slab_copies(it):
            cp.wait()
        for cp in slab_copies((it + 1) & (NIT - 1)):
            cp.start()
        acc = [None, None]

        def mod_job(q):
            for kk in range(2 * q, 2 * q + 2):
                cw = colb[pl.ds(kk * 8, 8), :]
                for t in range(2):
                    w = pltpu.bitcast(slab[it & 1, t, pl.ds(kk * 8, 8), :], U32)
                    v = lo16(w) * lo16(cw) + hi16(w) * hi16(cw)
                    acc[t] = v if acc[t] is None else acc[t] + v
            if q < D // 32 - 1:
                return pltpu.bitcast(acc[0], U32) | pltpu.bitcast(acc[1], U32)
            y = jnp.sum(jnp.concatenate(acc, axis=1), axis=0, keepdims=True).astype(BF16).astype(F32)
            y = jnp.broadcast_to(y + jnp.where((it >> 2) == 2, 1.0, 0.0), (8, 256))
            modb[it] = y
            return pltpu.bitcast(y[:, 0:128], U32)

        nxt2 = pl.multiple_of(jnp.minimum(it + 1, NIT - 1) * (IT_ROWS // 2), 16)
        pieces = list(range(IT_ROWS // 16))
        for k in range(UNROLL):
            side_jobs = {pos: functools.partial(mod_job, 8 * k + q) for q, pos in enumerate(MOD_SLOTS)}
            for pos in LN_SLOTS[k % 2:]:
                side_jobs[pos] = functools.partial(ln1_piece, nxt2 + 8 * pieces.pop(0))
            step(it, k, side_jobs)
        assert not pieces
        return carry

    with jax.named_scope("p2_steps"):
        lax.fori_loop(0, NIT, steps, 0)
    for cp in slab_copies(0):
        cp.wait()
    w1_copy.wait()
    w2_copy.wait()

    nb = S // FB
    HB = FB // 2
    QB = FB // 4

    def ln2_piece(hs, blk, off):
        x2 = (load_x16(pl.multiple_of(blk * HB, HB) + off // 2)
              + mrow(2, 16) * ha[pl.ds(pl.multiple_of(blk * FB, FB) + off, 16), :])
        h = _ln(x2) * mrow(4, 16) + mrow(3, 16)
        hs[off] = h
        return pltpu.bitcast(h[8:16, D - 128:], U32)

    def lhs1_loc(c, d):
        e = 7 * c + d
        return 32 * (e // 4), 256 * (e % 4)

    def lhs1_job(hs, k, t, c):
        def sub(ri, ki):
            def blk(ro, ko):
                c0 = (2 * ko + ki) * 256 + t * 128
                return hs[(2 * ro + ri) * QB + 16 * k][:, c0:c0 + 128]

            return _combo(_LHS_TERMS, c, blk)

        bits = None
        for d, v in enumerate(_lhs_combos(sub(0, 0), sub(0, 1), sub(1, 0), sub(1, 1))):
            r0, c0 = lhs1_loc(c, d)
            hn[pl.ds(r0 + 8 * k, 8), pl.ds(c0 + t * 128, 128)] = pltpu.bitcast(
                v.astype(BF16), F32)
            if d in TIE_L:
                b = pltpu.bitcast(v[8 * (d % 2):8 * (d % 2) + 8], U32)
                bits = b if bits is None else bits | b
        return bits

    def make_ln2(blk, plan, jobs):
        state = dict(piece=0, call=0)
        pending, hs = [], {}

        def issue():
            jobs.extend(pending)
            del pending[:]
            bits = []
            for _ in range(plan[state['call']]):
                k, r = state['piece'] // 4, state['piece'] % 4
                bits.append(ln2_piece(hs, blk, r * QB + 16 * k))
                if r == 3:
                    pending.extend(functools.partial(lhs1_job, hs, k, t, c)
                                   for t in range(2) for c in range(7))
                state['piece'] += 1
            state['call'] += 1
            return bits

        assert sum(plan) == FB // 16 and plan[-1] == 0
        return issue

    K1, N1, K2, N2 = D // 8, FF // 4, FF // 8, D // 4

    def rhs1_loc(c, d, n):
        e = _PAIRS.index((c, d)) * 7 + n
        return wqkv, e // 4, K1 * (e % 4)

    rhs2_slots = ([(wqkv, e, 0) for e in range(79, 96)] + [(qkb, e, 0) for e in range(H)]
                  + [(vring, e, 0) for e in range(H + 1)] + [(wx, e, 0) for e in range(8)])

    def rhs2_loc(c, d, n):
        return rhs2_slots[_PAIRS.index((c, d)) * 2 + n]

    def rhs_job(w, kq, nq, loc, n, r, cs):
        cache = {}

        def blk(ko, no, ki, ni):
            key = (2 * ko + ki, 2 * no + ni)
            if key not in cache:
                cache[key] = _bf(w[pl.ds(r + key[0] * kq, 8), pl.ds(n * 128 + key[1] * nq, 128)]).astype(F32)
            return cache[key]

        bits = None
        for c in cs:
            def sub(ki, ni):
                return _combo(_RHS_TERMS, c, lambda ko, no: blk(ko, no, ki, ni ^ _SWAP[c]))

            for d, v in enumerate(_rhs_combos(sub(0, 0), sub(0, 1), sub(1, 0), sub(1, 1))):
                if (c, d) in _PAIRS:
                    ref, idx, row = loc(c, d, n)
                    b = pack(v)
                    ref[idx, pl.ds(row + r, 8), :] = pltpu.bitcast(b, ref.dtype)
                    if d in TIE_R:
                        bits = b if bits is None else bits | b
        return bits

    def rhs_load(w, kq, nq, loc, c, d, n):
        if (c, d) not in _PAIRS:
            qk, qn = _plain_block(c, d)
            return w[pl.ds(qk * kq, kq), pl.ds(qn * nq + n * 128, 128)]
        ref, idx, row = loc(c, d, n)
        return pltpu.bitcast(ref[idx, pl.ds(row, kq), :], U32)

    def make_tie(jobs, credit):
        state = [credit]

        def tie(raw, density):
            if not jobs:
                return raw
            parts = []
            for r in range(0, raw.shape[0], 8):
                v = raw[r:r + 8]
                state[0] += density
                if jobs and state[0] >= 1.0:
                    state[0] -= 1.0
                    v = v | (jobs.pop(0)() & zerob[...])
                parts.append(v)
            return jnp.concatenate(parts, axis=0)

        return tie

    def bulk_o():
        spots = ([(w1, K1, N1, rhs1_loc, n, r) for n in range(7) for r in range(0, K1, 8)]
                 + [(w2, K2, N2, rhs2_loc, n, r) for n in range(2) for r in range(0, K2, 8)])
        ng = len(JOB_GROUPS)
        jobs = [functools.partial(rhs_job, *spots[(e + (len(spots) // ng) * gi) % len(spots)], cs)
                for e in range(len(spots)) for gi, cs in enumerate(JOB_GROUPS)]
        scale_d = (len(jobs) + 56 + 6) / (7 * 64 * sum(P3_WEIGHTS))
        state = dict(credit=-2.0)
        ln2_block0 = make_ln2(0, LN0_PLAN, jobs)

        def tie_lhs(tiles, density):
            tiles = [[t[8 * g:8 * g + 8] for g in range(16)] for t in tiles]
            for w in range(4):
                for g in range(16):
                    state['credit'] += density
                    for extra in range(2):
                        if jobs and state['credit'] >= 1.0:
                            state['credit'] -= 1.0
                            t = tiles[4 * w + (g + 2 * extra) % 4]
                            t[g] = t[g] | (jobs.pop(0)() & zerob[...])
            return _bf(jnp.concatenate([jnp.concatenate(t, axis=0) for t in tiles], axis=1))

        def a_blk(rh, kh):
            return jnp.concatenate([oring[h, pl.ds(rh * 256, 256), :]
                                    for h in range(16 * kh, 16 * kh + 16)], axis=1)

        lhs = [[pack(v[:, 128 * t:128 * t + 128]) for t in range(16)]
               for v in _lhs_combos(a_blk(0, 0), a_blk(0, 1), a_blk(1, 0), a_blk(1, 1))]
        for n in range(4):
            def prod(c):
                bits = ln2_block0()
                return after(_dot(tie_lhs(lhs[c], scale_d * P3_WEIGHTS[n]),
                                  _rhs_operand(c, lambda a, b: wo[n + 4 * b, pl.ds(a * 1024, 1024), :])), bits)

            def finish(y, rh, ch):
                ha[pl.ds(NSEG * TOK + rh * 256, 256), pl.ds((n + 4 * ch) * 128, 128)] = y

            _strassen(prod, finish)
        assert not jobs

    pks.pop(0)
    with jax.named_scope("p3_bulk_o"):
        bulk_o()

    pks.pop(0)
    out32 = out_hbm.bitcast(F32)

    def ffn(i, carry):
        nxt = (i + 1) & (nb - 1)
        half = i >> 2
        srow = pl.multiple_of((i & 3) * HB, HB)

        g = {(c, d): [] for c in range(7) for d in range(7)}
        for n in range(7):
            act = {}

            def prod1(c, d):
                r0, c0 = lhs1_loc(c, d)
                return _dot(_bf(hn[pl.ds(r0, QB // 2), pl.ds(c0, 256)]),
                            _bf(rhs_load(w1, K1, N1, rhs1_loc, c, d, n)))

            def activate(y, rh, ch):
                b1 = jnp.concatenate([biasb[:, pl.ds((2 * ch + ci) * N1 + n * 128, 128)] for ci in range(2)],
                                     axis=1)
                act[rh, ch] = jax.nn.gelu(y + rep(b1, HB), approximate=True)

            _strassen(lambda c: _strassen_value(prod1, c), activate)
            for c in range(7):
                o = _combo(_LHS_TERMS, c, lambda a, b: act[a, b])
                for d, v in enumerate(_lhs_combos(o[:QB, :128], o[:QB, 128:], o[QB:, :128], o[QB:, 128:])):
                    g[c, d].append(v.astype(BF16))

        jobs = []
        tie = make_tie(jobs, 0.0)
        next_block_ln = make_ln2(nxt, LN_PLAN, jobs)

        for n in range(2):
            def prod2(c, d):
                return _dot(jnp.concatenate(g[c, d], axis=1),
                            _bf(tie(rhs_load(w2, K2, N2, rhs2_loc, c, d, n), FFN_DENSITY)))

            def outer(c):
                bits = next_block_ln()
                return after(_strassen_value(prod2, c), bits, _SWAP[c])

            def finish(y, rh, ch):
                for ci in range(2):
                    nn = (2 * ch + ci) * 2 + n
                    cols = pl.ds(nn * 128, 128)
                    mcols = pl.ds((nn % 2) * 128, 128)
                    yy = y[:, ci * 128:(ci + 1) * 128] + rep(biasb[:, pl.ds(FF + nn * 128, 128)], HB)
                    xr = pl.ds(pl.multiple_of(i * HB, HB) + rh * (HB // 2), HB // 2)
                    ar = pl.ds(pl.multiple_of(i * FB, FB) + rh * HB, HB)
                    x2 = _bf(xs[xr, cols]).astype(F32) + rep(modb[nn // 2, :, mcols], HB) * ha[ar, cols]
                    qka[2 * nn + half, pl.ds(srow + rh * (HB // 2), HB // 2), :] = pack(
                        x2 + rep(modb[12 + nn // 2, :, mcols], HB) * yy, F32)
                    if rh == ch:
                        pltpu.make_async_copy(
                            qka.at[2 * nn + half, pl.ds(srow, HB), :],
                            out32.at[pl.ds(pl.multiple_of(i * HB, HB), HB), cols],
                            sem.at[SEM_OUT]).start()

            _strassen(outer, finish)
        assert not jobs
        return carry

    with jax.named_scope("p4_ffn"):
        lax.fori_loop(0, nb, ffn, 0)
    pltpu.make_async_copy(out32, out32, sem.at[SEM_OUT]).wait()


@jax.jit
def pallas_adaLN_cond__memory_aug_recurrent_mem_tr__dense_activation_gelu__prompt_kernel(
    A_x, A_mem0, A_Wq, A_Wk, A_Wv, A_Wo, A_seg_len, B_x, B_w1, B_b1, B_w2, B_b2, c, w_mod,
):
    assert A_x.shape == (1, S, D) and A_Wq.shape == (D, H, E) and A_mem0.shape == (1, M, D)
    any_spec = pl.BlockSpec(memory_space=pl.ANY)
    out = pl.pallas_call(
        _kernel,
        out_shape=jax.ShapeDtypeStruct((S, D), BF16),
        in_specs=[any_spec] * 12,
        out_specs=any_spec,
        scratch_shapes=[
            pltpu.VMEM((S // 2, D), U32),
            pltpu.VMEM((96, D // 2, E), U32),
            pltpu.VMEM((8, H * E // 2, 128), U32),
            pltpu.VMEM((D // 2, FF), U32),
            pltpu.VMEM((FF // 2, D), U32),
            pltpu.VMEM((H, RING, E), F32),
            pltpu.VMEM((H, RING, E), F32),
            pltpu.VMEM((H + 1, RING, E), F32),
            pltpu.VMEM((H, RING, E), F32),
            pltpu.VMEM((S, D), F32),
            pltpu.VMEM((S - PRE, D), F32),
            pltpu.VMEM((M, D), F32),
            pltpu.VMEM((NQ, 2, 8, KQ), F32),
            pltpu.VMEM((16, 8, 256), F32),
            pltpu.VMEM((8, D), U32),
            pltpu.VMEM((D // 2, 128), U32),
            pltpu.VMEM((2, 2, D // 2, 128), F32),
            pltpu.VMEM((8, FF + D), F32),
            pltpu.VMEM((80, 128), F32),
            pltpu.VMEM((8, 32, 128), F32),
            pltpu.VMEM((8, 128), U32),
            pltpu.VMEM((8, FF // 8, 128), U32),
            pltpu.VMEM((13 * 64, D), U32),
            pltpu.VMEM((128, 256), U32),
            pltpu.VMEM((128, 256), U32),
            pltpu.VMEM((128, 256), U32),
            pltpu.VMEM((128, 256), U32),
            pltpu.VMEM((M, D), BF16),
            pltpu.VMEM((FF,), BF16),
            pltpu.VMEM((D,), BF16),
            pltpu.VMEM((1, D), BF16),
            pltpu.SemaphoreType.DMA((NSEM,)),
        ],
        compiler_params=pltpu.CompilerParams(vmem_limit_bytes=127 * 1024 * 1024, disable_bounds_checks=True,
                                             disable_semaphore_checks=True),
    )(
        A_x.reshape(S, D), A_mem0.reshape(M, D),
        A_Wq.reshape(D // 2, 2, H, E), A_Wk.reshape(D // 2, 2, H, E), A_Wv.reshape(D // 2, 2, H, E),
        A_Wo.reshape(H * E, D), B_w1, B_b1, B_w2, B_b2, c, w_mod,
    )
    return out.reshape(1, S, D)
```

```python
import functools
import math

import jax
import jax.numpy as jnp
from jax import lax
import jax.experimental.pallas as pl
import jax.experimental.pallas.tpu as pltpu

F32 = jnp.float32
BF16 = jnp.bfloat16
U32 = jnp.uint32

S = 2048
D = 1024
H = 32
E = 128
M = 8
SEG = 32
NSEG = S // SEG
FF = 3584
NP = H // 2
TOK = 24
PRE = S - NSEG * TOK
RING = 576
OOFF = (-NSEG * TOK) % RING
LN_EPS = 1e-5
FB = 256
UNROLL = 4

ATT_COL, ATT_N1, ATT_N2 = 6, 2, 5
P3_WEIGHTS = (0.78, 1.0, 1.0, 1.0)
JOB_GROUPS = ([1, 3], [4, 2], [0], [5], [6])
LN0_PLAN = (0,) * 8 + (1,) * 16 + (0,) * 4
LN_PLAN = (1, 1, 1, 1, 1, 1, 1, 2, 2, 2, 2, 1, 0, 0)
FFN_DENSITY = 1.0 / 24
TIE_R, TIE_L = (5, 6), (0, 5, 6)

NQ = 4
KQ = D // NQ

FIRST_STARTS = [('m', 0), ('w', 0, 0, 4), ('w', 0, 4, 8), ('m', 1), ('w', 0, 8, 12), ('w', 1, 0, 8), ('m', 2),
                ('w', 1, 8, 12)]
P1A_BLOCKS = [
    ([], [('m', 0)]),
    ([], [('w', 0, 0, 4)]),
    ([], [('w', 0, 4, 8)]),
    ([('w', 2, 0, 8), ('m', 3), ('w', 2, 8, 12)], [('m', 1), ('w', 0, 8, 12)]),
    ([('w', 3, 0, 12)], [('w', 1, 0, 8)]),
    ([('g', 2), ('g', 3)], [('m', 2), ('w', 1, 8, 12)]),
    ([], [('w', 2, 0, 8)]),
    ([('g', 4), ('g', 5)], [('m', 3), ('w', 2, 8, 12)]),
    ([], [('w', 3, 0, 12)]),
]
W_ITEMS = [it for _, items in P1A_BLOCKS for it in items if it[0] == 'w']
IT_ROWS = TOK * UNROLL
X_CHUNKS = (PRE, PRE + IT_ROWS, PRE + 3 * IT_ROWS, S)
LN_SLOTS = ((0, 11), (1, 5))
MOD_SLOTS = ((0, 2), (0, 4), (0, 6), (1, 8), (1, 9), (1, 10), (1, 11), (2, 0))
NX0 = 4

SEM_C = 0
SEM_X0 = 1
SEM_MOD = SEM_X0 + NX0
SEM_WA = SEM_MOD + NQ + 2
SEM_WB = SEM_WA + len(W_ITEMS)
SEM_XC = SEM_WB + 6
SEM_WO = SEM_XC + 3
SEM_W1 = SEM_WO + 1
SEM_W2 = SEM_W1 + 1
SEM_OUT = SEM_W2 + 1
NSEM = SEM_OUT + 1


def _ln(x):
    m = jnp.mean(x, axis=-1, keepdims=True)
    xc = x - m
    v = jnp.mean(xc * xc, axis=-1, keepdims=True)
    return xc * lax.rsqrt(v + LN_EPS)


def _bf(w32):
    return pltpu.bitcast(w32, BF16)


def _as(v, dtype):
    return v if v.dtype == dtype else pltpu.bitcast(v, dtype)


def _dot(a, b):
    return jnp.dot(a, b, preferred_element_type=F32)


def _lhs_combos(a11, a12, a21, a22):
    return [a11 - a22, a21 - a22, a11, a22, a12 - a11, a21 - a11, a12 - a22]


def _rhs_combos(b11, b12, b21, b22):
    return [b11 - b22, b11, b12 + b22, b21 + b11, b22, b11 + b12, b21 + b22]


_LHS_TERMS = {0: ((0, 0), (1, 1), -1), 1: ((1, 0), (1, 1), -1), 2: ((0, 0), None, 0), 3: ((1, 1), None, 0),
              4: ((0, 1), (0, 0), -1), 5: ((1, 0), (0, 0), -1), 6: ((0, 1), (1, 1), -1)}
_RHS_TERMS = {0: ((0, 0), (1, 1), -1), 1: ((0, 0), None, 0), 2: ((0, 1), (1, 1), 1), 3: ((1, 0), (0, 0), 1),
              4: ((1, 1), None, 0), 5: ((0, 0), (0, 1), 1), 6: ((1, 0), (1, 1), 1)}
_SWAP = {c: int(c in (2, 4, 5, 6)) for c in range(7)}


def _combo(terms, c, blk):
    p, q, sign = terms[c]
    if q is None:
        return blk(*p)
    return blk(*p) + blk(*q) if sign > 0 else blk(*p) - blk(*q)


def _rhs_operand(c, blk):
    p, q, sign = _RHS_TERMS[c]
    a = _bf(blk(*p))
    if q is None:
        return a
    a = a.astype(F32)
    b = _bf(blk(*q)).astype(F32)
    return (a + b if sign > 0 else a - b).astype(BF16)


def _strassen(prod, finish):
    m1 = prod(1)
    m3 = prod(3)
    finish(m1 + m3, 1, 0)
    m2 = prod(2)
    m4 = prod(4)
    finish(m2 + m4, 0, 1)
    m0 = prod(0)
    m5 = prod(5)
    finish((m2 - m1) + m0 + m5, 1, 1)
    m6 = prod(6)
    finish((m3 - m4) + m0 + m6, 0, 0)


def _strassen_value(prod2, c):
    r = {}
    _strassen(functools.partial(prod2, c), lambda y, rh, ch: r.__setitem__((rh, ch ^ _SWAP[c]), y))
    return jnp.concatenate([jnp.concatenate([r[0, 0], r[0, 1]], axis=1),
                            jnp.concatenate([r[1, 0], r[1, 1]], axis=1)], axis=0)


_ORDER = (1, 3, 2, 4, 0, 5, 6)

_PAIRS = [(c, d) for c in range(7) for d in range(7) if not (c in (1, 4) and d in (1, 4))]


def _plain_block(c, d):
    return 2 * (c // 4) + d // 4, 2 * (c // 4) + ((d // 4) ^ _SWAP[c])


def _kernel(x_hbm, mem0_hbm, wq_hbm, wk_hbm, wv_hbm, wo_hbm, w1_hbm, b1_hbm, w2_hbm, b2_hbm,
            c_hbm, wmod_hbm, out_hbm,
            xs, wqkv, wo, w1, w2, qka, qkb, vring, oring, ha, hn, memb, moda, modb, scb, colb, slab, biasb,
            fillb, accb, zerob, wx, hb2, pk0, pk1, pk2, pk3, mem0_ref, b1_ref, b2_ref, c_ref, sem):
    qkv_hbm = [r.bitcast(U32) for r in (wq_hbm, wk_hbm, wv_hbm)]
    x32 = x_hbm.bitcast(U32)
    wo32 = wo_hbm.bitcast(U32)
    wmod32 = wmod_hbm.bitcast(F32)

    def wma(qq, k):
        return pl.ds(512 * (qq // 2), 512), pl.ds(512 * (qq % 2) + k * KQ, KQ)

    def hb_idx(c, q0, nq, row0=0, nrows=PRE // 4):
        return pl.ds(1024 + 128 * (c // 2) + row0, nrows), pl.ds(512 * (c % 2) + 128 * q0, 128 * nq)

    def units_start(lo, hi, rows, sem_idx):
        for u in range(lo, hi):
            j, m = u // 3, u % 3
            for p in range(2):
                pltpu.make_async_copy(qkv_hbm[m].at[rows, p, j, :], wqkv.at[2 * u + p, rows, :],
                                      sem.at[sem_idx]).start()

    def units_wait(lo, n, rows, sem_idx):
        blk = wqkv.at[pl.ds(2 * lo, 2 * n), rows, :]
        pltpu.make_async_copy(blk, blk, sem.at[sem_idx]).wait()

    def item_start(item):
        if item[0] == 'm':
            qq = item[1]
            for k in range(2):
                pltpu.make_async_copy(wmod32.at[:, pl.ds(k * D + qq * KQ, KQ)], ha.at[wma(qq, k)],
                                      sem.at[SEM_MOD + qq]).start()
        elif item[0] == 'w':
            _, qq, lo, hi = item
            units_start(lo, hi, pl.ds(qq * (KQ // 2), KQ // 2), SEM_WA + W_ITEMS.index(item))
        else:
            whole_start(item[1])

    def item_wait(item):
        if item[0] == 'm':
            qq = item[1]
            blk = ha.at[pl.ds(512 * (qq // 2), 512), pl.ds(512 * (qq % 2), 512)]
            pltpu.make_async_copy(blk, blk, sem.at[SEM_MOD + qq]).wait()
        else:
            _, qq, lo, hi = item
            units_wait(lo, hi - lo, pl.ds(qq * (KQ // 2), KQ // 2), SEM_WA + W_ITEMS.index(item))

    def whole_start(i):
        if i == 2:
            xc_copy(0).start()
        units_start(6 * i, 6 * i + 6, pl.ds(0, D // 2), SEM_WB + i - 2)

    def slab_copies(it):
        return [pltpu.make_async_copy(
            wmod32.at[:, pl.ds(pl.multiple_of(2 * D + it * 256 + t * 128, 128), 128)],
            slab.at[it & 1, t], sem.at[SEM_MOD + NQ + (it & 1)]) for t in range(2)]

    def x0_copy(i):
        n = PRE // 2 // NX0
        rows = pl.ds(pl.multiple_of(i * n, n), n)
        return pltpu.make_async_copy(x32.at[rows], xs.at[rows], sem.at[SEM_X0 + i])

    def xc_copy(i):
        rows = pl.ds(X_CHUNKS[i] // 2, (X_CHUNKS[i + 1] - X_CHUNKS[i]) // 2)
        return pltpu.make_async_copy(x32.at[rows], xs.at[rows], sem.at[SEM_XC + i])

    def wo_copy(n):
        return pltpu.make_async_copy(wo32.at[:, pl.ds(n * 128, 128)], wo.at[n], sem.at[SEM_WO])

    w1_copy = pltpu.make_async_copy(w1_hbm.bitcast(U32), w1, sem.at[SEM_W1])
    w2_copy = pltpu.make_async_copy(w2_hbm.bitcast(U32), w2, sem.at[SEM_W2])
    small_copies = [pltpu.make_async_copy(a, b, sem.at[SEM_C])
                    for a, b in ((c_hbm, c_ref), (mem0_hbm, mem0_ref), (b1_hbm, b1_ref),
                                 (b2_hbm, b2_ref))]

    def deinterleave(u, row0, nrows):
        for k in range(nrows // 64):
            rows = pl.ds(row0 + k * 64, 64)
            a = wqkv[2 * u, rows, :]
            b = wqkv[2 * u + 1, rows, :]
            wqkv[2 * u, rows, :] = (a & jnp.uint32(0xFFFF)) | (b << 16)
            wqkv[2 * u + 1, rows, :] = (a >> 16) | (b & jnp.uint32(0xFFFF0000))

    def load_x16(row2):
        return _bf(xs[pl.ds(row2, 8), :]).astype(F32)

    pks = [pk0, pk1, pk2, pk3]

    def pack(v, dtype=U32):
        rows = pl.ds(0, v.shape[0] // 2)
        pk = pks[0]
        pk[rows, pl.ds(0, 128)] = pltpu.bitcast(v.astype(BF16), U32)
        return _as(pk[rows, pl.ds(0, 128)], dtype)

    def or_rows(w, ties):
        parts, pos = [], 0
        for g in sorted(ties):
            if 8 * g > pos:
                parts.append(w[pos:8 * g])
            parts.append(w[8 * g:8 * g + 8] | (ties[g] & zerob[...]))
            pos = 8 * g + 8
        if pos == 0:
            return w
        if pos < w.shape[0]:
            parts.append(w[pos:])
        return jnp.concatenate(parts, axis=0)

    def rhs_operands(raw, c, cache):
        def quad(ko, no):
            if (ko, no) not in cache:
                cache[ko, no] = _bf(jnp.concatenate(
                    [raw(2 * ko + ki, 2 * no + ni) for ki in range(2) for ni in range(2)], axis=0)).astype(F32)
            return cache[ko, no]

        o = _combo(_RHS_TERMS, c, quad)
        sub = [o[16 * (2 * ki + (ni ^ _SWAP[c])):16 * (2 * ki + (ni ^ _SWAP[c])) + 16]
               for ki in range(2) for ni in range(2)]
        ds = [d for d in range(7) if (c, d) in _PAIRS]
        combos = _rhs_combos(*sub)
        packed = pack(jnp.concatenate([combos[d] for d in ds], axis=0))
        return {d: packed[8 * e:8 * e + 8] for e, d in enumerate(ds)}

    def after(y, bits, t=0):
        if not bits:
            return y
        top = [y[0:8, u * 128:(u + 1) * 128] for u in range(y.shape[1] // 128)]
        top[t] = pltpu.bitcast(pltpu.bitcast(top[t], U32)
                               | (functools.reduce(jnp.bitwise_or, bits) & zerob[...]), F32)
        return jnp.concatenate([jnp.concatenate(top, axis=1), y[8:]], axis=0)

    def rep(v8, n):
        return jnp.concatenate([v8] * (n // 8), axis=0)

    def mrow(k, n):
        if k < 2:
            return rep(jnp.concatenate([moda[qq, k] for qq in range(NQ)], axis=1), n)
        return rep(jnp.concatenate([modb[4 * (k - 2) + q] for q in range(4)], axis=1), n)

    for cp in small_copies:
        cp.start()
    for i in range(NX0):
        x0_copy(i).start()
    for item in FIRST_STARTS:
        item_start(item)

    def start_rest():
        xc_copy(1).start()
        for n in range(8):
            wo_copy(n).start()
        for cp in slab_copies(0):
            cp.start()
        xc_copy(2).start()
        w1_copy.start()
        w2_copy.start()

    r = lax.broadcasted_iota(jnp.int32, (80, 128), 0)
    q = lax.broadcasted_iota(jnp.int32, (80, 128), 1)
    r_tok = r < 64
    q_tok = q < 64
    r_head = jnp.where(r_tok, r >> 5, (r - 64) >> 3)
    q_head = jnp.where(q_tok, q >> 5, (q - 64) >> 3)
    same = (r_head == q_head) & (q < 80)
    causal_ok = jnp.logical_not(r_tok & q_tok & ((q & 31) > (r & 31)))
    scale = E ** (-0.5)
    fillb[...] = jnp.where(same, jnp.where(causal_ok, 0.0, -1e9 / scale), -jnp.inf).astype(F32)
    zerob[...] = jnp.zeros((8, 128), U32)

    for cp in small_copies:
        cp.wait()
    cf = c_ref[...].astype(F32)
    sc = (cf * jax.nn.sigmoid(cf)).astype(BF16)
    scb[...] = pltpu.bitcast(jnp.broadcast_to(sc, (16, D)), U32)
    scf = jnp.broadcast_to(sc.astype(F32), (128, D))
    for k in range(8):
        colb[pl.ds(k * 64, 64), :] = pltpu.bitcast(scf[:, k * 128:(k + 1) * 128].T.astype(BF16), U32)
    memb[...] = mem0_ref[...].astype(F32)
    biasb[:, pl.ds(0, FF)] = jnp.broadcast_to(b1_ref[...].astype(F32).reshape(1, FF), (8, FF))
    biasb[:, pl.ds(FF, D)] = jnp.broadcast_to(b2_ref[...].astype(F32).reshape(1, D), (8, D))

    def pre_norm(i, carry):
        x0_copy(i).wait()
        nr = PRE // NX0
        for z in range(nr // 16):
            xn = _ln(load_x16(pl.multiple_of(i * (nr // 2) + z * 8, 8)))
            for n in range(8):
                oring[n, pl.ds(pl.multiple_of(i * nr + z * 16, 16), 16), :] = xn[:, n * 128:(n + 1) * 128]
        return carry

    with jax.named_scope("p0_ln"):
        lax.fori_loop(0, NX0, pre_norm, 0)

    def dst_slot(i, k, p):
        cls, m = k // 3, k % 3
        if m == 2:
            return vring, 4 * i + 2 * cls + p
        return (qka, qkb)[cls], 4 * i + 2 * m + p

    PH = PRE // 2
    assert KQ == 256

    def item_run(item):
        if item[0] == 'm':
            qq = item[1]
            sc16 = _bf(scb[...])
            ca1 = 1.0 + _dot(sc16, _bf(ha[wma(qq, 1)]))[0:8].astype(BF16).astype(F32)
            sa = _dot(sc16, _bf(ha[wma(qq, 0)]))[0:8].astype(BF16).astype(F32)
            moda[qq, 0] = sa
            moda[qq, 1] = ca1
            for z in range(PH // 32):
                def h_blk(rh, kh):
                    cols = slice(kh * 128, (kh + 1) * 128)
                    return (oring[2 * qq + kh, pl.ds(rh * PH + z * 32, 32), :] * rep(ca1[:, cols], 32)
                            + rep(sa[:, cols], 32))

                for c, v in enumerate(_lhs_combos(h_blk(0, 0), h_blk(0, 1), h_blk(1, 0), h_blk(1, 1))):
                    ha[hb_idx(c, qq, 1, z * 16, 16)] = pltpu.bitcast(v.astype(BF16), F32)
            return
        _, qq, lo, hi = item
        if lo == 0 and qq >= 2:
            a_jobs.extend(functools.partial(lhs0_job, k, qq - 2, c) for k in range(PQ // 16) for c in range(7))
        for u in range(lo, hi):
            deinterleave(u, qq * (KQ // 2), KQ // 2)
            i, k = u // 6, u % 6

            def prod(c):
                lhs = pltpu.bitcast(ha[hb_idx(c, qq, 1)], U32)
                if u >= 2:
                    lhs = tie_rows(lhs, a_jobs, (1 + 4 * ((7 * u + _ORDER.index(c)) % 4),))
                rhs = _rhs_operand(c, lambda a, b: wqkv[2 * u + b, pl.ds((2 * qq + a) * 64, 64), :])
                return _dot(_bf(lhs), rhs)

            def finish(y, rh, ch):
                ref, idx = dst_slot(i, k, ch)
                rows = pl.ds(RING - PRE + rh * PH, PH)
                if qq > 0:
                    y = y + ref[idx, rows, :]
                ref[idx, rows, :] = y

            _strassen(prod, finish)

    def tie_rows(w, jobs, groups):
        if not jobs:
            return w
        ties = {g: jobs.pop(0)() for g in groups if jobs}
        if w.shape[1] == 128:
            return or_rows(w, ties)
        return jnp.concatenate([or_rows(w[:, 0:128], ties), w[:, 128:]], axis=1)

    PQ = PRE // 4
    a_jobs = []

    def lhs0_idx(c, d, k, nk, t, nt):
        e = 7 * c + d
        return pl.ds(64 * (e // 4) + 8 * k, 8 * nk), pl.ds(256 * (e % 4) + 128 * t, 128 * nt)

    def lhs0_job(k, t, c):
        def sub(ri, ki):
            def blk(ro, ko):
                n = 2 * ko + ki + 4 * t
                cols = pl.ds((n % 2) * 128, 128)
                return (oring[n, pl.ds((2 * ro + ri) * PQ + 16 * k, 16), :] * rep(moda[n // 2, 1, :, cols], 16)
                        + rep(moda[n // 2, 0, :, cols], 16))

            return _combo(_LHS_TERMS, c, blk)

        bits = None
        for d, v in enumerate(_lhs_combos(sub(0, 0), sub(0, 1), sub(1, 0), sub(1, 1))):
            hb2[lhs0_idx(c, d, k, 1, t, 1)] = pltpu.bitcast(v.astype(BF16), U32)
            if d in TIE_L:
                b = pltpu.bitcast(v[8 * (d % 2):8 * (d % 2) + 8], U32)
                bits = b if bits is None else bits | b
        return bits

    def ln1_piece(row2):
        h16 = _ln(load_x16(PRE // 2 + row2)) * mrow(1, 16) + mrow(0, 16)
        hn[pl.ds(pl.multiple_of(2 * row2, 16), 16), :] = h16
        return pltpu.bitcast(h16[8:16, D - 128:], U32)

    def phase1b(i, carry):
        @pl.when(i == 3)
        def _():
            whole_start(6)
            whole_start(7)
            start_rest()

        units_wait(6 * i, 6, pl.ds(0, D // 2), SEM_WB + i - 2)
        ln1_piece(pl.multiple_of((i - 2) * 8, 8))

        def raw(m, kq, nq, g):
            u = 6 * i + m + 3 * (nq // 2)
            return wqkv[2 * u + nq % 2, pl.ds((kq + 4 * (g // 8)) * 64 + 8 * (g % 8), 8), :]

        ops = {}

        def rhs0_job(m, c, g):
            out = rhs_operands(lambda kq, nq: raw(m, kq, nq, g), c, {})
            for d, v in out.items():
                ops[m, c, d, g] = v
            return functools.reduce(jnp.bitwise_or, out.values())

        seq = [(m, c) for m in range(3) for c in _ORDER]
        jobs = []
        count = [0]
        deinterleave(6 * i, 0, D // 2)
        deinterleave(6 * i + 3, 0, D // 2)
        for g in range(16):
            rhs0_job(*seq[0], g)
        for m in range(3):
            if m < 2:
                deinterleave(6 * i + m + 1, 0, D // 2)
                deinterleave(6 * i + m + 4, 0, D // 2)

            def prod(c, d):
                if (c, d) in _PAIRS:
                    rhs = [ops[m, c, d, g] for g in range(16)]
                else:
                    rhs = [raw(m, *_plain_block(c, d), g) for g in range(16)]
                lhs = tie_rows(hb2[lhs0_idx(c, d, 0, 8, 0, 2)], jobs, ((0, 3, 6), (1, 4, 7))[count[0] % 2])
                count[0] += 1
                return _dot(_bf(lhs), _bf(jnp.concatenate(rhs, axis=0)))

            def outer(c):
                assert not jobs
                count[0] = 0
                nx = seq.index((m, c)) + 1
                if nx < len(seq):
                    jobs.extend(functools.partial(rhs0_job, *seq[nx], g) for g in range(16))
                return _strassen_value(prod, c)

            def finish(y, rh, ch):
                for ci in range(2):
                    ref, idx = dst_slot(i, m + 3 * ch, ci)
                    ref[idx, pl.ds(RING - PRE + rh * PH, PH), :] = y[:, ci * 128:(ci + 1) * 128]

            _strassen(outer, finish)
        return carry

    for bi, (starts, items) in enumerate(P1A_BLOCKS):
        for item in starts:
            item_start(item)
        with jax.named_scope("p1a_wait%d" % bi):
            for item in items:
                item_wait(item)
        for item in items:
            item_run(item)
    assert not a_jobs
    xc_copy(0).wait()
    with jax.named_scope("p1b"):
        lax.fori_loop(2, 8, phase1b, 0)
    pks.pop(0)
    xc_copy(1).wait()
    for n in range(8):
        wo_copy(n).wait()

    cexp = scale * math.log2(math.e)
    NG = NP // 2
    grp = [(4 * (g // 2) + (g % 2), 4 * (g // 2) + (g % 2) + 2) for g in range(NG)]
    early = [2 * j + u for g in range(NG - 3) for j in grp[g] for u in range(2)]
    late = [h for h in range(H) if h not in early]

    def step(it, k, side_jobs):
        s = it * UNROLL + k
        split = k > 0
        base = TOK * UNROLL * it
        w0 = pl.multiple_of(lax.rem(base, RING), 32) + TOK * k
        r0 = pl.multiple_of(lax.rem(SEG * s + (RING - PRE), RING), 32)
        ow = pl.multiple_of(lax.rem(SEG * s + OOFF, RING), 32)
        o0 = pl.multiple_of(lax.rem(base + OOFF, RING), 32) + TOK * k
        a0 = pl.multiple_of(base, 32) + TOK * k
        X = jnp.concatenate([hn[pl.ds(a0, TOK), :], memb[...]], axis=0).astype(BF16)
        ym = [None] * 96
        probs = [None] * NP
        om = [None] * H
        order = (4, 5, 0, 1, 2, 3)

        if split:
            for t in order:
                accb[t] = _dot(X[:, :D // 2], _bf(wqkv[t, pl.ds(0, D // 4), :]))

        def slot(j, t):
            if t >= 4:
                return vring, 2 * j + t - 4
            return (qka, qkb)[j % 2], 4 * (j // 2) + t

        def proj(j, t, job):
            c = 6 * j + t
            bits = [] if job is None else [job()]
            if split and j == 0:
                y = accb[t] + _dot(X[:, D // 2:], _bf(wqkv[c, pl.ds(D // 4, D // 4), :]))
            else:
                y = _dot(X, _bf(wqkv[c]))
            ref, k = slot(j, t)
            ref[k, pl.ds(w0, TOK), :] = after(y, bits)[0:TOK]
            ym[c] = y[TOK:TOK + M]

        def gather(j, m, pad):
            c = 6 * j + 2 * m
            ref, k = slot(j, 2 * m)
            parts = [ref[k, pl.ds(r0, SEG), :], ref[k + 1, pl.ds(r0, SEG), :], ym[c], ym[c + 1]]
            if pad:
                parts.append(jnp.zeros((48, E), F32))
            return jnp.concatenate(parts, axis=0).astype(BF16)

        def scores(j):
            sc_ = lax.dot_general(gather(j, 0, False), gather(j, 1, True),
                                  (((1,), (1,)), ((), ())), preferred_element_type=F32)
            fill = fillb[...]
            sc_ = jnp.where(fill == 0.0, sc_, fill)
            mx = jnp.max(sc_, axis=-1, keepdims=True)
            p = jnp.exp2((sc_ - mx) * cexp)
            l = jnp.sum(p, axis=-1, keepdims=True)
            rl = pl.reciprocal(l, approx=True)
            rl = rl * (2.0 - l * rl)
            probs[j] = p * rl

        def park(j):
            vring[H, pl.ds(40 * (j % 8), 40), :] = pack(probs[j], F32)
            probs[j] = None

        def pv(j):
            if probs[j] is None:
                P = _bf(vring[H, pl.ds(40 * (j % 8), 40), :])
            else:
                P = probs[j].astype(BF16)
            o = _dot(P, gather(j, 2, True))
            oring[2 * j, pl.ds(ow, SEG), :] = o[0:32]
            oring[2 * j + 1, pl.ds(ow, SEG), :] = o[32:64]
            om[2 * j] = o[64:72]
            om[2 * j + 1] = o[72:80]

        def o_lhs(hs):
            return jnp.concatenate(
                [jnp.concatenate([oring[h, pl.ds(o0, TOK), :], om[h]], axis=0) for h in hs],
                axis=1).astype(BF16)

        def o_rhs(n, hs):
            return _bf(jnp.concatenate([wo[n, pl.ds(h * 64, 64), :] for h in hs], axis=0))

        for g in range(NG):
            cols = [(j, t) for j in grp[g] for t in order]
            if g == 2:
                cols = ([(j, t) for j in grp[g] for t in (4, 5)]
                        + [(j, t) for j in grp[g] for t in range(4)])
            for j in (grp[0] + grp[1] if g == 3 else grp[g - 2] if g >= 4 else ()):
                park(j)
            for ci, (j, t) in enumerate(cols):
                if g == 2 and ci == 4:
                    for jj in grp[0] + grp[1]:
                        scores(jj)
                if g >= 3 and ci == ATT_COL:
                    for jj in grp[g - 1]:
                        scores(jj)
                    for jj in grp[g - 3]:
                        pv(jj)
                proj(j, t, side_jobs.get((g, ci)))
        lo = o_lhs(early)
        for n in range(8):
            accb[n] = _dot(lo, o_rhs(n, early))
            if n == ATT_N1:
                for jj in grp[NG - 1]:
                    scores(jj)
                for jj in grp[NG - 3]:
                    pv(jj)
            if n == ATT_N2:
                for jj in grp[NG - 2] + grp[NG - 1]:
                    pv(jj)
        lo = o_lhs(late)
        for n in range(8):
            a = accb[n] + _dot(lo, o_rhs(n, late))
            ha[pl.ds(a0, TOK), pl.ds(n * 128, 128)] = a[0:TOK]
            memb[:, pl.ds(n * 128, 128)] = a[TOK:TOK + M]

    NIT = NSEG // UNROLL

    def lo16(w):
        return pltpu.bitcast(w << 16, F32)

    def hi16(w):
        return pltpu.bitcast(w & jnp.uint32(0xFFFF0000), F32)

    def steps(it, carry):
        @pl.when(it == 1)
        def _():
            xc_copy(2).wait()

        for cp in slab_copies(it):
            cp.wait()
        for cp in slab_copies((it + 1) & (NIT - 1)):
            cp.start()
        acc = [None, None]

        def mod_job(q):
            for kk in range(2 * q, 2 * q + 2):
                cw = colb[pl.ds(kk * 8, 8), :]
                for t in range(2):
                    w = pltpu.bitcast(slab[it & 1, t, pl.ds(kk * 8, 8), :], U32)
                    v = lo16(w) * lo16(cw) + hi16(w) * hi16(cw)
                    acc[t] = v if acc[t] is None else acc[t] + v
            if q < D // 32 - 1:
                return pltpu.bitcast(acc[0], U32) | pltpu.bitcast(acc[1], U32)
            y = jnp.sum(jnp.concatenate(acc, axis=1), axis=0, keepdims=True).astype(BF16).astype(F32)
            y = jnp.broadcast_to(y + jnp.where((it >> 2) == 2, 1.0, 0.0), (8, 256))
            modb[it] = y
            return pltpu.bitcast(y[:, 0:128], U32)

        nxt2 = pl.multiple_of(jnp.minimum(it + 1, NIT - 1) * (IT_ROWS // 2), 16)
        pieces = list(range(IT_ROWS // 16))
        for k in range(UNROLL):
            side_jobs = {pos: functools.partial(mod_job, 8 * k + q) for q, pos in enumerate(MOD_SLOTS)}
            for pos in LN_SLOTS[k % 2:]:
                side_jobs[pos] = functools.partial(ln1_piece, nxt2 + 8 * pieces.pop(0))
            step(it, k, side_jobs)
        assert not pieces
        return carry

    with jax.named_scope("p2_steps"):
        lax.fori_loop(0, NIT, steps, 0)
    for cp in slab_copies(0):
        cp.wait()
    w1_copy.wait()
    w2_copy.wait()

    nb = S // FB
    HB = FB // 2
    QB = FB // 4

    def ln2_piece(hs, blk, off):
        x2 = (load_x16(pl.multiple_of(blk * HB, HB) + off // 2)
              + mrow(2, 16) * ha[pl.ds(pl.multiple_of(blk * FB, FB) + off, 16), :])
        h = _ln(x2) * mrow(4, 16) + mrow(3, 16)
        hs[off] = h
        return pltpu.bitcast(h[8:16, D - 128:], U32)

    def lhs1_loc(c, d):
        e = 7 * c + d
        return 32 * (e // 4), 256 * (e % 4)

    def lhs1_job(hs, k, t, c):
        def sub(ri, ki):
            def blk(ro, ko):
                c0 = (2 * ko + ki) * 256 + t * 128
                return hs[(2 * ro + ri) * QB + 16 * k][:, c0:c0 + 128]

            return _combo(_LHS_TERMS, c, blk)

        bits = None
        for d, v in enumerate(_lhs_combos(sub(0, 0), sub(0, 1), sub(1, 0), sub(1, 1))):
            r0, c0 = lhs1_loc(c, d)
            hn[pl.ds(r0 + 8 * k, 8), pl.ds(c0 + t * 128, 128)] = pltpu.bitcast(
                v.astype(BF16), F32)
            if d in TIE_L:
                b = pltpu.bitcast(v[8 * (d % 2):8 * (d % 2) + 8], U32)
                bits = b if bits is None else bits | b
        return bits

    def make_ln2(blk, plan, jobs):
        state = dict(piece=0, call=0)
        pending, hs = [], {}

        def issue():
            jobs.extend(pending)
            del pending[:]
            bits = []
            for _ in range(plan[state['call']]):
                k, r = state['piece'] // 4, state['piece'] % 4
                bits.append(ln2_piece(hs, blk, r * QB + 16 * k))
                if r == 3:
                    pending.extend(functools.partial(lhs1_job, hs, k, t, c)
                                   for t in range(2) for c in range(7))
                state['piece'] += 1
            state['call'] += 1
            return bits

        assert sum(plan) == FB // 16 and plan[-1] == 0
        return issue

    K1, N1, K2, N2 = D // 8, FF // 4, FF // 8, D // 4

    def rhs1_loc(c, d, n):
        e = _PAIRS.index((c, d)) * 7 + n
        return wqkv, e // 4, K1 * (e % 4)

    rhs2_slots = ([(wqkv, e, 0) for e in range(79, 96)] + [(qkb, e, 0) for e in range(H)]
                  + [(vring, e, 0) for e in range(H + 1)] + [(wx, e, 0) for e in range(8)])

    def rhs2_loc(c, d, n):
        return rhs2_slots[_PAIRS.index((c, d)) * 2 + n]

    def rhs_job(w, kq, nq, loc, n, r, cs):
        cache, bits = {}, []
        for c in cs:
            out = rhs_operands(lambda a, b: w[pl.ds(r + a * kq, 8), pl.ds(n * 128 + b * nq, 128)], c, cache)
            for d, v in out.items():
                ref, idx, row = loc(c, d, n)
                ref[idx, pl.ds(row + r, 8), :] = _as(v, ref.dtype)
            bits += [out[d] for d in TIE_R]
        return functools.reduce(jnp.bitwise_or, bits)

    def rhs_load(w, kq, nq, loc, c, d, n):
        if (c, d) not in _PAIRS:
            qk, qn = _plain_block(c, d)
            return w[pl.ds(qk * kq, kq), pl.ds(qn * nq + n * 128, 128)]
        ref, idx, row = loc(c, d, n)
        return _as(ref[idx, pl.ds(row, kq), :], U32)

    def make_tie(jobs, credit):
        state = [credit]

        def tie(raw, density):
            if not jobs:
                return raw
            ties = {}
            for g in range(raw.shape[0] // 8):
                state[0] += density
                if jobs and state[0] >= 1.0:
                    state[0] -= 1.0
                    ties[g] = jobs.pop(0)()
            return or_rows(raw, ties)

        return tie

    def bulk_o():
        spots = ([(w1, K1, N1, rhs1_loc, n, r) for n in range(7) for r in range(0, K1, 8)]
                 + [(w2, K2, N2, rhs2_loc, n, r) for n in range(2) for r in range(0, K2, 8)])
        ng = len(JOB_GROUPS)
        jobs = [functools.partial(rhs_job, *spots[(e + (len(spots) // ng) * gi) % len(spots)], cs)
                for e in range(len(spots)) for gi, cs in enumerate(JOB_GROUPS)]
        scale_d = (len(jobs) + 56 + 6) / (7 * 64 * sum(P3_WEIGHTS))
        state = dict(credit=-2.0)
        ln2_block0 = make_ln2(0, LN0_PLAN, jobs)

        def tie_lhs(tiles, density):
            ties = [{} for _ in tiles]
            for w in range(4):
                for g in range(16):
                    state['credit'] += density
                    if jobs and state['credit'] >= 1.0:
                        state['credit'] -= 1.0
                        ties[4 * w + g % 4][g] = jobs.pop(0)()
            return _bf(jnp.concatenate([or_rows(t, z) for t, z in zip(tiles, ties)], axis=1))

        def a_blk(rh, kh):
            return jnp.concatenate([oring[h, pl.ds(rh * 256, 256), :]
                                    for h in range(16 * kh, 16 * kh + 16)], axis=1)

        lhs = [[pack(v[:, 128 * t:128 * t + 128]) for t in range(16)]
               for v in _lhs_combos(a_blk(0, 0), a_blk(0, 1), a_blk(1, 0), a_blk(1, 1))]
        for n in range(4):
            def prod(c):
                bits = ln2_block0()
                return after(_dot(tie_lhs(lhs[c], scale_d * P3_WEIGHTS[n]),
                                  _rhs_operand(c, lambda a, b: wo[n + 4 * b, pl.ds(a * 1024, 1024), :])), bits)

            def finish(y, rh, ch):
                ha[pl.ds(NSEG * TOK + rh * 256, 256), pl.ds((n + 4 * ch) * 128, 128)] = y

            _strassen(prod, finish)
        assert not jobs

    pks.pop(0)
    with jax.named_scope("p3_bulk_o"):
        bulk_o()

    pks.pop(0)
    out32 = out_hbm.bitcast(F32)

    def ffn(i, carry):
        nxt = (i + 1) & (nb - 1)
        half = i >> 2
        srow = pl.multiple_of((i & 3) * HB, HB)

        g = {(c, d): [] for c in range(7) for d in range(7)}
        for n in range(7):
            act = {}

            def prod1(c, d):
                r0, c0 = lhs1_loc(c, d)
                return _dot(_bf(hn[pl.ds(r0, QB // 2), pl.ds(c0, 256)]),
                            _bf(rhs_load(w1, K1, N1, rhs1_loc, c, d, n)))

            def activate(y, rh, ch):
                b1 = jnp.concatenate([biasb[:, pl.ds((2 * ch + ci) * N1 + n * 128, 128)] for ci in range(2)],
                                     axis=1)
                act[rh, ch] = jax.nn.gelu(y + rep(b1, HB), approximate=True)

            _strassen(lambda c: _strassen_value(prod1, c), activate)
            for c in range(7):
                o = _combo(_LHS_TERMS, c, lambda a, b: act[a, b])
                for d, v in enumerate(_lhs_combos(o[:QB, :128], o[:QB, 128:], o[QB:, :128], o[QB:, 128:])):
                    g[c, d].append(v.astype(BF16))

        jobs = []
        tie = make_tie(jobs, 0.0)
        next_block_ln = make_ln2(nxt, LN_PLAN, jobs)

        for n in range(2):
            def prod2(c, d):
                return _dot(jnp.concatenate(g[c, d], axis=1),
                            _bf(tie(rhs_load(w2, K2, N2, rhs2_loc, c, d, n), FFN_DENSITY)))

            def outer(c):
                bits = next_block_ln()
                return after(_strassen_value(prod2, c), bits, _SWAP[c])

            def finish(y, rh, ch):
                for ci in range(2):
                    nn = (2 * ch + ci) * 2 + n
                    cols = pl.ds(nn * 128, 128)
                    mcols = pl.ds((nn % 2) * 128, 128)
                    yy = y[:, ci * 128:(ci + 1) * 128] + rep(biasb[:, pl.ds(FF + nn * 128, 128)], HB)
                    xr = pl.ds(pl.multiple_of(i * HB, HB) + rh * (HB // 2), HB // 2)
                    ar = pl.ds(pl.multiple_of(i * FB, FB) + rh * HB, HB)
                    x2 = _bf(xs[xr, cols]).astype(F32) + rep(modb[nn // 2, :, mcols], HB) * ha[ar, cols]
                    qka[2 * nn + half, pl.ds(srow + rh * (HB // 2), HB // 2), :] = pack(
                        x2 + rep(modb[12 + nn // 2, :, mcols], HB) * yy, F32)
                    if rh == ch:
                        pltpu.make_async_copy(
                            qka.at[2 * nn + half, pl.ds(srow, HB), :],
                            out32.at[pl.ds(pl.multiple_of(i * HB, HB), HB), cols],
                            sem.at[SEM_OUT]).start()

            _strassen(outer, finish)
        assert not jobs
        return carry

    with jax.named_scope("p4_ffn"):
        lax.fori_loop(0, nb, ffn, 0)
    pltpu.make_async_copy(out32, out32, sem.at[SEM_OUT]).wait()


@jax.jit
def pallas_adaLN_cond__memory_aug_recurrent_mem_tr__dense_activation_gelu__prompt_kernel(
    A_x, A_mem0, A_Wq, A_Wk, A_Wv, A_Wo, A_seg_len, B_x, B_w1, B_b1, B_w2, B_b2, c, w_mod,
):
    assert A_x.shape == (1, S, D) and A_Wq.shape == (D, H, E) and A_mem0.shape == (1, M, D)
    any_spec = pl.BlockSpec(memory_space=pl.ANY)
    out = pl.pallas_call(
        _kernel,
        out_shape=jax.ShapeDtypeStruct((S, D), BF16),
        in_specs=[any_spec] * 12,
        out_specs=any_spec,
        scratch_shapes=[
            pltpu.VMEM((S // 2, D), U32),
            pltpu.VMEM((96, D // 2, E), U32),
            pltpu.VMEM((8, H * E // 2, 128), U32),
            pltpu.VMEM((D // 2, FF), U32),
            pltpu.VMEM((FF // 2, D), U32),
            pltpu.VMEM((H, RING, E), F32),
            pltpu.VMEM((H, RING, E), F32),
            pltpu.VMEM((H + 1, RING, E), F32),
            pltpu.VMEM((H, RING, E), F32),
            pltpu.VMEM((S, D), F32),
            pltpu.VMEM((S - PRE, D), F32),
            pltpu.VMEM((M, D), F32),
            pltpu.VMEM((NQ, 2, 8, KQ), F32),
            pltpu.VMEM((16, 8, 256), F32),
            pltpu.VMEM((8, D), U32),
            pltpu.VMEM((D // 2, 128), U32),
            pltpu.VMEM((2, 2, D // 2, 128), F32),
            pltpu.VMEM((8, FF + D), F32),
            pltpu.VMEM((80, 128), F32),
            pltpu.VMEM((8, 32, 128), F32),
            pltpu.VMEM((8, 128), U32),
            pltpu.VMEM((8, FF // 8, 128), U32),
            pltpu.VMEM((13 * 64, D), U32),
            pltpu.VMEM((128, 256), U32),
            pltpu.VMEM((128, 256), U32),
            pltpu.VMEM((128, 256), U32),
            pltpu.VMEM((128, 256), U32),
            pltpu.VMEM((M, D), BF16),
            pltpu.VMEM((FF,), BF16),
            pltpu.VMEM((D,), BF16),
            pltpu.VMEM((1, D), BF16),
            pltpu.SemaphoreType.DMA((NSEM,)),
        ],
        compiler_params=pltpu.CompilerParams(vmem_limit_bytes=127 * 1024 * 1024, disable_bounds_checks=True,
                                             disable_semaphore_checks=True),
    )(
        A_x.reshape(S, D), A_mem0.reshape(M, D),
        A_Wq.reshape(D // 2, 2, H, E), A_Wk.reshape(D // 2, 2, H, E), A_Wv.reshape(D // 2, 2, H, E),
        A_Wo.reshape(H * E, D), B_w1, B_b1, B_w2, B_b2, c, w_mod,
    )
    return out.reshape(1, S, D)
```

```python
import functools
import math

import jax
import jax.numpy as jnp
from jax import lax
import jax.experimental.pallas as pl
import jax.experimental.pallas.tpu as pltpu

F32 = jnp.float32
BF16 = jnp.bfloat16
U32 = jnp.uint32

S = 2048
D = 1024
H = 32
E = 128
M = 8
SEG = 32
NSEG = S // SEG
FF = 3584
NP = H // 2
TOK = 24
PRE = S - NSEG * TOK
RING = 576
OOFF = (-NSEG * TOK) % RING
LN_EPS = 1e-5
FB = 256
UNROLL = 4

ATT_COL, ATT_N1, ATT_N2 = 6, 2, 5
P3_WEIGHTS = (0.70, 1.0, 1.0, 1.0)
JOB_GROUPS = ([1, 3], [4, 2], [0], [5], [6])
LN0_PLAN = (0,) * 8 + (1,) * 16 + (0,) * 4
LN_PLAN = (1, 1, 1, 1, 1, 1, 1, 2, 2, 2, 2, 1, 0, 0)
FFN_DENSITY = 1.0 / 24
HB_SKIP = 6
FIRST_SPOTS = [(), (), (0, 2, 4, 6), (1, 3, 5, 7), (0, 2, 4, 6), (1, 3, 5, 7), ()]
TIE_R, TIE_L = (5, 6), (0, 5, 6)

NQ = 4
KQ = D // NQ

FIRST_STARTS = [('m', 0), ('w', 0, 0, 4), ('w', 0, 4, 8), ('m', 1), ('w', 0, 8, 12), ('w', 1, 0, 8), ('m', 2),
                ('w', 1, 8, 12)]
P1A_BLOCKS = [
    ([], [('m', 0)]),
    ([], [('w', 0, 0, 4)]),
    ([], [('w', 0, 4, 8)]),
    ([('w', 2, 0, 8), ('w', 2, 8, 12), ('m', 3), ('x',)], [('m', 1), ('w', 0, 8, 12)]),
    ([('w', 3, 0, 12)], [('w', 1, 0, 8)]),
    ([('g', 2), ('g', 3)], [('m', 2), ('w', 1, 8, 12)]),
    ([], [('w', 2, 0, 8)]),
    ([('g', 4), ('g', 5)], [('m', 3), ('w', 2, 8, 12)]),
    ([], [('w', 3, 0, 12)]),
]
W_ITEMS = [it for _, items in P1A_BLOCKS for it in items if it[0] == 'w']
IT_ROWS = TOK * UNROLL
X_CHUNKS = (PRE, PRE + IT_ROWS, PRE + 3 * IT_ROWS, S)
LN_SLOTS = ((0, 11), (1, 5))
MOD_SLOTS = ((0, 2), (0, 4), (0, 6), (1, 8), (1, 9), (1, 10), (1, 11), (2, 0))
NX0 = 4

SEM_C = 0
SEM_X0 = 1
SEM_MOD = SEM_X0 + NX0
SEM_WA = SEM_MOD + NQ + 2
SEM_WB = SEM_WA + len(W_ITEMS)
SEM_XC = SEM_WB + 6
SEM_WO = SEM_XC + 3
SEM_W1 = SEM_WO + 1
SEM_W2 = SEM_W1 + 1
SEM_OUT = SEM_W2 + 1
NSEM = SEM_OUT + 1


def _ln(x):
    m = jnp.mean(x, axis=-1, keepdims=True)
    xc = x - m
    v = jnp.mean(xc * xc, axis=-1, keepdims=True)
    return xc * lax.rsqrt(v + LN_EPS)


def _bf(w32):
    return pltpu.bitcast(w32, BF16)


def _as(v, dtype):
    return v if v.dtype == dtype else pltpu.bitcast(v, dtype)


def _dot(a, b):
    return jnp.dot(a, b, preferred_element_type=F32)


def _lhs_combos(a11, a12, a21, a22):
    return [a11 - a22, a21 - a22, a11, a22, a12 - a11, a21 - a11, a12 - a22]


def _rhs_combos(b11, b12, b21, b22):
    return [b11 - b22, b11, b12 + b22, b21 + b11, b22, b11 + b12, b21 + b22]


_LHS_TERMS = {0: ((0, 0), (1, 1), -1), 1: ((1, 0), (1, 1), -1), 2: ((0, 0), None, 0), 3: ((1, 1), None, 0),
              4: ((0, 1), (0, 0), -1), 5: ((1, 0), (0, 0), -1), 6: ((0, 1), (1, 1), -1)}
_RHS_TERMS = {0: ((0, 0), (1, 1), -1), 1: ((0, 0), None, 0), 2: ((0, 1), (1, 1), 1), 3: ((1, 0), (0, 0), 1),
              4: ((1, 1), None, 0), 5: ((0, 0), (0, 1), 1), 6: ((1, 0), (1, 1), 1)}
_SWAP = {c: int(c in (2, 4, 5, 6)) for c in range(7)}


def _combo(terms, c, blk):
    p, q, sign = terms[c]
    if q is None:
        return blk(*p)
    return blk(*p) + blk(*q) if sign > 0 else blk(*p) - blk(*q)


def _rhs_operand(c, blk):
    p, q, sign = _RHS_TERMS[c]
    a = _bf(blk(*p))
    if q is None:
        return a
    a = a.astype(F32)
    b = _bf(blk(*q)).astype(F32)
    return (a + b if sign > 0 else a - b).astype(BF16)


def _strassen(prod, finish):
    m1 = prod(1)
    m3 = prod(3)
    finish(m1 + m3, 1, 0)
    m2 = prod(2)
    m4 = prod(4)
    finish(m2 + m4, 0, 1)
    m0 = prod(0)
    m5 = prod(5)
    finish((m2 - m1) + m0 + m5, 1, 1)
    m6 = prod(6)
    finish((m3 - m4) + m0 + m6, 0, 0)


def _strassen_value(prod2, c):
    r = {}
    _strassen(functools.partial(prod2, c), lambda y, rh, ch: r.__setitem__((rh, ch ^ _SWAP[c]), y))
    return jnp.concatenate([jnp.concatenate([r[0, 0], r[0, 1]], axis=1),
                            jnp.concatenate([r[1, 0], r[1, 1]], axis=1)], axis=0)


_ORDER = (1, 3, 2, 4, 0, 5, 6)

_PAIRS = [(c, d) for c in range(7) for d in range(7) if not (c in (1, 4) and d in (1, 4))]


def _plain_block(c, d):
    return 2 * (c // 4) + d // 4, 2 * (c // 4) + ((d // 4) ^ _SWAP[c])


def _kernel(x_hbm, mem0_hbm, wq_hbm, wk_hbm, wv_hbm, wo_hbm, w1_hbm, b1_hbm, w2_hbm, b2_hbm,
            c_hbm, wmod_hbm, out_hbm,
            xs, wqkv, wo, w1, w2, qka, qkb, vring, oring, ha, hn, memb, moda, modb, scb, colb, slab, biasb,
            fillb, accb, accp, zerob, wx, hb2, pk0, pk1, pk2, pk3, mem0_ref, b1_ref, b2_ref, c_ref, sem):
    qkv_hbm = [r.bitcast(U32) for r in (wq_hbm, wk_hbm, wv_hbm)]
    x32 = x_hbm.bitcast(U32)
    wo32 = wo_hbm.bitcast(U32)
    wmod32 = wmod_hbm.bitcast(F32)

    def wma(qq, k):
        return pl.ds(512 * (qq // 2), 512), pl.ds(512 * (qq % 2) + k * KQ, KQ)

    def hb_idx(c, q0, nq, row0=0, nrows=PRE // 4):
        return pl.ds(1024 + 128 * (c // 2) + row0, nrows), pl.ds(512 * (c % 2) + 128 * q0, 128 * nq)

    def units_start(lo, hi, rows, sem_idx):
        for u in range(lo, hi):
            j, m = u // 3, u % 3
            for p in range(2):
                pltpu.make_async_copy(qkv_hbm[m].at[rows, p, j, :], wqkv.at[2 * u + p, rows, :],
                                      sem.at[sem_idx]).start()

    def units_wait(lo, n, rows, sem_idx):
        blk = wqkv.at[pl.ds(2 * lo, 2 * n), rows, :]
        pltpu.make_async_copy(blk, blk, sem.at[sem_idx]).wait()

    def item_start(item):
        if item[0] == 'm':
            qq = item[1]
            for k in range(2):
                pltpu.make_async_copy(wmod32.at[:, pl.ds(k * D + qq * KQ, KQ)], ha.at[wma(qq, k)],
                                      sem.at[SEM_MOD + qq]).start()
        elif item[0] == 'w':
            _, qq, lo, hi = item
            units_start(lo, hi, pl.ds(qq * (KQ // 2), KQ // 2), SEM_WA + W_ITEMS.index(item))
        elif item[0] == 'x':
            xc_copy(0).start()
        else:
            whole_start(item[1])

    def item_wait(item):
        if item[0] == 'm':
            qq = item[1]
            blk = ha.at[pl.ds(512 * (qq // 2), 512), pl.ds(512 * (qq % 2), 512)]
            pltpu.make_async_copy(blk, blk, sem.at[SEM_MOD + qq]).wait()
        else:
            _, qq, lo, hi = item
            units_wait(lo, hi - lo, pl.ds(qq * (KQ // 2), KQ // 2), SEM_WA + W_ITEMS.index(item))

    def whole_start(i):
        units_start(6 * i, 6 * i + 6, pl.ds(0, D // 2), SEM_WB + i - 2)

    def slab_copies(it):
        return [pltpu.make_async_copy(
            wmod32.at[:, pl.ds(pl.multiple_of(2 * D + it * 256 + t * 128, 128), 128)],
            slab.at[it & 1, t], sem.at[SEM_MOD + NQ + (it & 1)]) for t in range(2)]

    def x0_copy(i):
        n = PRE // 2 // NX0
        rows = pl.ds(pl.multiple_of(i * n, n), n)
        return pltpu.make_async_copy(x32.at[rows], xs.at[rows], sem.at[SEM_X0 + i])

    def xc_copy(i):
        rows = pl.ds(X_CHUNKS[i] // 2, (X_CHUNKS[i + 1] - X_CHUNKS[i]) // 2)
        return pltpu.make_async_copy(x32.at[rows], xs.at[rows], sem.at[SEM_XC + i])

    def wo_copy(n):
        return pltpu.make_async_copy(wo32.at[:, pl.ds(n * 128, 128)], wo.at[n], sem.at[SEM_WO])

    w1_copy = pltpu.make_async_copy(w1_hbm.bitcast(U32), w1, sem.at[SEM_W1])
    w2_copy = pltpu.make_async_copy(w2_hbm.bitcast(U32), w2, sem.at[SEM_W2])
    small_copies = [pltpu.make_async_copy(a, b, sem.at[SEM_C])
                    for a, b in ((c_hbm, c_ref), (mem0_hbm, mem0_ref), (b1_hbm, b1_ref),
                                 (b2_hbm, b2_ref))]

    def deinterleave(u, row0, nrows):
        for k in range(nrows // 64):
            rows = pl.ds(row0 + k * 64, 64)
            a = wqkv[2 * u, rows, :]
            b = wqkv[2 * u + 1, rows, :]
            wqkv[2 * u, rows, :] = (a & jnp.uint32(0xFFFF)) | (b << 16)
            wqkv[2 * u + 1, rows, :] = (a >> 16) | (b & jnp.uint32(0xFFFF0000))

    def load_x16(row2):
        return _bf(xs[pl.ds(row2, 8), :]).astype(F32)

    pks = [pk0, pk1, pk2, pk3]

    def pack(v, dtype=U32):
        rows = pl.ds(0, v.shape[0] // 2)
        pk = pks[0]
        pk[rows, pl.ds(0, 128)] = pltpu.bitcast(v.astype(BF16), U32)
        return _as(pk[rows, pl.ds(0, 128)], dtype)

    def or_rows(w, ties):
        parts, pos = [], 0
        for g in sorted(ties):
            if 8 * g > pos:
                parts.append(w[pos:8 * g])
            parts.append(w[8 * g:8 * g + 8] | (ties[g] & zerob[...]))
            pos = 8 * g + 8
        if pos == 0:
            return w
        if pos < w.shape[0]:
            parts.append(w[pos:])
        return jnp.concatenate(parts, axis=0)

    def rhs_operands(raw, c, cache):
        def quad(ko, no):
            if (ko, no) not in cache:
                cache[ko, no] = _bf(jnp.concatenate(
                    [raw(2 * ko + ki, 2 * no + ni) for ki in range(2) for ni in range(2)], axis=0)).astype(F32)
            return cache[ko, no]

        o = _combo(_RHS_TERMS, c, quad)
        sub = [o[16 * (2 * ki + (ni ^ _SWAP[c])):16 * (2 * ki + (ni ^ _SWAP[c])) + 16]
               for ki in range(2) for ni in range(2)]
        ds = [d for d in range(7) if (c, d) in _PAIRS]
        combos = _rhs_combos(*sub)
        packed = pack(jnp.concatenate([combos[d] for d in ds], axis=0))
        return {d: packed[8 * e:8 * e + 8] for e, d in enumerate(ds)}

    def after(y, bits, t=0):
        if not bits:
            return y
        top = [y[0:8, u * 128:(u + 1) * 128] for u in range(y.shape[1] // 128)]
        top[t] = pltpu.bitcast(pltpu.bitcast(top[t], U32)
                               | (functools.reduce(jnp.bitwise_or, bits) & zerob[...]), F32)
        return jnp.concatenate([jnp.concatenate(top, axis=1), y[8:]], axis=0)

    def rep(v8, n):
        return jnp.concatenate([v8] * (n // 8), axis=0)

    def mrow(k, n):
        if k < 2:
            return rep(jnp.concatenate([moda[qq, k] for qq in range(NQ)], axis=1), n)
        return rep(jnp.concatenate([modb[4 * (k - 2) + q] for q in range(4)], axis=1), n)

    for cp in small_copies:
        cp.start()
    for i in range(NX0):
        x0_copy(i).start()
    for item in FIRST_STARTS:
        item_start(item)

    def start_rest():
        xc_copy(1).start()
        for n in range(8):
            wo_copy(n).start()
        for cp in slab_copies(0):
            cp.start()
        xc_copy(2).start()
        w1_copy.start()
        w2_copy.start()

    r = lax.broadcasted_iota(jnp.int32, (80, 128), 0)
    q = lax.broadcasted_iota(jnp.int32, (80, 128), 1)
    r_tok = r < 64
    q_tok = q < 64
    r_head = jnp.where(r_tok, r >> 5, (r - 64) >> 3)
    q_head = jnp.where(q_tok, q >> 5, (q - 64) >> 3)
    same = (r_head == q_head) & (q < 80)
    causal_ok = jnp.logical_not(r_tok & q_tok & ((q & 31) > (r & 31)))
    scale = E ** (-0.5)
    fillb[...] = jnp.where(same, jnp.where(causal_ok, 0.0, -1e9 / scale), -jnp.inf).astype(F32)
    zerob[...] = jnp.zeros((8, 128), U32)

    for cp in small_copies:
        cp.wait()
    cf = c_ref[...].astype(F32)
    sc = (cf * jax.nn.sigmoid(cf)).astype(BF16)
    scb[...] = pltpu.bitcast(jnp.broadcast_to(sc, (16, D)), U32)
    scf = jnp.broadcast_to(sc.astype(F32), (128, D))
    for k in range(8):
        colb[pl.ds(k * 64, 64), :] = pltpu.bitcast(scf[:, k * 128:(k + 1) * 128].T.astype(BF16), U32)
    memb[...] = mem0_ref[...].astype(F32)
    biasb[:, pl.ds(0, FF)] = jnp.broadcast_to(b1_ref[...].astype(F32).reshape(1, FF), (8, FF))
    biasb[:, pl.ds(FF, D)] = jnp.broadcast_to(b2_ref[...].astype(F32).reshape(1, D), (8, D))

    def pre_norm(i, carry):
        x0_copy(i).wait()
        nr = PRE // NX0
        for z in range(nr // 16):
            xn = _ln(load_x16(pl.multiple_of(i * (nr // 2) + z * 8, 8)))
            for n in range(8):
                oring[n, pl.ds(pl.multiple_of(i * nr + z * 16, 16), 16), :] = xn[:, n * 128:(n + 1) * 128]
        return carry

    with jax.named_scope("p0_ln"):
        lax.fori_loop(0, NX0, pre_norm, 0)

    def dst_slot(i, k, p):
        cls, m = k // 3, k % 3
        if m == 2:
            return vring, 4 * i + 2 * cls + p
        return (qka, qkb)[cls], 4 * i + 2 * m + p

    PH = PRE // 2
    assert KQ == 256

    def item_run(item):
        if item[0] == 'm':
            qq = item[1]
            sc16 = _bf(scb[...])
            ca1 = 1.0 + _dot(sc16, _bf(ha[wma(qq, 1)]))[0:8].astype(BF16).astype(F32)
            sa = _dot(sc16, _bf(ha[wma(qq, 0)]))[0:8].astype(BF16).astype(F32)
            moda[qq, 0] = sa
            moda[qq, 1] = ca1
            def hb_job(z):
                def h_blk(rh, kh):
                    cols = slice(kh * 128, (kh + 1) * 128)
                    return (oring[2 * qq + kh, pl.ds(rh * PH + z * 16, 16), :] * rep(ca1[:, cols], 16)
                            + rep(sa[:, cols], 16))

                combos = _lhs_combos(h_blk(0, 0), h_blk(0, 1), h_blk(1, 0), h_blk(1, 1))
                for c, v in enumerate(combos):
                    ha[hb_idx(c, qq, 1, z * 8, 8)] = pltpu.bitcast(v.astype(BF16), F32)
                return pltpu.bitcast(combos[5][0:8], U32) | pltpu.bitcast(combos[6][8:16], U32)

            if qq == 0:
                for z in range(PH // 16):
                    hb_job(z)
            else:
                assert not a_jobs
                a_jobs.extend([None] * HB_SKIP + [functools.partial(hb_job, z) for z in range(PH // 16)])
            return
        _, qq, lo, hi = item
        if lo == 0:
            assert not a_jobs
        if lo == 0 and qq >= 2:
            a_jobs.extend(functools.partial(lhs0_job, k, qq - 2, c) for k in range(PQ // 16) for c in range(7))
        for u in range(lo, hi):
            deinterleave(u, qq * (KQ // 2), KQ // 2)
            i, k = u // 6, u % 6

            def prod(c):
                lhs = pltpu.bitcast(ha[hb_idx(c, qq, 1)], U32)
                g0 = 1 + 4 * ((7 * u + _ORDER.index(c)) % 4)
                if u >= 1:
                    lhs = tie_rows(lhs, a_jobs, (g0, (g0 + 8) % 16) if u == 4 else (g0,))
                rhs = _rhs_operand(c, lambda a, b: wqkv[2 * u + b, pl.ds((2 * qq + a) * 64, 64), :])
                return _dot(_bf(lhs), rhs)

            def finish(y, rh, ch):
                ref, idx = dst_slot(i, k, ch)
                rows = pl.ds(RING - PRE + rh * PH, PH)
                if qq > 0:
                    y = y + ref[idx, rows, :]
                ref[idx, rows, :] = y

            _strassen(prod, finish)

    def tie_rows(w, jobs, groups):
        if not jobs:
            return w
        picked = {g: jobs.pop(0) for g in groups if jobs}
        ties = {g: job() for g, job in picked.items() if job is not None}
        if w.shape[1] == 128:
            return or_rows(w, ties)
        return jnp.concatenate([or_rows(w[:, 0:128], ties), w[:, 128:]], axis=1)

    PQ = PRE // 4
    a_jobs = []

    def lhs0_idx(c, d, k, nk, t, nt):
        e = 7 * c + d
        return pl.ds(64 * (e // 4) + 8 * k, 8 * nk), pl.ds(256 * (e % 4) + 128 * t, 128 * nt)

    def lhs0_job(k, t, c):
        def sub(ri, ki):
            def blk(ro, ko):
                n = 2 * ko + ki + 4 * t
                cols = pl.ds((n % 2) * 128, 128)
                return (oring[n, pl.ds((2 * ro + ri) * PQ + 16 * k, 16), :] * rep(moda[n // 2, 1, :, cols], 16)
                        + rep(moda[n // 2, 0, :, cols], 16))

            return _combo(_LHS_TERMS, c, blk)

        bits = None
        for d, v in enumerate(_lhs_combos(sub(0, 0), sub(0, 1), sub(1, 0), sub(1, 1))):
            hb2[lhs0_idx(c, d, k, 1, t, 1)] = pltpu.bitcast(v.astype(BF16), U32)
            if d in TIE_L:
                b = pltpu.bitcast(v[8 * (d % 2):8 * (d % 2) + 8], U32)
                bits = b if bits is None else bits | b
        return bits

    def ln1_piece(row2):
        h16 = _ln(load_x16(PRE // 2 + row2)) * mrow(1, 16) + mrow(0, 16)
        hn[pl.ds(pl.multiple_of(2 * row2, 16), 16), :] = h16
        return pltpu.bitcast(h16[8:16, D - 128:], U32)

    def phase1b(i, carry):
        @pl.when(i == 3)
        def _():
            whole_start(6)
            whole_start(7)
            start_rest()

        units_wait(6 * i, 6, pl.ds(0, D // 2), SEM_WB + i - 2)
        ln1_piece(pl.multiple_of((i - 2) * 8, 8))

        def raw(m, kq, nq, g):
            u = 6 * i + m + 3 * (nq // 2)
            return wqkv[2 * u + nq % 2, pl.ds((kq + 4 * (g // 8)) * 64 + 8 * (g % 8), 8), :]

        ops = {}

        def rhs0_job(m, c, g):
            out = rhs_operands(lambda kq, nq: raw(m, kq, nq, g), c, {})
            for d, v in out.items():
                ops[m, c, d, g] = v
            return functools.reduce(jnp.bitwise_or, out.values())

        seq = [(m, c) for m in range(3) for c in _ORDER]
        jobs = []
        count = [0]
        spots = []
        deinterleave(6 * i, 0, D // 2)
        deinterleave(6 * i + 3, 0, D // 2)
        for g in range(16):
            rhs0_job(*seq[0], g)
        for m in range(3):
            if m < 2:
                deinterleave(6 * i + m + 1, 0, D // 2)
                deinterleave(6 * i + m + 4, 0, D // 2)

            def prod(c, d):
                if (c, d) in _PAIRS:
                    rhs = [ops[m, c, d, g] for g in range(16)]
                else:
                    rhs = [raw(m, *_plain_block(c, d), g) for g in range(16)]
                lhs = tie_rows(hb2[lhs0_idx(c, d, 0, 8, 0, 2)], jobs, spots[count[0] % len(spots)])
                count[0] += 1
                return _dot(_bf(lhs), _bf(jnp.concatenate(rhs, axis=0)))

            def outer(c):
                assert not jobs
                count[0] = 0
                spots[:] = [(0, 3, 6), (1, 4, 7)]
                nx = seq.index((m, c)) + 1
                if nx < len(seq):
                    jobs.extend(functools.partial(rhs0_job, *seq[nx], g) for g in range(16))
                if nx == 1:
                    spots[:] = FIRST_SPOTS
                    pre = {d: prod(c, d) for d in (1, 4)}
                    accp[...] = pre[4]
                    return _strassen_value(
                        lambda c, d: pre[1] if d == 1 else accp[...] if d == 4 else prod(c, d), c)
                return _strassen_value(prod, c)

            def finish(y, rh, ch):
                for ci in range(2):
                    ref, idx = dst_slot(i, m + 3 * ch, ci)
                    ref[idx, pl.ds(RING - PRE + rh * PH, PH), :] = y[:, ci * 128:(ci + 1) * 128]

            _strassen(outer, finish)
        return carry

    for bi, (starts, items) in enumerate(P1A_BLOCKS):
        for item in starts:
            item_start(item)
        with jax.named_scope("p1a_wait%d" % bi):
            for item in items:
                item_wait(item)
        for item in items:
            item_run(item)
    assert not a_jobs
    xc_copy(0).wait()
    with jax.named_scope("p1b"):
        lax.fori_loop(2, 8, phase1b, 0)
    pks.pop(0)
    xc_copy(1).wait()
    for n in range(8):
        wo_copy(n).wait()

    cexp = scale * math.log2(math.e)
    NG = NP // 2
    grp = [(4 * (g // 2) + (g % 2), 4 * (g // 2) + (g % 2) + 2) for g in range(NG)]
    early = [2 * j + u for g in range(NG - 3) for j in grp[g] for u in range(2)]
    late = [h for h in range(H) if h not in early]

    def step(it, k, side_jobs):
        s = it * UNROLL + k
        split = k > 0
        base = TOK * UNROLL * it
        w0 = pl.multiple_of(lax.rem(base, RING), 32) + TOK * k
        r0 = pl.multiple_of(lax.rem(SEG * s + (RING - PRE), RING), 32)
        ow = pl.multiple_of(lax.rem(SEG * s + OOFF, RING), 32)
        o0 = pl.multiple_of(lax.rem(base + OOFF, RING), 32) + TOK * k
        a0 = pl.multiple_of(base, 32) + TOK * k
        X = jnp.concatenate([hn[pl.ds(a0, TOK), :], memb[...]], axis=0).astype(BF16)
        ym = [None] * 96
        probs = [None] * NP
        om = [None] * H
        order = (4, 5, 0, 1, 2, 3)

        if split:
            for t in order:
                accb[t] = _dot(X[:, :D // 2], _bf(wqkv[t, pl.ds(0, D // 4), :]))

        def slot(j, t):
            if t >= 4:
                return vring, 2 * j + t - 4
            return (qka, qkb)[j % 2], 4 * (j // 2) + t

        def proj(j, t, job):
            c = 6 * j + t
            bits = [] if job is None else [job()]
            if split and j == 0:
                y = accb[t] + _dot(X[:, D // 2:], _bf(wqkv[c, pl.ds(D // 4, D // 4), :]))
            else:
                y = _dot(X, _bf(wqkv[c]))
            ref, k = slot(j, t)
            ref[k, pl.ds(w0, TOK), :] = after(y, bits)[0:TOK]
            ym[c] = y[TOK:TOK + M]

        def gather(j, m, pad):
            c = 6 * j + 2 * m
            ref, k = slot(j, 2 * m)
            parts = [ref[k, pl.ds(r0, SEG), :], ref[k + 1, pl.ds(r0, SEG), :], ym[c], ym[c + 1]]
            if pad:
                parts.append(jnp.zeros((48, E), F32))
            return jnp.concatenate(parts, axis=0).astype(BF16)

        def scores(j):
            sc_ = lax.dot_general(gather(j, 0, False), gather(j, 1, True),
                                  (((1,), (1,)), ((), ())), preferred_element_type=F32)
            fill = fillb[...]
            sc_ = jnp.where(fill == 0.0, sc_, fill)
            mx = jnp.max(sc_, axis=-1, keepdims=True)
            p = jnp.exp2((sc_ - mx) * cexp)
            l = jnp.sum(p, axis=-1, keepdims=True)
            rl = pl.reciprocal(l, approx=True)
            rl = rl * (2.0 - l * rl)
            probs[j] = p * rl

        def park(j):
            vring[H, pl.ds(40 * (j % 8), 40), :] = pack(probs[j], F32)
            probs[j] = None

        def pv(j):
            if probs[j] is None:
                P = _bf(vring[H, pl.ds(40 * (j % 8), 40), :])
            else:
                P = probs[j].astype(BF16)
            o = _dot(P, gather(j, 2, True))
            oring[2 * j, pl.ds(ow, SEG), :] = o[0:32]
            oring[2 * j + 1, pl.ds(ow, SEG), :] = o[32:64]
            om[2 * j] = o[64:72]
            om[2 * j + 1] = o[72:80]

        def o_lhs(hs):
            return jnp.concatenate(
                [jnp.concatenate([oring[h, pl.ds(o0, TOK), :], om[h]], axis=0) for h in hs],
                axis=1).astype(BF16)

        def o_rhs(n, hs):
            return _bf(jnp.concatenate([wo[n, pl.ds(h * 64, 64), :] for h in hs], axis=0))

        for g in range(NG):
            cols = [(j, t) for j in grp[g] for t in order]
            if g == 2:
                cols = ([(j, t) for j in grp[g] for t in (4, 5)]
                        + [(j, t) for j in grp[g] for t in range(4)])
            for j in (grp[0] + grp[1] if g == 3 else grp[g - 2] if g >= 4 else ()):
                park(j)
            for ci, (j, t) in enumerate(cols):
                if g == 2 and ci == 4:
                    for jj in grp[0] + grp[1]:
                        scores(jj)
                if g >= 3 and ci == ATT_COL:
                    for jj in grp[g - 1]:
                        scores(jj)
                    for jj in grp[g - 3]:
                        pv(jj)
                proj(j, t, side_jobs.get((g, ci)))
        lo = o_lhs(early)
        for n in range(8):
            accb[n] = _dot(lo, o_rhs(n, early))
            if n == ATT_N1:
                for jj in grp[NG - 1]:
                    scores(jj)
                for jj in grp[NG - 3]:
                    pv(jj)
            if n == ATT_N2:
                for jj in grp[NG - 2] + grp[NG - 1]:
                    pv(jj)
        lo = o_lhs(late)
        for n in range(8):
            a = accb[n] + _dot(lo, o_rhs(n, late))
            ha[pl.ds(a0, TOK), pl.ds(n * 128, 128)] = a[0:TOK]
            memb[:, pl.ds(n * 128, 128)] = a[TOK:TOK + M]

    NIT = NSEG // UNROLL

    def lo16(w):
        return pltpu.bitcast(w << 16, F32)

    def hi16(w):
        return pltpu.bitcast(w & jnp.uint32(0xFFFF0000), F32)

    def steps(it, carry):
        @pl.when(it == 1)
        def _():
            xc_copy(2).wait()

        for cp in slab_copies(it):
            cp.wait()
        for cp in slab_copies((it + 1) & (NIT - 1)):
            cp.start()
        acc = [None, None]

        def mod_job(q):
            for kk in range(2 * q, 2 * q + 2):
                cw = colb[pl.ds(kk * 8, 8), :]
                for t in range(2):
                    w = pltpu.bitcast(slab[it & 1, t, pl.ds(kk * 8, 8), :], U32)
                    v = lo16(w) * lo16(cw) + hi16(w) * hi16(cw)
                    acc[t] = v if acc[t] is None else acc[t] + v
            if q < D // 32 - 1:
                return pltpu.bitcast(acc[0], U32) | pltpu.bitcast(acc[1], U32)
            y = jnp.sum(jnp.concatenate(acc, axis=1), axis=0, keepdims=True).astype(BF16).astype(F32)
            y = jnp.broadcast_to(y + jnp.where((it >> 2) == 2, 1.0, 0.0), (8, 256))
            modb[it] = y
            return pltpu.bitcast(y[:, 0:128], U32)

        nxt2 = pl.multiple_of(jnp.minimum(it + 1, NIT - 1) * (IT_ROWS // 2), 16)
        pieces = list(range(IT_ROWS // 16))
        for k in range(UNROLL):
            side_jobs = {pos: functools.partial(mod_job, 8 * k + q) for q, pos in enumerate(MOD_SLOTS)}
            for pos in LN_SLOTS[k % 2:]:
                side_jobs[pos] = functools.partial(ln1_piece, nxt2 + 8 * pieces.pop(0))
            step(it, k, side_jobs)
        assert not pieces
        return carry

    with jax.named_scope("p2_steps"):
        lax.fori_loop(0, NIT, steps, 0)
    for cp in slab_copies(0):
        cp.wait()
    w1_copy.wait()
    w2_copy.wait()

    nb = S // FB
    HB = FB // 2
    QB = FB // 4

    def ln2_piece(hs, blk, off):
        x2 = (load_x16(pl.multiple_of(blk * HB, HB) + off // 2)
              + mrow(2, 16) * ha[pl.ds(pl.multiple_of(blk * FB, FB) + off, 16), :])
        h = _ln(x2) * mrow(4, 16) + mrow(3, 16)
        hs[off] = h
        return pltpu.bitcast(h[8:16, D - 128:], U32)

    def lhs1_loc(c, d):
        e = 7 * c + d
        return 32 * (e // 4), 256 * (e % 4)

    def lhs1_job(hs, k, t, c):
        def sub(ri, ki):
            def blk(ro, ko):
                c0 = (2 * ko + ki) * 256 + t * 128
                return hs[(2 * ro + ri) * QB + 16 * k][:, c0:c0 + 128]

            return _combo(_LHS_TERMS, c, blk)

        bits = None
        for d, v in enumerate(_lhs_combos(sub(0, 0), sub(0, 1), sub(1, 0), sub(1, 1))):
            r0, c0 = lhs1_loc(c, d)
            hn[pl.ds(r0 + 8 * k, 8), pl.ds(c0 + t * 128, 128)] = pltpu.bitcast(
                v.astype(BF16), F32)
            if d in TIE_L:
                b = pltpu.bitcast(v[8 * (d % 2):8 * (d % 2) + 8], U32)
                bits = b if bits is None else bits | b
        return bits

    def make_ln2(blk, plan, jobs):
        state = dict(piece=0, call=0)
        pending, hs = [], {}

        def issue():
            jobs.extend(pending)
            del pending[:]
            bits = []
            for _ in range(plan[state['call']]):
                k, r = state['piece'] // 4, state['piece'] % 4
                bits.append(ln2_piece(hs, blk, r * QB + 16 * k))
                if r == 3:
                    pending.extend(functools.partial(lhs1_job, hs, k, t, c)
                                   for t in range(2) for c in range(7))
                state['piece'] += 1
            state['call'] += 1
            return bits

        assert sum(plan) == FB // 16 and plan[-1] == 0
        return issue

    K1, N1, K2, N2 = D // 8, FF // 4, FF // 8, D // 4

    def rhs1_loc(c, d, n):
        e = _PAIRS.index((c, d)) * 7 + n
        return wqkv, e // 4, K1 * (e % 4)

    rhs2_slots = ([(wqkv, e, 0) for e in range(79, 96)] + [(qkb, e, 0) for e in range(H)]
                  + [(vring, e, 0) for e in range(H + 1)] + [(wx, e, 0) for e in range(8)])

    def rhs2_loc(c, d, n):
        return rhs2_slots[_PAIRS.index((c, d)) * 2 + n]

    def rhs_job(w, kq, nq, loc, n, r, cs):
        cache, bits = {}, []
        for c in cs:
            out = rhs_operands(lambda a, b: w[pl.ds(r + a * kq, 8), pl.ds(n * 128 + b * nq, 128)], c, cache)
            for d, v in out.items():
                ref, idx, row = loc(c, d, n)
                ref[idx, pl.ds(row + r, 8), :] = _as(v, ref.dtype)
            bits += [out[d] for d in TIE_R]
        return functools.reduce(jnp.bitwise_or, bits)

    def rhs_load(w, kq, nq, loc, c, d, n):
        if (c, d) not in _PAIRS:
            qk, qn = _plain_block(c, d)
            return w[pl.ds(qk * kq, kq), pl.ds(qn * nq + n * 128, 128)]
        ref, idx, row = loc(c, d, n)
        return _as(ref[idx, pl.ds(row, kq), :], U32)

    def make_tie(jobs, credit):
        state = [credit]

        def tie(raw, density):
            if not jobs:
                return raw
            ties = {}
            for g in range(raw.shape[0] // 8):
                state[0] += density
                if jobs and state[0] >= 1.0:
                    state[0] -= 1.0
                    ties[g] = jobs.pop(0)()
            return or_rows(raw, ties)

        return tie

    def bulk_o():
        spots = ([(w1, K1, N1, rhs1_loc, n, r) for n in range(7) for r in range(0, K1, 8)]
                 + [(w2, K2, N2, rhs2_loc, n, r) for n in range(2) for r in range(0, K2, 8)])
        ng = len(JOB_GROUPS)
        jobs = [functools.partial(rhs_job, *spots[(e + (len(spots) // ng) * gi) % len(spots)], cs)
                for e in range(len(spots)) for gi, cs in enumerate(JOB_GROUPS)]
        scale_d = (len(jobs) + 56 + 6) / (7 * 64 * sum(P3_WEIGHTS))
        state = dict(credit=-2.0)
        ln2_block0 = make_ln2(0, LN0_PLAN, jobs)

        def tie_lhs(tiles, density):
            ties = [{} for _ in tiles]
            for w in range(4):
                for g in range(16):
                    state['credit'] += density
                    if jobs and state['credit'] >= 1.0:
                        state['credit'] -= 1.0
                        ties[4 * w + g % 4][g] = jobs.pop(0)()
            return _bf(jnp.concatenate([or_rows(t, z) for t, z in zip(tiles, ties)], axis=1))

        def a_blk(rh, kh):
            return jnp.concatenate([oring[h, pl.ds(rh * 256, 256), :]
                                    for h in range(16 * kh, 16 * kh + 16)], axis=1)

        lhs = [[pack(v[:, 128 * t:128 * t + 128]) for t in range(16)]
               for v in _lhs_combos(a_blk(0, 0), a_blk(0, 1), a_blk(1, 0), a_blk(1, 1))]
        for n in range(4):
            def prod(c):
                bits = ln2_block0()
                return after(_dot(tie_lhs(lhs[c], scale_d * P3_WEIGHTS[n]),
                                  _rhs_operand(c, lambda a, b: wo[n + 4 * b, pl.ds(a * 1024, 1024), :])), bits)

            def finish(y, rh, ch):
                ha[pl.ds(NSEG * TOK + rh * 256, 256), pl.ds((n + 4 * ch) * 128, 128)] = y

            _strassen(prod, finish)
        assert not jobs

    pks.pop(0)
    with jax.named_scope("p3_bulk_o"):
        bulk_o()

    pks.pop(0)
    out32 = out_hbm.bitcast(F32)

    def ffn(i, carry):
        nxt = (i + 1) & (nb - 1)
        half = i >> 2
        srow = pl.multiple_of((i & 3) * HB, HB)

        g = {(c, d): [] for c in range(7) for d in range(7)}
        for n in range(7):
            act = {}

            def prod1(c, d):
                r0, c0 = lhs1_loc(c, d)
                return _dot(_bf(hn[pl.ds(r0, QB // 2), pl.ds(c0, 256)]),
                            _bf(rhs_load(w1, K1, N1, rhs1_loc, c, d, n)))

            def activate(y, rh, ch):
                b1 = jnp.concatenate([biasb[:, pl.ds((2 * ch + ci) * N1 + n * 128, 128)] for ci in range(2)],
                                     axis=1)
                act[rh, ch] = jax.nn.gelu(y + rep(b1, HB), approximate=True)

            _strassen(lambda c: _strassen_value(prod1, c), activate)
            for c in range(7):
                o = _combo(_LHS_TERMS, c, lambda a, b: act[a, b])
                for d, v in enumerate(_lhs_combos(o[:QB, :128], o[:QB, 128:], o[QB:, :128], o[QB:, 128:])):
                    g[c, d].append(v.astype(BF16))

        jobs = []
        tie = make_tie(jobs, 0.0)
        next_block_ln = make_ln2(nxt, LN_PLAN, jobs)

        for n in range(2):
            def prod2(c, d):
                return _dot(jnp.concatenate(g[c, d], axis=1),
                            _bf(tie(rhs_load(w2, K2, N2, rhs2_loc, c, d, n), FFN_DENSITY)))

            def outer(c):
                bits = next_block_ln()
                return after(_strassen_value(prod2, c), bits, _SWAP[c])

            def finish(y, rh, ch):
                for ci in range(2):
                    nn = (2 * ch + ci) * 2 + n
                    cols = pl.ds(nn * 128, 128)
                    mcols = pl.ds((nn % 2) * 128, 128)
                    yy = y[:, ci * 128:(ci + 1) * 128] + rep(biasb[:, pl.ds(FF + nn * 128, 128)], HB)
                    xr = pl.ds(pl.multiple_of(i * HB, HB) + rh * (HB // 2), HB // 2)
                    ar = pl.ds(pl.multiple_of(i * FB, FB) + rh * HB, HB)
                    x2 = _bf(xs[xr, cols]).astype(F32) + rep(modb[nn // 2, :, mcols], HB) * ha[ar, cols]
                    qka[2 * nn + half, pl.ds(srow + rh * (HB // 2), HB // 2), :] = pack(
                        x2 + rep(modb[12 + nn // 2, :, mcols], HB) * yy, F32)
                    if rh == ch:
                        pltpu.make_async_copy(
                            qka.at[2 * nn + half, pl.ds(srow, HB), :],
                            out32.at[pl.ds(pl.multiple_of(i * HB, HB), HB), cols],
                            sem.at[SEM_OUT]).start()

            _strassen(outer, finish)
        assert not jobs
        return carry

    with jax.named_scope("p4_ffn"):
        lax.fori_loop(0, nb, ffn, 0)
    pltpu.make_async_copy(out32, out32, sem.at[SEM_OUT]).wait()


@jax.jit
def pallas_adaLN_cond__memory_aug_recurrent_mem_tr__dense_activation_gelu__prompt_kernel(
    A_x, A_mem0, A_Wq, A_Wk, A_Wv, A_Wo, A_seg_len, B_x, B_w1, B_b1, B_w2, B_b2, c, w_mod,
):
    assert A_x.shape == (1, S, D) and A_Wq.shape == (D, H, E) and A_mem0.shape == (1, M, D)
    any_spec = pl.BlockSpec(memory_space=pl.ANY)
    out = pl.pallas_call(
        _kernel,
        out_shape=jax.ShapeDtypeStruct((S, D), BF16),
        in_specs=[any_spec] * 12,
        out_specs=any_spec,
        scratch_shapes=[
            pltpu.VMEM((S // 2, D), U32),
            pltpu.VMEM((96, D // 2, E), U32),
            pltpu.VMEM((8, H * E // 2, 128), U32),
            pltpu.VMEM((D // 2, FF), U32),
            pltpu.VMEM((FF // 2, D), U32),
            pltpu.VMEM((H, RING, E), F32),
            pltpu.VMEM((H, RING, E), F32),
            pltpu.VMEM((H + 1, RING, E), F32),
            pltpu.VMEM((H, RING, E), F32),
            pltpu.VMEM((S, D), F32),
            pltpu.VMEM((S - PRE, D), F32),
            pltpu.VMEM((M, D), F32),
            pltpu.VMEM((NQ, 2, 8, KQ), F32),
            pltpu.VMEM((16, 8, 256), F32),
            pltpu.VMEM((8, D), U32),
            pltpu.VMEM((D // 2, 128), U32),
            pltpu.VMEM((2, 2, D // 2, 128), F32),
            pltpu.VMEM((8, FF + D), F32),
            pltpu.VMEM((80, 128), F32),
            pltpu.VMEM((8, 32, 128), F32),
            pltpu.VMEM((128, 128), F32),
            pltpu.VMEM((8, 128), U32),
            pltpu.VMEM((8, FF // 8, 128), U32),
            pltpu.VMEM((13 * 64, D), U32),
            pltpu.VMEM((128, 256), U32),
            pltpu.VMEM((128, 256), U32),
            pltpu.VMEM((128, 256), U32),
            pltpu.VMEM((128, 256), U32),
            pltpu.VMEM((M, D), BF16),
            pltpu.VMEM((FF,), BF16),
            pltpu.VMEM((D,), BF16),
            pltpu.VMEM((1, D), BF16),
            pltpu.SemaphoreType.DMA((NSEM,)),
        ],
        compiler_params=pltpu.CompilerParams(vmem_limit_bytes=127 * 1024 * 1024, disable_bounds_checks=True,
                                             disable_semaphore_checks=True),
    )(
        A_x.reshape(S, D), A_mem0.reshape(M, D),
        A_Wq.reshape(D // 2, 2, H, E), A_Wk.reshape(D // 2, 2, H, E), A_Wv.reshape(D // 2, 2, H, E),
        A_Wo.reshape(H * E, D), B_w1, B_b1, B_w2, B_b2, c, w_mod,
    )
    return out.reshape(1, S, D)
```
